```python
import jax
import jax.numpy as jnp

def _softmax(x, axis=-1):
    return jax.nn.softmax(x, axis=axis)
def _gelu(x):
    return jax.nn.gelu(x, approximate=True)
def _silu(x):
    return jax.nn.silu(x)
def _sigmoid(x):
    return jax.nn.sigmoid(x)
def _layernorm(x, axis=-1, eps=1e-5):
    m = jnp.mean(x, axis=axis, keepdims=True)
    v = jnp.var(x, axis=axis, keepdims=True)
    return (x - m) / jnp.sqrt(v + eps)
def _scatter_add(tgt, idx, src, axis=0):
    return tgt.at[idx].add(src)
def _segment_sum(src, seg, n):
    return jax.ops.segment_sum(src, seg, n)
class _Rng:
    def __init__(self, key):
        self._k = key
    def _next(self):
        self._k, sub = jax.random.split(self._k)
        return sub
    def normal(self, shape):
        return jax.random.normal(self._next(), shape, dtype=jnp.bfloat16)
    def randint(self, lo, hi, shape):
        return jax.random.randint(self._next(), shape, lo, hi, dtype=jnp.int32)
    def uniform(self, shape, lo=0.0, hi=1.0):
        return jax.random.uniform(self._next(), shape, jnp.bfloat16, lo, hi)
    def permutation(self, n):
        return jax.random.permutation(self._next(), n)


kernel_name = 'interleave_layers__spectral_gfnet__sliding_local_dilated__prompt'

def setup_inputs():
    _rng = _Rng(jax.random.key(int.from_bytes(__import__("os").urandom(4), "little")))
    _w = (lambda a: (lambda t: t.astype(jnp.bfloat16) if jnp.issubdtype(t.dtype, jnp.floating) else t)(jnp.asarray(a)))
    def _A_setup():
        B, S, D = 1, 2048, 1024
        Df = D // 2 + 1
        return {
            "x": _w((lambda *s: _rng.normal(s) * 0.05)(B, S, D)),
            "w_r": _w((lambda *s: _rng.normal(s) * 0.05)(S, Df) * 0.02),
            "w_i": _w((lambda *s: _rng.normal(s) * 0.05)(S, Df) * 0.02),
        }
    _A_in = _A_setup()

    def _B_setup():
        B, S, D = 1, 2048, 1024
        return {
            "x": _w((lambda *s: _rng.normal(s) * 0.05)(B, S, D)),
            "wqkv": _w((lambda *s: _rng.normal(s) * 0.05)(D, 3 * D)),
            "wo": _w((lambda *s: _rng.normal(s) * 0.05)(D, D)),
        }
    _B_in = _B_setup()

    return {
        "A_x": _A_in["x"],
        "A_w_r": _A_in["w_r"],
        "A_w_i": _A_in["w_i"],
        "B_x": _B_in["x"],
        "B_wqkv": _B_in["wqkv"],
        "B_wo": _B_in["wo"],
    }

def reference(A_x, A_w_r, A_w_i, B_x, B_wqkv, B_wo):
    def _A_ref(x, w_r, w_i):
        B, S, D = x.shape
        X = (lambda x, axes=(-2,-1): jnp.fft.rfft2(x.astype(jnp.float32), axes=axes))(x, axes=(-2, -1))
        W = w_r + 1j * w_i
        X = X * W
        y = (lambda x, s, axes=(-2,-1): jnp.fft.irfft2(x, s=s, axes=axes).astype(jnp.bfloat16))(X, (S, D), axes=(-2, -1))
        return y

    def _B_ref(x, wqkv, wo):
        B, S, D = x.shape
        H = 32; Dh = D // H
        W, dil = 8, 2
        qkv = (lambda x, *d: x.transpose(*d))((x @ wqkv).reshape(B, S, 3, H, Dh), 2, 0, 3, 1, 4)
        q, k, v = qkv[0], qkv[1], qkv[2]
        scale = Dh ** -0.5
        pos = jnp.arange(S)
        off = jnp.arange(W) * dil
        idx = pos[:, None] - off[None, :]
        mask = idx >= 0
        idx_c = jnp.where(mask, idx, 0).reshape(-1)
        kg = k[:, :, idx_c, :].reshape(B, H, S, W, Dh)
        vg = v[:, :, idx_c, :].reshape(B, H, S, W, Dh)
        logits = jnp.einsum("bhsd,bhswd->bhsw", q, kg) * scale
        logits = jnp.where(mask[None, None, :, :], logits, -1e9)
        attn = _softmax(logits, axis=-1)
        o = jnp.einsum("bhsw,bhswd->bhsd", attn, vg)
        return (lambda x, *d: x.transpose(*d))(o, 0, 2, 1, 3).reshape(B, S, D) @ wo

    x = A_x
    x = x + _A_ref(_layernorm(x, axis=-1), A_w_r, A_w_i)
    x = x + _B_ref(_layernorm(x, axis=-1), B_wqkv, B_wo)
    x = x + _A_ref(_layernorm(x, axis=-1), A_w_r, A_w_i)
    x = x + _B_ref(_layernorm(x, axis=-1), B_wqkv, B_wo)
    return x
```

```python
import numpy as np

import jax
import jax.numpy as jnp
import jax.experimental.pallas as pl
import jax.experimental.pallas.tpu as pltpu

S, D, NB = 2048, 1024, 16
ZR = 520
F32, BF16, U32, I32 = jnp.float32, jnp.bfloat16, jnp.uint32, jnp.int32
EPS = 1e-5
SCALE = 32 ** -0.5
RSQ2 = float(np.sqrt(0.5))
UTIL = 0.80
DEFER = 2

M_FA, M_FB, M_R, M_C4, M_RT, M_C4T, M_R0T = 0, 16, 32, 33, 34, 35, 36
L_MU, L_NU, L_KU, L_KV = 0, 16, 32, 48


def _bf16_bits(a):
    u = np.ascontiguousarray(a, dtype=np.float32).view(np.uint32).astype(np.uint64)
    return ((u + 0x7FFF + ((u >> 16) & 1)) >> 16).astype(np.uint32)


def _bf16_round(a):
    return (_bf16_bits(a) << 16).view(np.float32).astype(np.float64)


def _constants():
    a = np.arange(128)
    k1 = np.arange(64)
    alt = (-1.0) ** a
    mats = np.zeros((37, 128, 128))
    lanes = np.zeros((64, 128))
    for j in range(NB):
        t = 2 * np.pi * np.outer(16 * a + j, k1) / S
        ang = 2 * np.pi * j / 32 + np.pi / 32
        p, q = _bf16_round(np.array([np.cos(ang), np.sin(ang)]))
        fa = np.concatenate([np.cos(t), -np.sin(t)], 1)
        fb = np.concatenate([np.sin(t), -np.cos(t)], 1)
        fa[:, 0], fb[:, 0] = RSQ2, -RSQ2
        fa[:, 64], fb[:, 64] = p * alt, -q * alt
        mats[M_FA + j], mats[M_FB + j] = fa, fb
        lanes[L_MU + j, 0], lanes[L_MU + j, 64] = 1.0, (q / p + p / q) / 2
        lanes[L_NU + j, 0], lanes[L_NU + j, 64] = 0.0, (q / p - p / q) / 2
        lanes[L_KU + j, 0], lanes[L_KU + j, 64] = 1.0, q / p
        lanes[L_KV + j, 0], lanes[L_KV + j, 64] = 1.0, p / q
    th = 2 * np.pi * np.outer(k1, a) / 128
    r = np.concatenate([np.cos(th), -np.sin(th)], 0)
    r[64] = alt
    th = 2 * np.pi * np.outer(2 * k1 + 1, a) / 256
    c4 = np.concatenate([np.cos(th), -np.sin(th)], 0)
    inv = 2.0 / (S * D)
    mats[M_R], mats[M_C4], mats[M_RT], mats[M_C4T] = r, c4, inv * r.T, inv * c4.T
    mats[M_R0T] = mats[M_RT]
    mats[M_R0T, :, 0::64] *= 0.5
    bits = _bf16_bits(mats)
    mats_u32 = bits[:, 0::2] | (bits[:, 1::2] << 16)
    tw = np.zeros((6, 128, 128), np.float32)
    for k in (1, 2, 3):
        tw[2 * k - 2] = np.cos(2 * np.pi * a * k / D)[:, None]
        tw[2 * k - 1] = np.sin(2 * np.pi * a * k / D)[:, None]
    ang = 2 * np.pi * np.outer(np.arange(4), np.arange(4)).ravel() / 16
    rot = np.concatenate([np.cos(ang), np.sin(ang)]).astype(np.float32)
    return mats_u32, lanes.astype(np.float32), tw, rot


_MATS, _LANES, _TWID, _ROT = _constants()
_ZERO = np.zeros((1,), np.int32)


class _Step:
    def __init__(self, cost, anchors=(), delay=0, marks=()):
        self.cost, self.anchors, self.delay, self.marks = cost, list(anchors), delay, list(marks)


class _Wait:
    def __init__(self, *names):
        self.names = names


class _Task:
    def __init__(self, gen):
        self.gen, self.blocked, self.not_before = gen, (), 0


class _Sched:
    def __init__(self):
        self.tasks, self.done, self.producer = [], {}, {}
        self.slot, self.credit, self.anchors = 0, 0.0, []

    def add(self, gen, name):
        self.producer[name] = _Task(gen)
        self.tasks.append(self.producer[name])

    def _ready(self, t):
        return t.not_before <= self.slot and all(
            n in self.done and self.done[n] <= self.slot for n in t.blocked)

    def _advance(self, t):
        item = next(t.gen, None)
        if item is None:
            self.tasks.remove(t)
        elif isinstance(item, _Wait):
            t.blocked = item.names
        else:
            t.blocked = ()
            t.not_before = self.slot + item.delay
            self.credit -= item.cost
            self.anchors += item.anchors
            for n in item.marks:
                self.done[n] = self.slot + item.delay

    def run(self, *names):
        while not all(n in self.done for n in names):
            for n in names:
                if n not in self.done:
                    for b in self.producer[n].blocked:
                        self.run(b)
                    self._advance(self.producer[n])

    def finish(self):
        self.run(*self.producer)

    def chunk(self, emit, cycles, own, needs=(), marks=()):
        for n in needs:
            self.run(n)
        self.credit = min(self.credit, 0.0) + cycles * 4 * UTIL - own
        while self.credit > 0:
            t = next((t for t in self.tasks if self._ready(t)), None)
            if t is None:
                break
            self._advance(t)
        anchors, self.anchors = self.anchors, []
        emit(anchors)
        self.slot += 1
        for n in marks:
            self.done[n] = self.slot + 1


def _dot(a, b):
    return jnp.dot(a, b, preferred_element_type=F32)


def _dot_t(a, b):
    return jax.lax.dot_general(a, b, (((1,), (1,)), ((), ())), preferred_element_type=F32)


def _bf(u):
    return pltpu.bitcast(u, BF16)


def _iota(rows, dim):
    return jax.lax.broadcasted_iota(I32, (rows, 128), dim)


def _radix4(z, inverse):
    (r0, i0), (r1, i1), (r2, i2), (r3, i3) = z
    ar, ai, cr, ci = r0 + r2, i0 + i2, r0 - r2, i0 - i2
    br, bi, dr, di = r1 + r3, i1 + i3, r1 - r3, i1 - i3
    lo, hi = (cr + di, ci - dr), (cr - di, ci + dr)
    if inverse:
        lo, hi = hi, lo
    return [(ar + br, ai + bi), lo, (ar - br, ai - bi), hi]


def _all_sublanes(v, op, axis):
    for sh in (4, 2, 1):
        v = op(v, pltpu.roll(v, sh, axis))
    return v


def _loop(n, body):
    def step(i, carry):
        body(i)
        return carry
    jax.lax.fori_loop(0, n, step, 0)


def _kernel(zero_ref, rot, mats, lanes, twid, x_hbm, wr_hbm, wi_hbm, wqkv_hbm, wo_hbm, out_hbm,
            X, HB, KE, VE, QB, Z, WS, WT, UB, AB, PB, XR, WRI, WN, WRAW, sems):
    zero = zero_ref[0]
    never = zero != 0
    hbu, ubu, abu, xru, wsu = (r.bitcast(U32) for r in (HB, UB, AB, XR, WRI))

    def anchor(ref, idx, row, col=0):
        return lambda: ref[idx, pl.ds(pl.multiple_of(row + zero * 8, 8), 8), pl.ds(col, 128)]

    def mat(i):
        return _bf(mats[i])

    def lane_vec(i, rows):
        return jnp.broadcast_to(lanes[pl.ds(i, 1), :], (rows, 128))

    def x_copy(c):
        return pltpu.make_async_copy(
            x_hbm.at[:, pl.ds(pl.multiple_of(128 * c, 128), 128)], XR.at[c], sems.at[c])

    def out_copy(c):
        return pltpu.make_async_copy(
            XR.at[c], out_hbm.at[:, pl.ds(pl.multiple_of(128 * c, 128), 128)], sems.at[8 + c])

    spec_copies = [[pltpu.make_async_copy(w.at[pl.ds(0, 512), pl.ds(128 * k2, 128)], WRI.at[u, k2],
                                          sems.at[16 + u]) for k2 in range(16)]
                   + [pltpu.make_async_copy(w.at[pl.ds(512, 1), :], WN.at[u], sems.at[22 + u])]
                   for u, w in enumerate((wr_hbm, wi_hbm))]

    def start_all(copies):
        for c in copies:
            c.start()
    w_copies = [pltpu.make_async_copy(wqkv_hbm.at[:, pl.ds(D * w, D)], WRAW.at[w], sems.at[18 + w])
                for w in range(3)] + [pltpu.make_async_copy(wo_hbm, WRAW.at[3], sems.at[21])]

    def ln_finish(n, mean, t):
        acc = None
        for r in range(8):
            d = X[n, pl.ds(128 * r, 128), :].reshape(16, 8, 128) - mean[None]
            v = (d * d).sum(0)
            acc = v if acc is None else acc + v
            if r == 3:
                yield _Step(200)
        PB[t, pl.ds(1040, 8), :] = mean
        PB[t, pl.ds(1048, 8), :] = jax.lax.rsqrt(_all_sublanes(acc, jnp.add, 0) * (1.0 / D) + EPS)
        yield _Step(210, [anchor(PB, t, 1048)])

    def fwd_block(g, i, name, needs):
        n, j, t = 4 * g + i, g + 4 * i, 2 + i % 2
        yield _Wait(*needs)
        acc = None
        for r in range(8):
            v = X[n, pl.ds(128 * r, 128), :].reshape(16, 8, 128).sum(0)
            acc = v if acc is None else acc + v
        mean = _all_sublanes(acc, jnp.add, 0) * (1.0 / D)
        yield _Step(140)
        yield from ln_finish(n, mean, t)
        for r in range(8):
            rows = pl.ds(16 * r, 16)
            mean8 = jnp.concatenate([PB[t, pl.ds(1040, 8), :] * 8.0] * 2, 0)
            rstd = jnp.concatenate([PB[t, pl.ds(1048, 8), :]] * 2, 0)
            x = [X[n, pl.ds(128 * b + 16 * r, 16), :] for b in range(8)]
            s = [x[b] + x[b + 4] for b in range(4)]
            d = [x[b] - x[b + 4] for b in range(4)]
            e, o = s[0] + s[2], s[1] + s[3]
            UB[t, rows, :] = ((e + o - mean8) * rstd).astype(BF16)
            UB[t, pl.ds(128 + 16 * r, 16), :] = ((e - o) * rstd).astype(BF16)
            t1, t2 = (d[1] - d[3]) * RSQ2, (d[1] + d[3]) * RSQ2
            u = {1: (d[0] + t1, d[2] + t2), 2: (s[0] - s[2], s[1] - s[3]), 3: (d[0] - t1, d[2] - t2)}
            for k in (1, 2, 3):
                c, sn = twid[2 * k - 2, rows, :] * rstd, twid[2 * k - 1, rows, :] * rstd
                re, m = u[k]
                if k == 3:
                    ur, ui = re * c + m * sn, m * c - re * sn
                else:
                    ur, ui = re * c - m * sn, m * c + re * sn
                UB[t, pl.ds(256 * k + 16 * r, 16), :] = ur.astype(BF16)
                UB[t, pl.ds(256 * k + 128 + 16 * r, 16), :] = ui.astype(BF16)
            yield _Step(110, [anchor(ubu, t, 448 + 8 * r)])
        for c in range(8):
            PB[t, pl.ds(128 * c, 128), :] = _dot(mat(M_C4 if c == 1 else M_R),
                                                 _bf(ubu[t, pl.ds(64 * c, 64), :]))
        yield _Step(0, delay=2)
        first = _iota(64, 0) == 0

        def fix(v, v0):
            return jnp.concatenate([jnp.where(first[:8], v0, v[:8]), v[8:]], 0).astype(BF16)

        p1, p2 = PB[t, pl.ds(0, 64), :], PB[t, pl.ds(64, 64), :]
        AB[t, pl.ds(0, 64), :] = p1.astype(BF16)
        AB[t, pl.ds(528, 64), :] = jnp.where(first, 0.0, p2).astype(BF16)
        AB[t, pl.ds(512, 16), :] = jnp.where(first[:16], p2[:16], 0.0).astype(BF16)
        AB[t, pl.ds(256, 64), :] = PB[t, pl.ds(128, 64), :].astype(BF16)
        AB[t, pl.ds(528 + 256, 64), :] = PB[t, pl.ds(192, 64), :].astype(BF16)
        for k in (1, 2, 3):
            p1, p2 = PB[t, pl.ds(256 * k, 64), :], PB[t, pl.ds(256 * k + 64, 64), :]
            q1, q2 = PB[t, pl.ds(256 * k + 128, 64), :], PB[t, pl.ds(256 * k + 192, 64), :]
            if k == 3:
                pr, pi, mr, mi = p1 - q2, p2 + q1, p1 + q2, p2 - q1
                pi0, mi0 = q1[:8], -q2[:8]
            else:
                pr, pi, mr, mi = p1 + q2, p2 - q1, p1 - q2, p2 + q1
                pi0, mi0 = -q1[:8], q2[:8]
            AB[t, pl.ds(64 * k, 64), :] = fix(pr, p1[:8])
            AB[t, pl.ds(64 * (8 - k), 64), :] = fix(mr, p2[:8])
            AB[t, pl.ds(528 + 64 * k, 64), :] = fix(pi, pi0)
            AB[t, pl.ds(528 + 64 * (8 - k), 64), :] = fix(mi, mi0)
        yield _Step(190, [anchor(abu, t, 424)])
        fa, fb = mat(M_FA + j), mat(M_FB + j)
        PB[t, pl.ds(0, 256), :] = _dot(_bf(abu[t, pl.ds(0, 128), :]), fa)
        PB[t, pl.ds(528, 256), :] = _dot(_bf(abu[t, pl.ds(264, 128), :]), fb)
        PB[t, pl.ds(256, 272), :] = _dot(_bf(abu[t, pl.ds(128, 136), :]), fa)
        PB[t, pl.ds(784, 256), :] = _dot(_bf(abu[t, pl.ds(392, 128), :]), fb)
        yield _Step(0, delay=2)
        for r0, rn in ((0, 176), (176, 176), (352, 160), (512, 8)):
            u = PB[t, pl.ds(r0, rn), :]
            if r0 < 512:
                v = PB[t, pl.ds(528 + r0, rn), :]
                re, m = u + v, u - v
            else:
                re = m = u
            edge = (_iota(rn, 1) & 63) == 0
            Z[2 * n, pl.ds(r0, rn), :] = re
            Z[2 * n + 1, pl.ds(r0, rn), :] = jnp.where(
                edge, lane_vec(L_MU + j, rn) * m + lane_vec(L_NU + j, rn) * re, pltpu.roll(m, 64, 1))
            if r0 < 352:
                yield _Step(140, [anchor(Z, 2 * n + 1, r0)])
        yield _Step(140, [anchor(Z, 2 * n + 1, 512)], marks=[name])

    def group_stage(g, name, needs, inverse):
        yield _Wait(*needs)

        def turn(z, k):
            if k == 0:
                return z
            c, s = rot[4 * g + k], rot[16 + 4 * g + k]
            if inverse:
                return z[0] * c - z[1] * s, z[1] * c + z[0] * s
            return z[0] * c + z[1] * s, z[1] * c - z[0] * s

        for r in range(13):
            rows = pl.ds(40 * r, 40)
            z = [(Z[8 * g + 2 * i, rows, :], Z[8 * g + 2 * i + 1, rows, :]) for i in range(4)]
            if inverse:
                z = _radix4([turn(z[k], k) for k in range(4)], True)
            else:
                z = [turn(v, k) for k, v in enumerate(_radix4(z, False))]
            for i in range(4):
                Z[8 * g + 2 * i, rows, :], Z[8 * g + 2 * i + 1, rows, :] = z[i]
            yield _Step(170, [anchor(Z, 8 * g + 7, 40 * r)], marks=[name] if r == 12 else [])

    def spectral(k0):
        for r in range(33):
            rows = pl.ds(16 * r, 16 if r < 32 else 8)
            z = _radix4([(Z[8 * g + 2 * k0, rows, :], Z[8 * g + 2 * k0 + 1, rows, :])
                         for g in range(4)], False)
            y = []
            for k1, (re, im) in enumerate(z):
                w = WS[k0 + 4 * k1, rows, :]
                wr = pltpu.bitcast(w << 16, F32)
                wi = pltpu.bitcast(w & np.uint32(0xFFFF0000), F32)
                y.append((re * wr - im * wi, re * wi + im * wr))
            y = _radix4(y, True)
            for g in range(4):
                Z[8 * g + 2 * k0, rows, :], Z[8 * g + 2 * k0 + 1, rows, :] = y[g]

    def inv_block(g, i, name, needs, n=None):
        zn, j, t = 4 * g + i, g + 4 * i, i % 2
        n = zn if n is None else n
        yield _Wait(*needs)
        for r0, rn in ((0, 176), (176, 176), (352, 160), (512, 8)):
            re, im = Z[2 * zn, pl.ds(r0, rn), :], Z[2 * zn + 1, pl.ds(r0, rn), :]
            edge = (_iota(rn, 1) & 63) == 0
            rolled = pltpu.roll(im, 64, 1)
            u = re + jnp.where(edge, lane_vec(L_KU + j, rn) * im, rolled)
            if r0 < 512:
                v = re - jnp.where(edge, lane_vec(L_KV + j, rn) * im, rolled)
                AB[t, pl.ds(r0, rn), :] = u.astype(BF16)
                AB[t, pl.ds(528 + r0, rn), :] = v.astype(BF16)
            else:
                AB[t, pl.ds(512, 16), :] = jnp.concatenate([u, jnp.zeros_like(u)], 0).astype(BF16)
            if r0 < 352:
                yield _Step(160, [anchor(abu, t, 264 + r0 // 2)])
        yield _Step(160, [anchor(abu, t, 256)])
        fa, fb = mat(M_FA + j), mat(M_FB + j)
        PB[t, pl.ds(0, 256), :] = _dot_t(_bf(abu[t, pl.ds(0, 128), :]), fa)
        PB[t, pl.ds(528, 256), :] = _dot_t(_bf(abu[t, pl.ds(264, 128), :]), fb)
        PB[t, pl.ds(256, 272), :] = _dot_t(_bf(abu[t, pl.ds(128, 136), :]), fa)
        PB[t, pl.ds(784, 256), :] = _dot_t(_bf(abu[t, pl.ds(392, 128), :]), fb)
        yield _Step(0, delay=2)
        first = _iota(8, 0) == 0

        def fix(v, v0):
            return jnp.concatenate([jnp.where(first, v0, v[:8]), v[8:]], 0).astype(BF16)

        UB[t, pl.ds(0, 64), :] = PB[t, pl.ds(0, 64), :].astype(BF16)
        UB[t, pl.ds(64, 64), :] = fix(PB[t, pl.ds(528, 64), :], PB[t, pl.ds(512, 8), :])
        UB[t, pl.ds(128, 64), :] = PB[t, pl.ds(256, 64), :].astype(BF16)
        UB[t, pl.ds(192, 64), :] = PB[t, pl.ds(528 + 256, 64), :].astype(BF16)
        for k in (1, 2, 3):
            pr, pi = PB[t, pl.ds(64 * k, 64), :], PB[t, pl.ds(528 + 64 * k, 64), :]
            mr, mi = PB[t, pl.ds(64 * (8 - k), 64), :], PB[t, pl.ds(528 + 64 * (8 - k), 64), :]
            UB[t, pl.ds(256 * k, 64), :] = fix(pr + mr, pr[:8])
            UB[t, pl.ds(256 * k + 64, 64), :] = fix(pi + mi, mr[:8])
            UB[t, pl.ds(256 * k + 128, 64), :] = fix(pi - mi, pi[:8])
            UB[t, pl.ds(256 * k + 192, 64), :] = fix(mr - pr, -mi[:8])
        yield _Step(190, [anchor(ubu, t, 480)])
        for c in range(8):
            PB[t, pl.ds(128 * c, 128), :] = _dot(mat({0: M_R0T, 1: M_C4T}.get(c, M_RT)),
                                                 _bf(ubu[t, pl.ds(64 * c, 64), :]))
        yield _Step(0, delay=2)
        acc = None
        for r in range(8):
            rows = pl.ds(16 * r, 16)
            t0, t4 = PB[t, rows, :], PB[t, pl.ds(128 + 16 * r, 16), :]
            tk = {}
            for k in (1, 2, 3):
                c, sn = twid[2 * k - 2, rows, :], twid[2 * k - 1, rows, :]
                re = PB[t, pl.ds(256 * k + 16 * r, 16), :]
                im = PB[t, pl.ds(256 * k + 128 + 16 * r, 16), :]
                tk[k] = (re * c - im * sn, re * sn + im * c)
            e0, e1 = t0 + t4, t0 - t4
            s = [e0 + tk[2][0], e1 - tk[2][1], e0 - tk[2][0], e1 + tk[2][1]]
            al, be = tk[1][0] - tk[3][0], tk[1][1] + tk[3][1]
            o = [tk[1][0] + tk[3][0], (al - be) * RSQ2, tk[3][1] - tk[1][1], (al + be) * -RSQ2]
            for b in range(8):
                y = s[b] + o[b] if b < 4 else s[b - 4] - o[b - 4]
                v = X[zn, pl.ds(128 * b + 16 * r, 16), :] + y
                X[n, pl.ds(128 * b + 16 * r, 16), :] = v
                acc = v if acc is None else acc + v
            yield _Step(115, [anchor(X, n, 896 + 16 * r)])
        yield from ln_finish(n, _all_sublanes(acc[:8] + acc[8:], jnp.add, 0) * (1.0 / D), t)
        for r in range(2):
            mean, rstd = PB[t, pl.ds(1040, 8), :], PB[t, pl.ds(1048, 8), :]
            v = X[n, pl.ds(512 * r, 512), :].reshape(64, 8, 128)
            HB[n, pl.ds(512 * r, 512), :] = ((v - mean[None]) * rstd[None]).reshape(512, 128).astype(BF16)
            yield _Step(160, [anchor(hbu, n, 256 * r + 248)], marks=[name] if r == 1 else [])

    def attend(g, i, name, needs):
        n, j = 4 * g + i, g + 4 * i
        yield _Wait(*needs)
        sub = jax.lax.broadcasted_iota(I32, (1, 8, 128), 1)
        lane = jax.lax.broadcasted_iota(I32, (1, 8, 128), 2)
        wrapped = (lane == 0) & (2 * sub > j)

        def merge(a, b, pos_a, shift):
            sel = ((sum(1 << p for p in pos_a) >> sub) & 1) == 1
            return jnp.where(sel, a, b) + pltpu.roll(jnp.where(sel, b, a), 8 - shift, 1)

        def fold8(s):
            def quad(ws, o):
                z1 = merge(s[ws[0]], s[ws[1]], [(o + u) % 8 for u in range(4)], 4)
                z2 = merge(s[ws[2]], s[ws[3]], [(o + 2 + u) % 8 for u in range(4)], 4)
                return merge(z1, z2, [(o + u) % 8 for u in (0, 1, 4, 5)], 2)
            return merge(quad((0, 4, 2, 6), 0), quad((1, 5, 3, 7), 1), [0, 2, 4, 6], 1)

        hp = 2
        for h in range(0, 32, hp):
            rows = pl.ds(32 * h, 32 * hp)
            q = QB[i, rows, :]
            s = [(q * KE[j + 14 - 2 * w, rows, :]).reshape(hp, 4, 8, 128).sum(1) for w in range(8)]
            lg = jnp.where(wrapped, -1e9, fold8(s) * SCALE)
            e = jnp.exp(lg - _all_sublanes(lg, jnp.maximum, 1))
            p = e / _all_sublanes(e, jnp.add, 1)
            acc = None
            for w in range(8):
                pw = jnp.broadcast_to(p[:, w:w + 1, :], (hp, 32, 128)).reshape(32 * hp, 128)
                v = pw * VE[j + 14 - 2 * w, rows, :]
                acc = v if acc is None else acc + v
            HB[n, rows, :] = acc.astype(BF16)
            yield _Step(180 * hp, [anchor(hbu, n, 16 * h)], marks=[name] if h == 32 - hp else [])

    def proj(sch, w, n, m, store, needs, marks, own=120):
        def emit(anchors):
            lhs = WT[w, pl.ds(pl.multiple_of(64 * m, 64), 64), :]
            if anchors:
                head = lhs[:8, :128]
                for a in anchors:
                    head = jnp.where(never, pltpu.bitcast(a(), U32), head)
                top = jnp.concatenate([head, lhs[:8, 128:]], 1)
                lhs = jnp.concatenate([top, lhs[8:]], 0)
            store(_dot(_bf(lhs), _bf(hbu[n])), pl.ds(pl.multiple_of(128 * m, 128), 128))
        sch.chunk(emit, 256, own, needs, marks)

    def kv_proj(sch, g, i, needs):
        j = g + 4 * i
        shifted = j - 2 if i else jnp.where(g >= 2, g - 2, g + 30)
        for w, ref in ((1, KE), (2, VE)):
            def store(v, rows):
                ref[j + 14, rows, :] = v
                r = pltpu.roll(v, 1, 1)
                if w == 2:
                    r = jnp.where(_iota(128, 1) == 0, ref[14, rows, :], r)
                ref[shifted, rows, :] = r
            for m in range(8):
                proj(sch, w, 4 * g + i, m, store, needs, [], own=150)

    def q_proj(sch, g, i, name):
        def store(v, rows):
            QB[i, rows, :] = v
        for m in range(8):
            proj(sch, 0, 4 * g + i, m, store, [], [name] if m == 7 else [])

    def o_proj(sch, n, m, needs, marks):
        def store(v, rows):
            X[n, rows, :] = X[n, rows, :] + v
        proj(sch, 3, n, m, store, needs, marks, own=135)

    def transpose_weight(src, dst, name):
        for r in range(4):
            for c in range(4):
                WT[dst, pl.ds(128 * c, 128), pl.ds(256 * r, 256)] = pltpu.bitcast(
                    WRAW[src, pl.ds(256 * r, 256), pl.ds(256 * c, 256)].T, U32)
                yield _Step(140, [anchor(WT, dst, 128 * c, 256 * r)],
                            marks=[name] if r == 3 and c == 3 else [])

    def prep_spectral_weights(c2):
        lane = _iota(8, 1)
        order = jnp.where(lane > 64, 192 - lane, lane)

        def words(k2):
            re, im = (wsu[u, k2, pl.ds(c2, 64, stride=4), :] for u in range(2))
            return ((re & np.uint32(0xFFFF)) | (im << 16), (re >> 16) | (im & np.uint32(0xFFFF0000)))

        def arrange(w, below):
            w = jnp.where(_iota(w.shape[0], 1) < 64, w, below)
            return jnp.concatenate([jnp.take_along_axis(w[u:u + 8], order, axis=1)
                                    for u in range(0, w.shape[0], 8)], 0)

        below = words(15)
        for k2 in range(16):
            here = words(k2)
            for e in range(2):
                cl = 2 * c2 + e
                w = arrange(here[e], below[e])
                WS[k2, pl.ds(64 * cl, 64), :] = pltpu.roll(w, 1, 0) if cl > 4 else w
            below = here
        if c2 == 0:
            def nyquist(k2):
                re, im = (jnp.broadcast_to(WN[u, :, pl.ds(128 * k2, 128)].astype(F32), (8, 128))
                          for u in range(2))
                return pltpu.pack_elementwise([re, im], packed_dtype=BF16)
            for k2 in range(16):
                WS[k2, pl.ds(512, 8), :] = arrange(nyquist(k2), nyquist((k2 + 15) % 16))

    def write_out(lo, hi, p, c, name, needs):
        yield _Wait(*needs)
        rows = pl.ds(pl.multiple_of(128 * c, 128), 128)
        w = pltpu.pack_elementwise([X[lo, rows, :], X[hi, rows, :]], packed_dtype=BF16)
        xru[c, pl.ds(p, 128, stride=8), :] = w.T
        yield _Step(60, [anchor(xru, c, 0)], marks=[name])

    x_copy(0).start()
    x_copy(1).start()

    def load_x(c):
        x_copy(c).wait()
        pl.when(c < 6)(lambda: x_copy(c + 2).start())
        pl.when(c == 6)(lambda: start_all(spec_copies[0]))
        pl.when(c == 7)(lambda: start_all(spec_copies[1]))
        rows = pl.ds(pl.multiple_of(128 * c, 128), 128)
        for p in range(8):
            w = xru[c, pl.ds(p, 128, stride=8), :].T
            X[4 * (2 * p % 4) + p // 2, rows, :] = pltpu.bitcast(w << 16, F32)
            X[4 * ((2 * p + 1) % 4) + p // 2, rows, :] = pltpu.bitcast(w & np.uint32(0xFFFF0000), F32)

    _loop(8, load_x)

    def first_forward(g):
        pl.when(g == 1)(w_copies[1].start)
        pl.when(g == 2)(w_copies[2].start)
        sch = _Sched()
        for i in range(4):
            sch.add(fwd_block(g, i, ("f", i), [("f", i - 2)] if i >= 2 else []), ("f", i))
        sch.add(group_stage(g, "r", [("f", i) for i in range(4)], False), "r")
        sch.run(("f", 0), ("f", 1))
        sch.run(("f", 2), ("f", 3))
        sch.finish()

    _loop(4, first_forward)
    w_copies[0].start()
    w_copies[3].start()
    for c in spec_copies[0] + spec_copies[1]:
        c.wait()
    for c2 in range(4):
        prep_spectral_weights(c2)
    w_copies[1].wait()
    w_copies[2].wait()

    def first_weights(u):
        for _ in transpose_weight(1 + u, 1 + u, None):
            pass

    _loop(2, first_weights)

    def keys_values(layer, g):
        pl.when((layer == 0) & (g == 1))(w_copies[0].wait)
        pl.when((layer == 0) & (g == 2))(w_copies[3].wait)
        sch = _Sched()
        for i in range(1, 4):
            sch.add(inv_block(g, i, ("i", i), [("i", i - 2)] if i >= 2 else []), ("i", i))
            if i == 1:
                sch.done[("i", 0)] = 0
        nxt = (g + 1) % 4
        sch.add(group_stage(nxt, "r", [], True), "r")
        sch.add(inv_block(nxt, 0, ("i", 4), ["r", ("i", 2)], n=4 * g + 4), ("i", 4))
        src = jnp.where(g == 1, 0, jnp.where(g == 2, 3, 1))
        sch.add(transpose_weight(src, jnp.where(src == 1, 4, src), "w"), "w")
        for i in range(4):
            kv_proj(sch, g, i, [("i", i)])
        sch.finish()

    def block_of(g, i):
        return g + i // 4, i % 4

    def mix(g, last, tail):
        sch = _Sched()
        now = 8 - DEFER if last else 8
        sch.done[("a", 0)] = 0
        if not last:
            sch.add(group_stage((g + 3) % 4, "r", [], False), "r")
        for i in range(4):
            if i < 3 or not tail:
                sch.add(attend(*block_of(g, i + 1), ("a", i + 1), [("q", i + 1)] if i else []),
                        ("a", i + 1))
            if not last:
                sch.add(fwd_block(g, i, ("f", i), [("o", i, 7)] + ([("f", i - 2)] if i >= 2 else [])),
                        ("f", i))
            else:
                pair = 2 if tail else 0
                for c in range(now):
                    sch.add(write_out(4 * pair + i, 4 * pair + 4 + i, pair // 2 + 2 * i, c,
                                      ("w", i, c), [("o", i, c)]), ("w", i, c))
        for i in range(4):
            for m in range(now):
                o_proj(sch, 4 * g + i, m, [("a", i)], [("o", i, m)])
            if i < 2 or not tail:
                q_proj(sch, *block_of(g, i + 2), ("q", i + 2))
        if tail and not last:
            sch.add(group_stage(g, "s", [("f", i) for i in range(4)], False), "s")
        sch.finish()

    def postponed(u):
        c = 8 - DEFER + u
        sch = _Sched()
        for p in range(8):
            lo = 4 * (2 * p % 4) + p // 2
            sch.add(write_out(lo, lo + 4, p, c, ("w", p), [("o", p)]), ("w", p))
            o_proj(sch, lo, c, [], [])
            o_proj(sch, lo + 4, c, [], [("o", p)])
        sch.finish()
        out_copy(c).start()

    def layer_body(layer):
        _loop(4, spectral)
        sch = _Sched()
        sch.add(group_stage(0, "r", [], True), "r")
        sch.add(inv_block(0, 0, "i", ["r"]), "i")
        sch.finish()
        _loop(4, lambda g: keys_values(layer, g))
        sch = _Sched()
        sch.add(attend(0, 0, "a", ["q"]), "a")
        q_proj(sch, 0, 0, "q")
        q_proj(sch, 0, 1, None)
        sch.finish()

        @pl.when(layer == 0)
        def _():
            _loop(3, lambda g: mix(g, False, False))
            mix(3, False, True)

        @pl.when(layer == 1)
        def _():
            _loop(3, lambda g: mix(g, True, False))
            mix(3, True, True)
            for c in range(8 - DEFER):
                out_copy(c).start()
            _loop(DEFER, postponed)

    _loop(2, layer_body)
    for c in range(8):
        out_copy(c).wait()


@jax.jit
def pallas_interleave_layers__spectral_gfnet__sliding_local_dilated__prompt_kernel(
    A_x: jax.Array,
    A_w_r: jax.Array,
    A_w_i: jax.Array,
    B_x: jax.Array,
    B_wqkv: jax.Array,
    B_wo: jax.Array,
):
    del B_x
    hbm = pl.BlockSpec(memory_space=pl.ANY)
    smem = pl.BlockSpec(memory_space=pltpu.SMEM)
    out = pl.pallas_call(
        _kernel,
        out_shape=jax.ShapeDtypeStruct((S, D), BF16),
        in_specs=[smem, smem, pl.BlockSpec(), pl.BlockSpec(), pl.BlockSpec(), hbm, hbm, hbm, hbm, hbm],
        out_specs=hbm,
        scratch_shapes=[
            pltpu.VMEM((NB + 1, D, 128), F32),
            pltpu.VMEM((NB + 1, D, 128), BF16),
            pltpu.VMEM((32, D, 128), F32),
            pltpu.VMEM((32, D, 128), F32),
            pltpu.VMEM((4, D, 128), F32),
            pltpu.VMEM((2 * NB, ZR, 128), F32),
            pltpu.VMEM((NB, ZR, 128), U32),
            pltpu.VMEM((5, D // 2, D), U32),
            pltpu.VMEM((4, D, 128), BF16),
            pltpu.VMEM((4, 1040, 128), BF16),
            pltpu.VMEM((4, 1056, 128), F32),
            pltpu.VMEM((8, S, 128), BF16),
            pltpu.VMEM((2, NB, D // 2, 128), BF16),
            pltpu.VMEM((2, 1, S), BF16),
            pltpu.VMEM((4, D, D), BF16),
            pltpu.SemaphoreType.DMA((24,)),
        ],
        compiler_params=pltpu.CompilerParams(vmem_limit_bytes=124 * 2 ** 20),
    )(_ZERO, _ROT, _MATS, _LANES, _TWID, A_x.reshape(S, D), A_w_r.T, A_w_i.T, B_wqkv, B_wo)
    return out.reshape(1, S, D)
```

```python
import numpy as np

import jax
import jax.numpy as jnp
import jax.experimental.pallas as pl
import jax.experimental.pallas.tpu as pltpu

S, D, NB = 2048, 1024, 16
ZR = 520
F32, BF16, U32, I32 = jnp.float32, jnp.bfloat16, jnp.uint32, jnp.int32
EPS = 1e-5
SCALE = 32 ** -0.5
RSQ2 = float(np.sqrt(0.5))
DEFER = 2

_S_ROWS = [(64 * u, 64) for u in range(8)] + [(512, 8)]

M_FA, M_FB, M_R, M_C4, M_RT, M_C4T, M_R0T = 0, 16, 32, 33, 34, 35, 36
L_MU, L_NU, L_KU, L_KV = 0, 16, 32, 48


def _bf16_bits(a):
    u = np.ascontiguousarray(a, dtype=np.float32).view(np.uint32).astype(np.uint64)
    return ((u + 0x7FFF + ((u >> 16) & 1)) >> 16).astype(np.uint32)


def _bf16_round(a):
    return (_bf16_bits(a) << 16).view(np.float32).astype(np.float64)


def _constants():
    a = np.arange(128)
    k1 = np.arange(64)
    alt = (-1.0) ** a
    mats = np.zeros((37, 128, 128))
    lanes = np.zeros((64, 128))
    for j in range(NB):
        t = 2 * np.pi * np.outer(16 * a + j, k1) / S
        ang = 2 * np.pi * j / 32 + np.pi / 32
        p, q = _bf16_round(np.array([np.cos(ang), np.sin(ang)]))
        fa = np.concatenate([np.cos(t), -np.sin(t)], 1)
        fb = np.concatenate([np.sin(t), -np.cos(t)], 1)
        fa[:, 0], fb[:, 0] = RSQ2, -RSQ2
        fa[:, 64], fb[:, 64] = p * alt, -q * alt
        mats[M_FA + j], mats[M_FB + j] = fa, fb
        lanes[L_MU + j, 0], lanes[L_MU + j, 64] = 1.0, (q / p + p / q) / 2
        lanes[L_NU + j, 0], lanes[L_NU + j, 64] = 0.0, (q / p - p / q) / 2
        lanes[L_KU + j, 0], lanes[L_KU + j, 64] = 1.0, q / p
        lanes[L_KV + j, 0], lanes[L_KV + j, 64] = 1.0, p / q
    th = 2 * np.pi * np.outer(k1, a) / 128
    r = np.concatenate([np.cos(th), -np.sin(th)], 0)
    r[64] = alt
    th = 2 * np.pi * np.outer(2 * k1 + 1, a) / 256
    c4 = np.concatenate([np.cos(th), -np.sin(th)], 0)
    inv = 2.0 / (S * D)
    mats[M_R], mats[M_C4], mats[M_RT], mats[M_C4T] = r, c4, inv * r.T, inv * c4.T
    mats[M_R0T] = mats[M_RT]
    mats[M_R0T, :, 0::64] *= 0.5
    bits = _bf16_bits(mats)
    mats_u32 = bits[:, 0::2] | (bits[:, 1::2] << 16)
    tw = np.zeros((6, 128, 128), np.float32)
    for k in (1, 2, 3):
        tw[2 * k - 2] = np.cos(2 * np.pi * a * k / D)[:, None]
        tw[2 * k - 1] = np.sin(2 * np.pi * a * k / D)[:, None]
    ang = 2 * np.pi * np.outer(np.arange(4), np.arange(4)).ravel() / 16
    rot = np.concatenate([np.cos(ang), np.sin(ang)]).astype(np.float32)
    return mats_u32, lanes.astype(np.float32), tw, rot


_MATS, _LANES, _TWID, _ROT = _constants()
_ZERO = np.zeros((1,), np.int32)


class _Step:
    def __init__(self, cost, anchors=(), delay=0, marks=()):
        self.cost, self.anchors, self.delay, self.marks = cost, list(anchors), delay, list(marks)


class _Wait:
    def __init__(self, *names):
        self.names = names


class _Task:
    def __init__(self, gen, pace):
        self.gen, self.pace, self.blocked, self.not_before = gen, pace, (), 0


class _Sched:
    def __init__(self, share=0.5):
        self.share = share
        self.tasks, self.done, self.producer = [], {}, {}
        self.slot, self.credit, self.anchors = 0, 0.0, []

    def add(self, gen, name, pace=3):
        self.producer[name] = _Task(gen, pace)
        self.tasks.append(self.producer[name])

    def _ready(self, t):
        return t.not_before <= self.slot and all(
            n in self.done and self.done[n] <= self.slot for n in t.blocked)

    def _advance(self, t):
        item = next(t.gen, None)
        if item is None:
            self.tasks.remove(t)
        elif isinstance(item, _Wait):
            t.blocked = item.names
        else:
            t.blocked = ()
            t.not_before = self.slot + item.delay
            self.credit -= item.cost
            self.anchors += item.anchors
            for n in item.marks:
                self.done[n] = self.slot + item.delay

    def run(self, *names):
        while not all(n in self.done for n in names):
            for n in names:
                if n not in self.done:
                    for b in self.producer[n].blocked:
                        self.run(b)
                    self._advance(self.producer[n])

    def finish(self):
        self.run(*self.producer)

    def chunk(self, emit, cycles, own, needs=(), marks=()):
        for n in needs:
            self.run(n)
        self.credit = min(self.credit, 100.0) + cycles * 4 * self.share - own
        stepped = []
        while self.credit > 0:
            t = next((t for t in self.tasks if self._ready(t) and stepped.count(t) < t.pace), None)
            if t is None:
                break
            stepped.append(t)
            self._advance(t)
        anchors, self.anchors = self.anchors, []
        emit(anchors)
        self.slot += 1
        for n in marks:
            self.done[n] = self.slot + 1


def _dot(a, b):
    return jnp.dot(a, b, preferred_element_type=F32)


def _dot_t(a, b):
    return jax.lax.dot_general(a, b, (((1,), (1,)), ((), ())), preferred_element_type=F32)


def _bf(u):
    return pltpu.bitcast(u, BF16)


def _iota(rows, dim):
    return jax.lax.broadcasted_iota(I32, (rows, 128), dim)


def _radix4(z, inverse):
    (r0, i0), (r1, i1), (r2, i2), (r3, i3) = z
    ar, ai, cr, ci = r0 + r2, i0 + i2, r0 - r2, i0 - i2
    br, bi, dr, di = r1 + r3, i1 + i3, r1 - r3, i1 - i3
    lo, hi = (cr + di, ci - dr), (cr - di, ci + dr)
    if inverse:
        lo, hi = hi, lo
    return [(ar + br, ai + bi), lo, (ar - br, ai - bi), hi]


def _all_sublanes(v, op, axis):
    for sh in (4, 2, 1):
        v = op(v, pltpu.roll(v, sh, axis))
    return v


def _loop(n, body, name):
    def step(i, carry):
        body(i)
        return carry
    with jax.named_scope(name):
        jax.lax.fori_loop(0, n, step, 0)


def _kernel(zero_ref, rot, mats, lanes, twid, x_hbm, wr_hbm, wi_hbm, wqkv_hbm, wo_hbm, out_hbm,
            X, HB, KE, VE, QB, Z, WS, WT, UB, AB, PB, XR, WRI, WN, WRAW, sems):
    zero = zero_ref[0]
    never = zero != 0
    hbu, ubu, abu, xru, wsu = (r.bitcast(U32) for r in (HB, UB, AB, XR, WRI))

    def anchor(ref, idx, row, col=0):
        return lambda: ref[idx, pl.ds(pl.multiple_of(row + zero * 8, 8), 8), pl.ds(col, 128)]

    def mat(i):
        return _bf(mats[i])

    def lane_vec(i, rows):
        return jnp.broadcast_to(lanes[pl.ds(i, 1), :], (rows, 128))

    def x_copy(c):
        return pltpu.make_async_copy(
            x_hbm.at[:, pl.ds(pl.multiple_of(128 * c, 128), 128)], XR.at[c], sems.at[c])

    def out_copy(c):
        return pltpu.make_async_copy(
            XR.at[c], out_hbm.at[:, pl.ds(pl.multiple_of(128 * c, 128), 128)], sems.at[8 + c])

    spec_copies = [[pltpu.make_async_copy(w.at[pl.ds(0, 512), pl.ds(128 * k2, 128)], WRI.at[u, k2],
                                          sems.at[16 + u]) for k2 in range(16)]
                   + [pltpu.make_async_copy(w.at[pl.ds(512, 1), :], WN.at[u], sems.at[22 + u])]
                   for u, w in enumerate((wr_hbm, wi_hbm))]

    def start_all(copies):
        for c in copies:
            c.start()
    w_copies = [pltpu.make_async_copy(wqkv_hbm.at[:, pl.ds(D * w, D)], WRAW.at[w], sems.at[18 + w])
                for w in range(3)] + [pltpu.make_async_copy(wo_hbm, WRAW.at[3], sems.at[21])]

    def ln_finish(n, mean, t):
        acc = None
        for r in range(8):
            d = X[n, pl.ds(128 * r, 128), :].reshape(16, 8, 128) - mean[None]
            v = (d * d).sum(0)
            acc = v if acc is None else acc + v
            if r == 3:
                yield _Step(200)
        PB[t, pl.ds(1040, 8), :] = mean
        PB[t, pl.ds(1048, 8), :] = jax.lax.rsqrt(_all_sublanes(acc, jnp.add, 0) * (1.0 / D) + EPS)
        yield _Step(210, [anchor(PB, t, 1048)])

    def fwd_block(g, i, name, needs):
        n, j, t = 4 * g + i, g + 4 * i, 2 + i % 2
        yield _Wait(*needs)
        acc = None
        for r in range(8):
            v = X[n, pl.ds(128 * r, 128), :].reshape(16, 8, 128).sum(0)
            acc = v if acc is None else acc + v
        mean = _all_sublanes(acc, jnp.add, 0) * (1.0 / D)
        yield _Step(140)
        yield from ln_finish(n, mean, t)
        for r in range(8):
            rows = pl.ds(16 * r, 16)
            mean8 = jnp.concatenate([PB[t, pl.ds(1040, 8), :] * 8.0] * 2, 0)
            rstd = jnp.concatenate([PB[t, pl.ds(1048, 8), :]] * 2, 0)
            x = [X[n, pl.ds(128 * b + 16 * r, 16), :] for b in range(8)]
            s = [x[b] + x[b + 4] for b in range(4)]
            d = [x[b] - x[b + 4] for b in range(4)]
            e, o = s[0] + s[2], s[1] + s[3]
            UB[t, rows, :] = ((e + o - mean8) * rstd).astype(BF16)
            UB[t, pl.ds(128 + 16 * r, 16), :] = ((e - o) * rstd).astype(BF16)
            t1, t2 = (d[1] - d[3]) * RSQ2, (d[1] + d[3]) * RSQ2
            u = {1: (d[0] + t1, d[2] + t2), 2: (s[0] - s[2], s[1] - s[3]), 3: (d[0] - t1, d[2] - t2)}
            for k in (1, 2, 3):
                c, sn = twid[2 * k - 2, rows, :] * rstd, twid[2 * k - 1, rows, :] * rstd
                re, m = u[k]
                if k == 3:
                    ur, ui = re * c + m * sn, m * c - re * sn
                else:
                    ur, ui = re * c - m * sn, m * c + re * sn
                UB[t, pl.ds(256 * k + 16 * r, 16), :] = ur.astype(BF16)
                UB[t, pl.ds(256 * k + 128 + 16 * r, 16), :] = ui.astype(BF16)
            yield _Step(110, [anchor(ubu, t, 448 + 8 * r)])
        for c in range(8):
            PB[t, pl.ds(128 * c, 128), :] = _dot(mat(M_C4 if c == 1 else M_R),
                                                 _bf(ubu[t, pl.ds(64 * c, 64), :]))
        yield _Step(-400, delay=2)
        first = _iota(64, 0) == 0

        def fix(v, v0):
            return jnp.concatenate([jnp.where(first[:8], v0, v[:8]), v[8:]], 0).astype(BF16)

        p1, p2 = PB[t, pl.ds(0, 64), :], PB[t, pl.ds(64, 64), :]
        AB[t, pl.ds(0, 64), :] = p1.astype(BF16)
        AB[t, pl.ds(528, 64), :] = jnp.where(first, 0.0, p2).astype(BF16)
        AB[t, pl.ds(512, 16), :] = jnp.where(first[:16], p2[:16], 0.0).astype(BF16)
        AB[t, pl.ds(256, 64), :] = PB[t, pl.ds(128, 64), :].astype(BF16)
        AB[t, pl.ds(528 + 256, 64), :] = PB[t, pl.ds(192, 64), :].astype(BF16)
        for k in (1, 2, 3):
            p1, p2 = PB[t, pl.ds(256 * k, 64), :], PB[t, pl.ds(256 * k + 64, 64), :]
            q1, q2 = PB[t, pl.ds(256 * k + 128, 64), :], PB[t, pl.ds(256 * k + 192, 64), :]
            if k == 3:
                pr, pi, mr, mi = p1 - q2, p2 + q1, p1 + q2, p2 - q1
                pi0, mi0 = q1[:8], -q2[:8]
            else:
                pr, pi, mr, mi = p1 + q2, p2 - q1, p1 - q2, p2 + q1
                pi0, mi0 = -q1[:8], q2[:8]
            AB[t, pl.ds(64 * k, 64), :] = fix(pr, p1[:8])
            AB[t, pl.ds(64 * (8 - k), 64), :] = fix(mr, p2[:8])
            AB[t, pl.ds(528 + 64 * k, 64), :] = fix(pi, pi0)
            AB[t, pl.ds(528 + 64 * (8 - k), 64), :] = fix(mi, mi0)
        yield _Step(190, [anchor(abu, t, 424)])
        fa, fb = mat(M_FA + j), mat(M_FB + j)
        PB[t, pl.ds(0, 256), :] = _dot(_bf(abu[t, pl.ds(0, 128), :]), fa)
        PB[t, pl.ds(528, 256), :] = _dot(_bf(abu[t, pl.ds(264, 128), :]), fb)
        PB[t, pl.ds(256, 272), :] = _dot(_bf(abu[t, pl.ds(128, 136), :]), fa)
        PB[t, pl.ds(784, 256), :] = _dot(_bf(abu[t, pl.ds(392, 128), :]), fb)
        yield _Step(-400, delay=2)
        for r0, rn in _S_ROWS:
            u = PB[t, pl.ds(r0, rn), :]
            if r0 < 512:
                v = PB[t, pl.ds(528 + r0, rn), :]
                re, m = u + v, u - v
            else:
                re = m = u
            edge = (_iota(rn, 1) & 63) == 0
            Z[2 * n, pl.ds(r0, rn), :] = re
            Z[2 * n + 1, pl.ds(r0, rn), :] = jnp.where(
                edge, lane_vec(L_MU + j, rn) * m + lane_vec(L_NU + j, rn) * re, pltpu.roll(m, 64, 1))
            if r0 % 128 == 64:
                yield _Step(110, [anchor(Z, 2 * n + 1, r0)])
        yield _Step(10, [anchor(Z, 2 * n + 1, 512)], marks=[name])

    def group_stage(g, name, needs, inverse):
        yield _Wait(*needs)

        def turn(z, k):
            if k == 0:
                return z
            c, s = rot[4 * g + k], rot[16 + 4 * g + k]
            if inverse:
                return z[0] * c - z[1] * s, z[1] * c + z[0] * s
            return z[0] * c + z[1] * s, z[1] * c - z[0] * s

        for r in range(33):
            rows = pl.ds(16 * r, 16 if r < 32 else 8)
            z = [(Z[8 * g + 2 * i, rows, :], Z[8 * g + 2 * i + 1, rows, :]) for i in range(4)]
            if inverse:
                z = _radix4([turn(z[k], k) for k in range(4)], True)
            else:
                z = [turn(v, k) for k, v in enumerate(_radix4(z, False))]
            for i in range(4):
                Z[8 * g + 2 * i, rows, :], Z[8 * g + 2 * i + 1, rows, :] = z[i]
            if r % 2 == 0:
                yield _Step(140, [anchor(Z, 8 * g + 7, 16 * r)], marks=[name] if r == 32 else [])

    def spectral(row, size):
        rows = pl.ds(row, size)
        for k0 in range(4):
            z = _radix4([(Z[8 * g + 2 * k0, rows, :], Z[8 * g + 2 * k0 + 1, rows, :])
                         for g in range(4)], False)
            y = []
            for k1, (re, im) in enumerate(z):
                w = WS[k0 + 4 * k1, rows, :]
                wr = pltpu.bitcast(w << 16, F32)
                wi = pltpu.bitcast(w & np.uint32(0xFFFF0000), F32)
                y.append((re * wr - im * wi, re * wi + im * wr))
            y = _radix4(y, True)
            for g in range(4):
                Z[8 * g + 2 * k0, rows, :], Z[8 * g + 2 * k0 + 1, rows, :] = y[g]

    def spectral_rows(c2):
        for r in range(8):
            spectral(pl.multiple_of(128 * c2 + 16 * r, 16), 16)

    def inv_block(g, i, name, needs, n=None):
        zn, j, t = 4 * g + i, g + 4 * i, i % 2
        n = zn if n is None else n
        yield _Wait(*needs)
        for r0, rn in _S_ROWS:
            re, im = Z[2 * zn, pl.ds(r0, rn), :], Z[2 * zn + 1, pl.ds(r0, rn), :]
            edge = (_iota(rn, 1) & 63) == 0
            rolled = pltpu.roll(im, 64, 1)
            u = re + jnp.where(edge, lane_vec(L_KU + j, rn) * im, rolled)
            if r0 < 512:
                v = re - jnp.where(edge, lane_vec(L_KV + j, rn) * im, rolled)
                AB[t, pl.ds(r0, rn), :] = u.astype(BF16)
                AB[t, pl.ds(528 + r0, rn), :] = v.astype(BF16)
            else:
                AB[t, pl.ds(512, 16), :] = jnp.concatenate([u, jnp.zeros_like(u)], 0).astype(BF16)
            if r0 % 128 == 64:
                yield _Step(125, [anchor(abu, t, 264 + r0 // 2)])
        yield _Step(10, [anchor(abu, t, 256)])
        fa, fb = mat(M_FA + j), mat(M_FB + j)
        PB[t, pl.ds(0, 256), :] = _dot_t(_bf(abu[t, pl.ds(0, 128), :]), fa)
        PB[t, pl.ds(528, 256), :] = _dot_t(_bf(abu[t, pl.ds(264, 128), :]), fb)
        PB[t, pl.ds(256, 272), :] = _dot_t(_bf(abu[t, pl.ds(128, 136), :]), fa)
        PB[t, pl.ds(784, 256), :] = _dot_t(_bf(abu[t, pl.ds(392, 128), :]), fb)
        yield _Step(-400, delay=2)
        first = _iota(8, 0) == 0

        def fix(v, v0):
            return jnp.concatenate([jnp.where(first, v0, v[:8]), v[8:]], 0).astype(BF16)

        UB[t, pl.ds(0, 64), :] = PB[t, pl.ds(0, 64), :].astype(BF16)
        UB[t, pl.ds(64, 64), :] = fix(PB[t, pl.ds(528, 64), :], PB[t, pl.ds(512, 8), :])
        UB[t, pl.ds(128, 64), :] = PB[t, pl.ds(256, 64), :].astype(BF16)
        UB[t, pl.ds(192, 64), :] = PB[t, pl.ds(528 + 256, 64), :].astype(BF16)
        for k in (1, 2, 3):
            pr, pi = PB[t, pl.ds(64 * k, 64), :], PB[t, pl.ds(528 + 64 * k, 64), :]
            mr, mi = PB[t, pl.ds(64 * (8 - k), 64), :], PB[t, pl.ds(528 + 64 * (8 - k), 64), :]
            UB[t, pl.ds(256 * k, 64), :] = fix(pr + mr, pr[:8])
            UB[t, pl.ds(256 * k + 64, 64), :] = fix(pi + mi, mr[:8])
            UB[t, pl.ds(256 * k + 128, 64), :] = fix(pi - mi, pi[:8])
            UB[t, pl.ds(256 * k + 192, 64), :] = fix(mr - pr, -mi[:8])
        yield _Step(190, [anchor(ubu, t, 480)])
        for c in range(8):
            PB[t, pl.ds(128 * c, 128), :] = _dot(mat({0: M_R0T, 1: M_C4T}.get(c, M_RT)),
                                                 _bf(ubu[t, pl.ds(64 * c, 64), :]))
        yield _Step(-400, delay=2)
        acc = None
        for r in range(8):
            rows = pl.ds(16 * r, 16)
            t0, t4 = PB[t, rows, :], PB[t, pl.ds(128 + 16 * r, 16), :]
            tk = {}
            for k in (1, 2, 3):
                c, sn = twid[2 * k - 2, rows, :], twid[2 * k - 1, rows, :]
                re = PB[t, pl.ds(256 * k + 16 * r, 16), :]
                im = PB[t, pl.ds(256 * k + 128 + 16 * r, 16), :]
                tk[k] = (re * c - im * sn, re * sn + im * c)
            e0, e1 = t0 + t4, t0 - t4
            s = [e0 + tk[2][0], e1 - tk[2][1], e0 - tk[2][0], e1 + tk[2][1]]
            al, be = tk[1][0] - tk[3][0], tk[1][1] + tk[3][1]
            o = [tk[1][0] + tk[3][0], (al - be) * RSQ2, tk[3][1] - tk[1][1], (al + be) * -RSQ2]
            for b in range(8):
                y = s[b] + o[b] if b < 4 else s[b - 4] - o[b - 4]
                v = X[zn, pl.ds(128 * b + 16 * r, 16), :] + y
                X[n, pl.ds(128 * b + 16 * r, 16), :] = v
                acc = v if acc is None else acc + v
            yield _Step(115, [anchor(X, n, 896 + 16 * r)])
        yield from ln_finish(n, _all_sublanes(acc[:8] + acc[8:], jnp.add, 0) * (1.0 / D), t)
        for r in range(2):
            mean, rstd = PB[t, pl.ds(1040, 8), :], PB[t, pl.ds(1048, 8), :]
            v = X[n, pl.ds(512 * r, 512), :].reshape(64, 8, 128)
            HB[n, pl.ds(512 * r, 512), :] = ((v - mean[None]) * rstd[None]).reshape(512, 128).astype(BF16)
            yield _Step(160, [anchor(hbu, n, 256 * r + 248)], marks=[name] if r == 1 else [])

    def attend(g, i, name, needs):
        n, j = 4 * g + i, g + 4 * i
        yield _Wait(*needs)
        sub = jax.lax.broadcasted_iota(I32, (1, 8, 128), 1)
        lane = jax.lax.broadcasted_iota(I32, (1, 8, 128), 2)
        wrapped = (lane == 0) & (2 * sub > j)

        def merge(a, b, pos_a, shift):
            sel = ((sum(1 << p for p in pos_a) >> sub) & 1) == 1
            return jnp.where(sel, a, b) + pltpu.roll(jnp.where(sel, b, a), 8 - shift, 1)

        def fold8(s):
            def quad(ws, o):
                z1 = merge(s[ws[0]], s[ws[1]], [(o + u) % 8 for u in range(4)], 4)
                z2 = merge(s[ws[2]], s[ws[3]], [(o + 2 + u) % 8 for u in range(4)], 4)
                return merge(z1, z2, [(o + u) % 8 for u in (0, 1, 4, 5)], 2)
            return merge(quad((0, 4, 2, 6), 0), quad((1, 5, 3, 7), 1), [0, 2, 4, 6], 1)

        hp = 2
        for h in range(0, 32, hp):
            rows = pl.ds(32 * h, 32 * hp)
            q = QB[i, rows, :]
            s = [(q * KE[j + 14 - 2 * w, rows, :]).reshape(hp, 4, 8, 128).sum(1) for w in range(8)]
            lg = jnp.where(wrapped, -1e9, fold8(s) * SCALE)
            e = jnp.exp(lg - _all_sublanes(lg, jnp.maximum, 1))
            p = e / _all_sublanes(e, jnp.add, 1)
            acc = None
            for w in range(8):
                pw = jnp.broadcast_to(p[:, w:w + 1, :], (hp, 32, 128)).reshape(32 * hp, 128)
                v = pw * VE[j + 14 - 2 * w, rows, :]
                acc = v if acc is None else acc + v
            HB[n, rows, :] = acc.astype(BF16)
            yield _Step(180 * hp, [anchor(hbu, n, 16 * h)], marks=[name] if h == 32 - hp else [])

    def proj(sch, w, n, m, store, needs, marks, own=120):
        def emit(anchors):
            lhs = WT[w, pl.ds(pl.multiple_of(64 * m, 64), 64), :]
            if anchors:
                head = lhs[:8, :128]
                for a in anchors:
                    head = jnp.where(never, pltpu.bitcast(a(), U32), head)
                top = jnp.concatenate([head, lhs[:8, 128:]], 1)
                lhs = jnp.concatenate([top, lhs[8:]], 0)
            store(_dot(_bf(lhs), _bf(hbu[n])), pl.ds(pl.multiple_of(128 * m, 128), 128))
        sch.chunk(emit, 256, own, needs, marks)

    def kv_proj(sch, g, i, needs):
        j = g + 4 * i
        shifted = j - 2 if i else jnp.where(g >= 2, g - 2, g + 30)
        for w, ref in ((1, KE), (2, VE)):
            def store(v, rows):
                ref[j + 14, rows, :] = v
                r = pltpu.roll(v, 1, 1)
                if w == 2:
                    r = jnp.where(_iota(128, 1) == 0, ref[14, rows, :], r)
                ref[shifted, rows, :] = r
            for m in range(8):
                proj(sch, w, 4 * g + i, m, store, needs, [], own=150)

    def q_proj(sch, g, i, name):
        def store(v, rows):
            QB[i, rows, :] = v
        for m in range(8):
            proj(sch, 0, 4 * g + i, m, store, [], [name] if m == 7 else [])

    def o_proj(sch, n, m, needs, marks):
        def store(v, rows):
            X[n, rows, :] = X[n, rows, :] + v
        proj(sch, 3, n, m, store, needs, marks, own=135)

    def transpose_weight(src, dst, name):
        for r in range(4):
            for c in range(4):
                WT[dst, pl.ds(128 * c, 128), pl.ds(256 * r, 256)] = pltpu.bitcast(
                    WRAW[src, pl.ds(256 * r, 256), pl.ds(256 * c, 256)].T, U32)
                yield _Step(140, [anchor(WT, dst, 128 * c, 256 * r)],
                            marks=[name] if r == 3 and c == 3 else [])

    def prep_spectral_weights(c2):
        lane = _iota(8, 1)
        order = jnp.where(lane > 64, 192 - lane, lane)

        def words(k2):
            re, im = (wsu[u, k2, pl.ds(c2, 64, stride=4), :] for u in range(2))
            return ((re & np.uint32(0xFFFF)) | (im << 16), (re >> 16) | (im & np.uint32(0xFFFF0000)))

        def arrange(w, below):
            w = jnp.where(_iota(w.shape[0], 1) < 64, w, below)
            return jnp.concatenate([jnp.take_along_axis(w[u:u + 8], order, axis=1)
                                    for u in range(0, w.shape[0], 8)], 0)

        below = words(15)
        for k2 in range(16):
            here = words(k2)
            for e in range(2):
                cl = 2 * c2 + e
                w = arrange(here[e], below[e])
                WS[k2, pl.ds(64 * cl, 64), :] = pltpu.roll(w, 1, 0) if cl > 4 else w
            below = here
        if c2 == 0:
            def nyquist(k2):
                re, im = (jnp.broadcast_to(WN[u, :, pl.ds(128 * k2, 128)].astype(F32), (8, 128))
                          for u in range(2))
                return pltpu.pack_elementwise([re, im], packed_dtype=BF16)
            for k2 in range(16):
                WS[k2, pl.ds(512, 8), :] = arrange(nyquist(k2), nyquist((k2 + 15) % 16))

    def write_out(lo, hi, p, c, name, needs):
        yield _Wait(*needs)
        rows = pl.ds(pl.multiple_of(128 * c, 128), 128)
        w = pltpu.pack_elementwise([X[lo, rows, :], X[hi, rows, :]], packed_dtype=BF16)
        xru[c, pl.ds(p, 128, stride=8), :] = w.T
        yield _Step(60, [anchor(xru, c, 0)], marks=[name])

    x_copy(0).start()
    x_copy(1).start()

    def load_x(c):
        x_copy(c).wait()
        pl.when(c < 6)(lambda: x_copy(c + 2).start())
        pl.when(c == 6)(lambda: start_all(spec_copies[0]))
        pl.when(c == 7)(lambda: start_all(spec_copies[1]))
        rows = pl.ds(pl.multiple_of(128 * c, 128), 128)
        for p in range(8):
            w = xru[c, pl.ds(p, 128, stride=8), :].T
            X[4 * (2 * p % 4) + p // 2, rows, :] = pltpu.bitcast(w << 16, F32)
            X[4 * ((2 * p + 1) % 4) + p // 2, rows, :] = pltpu.bitcast(w & np.uint32(0xFFFF0000), F32)

    _loop(8, load_x, 'load_x')

    def first_forward(g):
        pl.when(g == 1)(w_copies[1].start)
        pl.when(g == 2)(w_copies[2].start)
        sch = _Sched()
        for i in range(4):
            sch.add(fwd_block(g, i, ("f", i), [("f", i - 2)] if i >= 2 else []), ("f", i))
        sch.add(group_stage(g, "r", [("f", i) for i in range(4)], False), "r")
        sch.run(("f", 0), ("f", 1))
        sch.run(("f", 2), ("f", 3))
        sch.finish()

    _loop(4, first_forward, 'first_forward')
    w_copies[0].start()
    w_copies[3].start()
    for c in spec_copies[0] + spec_copies[1]:
        c.wait()

    def keys_values(layer, g):
        sch = _Sched(0.36 if layer == 0 else 0.33)
        if layer == 0:
            pl.when(g == 1)(w_copies[0].wait)
            pl.when(g == 2)(w_copies[3].wait)
        sch.done[("i", 0)] = 0
        for i in range(1, 3):
            sch.add(inv_block(g, i, ("i", i), []), ("i", i))
        nxt = (g + 1) % 4
        sch.add(inv_block(g, 3, ("i", 3), [("i", 1)]), ("i", 3))
        sch.add(group_stage(nxt, "r", [], True), "r")
        sch.add(inv_block(nxt, 0, ("i", 4), ["r", ("i", 2)], n=4 * g + 4), ("i", 4))
        if layer == 0:
            src = jnp.where(g == 1, 0, jnp.where(g == 2, 3, 1))
            sch.add(transpose_weight(src, jnp.where(src == 1, 4, src), "w"), "w", pace=1)
        for i in range(4):
            kv_proj(sch, g, i, [("i", i)])
        sch.finish()

    def block_of(g, i):
        return g + i // 4, i % 4

    def mix(g, last, tail):
        sch = _Sched(0.62)
        now = 8 - DEFER if last else 8
        sch.done[("a", 0)] = 0
        if not last:
            sch.add(group_stage((g + 3) % 4, "r", [], False), "r")
        for i in range(4):
            if i < 3 or not tail:
                sch.add(attend(*block_of(g, i + 1), ("a", i + 1), [("q", i + 1)] if i else []),
                        ("a", i + 1), pace=2 if last or tail else 1)
            if not last:
                sch.add(fwd_block(g, i, ("f", i), [("o", i, 7)] + ([("f", i - 2)] if i >= 2 else [])),
                        ("f", i))
            else:
                pair = 2 if tail else 0
                for c in range(now):
                    sch.add(write_out(4 * pair + i, 4 * pair + 4 + i, pair // 2 + 2 * i, c,
                                      ("w", i, c), [("o", i, c)]), ("w", i, c))
        if tail:
            q_proj(sch, g, 2, ("q", 2))
            q_proj(sch, g, 3, ("q", 3))
        for i in range(4):
            for m in range(now):
                o_proj(sch, 4 * g + i, m, [("a", i)], [("o", i, m)])
            if not tail:
                q_proj(sch, *block_of(g, i + 2), ("q", i + 2))
        if tail and not last:
            sch.add(group_stage(g, "s", [("f", i) for i in range(4)], False), "s")
        sch.finish()

    def postponed(u):
        c = 8 - DEFER + u
        sch = _Sched()
        for p in range(8):
            lo = 4 * (2 * p % 4) + p // 2
            sch.add(write_out(lo, lo + 4, p, c, ("w", p), [("o", p)]), ("w", p))
            o_proj(sch, lo, c, [], [])
            o_proj(sch, lo + 4, c, [], [("o", p)])
        sch.finish()
        out_copy(c).start()

    for layer in range(2):
        with jax.named_scope("spectral"):
            if layer == 0:
                prep_spectral_weights(0)
                for c2 in range(4):
                    if c2 < 3:
                        prep_spectral_weights(c2 + 1)
                    if c2 >= 2:
                        w_copies[c2 - 1].wait()
                        for _ in transpose_weight(c2 - 1, c2 - 1, None):
                            pass
                    spectral_rows(c2)
            else:
                _loop(4, spectral_rows, "rows")
            spectral(512, 8)
        sch = _Sched()
        sch.add(group_stage(0, "r", [], True), "r")
        sch.add(inv_block(0, 0, "i", ["r"]), "i")
        sch.finish()
        _loop(4, lambda g: keys_values(layer, g), "keys_values")
        sch = _Sched(0.6)
        sch.add(attend(0, 0, "a", ["q"]), "a", pace=2)
        q_proj(sch, 0, 0, "q")
        q_proj(sch, 0, 1, None)
        sch.finish()
        _loop(3, lambda g: mix(g, layer == 1, False), "mix")
        mix(3, layer == 1, True)
    for c in range(8 - DEFER):
        out_copy(c).start()
    _loop(DEFER, postponed, "postponed")
    for c in range(8):
        out_copy(c).wait()


@jax.jit
def pallas_interleave_layers__spectral_gfnet__sliding_local_dilated__prompt_kernel(
    A_x: jax.Array,
    A_w_r: jax.Array,
    A_w_i: jax.Array,
    B_x: jax.Array,
    B_wqkv: jax.Array,
    B_wo: jax.Array,
):
    del B_x
    hbm = pl.BlockSpec(memory_space=pl.ANY)
    smem = pl.BlockSpec(memory_space=pltpu.SMEM)
    out = pl.pallas_call(
        _kernel,
        out_shape=jax.ShapeDtypeStruct((S, D), BF16),
        in_specs=[smem, smem, pl.BlockSpec(), pl.BlockSpec(), pl.BlockSpec(), hbm, hbm, hbm, hbm, hbm],
        out_specs=hbm,
        scratch_shapes=[
            pltpu.VMEM((NB + 1, D, 128), F32),
            pltpu.VMEM((NB + 1, D, 128), BF16),
            pltpu.VMEM((32, D, 128), F32),
            pltpu.VMEM((32, D, 128), F32),
            pltpu.VMEM((4, D, 128), F32),
            pltpu.VMEM((2 * NB, ZR, 128), F32),
            pltpu.VMEM((NB, ZR, 128), U32),
            pltpu.VMEM((5, D // 2, D), U32),
            pltpu.VMEM((4, D, 128), BF16),
            pltpu.VMEM((4, 1040, 128), BF16),
            pltpu.VMEM((4, 1056, 128), F32),
            pltpu.VMEM((8, S, 128), BF16),
            pltpu.VMEM((2, NB, D // 2, 128), BF16),
            pltpu.VMEM((2, 1, S), BF16),
            pltpu.VMEM((4, D, D), BF16),
            pltpu.SemaphoreType.DMA((24,)),
        ],
        compiler_params=pltpu.CompilerParams(vmem_limit_bytes=124 * 2 ** 20),
    )(_ZERO, _ROT, _MATS, _LANES, _TWID, A_x.reshape(S, D), A_w_r.T, A_w_i.T, B_wqkv, B_wo)
    return out.reshape(1, S, D)
```

```python
import numpy as np

import jax
import jax.numpy as jnp
import jax.experimental.pallas as pl
import jax.experimental.pallas.tpu as pltpu

S, D, NB = 2048, 1024, 16
ZR = 520
F32, BF16, U32, I32 = jnp.float32, jnp.bfloat16, jnp.uint32, jnp.int32
EPS = 1e-5
SCALE = 32 ** -0.5
RSQ2 = float(np.sqrt(0.5))
WAIT = 16
LAG = 3
DEFER = 2

_S_ROWS = [(32 * u, 32) for u in range(16)] + [(512, 8)]

M_FA, M_FB, M_R, M_C4, M_RT, M_C4T, M_R0T = 0, 16, 32, 33, 34, 35, 36
L_MU, L_NU, L_KU, L_KV = 0, 16, 32, 48


def _bf16_bits(a):
    u = np.ascontiguousarray(a, dtype=np.float32).view(np.uint32).astype(np.uint64)
    return ((u + 0x7FFF + ((u >> 16) & 1)) >> 16).astype(np.uint32)


def _bf16_round(a):
    return (_bf16_bits(a) << 16).view(np.float32).astype(np.float64)


def _constants():
    a = np.arange(128)
    k1 = np.arange(64)
    alt = (-1.0) ** a
    mats = np.zeros((37, 128, 128))
    lanes = np.zeros((64, 128))
    for j in range(NB):
        t = 2 * np.pi * np.outer(16 * a + j, k1) / S
        ang = 2 * np.pi * j / 32 + np.pi / 32
        p, q = _bf16_round(np.array([np.cos(ang), np.sin(ang)]))
        fa = np.concatenate([np.cos(t), -np.sin(t)], 1)
        fb = np.concatenate([np.sin(t), -np.cos(t)], 1)
        fa[:, 0], fb[:, 0] = RSQ2, -RSQ2
        fa[:, 64], fb[:, 64] = p * alt, -q * alt
        mats[M_FA + j], mats[M_FB + j] = fa, fb
        lanes[L_MU + j, 0], lanes[L_MU + j, 64] = 1.0, (q / p + p / q) / 2
        lanes[L_NU + j, 0], lanes[L_NU + j, 64] = 0.0, (q / p - p / q) / 2
        lanes[L_KU + j, 0], lanes[L_KU + j, 64] = 1.0, q / p
        lanes[L_KV + j, 0], lanes[L_KV + j, 64] = 1.0, p / q
    th = 2 * np.pi * np.outer(k1, a) / 128
    r = np.concatenate([np.cos(th), -np.sin(th)], 0)
    r[64] = alt
    th = 2 * np.pi * np.outer(2 * k1 + 1, a) / 256
    c4 = np.concatenate([np.cos(th), -np.sin(th)], 0)
    inv = 2.0 / (S * D)
    mats[M_R], mats[M_C4], mats[M_RT], mats[M_C4T] = r, c4, inv * r.T, inv * c4.T
    mats[M_R0T] = mats[M_RT]
    mats[M_R0T, :, 0::64] *= 0.5
    bits = _bf16_bits(mats)
    mats_u32 = bits[:, 0::2] | (bits[:, 1::2] << 16)
    tw = np.zeros((6, 128, 128), np.float32)
    for k in (1, 2, 3):
        tw[2 * k - 2] = np.cos(2 * np.pi * a * k / D)[:, None]
        tw[2 * k - 1] = np.sin(2 * np.pi * a * k / D)[:, None]
    ang = 2 * np.pi * np.outer(np.arange(4), np.arange(4)).ravel() / 16
    rot = np.concatenate([np.cos(ang), np.sin(ang)]).astype(np.float32)
    return mats_u32, lanes.astype(np.float32), tw, rot


_MATS, _LANES, _TWID, _ROT = _constants()
_ZERO = np.zeros((1,), np.int32)


class _Step:
    def __init__(self, cost, anchors=(), delay=0, marks=()):
        self.cost, self.anchors, self.delay, self.marks = cost, list(anchors), delay, list(marks)


class _Wait:
    def __init__(self, *names):
        self.names = names


class _Mat:
    def __init__(self, emit):
        self.emit = emit


class _Hold:
    def __init__(self, store):
        self.store = store


class _Task:
    def __init__(self, gen, pace):
        self.gen, self.pace, self.blocked, self.not_before, self.held = gen, pace, (), 0, None
        self.allowed = 0.0


class _Sched:
    def __init__(self, share=0.0):
        self.share = share
        self.tasks, self.done, self.producer = [], {}, {}
        self.slot, self.credit, self.anchors, self.results = 0, 0.0, [], []
        self.fresh = False

    def add(self, gen, name, pace=99):
        self.producer[name] = self.producer["read", name] = _Task(gen, pace)
        self.tasks.append(self.producer[name])

    def _ready(self, t):
        return t.not_before <= self.slot and all(
            n in self.done and self.done[n] <= self.slot for n in t.blocked)

    def _advance(self, t, mats=True):
        item, t.held = t.held or next(t.gen, None), None
        if item is None:
            self.tasks.remove(t)
        elif isinstance(item, _Wait):
            t.blocked = item.names
        elif isinstance(item, _Hold):
            if len(self.results) >= LAG:
                item.store(self.results[-LAG])
        elif isinstance(item, _Mat):
            if mats:
                t.not_before = float("inf")
                self.fresh = False
                item.emit(lambda: self.point(0.0))
                t.not_before = self.slot + WAIT
            else:
                t.held, t.not_before = item, self.slot + 1
        else:
            t.blocked = ()
            t.not_before = self.slot + item.delay
            self.credit -= item.cost
            self.anchors += item.anchors
            for n in item.marks:
                self.done[n] = self.slot + item.delay
            return True

    def run(self, *names):
        while not all(n in self.done for n in names):
            for n in names:
                if n not in self.done:
                    for b in self.producer[n].blocked:
                        self.run(b)
                    self._advance(self.producer[n])

    def finish(self):
        self.run(*[n for n in self.producer if n[0] != "read"])

    def point(self, own):
        for t in self.tasks:
            t.allowed = min(t.allowed, 0.0) + t.pace
        while self.credit > 0:
            t = next((t for t in self.tasks if self._ready(t) and t.allowed > 0), None)
            if t is None:
                break
            if self._advance(t, self.fresh):
                t.allowed -= 1
        anchors, self.anchors = self.anchors, []
        self.credit = min(self.credit, 10.0) + 64 * self.share - own
        self.fresh = False
        self.slot += 1
        return anchors


def _dot(a, b):
    return jnp.dot(a, b, preferred_element_type=F32)


def _dot_t(a, b):
    return jax.lax.dot_general(a, b, (((1,), (1,)), ((), ())), preferred_element_type=F32)


def _bf(u):
    return pltpu.bitcast(u, BF16)


def _iota(rows, dim):
    return jax.lax.broadcasted_iota(I32, (rows, 128), dim)


def _radix4(z, inverse):
    (r0, i0), (r1, i1), (r2, i2), (r3, i3) = z
    ar, ai, cr, ci = r0 + r2, i0 + i2, r0 - r2, i0 - i2
    br, bi, dr, di = r1 + r3, i1 + i3, r1 - r3, i1 - i3
    lo, hi = (cr + di, ci - dr), (cr - di, ci + dr)
    if inverse:
        lo, hi = hi, lo
    return [(ar + br, ai + bi), lo, (ar - br, ai - bi), hi]


def _all_sublanes(v, op, axis):
    for sh in (4, 2, 1):
        v = op(v, pltpu.roll(v, sh, axis))
    return v


def _loop(n, body, name):
    def step(i, carry):
        body(i)
        return carry
    with jax.named_scope(name):
        jax.lax.fori_loop(0, n, step, 0)


def _kernel(zero_ref, rot, mats, lanes, twid, x_hbm, wr_hbm, wi_hbm, wqkv_hbm, wo_hbm, out_hbm,
            KE, VE, Z, ZT, WS, WT, XR, WRI, WN, WRAW, sems, *split):
    zero = zero_ref[0]
    never = zero != 0
    X, HB, QB = split[0::6], split[1::6], split[2::6]
    hbu = [r.bitcast(U32) for r in HB]
    xru, wsu = XR.bitcast(U32), WRI.bitcast(U32)
    temps = [(ub, ab, pb, ub.bitcast(U32), ab.bitcast(U32))
             for ub, ab, pb in zip(split[3::6], split[4::6], split[5::6])]
    counter = [0]

    def opaque():
        counter[0] += 1
        return zero * counter[0]

    def anchor(ref, idx, row, col=0):
        return lambda: ref[idx, pl.ds(pl.multiple_of(row + zero * 8, 8), 8), pl.ds(col, 128)]

    def hold(ref, spare):
        def store(v):
            ref[spare, pl.ds(pl.multiple_of(zero * 8, 8), 8), :] = v
        return _Hold(store)

    def tied(load, vregs, point):
        parts = []
        for r in range(vregs):
            anchors = point()
            u = load(8 * r)
            for a in anchors:
                u = jnp.where(never, pltpu.bitcast(a(), U32), u)
            parts.append(u)
        return jnp.concatenate(parts, 0)

    def mat(i):
        return _bf(mats[i])

    def d_stage(t, which):
        UB, AB, PB, ubu, abu = temps[t]

        def emit(point):
            z = opaque()
            for c in range(8):
                lhs = mat(which(c) + opaque()) if c % 4 else _bf(
                    tied(lambda r, u=which(c) + opaque(): mats[u, pl.ds(r, 8), :], 8, point))
                PB[0, pl.ds(128 * c, 128), :] = _dot(lhs, _bf(ubu[z, pl.ds(64 * c, 64), :]))
        return _Mat(emit)

    def s_stage(t, j, dot):
        UB, AB, PB, ubu, abu = temps[t]

        def emit(point):
            z = opaque()
            lhs = _bf(tied(lambda r: abu[z, pl.ds(r, 8), :], 16, point))
            fa, fb = mat(M_FA + j), mat(M_FB + j)
            PB[0, pl.ds(0, 256), :] = dot(lhs, fa)
            PB[0, pl.ds(528, 256), :] = dot(_bf(abu[z, pl.ds(264, 128), :]), fb)
            PB[0, pl.ds(256, 272), :] = dot(_bf(abu[z, pl.ds(128, 136), :]), fa)
            PB[0, pl.ds(784, 256), :] = dot(_bf(abu[z, pl.ds(392, 128), :]), fb)
        return _Mat(emit)

    def lane_vec(i, rows):
        return jnp.broadcast_to(lanes[pl.ds(i, 1), :], (rows, 128))

    def x_copy(c):
        return pltpu.make_async_copy(
            x_hbm.at[:, pl.ds(pl.multiple_of(128 * c, 128), 128)], XR.at[c], sems.at[c])

    def out_copy(c):
        return pltpu.make_async_copy(
            XR.at[c], out_hbm.at[:, pl.ds(pl.multiple_of(128 * c, 128), 128)], sems.at[8 + c])

    spec_copies = [[pltpu.make_async_copy(w.at[pl.ds(0, 512), pl.ds(128 * k2, 128)], WRI.at[u, k2],
                                          sems.at[16 + u]) for k2 in range(16)]
                   + [pltpu.make_async_copy(w.at[pl.ds(512, 1), :], WN.at[u], sems.at[22 + u])]
                   for u, w in enumerate((wr_hbm, wi_hbm))]

    def start_all(copies):
        for c in copies:
            c.start()
    w_copies = [pltpu.make_async_copy(wqkv_hbm.at[:, pl.ds(D * w, D)], WRAW.at[w], sems.at[18 + w])
                for w in range(3)] + [pltpu.make_async_copy(wo_hbm, WRAW.at[3], sems.at[21])]

    def ln_rstd(g, i, mean):
        acc, m = None, g + opaque()
        for r in range(8):
            d = X[i][m, pl.ds(128 * r, 128), :].reshape(16, 8, 128) - mean[None]
            v = (d * d).sum(0)
            acc = v if acc is None else acc + v
            if r < 7:
                yield _Step(50, [lambda acc=acc: acc], delay=3)
        rstd = jax.lax.rsqrt(_all_sublanes(acc, jnp.add, 0) * (1.0 / D) + EPS)
        yield _Step(50, delay=8)
        yield _Step(10, [lambda: rstd], delay=1)
        return rstd

    def fwd_block(g, i, name, needs, free=()):
        j, t = g + 4 * i, 2 + i % 2
        UB, AB, PB, ubu, abu = temps[t]
        yield _Wait(*needs)
        acc, m = None, g + opaque()
        for r in range(8):
            v = X[i][m, pl.ds(128 * r, 128), :].reshape(16, 8, 128).sum(0)
            acc = v if acc is None else acc + v
            if r % 2:
                yield _Step(35, [lambda acc=acc: acc], delay=7 if r == 7 else 3)
        mean = _all_sublanes(acc, jnp.add, 0) * (1.0 / D)
        rstd = yield from ln_rstd(g, i, mean)
        mean8, rstd = (jnp.concatenate([v, v], 0) for v in (mean * 8.0, rstd))
        z = opaque()
        for r in range(8):
            rows = pl.ds(16 * r, 16)
            x = [X[i][g + z, pl.ds(128 * b + 16 * r, 16), :] for b in range(8)]
            s = [x[b] + x[b + 4] for b in range(4)]
            d = [x[b] - x[b + 4] for b in range(4)]
            e, o = s[0] + s[2], s[1] + s[3]
            UB[0, rows, :] = ((e + o - mean8) * rstd).astype(BF16)
            UB[0, pl.ds(128 + 16 * r, 16), :] = ((e - o) * rstd).astype(BF16)
            t1, t2 = (d[1] - d[3]) * RSQ2, (d[1] + d[3]) * RSQ2
            u = {1: (d[0] + t1, d[2] + t2), 2: (s[0] - s[2], s[1] - s[3]), 3: (d[0] - t1, d[2] - t2)}
            yield _Step(34, [anchor(ubu, 0, 64 + 8 * r)], delay=1)
            for k in (1, 2, 3):
                c, sn = twid[z + 2 * k - 2, rows, :] * rstd, twid[z + 2 * k - 1, rows, :] * rstd
                re, m = u[k]
                if k == 3:
                    ur, ui = re * c + m * sn, m * c - re * sn
                else:
                    ur, ui = re * c - m * sn, m * c + re * sn
                UB[0, pl.ds(256 * k + 16 * r, 16), :] = ur.astype(BF16)
                UB[0, pl.ds(256 * k + 128 + 16 * r, 16), :] = ui.astype(BF16)
                yield _Step(26, [anchor(ubu, 0, 128 * k + 64 + 8 * r)], delay=1)
        yield d_stage(t, lambda c: M_C4 if c == 1 else M_R)
        z = opaque()
        first = _iota(64, 0) == 0

        def fix(v, v0):
            return jnp.concatenate([jnp.where(first[:8], v0, v[:8]), v[8:]], 0).astype(BF16)

        p1, p2 = PB[z, pl.ds(0, 64), :], PB[z, pl.ds(64, 64), :]
        AB[0, pl.ds(0, 64), :] = p1.astype(BF16)
        AB[0, pl.ds(528, 64), :] = jnp.where(first, 0.0, p2).astype(BF16)
        AB[0, pl.ds(512, 16), :] = jnp.where(first[:16], p2[:16], 0.0).astype(BF16)
        AB[0, pl.ds(256, 64), :] = PB[z, pl.ds(128, 64), :].astype(BF16)
        AB[0, pl.ds(528 + 256, 64), :] = PB[z, pl.ds(192, 64), :].astype(BF16)
        yield _Step(40, [anchor(abu, 0, 392)], delay=2)
        for k in (1, 2, 3):
            p1, p2 = PB[z, pl.ds(256 * k, 64), :], PB[z, pl.ds(256 * k + 64, 64), :]
            q1, q2 = PB[z, pl.ds(256 * k + 128, 64), :], PB[z, pl.ds(256 * k + 192, 64), :]
            if k == 3:
                pr, pi, mr, mi = p1 - q2, p2 + q1, p1 + q2, p2 - q1
                pi0, mi0 = q1[:8], -q2[:8]
            else:
                pr, pi, mr, mi = p1 + q2, p2 - q1, p1 - q2, p2 + q1
                pi0, mi0 = -q1[:8], q2[:8]
            AB[0, pl.ds(64 * k, 64), :] = fix(pr, p1[:8])
            AB[0, pl.ds(64 * (8 - k), 64), :] = fix(mr, p2[:8])
            AB[0, pl.ds(528 + 64 * k, 64), :] = fix(pi, pi0)
            AB[0, pl.ds(528 + 64 * (8 - k), 64), :] = fix(mi, mi0)
            yield _Step(55, [anchor(abu, 0, 264 + 32 * (8 - k))], delay=2)
        yield s_stage(t, j, _dot)
        z = opaque()
        yield _Wait(*free)
        for r0, rn in _S_ROWS:
            u = PB[z, pl.ds(r0, rn), :]
            if r0 < 512:
                v = PB[z, pl.ds(528 + r0, rn), :]
                re, m = u + v, u - v
            else:
                re = m = u
            edge = (_iota(rn, 1) & 63) == 0
            ZT[2 * i, pl.ds(r0, rn), :] = re
            ZT[2 * i + 1, pl.ds(r0, rn), :] = jnp.where(
                edge, lane_vec(L_MU + j, rn) * m + lane_vec(L_NU + j, rn) * re, pltpu.roll(m, 64, 1))
            yield _Step(rn, [anchor(ZT, 2 * i + 1, r0)], delay=1, marks=[name] if r0 == 512 else [])

    def group_stage(g, name, needs, inverse):
        yield _Wait(*needs)

        def turn(z, k):
            if k == 0:
                return z
            c, s = rot[4 * g + k], rot[16 + 4 * g + k]
            if inverse:
                return z[0] * c - z[1] * s, z[1] * c + z[0] * s
            return z[0] * c + z[1] * s, z[1] * c - z[0] * s

        (src, a), (dst, b) = ((Z, 8 * g), (ZT, 0)) if inverse else ((ZT, opaque()), (Z, 8 * g))
        for r in range(65):
            if r % 4 == 0:
                yield hold(src, 2 * NB if inverse else 8)
            rows = pl.ds(8 * r, 8)
            z = [(src[a + 2 * i, rows, :], src[a + 2 * i + 1, rows, :]) for i in range(4)]
            if inverse:
                z = _radix4([turn(z[k], k) for k in range(4)], True)
            else:
                z = [turn(v, k) for k, v in enumerate(_radix4(z, False))]
            for i in range(4):
                dst[b + 2 * i, rows, :], dst[b + 2 * i + 1, rows, :] = z[i]
            yield _Step(35, [anchor(dst, b + 7, 8 * r)], delay=1, marks=[name] if r == 64 else [])

    def spectral(row, size):
        rows = pl.ds(row, size)
        for k0 in range(4):
            z = _radix4([(Z[8 * g + 2 * k0, rows, :], Z[8 * g + 2 * k0 + 1, rows, :])
                         for g in range(4)], False)
            y = []
            for k1, (re, im) in enumerate(z):
                w = WS[k0 + 4 * k1, rows, :]
                wr = pltpu.bitcast(w << 16, F32)
                wi = pltpu.bitcast(w & np.uint32(0xFFFF0000), F32)
                y.append((re * wr - im * wi, re * wi + im * wr))
            y = _radix4(y, True)
            for g in range(4):
                Z[8 * g + 2 * k0, rows, :], Z[8 * g + 2 * k0 + 1, rows, :] = y[g]

    def spectral_rows(c2):
        for r in range(8):
            spectral(pl.multiple_of(128 * c2 + 16 * r, 16), 16)

    def inv_block(g, i, name, needs, n=None):
        j, t = g + 4 * i, i % 2
        UB, AB, PB, ubu, abu = temps[t]
        n = g if n is None else n
        z = opaque()
        yield _Wait(*needs)
        for r0, rn in _S_ROWS:
            if r0 == 0:
                yield hold(ZT, 8)
            re, im = ZT[z + 2 * i, pl.ds(r0, rn), :], ZT[z + 2 * i + 1, pl.ds(r0, rn), :]
            edge = (_iota(rn, 1) & 63) == 0
            rolled = pltpu.roll(im, 64, 1)
            u = re + jnp.where(edge, lane_vec(L_KU + j, rn) * im, rolled)
            if r0 < 512:
                v = re - jnp.where(edge, lane_vec(L_KV + j, rn) * im, rolled)
                AB[0, pl.ds(r0, rn), :] = u.astype(BF16)
                AB[0, pl.ds(528 + r0, rn), :] = v.astype(BF16)
            else:
                AB[0, pl.ds(512, 16), :] = jnp.concatenate([u, jnp.zeros_like(u)], 0).astype(BF16)
            yield _Step(rn, [anchor(abu, 0, r0 // 2)], delay=1, marks=[("read", name)] if r0 == 512 else [])
        yield s_stage(t, j, _dot_t)
        z = opaque()
        first = _iota(8, 0) == 0

        def fix(v, v0):
            return jnp.concatenate([jnp.where(first, v0, v[:8]), v[8:]], 0).astype(BF16)

        UB[0, pl.ds(0, 64), :] = PB[z, pl.ds(0, 64), :].astype(BF16)
        UB[0, pl.ds(64, 64), :] = fix(PB[z, pl.ds(528, 64), :], PB[z, pl.ds(512, 8), :])
        UB[0, pl.ds(128, 64), :] = PB[z, pl.ds(256, 64), :].astype(BF16)
        UB[0, pl.ds(192, 64), :] = PB[z, pl.ds(528 + 256, 64), :].astype(BF16)
        yield _Step(40, [anchor(ubu, 0, 96)], delay=2)
        for k in (1, 2, 3):
            pr, pi = PB[z, pl.ds(64 * k, 64), :], PB[z, pl.ds(528 + 64 * k, 64), :]
            mr, mi = PB[z, pl.ds(64 * (8 - k), 64), :], PB[z, pl.ds(528 + 64 * (8 - k), 64), :]
            UB[0, pl.ds(256 * k, 64), :] = fix(pr + mr, pr[:8])
            UB[0, pl.ds(256 * k + 64, 64), :] = fix(pi + mi, mr[:8])
            UB[0, pl.ds(256 * k + 128, 64), :] = fix(pi - mi, pi[:8])
            UB[0, pl.ds(256 * k + 192, 64), :] = fix(mr - pr, -mi[:8])
            yield _Step(55, [anchor(ubu, 0, 128 * k + 96)], delay=2)
        yield d_stage(t, lambda c: {0: M_R0T, 1: M_C4T}.get(c, M_RT))
        z = opaque()
        acc = None
        for r in range(16):
            rows = pl.ds(8 * r, 8)
            t0, t4 = PB[z, rows, :], PB[z, pl.ds(128 + 8 * r, 8), :]
            tk = {}
            for k in (1, 2, 3):
                c, sn = twid[z + 2 * k - 2, rows, :], twid[z + 2 * k - 1, rows, :]
                re = PB[z, pl.ds(256 * k + 8 * r, 8), :]
                im = PB[z, pl.ds(256 * k + 128 + 8 * r, 8), :]
                tk[k] = (re * c - im * sn, re * sn + im * c)
            e0, e1 = t0 + t4, t0 - t4
            s = [e0 + tk[2][0], e1 - tk[2][1], e0 - tk[2][0], e1 + tk[2][1]]
            al, be = tk[1][0] - tk[3][0], tk[1][1] + tk[3][1]
            o = [tk[1][0] + tk[3][0], (al - be) * RSQ2, tk[3][1] - tk[1][1], (al + be) * -RSQ2]
            for b in range(8):
                y = s[b] + o[b] if b < 4 else s[b - 4] - o[b - 4]
                v = X[i][g, pl.ds(128 * b + 8 * r, 8), :] + y
                X[i][n, pl.ds(128 * b + 8 * r, 8), :] = v
                acc = v if acc is None else acc + v
            yield _Step(57, [lambda v=acc: v], delay=5 if r == 15 else 2)
        mean = _all_sublanes(acc, jnp.add, 0) * (1.0 / D)
        rstd = yield from ln_rstd(n, i, mean)
        z = opaque()
        for r in range(8):
            v = X[i][n + z, pl.ds(128 * r, 128), :].reshape(16, 8, 128)
            HB[i][n, pl.ds(128 * r, 128), :] = ((v - mean[None]) * rstd[None]).reshape(128, 128).astype(BF16)
            yield _Step(41, [anchor(hbu[i], n, 64 * r + 56)], delay=1, marks=[name] if r == 7 else [])

    def attend(g, i, name, needs):
        j = g + 4 * i
        yield _Wait(*needs)
        z = opaque()
        jz = j + z
        sub = _iota(8, 0)
        wrapped = (_iota(8, 1) == 0) & (2 * sub > j)

        def merge(a, b, pos_a, shift):
            sel = ((sum(1 << p for p in pos_a) >> sub) & 1) == 1
            return jnp.where(sel, a, b) + pltpu.roll(jnp.where(sel, b, a), 8 - shift, 0)

        def quad(q, rows, ws, o):
            s = [(q * KE[jz + 14 - 2 * w, rows, :]).reshape(4, 8, 128).sum(0) for w in ws]
            z1 = merge(s[0], s[1], [(o + u) % 8 for u in range(4)], 4)
            z2 = merge(s[2], s[3], [(o + 2 + u) % 8 for u in range(4)], 4)
            return merge(z1, z2, [(o + u) % 8 for u in (0, 1, 4, 5)], 2)

        def mix_values(h, u, pw):
            rows = pl.ds(32 * h + 16 * u, 16)
            acc = None
            for w in range(8):
                v = pw[w] * VE[jz + 14 - 2 * w, rows, :]
                acc = v if acc is None else acc + v
            HB[i][g, rows, :] = acc.astype(BF16)
            return _Step(40 - 8 * u, [anchor(hbu[i], g, 16 * h + 8 * u)],
                         marks=[name] if h == 31 and u else [])

        p = None
        for h in range(33):
            if h < 32:
                rows = pl.ds(32 * h, 32)
                q = QB[i][z, rows, :]
                even = quad(q, rows, (0, 4, 2, 6), 0)
                yield _Step(41, [lambda v=even: v])
                odd = quad(q, rows, (1, 5, 3, 7), 1)
                yield _Step(41, [lambda v=odd: v], delay=0 if h else 2)
            if h > 0:
                pw = [jnp.broadcast_to(p[w:w + 1, :], (16, 128)) for w in range(8)]
                yield mix_values(h - 1, 0, pw)
            if h < 32:
                lg = merge(even, odd, [0, 2, 4, 6], 1)
                lg = jnp.where(wrapped, -1e9, lg * SCALE)
                e = jnp.exp(lg - _all_sublanes(lg, jnp.maximum, 0))
                yield _Step(17, [lambda v=e: v], delay=0 if h else 2)
            if h > 0:
                yield mix_values(h - 1, 1, pw)
            if h < 32:
                p = e / _all_sublanes(e, jnp.add, 0)
                yield _Step(18, [lambda v=p: v], delay=2 if h == 31 else 0)

    def proj(sch, w, g, i, m, store, needs, marks, own=120):
        for name in needs:
            sch.run(name)
        row, w = pl.multiple_of(64 * m, 64), w + opaque()
        parts = []
        sch.fresh = True
        for col in (0, 512):
            parts.append(tied(lambda r: WT[w, pl.ds(row + r, 8), pl.ds(col, 128)], 8,
                              lambda: sch.point(own / 16)))
            parts.append(WT[w, pl.ds(row, 64), pl.ds(col + 128, 384)])
        v = _dot(_bf(jnp.concatenate(parts, 1)), _bf(hbu[i][g + opaque()]))
        store(v, pl.ds(pl.multiple_of(128 * m, 128), 128))
        sch.results.append(v[:8])
        for name in marks:
            sch.done[name] = sch.slot + WAIT

    def kv_proj(sch, g, i, needs):
        j = g + 4 * i
        shifted = j - 2 if i else jnp.where(g >= 2, g - 2, g + 30)
        for w, ref in ((1, KE), (2, VE)):
            def store(v, rows):
                ref[j + 14, rows, :] = v
                r = pltpu.roll(v, 1, 1)
                if w == 2:
                    r = jnp.where(_iota(128, 1) == 0, ref[14 + opaque(), rows, :], r)
                ref[shifted, rows, :] = r
            for m in range(8):
                proj(sch, w, g, i, m, store, needs, [], own=150)

    def q_proj(sch, g, i, name):
        def store(v, rows):
            QB[i][0, rows, :] = v
        for m in range(8):
            proj(sch, 0, g, i, m, store, [], [name] if m == 7 else [])

    def o_proj(sch, g, i, m, needs, marks):
        def store(v, rows):
            X[i][g, rows, :] = X[i][g, rows, :] + v
        proj(sch, 3, g, i, m, store, needs, marks, own=135)

    def transpose_weight(src, dst, name):
        for r in range(4):
            for c in range(4):
                WT[dst, pl.ds(128 * c, 128), pl.ds(256 * r, 256)] = pltpu.bitcast(
                    WRAW[src, pl.ds(256 * r, 256), pl.ds(256 * c, 256)].T, U32)
                yield _Step(40, delay=20)
                yield _Step(4, [anchor(WT, dst, 128 * c, 256 * r)],
                            marks=[name] if r == 3 and c == 3 else [])

    def prep_spectral_weights(c2):
        lane = _iota(8, 1)
        order = jnp.where(lane > 64, 192 - lane, lane)

        def words(k2):
            re, im = (wsu[u, k2, pl.ds(c2, 64, stride=4), :] for u in range(2))
            return ((re & np.uint32(0xFFFF)) | (im << 16), (re >> 16) | (im & np.uint32(0xFFFF0000)))

        def arrange(w, below):
            w = jnp.where(_iota(w.shape[0], 1) < 64, w, below)
            return jnp.concatenate([jnp.take_along_axis(w[u:u + 8], order, axis=1)
                                    for u in range(0, w.shape[0], 8)], 0)

        below = words(15)
        for k2 in range(16):
            here = words(k2)
            for e in range(2):
                cl = 2 * c2 + e
                w = arrange(here[e], below[e])
                WS[k2, pl.ds(64 * cl, 64), :] = pltpu.roll(w, 1, 0) if cl > 4 else w
            below = here
        if c2 == 0:
            def nyquist(k2):
                re, im = (jnp.broadcast_to(WN[u, :, pl.ds(128 * k2, 128)].astype(F32), (8, 128))
                          for u in range(2))
                return pltpu.pack_elementwise([re, im], packed_dtype=BF16)
            for k2 in range(16):
                WS[k2, pl.ds(512, 8), :] = arrange(nyquist(k2), nyquist((k2 + 15) % 16))

    def write_out(p, c, name, needs):
        yield _Wait(*needs)
        rows = pl.ds(pl.multiple_of(128 * c, 128), 128)
        g, i = 2 * p % 4 + opaque(), p // 2
        w = pltpu.pack_elementwise([X[i][g, rows, :], X[i][g + 1, rows, :]], packed_dtype=BF16)
        xru[c, pl.ds(p, 128, stride=8), :] = w.T
        yield _Step(30, marks=[name])

    x_copy(0).start()
    x_copy(1).start()

    def load_x(c):
        x_copy(c).wait()
        pl.when(c < 6)(lambda: x_copy(c + 2).start())
        pl.when(c == 6)(lambda: start_all(spec_copies[0]))
        pl.when(c == 7)(lambda: start_all(spec_copies[1]))
        rows = pl.ds(pl.multiple_of(128 * c, 128), 128)
        for p in range(8):
            w = xru[c, pl.ds(p, 128, stride=8), :].T
            X[p // 2][2 * p % 4, rows, :] = pltpu.bitcast(w << 16, F32)
            X[p // 2][2 * p % 4 + 1, rows, :] = pltpu.bitcast(w & np.uint32(0xFFFF0000), F32)

    _loop(8, load_x, 'load_x')

    def first_forward(g):
        pl.when(g == 1)(w_copies[1].start)
        pl.when(g == 2)(w_copies[2].start)
        sch = _Sched()
        for i in range(4):
            sch.add(fwd_block(g, i, ("f", i), [("f", i - 2)] if i >= 2 else []), ("f", i))
        sch.add(group_stage(g, "r", [("f", i) for i in range(4)], False), "r")
        sch.run(("f", 0), ("f", 1))
        sch.run(("f", 2), ("f", 3))
        sch.finish()

    _loop(4, first_forward, 'first_forward')
    w_copies[0].start()
    w_copies[3].start()
    for c in spec_copies[0] + spec_copies[1]:
        c.wait()

    def keys_values(layer, g):
        sch = _Sched(0.36 if layer == 0 else 0.33)
        if layer == 0:
            pl.when(g == 1)(w_copies[0].wait)
            pl.when(g == 2)(w_copies[3].wait)
        sch.done[("i", 0)] = 0
        for i in range(1, 3):
            sch.add(inv_block(g, i, ("i", i), [("read", ("i", 1))] if i == 2 else []), ("i", i))
        nxt = (g + 1) % 4
        sch.add(inv_block(g, 3, ("i", 3), [("i", 1)]), ("i", 3))
        sch.add(group_stage(nxt, "r", [("read", ("i", i)) for i in (1, 2, 3)], True), "r")
        sch.add(inv_block(nxt, 0, ("i", 4), ["r", ("i", 2)], n=g + 1), ("i", 4))
        if layer == 0:
            src = jnp.where(g == 1, 0, jnp.where(g == 2, 3, 1))
            sch.add(transpose_weight(src, jnp.where(src == 1, 4, src), "w"), "w")
        for i in range(4):
            kv_proj(sch, g, i, [("i", i)])
        sch.finish()

    def block_of(g, i):
        return g + i // 4, i % 4

    def mix(g, last, tail):
        sch = _Sched(0.67 if last else 0.63)
        now = 8 - DEFER if last else 8
        sch.done[("a", 0)] = 0
        for i in range(3 if tail else 4):
            sch.add(attend(*block_of(g, i + 1), ("a", i + 1),
                           [("q", i + 1), ("a", i)] if i else []),
                    ("a", i + 1), pace=1.03 if last or tail else 0.87)
        if not last:
            sch.add(group_stage((g + 3) % 4, "r", [], False), "r")
        for i in range(4):
            if not last:
                sch.add(fwd_block(g, i, ("f", i), [("o", i, 7)] + ([("f", i - 2)] if i >= 2 else []), ["r"]),
                        ("f", i))
            else:
                for c in range(now):
                    sch.add(write_out(2 * i + (1 if tail else 0), c,
                                      ("w", i, c), [("o", i, c)]), ("w", i, c))
        if tail:
            q_proj(sch, g, 2, ("q", 2))
            q_proj(sch, g, 3, ("q", 3))
        for i in range(4):
            for m in range(now):
                o_proj(sch, g, i, m, [("a", i)], [("o", i, m)])
            if not tail:
                q_proj(sch, *block_of(g, i + 2), ("q", i + 2))
        if tail and not last:
            sch.add(group_stage(g, "s", [("f", i) for i in range(4)], False), "s")
        sch.finish()

    def postponed(u):
        c = 8 - DEFER + u
        sch = _Sched(0.5)
        for p in range(8):
            sch.add(write_out(p, c, ("w", p), [("o", p)]), ("w", p))
            o_proj(sch, 2 * p % 4, p // 2, c, [], [])
            o_proj(sch, 2 * p % 4 + 1, p // 2, c, [], [("o", p)])
        sch.finish()
        out_copy(c).start()

    for layer in range(2):
        with jax.named_scope("spectral"):
            if layer == 0:
                prep_spectral_weights(0)
                for c2 in range(4):
                    if c2 < 3:
                        prep_spectral_weights(c2 + 1)
                    if c2 >= 2:
                        w_copies[c2 - 1].wait()
                        for _ in transpose_weight(c2 - 1, c2 - 1, None):
                            pass
                    spectral_rows(c2)
            else:
                _loop(4, spectral_rows, "rows")
            spectral(512, 8)
        sch = _Sched()
        sch.add(group_stage(0, "r", [], True), "r")
        sch.add(inv_block(0, 0, "i", ["r"]), "i")
        sch.finish()
        _loop(4, lambda g: keys_values(layer, g), "keys_values")
        sch = _Sched(0.66)
        sch.add(attend(0, 0, "a", ["q"]), "a")
        q_proj(sch, 0, 0, "q")
        q_proj(sch, 0, 1, None)
        sch.finish()
        _loop(3, lambda g: mix(g, layer == 1, False), "mix")
        mix(3, layer == 1, True)
    for c in range(8 - DEFER):
        out_copy(c).start()
    _loop(DEFER, postponed, "postponed")
    for c in range(8):
        out_copy(c).wait()


@jax.jit
def pallas_interleave_layers__spectral_gfnet__sliding_local_dilated__prompt_kernel(
    A_x: jax.Array,
    A_w_r: jax.Array,
    A_w_i: jax.Array,
    B_x: jax.Array,
    B_wqkv: jax.Array,
    B_wo: jax.Array,
):
    del B_x
    hbm = pl.BlockSpec(memory_space=pl.ANY)
    smem = pl.BlockSpec(memory_space=pltpu.SMEM)
    out = pl.pallas_call(
        _kernel,
        out_shape=jax.ShapeDtypeStruct((S, D), BF16),
        in_specs=[smem, smem, pl.BlockSpec(), pl.BlockSpec(), pl.BlockSpec(), hbm, hbm, hbm, hbm, hbm],
        out_specs=hbm,
        scratch_shapes=[
            pltpu.VMEM((32, D, 128), F32),
            pltpu.VMEM((32, D, 128), F32),
            pltpu.VMEM((2 * NB + 1, ZR, 128), F32),
            pltpu.VMEM((9, ZR, 128), F32),
            pltpu.VMEM((NB, ZR, 128), U32),
            pltpu.VMEM((5, D // 2, D), U32),
            pltpu.VMEM((8, S, 128), BF16),
            pltpu.VMEM((2, NB, D // 2, 128), BF16),
            pltpu.VMEM((2, 1, S), BF16),
            pltpu.VMEM((4, D, D), BF16),
            pltpu.SemaphoreType.DMA((24,)),
        ] + 4 * [
            pltpu.VMEM((5, D, 128), F32),
            pltpu.VMEM((5, D, 128), BF16),
            pltpu.VMEM((1, D, 128), F32),
            pltpu.VMEM((1, D, 128), BF16),
            pltpu.VMEM((1, 1040, 128), BF16),
            pltpu.VMEM((1, 1040, 128), F32),
        ],
        compiler_params=pltpu.CompilerParams(vmem_limit_bytes=124 * 2 ** 20),
    )(_ZERO, _ROT, _MATS, _LANES, _TWID, A_x.reshape(S, D), A_w_r.T, A_w_i.T, B_wqkv, B_wo)
    return out.reshape(1, S, D)
```

```python
import functools

import numpy as np

import jax
import jax.numpy as jnp
import jax.experimental.pallas as pl
import jax.experimental.pallas.tpu as pltpu

S, D, NB = 2048, 1024, 16
ZR = 520
F32, BF16, U32, I32 = jnp.float32, jnp.bfloat16, jnp.uint32, jnp.int32
EPS = 1e-5
SCALE = 32 ** -0.5
RSQ2 = float(np.sqrt(0.5))
WAIT = 16
GRAIN = 1
SETTLE = 3
LAG = 3
DEFER = 2

_S_ROWS = [(32 * u, 32) for u in range(16)] + [(512, 8)]

M_FA, M_FB, M_R, M_C4, M_RT, M_C4T, M_R0T = 0, 16, 32, 33, 34, 35, 36
L_MU, L_NU, L_KU, L_KV, L_COS, L_SIN, L_TWID, L_FA, L_FB = 0, 16, 32, 48, 64, 80, 96, 104, 232


def _bf16_bits(a):
    u = np.ascontiguousarray(a, dtype=np.float32).view(np.uint32).astype(np.uint64)
    return ((u + 0x7FFF + ((u >> 16) & 1)) >> 16).astype(np.uint32)


def _constants():
    a = np.arange(128)
    k1 = np.arange(64)
    alt = (-1.0) ** a
    lanes = np.zeros((L_FB + 128, 128))
    t = 2 * np.pi * np.outer(a, k1) / 128
    fa = np.concatenate([np.cos(t), -np.sin(t)], 1)
    fb = np.concatenate([np.sin(t), -np.cos(t)], 1)
    fa[:, 0], fb[:, 0] = RSQ2, -RSQ2
    fa[:, 64], fb[:, 64] = alt, 0.0
    lanes[L_FA:L_FA + 128], lanes[L_FB:L_FB + 128] = fa, fb
    for j in range(NB):
        ang = 2 * np.pi * j / 32 + np.pi / 32
        p, q = (_bf16_bits([np.cos(ang), np.sin(ang)]) << 16).view(np.float32).astype(np.float64)
        turn = 2 * np.pi * j * np.tile(k1, 2) / S
        lanes[L_COS + j], lanes[L_SIN + j] = np.cos(turn), -np.sin(turn)
        lanes[L_COS + j, 64], lanes[L_SIN + j, 64] = p, q
        lanes[L_MU + j, 0], lanes[L_MU + j, 64] = 1.0, (q / p + p / q) / 2
        lanes[L_NU + j, 0], lanes[L_NU + j, 64] = 0.0, (q / p - p / q) / 2
        lanes[L_KU + j, 0], lanes[L_KU + j, 64] = 1.0, q / p
        lanes[L_KV + j, 0], lanes[L_KV + j, 64] = 1.0, p / q
    for k in (1, 2, 3):
        lanes[L_TWID + 2 * k - 2] = np.cos(2 * np.pi * a * k / D)
        lanes[L_TWID + 2 * k - 1] = np.sin(2 * np.pi * a * k / D)
    th = 2 * np.pi * np.outer(k1, a) / 128
    r = np.concatenate([np.cos(th), -np.sin(th)], 0)
    r[64] = alt
    th = 2 * np.pi * np.outer(2 * k1 + 1, a) / 256
    c4 = np.concatenate([np.cos(th), -np.sin(th)], 0)
    inv = 2.0 / (S * D)
    r0t = inv * r.T
    r0t[:, 0::64] *= 0.5
    rows = np.arange(128).reshape(2, 4, 16).transpose(1, 0, 2).ravel()
    bits = _bf16_bits(np.stack([r[rows], c4[rows], inv * r.T, inv * c4.T, r0t]))
    ang = 2 * np.pi * np.outer(np.arange(4), np.arange(4)).ravel() / 16
    rot = np.concatenate([np.cos(ang), np.sin(ang)]).astype(np.float32)
    return bits[:, 0::2] | (bits[:, 1::2] << 16), lanes.astype(np.float32), rot


_MATS, _LANES, _ROT = _constants()
_ZERO = np.zeros((1,), np.int32)


class _Step:
    def __init__(self, cost, anchors=(), delay=0, marks=()):
        self.cost, self.anchors, self.delay, self.marks = cost, list(anchors), delay, list(marks)


class _Wait:
    def __init__(self, *names):
        self.names = names


class _Mat:
    def __init__(self, emit):
        self.emit = emit


class _Hold:
    def __init__(self, store):
        self.store = store


class _Task:
    def __init__(self, gen, pace):
        self.gen, self.pace, self.blocked, self.not_before, self.held = gen, pace, (), 0, None
        self.allowed = 0.0


class _Sched:
    def __init__(self, share=0.0):
        self.share = share
        self.tasks, self.done, self.producer = [], {}, {}
        self.slot, self.credit, self.anchors, self.results = 0, 0.0, [], []
        self.fresh = False

    def add(self, gen, name, pace=99):
        self.producer[name] = self.producer["read", name] = _Task(gen, pace)
        self.tasks.append(self.producer[name])

    def _ready(self, t):
        return t.not_before <= self.slot and all(
            n in self.done and self.done[n] <= self.slot for n in t.blocked)

    def _advance(self, t, mats=True):
        item, t.held = t.held or next(t.gen, None), None
        if item is None:
            self.tasks.remove(t)
        elif isinstance(item, _Wait):
            t.blocked = item.names
        elif isinstance(item, _Hold):
            if len(self.results) >= LAG:
                item.store(self.results[-LAG])
        elif isinstance(item, _Mat):
            if mats:
                t.not_before = float("inf")
                self.fresh = False
                self.credit -= item.emit(lambda: self.point(0.0)) or 0
                t.not_before = self.slot + WAIT
            else:
                t.held, t.not_before = item, self.slot + 1
        else:
            t.blocked = ()
            t.not_before = self.slot + item.delay
            self.credit -= item.cost
            self.anchors += item.anchors
            for n in item.marks:
                self.done[n] = self.slot + item.delay
            return True

    def run(self, *names):
        while not all(n in self.done for n in names):
            for n in names:
                if n not in self.done:
                    for b in self.producer[n].blocked:
                        self.run(b)
                    self._advance(self.producer[n])

    def drive(self):
        while self.tasks:
            ready = [t for t in self.tasks if self._ready(t)]
            if not ready:
                self.slot += 1
                continue
            self.anchors, self.credit = self.anchors[-2:], 0.0
            self._advance(next((t for t in ready if t.held), ready[0]))
            self.slot -= min(self.credit, 0.0) / 60

    def finish(self):
        self.run(*[n for n in self.producer if n[0] != "read"])

    def point(self, own):
        for t in self.tasks:
            t.allowed = min(t.allowed, 0.0) + t.pace
        while True:
            t = next((t for t in self.tasks if self._ready(t) and t.allowed > 0
                      and self.credit > 0), None)
            if t is None:
                break
            if self._advance(t, self.fresh):
                t.allowed -= 1
        anchors, self.anchors = self.anchors, []
        self.credit = min(self.credit, 10.0) + 64 * self.share - own
        self.fresh = False
        self.slot += 1
        return anchors


def _dot(a, b):
    return jnp.dot(a, b, preferred_element_type=F32)


def _dot_t(a, b):
    return jax.lax.dot_general(a, b, (((1,), (1,)), ((), ())), preferred_element_type=F32)


def _bf(u):
    return pltpu.bitcast(u, BF16)


def _iota(rows, dim):
    return jax.lax.broadcasted_iota(I32, (rows, 128), dim)


def _radix4(z, inverse):
    (r0, i0), (r1, i1), (r2, i2), (r3, i3) = z
    ar, ai, cr, ci = r0 + r2, i0 + i2, r0 - r2, i0 - i2
    br, bi, dr, di = r1 + r3, i1 + i3, r1 - r3, i1 - i3
    lo, hi = (cr + di, ci - dr), (cr - di, ci + dr)
    if inverse:
        lo, hi = hi, lo
    return [(ar + br, ai + bi), lo, (ar - br, ai - bi), hi]


def _all_sublanes(v, op, axis):
    for sh in (4, 2, 1):
        v = op(v, pltpu.roll(v, sh, axis))
    return v


def _loop(n, body, name):
    def step(i, carry):
        body(i)
        return carry
    with jax.named_scope(name):
        jax.lax.fori_loop(0, n, step, 0)


def _kernel(zero_ref, rot, d_mats, lanes, x_hbm, wr_hbm, wi_hbm, wqkv_hbm, wo_hbm, out_hbm,
            mats, twid, STAT, KE, VE, KS, VS, Z, ZT, WS, WT, XR, WRI, WN, WRAW, WO, TR, PW0, PW1, sems, *split):
    zero = zero_ref[0]
    never = zero != 0
    X, HB, QB = split[0::6], split[1::6], split[2::6]
    hbu = [r.bitcast(U32) for r in HB]
    xru, wsu, wou = XR.bitcast(U32), WRI.bitcast(U32), WO.bitcast(U32)
    temps = [(ub, ab, pb, ub.bitcast(U32), ab.bitcast(U32))
             for ub, ab, pb in zip(split[3::6], split[4::6], split[5::6])]
    PW = (PW0, PW1)
    counter = [0]

    def opaque():
        counter[0] += 1
        return zero * counter[0]

    def anchor(ref):
        return lambda: ref[0, pl.ds(pl.multiple_of(zero * 8, 8), 8), pl.ds(0, 128)]

    def settle(ref):
        return _Step(2, [anchor(ref)], delay=SETTLE)

    def hold(ref, spare, row=0):
        def store(v):
            ref[spare, pl.ds(pl.multiple_of(row + zero * 8, 8), 8), :] = v
        return _Hold(store)

    def tied(load, vregs, point):
        parts = []
        for r in range(vregs):
            anchors = [a for _ in range(GRAIN) for a in point()] if r % GRAIN == 0 else []
            u = load(8 * r)
            for a in anchors:
                u = jnp.where(never, pltpu.bitcast(a(), U32), u)
            parts.append(u)
        return jnp.concatenate(parts, 0)

    def mat(i):
        return _bf(mats[i])

    def d_stage(t, which):
        UB, AB, PB, ubu, abu = temps[t]

        def emit(point):
            z = opaque()
            for c in range(8):
                lhs = mat(which(c) + opaque()) if c % 4 else _bf(
                    tied(lambda r, u=which(c) + opaque(): mats[u, pl.ds(r, 8), :], 8, point))
                PB[0, pl.ds(128 * c, 128), :] = _dot(lhs, _bf(ubu[z, pl.ds(64 * c, 64), :]))
        return _Mat(emit)

    def lane_vec(i, rows):
        return jnp.broadcast_to(lanes[pl.ds(i, 1), :], (rows, 128))

    def x_copy(c):
        return pltpu.make_async_copy(
            x_hbm.at[:, pl.ds(pl.multiple_of(128 * c, 128), 128)], XR.at[c], sems.at[c])

    def out_copy(c):
        return pltpu.make_async_copy(
            XR.at[c], out_hbm.at[:, pl.ds(pl.multiple_of(128 * c, 128), 128)], sems.at[8 + c])

    spec_copies = [[pltpu.make_async_copy(w.at[pl.ds(0, 512), pl.ds(128 * k2, 128)], WRI.at[u, k2],
                                          sems.at[16 + u]) for k2 in range(16)]
                   + [pltpu.make_async_copy(w.at[pl.ds(512, 1), :], WN.at[u], sems.at[22 + u])]
                   for u, w in enumerate((wr_hbm, wi_hbm))]

    def start_all(copies):
        for c in copies:
            c.start()
    w_copies = [pltpu.make_async_copy(wqkv_hbm.at[:, pl.ds(D * w, D)], WRAW.at[w], sems.at[18 + w])
                for w in range(3)]
    wo_copies = [pltpu.make_async_copy(wo_hbm.at[:, pl.ds(128 * c, 128)], WO.at[c], sems.at[21])
                 for c in range(8)]

    def ln_rstd(g, i, mean):
        acc, m = None, g + opaque()
        for r in range(8):
            d = X[i][m, pl.ds(128 * r, 128), :].reshape(16, 8, 128) - mean[None]
            v = (d * d).sum(0)
            acc = v if acc is None else acc + v
            if r < 7:
                yield _Step(50, [lambda acc=acc: acc], delay=3)
        rstd = jax.lax.rsqrt(_all_sublanes(acc, jnp.add, 0) * (1.0 / D) + EPS)
        yield _Step(50, delay=8)
        yield _Step(10, [lambda: rstd], delay=1)
        return rstd

    def fwd_block(g, i, name, needs, free=(), known=False):
        j, t = g + 4 * i, i
        UB, AB, PB, ubu, abu = temps[t]
        yield _Wait(*needs)
        if known:
            means, squares = STAT[4 * g + i, pl.ds(0, 8)], STAT[4 * g + i, pl.ds(8, 8)]
            mean = means.sum(0) * 0.125
            var = (squares.sum(0) + 128.0 * ((means - mean) ** 2).sum(0)) * (1.0 / D)
            rstd = jax.lax.rsqrt(var + EPS)
            yield _Step(50, delay=6)
        else:
            yield settle(X[i])
            acc, m = None, g + opaque()
            for r in range(8):
                v = X[i][m, pl.ds(128 * r, 128), :].reshape(16, 8, 128).sum(0)
                acc = v if acc is None else acc + v
                if r % 2:
                    yield _Step(35, [lambda acc=acc: acc], delay=7 if r == 7 else 3)
            mean = _all_sublanes(acc, jnp.add, 0) * (1.0 / D)
            rstd = yield from ln_rstd(g, i, mean)
        mean8, rstd = (jnp.concatenate([v, v], 0) for v in (mean * 8.0, rstd))
        z = opaque()
        for r in range(8):
            rows = pl.ds(16 * r, 16)
            x = [X[i][g + z, pl.ds(128 * b + 16 * r, 16), :] for b in range(8)]
            s = [x[b] + x[b + 4] for b in range(4)]
            d = [x[b] - x[b + 4] for b in range(4)]
            e, o = s[0] + s[2], s[1] + s[3]
            UB[0, rows, :] = ((e + o - mean8) * rstd).astype(BF16)
            UB[0, pl.ds(128 + 16 * r, 16), :] = ((e - o) * rstd).astype(BF16)
            t1, t2 = (d[1] - d[3]) * RSQ2, (d[1] + d[3]) * RSQ2
            u = {1: (d[0] + t1, d[2] + t2), 2: (s[0] - s[2], s[1] - s[3]), 3: (d[0] - t1, d[2] - t2)}
            yield _Step(34, [anchor(ubu)], delay=1)
            for k in (1, 2, 3):
                c, sn = twid[z + 2 * k - 2, rows, :] * rstd, twid[z + 2 * k - 1, rows, :] * rstd
                re, m = u[k]
                if k == 3:
                    ur, ui = re * c + m * sn, m * c - re * sn
                else:
                    ur, ui = re * c - m * sn, m * c + re * sn
                UB[0, pl.ds(256 * k + 16 * r, 16), :] = ur.astype(BF16)
                UB[0, pl.ds(256 * k + 128 + 16 * r, 16), :] = ui.astype(BF16)
                yield _Step(26, [anchor(ubu)], delay=1)
        yield settle(ubu)

        def d_forward(point):
            z = opaque()
            first = _iota(8, 0) == 0

            def stage(c):
                u = (M_C4 if c == 1 else M_R) + opaque()
                lhs = mat(u) if c % 4 else _bf(tied(lambda r: mats[u, pl.ds(r, 8), :], 8, point))
                v = _dot(lhs, _bf(ubu[z, pl.ds(64 * c, 64), :]))
                return [(v[32 * u:32 * u + 16], v[32 * u + 16:32 * u + 32]) for u in range(4)]

            def put(row, u, v, v0=None):
                if u == 0 and v0 is not None:
                    v = jnp.concatenate([jnp.where(first, v0, v[:8]), v[8:]], 0)
                AB[0, pl.ds(row + 16 * u, 16), :] = v.astype(BF16)

            for u, (p1, p2) in enumerate(stage(0)):
                put(0, u, p1)
                put(528, u, p2, 0.0)
                if u == 0:
                    put(512, 0, jnp.zeros_like(p2), p2[:8])
            for u, (p1, p2) in enumerate(stage(1)):
                put(256, u, p1)
                put(528 + 256, u, p2)
            for k in (1, 2, 3):
                for u, ((p1, p2), (q1, q2)) in enumerate(zip(stage(2 * k), stage(2 * k + 1))):
                    if k == 3:
                        pr, pi, mr, mi = p1 - q2, p2 + q1, p1 + q2, p2 - q1
                        pi0, mi0 = q1[:8], -q2[:8]
                    else:
                        pr, pi, mr, mi = p1 + q2, p2 - q1, p1 - q2, p2 + q1
                        pi0, mi0 = -q1[:8], q2[:8]
                    put(64 * k, u, pr, p1[:8])
                    put(64 * (8 - k), u, mr, p2[:8])
                    put(528 + 64 * k, u, pi, pi0)
                    put(528 + 64 * (8 - k), u, mi, mi0)
            return 190

        yield _Mat(d_forward)
        yield settle(abu)
        yield _Wait(*free)

        def s_forward(point):
            z = opaque()
            fa, fb = mat(M_FA + j + z), mat(M_FB + j + z)
            for r0, rn in ((0, 256), (256, 272)):
                lhs = abu[z, pl.ds(r0 // 2, rn // 2), :] if r0 else tied(
                    lambda r: abu[z, pl.ds(r, 8), :], 16, point)
                u = _dot(_bf(lhs), fa)
                v = _dot(_bf(abu[z, pl.ds(264 + r0 // 2, 128), :]), fb)
                re, m = u[:256] + v, u[:256] - v
                if r0:
                    re, m = (jnp.concatenate([a, u[256:264]], 0) for a in (re, m))
                rn = re.shape[0]
                edge = (_iota(rn, 1) & 63) == 0
                ZT[2 * i, pl.ds(r0, rn), :] = re
                ZT[2 * i + 1, pl.ds(r0, rn), :] = jnp.where(
                    edge, lane_vec(L_MU + j, rn) * m + lane_vec(L_NU + j, rn) * re, pltpu.roll(m, 64, 1))
            return 400

        yield _Mat(s_forward)
        yield _Step(2, [anchor(ZT)], delay=SETTLE, marks=[name])

    def group_stage(g, name, needs, inverse):
        yield _Wait(*needs)

        def turn(z, k):
            if k == 0:
                return z
            c, s = rot[4 * g + k], rot[16 + 4 * g + k]
            if inverse:
                return z[0] * c - z[1] * s, z[1] * c + z[0] * s
            return z[0] * c + z[1] * s, z[1] * c - z[0] * s

        (src, a), (dst, b) = ((Z, 8 * g), (ZT, 0)) if inverse else ((ZT, opaque()), (Z, 8 * g))
        for r in range(65):
            if r % 4 == 0:
                yield hold(src, 2 * NB if inverse else 8)
            rows = pl.ds(8 * r, 8)
            z = [(src[a + 2 * i, rows, :], src[a + 2 * i + 1, rows, :]) for i in range(4)]
            if inverse:
                z = _radix4([turn(z[k], k) for k in range(4)], True)
            else:
                z = [turn(v, k) for k, v in enumerate(_radix4(z, False))]
            for i in range(4):
                dst[b + 2 * i, rows, :], dst[b + 2 * i + 1, rows, :] = z[i]
            yield _Step(35, [anchor(dst)], delay=1, marks=[name] if r == 64 else [])

    def spectral(row, size):
        rows = pl.ds(row, size)
        for k0 in range(4):
            z = _radix4([(Z[8 * g + 2 * k0, rows, :], Z[8 * g + 2 * k0 + 1, rows, :])
                         for g in range(4)], False)
            y = []
            for k1, (re, im) in enumerate(z):
                w = WS[k0 + 4 * k1, rows, :]
                wr = pltpu.bitcast(w << 16, F32)
                wi = pltpu.bitcast(w & np.uint32(0xFFFF0000), F32)
                y.append((re * wr - im * wi, re * wi + im * wr))
            y = _radix4(y, True)
            for g in range(4):
                Z[8 * g + 2 * k0, rows, :], Z[8 * g + 2 * k0 + 1, rows, :] = y[g]

    def spectral_rows(c2):
        for r in range(8):
            spectral(pl.multiple_of(128 * c2 + 16 * r, 16), 16)

    def inv_block(g, i, name, needs, n=None):
        j, t = g + 4 * i, i % 2
        UB, AB, PB, ubu, abu = temps[t]
        n = g if n is None else n
        z = opaque()
        yield _Wait(*needs)
        for r0, rn in _S_ROWS:
            if r0 == 0:
                yield hold(ZT, 8)
            re, im = ZT[z + 2 * i, pl.ds(r0, rn), :], ZT[z + 2 * i + 1, pl.ds(r0, rn), :]
            edge = (_iota(rn, 1) & 63) == 0
            rolled = pltpu.roll(im, 64, 1)
            u = re + jnp.where(edge, lane_vec(L_KU + j, rn) * im, rolled)
            if r0 < 512:
                v = re - jnp.where(edge, lane_vec(L_KV + j, rn) * im, rolled)
                AB[0, pl.ds(r0, rn), :] = u.astype(BF16)
                AB[0, pl.ds(528 + r0, rn), :] = v.astype(BF16)
            else:
                AB[0, pl.ds(512, 16), :] = jnp.concatenate([u, jnp.zeros_like(u)], 0).astype(BF16)
            yield _Step(rn, [anchor(abu)], delay=1, marks=[("read", name)] if r0 == 512 else [])
        yield settle(abu)

        def s_inverse(point):
            z = opaque()
            fa, fb = mat(M_FA + j + z), mat(M_FB + j + z)
            first = _iota(8, 0) == 0

            def put(row, v, v0=None):
                if v0 is not None:
                    v = jnp.concatenate([jnp.where(first, v0, v[:8]), v[8:]], 0)
                UB[0, pl.ds(row, 64), :] = v.astype(BF16)

            for k in range(4):
                lo, hi = 32 * k, 32 * (8 - k if k else 4)
                a = [abu[z, pl.ds(lo, 32), :], abu[z, pl.ds(hi, 32), :]] if k % 2 else [
                    tied(lambda r, o=o: abu[z, pl.ds(o + r, 8), :], 4, point) for o in (lo, hi)]
                if k == 0:
                    a.append(abu[z, pl.ds(256, 8), :])
                re = _dot_t(_bf(jnp.concatenate(a, 0)), fa)
                im = _dot_t(_bf(jnp.concatenate(
                    [abu[z, pl.ds(264 + lo, 32), :], abu[z, pl.ds(264 + hi, 32), :]], 0)), fb)
                pr, mr, pi, mi = re[:64], re[64:128], im[:64], im[64:]
                if k == 0:
                    put(0, pr)
                    put(64, pi, re[128:136])
                    put(128, mr)
                    put(192, mi)
                else:
                    put(256 * k, pr + mr, pr[:8])
                    put(256 * k + 64, pi + mi, mr[:8])
                    put(256 * k + 128, pi - mi, pi[:8])
                    put(256 * k + 192, mr - pr, -mi[:8])
            return 190

        yield _Mat(s_inverse)
        yield settle(ubu)
        yield d_stage(t, lambda c: {0: M_R0T, 1: M_C4T}.get(c, M_RT))
        yield settle(PB)
        z = opaque()
        acc = None
        for r in range(16):
            rows = pl.ds(8 * r, 8)
            t0, t4 = PB[z, rows, :], PB[z, pl.ds(128 + 8 * r, 8), :]
            tk = {}
            for k in (1, 2, 3):
                c, sn = twid[z + 2 * k - 2, rows, :], twid[z + 2 * k - 1, rows, :]
                re = PB[z, pl.ds(256 * k + 8 * r, 8), :]
                im = PB[z, pl.ds(256 * k + 128 + 8 * r, 8), :]
                tk[k] = (re * c - im * sn, re * sn + im * c)
            e0, e1 = t0 + t4, t0 - t4
            s = [e0 + tk[2][0], e1 - tk[2][1], e0 - tk[2][0], e1 + tk[2][1]]
            al, be = tk[1][0] - tk[3][0], tk[1][1] + tk[3][1]
            o = [tk[1][0] + tk[3][0], (al - be) * RSQ2, tk[3][1] - tk[1][1], (al + be) * -RSQ2]
            for b in range(8):
                y = s[b] + o[b] if b < 4 else s[b - 4] - o[b - 4]
                v = X[i][g, pl.ds(128 * b + 8 * r, 8), :] + y
                X[i][n, pl.ds(128 * b + 8 * r, 8), :] = v
                acc = v if acc is None else acc + v
            yield _Step(57, [lambda v=acc: v], delay=5 if r == 15 else 2)
        yield settle(X[i])
        mean = _all_sublanes(acc, jnp.add, 0) * (1.0 / D)
        rstd = yield from ln_rstd(n, i, mean)
        z = opaque()
        for r in range(8):
            v = X[i][n + z, pl.ds(128 * r, 128), :].reshape(16, 8, 128)
            HB[i][n, pl.ds(128 * r, 128), :] = ((v - mean[None]) * rstd[None]).reshape(128, 128).astype(BF16)
            yield _Step(41, [anchor(hbu[i])], delay=1, marks=[name] if r == 7 else [])

    def attend(g, i, name, needs):
        yield _Wait(*needs)
        yield settle(QB[i])
        j, z = g + 4 * i, opaque()
        even = (_iota(8, 0) & 1) == 0
        edge = _iota(8, 1) == 0

        def window(near, far, w, rows):
            return near[j + z + 4 - 2 * w, rows, :] if w <= 2 * i + 2 else far[j + z + 16 - 2 * w, rows, :]

        def mix_values(h, u):
            p = PW[h % 2][opaque()]
            for rows in (pl.ds(256 * h + 16 * u, 16), pl.ds(256 * h + 16 * u + 16, 16)):
                acc = functools.reduce(jnp.add, [p[16 * w:16 * w + 16] * window(VE, VS, w, rows)
                                                 for w in range(8)])
                HB[i][g, rows, :] = acc.astype(BF16)
            return _Step(63, [anchor(hbu[i])], delay=1, marks=[name] if (h, u) == (3, 14) else [])

        for h in range(5):
            logits = []
            for w0 in range(0, 8, 2):
                if h < 4:
                    rows = pl.ds(256 * h, 256)
                    q = QB[i][opaque(), rows, :]
                    for w in (w0, w0 + 1):
                        v = (q * window(KE, KS, w, rows)).reshape(16, 16, 128).sum(0)
                        v = jnp.where(even, v[:8], v[8:]) + pltpu.roll(jnp.where(even, v[8:], v[:8]), 7, 0)
                        logits.append(jnp.where(edge & (2 * w > j), -1e9, v * SCALE) if w > 2 * i
                                      else v * SCALE)
                    yield _Step(138, [lambda v=v: v for v in logits[-2:]], delay=2)
                if h > 0:
                    yield mix_values(h - 1, 2 * w0)
                    yield mix_values(h - 1, 2 * w0 + 2)
            if h < 4:
                top = functools.reduce(jnp.maximum, logits)
                e = [jnp.exp(v - top) for v in logits]
                total = functools.reduce(jnp.add, e)
                yield _Step(30, [lambda v=total: v], delay=3)
                scale = 1.0 / total
                for w in range(8):
                    v = e[w] * scale
                    PW[h % 2][0, pl.ds(16 * w, 8), :] = jnp.where(even, v, pltpu.roll(v, 1, 0))
                    PW[h % 2][0, pl.ds(16 * w + 8, 8), :] = jnp.where(even, pltpu.roll(v, 7, 0), v)
                yield _Step(50, [anchor(PW[h % 2])], delay=6 if h == 3 else 1)

    def proj(sch, w, g, i, m, store, needs, marks, own=120):
        for name in needs:
            sch.run(name)
        row, w = pl.multiple_of(64 * m, 64), w + opaque()
        parts = []
        sch.fresh = True
        for col in (0, 512):
            parts.append(tied(lambda r: WT[w, pl.ds(row + r, 8), pl.ds(col, 128)], 8,
                              lambda: sch.point(own / 16)))
            parts.append(WT[w, pl.ds(row, 64), pl.ds(col + 128, 384)])
        v = _dot(_bf(jnp.concatenate(parts, 1)), _bf(hbu[i][g + opaque()]))
        store(v, pl.ds(pl.multiple_of(128 * m, 128), 128))
        sch.results.append(v[:8])
        for name in marks:
            sch.done[name] = sch.slot + WAIT

    def kv_proj(sch, g, i, needs):
        for w, ref in ((1, KE), (2, VE)):
            def store(v, rows):
                ref[g + 4 * i + 4, rows, :] = v
            for m in range(8):
                proj(sch, w, g, i, m, store, needs, [("kv", i)] if (w, m) == (2, 7) else [])

    def shift_block(g, i, name, needs):
        yield _Wait(*needs)
        j, z = g + 4 * i, opaque()
        for m in range(16):
            rows = pl.ds(64 * m, 64)
            for ref, to in ((KE, KS), (VE, VS)):
                v = pltpu.roll(ref[j + 4 + z, rows, :], 1, 1)
                if ref is VE:
                    v = jnp.where(_iota(64, 1) == 0, ref[4 + z, rows, :], v)
                to[j, rows, :] = v
                if i == 3:
                    ref[g, rows, :] = v
            yield _Step(12, delay=8 if i == 3 else 4, marks=[name] if m == 15 else [])

    def q_proj(sch, g, i, name):
        def store(v, rows):
            QB[i][0, rows, :] = v
        for m in range(8):
            proj(sch, 0, g, i, m, store, [], [name] if m == 7 else [])

    def o_proj(sch, g, i, m, needs, marks):
        def store(v, rows):
            X[i][g, rows, :] = X[i][g, rows, :] + v
        proj(sch, 3, g, i, m, store, needs, marks, own=135)

    def transpose_weight(src, dst, name):
        for r in range(4):
            for h in range(4):
                v = pltpu.bitcast(WRAW[src, pl.ds(256 * r, 256), pl.ds(256 * h, 256)].T, U32)
                TR[h % 2, 0], TR[h % 2, 1] = v[:, :128], v[:, 128:]
                yield _Step(40, delay=20)
                z = h % 2 + opaque()
                for e in range(2):
                    WT[dst, pl.ds(128 * h, 128), pl.ds(256 * r + 128 * e, 128)] = jnp.concatenate(
                        [TR[z, e, pl.ds(u, 8, stride=16), :] for u in range(16)], 0)
                yield _Step(40, marks=[name] if r == 3 and h == 3 else [])

    def transpose_wo(name):
        for c in range(8):
            for h in range(4):
                v = jnp.concatenate([wou[c, pl.ds(128 * h + u, 8, stride=16), :] for u in range(16)], 0)
                WT[3, pl.ds(64 * c, 64), pl.ds(256 * h, 256)] = pltpu.bitcast(_bf(v).T, U32)
                yield _Step(20, delay=10, marks=[name] if c == 7 and h == 3 else [])

    def prep_spectral_weights(c2):
        lane = _iota(8, 1)
        order = jnp.where(lane > 64, 192 - lane, lane)

        def words(k2):
            re, im = (wsu[u, k2, pl.ds(c2, 64, stride=4), :] for u in range(2))
            return ((re & np.uint32(0xFFFF)) | (im << 16), (re >> 16) | (im & np.uint32(0xFFFF0000)))

        def arrange(w, below):
            w = jnp.where(_iota(w.shape[0], 1) < 64, w, below)
            return jnp.concatenate([jnp.take_along_axis(w[u:u + 8], order, axis=1)
                                    for u in range(0, w.shape[0], 8)], 0)

        below = words(15)
        for k2 in range(16):
            here = words(k2)
            for e in range(2):
                cl = 2 * c2 + e
                w = arrange(here[e], below[e])
                WS[k2, pl.ds(64 * cl, 64), :] = pltpu.roll(w, 1, 0) if cl > 4 else w
            below = here
            yield _Step(100)
        if c2 == 0:
            def nyquist(k2):
                re, im = (jnp.broadcast_to(WN[u, :, pl.ds(128 * k2, 128)].astype(F32), (8, 128))
                          for u in range(2))
                return pltpu.pack_elementwise([re, im], packed_dtype=BF16)
            for k2 in range(16):
                WS[k2, pl.ds(512, 8), :] = arrange(nyquist(k2), nyquist((k2 + 15) % 16))

    def write_out(p, c, name, needs):
        yield _Wait(*needs)
        rows = pl.ds(pl.multiple_of(128 * c, 128), 128)
        g, i = 2 * p % 4 + opaque(), p // 2
        w = pltpu.pack_elementwise([X[i][g, rows, :], X[i][g + 1, rows, :]], packed_dtype=BF16)
        xru[c, pl.ds(p, 128, stride=8), :] = w.T
        yield _Step(30, marks=[name])

    for c in range(8):
        x_copy(c).start()
    for c in range(5):
        mats[M_R + c] = d_mats[c]

    def make_twiddle(k):
        PB = temps[0][2]
        PB[0, pl.ds(0, 128), :] = lane_vec(L_TWID + k, 128)
        twid[k] = PB[opaque(), pl.ds(0, 128), :].T

    _loop(6, make_twiddle, "make_twiddle")

    def make_dft(j):
        fa, fb = lanes[pl.ds(L_FA, 128), :], lanes[pl.ds(L_FB, 128), :]
        c, sn = lane_vec(L_COS + j, 128), lane_vec(L_SIN + j, 128)
        UB, _, _, ubu, _ = temps[0]
        UB[0, pl.ds(0, 128), :] = (fa * c + fb * sn).astype(BF16)
        UB[0, pl.ds(128, 128), :] = (fb * c - fa * sn).astype(BF16)
        mats[M_FA + j], mats[M_FB + j] = ubu[0, pl.ds(0, 64), :], ubu[0, pl.ds(64, 64), :]

    _loop(NB, make_dft, "make_dft")

    def load_x(c):
        x_copy(c).wait()
        pl.when(c == 5)(lambda: start_all(spec_copies[0]))
        pl.when(c == 7)(lambda: start_all(spec_copies[1]))
        rows = pl.ds(pl.multiple_of(128 * c, 128), 128)
        for p in range(8):
            w = xru[c, pl.ds(p, 128, stride=8), :].T
            for e, bits in enumerate((w << 16, w & np.uint32(0xFFFF0000))):
                g, i = 2 * p % 4 + e, p // 2
                v = pltpu.bitcast(bits, F32)
                X[i][g, rows, :] = v
                v = v.reshape(16, 8, 128)
                mean = _all_sublanes(v.sum(0), jnp.add, 0) * (1.0 / 128)
                STAT[4 * g + i, c] = mean
                STAT[4 * g + i, 8 + c] = _all_sublanes(((v - mean) ** 2).sum(0), jnp.add, 0)

    _loop(8, load_x, "load_x")

    def after(name, action):
        yield _Wait(name)
        action()

    def spectral_weights():
        yield _Wait(("f", 2, 1))
        for c in spec_copies[0] + spec_copies[1]:
            c.wait()
        for c2 in range(4):
            yield from prep_spectral_weights(c2)

    with jax.named_scope("first_forward"):
        sch = _Sched(0.92)
        sch.add(after(("f", 0, 1), w_copies[1].start), "k")
        sch.add(after(("f", 1, 3), w_copies[2].start), "v")
        for g in range(4):
            for i in range(4):
                sch.add(fwd_block(g, i, ("f", g, i), [("f", g - 1, i)] if g else [],
                                  [("r", g - 1)] if g else [], True), ("f", g, i))
            sch.add(group_stage(g, ("r", g), [("f", g, i) for i in range(4)], False), ("r", g))
        sch.add(spectral_weights(), "s")
        sch.drive()
    w_copies[0].start()
    start_all(wo_copies)

    def keys_values(layer, g):
        sch = _Sched(0.36 if layer == 0 else 0.33)
        if layer == 0:
            pl.when(g == 1)(w_copies[0].wait)
        sch.done[("i", 0)] = 0
        for i in range(1, 3):
            sch.add(inv_block(g, i, ("i", i), [("read", ("i", 1))] if i == 2 else []), ("i", i))
        nxt = (g + 1) % 4
        sch.add(inv_block(g, 3, ("i", 3), [("i", 1)]), ("i", 3))
        sch.add(group_stage(nxt, "r", [("read", ("i", i)) for i in (1, 2, 3)], True), "r")
        sch.add(inv_block(nxt, 0, ("i", 4), ["r", ("i", 2)], n=g + 1), ("i", 4))
        if layer == 0:
            sch.add(transpose_weight(jnp.where(g == 0, 1, 0), 0, "w"), "w")
        sch.add(shift_block((g + 3) % 4, 3, ("s", 0), []), ("s", 0))
        for i in range(1, 4):
            sch.add(shift_block(g, i - 1, ("s", i), [("kv", i - 1)]), ("s", i))
        for i in range(4):
            kv_proj(sch, g, i, [("i", i)])
        sch.finish()

    def mix(g, after, last, write):
        sch = _Sched(0.67 if last else 0.63)
        now = 8 - DEFER if last else 8
        tail = after is None

        def block(i):
            return (g, i) if i < 4 else (after, i - 4)

        sch.done[("a", 0)] = 0
        for i in range(3 if tail else 4):
            sch.add(attend(*block(i + 1), ("a", i + 1), [("q", i + 1), ("a", i)] if i else []),
                    ("a", i + 1), pace=0.30 if last or tail else 0.26)
        if not last:
            sch.add(group_stage((g + 3) % 4, "r", [], False), "r")
            for i in range(4):
                sch.add(fwd_block(g, i, ("f", i), [("o", i, 7)], ["r"]), ("f", i))
        for i in range(4 if write else 0):
            for c in range(now):
                sch.add(write_out(2 * i + g // 2, c, ("w", i, c), [("o", i, c)]), ("w", i, c))
        if tail:
            q_proj(sch, g, 2, ("q", 2))
            q_proj(sch, g, 3, ("q", 3))
        for i in range(4):
            for m in range(now):
                o_proj(sch, g, i, m, [("a", i)], [("o", i, m)])
            if not tail:
                q_proj(sch, *block(i + 2), ("q", i + 2))
        if tail and not last:
            sch.add(group_stage(g, "s", [("f", i) for i in range(4)], False), "s")
        sch.finish()

    def postponed(u):
        c = 8 - DEFER + u
        sch = _Sched(0.5)
        for p in range(8):
            sch.add(write_out(p, c, ("w", p), [("o", p)]), ("w", p))
            o_proj(sch, 2 * p % 4, p // 2, c, [], [])
            o_proj(sch, 2 * p % 4 + 1, p // 2, c, [], [("o", p)])
        sch.finish()
        out_copy(c).start()

    def spectral_and_weights(u):
        spectral_rows(2 * u)
        pl.when(u == 0)(w_copies[1].wait)
        pl.when(u == 1)(w_copies[2].wait)
        for _ in transpose_weight(1 + u, 1 + u, None):
            pass
        spectral_rows(2 * u + 1)

    for layer in range(2):
        with jax.named_scope("spectral"):
            if layer == 0:
                _loop(2, spectral_and_weights, "rows")
            else:
                _loop(4, spectral_rows, "rows")
            spectral(512, 8)
        sch = _Sched()
        sch.add(group_stage(0, "r", [], True), "r")
        sch.add(inv_block(0, 0, "i", ["r"]), "i")
        sch.finish()
        _loop(4, lambda g: keys_values(layer, g), "keys_values")
        sch = _Sched(0.66)
        sch.add(attend(0, 0, "a", ["q"]), "a")
        sch.add(shift_block(3, 3, "s", []), "s")
        if layer == 0:
            for c in wo_copies:
                c.wait()
            sch.add(transpose_wo("w"), "w")
        q_proj(sch, 0, 0, "q")
        q_proj(sch, 0, 1, None)
        sch.finish()
        if layer == 0:
            _loop(3, lambda g: mix(g, g + 1, False, False), "mix")
            mix(3, None, False, False)
        else:
            _loop(2, lambda u: mix(2 * u, 2 - u, True, False), "mix")
            mix(1, 3, True, True)
            mix(3, None, True, True)
    for c in range(8 - DEFER):
        out_copy(c).start()
    _loop(DEFER, postponed, "postponed")
    for c in range(8):
        out_copy(c).wait()


@jax.jit
def pallas_interleave_layers__spectral_gfnet__sliding_local_dilated__prompt_kernel(
    A_x: jax.Array,
    A_w_r: jax.Array,
    A_w_i: jax.Array,
    B_x: jax.Array,
    B_wqkv: jax.Array,
    B_wo: jax.Array,
):
    del B_x
    hbm = pl.BlockSpec(memory_space=pl.ANY)
    smem = pl.BlockSpec(memory_space=pltpu.SMEM)
    out = pl.pallas_call(
        _kernel,
        out_shape=jax.ShapeDtypeStruct((S, D), BF16),
        in_specs=[smem, smem, pl.BlockSpec(), pl.BlockSpec(), hbm, hbm, hbm, hbm, hbm],
        out_specs=hbm,
        scratch_shapes=[
            pltpu.VMEM((37, 64, 128), U32),
            pltpu.VMEM((6, 128, 128), F32),
            pltpu.VMEM((NB, 16, 8, 128), F32),
            pltpu.VMEM((NB + 4, D, 128), F32),
            pltpu.VMEM((NB + 4, D, 128), F32),
            pltpu.VMEM((NB, D, 128), F32),
            pltpu.VMEM((NB, D, 128), F32),
            pltpu.VMEM((2 * NB + 1, ZR, 128), F32),
            pltpu.VMEM((9, ZR, 128), F32),
            pltpu.VMEM((NB, ZR, 128), U32),
            pltpu.VMEM((4, D // 2, D), U32),
            pltpu.VMEM((8, S, 128), BF16),
            pltpu.VMEM((2, NB, D // 2, 128), BF16),
            pltpu.VMEM((2, 1, S), BF16),
            pltpu.VMEM((3, D, D), BF16),
            pltpu.VMEM((8, D, 128), BF16),
            pltpu.VMEM((2, 2, 128, 128), U32),
            pltpu.VMEM((1, 128, 128), F32),
            pltpu.VMEM((1, 128, 128), F32),
            pltpu.SemaphoreType.DMA((24,)),
        ] + 4 * [
            pltpu.VMEM((5, D, 128), F32),
            pltpu.VMEM((5, D, 128), BF16),
            pltpu.VMEM((1, D, 128), F32),
            pltpu.VMEM((1, D, 128), BF16),
            pltpu.VMEM((1, 1040, 128), BF16),
            pltpu.VMEM((1, 1040, 128), F32),
        ],
        compiler_params=pltpu.CompilerParams(vmem_limit_bytes=124 * 2 ** 20),
    )(_ZERO, _ROT, _MATS, _LANES, A_x.reshape(S, D), A_w_r.T, A_w_i.T, B_wqkv, B_wo)
    return out.reshape(1, S, D)
```

```python
import functools

import numpy as np

import jax
import jax.numpy as jnp
import jax.experimental.pallas as pl
import jax.experimental.pallas.tpu as pltpu

S, D, NB = 2048, 1024, 16
ZR = 576
F32, BF16, U32, I32 = jnp.float32, jnp.bfloat16, jnp.uint32, jnp.int32
EPS = 1e-5
SCALE = 32 ** -0.5
RSQ2 = float(np.sqrt(0.5))
WAIT = 16
GRAIN = 1
SETTLE = 3
LAG = 3
DEFER = 2

_S_ROWS = [(32 * u, 32) for u in range(16)] + [(512, 8)]

M_FA, M_FB, M_R, M_C4, M_RT, M_C4T, M_R0T = 0, 16, 32, 33, 34, 35, 36
L_MU, L_NU, L_KU, L_KV, L_COS, L_SIN, L_TWID, L_FA, L_FB = 0, 16, 32, 48, 64, 80, 96, 104, 232


def _bf16_bits(a):
    u = np.ascontiguousarray(a, dtype=np.float32).view(np.uint32).astype(np.uint64)
    return ((u + 0x7FFF + ((u >> 16) & 1)) >> 16).astype(np.uint32)


def _constants():
    a = np.arange(128)
    k1 = np.arange(64)
    alt = (-1.0) ** a
    lanes = np.zeros((L_FB + 128, 128))
    t = 2 * np.pi * np.outer(a, k1) / 128
    fa = np.concatenate([np.cos(t), -np.sin(t)], 1)
    fb = np.concatenate([np.sin(t), -np.cos(t)], 1)
    fa[:, 0], fb[:, 0] = RSQ2, -RSQ2
    fa[:, 64], fb[:, 64] = alt, 0.0
    lanes[L_FA:L_FA + 128], lanes[L_FB:L_FB + 128] = fa, fb
    for j in range(NB):
        ang = 2 * np.pi * j / 32 + np.pi / 32
        p, q = (_bf16_bits([np.cos(ang), np.sin(ang)]) << 16).view(np.float32).astype(np.float64)
        turn = 2 * np.pi * j * np.tile(k1, 2) / S
        lanes[L_COS + j], lanes[L_SIN + j] = np.cos(turn), np.repeat([-1.0, 1.0], 64) * np.sin(turn)
        lanes[L_COS + j, 64], lanes[L_SIN + j, 64] = p, q
        lanes[L_MU + j, 0], lanes[L_MU + j, 64] = 1.0, (q / p + p / q) / 2
        lanes[L_NU + j, 0], lanes[L_NU + j, 64] = 0.0, (q / p - p / q) / 2
        lanes[L_KU + j, 0], lanes[L_KU + j, 64] = 1.0, q / p
        lanes[L_KV + j, 0], lanes[L_KV + j, 64] = 1.0, p / q
    for k in (1, 2, 3):
        lanes[L_TWID + 2 * k - 2] = np.cos(2 * np.pi * a * k / D)
        lanes[L_TWID + 2 * k - 1] = np.sin(2 * np.pi * a * k / D)
    th = 2 * np.pi * np.outer(k1, a) / 128
    r = np.concatenate([np.cos(th), -np.sin(th)], 0)
    r[64] = alt
    th = 2 * np.pi * np.outer(2 * k1 + 1, a) / 256
    c4 = np.concatenate([np.cos(th), -np.sin(th)], 0)
    inv = 2.0 / (S * D)
    r0t = inv * r.T
    r0t[:, 0::64] *= 0.5
    rows = np.arange(128).reshape(2, 4, 16).transpose(1, 0, 2).ravel()
    bits = _bf16_bits(np.stack([r[rows], c4[rows], inv * r.T, inv * c4.T, r0t]))
    ang = 2 * np.pi * np.outer(np.arange(4), np.arange(4)).ravel() / 16
    rot = np.concatenate([np.cos(ang), np.sin(ang)]).astype(np.float32)
    return bits[:, 0::2] | (bits[:, 1::2] << 16), lanes.astype(np.float32), rot


_MATS, _LANES, _ROT = _constants()
_ZERO = np.zeros((1,), np.int32)


class _Step:
    def __init__(self, cost, anchors=(), delay=0, marks=()):
        self.cost, self.anchors, self.delay, self.marks = cost, list(anchors), delay, list(marks)


class _Wait:
    def __init__(self, *names):
        self.names = names


class _Mat:
    def __init__(self, emit):
        self.emit = emit


class _Hold:
    def __init__(self, store):
        self.store = store


class _Task:
    def __init__(self, gen, pace):
        self.gen, self.pace, self.blocked, self.not_before, self.held = gen, pace, (), 0, None
        self.allowed = 0.0


class _Sched:
    def __init__(self, share=0.0):
        self.share = share
        self.tasks, self.done, self.producer = [], {}, {}
        self.slot, self.credit, self.anchors, self.results = 0, 0.0, [], []
        self.fresh = False

    def add(self, gen, name, pace=99):
        self.producer[name] = self.producer["read", name] = _Task(gen, pace)
        self.tasks.append(self.producer[name])

    def _ready(self, t):
        return t.not_before <= self.slot and all(
            n in self.done and self.done[n] <= self.slot for n in t.blocked)

    def _advance(self, t, mats=True):
        item, t.held = t.held or next(t.gen, None), None
        if item is None:
            self.tasks.remove(t)
        elif isinstance(item, _Wait):
            t.blocked = item.names
        elif isinstance(item, _Hold):
            if len(self.results) >= LAG:
                item.store(self.results[-LAG])
        elif isinstance(item, _Mat):
            if mats:
                t.not_before = float("inf")
                self.fresh = False
                self.credit -= item.emit(lambda: self.point(0.0)) or 0
                t.not_before = self.slot + WAIT
            else:
                t.held, t.not_before = item, self.slot + 1
        else:
            t.blocked = ()
            t.not_before = self.slot + item.delay
            self.credit -= item.cost
            self.anchors += item.anchors
            for n in item.marks:
                self.done[n] = self.slot + item.delay
            return True

    def run(self, *names):
        while not all(n in self.done for n in names):
            for n in names:
                if n not in self.done:
                    for b in self.producer[n].blocked:
                        self.run(b)
                    self._advance(self.producer[n])

    def drive(self):
        while self.tasks:
            ready = [t for t in self.tasks if self._ready(t)]
            if not ready:
                self.slot += 1
                continue
            self.anchors, self.credit = self.anchors[-2:], 0.0
            self._advance(next((t for t in ready if t.held), ready[0]))
            self.slot -= min(self.credit, 0.0) / 60

    def finish(self):
        self.run(*[n for n in self.producer if n[0] != "read"])

    def point(self, own):
        for t in self.tasks:
            t.allowed = min(t.allowed, 0.0) + t.pace
        while True:
            t = next((t for t in self.tasks if self._ready(t) and t.allowed > 0
                      and self.credit > 0), None)
            if t is None:
                break
            if self._advance(t, self.fresh):
                t.allowed -= 1
        anchors, self.anchors = self.anchors, []
        self.credit = min(self.credit, 10.0) + 64 * self.share - own
        self.fresh = False
        self.slot += 1
        return anchors


def _dot(a, b):
    return jnp.dot(a, b, preferred_element_type=F32)


def _dot_t(a, b):
    return jax.lax.dot_general(a, b, (((1,), (1,)), ((), ())), preferred_element_type=F32)


def _bf(u):
    return pltpu.bitcast(u, BF16)


def _iota(rows, dim):
    return jax.lax.broadcasted_iota(I32, (rows, 128), dim)


def _radix4(z, inverse):
    (r0, i0), (r1, i1), (r2, i2), (r3, i3) = z
    ar, ai, cr, ci = r0 + r2, i0 + i2, r0 - r2, i0 - i2
    br, bi, dr, di = r1 + r3, i1 + i3, r1 - r3, i1 - i3
    lo, hi = (cr + di, ci - dr), (cr - di, ci + dr)
    if inverse:
        lo, hi = hi, lo
    return [(ar + br, ai + bi), lo, (ar - br, ai - bi), hi]


def _all_sublanes(v, op, axis):
    for sh in (4, 2, 1):
        v = op(v, pltpu.roll(v, sh, axis))
    return v


def _loop(n, body, name):
    def step(i, carry):
        body(i)
        return carry
    with jax.named_scope(name):
        jax.lax.fori_loop(0, n, step, 0)


def _kernel(zero_ref, rot, d_mats, lanes, x_hbm, wr_hbm, wi_hbm, wqkv_hbm, wo_hbm, out_hbm,
            mats, twid, STAT, KE, VE, KS, VS, Z, ZT, WS, WQ, WK, WV, WP, XR, WRI, WN, WRAW, WO, TR, PW0, PW1, sems, *split):
    zero = zero_ref[0]
    never = zero != 0
    X, HB, QB = split[0::6], split[1::6], split[2::6]
    hbu = [r.bitcast(U32) for r in HB]
    xru, wsu, wou = XR.bitcast(U32), WRI.bitcast(U32), WO.bitcast(U32)
    temps = [(ub, ab, pb, ub.bitcast(U32), ab.bitcast(U32))
             for ub, ab, pb in zip(split[3::6], split[4::6], split[5::6])]
    PW, WT = (PW0, PW1), (WQ, WK, WV, WP)
    counter = [0]

    def opaque():
        counter[0] += 1
        return zero * counter[0]

    def anchor(ref):
        return lambda: ref[0, pl.ds(pl.multiple_of(zero * 8, 8), 8), pl.ds(0, 128)]

    def settle(ref):
        return _Step(2, [anchor(ref)], delay=SETTLE)

    def hold(ref, spare, row=0):
        def store(v):
            ref[spare, pl.ds(pl.multiple_of(row + zero * 8, 8), 8), :] = v
        return _Hold(store)

    def tied(load, vregs, point):
        parts = []
        for r in range(vregs):
            anchors = [a for _ in range(GRAIN) for a in point()] if r % GRAIN == 0 else []
            u = load(8 * r)
            for a in anchors:
                u = jnp.where(never, pltpu.bitcast(a(), U32), u)
            parts.append(u)
        return jnp.concatenate(parts, 0)

    def mat(i):
        return _bf(mats[i])

    def d_stage(t, which):
        UB, AB, PB, ubu, abu = temps[t]

        def emit(point):
            z = opaque()
            for c in range(8):
                lhs = mat(which(c) + opaque()) if c % 4 else _bf(
                    tied(lambda r, u=which(c) + opaque(): mats[u, pl.ds(r, 8), :], 8, point))
                PB[0, pl.ds(128 * c, 128), :] = _dot(lhs, _bf(ubu[z, pl.ds(64 * c, 64), :]))
        return _Mat(emit)

    def lane_vec(i, rows):
        return jnp.broadcast_to(lanes[pl.ds(i, 1), :], (rows, 128))

    def x_copy(c):
        return pltpu.make_async_copy(
            x_hbm.at[:, pl.ds(pl.multiple_of(128 * c, 128), 128)], XR.at[c], sems.at[c])

    def out_copy(c):
        return pltpu.make_async_copy(
            XR.at[c], out_hbm.at[:, pl.ds(pl.multiple_of(128 * c, 128), 128)], sems.at[8 + c])

    spec_copies = [[pltpu.make_async_copy(w.at[pl.ds(0, 512), pl.ds(128 * k2, 128)], WRI.at[u, k2],
                                          sems.at[16 + u]) for k2 in range(16)]
                   + [pltpu.make_async_copy(w.at[pl.ds(512, 1), :], WN.at[u], sems.at[22 + u])]
                   for u, w in enumerate((wr_hbm, wi_hbm))]

    def start_all(copies):
        for c in copies:
            c.start()
    w_copies = [pltpu.make_async_copy(wqkv_hbm.at[:, pl.ds(D * w, D)], WRAW.at[w], sems.at[18 + w])
                for w in range(3)]
    wo_copies = [pltpu.make_async_copy(wo_hbm.at[:, pl.ds(128 * c, 128)], WO.at[c], sems.at[21])
                 for c in range(8)]

    def ln_rstd(g, i, mean):
        acc, m = None, g + opaque()
        for r in range(8):
            d = X[i][m, pl.ds(128 * r, 128), :].reshape(16, 8, 128) - mean[None]
            v = (d * d).sum(0)
            acc = v if acc is None else acc + v
            if r < 7:
                yield _Step(50, [lambda acc=acc: acc], delay=3)
        rstd = jax.lax.rsqrt(_all_sublanes(acc, jnp.add, 0) * (1.0 / D) + EPS)
        yield _Step(50, delay=8)
        yield _Step(10, [lambda: rstd], delay=1)
        return rstd

    def fwd_block(g, i, name, needs, free=(), known=False):
        j, t = g + 4 * i, i
        UB, AB, PB, ubu, abu = temps[t]
        yield _Wait(*needs)
        if known:
            means, squares = STAT[4 * g + i, pl.ds(0, 8)], STAT[4 * g + i, pl.ds(8, 8)]
            mean = means.sum(0) * 0.125
            var = (squares.sum(0) + 128.0 * ((means - mean) ** 2).sum(0)) * (1.0 / D)
            rstd = jax.lax.rsqrt(var + EPS)
            yield _Step(50, delay=6)
        else:
            yield settle(X[i])
            acc, m = None, g + opaque()
            for r in range(8):
                v = X[i][m, pl.ds(128 * r, 128), :].reshape(16, 8, 128).sum(0)
                acc = v if acc is None else acc + v
                if r % 2:
                    yield _Step(35, [lambda acc=acc: acc], delay=7 if r == 7 else 3)
            mean = _all_sublanes(acc, jnp.add, 0) * (1.0 / D)
            rstd = yield from ln_rstd(g, i, mean)
        mean8, rstd = (jnp.concatenate([v, v], 0) for v in (mean * 8.0, rstd))
        z = opaque()
        for r in range(8):
            rows = pl.ds(16 * r, 16)
            x = [X[i][g + z, pl.ds(128 * b + 16 * r, 16), :] for b in range(8)]
            s = [x[b] + x[b + 4] for b in range(4)]
            d = [x[b] - x[b + 4] for b in range(4)]
            e, o = s[0] + s[2], s[1] + s[3]
            UB[0, rows, :] = ((e + o - mean8) * rstd).astype(BF16)
            UB[0, pl.ds(128 + 16 * r, 16), :] = ((e - o) * rstd).astype(BF16)
            t1, t2 = (d[1] - d[3]) * RSQ2, (d[1] + d[3]) * RSQ2
            u = {1: (d[0] + t1, d[2] + t2), 2: (s[0] - s[2], s[1] - s[3]), 3: (d[0] - t1, d[2] - t2)}
            yield _Step(34, [anchor(ubu)], delay=1)
            for k in (1, 2, 3):
                c, sn = twid[z + 2 * k - 2, rows, :] * rstd, twid[z + 2 * k - 1, rows, :] * rstd
                re, m = u[k]
                if k == 3:
                    ur, ui = re * c + m * sn, m * c - re * sn
                else:
                    ur, ui = re * c - m * sn, m * c + re * sn
                UB[0, pl.ds(256 * k + 16 * r, 16), :] = ur.astype(BF16)
                UB[0, pl.ds(256 * k + 128 + 16 * r, 16), :] = ui.astype(BF16)
                yield _Step(26, [anchor(ubu)], delay=1)
        yield settle(ubu)

        def d_forward(point):
            z = opaque()
            first = _iota(8, 0) == 0

            def stage(c):
                u = (M_C4 if c == 1 else M_R) + opaque()
                lhs = mat(u) if c % 4 else _bf(tied(lambda r: mats[u, pl.ds(r, 8), :], 8, point))
                v = _dot(lhs, _bf(ubu[z, pl.ds(64 * c, 64), :]))
                return [(v[32 * u:32 * u + 16], v[32 * u + 16:32 * u + 32]) for u in range(4)]

            def put(row, u, v, v0=None):
                if u == 0 and v0 is not None:
                    v = jnp.concatenate([jnp.where(first, v0, v[:8]), v[8:]], 0)
                AB[0, pl.ds(row + 16 * u, 16), :] = v.astype(BF16)

            for u, (p1, p2) in enumerate(stage(0)):
                put(0, u, p1)
                put(528, u, p2, 0.0)
                if u == 0:
                    put(512, 0, jnp.zeros_like(p2), p2[:8])
            for u, (p1, p2) in enumerate(stage(1)):
                put(256, u, p1)
                put(528 + 256, u, p2)
            for k in (1, 2, 3):
                for u, ((p1, p2), (q1, q2)) in enumerate(zip(stage(2 * k), stage(2 * k + 1))):
                    if k == 3:
                        pr, pi, mr, mi = p1 - q2, p2 + q1, p1 + q2, p2 - q1
                        pi0, mi0 = q1[:8], -q2[:8]
                    else:
                        pr, pi, mr, mi = p1 + q2, p2 - q1, p1 - q2, p2 + q1
                        pi0, mi0 = -q1[:8], q2[:8]
                    put(64 * k, u, pr, p1[:8])
                    put(64 * (8 - k), u, mr, p2[:8])
                    put(528 + 64 * k, u, pi, pi0)
                    put(528 + 64 * (8 - k), u, mi, mi0)
            return 190

        yield _Mat(d_forward)
        yield settle(abu)
        yield _Wait(*free)

        def s_forward(point):
            z = opaque()
            fa, fb = mat(M_FA + j + z), mat(M_FB + j + z)
            for r0, rn in ((0, 256), (256, 272)):
                lhs = abu[z, pl.ds(r0 // 2, rn // 2), :] if r0 else tied(
                    lambda r: abu[z, pl.ds(r, 8), :], 16, point)
                u = _dot(_bf(lhs), fa)
                v = _dot(_bf(abu[z, pl.ds(264 + r0 // 2, 128), :]), fb)
                re, m = u[:256] + v, u[:256] - v
                if r0:
                    re, m = (jnp.concatenate([a, u[256:264]], 0) for a in (re, m))
                rn = re.shape[0]
                edge = (_iota(rn, 1) & 63) == 0
                ZT[2 * i, pl.ds(r0, rn), :] = re
                ZT[2 * i + 1, pl.ds(r0, rn), :] = jnp.where(
                    edge, lane_vec(L_MU + j, rn) * m + lane_vec(L_NU + j, rn) * re, pltpu.roll(m, 64, 1))
            return 400

        yield _Mat(s_forward)
        yield _Step(2, [anchor(ZT)], delay=SETTLE, marks=[name])

    def group_stage(g, name, needs, inverse):
        yield _Wait(*needs)

        def turn(z, k):
            if k == 0:
                return z
            c, s = rot[4 * g + k], rot[16 + 4 * g + k]
            if inverse:
                return z[0] * c - z[1] * s, z[1] * c + z[0] * s
            return z[0] * c + z[1] * s, z[1] * c - z[0] * s

        (src, a), (dst, b) = ((Z, 8 * g), (ZT, 0)) if inverse else ((ZT, opaque()), (Z, 8 * g))
        for r in range(65):
            if r % 4 == 0:
                yield hold(src, 2 * NB if inverse else 8)
            rows = pl.ds(8 * r, 8)
            z = [(src[a + 2 * i, rows, :], src[a + 2 * i + 1, rows, :]) for i in range(4)]
            if inverse:
                z = _radix4([turn(z[k], k) for k in range(4)], True)
            else:
                z = [turn(v, k) for k, v in enumerate(_radix4(z, False))]
            for i in range(4):
                dst[b + 2 * i, rows, :], dst[b + 2 * i + 1, rows, :] = z[i]
            yield _Step(35, [anchor(dst)], delay=1, marks=[name] if r == 64 else [])

    def spectral(row, size):
        rows = pl.ds(row, size)
        for k0 in range(4):
            z = _radix4([(Z[8 * g + 2 * k0, rows, :], Z[8 * g + 2 * k0 + 1, rows, :])
                         for g in range(4)], False)
            y = []
            for k1, (re, im) in enumerate(z):
                w = WS[k0 + 4 * k1, rows, :]
                wr = pltpu.bitcast(w << 16, F32)
                wi = pltpu.bitcast(w & np.uint32(0xFFFF0000), F32)
                y.append((re * wr - im * wi, re * wi + im * wr))
            y = _radix4(y, True)
            for g in range(4):
                Z[8 * g + 2 * k0, rows, :], Z[8 * g + 2 * k0 + 1, rows, :] = y[g]

    def spectral_rows(c2):
        for r in range(8):
            spectral(pl.multiple_of(128 * c2 + 16 * r, 16), 16)

    def inv_block(g, i, name, needs, n=None):
        j, t = g + 4 * i, i % 2
        UB, AB, PB, ubu, abu = temps[t]
        n = g if n is None else n
        z = opaque()
        yield _Wait(*needs)
        for r0, rn in _S_ROWS:
            if r0 == 0:
                yield hold(ZT, 8)
            re, im = ZT[z + 2 * i, pl.ds(r0, rn), :], ZT[z + 2 * i + 1, pl.ds(r0, rn), :]
            edge = (_iota(rn, 1) & 63) == 0
            rolled = pltpu.roll(im, 64, 1)
            u = re + jnp.where(edge, lane_vec(L_KU + j, rn) * im, rolled)
            if r0 < 512:
                v = re - jnp.where(edge, lane_vec(L_KV + j, rn) * im, rolled)
                AB[0, pl.ds(r0, rn), :] = u.astype(BF16)
                AB[0, pl.ds(528 + r0, rn), :] = v.astype(BF16)
            else:
                AB[0, pl.ds(512, 16), :] = jnp.concatenate([u, jnp.zeros_like(u)], 0).astype(BF16)
            yield _Step(rn, [anchor(abu)], delay=1, marks=[("read", name)] if r0 == 512 else [])
        yield settle(abu)

        def s_inverse(point):
            z = opaque()
            fa, fb = mat(M_FA + j + z), mat(M_FB + j + z)
            first = _iota(8, 0) == 0

            def put(row, v, v0=None):
                if v0 is not None:
                    v = jnp.concatenate([jnp.where(first, v0, v[:8]), v[8:]], 0)
                UB[0, pl.ds(row, 64), :] = v.astype(BF16)

            for k in range(4):
                lo, hi = 32 * k, 32 * (8 - k if k else 4)
                a = [abu[z, pl.ds(lo, 32), :], abu[z, pl.ds(hi, 32), :]] if k % 2 else [
                    tied(lambda r, o=o: abu[z, pl.ds(o + r, 8), :], 4, point) for o in (lo, hi)]
                if k == 0:
                    a.append(abu[z, pl.ds(256, 8), :])
                re = _dot_t(_bf(jnp.concatenate(a, 0)), fa)
                im = _dot_t(_bf(jnp.concatenate(
                    [abu[z, pl.ds(264 + lo, 32), :], abu[z, pl.ds(264 + hi, 32), :]], 0)), fb)
                pr, mr, pi, mi = re[:64], re[64:128], im[:64], im[64:]
                if k == 0:
                    put(0, pr)
                    put(64, pi, re[128:136])
                    put(128, mr)
                    put(192, mi)
                else:
                    put(256 * k, pr + mr, pr[:8])
                    put(256 * k + 64, pi + mi, mr[:8])
                    put(256 * k + 128, pi - mi, pi[:8])
                    put(256 * k + 192, mr - pr, -mi[:8])
            return 190

        yield _Mat(s_inverse)
        yield settle(ubu)
        yield d_stage(t, lambda c: {0: M_R0T, 1: M_C4T}.get(c, M_RT))
        yield settle(PB)
        z = opaque()
        acc = None
        for r in range(16):
            rows = pl.ds(8 * r, 8)
            t0, t4 = PB[z, rows, :], PB[z, pl.ds(128 + 8 * r, 8), :]
            tk = {}
            for k in (1, 2, 3):
                c, sn = twid[z + 2 * k - 2, rows, :], twid[z + 2 * k - 1, rows, :]
                re = PB[z, pl.ds(256 * k + 8 * r, 8), :]
                im = PB[z, pl.ds(256 * k + 128 + 8 * r, 8), :]
                tk[k] = (re * c - im * sn, re * sn + im * c)
            e0, e1 = t0 + t4, t0 - t4
            s = [e0 + tk[2][0], e1 - tk[2][1], e0 - tk[2][0], e1 + tk[2][1]]
            al, be = tk[1][0] - tk[3][0], tk[1][1] + tk[3][1]
            o = [tk[1][0] + tk[3][0], (al - be) * RSQ2, tk[3][1] - tk[1][1], (al + be) * -RSQ2]
            for b in range(8):
                y = s[b] + o[b] if b < 4 else s[b - 4] - o[b - 4]
                v = X[i][g, pl.ds(128 * b + 8 * r, 8), :] + y
                X[i][n, pl.ds(128 * b + 8 * r, 8), :] = v
                acc = v if acc is None else acc + v
            yield _Step(57, [lambda v=acc: v], delay=5 if r == 15 else 2)
        yield settle(X[i])
        mean = _all_sublanes(acc, jnp.add, 0) * (1.0 / D)
        rstd = yield from ln_rstd(n, i, mean)
        z = opaque()
        for r in range(8):
            v = X[i][n + z, pl.ds(128 * r, 128), :].reshape(16, 8, 128)
            HB[i][n, pl.ds(128 * r, 128), :] = ((v - mean[None]) * rstd[None]).reshape(128, 128).astype(BF16)
            yield _Step(41, [anchor(hbu[i])], delay=1, marks=[name] if r == 7 else [])

    def attend(g, i, name, needs):
        yield _Wait(*needs)
        yield settle(QB[i])
        j, z = g + 4 * i, opaque()
        even = (_iota(8, 0) & 1) == 0
        edge = _iota(8, 1) == 0

        def window(near, far, w, rows):
            return near[j + z + 4 - 2 * w, rows, :] if w <= 2 * i + 2 else far[j + z + 16 - 2 * w, rows, :]

        def mix_values(h, u):
            p = PW[h % 2][opaque()]
            for rows in (pl.ds(256 * h + 16 * u, 16), pl.ds(256 * h + 16 * u + 16, 16)):
                acc = functools.reduce(jnp.add, [p[16 * w:16 * w + 16] * window(VE, VS, w, rows)
                                                 for w in range(8)])
                HB[i][g, rows, :] = acc.astype(BF16)
            return _Step(63, [anchor(hbu[i])], delay=1, marks=[name] if (h, u) == (3, 14) else [])

        for h in range(5):
            logits = []
            for w0 in range(0, 8, 2):
                if h < 4:
                    rows = pl.ds(256 * h, 256)
                    q = QB[i][opaque(), rows, :]
                    for w in (w0, w0 + 1):
                        v = (q * window(KE, KS, w, rows)).reshape(16, 16, 128).sum(0)
                        v = jnp.where(even, v[:8] + pltpu.roll(v[:8], 7, 0), v[8:] + pltpu.roll(v[8:], 1, 0))
                        logits.append(jnp.where(edge & (2 * w > j), -1e9, v * SCALE) if w > 2 * i
                                      else v * SCALE)
                    yield _Step(138, [lambda v=v: v for v in logits[-2:]], delay=2)
                if h > 0:
                    yield mix_values(h - 1, 2 * w0)
                    yield mix_values(h - 1, 2 * w0 + 2)
            if h < 4:
                top = functools.reduce(jnp.maximum, logits)
                e = [jnp.exp(v - top) for v in logits]
                total = functools.reduce(jnp.add, e)
                yield _Step(30, [lambda v=total: v], delay=3)
                scale = 1.0 / total
                for w in range(8):
                    v = e[w] * scale
                    PW[h % 2][0, pl.ds(16 * w, 8), :] = jnp.where(even, v, pltpu.roll(v, 1, 0))
                    PW[h % 2][0, pl.ds(16 * w + 8, 8), :] = jnp.where(even, pltpu.roll(v, 7, 0), v)
                yield _Step(50, [anchor(PW[h % 2])], delay=6 if h == 3 else 1)

    def proj(sch, w, g, i, m, store, needs, marks, own=120):
        for name in needs:
            sch.run(name)
        row = pl.multiple_of(64 * m, 64)
        parts = []
        sch.fresh = True
        for col in (0, 512):
            parts.append(tied(lambda r: WT[w][pl.ds(row + r, 8), pl.ds(col, 128)], 8,
                              lambda: sch.point(own / 16)))
            parts.append(WT[w][pl.ds(row, 64), pl.ds(col + 128, 384)])
        v = _dot(_bf(jnp.concatenate(parts, 1)), _bf(hbu[i][g + opaque()]))
        store(v, pl.ds(pl.multiple_of(128 * m, 128), 128))
        sch.results.append(v[:8])
        for name in marks:
            sch.done[name] = sch.slot + WAIT

    def kv_proj(sch, g, i, needs):
        for w, ref in ((1, KE), (2, VE)):
            def store(v, rows):
                ref[g + 4 * i + 4, rows, :] = v
            for m in range(8):
                proj(sch, w, g, i, m, store, needs, [("kv", i)] if (w, m) == (2, 7) else [])

    def shift_block(g, i, name, needs):
        yield _Wait(*needs)
        j, z = g + 4 * i, opaque()
        for m in range(16):
            rows = pl.ds(64 * m, 64)
            for ref, to in ((KE, KS), (VE, VS)):
                v = pltpu.roll(ref[j + 4 + z, rows, :], 1, 1)
                if ref is VE:
                    v = jnp.where(_iota(64, 1) == 0, ref[4 + z, rows, :], v)
                to[j, rows, :] = v
                if i == 3:
                    ref[g, rows, :] = v
            yield _Step(12, delay=8 if i == 3 else 4, marks=[name] if m == 15 else [])

    def q_proj(sch, g, i, name):
        def store(v, rows):
            QB[i][0, rows, :] = v
        for m in range(8):
            proj(sch, 0, g, i, m, store, [], [name] if m == 7 else [])

    def o_proj(sch, g, i, m, needs, marks):
        def store(v, rows):
            X[i][g, rows, :] = X[i][g, rows, :] + v
        proj(sch, 3, g, i, m, store, needs, marks, own=135)

    def transpose_weight(w, quarters, name):
        for h in quarters:
            for r in range(4):
                v = WRAW[w, pl.ds(256 * r, 256), pl.ds(pl.multiple_of(256 * h, 256), 256)]
                v = pltpu.bitcast(v.T, U32)
                TR[2 * r], TR[2 * r + 1] = v[:, :128], v[:, 128:]
                yield _Step(40, delay=16)
            z = opaque()
            for c in range(8):
                WT[w][pl.ds(pl.multiple_of(128 * h, 128), 128), pl.ds(128 * c, 128)] = jnp.concatenate(
                    [TR[c + z, pl.ds(u, 8, stride=16), :] for u in range(16)], 0)
                yield _Step(20, delay=4, marks=[name] if c == 7 else [])

    def transpose_wo(name):
        for c in range(8):
            for h in range(4):
                v = jnp.concatenate([wou[c, pl.ds(128 * h + u, 8, stride=16), :] for u in range(16)], 0)
                WP[pl.ds(64 * c, 64), pl.ds(256 * h, 256)] = pltpu.bitcast(_bf(v).T, U32)
                yield _Step(20, delay=10, marks=[name] if c == 7 and h == 3 else [])

    def prep_spectral_weights(c2):
        lane = _iota(8, 1)
        order = jnp.where(lane > 64, 192 - lane, lane)

        def words(k2):
            re, im = (wsu[u, k2, pl.ds(c2, 64, stride=4), :] for u in range(2))
            return ((re & np.uint32(0xFFFF)) | (im << 16), (re >> 16) | (im & np.uint32(0xFFFF0000)))

        def arrange(w, below):
            w = jnp.where(_iota(w.shape[0], 1) < 64, w, below)
            return jnp.concatenate([jnp.take_along_axis(w[u:u + 8], order, axis=1)
                                    for u in range(0, w.shape[0], 8)], 0)

        below = words(15)
        for k2 in range(16):
            here = words(k2)
            for e in range(2):
                cl = 2 * c2 + e
                w = arrange(here[e], below[e])
                WS[k2, pl.ds(64 * cl, 64), :] = pltpu.roll(w, 1, 0) if cl > 4 else w
            below = here
            yield _Step(100)
        if c2 == 0:
            def nyquist(k2):
                re, im = (jnp.broadcast_to(WN[u, :, pl.ds(128 * k2, 128)].astype(F32), (8, 128))
                          for u in range(2))
                return pltpu.pack_elementwise([re, im], packed_dtype=BF16)
            for k2 in range(16):
                WS[k2, pl.ds(512, 8), :] = arrange(nyquist(k2), nyquist((k2 + 15) % 16))

    def write_out(p, c, name, needs):
        yield _Wait(*needs)
        rows = pl.ds(pl.multiple_of(128 * c, 128), 128)
        g, i = 2 * p % 4 + opaque(), p // 2
        w = pltpu.pack_elementwise([X[i][g, rows, :], X[i][g + 1, rows, :]], packed_dtype=BF16)
        xru[c, pl.ds(p, 128, stride=8), :] = w.T
        yield _Step(30, marks=[name])

    for c in range(8):
        x_copy(c).start()
    for c in range(5):
        mats[M_R + c] = d_mats[c]

    def make_twiddle(k):
        PB = temps[0][2]
        PB[0, pl.ds(0, 128), :] = lane_vec(L_TWID + k, 128)
        twid[k] = PB[opaque(), pl.ds(0, 128), :].T

    _loop(6, make_twiddle, "make_twiddle")

    def make_dft(j):
        fa, fb = lanes[pl.ds(L_FA, 128), :], lanes[pl.ds(L_FB, 128), :]
        c, sn = lane_vec(L_COS + j, 128), lane_vec(L_SIN + j, 128)
        UB, _, _, ubu, _ = temps[0]
        UB[0, pl.ds(0, 128), :] = (fa * c + fb * sn).astype(BF16)
        UB[0, pl.ds(128, 128), :] = (fb * c - fa * sn).astype(BF16)
        mats[M_FA + j], mats[M_FB + j] = ubu[0, pl.ds(0, 64), :], ubu[0, pl.ds(64, 64), :]

    _loop(NB, make_dft, "make_dft")

    def load_x(c):
        x_copy(c).wait()
        pl.when(c == 5)(lambda: start_all(spec_copies[0]))
        pl.when(c == 7)(lambda: start_all(spec_copies[1]))
        rows = pl.ds(pl.multiple_of(128 * c, 128), 128)
        for p in range(8):
            w = xru[c, pl.ds(p, 128, stride=8), :].T
            for e, bits in enumerate((w << 16, w & np.uint32(0xFFFF0000))):
                g, i = 2 * p % 4 + e, p // 2
                v = pltpu.bitcast(bits, F32)
                X[i][g, rows, :] = v
                v = v.reshape(16, 8, 128)
                mean = _all_sublanes(v.sum(0), jnp.add, 0) * (1.0 / 128)
                STAT[4 * g + i, c] = mean
                STAT[4 * g + i, 8 + c] = _all_sublanes(((v - mean) ** 2).sum(0), jnp.add, 0)

    _loop(8, load_x, "load_x")

    def after(name, action):
        yield _Wait(name)
        action()

    def spectral_weights():
        yield _Wait(("f", 2, 1))
        for c in spec_copies[0] + spec_copies[1]:
            c.wait()
        for c2 in range(4):
            yield from prep_spectral_weights(c2)

    with jax.named_scope("first_forward"):
        sch = _Sched(0.92)
        sch.add(after(("f", 0, 1), w_copies[1].start), "k")
        sch.add(after(("f", 1, 1), w_copies[2].start), "v")
        sch.add(after(("f", 2, 3), w_copies[0].start), "q")
        for g in range(4):
            for i in range(4):
                sch.add(fwd_block(g, i, ("f", g, i), [("f", g - 1, i)] if g else [],
                                  [("r", g - 1)] if g else [], True), ("f", g, i))
            sch.add(group_stage(g, ("r", g), [("f", g, i) for i in range(4)], False), ("r", g))
        sch.add(spectral_weights(), "s")
        sch.drive()
    start_all(wo_copies)

    def keys_values(layer, g):
        sch = _Sched(0.36 if layer == 0 else 0.33)
        sch.done[("i", 0)] = 0
        for i in range(1, 3):
            sch.add(inv_block(g, i, ("i", i), [("read", ("i", 1))] if i == 2 else []), ("i", i))
        nxt = (g + 1) % 4
        sch.add(inv_block(g, 3, ("i", 3), [("i", 1)]), ("i", 3))
        sch.add(group_stage(nxt, "r", [("read", ("i", i)) for i in (1, 2, 3)], True), "r")
        sch.add(inv_block(nxt, 0, ("i", 4), ["r", ("i", 2)], n=g + 1), ("i", 4))
        if layer == 0:
            sch.add(transpose_weight(0, [g], "w"), "w")
        sch.add(shift_block((g + 3) % 4, 3, ("s", 0), []), ("s", 0))
        for i in range(1, 4):
            sch.add(shift_block(g, i - 1, ("s", i), [("kv", i - 1)]), ("s", i))
        for i in range(4):
            kv_proj(sch, g, i, [("i", i)])
        sch.finish()

    def mix(g, after, last, write):
        sch = _Sched(0.67 if last else 0.63)
        now = 8 - DEFER if last else 8
        tail = after is None

        def block(i):
            return (g, i) if i < 4 else (after, i - 4)

        sch.done[("a", 0)] = 0
        for i in range(3 if tail else 4):
            sch.add(attend(*block(i + 1), ("a", i + 1), [("q", i + 1), ("a", i)] if i else []),
                    ("a", i + 1), pace=0.30 if last or tail else 0.26)
        if not last:
            sch.add(group_stage((g + 3) % 4, "r", [], False), "r")
            for i in range(4):
                sch.add(fwd_block(g, i, ("f", i), [("o", i, 7)], ["r"]), ("f", i))
        for i in range(4 if write else 0):
            for c in range(now):
                sch.add(write_out(2 * i + g // 2, c, ("w", i, c), [("o", i, c)]), ("w", i, c))
        if tail:
            q_proj(sch, g, 2, ("q", 2))
            q_proj(sch, g, 3, ("q", 3))
        for i in range(4):
            for m in range(now):
                o_proj(sch, g, i, m, [("a", i)], [("o", i, m)])
            if not tail:
                q_proj(sch, *block(i + 2), ("q", i + 2))
        if tail and not last:
            sch.add(group_stage(g, "s", [("f", i) for i in range(4)], False), "s")
        sch.finish()

    def postponed(u):
        c = 8 - DEFER + u
        sch = _Sched(0.5)
        for p in range(8):
            sch.add(write_out(p, c, ("w", p), [("o", p)]), ("w", p))
            o_proj(sch, 2 * p % 4, p // 2, c, [], [])
            o_proj(sch, 2 * p % 4 + 1, p // 2, c, [], [("o", p)])
        sch.finish()
        out_copy(c).start()

    def spectral_and_weights(h):
        for _ in transpose_weight(1, [h], None):
            pass
        spectral_rows(h)
        for _ in transpose_weight(2, [h], None):
            pass

    for layer in range(2):
        with jax.named_scope("spectral"):
            if layer == 0:
                w_copies[1].wait()
                w_copies[2].wait()
                _loop(4, spectral_and_weights, "rows")
            else:
                _loop(4, spectral_rows, "rows")
            spectral(512, 8)
        sch = _Sched()
        sch.add(group_stage(0, "r", [], True), "r")
        sch.add(inv_block(0, 0, "i", ["r"]), "i")
        sch.finish()
        if layer == 0:
            w_copies[0].wait()
        _loop(4, lambda g: keys_values(layer, g), "keys_values")
        sch = _Sched(0.66)
        sch.add(attend(0, 0, "a", ["q"]), "a")
        sch.add(shift_block(3, 3, "s", []), "s")
        if layer == 0:
            for c in wo_copies:
                c.wait()
            sch.add(transpose_wo("w"), "w")
        q_proj(sch, 0, 0, "q")
        q_proj(sch, 0, 1, None)
        sch.finish()
        if layer == 0:
            _loop(3, lambda g: mix(g, g + 1, False, False), "mix")
            mix(3, None, False, False)
        else:
            _loop(2, lambda u: mix(2 * u, 2 - u, True, False), "mix")
            mix(1, 3, True, True)
            mix(3, None, True, True)
    for c in range(8 - DEFER):
        out_copy(c).start()
    _loop(DEFER, postponed, "postponed")
    for c in range(8):
        out_copy(c).wait()


@jax.jit
def pallas_interleave_layers__spectral_gfnet__sliding_local_dilated__prompt_kernel(
    A_x: jax.Array,
    A_w_r: jax.Array,
    A_w_i: jax.Array,
    B_x: jax.Array,
    B_wqkv: jax.Array,
    B_wo: jax.Array,
):
    del B_x
    hbm = pl.BlockSpec(memory_space=pl.ANY)
    smem = pl.BlockSpec(memory_space=pltpu.SMEM)
    out = pl.pallas_call(
        _kernel,
        out_shape=jax.ShapeDtypeStruct((S, D), BF16),
        in_specs=[smem, smem, pl.BlockSpec(), pl.BlockSpec(), hbm, hbm, hbm, hbm, hbm],
        out_specs=hbm,
        scratch_shapes=[
            pltpu.VMEM((37, 64, 128), U32),
            pltpu.VMEM((6, 128, 128), F32),
            pltpu.VMEM((NB, 16, 8, 128), F32),
            pltpu.VMEM((NB + 4, D, 128), F32),
            pltpu.VMEM((NB + 4, D, 128), F32),
            pltpu.VMEM((NB, D, 128), F32),
            pltpu.VMEM((NB, D, 128), F32),
            pltpu.VMEM((2 * NB + 1, ZR, 128), F32),
            pltpu.VMEM((9, ZR, 128), F32),
            pltpu.VMEM((NB, ZR, 128), U32),
            *4 * [pltpu.VMEM((D // 2, D), U32)],
            pltpu.VMEM((8, S, 128), BF16),
            pltpu.VMEM((2, NB, D // 2, 128), BF16),
            pltpu.VMEM((2, 1, S), BF16),
            pltpu.VMEM((3, D, D), BF16),
            pltpu.VMEM((8, D, 128), BF16),
            pltpu.VMEM((8, 128, 128), U32),
            pltpu.VMEM((1, 128, 128), F32),
            pltpu.VMEM((1, 128, 128), F32),
            pltpu.SemaphoreType.DMA((24,)),
        ] + 4 * [
            pltpu.VMEM((5, D, 128), F32),
            pltpu.VMEM((5, D, 128), BF16),
            pltpu.VMEM((1, D, 128), F32),
            pltpu.VMEM((1, D, 128), BF16),
            pltpu.VMEM((1, 1152, 128), BF16),
            pltpu.VMEM((1, D, 128), F32),
        ],
        compiler_params=pltpu.CompilerParams(vmem_limit_bytes=124 * 2 ** 20),
    )(_ZERO, _ROT, _MATS, _LANES, A_x.reshape(S, D), A_w_r.T, A_w_i.T, B_wqkv, B_wo)
    return out.reshape(1, S, D)
```

```python
import functools

import numpy as np

import jax
import jax.numpy as jnp
import jax.experimental.pallas as pl
import jax.experimental.pallas.tpu as pltpu

S, D, NB = 2048, 1024, 16
ZR = 576
F32, BF16, U32, I32 = jnp.float32, jnp.bfloat16, jnp.uint32, jnp.int32
EPS = 1e-5
SCALE = 32 ** -0.5
RSQ2 = float(np.sqrt(0.5))
WAIT = 24
GRAIN = 1
SETTLE = 6
LAG = 3

_S_ROWS = [(32 * u, 32) for u in range(16)] + [(512, 8)]

M_FA, M_FB, M_R, M_C4, M_RT, M_C4T, M_R0T = 0, 16, 32, 33, 34, 35, 36
L_MU, L_NU, L_KU, L_KV, L_COS, L_SIN, L_TWID, L_FA, L_FB = 0, 16, 32, 48, 64, 80, 96, 104, 232


def _bf16_bits(a):
    u = np.ascontiguousarray(a, dtype=np.float32).view(np.uint32).astype(np.uint64)
    return ((u + 0x7FFF + ((u >> 16) & 1)) >> 16).astype(np.uint32)


def _constants():
    a = np.arange(128)
    k1 = np.arange(64)
    alt = (-1.0) ** a
    lanes = np.zeros((L_FB + 128, 128))
    t = 2 * np.pi * np.outer(a, k1) / 128
    fa = np.concatenate([np.cos(t), -np.sin(t)], 1)
    fb = np.concatenate([np.sin(t), -np.cos(t)], 1)
    fa[:, 0], fb[:, 0] = RSQ2, -RSQ2
    fa[:, 64], fb[:, 64] = alt, 0.0
    lanes[L_FA:L_FA + 128], lanes[L_FB:L_FB + 128] = fa, fb
    for j in range(NB):
        ang = 2 * np.pi * j / 32 + np.pi / 32
        p, q = (_bf16_bits([np.cos(ang), np.sin(ang)]) << 16).view(np.float32).astype(np.float64)
        turn = 2 * np.pi * j * np.tile(k1, 2) / S
        lanes[L_COS + j], lanes[L_SIN + j] = np.cos(turn), np.repeat([-1.0, 1.0], 64) * np.sin(turn)
        lanes[L_COS + j, 64], lanes[L_SIN + j, 64] = p, q
        lanes[L_MU + j, 0], lanes[L_MU + j, 64] = 1.0, (q / p + p / q) / 2
        lanes[L_NU + j, 0], lanes[L_NU + j, 64] = 0.0, (q / p - p / q) / 2
        lanes[L_KU + j, 0], lanes[L_KU + j, 64] = 1.0, q / p
        lanes[L_KV + j, 0], lanes[L_KV + j, 64] = 1.0, p / q
    for k in (1, 2, 3):
        lanes[L_TWID + 2 * k - 2] = np.cos(2 * np.pi * a * k / D)
        lanes[L_TWID + 2 * k - 1] = np.sin(2 * np.pi * a * k / D)
    th = 2 * np.pi * np.outer(k1, a) / 128
    r = np.concatenate([np.cos(th), -np.sin(th)], 0)
    r[64] = alt
    th = 2 * np.pi * np.outer(2 * k1 + 1, a) / 256
    c4 = np.concatenate([np.cos(th), -np.sin(th)], 0)
    inv = 2.0 / (S * D)
    r0t = inv * r.T
    r0t[:, 0::64] *= 0.5
    rows = np.arange(128).reshape(2, 4, 16).transpose(1, 0, 2).ravel()
    bits = _bf16_bits(np.stack([r[rows], c4[rows], inv * r.T, inv * c4.T, r0t]))
    ang = 2 * np.pi * np.outer(np.arange(4), np.arange(4)).ravel() / 16
    rot = np.concatenate([np.cos(ang), np.sin(ang)]).astype(np.float32)
    return bits[:, 0::2] | (bits[:, 1::2] << 16), lanes.astype(np.float32), rot


_MATS, _LANES, _ROT = _constants()
_ZERO = np.zeros((1,), np.int32)


class _Step:
    def __init__(self, cost, anchors=(), delay=0, marks=()):
        self.cost, self.anchors, self.delay, self.marks = cost, list(anchors), delay, list(marks)


class _Wait:
    def __init__(self, *names):
        self.names = names


class _Mat:
    def __init__(self, emit):
        self.emit = emit


class _Hold:
    def __init__(self, store):
        self.store = store


class _Task:
    def __init__(self, gen, pace):
        self.gen, self.pace, self.blocked, self.not_before, self.held = gen, pace, (), 0, None
        self.allowed = 0.0


class _Sched:
    def __init__(self, share=0.0):
        self.share = share
        self.tasks, self.done, self.producer = [], {}, {}
        self.slot, self.credit, self.anchors, self.results = 0, 0.0, [], []
        self.fresh = False

    def add(self, gen, name, pace=99):
        self.producer[name] = self.producer["read", name] = _Task(gen, pace)
        self.tasks.append(self.producer[name])

    def _ready(self, t):
        return t.not_before <= self.slot and all(
            n in self.done and self.done[n] <= self.slot for n in t.blocked)

    def _advance(self, t, mats=True):
        item, t.held = t.held or next(t.gen, None), None
        if item is None:
            self.tasks.remove(t)
        elif isinstance(item, _Wait):
            t.blocked = item.names
        elif isinstance(item, _Hold):
            if len(self.results) >= LAG:
                item.store(self.results[-LAG])
        elif isinstance(item, _Mat):
            if mats:
                t.not_before = float("inf")
                self.fresh = False
                self.credit -= item.emit(lambda: self.point(0.0)) or 0
                t.not_before = self.slot + WAIT
            else:
                t.held, t.not_before = item, self.slot + 1
        else:
            t.blocked = ()
            t.not_before = self.slot + item.delay
            self.credit -= item.cost
            self.anchors += item.anchors
            for n in item.marks:
                self.done[n] = self.slot + item.delay
            return True

    def run(self, *names):
        while not all(n in self.done for n in names):
            for n in names:
                if n not in self.done:
                    for b in self.producer[n].blocked:
                        self.run(b)
                    self._advance(self.producer[n])

    def drive(self):
        while self.tasks:
            ready = [t for t in self.tasks if self._ready(t)]
            if not ready:
                self.slot += 1
                continue
            self.anchors, self.credit = self.anchors[-2:], 0.0
            self._advance(next((t for t in ready if t.held), ready[0]))
            self.slot -= min(self.credit, 0.0) / 60

    def finish(self):
        self.run(*[n for n in self.producer if n[0] != "read"])

    def point(self, own):
        for t in self.tasks:
            t.allowed = min(t.allowed, 0.0) + t.pace
        while True:
            t = next((t for t in self.tasks if self._ready(t) and t.allowed > 0
                      and self.credit > 0), None)
            if t is None:
                break
            if self._advance(t, self.fresh):
                t.allowed -= 1
        anchors, self.anchors = self.anchors, []
        self.credit = min(self.credit, 10.0) + 64 * self.share - own
        self.fresh = False
        self.slot += 1
        return anchors


def _dot(a, b):
    return jnp.dot(a, b, preferred_element_type=F32)


def _dot_t(a, b):
    return jax.lax.dot_general(a, b, (((1,), (1,)), ((), ())), preferred_element_type=F32)


def _bf(u):
    return pltpu.bitcast(u, BF16)


def _iota(rows, dim):
    return jax.lax.broadcasted_iota(I32, (rows, 128), dim)


def _radix4(z, inverse):
    (r0, i0), (r1, i1), (r2, i2), (r3, i3) = z
    ar, ai, cr, ci = r0 + r2, i0 + i2, r0 - r2, i0 - i2
    br, bi, dr, di = r1 + r3, i1 + i3, r1 - r3, i1 - i3
    lo, hi = (cr + di, ci - dr), (cr - di, ci + dr)
    if inverse:
        lo, hi = hi, lo
    return [(ar + br, ai + bi), lo, (ar - br, ai - bi), hi]


def _all_sublanes(v, op, axis):
    for sh in (4, 2, 1):
        v = op(v, pltpu.roll(v, sh, axis))
    return v


def _loop(n, body, name):
    def step(i, carry):
        body(i)
        return carry
    with jax.named_scope(name):
        jax.lax.fori_loop(0, n, step, 0)


def _kernel(zero_ref, rot, d_mats, lanes, x_hbm, wr_hbm, wi_hbm, wqkv_hbm, wo_hbm, out_hbm,
            mats, twid, STAT, KE, VE, KS, VS, Z, ZT, WS, WQ, WK, WV, WP, WS5, WQ5, WP5, SB0, SB1, SB2, SB3, XR, WRI, WN, WRAW, WO, TR, PW0, PW1, sems, *split):
    zero = zero_ref[0]
    never = zero != 0
    X, HB, QB = split[0::6], split[1::6], split[2::6]
    hbu = [r.bitcast(U32) for r in HB]
    xru, wsu, wou = XR.bitcast(U32), WRI.bitcast(U32), WO.bitcast(U32)
    temps = [(ub, ab, pb, ub.bitcast(U32), ab.bitcast(U32))
             for ub, ab, pb in zip(split[3::6], split[4::6], split[5::6])]
    PW, SB, WT = (PW0, PW1), (SB0, SB1, SB2, SB3), (WQ, WK, WV, WP)
    counter = [0]

    def opaque():
        counter[0] += 1
        return zero * counter[0]

    def anchor(ref):
        return lambda: ref[0, pl.ds(pl.multiple_of(zero * 8, 8), 8), pl.ds(0, 128)]

    def settle(ref):
        return _Step(2, [anchor(ref)], delay=SETTLE)

    def hold(ref, spare, row=0):
        def store(v):
            ref[spare, pl.ds(pl.multiple_of(row + zero * 8, 8), 8), :] = v
        return _Hold(store)

    def tied(load, vregs, point):
        parts = []
        for r in range(vregs):
            anchors = [a for _ in range(GRAIN) for a in point()] if r % GRAIN == 0 else []
            u = load(8 * r)
            for a in anchors:
                u = jnp.where(never, pltpu.bitcast(a(), U32), u)
            parts.append(u)
        return jnp.concatenate(parts, 0)

    def mat(i):
        return _bf(mats[i])

    def d_stage(t, which):
        UB, AB, PB, ubu, abu = temps[t]

        def emit(point):
            z = opaque()
            for c in range(8):
                lhs = mat(which(c) + opaque()) if c % 4 else _bf(
                    tied(lambda r, u=which(c) + opaque(): mats[u, pl.ds(r, 8), :], 8, point))
                PB[0, pl.ds(128 * c, 128), :] = _dot(lhs, _bf(ubu[z, pl.ds(64 * c, 64), :]))
        return _Mat(emit)

    def lane_vec(i, rows):
        return jnp.broadcast_to(lanes[pl.ds(i, 1), :], (rows, 128))

    def x_copy(c):
        return pltpu.make_async_copy(
            x_hbm.at[:, pl.ds(pl.multiple_of(128 * c, 128), 128)], XR.at[c], sems.at[c])

    def out_copy(c):
        return pltpu.make_async_copy(
            XR.at[c], out_hbm.at[:, pl.ds(pl.multiple_of(128 * c, 128), 128)], sems.at[8 + c])

    spec_copies = [[pltpu.make_async_copy(w.at[pl.ds(0, 512), pl.ds(128 * k2, 128)], WRI.at[u, k2],
                                          sems.at[16 + u]) for k2 in range(16)]
                   + [pltpu.make_async_copy(w.at[pl.ds(512, 1), :], WN.at[u], sems.at[22 + u])]
                   for u, w in enumerate((wr_hbm, wi_hbm))]

    def start_all(copies):
        for c in copies:
            c.start()
    w_copies = [pltpu.make_async_copy(wqkv_hbm.at[:, pl.ds(D * w, D)], WRAW.at[w], sems.at[18 + w])
                for w in range(3)]
    wo_copies = [pltpu.make_async_copy(wo_hbm.at[:, pl.ds(128 * c, 128)], WO.at[c], sems.at[21])
                 for c in range(8)]

    def ln_rstd(g, i, mean):
        acc, m = None, g + opaque()
        for r in range(8):
            d = X[i][m, pl.ds(128 * r, 128), :].reshape(16, 8, 128) - mean[None]
            v = (d * d).sum(0)
            acc = v if acc is None else acc + v
            if r < 7:
                yield _Step(50, [lambda acc=acc: acc], delay=3)
        rstd = jax.lax.rsqrt(_all_sublanes(acc, jnp.add, 0) * (1.0 / D) + EPS)
        yield _Step(50, delay=8)
        yield _Step(10, [lambda: rstd], delay=1)
        return rstd

    def fwd_block(g, i, name, needs, free=(), known=False):
        j, t = g + 4 * i, i
        UB, AB, PB, ubu, abu = temps[t]
        yield _Wait(*needs)
        if known:
            means, squares = STAT[4 * g + i, pl.ds(0, 8)], STAT[4 * g + i, pl.ds(8, 8)]
            mean = means.sum(0) * 0.125
            var = (squares.sum(0) + 128.0 * ((means - mean) ** 2).sum(0)) * (1.0 / D)
            rstd = jax.lax.rsqrt(var + EPS)
            yield _Step(50, delay=6)
        else:
            yield settle(X[i])
            acc, m = None, g + opaque()
            for r in range(8):
                v = X[i][m, pl.ds(128 * r, 128), :].reshape(16, 8, 128).sum(0)
                acc = v if acc is None else acc + v
                if r % 2:
                    yield _Step(35, [lambda acc=acc: acc], delay=7 if r == 7 else 3)
            mean = _all_sublanes(acc, jnp.add, 0) * (1.0 / D)
            rstd = yield from ln_rstd(g, i, mean)
        mean8, rstd = (jnp.concatenate([v, v], 0) for v in (mean * 8.0, rstd))
        z = opaque()
        for r in range(8):
            rows = pl.ds(16 * r, 16)
            x = [X[i][g + z, pl.ds(128 * b + 16 * r, 16), :] for b in range(8)]
            s = [x[b] + x[b + 4] for b in range(4)]
            d = [x[b] - x[b + 4] for b in range(4)]
            e, o = s[0] + s[2], s[1] + s[3]
            UB[0, rows, :] = ((e + o - mean8) * rstd).astype(BF16)
            UB[0, pl.ds(128 + 16 * r, 16), :] = ((e - o) * rstd).astype(BF16)
            t1, t2 = (d[1] - d[3]) * RSQ2, (d[1] + d[3]) * RSQ2
            u = {1: (d[0] + t1, d[2] + t2), 2: (s[0] - s[2], s[1] - s[3]), 3: (d[0] - t1, d[2] - t2)}
            yield _Step(34, [anchor(ubu)], delay=1)
            for k in (1, 2, 3):
                c, sn = twid[z + 2 * k - 2, rows, :] * rstd, twid[z + 2 * k - 1, rows, :] * rstd
                re, m = u[k]
                if k == 3:
                    ur, ui = re * c + m * sn, m * c - re * sn
                else:
                    ur, ui = re * c - m * sn, m * c + re * sn
                UB[0, pl.ds(256 * k + 16 * r, 16), :] = ur.astype(BF16)
                UB[0, pl.ds(256 * k + 128 + 16 * r, 16), :] = ui.astype(BF16)
                yield _Step(26, [anchor(ubu)], delay=1)
        yield settle(ubu)

        def d_forward(point):
            z = opaque()
            first = _iota(8, 0) == 0

            def stage(c):
                u = (M_C4 if c == 1 else M_R) + opaque()
                lhs = mat(u) if c % 4 else _bf(tied(lambda r: mats[u, pl.ds(r, 8), :], 8, point))
                v = _dot(lhs, _bf(ubu[z, pl.ds(64 * c, 64), :]))
                return [(v[32 * u:32 * u + 16], v[32 * u + 16:32 * u + 32]) for u in range(4)]

            def put(row, u, v, v0=None):
                if u == 0 and v0 is not None:
                    v = jnp.concatenate([jnp.where(first, v0, v[:8]), v[8:]], 0)
                AB[0, pl.ds(row + 16 * u, 16), :] = v.astype(BF16)

            for u, (p1, p2) in enumerate(stage(0)):
                put(0, u, p1)
                put(528, u, p2, 0.0)
                if u == 0:
                    put(512, 0, jnp.zeros_like(p2), p2[:8])
            for u, (p1, p2) in enumerate(stage(1)):
                put(256, u, p1)
                put(528 + 256, u, p2)
            for k in (1, 2, 3):
                for u, ((p1, p2), (q1, q2)) in enumerate(zip(stage(2 * k), stage(2 * k + 1))):
                    if k == 3:
                        pr, pi, mr, mi = p1 - q2, p2 + q1, p1 + q2, p2 - q1
                        pi0, mi0 = q1[:8], -q2[:8]
                    else:
                        pr, pi, mr, mi = p1 + q2, p2 - q1, p1 - q2, p2 + q1
                        pi0, mi0 = -q1[:8], q2[:8]
                    put(64 * k, u, pr, p1[:8])
                    put(64 * (8 - k), u, mr, p2[:8])
                    put(528 + 64 * k, u, pi, pi0)
                    put(528 + 64 * (8 - k), u, mi, mi0)
            return 190

        yield _Mat(d_forward)
        yield settle(abu)
        yield _Wait(*free)

        def s_forward(point):
            z = opaque()
            fa, fb = mat(M_FA + j + z), mat(M_FB + j + z)
            for r0, rn in ((0, 256), (256, 272)):
                lhs = abu[z, pl.ds(r0 // 2, rn // 2), :] if r0 else tied(
                    lambda r: abu[z, pl.ds(r, 8), :], 16, point)
                u = _dot(_bf(lhs), fa)
                v = _dot(_bf(abu[z, pl.ds(264 + r0 // 2, 128), :]), fb)
                re, m = u[:256] + v, u[:256] - v
                if r0:
                    re, m = (jnp.concatenate([a, u[256:264]], 0) for a in (re, m))
                rn = re.shape[0]
                edge = (_iota(rn, 1) & 63) == 0
                ZT[2 * i, pl.ds(r0, rn), :] = re
                ZT[2 * i + 1, pl.ds(r0, rn), :] = jnp.where(
                    edge, lane_vec(L_MU + j, rn) * m + lane_vec(L_NU + j, rn) * re, pltpu.roll(m, 64, 1))
            return 400

        yield _Mat(s_forward)
        yield _Step(2, [anchor(ZT)], delay=SETTLE, marks=[name])

    def group_stage(g, name, needs, inverse):
        yield _Wait(*needs)

        def turn(z, k):
            if k == 0:
                return z
            c, s = rot[4 * g + k], rot[16 + 4 * g + k]
            if inverse:
                return z[0] * c - z[1] * s, z[1] * c + z[0] * s
            return z[0] * c + z[1] * s, z[1] * c - z[0] * s

        (src, a), (dst, b) = ((Z, 8 * g), (ZT, 0)) if inverse else ((ZT, opaque()), (Z, 8 * g))
        for r in range(65):
            if r % 4 == 0:
                yield hold(src, 2 * NB if inverse else 8)
            rows = pl.ds(8 * r, 8)
            z = [(src[a + 2 * i, rows, :], src[a + 2 * i + 1, rows, :]) for i in range(4)]
            if inverse:
                z = _radix4([turn(z[k], k) for k in range(4)], True)
            else:
                z = [turn(v, k) for k, v in enumerate(_radix4(z, False))]
            for i in range(4):
                dst[b + 2 * i, rows, :], dst[b + 2 * i + 1, rows, :] = z[i]
            yield _Step(35, [anchor(dst)], delay=1, marks=[name] if r == 64 else [])

    def spectral(row, size):
        rows = pl.ds(row, size)
        for k0 in range(4):
            z = _radix4([(Z[8 * g + 2 * k0, rows, :], Z[8 * g + 2 * k0 + 1, rows, :])
                         for g in range(4)], False)
            y = []
            for k1, (re, im) in enumerate(z):
                w = WS[k0 + 4 * k1, rows, :]
                wr = pltpu.bitcast(w << 16, F32)
                wi = pltpu.bitcast(w & np.uint32(0xFFFF0000), F32)
                y.append((re * wr - im * wi, re * wi + im * wr))
            y = _radix4(y, True)
            for g in range(4):
                Z[8 * g + 2 * k0, rows, :], Z[8 * g + 2 * k0 + 1, rows, :] = y[g]

    def spectral_rows(c2):
        for r in range(8):
            spectral(pl.multiple_of(128 * c2 + 16 * r, 16), 16)

    def inv_block(g, i, name, needs, n=None):
        j, t = g + 4 * i, i % 2
        UB, AB, PB, ubu, abu = temps[t]
        n = g if n is None else n
        z = opaque()
        yield _Wait(*needs)
        for r0, rn in _S_ROWS:
            if r0 == 0:
                yield hold(ZT, 8)
            re, im = ZT[z + 2 * i, pl.ds(r0, rn), :], ZT[z + 2 * i + 1, pl.ds(r0, rn), :]
            edge = (_iota(rn, 1) & 63) == 0
            rolled = pltpu.roll(im, 64, 1)
            u = re + jnp.where(edge, lane_vec(L_KU + j, rn) * im, rolled)
            if r0 < 512:
                v = re - jnp.where(edge, lane_vec(L_KV + j, rn) * im, rolled)
                AB[0, pl.ds(r0, rn), :] = u.astype(BF16)
                AB[0, pl.ds(528 + r0, rn), :] = v.astype(BF16)
            else:
                AB[0, pl.ds(512, 16), :] = jnp.concatenate([u, jnp.zeros_like(u)], 0).astype(BF16)
            yield _Step(rn, [anchor(abu)], delay=1, marks=[("read", name)] if r0 == 512 else [])
        yield settle(abu)

        def s_inverse(point):
            z = opaque()
            fa, fb = mat(M_FA + j + z), mat(M_FB + j + z)
            first = _iota(8, 0) == 0

            def put(row, v, v0=None):
                if v0 is not None:
                    v = jnp.concatenate([jnp.where(first, v0, v[:8]), v[8:]], 0)
                UB[0, pl.ds(row, 64), :] = v.astype(BF16)

            for k in range(4):
                lo, hi = 32 * k, 32 * (8 - k if k else 4)
                a = [abu[z, pl.ds(lo, 32), :], abu[z, pl.ds(hi, 32), :]] if k % 2 else [
                    tied(lambda r, o=o: abu[z, pl.ds(o + r, 8), :], 4, point) for o in (lo, hi)]
                if k == 0:
                    a.append(abu[z, pl.ds(256, 8), :])
                re = _dot_t(_bf(jnp.concatenate(a, 0)), fa)
                im = _dot_t(_bf(jnp.concatenate(
                    [abu[z, pl.ds(264 + lo, 32), :], abu[z, pl.ds(264 + hi, 32), :]], 0)), fb)
                pr, mr, pi, mi = re[:64], re[64:128], im[:64], im[64:]
                if k == 0:
                    put(0, pr)
                    put(64, pi, re[128:136])
                    put(128, mr)
                    put(192, mi)
                else:
                    put(256 * k, pr + mr, pr[:8])
                    put(256 * k + 64, pi + mi, mr[:8])
                    put(256 * k + 128, pi - mi, pi[:8])
                    put(256 * k + 192, mr - pr, -mi[:8])
            return 190

        yield _Mat(s_inverse)
        yield settle(ubu)
        yield d_stage(t, lambda c: {0: M_R0T, 1: M_C4T}.get(c, M_RT))
        yield settle(PB)
        z = opaque()
        acc = None
        for r in range(16):
            rows = pl.ds(8 * r, 8)
            t0, t4 = PB[z, rows, :], PB[z, pl.ds(128 + 8 * r, 8), :]
            tk = {}
            for k in (1, 2, 3):
                c, sn = twid[z + 2 * k - 2, rows, :], twid[z + 2 * k - 1, rows, :]
                re = PB[z, pl.ds(256 * k + 8 * r, 8), :]
                im = PB[z, pl.ds(256 * k + 128 + 8 * r, 8), :]
                tk[k] = (re * c - im * sn, re * sn + im * c)
            e0, e1 = t0 + t4, t0 - t4
            s = [e0 + tk[2][0], e1 - tk[2][1], e0 - tk[2][0], e1 + tk[2][1]]
            al, be = tk[1][0] - tk[3][0], tk[1][1] + tk[3][1]
            o = [tk[1][0] + tk[3][0], (al - be) * RSQ2, tk[3][1] - tk[1][1], (al + be) * -RSQ2]
            for b in range(8):
                y = s[b] + o[b] if b < 4 else s[b - 4] - o[b - 4]
                v = X[i][g, pl.ds(128 * b + 8 * r, 8), :] + y
                X[i][n, pl.ds(128 * b + 8 * r, 8), :] = v
                acc = v if acc is None else acc + v
            yield _Step(57, [lambda v=acc: v], delay=5 if r == 15 else 2)
        yield settle(X[i])
        mean = _all_sublanes(acc, jnp.add, 0) * (1.0 / D)
        rstd = yield from ln_rstd(n, i, mean)
        z = opaque()
        for r in range(8):
            v = X[i][n + z, pl.ds(128 * r, 128), :].reshape(16, 8, 128)
            HB[i][n, pl.ds(128 * r, 128), :] = ((v - mean[None]) * rstd[None]).reshape(128, 128).astype(BF16)
            yield _Step(41, [anchor(hbu[i])], delay=1, marks=[name] if r == 7 else [])

    def attend(g, i, name, needs):
        yield _Wait(*needs)
        yield settle(QB[i])
        j, z = g + 4 * i, opaque()
        even = (_iota(8, 0) & 1) == 0
        edge = _iota(8, 1) == 0

        def window(near, far, w, rows):
            return near[j + z + 4 - 2 * w, rows, :] if w <= 2 * i + 2 else far[j + z + 16 - 2 * w, rows, :]

        def mix_values(h, u):
            p = PW[h % 2][opaque()]
            for rows in (pl.ds(256 * h + 16 * u, 16), pl.ds(256 * h + 16 * u + 16, 16)):
                acc = functools.reduce(jnp.add, [p[16 * w:16 * w + 16] * window(VE, VS, w, rows)
                                                 for w in range(8)])
                HB[i][g, rows, :] = acc.astype(BF16)
            return _Step(63, [anchor(hbu[i])], delay=1, marks=[name] if (h, u) == (3, 14) else [])

        for h in range(5):
            logits = []
            for w0 in range(0, 8, 2):
                if h < 4:
                    rows = pl.ds(256 * h, 256)
                    q = QB[i][opaque(), rows, :]
                    for w in (w0, w0 + 1):
                        v = (q * window(KE, KS, w, rows)).reshape(16, 16, 128).sum(0)
                        v = jnp.where(even, v[:8] + pltpu.roll(v[:8], 7, 0), v[8:] + pltpu.roll(v[8:], 1, 0))
                        logits.append(jnp.where(edge & (2 * w > j), -1e9, v * SCALE) if w > 2 * i
                                      else v * SCALE)
                    yield _Step(138, [lambda v=v: v for v in logits[-2:]], delay=2)
                if h > 0:
                    yield mix_values(h - 1, 2 * w0)
                    yield mix_values(h - 1, 2 * w0 + 2)
            if h < 4:
                top = functools.reduce(jnp.maximum, logits)
                e = [jnp.exp(v - top) for v in logits]
                total = functools.reduce(jnp.add, e)
                yield _Step(30, [lambda v=total: v], delay=3)
                scale = 1.0 / total
                for w in range(8):
                    v = e[w] * scale
                    PW[h % 2][0, pl.ds(16 * w, 8), :] = jnp.where(even, v, pltpu.roll(v, 1, 0))
                    PW[h % 2][0, pl.ds(16 * w + 8, 8), :] = jnp.where(even, pltpu.roll(v, 7, 0), v)
                yield _Step(50, [anchor(PW[h % 2])], delay=6 if h == 3 else 1)

    def packed_sums(terms, signs):
        lo = [pltpu.bitcast(u << 16, F32) for u in terms]
        hi = [pltpu.bitcast(u & np.uint32(0xFFFF0000), F32) for u in terms]
        return [pltpu.pack_elementwise([v[p] + v[q] if s > 0 else v[p] - v[q] for v in (lo, hi)],
                                       packed_dtype=BF16) for p, s, q in signs]

    def half(ref, row):
        return lambda r, size, cols: ref[pl.ds(pl.multiple_of(row + r, 8), size), cols]

    kv_weight = (WS5, half(WK, 0), half(WV, 0))
    q_weight = (WQ5, half(WQ, 0), half(WQ, D // 4))
    o_weight = (WP5, half(WP, 0), half(WP, D // 4))

    def left_sums(weight, row, size, needs=()):
        yield _Wait(*needs)
        sums, top, bottom = weight
        for r in range(0, size, 8):
            a = [ref(row + r, 8, pl.ds(c, 512)) for ref in (top, bottom) for c in (0, 512)]
            for e, v in enumerate(packed_sums(a, ((0, 1, 3), (2, 1, 3), (0, 1, 1), (2, -1, 0), (1, -1, 3)))):
                sums[e, pl.ds(pl.multiple_of(row + r, 8), 8), :] = v
            yield _Step(92, delay=2, marks=["sums"] if r == size - 8 else [])

    def right_sums(dst, g, i, name, needs):
        yield _Wait(*needs)
        z = g + opaque()
        for r in range(0, 256, 16):
            b = [hbu[n][z, pl.ds(k + r, 16), :] for k in (0, 256) for n in (i, i + 1)]
            for e, v in enumerate(packed_sums(b, ((0, 1, 3), (1, -1, 3), (2, -1, 0), (0, 1, 1), (2, 1, 3)))):
                dst[e, pl.ds(r, 16), :] = v
            yield _Step(47, [anchor(dst)], delay=SETTLE if r == 240 else 1,
                        marks=[name] if r == 240 else [])

    def strassen(sch, weight, right, g, i, m, store, needs, marks):
        for n in needs:
            sch.run(n)
        sums, top, bottom = weight
        rows = pl.ds(pl.multiple_of(64 * m, 64), 64)
        sch.fresh = True

        def product(left, b):
            head = tied(lambda r: left(32 * m + r, 8, pl.ds(0, 128)), 4, lambda: sch.point(8.0))
            return _dot(_bf(jnp.concatenate([head, left(32 * m, 32, pl.ds(128, 384))], 1)), _bf(b))

        def a(e):
            return lambda r, size, cols: sums[e, pl.ds(pl.multiple_of(r, 8), size), cols]

        def b(e):
            return right[e + opaque()]

        m2 = product(a(1), hbu[i][g + opaque(), pl.ds(0, 256), :])
        m4 = product(lambda r, size, cols: bottom(r, size, pl.ds(512 + cols.start, cols.size)), b(2))
        store(1, i, rows, m2 + m4)
        m1 = product(a(0), b(0))
        c11, c22 = m1 + m4, m1 - m2
        m5 = product(a(2), hbu[i + 1][g + opaque(), pl.ds(256, 256), :])
        c11 = c11 - m5
        store(0, i, rows, c11 + product(a(4), b(4)))
        m3 = product(top, b(1))
        store(0, i + 1, rows, m3 + m5)
        c22 = c22 + m3
        v = product(a(3), b(3))
        store(1, i + 1, rows, c22 + v)
        sch.results.append(v[:8])
        for name in marks:
            sch.done[name] = sch.slot + WAIT

    def kv_proj(sch, g, i, name, needs):
        def store(lower, n, rows, v):
            (KE, VE)[lower][g + 4 * n + 4, rows, :] = v
        for m in range(16):
            strassen(sch, kv_weight, SB[i // 2], g, i, m, store, needs, [name] if m == 15 else [])

    def q_proj(sch, g, i, name, needs):
        def store(lower, n, rows, v):
            QB[n][0, pl.ds(512 * lower + rows.start, 64), :] = v
        for m in range(8):
            strassen(sch, q_weight, SB[i // 2], g, i, m, store, needs, [name] if m == 7 else [])

    def o_proj(sch, g, i, m, needs, marks):
        def store(lower, n, rows, v):
            rows = pl.ds(512 * lower + rows.start, 64)
            X[n][g, rows, :] = X[n][g, rows, :] + v
        strassen(sch, o_weight, SB[2 + i // 2], g, i, m, store, needs, marks)

    def shift_block(g, i, name, needs):
        yield _Wait(*needs)
        j, z = g + 4 * i, opaque()
        for m in range(16):
            rows = pl.ds(64 * m, 64)
            for ref, to in ((KE, KS), (VE, VS)):
                v = pltpu.roll(ref[j + 4 + z, rows, :], 1, 1)
                if ref is VE:
                    v = jnp.where(_iota(64, 1) == 0, ref[4 + z, rows, :], v)
                to[j, rows, :] = v
                if i == 3:
                    ref[g, rows, :] = v
            yield _Step(12, delay=8 if i == 3 else 4, marks=[name] if m == 15 else [])

    def transpose_weight(w, quarters, name):
        for h in quarters:
            for r in range(4):
                v = WRAW[w, pl.ds(256 * r, 256), pl.ds(pl.multiple_of(256 * h, 256), 256)]
                v = pltpu.bitcast(v.T, U32)
                TR[2 * r], TR[2 * r + 1] = v[:, :128], v[:, 128:]
                yield _Step(40, delay=16)
            z = opaque()
            for c in range(8):
                WT[w][pl.ds(pl.multiple_of(128 * h, 128), 128), pl.ds(128 * c, 128)] = jnp.concatenate(
                    [TR[c + z, pl.ds(u, 8, stride=16), :] for u in range(16)], 0)
                yield _Step(20, delay=4, marks=[name] if c == 7 else [])

    def transpose_wo(name):
        for c in range(8):
            for h in range(4):
                v = jnp.concatenate([wou[c, pl.ds(128 * h + u, 8, stride=16), :] for u in range(16)], 0)
                WP[pl.ds(64 * c, 64), pl.ds(256 * h, 256)] = pltpu.bitcast(_bf(v).T, U32)
                yield _Step(20, delay=10, marks=[name] if c == 7 and h == 3 else [])

    def prep_spectral_weights(c2):
        lane = _iota(8, 1)
        order = jnp.where(lane > 64, 192 - lane, lane)

        def words(k2):
            re, im = (wsu[u, k2, pl.ds(c2, 64, stride=4), :] for u in range(2))
            return ((re & np.uint32(0xFFFF)) | (im << 16), (re >> 16) | (im & np.uint32(0xFFFF0000)))

        def arrange(w, below):
            w = jnp.where(_iota(w.shape[0], 1) < 64, w, below)
            return jnp.concatenate([jnp.take_along_axis(w[u:u + 8], order, axis=1)
                                    for u in range(0, w.shape[0], 8)], 0)

        below = words(15)
        for k2 in range(16):
            here = words(k2)
            for e in range(2):
                cl = 2 * c2 + e
                w = arrange(here[e], below[e])
                WS[k2, pl.ds(64 * cl, 64), :] = pltpu.roll(w, 1, 0) if cl > 4 else w
            below = here
            yield _Step(100)
        if c2 == 0:
            def nyquist(k2):
                re, im = (jnp.broadcast_to(WN[u, :, pl.ds(128 * k2, 128)].astype(F32), (8, 128))
                          for u in range(2))
                return pltpu.pack_elementwise([re, im], packed_dtype=BF16)
            for k2 in range(16):
                WS[k2, pl.ds(512, 8), :] = arrange(nyquist(k2), nyquist((k2 + 15) % 16))

    def write_out(p, c, name, needs):
        yield _Wait(*needs)
        rows = pl.ds(pl.multiple_of(128 * c, 128), 128)
        g, i = 2 * p % 4 + opaque(), p // 2
        w = pltpu.pack_elementwise([X[i][g, rows, :], X[i][g + 1, rows, :]], packed_dtype=BF16)
        xru[c, pl.ds(p, 128, stride=8), :] = w.T
        yield _Step(30, marks=[name])

    for c in range(8):
        x_copy(c).start()
    for c in range(5):
        mats[M_R + c] = d_mats[c]

    def make_twiddle(k):
        PB = temps[0][2]
        PB[0, pl.ds(0, 128), :] = lane_vec(L_TWID + k, 128)
        twid[k] = PB[opaque(), pl.ds(0, 128), :].T

    _loop(6, make_twiddle, "make_twiddle")

    def make_dft(j):
        fa, fb = lanes[pl.ds(L_FA, 128), :], lanes[pl.ds(L_FB, 128), :]
        c, sn = lane_vec(L_COS + j, 128), lane_vec(L_SIN + j, 128)
        UB, _, _, ubu, _ = temps[0]
        UB[0, pl.ds(0, 128), :] = (fa * c + fb * sn).astype(BF16)
        UB[0, pl.ds(128, 128), :] = (fb * c - fa * sn).astype(BF16)
        mats[M_FA + j], mats[M_FB + j] = ubu[0, pl.ds(0, 64), :], ubu[0, pl.ds(64, 64), :]

    _loop(NB, make_dft, "make_dft")

    def load_x(c):
        x_copy(c).wait()
        pl.when(c == 5)(lambda: start_all(spec_copies[0]))
        pl.when(c == 7)(lambda: start_all(spec_copies[1]))
        rows = pl.ds(pl.multiple_of(128 * c, 128), 128)
        for p in range(8):
            w = xru[c, pl.ds(p, 128, stride=8), :].T
            for e, bits in enumerate((w << 16, w & np.uint32(0xFFFF0000))):
                g, i = 2 * p % 4 + e, p // 2
                v = pltpu.bitcast(bits, F32)
                X[i][g, rows, :] = v
                v = v.reshape(16, 8, 128)
                mean = _all_sublanes(v.sum(0), jnp.add, 0) * (1.0 / 128)
                STAT[4 * g + i, c] = mean
                STAT[4 * g + i, 8 + c] = _all_sublanes(((v - mean) ** 2).sum(0), jnp.add, 0)

    _loop(8, load_x, "load_x")

    def after(name, action):
        yield _Wait(name)
        action()

    def spectral_weights():
        yield _Wait(("f", 2, 1))
        for c in spec_copies[0] + spec_copies[1]:
            c.wait()
        for c2 in range(4):
            yield from prep_spectral_weights(c2)

    with jax.named_scope("first_forward"):
        sch = _Sched(0.92)
        sch.add(after(("f", 0, 1), w_copies[1].start), "k")
        sch.add(after(("f", 1, 1), w_copies[2].start), "v")
        sch.add(after(("f", 2, 3), w_copies[0].start), "q")
        for g in range(4):
            for i in range(4):
                sch.add(fwd_block(g, i, ("f", g, i), [("f", g - 1, i)] if g else [],
                                  [("r", g - 1)] if g else [], True), ("f", g, i))
            sch.add(group_stage(g, ("r", g), [("f", g, i) for i in range(4)], False), ("r", g))
        sch.add(spectral_weights(), "s")
        sch.drive()
    start_all(wo_copies)

    def keys_values(layer, g):
        sch = _Sched(0.42 if layer == 0 else 0.40)
        nxt = (g + 1) % 4
        sch.add(inv_block(g, 2, ("i", 2), []), ("i", 2))
        sch.add(inv_block(g, 3, ("i", 3), [("read", ("i", 2))]), ("i", 3))
        sch.add(right_sums(SB[1], g, 2, ("b", 2), [("i", 2), ("i", 3)]), ("b", 2))
        sch.add(group_stage(nxt, "r", [("read", ("i", 3))], True), "r")
        sch.add(inv_block(nxt, 0, ("i", 4), ["r", ("i", 2)], n=g + 1), ("i", 4))
        sch.add(inv_block(nxt, 1, ("i", 5), [("read", ("i", 4)), ("i", 3)], n=g + 1), ("i", 5))
        if layer == 0:
            sch.add(transpose_weight(0, [g], "w"), "w")
            sch.add(left_sums(q_weight, 128 * (g % 2), 128, ["w"]), "sums")
        for i in (2, 3):
            sch.add(shift_block((g + 3) % 4, i, ("s", i), []), ("s", i))
        for i in (0, 1):
            sch.add(shift_block(g, i, ("s", i), [("kv", 0)]), ("s", i))
        sch.add(right_sums(SB[0], g + 1, 0, ("b", 4), [("i", 4), ("i", 5), ("kv", 0)]), ("b", 4))
        kv_proj(sch, g, 0, ("kv", 0), [])
        kv_proj(sch, g, 2, ("kv", 2), [("b", 2)])
        sch.finish()

    def mix(g, after, last, write):
        sch = _Sched(0.62)
        tail = after is None
        pace = 0.36 if tail else 0.33 if last else 0.29
        ahead = [(g, 2), (g, 3)] + ([] if tail else [(after, 0), (after, 1)])
        for n, block in enumerate(ahead):
            sch.add(attend(*block, ("a", n), [[], [("a", 0)], [("a", 1), ("q", 0)], [("a", 2)]][n]),
                    ("a", n), pace=pace)
            if n % 2:
                sch.add(right_sums(SB[2 + block[1] // 2], block[0], block[1] - 1, ("b", n),
                                   [("a", n)] + ([("o", 0, 0, "all")] if n == 3 else [])), ("b", n))
        for i in () if tail else (0, 2):
            sch.add(right_sums(SB[i // 2], after, i, ("h", i), [("q", 0)] if i else []), ("h", i))
        if not last:
            sch.add(group_stage((g + 3) % 4, "r", [], False), "r")
            for i in range(4):
                sch.add(fwd_block(g, i, ("f", i), [("o", i - i % 2, 7)], ["r"]), ("f", i))
        now = 6 if last else 8
        for i in range(4 if write else 0):
            for c in (0, 4, 1, 5, 2, 6):
                sch.add(write_out(2 * i + g // 2, c, ("w", i, c), [("o", i - i % 2, 2 * (c % 4) + 1)]),
                        ("w", i, c))
        for i in (0, 2):
            for m in range(now):
                o_proj(sch, g, i, m, [("b", 1)] if i else [],
                       [("o", i, m)] + ([("o", i, 0, "all")] if m == now - 1 else []))
            if not tail:
                q_proj(sch, after, i, ("q", i), [("h", i)])
        if tail and not last:
            sch.add(group_stage(g, "s", [("f", i) for i in range(4)], False), "s")
        sch.share = 0.92
        sch.drive()

    def postponed():
        sch = _Sched(0.5)
        pairs = [(g, i) for g in range(4) for i in (0, 2)]
        for n, (g, i) in enumerate(pairs):
            sch.add(right_sums(SB[2 + i // 2], g, i, ("b", n), [("o", n - 2)] if n >= 2 else []), ("b", n))
            for c in (3, 7) if g % 2 else ():
                for e in (i, i + 1):
                    sch.add(write_out(2 * e + g // 2, c, ("w", n, c, e), [("o", n)]), ("w", n, c, e))
        for n, (g, i) in enumerate(pairs):
            for m in (6, 7):
                o_proj(sch, g, i, m, [("b", n)], [("o", n)] if m == 7 else [])
        sch.finish()

    def spectral_and_weights(h):
        for _ in transpose_weight(1, [h], None):
            pass
        spectral_rows(h)
        for _ in transpose_weight(2, [h], None):
            pass
        for _ in left_sums(kv_weight, 128 * h, 128):
            pass

    for layer in range(2):
        with jax.named_scope("spectral"):
            if layer == 0:
                w_copies[1].wait()
                w_copies[2].wait()
                _loop(4, spectral_and_weights, "rows")
            else:
                _loop(4, spectral_rows, "rows")
            spectral(512, 8)
        sch = _Sched(0.92)
        sch.add(group_stage(0, "r", [], True), "r")
        sch.add(inv_block(0, 0, ("i", 0), ["r"]), ("i", 0))
        sch.add(inv_block(0, 1, ("i", 1), ["r"]), ("i", 1))
        sch.add(right_sums(SB[0], 0, 0, "b", [("i", 0), ("i", 1)]), "b")
        sch.drive()
        if layer == 0:
            w_copies[0].wait()
        _loop(4, lambda g: keys_values(layer, g), "keys_values")
        sch = _Sched(0.62)
        sch.add(right_sums(SB[0], 0, 0, ("h", 0), []), ("h", 0))
        sch.add(right_sums(SB[1], 0, 2, ("h", 2), []), ("h", 2))
        sch.add(shift_block(3, 2, "s", []), "s")
        sch.add(attend(0, 0, ("a", 0), ["q"]), ("a", 0), pace=0.4)
        sch.add(attend(0, 1, ("a", 1), [("a", 0)]), ("a", 1), pace=0.4)
        sch.add(right_sums(SB[2], 0, 0, "b", [("a", 1)]), "b")
        sch.add(shift_block(3, 3, "t", []), "t")
        if layer == 0:
            for c in wo_copies:
                c.wait()
            sch.add(transpose_wo("w"), "w")
            sch.add(left_sums(o_weight, 0, 256, ["w"]), "sums")
        q_proj(sch, 0, 0, "q", [("h", 0)])
        q_proj(sch, 0, 2, None, [("h", 2)])
        sch.finish()
        if layer == 0:
            _loop(3, lambda g: mix(g, g + 1, False, False), "mix")
            mix(3, None, False, False)
        else:
            _loop(2, lambda u: mix(2 * u, 2 - u, True, False), "mix")
            mix(1, 3, True, True)
            mix(3, None, True, True)
    for c in (0, 1, 2, 4, 5, 6):
        out_copy(c).start()
    with jax.named_scope("postponed"):
        postponed()
    for c in (3, 7):
        out_copy(c).start()
    for c in range(8):
        out_copy(c).wait()


@jax.jit
def pallas_interleave_layers__spectral_gfnet__sliding_local_dilated__prompt_kernel(
    A_x: jax.Array,
    A_w_r: jax.Array,
    A_w_i: jax.Array,
    B_x: jax.Array,
    B_wqkv: jax.Array,
    B_wo: jax.Array,
):
    del B_x
    hbm = pl.BlockSpec(memory_space=pl.ANY)
    smem = pl.BlockSpec(memory_space=pltpu.SMEM)
    out = pl.pallas_call(
        _kernel,
        out_shape=jax.ShapeDtypeStruct((S, D), BF16),
        in_specs=[smem, smem, pl.BlockSpec(), pl.BlockSpec(), hbm, hbm, hbm, hbm, hbm],
        out_specs=hbm,
        scratch_shapes=[
            pltpu.VMEM((37, 64, 128), U32),
            pltpu.VMEM((6, 128, 128), F32),
            pltpu.VMEM((NB, 16, 8, 128), F32),
            pltpu.VMEM((NB + 4, D, 128), F32),
            pltpu.VMEM((NB + 4, D, 128), F32),
            pltpu.VMEM((NB, D, 128), F32),
            pltpu.VMEM((NB, D, 128), F32),
            pltpu.VMEM((2 * NB + 1, ZR, 128), F32),
            pltpu.VMEM((9, ZR, 128), F32),
            pltpu.VMEM((NB, ZR, 128), U32),
            *4 * [pltpu.VMEM((D // 2, D), U32)],
            pltpu.VMEM((5, D // 2, D // 2), U32),
            *2 * [pltpu.VMEM((5, D // 4, D // 2), U32)],
            *4 * [pltpu.VMEM((5, D // 4, 128), U32)],
            pltpu.VMEM((8, S, 128), BF16),
            pltpu.VMEM((2, NB, D // 2, 128), BF16),
            pltpu.VMEM((2, 1, S), BF16),
            pltpu.VMEM((3, D, D), BF16),
            pltpu.VMEM((8, D, 128), BF16),
            pltpu.VMEM((8, 128, 128), U32),
            pltpu.VMEM((1, 128, 128), F32),
            pltpu.VMEM((1, 128, 128), F32),
            pltpu.SemaphoreType.DMA((24,)),
        ] + 4 * [
            pltpu.VMEM((5, D, 128), F32),
            pltpu.VMEM((5, D, 128), BF16),
            pltpu.VMEM((1, D, 128), F32),
            pltpu.VMEM((1, D, 128), BF16),
            pltpu.VMEM((1, 1152, 128), BF16),
            pltpu.VMEM((1, D, 128), F32),
        ],
        compiler_params=pltpu.CompilerParams(vmem_limit_bytes=124 * 2 ** 20),
    )(_ZERO, _ROT, _MATS, _LANES, A_x.reshape(S, D), A_w_r.T, A_w_i.T, B_wqkv, B_wo)
    return out.reshape(1, S, D)
```

```python
import functools

import numpy as np

import jax
import jax.numpy as jnp
import jax.experimental.pallas as pl
import jax.experimental.pallas.tpu as pltpu

S, D, NB = 2048, 1024, 16
ZR = 576
F32, BF16, U32, I32 = jnp.float32, jnp.bfloat16, jnp.uint32, jnp.int32
EPS = 1e-5
SCALE = 32 ** -0.5
RSQ2 = float(np.sqrt(0.5))
WAIT = 24
GRAIN = 1
SETTLE = 6
LAG = 3

_S_ROWS = [(32 * u, 32) for u in range(16)] + [(512, 8)]

M_FA, M_FB, M_R, M_C4, M_RT, M_C4T, M_R0T = 0, 16, 32, 33, 34, 35, 36
L_MU, L_NU, L_KU, L_KV, L_COS, L_SIN, L_TWID, L_FA, L_FB = 0, 16, 32, 48, 64, 80, 96, 104, 232


def _bf16_bits(a):
    u = np.ascontiguousarray(a, dtype=np.float32).view(np.uint32).astype(np.uint64)
    return ((u + 0x7FFF + ((u >> 16) & 1)) >> 16).astype(np.uint32)


def _constants():
    a = np.arange(128)
    k1 = np.arange(64)
    alt = (-1.0) ** a
    lanes = np.zeros((L_FB + 128, 128))
    t = 2 * np.pi * np.outer(a, k1) / 128
    fa = np.concatenate([np.cos(t), -np.sin(t)], 1)
    fb = np.concatenate([np.sin(t), -np.cos(t)], 1)
    fa[:, 0], fb[:, 0] = RSQ2, -RSQ2
    fa[:, 64], fb[:, 64] = alt, 0.0
    lanes[L_FA:L_FA + 128], lanes[L_FB:L_FB + 128] = fa, fb
    for j in range(NB):
        ang = 2 * np.pi * j / 32 + np.pi / 32
        p, q = (_bf16_bits([np.cos(ang), np.sin(ang)]) << 16).view(np.float32).astype(np.float64)
        turn = 2 * np.pi * j * np.tile(k1, 2) / S
        lanes[L_COS + j], lanes[L_SIN + j] = np.cos(turn), np.repeat([-1.0, 1.0], 64) * np.sin(turn)
        lanes[L_COS + j, 64], lanes[L_SIN + j, 64] = p, q
        lanes[L_MU + j, 0], lanes[L_MU + j, 64] = 1.0, (q / p + p / q) / 2
        lanes[L_NU + j, 0], lanes[L_NU + j, 64] = 0.0, (q / p - p / q) / 2
        lanes[L_KU + j, 0], lanes[L_KU + j, 64] = 1.0, q / p
        lanes[L_KV + j, 0], lanes[L_KV + j, 64] = 1.0, p / q
    for k in (1, 2, 3):
        lanes[L_TWID + 2 * k - 2] = np.cos(2 * np.pi * a * k / D)
        lanes[L_TWID + 2 * k - 1] = np.sin(2 * np.pi * a * k / D)
    th = 2 * np.pi * np.outer(k1, a) / 128
    r = np.concatenate([np.cos(th), -np.sin(th)], 0)
    r[64] = alt
    th = 2 * np.pi * np.outer(2 * k1 + 1, a) / 256
    c4 = np.concatenate([np.cos(th), -np.sin(th)], 0)
    inv = 2.0 / (S * D)
    r0t = inv * r.T
    r0t[:, 0::64] *= 0.5
    rows = np.arange(128).reshape(2, 4, 16).transpose(1, 0, 2).ravel()
    bits = _bf16_bits(np.stack([r[rows], c4[rows], inv * r.T, inv * c4.T, r0t]))
    ang = 2 * np.pi * np.outer(np.arange(4), np.arange(4)).ravel() / 16
    rot = np.concatenate([np.cos(ang), np.sin(ang)]).astype(np.float32)
    return bits[:, 0::2] | (bits[:, 1::2] << 16), lanes.astype(np.float32), rot


_MATS, _LANES, _ROT = _constants()
_ZERO = np.zeros((1,), np.int32)


class _Step:
    def __init__(self, cost, anchors=(), delay=0, marks=()):
        self.cost, self.anchors, self.delay, self.marks = cost, list(anchors), delay, list(marks)


class _Wait:
    def __init__(self, *names):
        self.names = names


class _Mat:
    def __init__(self, emit):
        self.emit = emit


class _Hold:
    def __init__(self, store):
        self.store = store


class _Task:
    def __init__(self, gen, pace):
        self.gen, self.pace, self.blocked, self.not_before, self.held = gen, pace, (), 0, None
        self.allowed = 0.0


class _Sched:
    def __init__(self, share=0.0):
        self.share = share
        self.tasks, self.done, self.producer = [], {}, {}
        self.slot, self.credit, self.anchors, self.results = 0, 0.0, [], []
        self.fresh = False

    def add(self, gen, name, pace=99):
        self.producer[name] = self.producer["read", name] = _Task(gen, pace)
        self.tasks.append(self.producer[name])

    def _ready(self, t):
        return t.not_before <= self.slot and all(
            n in self.done and self.done[n] <= self.slot for n in t.blocked)

    def _advance(self, t, mats=True):
        item, t.held = t.held or next(t.gen, None), None
        if item is None:
            self.tasks.remove(t)
        elif isinstance(item, _Wait):
            t.blocked = item.names
        elif isinstance(item, _Hold):
            if len(self.results) >= LAG:
                item.store(self.results[-LAG])
        elif isinstance(item, _Mat):
            if mats:
                t.not_before = float("inf")
                self.fresh = False
                self.credit -= item.emit(lambda: self.point(0.0)) or 0
                t.not_before = self.slot + WAIT
            else:
                t.held, t.not_before = item, self.slot + 1
        else:
            t.blocked = ()
            t.not_before = self.slot + item.delay
            self.credit -= item.cost
            self.anchors += item.anchors
            for n in item.marks:
                self.done[n] = self.slot + item.delay
            return True

    def run(self, *names):
        while not all(n in self.done for n in names):
            for n in names:
                if n not in self.done:
                    for b in self.producer[n].blocked:
                        self.run(b)
                    self._advance(self.producer[n])

    def drive(self):
        while self.tasks:
            ready = [t for t in self.tasks if self._ready(t)]
            if not ready:
                self.slot += 1
                continue
            self.anchors, self.credit = self.anchors[-2:], 0.0
            self._advance(next((t for t in ready if t.held), ready[0]))
            self.slot -= min(self.credit, 0.0) / 60

    def finish(self):
        self.run(*[n for n in self.producer if n[0] != "read"])

    def point(self, own):
        for t in self.tasks:
            t.allowed = min(t.allowed, 0.0) + t.pace
        while True:
            t = next((t for t in self.tasks if self._ready(t) and t.allowed > 0
                      and self.credit > 0), None)
            if t is None:
                break
            if self._advance(t, self.fresh):
                t.allowed -= 1
        anchors, self.anchors = self.anchors, []
        self.credit = min(self.credit, 10.0) + 64 * self.share - own
        self.fresh = False
        self.slot += 1
        return anchors


def _dot(a, b):
    return jnp.dot(a, b, preferred_element_type=F32)


def _dot_t(a, b):
    return jax.lax.dot_general(a, b, (((1,), (1,)), ((), ())), preferred_element_type=F32)


def _bf(u):
    return pltpu.bitcast(u, BF16)


def _iota(rows, dim):
    return jax.lax.broadcasted_iota(I32, (rows, 128), dim)


def _radix4(z, inverse):
    (r0, i0), (r1, i1), (r2, i2), (r3, i3) = z
    ar, ai, cr, ci = r0 + r2, i0 + i2, r0 - r2, i0 - i2
    br, bi, dr, di = r1 + r3, i1 + i3, r1 - r3, i1 - i3
    lo, hi = (cr + di, ci - dr), (cr - di, ci + dr)
    if inverse:
        lo, hi = hi, lo
    return [(ar + br, ai + bi), lo, (ar - br, ai - bi), hi]


def _all_sublanes(v, op, axis):
    for sh in (4, 2, 1):
        v = op(v, pltpu.roll(v, sh, axis))
    return v


def _loop(n, body, name):
    def step(i, carry):
        body(i)
        return carry
    with jax.named_scope(name):
        jax.lax.fori_loop(0, n, step, 0)


def _kernel(zero_ref, rot, d_mats, lanes, x_hbm, wr_hbm, wi_hbm, wqkv_hbm, wo_hbm, out_hbm,
            mats, twid, STAT, KE, VE, KS, VS, Z, ZT, WS, WQ, WK, WV, WP, WS5, WQ5, WP5, SB0, SB1, SB2, SB3, XR, WRI, WN, WRAW, WO, TR, PW0, PW1, sems, *split):
    zero = zero_ref[0]
    never = zero != 0
    X, HB, QB = split[0::6], split[1::6], split[2::6]
    hbu = [r.bitcast(U32) for r in HB]
    xru, wsu, wou = XR.bitcast(U32), WRI.bitcast(U32), WO.bitcast(U32)
    temps = [(ub, ab, pb, ub.bitcast(U32), ab.bitcast(U32))
             for ub, ab, pb in zip(split[3::6], split[4::6], split[5::6])]
    PW, SB, WT = (PW0, PW1), (SB0, SB1, SB2, SB3), (WQ, WK, WV, WP)
    counter = [0]

    def opaque():
        counter[0] += 1
        return zero * counter[0]

    def anchor(ref):
        return lambda: ref[0, pl.ds(pl.multiple_of(zero * 8, 8), 8), pl.ds(0, 128)]

    def settle(ref):
        return _Step(2, [anchor(ref)], delay=SETTLE)

    def hold(ref, spare, row=0):
        def store(v):
            ref[spare, pl.ds(pl.multiple_of(row + zero * 8, 8), 8), :] = v
        return _Hold(store)

    def tied(load, vregs, point):
        parts = []
        for r in range(vregs):
            anchors = [a for _ in range(GRAIN) for a in point()] if r % GRAIN == 0 else []
            u = load(8 * r)
            for a in anchors:
                u = jnp.where(never, pltpu.bitcast(a(), U32), u)
            parts.append(u)
        return jnp.concatenate(parts, 0)

    def mat(i):
        return _bf(mats[i])

    def d_stage(t, which):
        UB, AB, PB, ubu, abu = temps[t]

        def emit(point):
            z = opaque()
            for c in range(8):
                lhs = mat(which(c) + opaque()) if c % 4 else _bf(
                    tied(lambda r, u=which(c) + opaque(): mats[u, pl.ds(r, 8), :], 8, point))
                PB[0, pl.ds(128 * c, 128), :] = _dot(lhs, _bf(ubu[z, pl.ds(64 * c, 64), :]))
        return _Mat(emit)

    def lane_vec(i, rows):
        return jnp.broadcast_to(lanes[pl.ds(i, 1), :], (rows, 128))

    def x_copy(c):
        return pltpu.make_async_copy(
            x_hbm.at[:, pl.ds(pl.multiple_of(128 * c, 128), 128)], XR.at[c], sems.at[c])

    def out_copy(c):
        return pltpu.make_async_copy(
            XR.at[c], out_hbm.at[:, pl.ds(pl.multiple_of(128 * c, 128), 128)], sems.at[8 + c])

    spec_copies = [[pltpu.make_async_copy(w.at[pl.ds(0, 512), pl.ds(128 * k2, 128)], WRI.at[u, k2],
                                          sems.at[16 + u]) for k2 in range(16)]
                   + [pltpu.make_async_copy(w.at[pl.ds(512, 1), :], WN.at[u], sems.at[22 + u])]
                   for u, w in enumerate((wr_hbm, wi_hbm))]

    def start_all(copies):
        for c in copies:
            c.start()
    w_copies = [pltpu.make_async_copy(wqkv_hbm.at[:, pl.ds(D * w, D)], WRAW.at[w], sems.at[18 + w])
                for w in range(3)]
    wo_copies = [pltpu.make_async_copy(wo_hbm.at[:, pl.ds(128 * c, 128)], WO.at[c], sems.at[21])
                 for c in range(8)]

    def ln_rstd(g, i, mean):
        acc, m = None, g + opaque()
        for r in range(8):
            d = X[i][m, pl.ds(128 * r, 128), :].reshape(16, 8, 128) - mean[None]
            v = (d * d).sum(0)
            acc = v if acc is None else acc + v
            if r < 7:
                yield _Step(50, [lambda acc=acc: acc], delay=3)
        rstd = jax.lax.rsqrt(_all_sublanes(acc, jnp.add, 0) * (1.0 / D) + EPS)
        yield _Step(50, delay=8)
        yield _Step(10, [lambda: rstd], delay=1)
        return rstd

    def fwd_block(g, i, name, needs, free=(), known=False):
        j, t = g + 4 * i, i
        UB, AB, PB, ubu, abu = temps[t]
        yield _Wait(*needs)
        if known:
            means, squares = STAT[4 * g + i, pl.ds(0, 8)], STAT[4 * g + i, pl.ds(8, 8)]
            mean = means.sum(0) * 0.125
            var = (squares.sum(0) + 128.0 * ((means - mean) ** 2).sum(0)) * (1.0 / D)
            rstd = jax.lax.rsqrt(var + EPS)
            yield _Step(50, delay=6)
        else:
            yield settle(X[i])
            acc, m = None, g + opaque()
            for r in range(8):
                v = X[i][m, pl.ds(128 * r, 128), :].reshape(16, 8, 128).sum(0)
                acc = v if acc is None else acc + v
                if r % 2:
                    yield _Step(35, [lambda acc=acc: acc], delay=7 if r == 7 else 3)
            mean = _all_sublanes(acc, jnp.add, 0) * (1.0 / D)
            rstd = yield from ln_rstd(g, i, mean)
        mean8, rstd = (jnp.concatenate([v, v], 0) for v in (mean * 8.0, rstd))
        z = opaque()
        for r in range(8):
            rows = pl.ds(16 * r, 16)
            x = [X[i][g + z, pl.ds(128 * b + 16 * r, 16), :] for b in range(8)]
            s = [x[b] + x[b + 4] for b in range(4)]
            d = [x[b] - x[b + 4] for b in range(4)]
            e, o = s[0] + s[2], s[1] + s[3]
            UB[0, rows, :] = ((e + o - mean8) * rstd).astype(BF16)
            UB[0, pl.ds(128 + 16 * r, 16), :] = ((e - o) * rstd).astype(BF16)
            t1, t2 = (d[1] - d[3]) * RSQ2, (d[1] + d[3]) * RSQ2
            u = {1: (d[0] + t1, d[2] + t2), 2: (s[0] - s[2], s[1] - s[3]), 3: (d[0] - t1, d[2] - t2)}
            yield _Step(34, [anchor(ubu)], delay=1)
            for k in (1, 2, 3):
                c, sn = twid[z + 2 * k - 2, rows, :] * rstd, twid[z + 2 * k - 1, rows, :] * rstd
                re, m = u[k]
                if k == 3:
                    ur, ui = re * c + m * sn, m * c - re * sn
                else:
                    ur, ui = re * c - m * sn, m * c + re * sn
                UB[0, pl.ds(256 * k + 16 * r, 16), :] = ur.astype(BF16)
                UB[0, pl.ds(256 * k + 128 + 16 * r, 16), :] = ui.astype(BF16)
                yield _Step(26, [anchor(ubu)], delay=1)
        yield settle(ubu)

        def d_forward(point):
            z = opaque()
            first = _iota(8, 0) == 0

            def stage(c):
                u = (M_C4 if c == 1 else M_R) + opaque()
                lhs = mat(u) if c % 4 else _bf(tied(lambda r: mats[u, pl.ds(r, 8), :], 8, point))
                v = _dot(lhs, _bf(ubu[z, pl.ds(64 * c, 64), :]))
                return [(v[32 * u:32 * u + 16], v[32 * u + 16:32 * u + 32]) for u in range(4)]

            def put(row, u, v, v0=None):
                if u == 0 and v0 is not None:
                    v = jnp.concatenate([jnp.where(first, v0, v[:8]), v[8:]], 0)
                AB[0, pl.ds(row + 16 * u, 16), :] = v.astype(BF16)

            for u, (p1, p2) in enumerate(stage(0)):
                put(0, u, p1)
                put(528, u, p2, 0.0)
                if u == 0:
                    put(512, 0, jnp.zeros_like(p2), p2[:8])
            for u, (p1, p2) in enumerate(stage(1)):
                put(256, u, p1)
                put(528 + 256, u, p2)
            for k in (1, 2, 3):
                for u, ((p1, p2), (q1, q2)) in enumerate(zip(stage(2 * k), stage(2 * k + 1))):
                    if k == 3:
                        pr, pi, mr, mi = p1 - q2, p2 + q1, p1 + q2, p2 - q1
                        pi0, mi0 = q1[:8], -q2[:8]
                    else:
                        pr, pi, mr, mi = p1 + q2, p2 - q1, p1 - q2, p2 + q1
                        pi0, mi0 = -q1[:8], q2[:8]
                    put(64 * k, u, pr, p1[:8])
                    put(64 * (8 - k), u, mr, p2[:8])
                    put(528 + 64 * k, u, pi, pi0)
                    put(528 + 64 * (8 - k), u, mi, mi0)
            return 190

        yield _Mat(d_forward)
        yield settle(abu)
        yield _Wait(*free)

        def s_forward(point):
            z = opaque()
            fa, fb = mat(M_FA + j + z), mat(M_FB + j + z)
            for r0, rn in ((0, 256), (256, 272)):
                lhs = abu[z, pl.ds(r0 // 2, rn // 2), :] if r0 else tied(
                    lambda r: abu[z, pl.ds(r, 8), :], 16, point)
                u = _dot(_bf(lhs), fa)
                v = _dot(_bf(abu[z, pl.ds(264 + r0 // 2, 128), :]), fb)
                re, m = u[:256] + v, u[:256] - v
                if r0:
                    re, m = (jnp.concatenate([a, u[256:264]], 0) for a in (re, m))
                rn = re.shape[0]
                edge = (_iota(rn, 1) & 63) == 0
                ZT[2 * i, pl.ds(r0, rn), :] = re
                ZT[2 * i + 1, pl.ds(r0, rn), :] = jnp.where(
                    edge, lane_vec(L_MU + j, rn) * m + lane_vec(L_NU + j, rn) * re, pltpu.roll(m, 64, 1))
            return 400

        yield _Mat(s_forward)
        yield _Step(2, [anchor(ZT)], delay=SETTLE, marks=[name])

    def group_stage(g, name, needs, inverse):
        yield _Wait(*needs)

        def turn(z, k):
            if k == 0:
                return z
            c, s = rot[4 * g + k], rot[16 + 4 * g + k]
            if inverse:
                return z[0] * c - z[1] * s, z[1] * c + z[0] * s
            return z[0] * c + z[1] * s, z[1] * c - z[0] * s

        (src, a), (dst, b) = ((Z, 8 * g), (ZT, 0)) if inverse else ((ZT, opaque()), (Z, 8 * g))
        for r in range(65):
            if r % 4 == 0:
                yield hold(src, 2 * NB if inverse else 8)
            rows = pl.ds(8 * r, 8)
            z = [(src[a + 2 * i, rows, :], src[a + 2 * i + 1, rows, :]) for i in range(4)]
            if inverse:
                z = _radix4([turn(z[k], k) for k in range(4)], True)
            else:
                z = [turn(v, k) for k, v in enumerate(_radix4(z, False))]
            for i in range(4):
                dst[b + 2 * i, rows, :], dst[b + 2 * i + 1, rows, :] = z[i]
            yield _Step(35, [anchor(dst)], delay=1, marks=[name] if r == 64 else [])

    def spectral(row, size):
        rows = pl.ds(row, size)
        for k0 in range(4):
            z = _radix4([(Z[8 * g + 2 * k0, rows, :], Z[8 * g + 2 * k0 + 1, rows, :])
                         for g in range(4)], False)
            y = []
            for k1, (re, im) in enumerate(z):
                w = WS[k0 + 4 * k1, rows, :]
                wr = pltpu.bitcast(w << 16, F32)
                wi = pltpu.bitcast(w & np.uint32(0xFFFF0000), F32)
                y.append((re * wr - im * wi, re * wi + im * wr))
            y = _radix4(y, True)
            for g in range(4):
                Z[8 * g + 2 * k0, rows, :], Z[8 * g + 2 * k0 + 1, rows, :] = y[g]

    def spectral_rows(c2):
        for r in range(8):
            spectral(pl.multiple_of(128 * c2 + 16 * r, 16), 16)

    def inv_block(g, i, name, needs, n=None):
        j, t = g + 4 * i, i % 2
        UB, AB, PB, ubu, abu = temps[t]
        n = g if n is None else n
        z = opaque()
        yield _Wait(*needs)
        for r0, rn in _S_ROWS:
            if r0 == 0:
                yield hold(ZT, 8)
            re, im = ZT[z + 2 * i, pl.ds(r0, rn), :], ZT[z + 2 * i + 1, pl.ds(r0, rn), :]
            edge = (_iota(rn, 1) & 63) == 0
            rolled = pltpu.roll(im, 64, 1)
            u = re + jnp.where(edge, lane_vec(L_KU + j, rn) * im, rolled)
            if r0 < 512:
                v = re - jnp.where(edge, lane_vec(L_KV + j, rn) * im, rolled)
                AB[0, pl.ds(r0, rn), :] = u.astype(BF16)
                AB[0, pl.ds(528 + r0, rn), :] = v.astype(BF16)
            else:
                AB[0, pl.ds(512, 16), :] = jnp.concatenate([u, jnp.zeros_like(u)], 0).astype(BF16)
            yield _Step(rn, [anchor(abu)], delay=1, marks=[("read", name)] if r0 == 512 else [])
        yield settle(abu)

        def s_inverse(point):
            z = opaque()
            fa, fb = mat(M_FA + j + z), mat(M_FB + j + z)
            first = _iota(8, 0) == 0

            def put(row, v, v0=None):
                if v0 is not None:
                    v = jnp.concatenate([jnp.where(first, v0, v[:8]), v[8:]], 0)
                UB[0, pl.ds(row, 64), :] = v.astype(BF16)

            for k in range(4):
                lo, hi = 32 * k, 32 * (8 - k if k else 4)
                a = [abu[z, pl.ds(lo, 32), :], abu[z, pl.ds(hi, 32), :]] if k % 2 else [
                    tied(lambda r, o=o: abu[z, pl.ds(o + r, 8), :], 4, point) for o in (lo, hi)]
                if k == 0:
                    a.append(abu[z, pl.ds(256, 8), :])
                re = _dot_t(_bf(jnp.concatenate(a, 0)), fa)
                im = _dot_t(_bf(jnp.concatenate(
                    [abu[z, pl.ds(264 + lo, 32), :], abu[z, pl.ds(264 + hi, 32), :]], 0)), fb)
                pr, mr, pi, mi = re[:64], re[64:128], im[:64], im[64:]
                if k == 0:
                    put(0, pr)
                    put(64, pi, re[128:136])
                    put(128, mr)
                    put(192, mi)
                else:
                    put(256 * k, pr + mr, pr[:8])
                    put(256 * k + 64, pi + mi, mr[:8])
                    put(256 * k + 128, pi - mi, pi[:8])
                    put(256 * k + 192, mr - pr, -mi[:8])
            return 190

        yield _Mat(s_inverse)
        yield settle(ubu)
        yield d_stage(t, lambda c: {0: M_R0T, 1: M_C4T}.get(c, M_RT))
        yield settle(PB)
        z = opaque()
        acc = None
        for r in range(16):
            rows = pl.ds(8 * r, 8)
            t0, t4 = PB[z, rows, :], PB[z, pl.ds(128 + 8 * r, 8), :]
            tk = {}
            for k in (1, 2, 3):
                c, sn = twid[z + 2 * k - 2, rows, :], twid[z + 2 * k - 1, rows, :]
                re = PB[z, pl.ds(256 * k + 8 * r, 8), :]
                im = PB[z, pl.ds(256 * k + 128 + 8 * r, 8), :]
                tk[k] = (re * c - im * sn, re * sn + im * c)
            e0, e1 = t0 + t4, t0 - t4
            s = [e0 + tk[2][0], e1 - tk[2][1], e0 - tk[2][0], e1 + tk[2][1]]
            al, be = tk[1][0] - tk[3][0], tk[1][1] + tk[3][1]
            o = [tk[1][0] + tk[3][0], (al - be) * RSQ2, tk[3][1] - tk[1][1], (al + be) * -RSQ2]
            for b in range(8):
                y = s[b] + o[b] if b < 4 else s[b - 4] - o[b - 4]
                v = X[i][g, pl.ds(128 * b + 8 * r, 8), :] + y
                X[i][n, pl.ds(128 * b + 8 * r, 8), :] = v
                acc = v if acc is None else acc + v
            yield _Step(57, [lambda v=acc: v], delay=5 if r == 15 else 2)
        yield settle(X[i])
        mean = _all_sublanes(acc, jnp.add, 0) * (1.0 / D)
        rstd = yield from ln_rstd(n, i, mean)
        z = opaque()
        for r in range(8):
            v = X[i][n + z, pl.ds(128 * r, 128), :].reshape(16, 8, 128)
            HB[i][n, pl.ds(128 * r, 128), :] = ((v - mean[None]) * rstd[None]).reshape(128, 128).astype(BF16)
            yield _Step(41, [anchor(hbu[i])], delay=1, marks=[name] if r == 7 else [])

    def attend(g, i, name, needs):
        yield _Wait(*needs)
        yield settle(QB[i])
        j, z = g + 4 * i, opaque()
        even = (_iota(8, 0) & 1) == 0
        edge = _iota(8, 1) == 0

        def window(near, far, w, rows):
            return near[j + z + 4 - 2 * w, rows, :] if w <= 2 * i + 2 else far[j + z + 16 - 2 * w, rows, :]

        def mix_values(h, u):
            p = PW[h % 2][opaque()]
            for rows in (pl.ds(256 * h + 16 * u, 16), pl.ds(256 * h + 16 * u + 16, 16)):
                acc = functools.reduce(jnp.add, [p[16 * w:16 * w + 16] * window(VE, VS, w, rows)
                                                 for w in range(8)])
                HB[i][g, rows, :] = acc.astype(BF16)
            return _Step(63, [anchor(hbu[i])], delay=1, marks=[name] if (h, u) == (3, 14) else [])

        for h in range(5):
            logits = []
            for w0 in range(0, 8, 2):
                if h < 4:
                    rows = pl.ds(256 * h, 256)
                    q = QB[i][opaque(), rows, :]
                    for w in (w0, w0 + 1):
                        v = (q * window(KE, KS, w, rows)).reshape(16, 16, 128).sum(0)
                        v = jnp.where(even, v[:8] + pltpu.roll(v[:8], 7, 0), v[8:] + pltpu.roll(v[8:], 1, 0))
                        logits.append(jnp.where(edge & (2 * w > j), -1e9, v * SCALE) if w > 2 * i
                                      else v * SCALE)
                    yield _Step(138, [lambda v=v: v for v in logits[-2:]], delay=2)
                if h > 0:
                    yield mix_values(h - 1, 2 * w0)
                    yield mix_values(h - 1, 2 * w0 + 2)
            if h < 4:
                top = functools.reduce(jnp.maximum, logits)
                e = [jnp.exp(v - top) for v in logits]
                total = functools.reduce(jnp.add, e)
                yield _Step(30, [lambda v=total: v], delay=3)
                scale = 1.0 / total
                for w in range(8):
                    v = e[w] * scale
                    PW[h % 2][0, pl.ds(16 * w, 8), :] = jnp.where(even, v, pltpu.roll(v, 1, 0))
                    PW[h % 2][0, pl.ds(16 * w + 8, 8), :] = jnp.where(even, pltpu.roll(v, 7, 0), v)
                yield _Step(50, [anchor(PW[h % 2])], delay=6 if h == 3 else 1)

    def packed_sums(terms, signs):
        lo = [pltpu.bitcast(u << 16, F32) for u in terms]
        hi = [pltpu.bitcast(u & np.uint32(0xFFFF0000), F32) for u in terms]
        return [pltpu.pack_elementwise([v[p] + v[q] if s > 0 else v[p] - v[q] for v in (lo, hi)],
                                       packed_dtype=BF16) for p, s, q in signs]

    def half(ref, row):
        return lambda r, size, cols: ref[pl.ds(pl.multiple_of(row + r, 8), size), cols]

    kv_weight = (WS5, half(WK, 0), half(WV, 0))
    q_weight = (WQ5, half(WQ, 0), half(WQ, D // 4))
    o_weight = (WP5, half(WP, 0), half(WP, D // 4))

    def left_sums(weight, row, size, needs=()):
        yield _Wait(*needs)
        sums, top, bottom = weight
        for r in range(0, size, 8):
            a = [ref(row + r, 8, pl.ds(c, 512)) for ref in (top, bottom) for c in (0, 512)]
            for e, v in enumerate(packed_sums(a, ((0, 1, 3), (2, 1, 3), (0, 1, 1), (2, -1, 0), (1, -1, 3)))):
                sums[e, pl.ds(pl.multiple_of(row + r, 8), 8), :] = v
            yield _Step(92, delay=2, marks=["sums"] if r == size - 8 else [])

    def right_sums(dst, g, i, name, needs):
        yield _Wait(*needs)
        z = g + opaque()
        for r in range(0, 256, 16):
            b = [hbu[n][z, pl.ds(k + r, 16), :] for k in (0, 256) for n in (i, i + 1)]
            for e, v in enumerate(packed_sums(b, ((0, 1, 3), (1, -1, 3), (2, -1, 0), (0, 1, 1), (2, 1, 3)))):
                dst[e, pl.ds(r, 16), :] = v
            yield _Step(47, [anchor(dst)], delay=SETTLE if r == 240 else 1,
                        marks=[name] if r == 240 else [])

    def strassen(sch, weight, right, g, i, m, store, needs, marks):
        for n in needs:
            sch.run(n)
        sums, top, bottom = weight
        rows = pl.ds(pl.multiple_of(64 * m, 64), 64)
        sch.fresh = True

        def product(left, b):
            head = tied(lambda r: left(32 * m + r, 8, pl.ds(0, 128)), 4, lambda: sch.point(8.0))
            return _dot(_bf(jnp.concatenate([head, left(32 * m, 32, pl.ds(128, 384))], 1)), _bf(b))

        def a(e):
            return lambda r, size, cols: sums[e, pl.ds(pl.multiple_of(r, 8), size), cols]

        def b(e):
            return right[e + opaque()]

        m2 = product(a(1), hbu[i][g + opaque(), pl.ds(0, 256), :])
        m4 = product(lambda r, size, cols: bottom(r, size, pl.ds(512 + cols.start, cols.size)), b(2))
        store(1, i, rows, m2 + m4)
        m1 = product(a(0), b(0))
        c11, c22 = m1 + m4, m1 - m2
        m5 = product(a(2), hbu[i + 1][g + opaque(), pl.ds(256, 256), :])
        c11 = c11 - m5
        store(0, i, rows, c11 + product(a(4), b(4)))
        m3 = product(top, b(1))
        store(0, i + 1, rows, m3 + m5)
        c22 = c22 + m3
        v = product(a(3), b(3))
        store(1, i + 1, rows, c22 + v)
        sch.results.append(v[:8])
        for name in marks:
            sch.done[name] = sch.slot + WAIT

    def kv_proj(sch, g, i, name, needs):
        def store(lower, n, rows, v):
            (KE, VE)[lower][g + 4 * n + 4, rows, :] = v
        for m in range(16):
            strassen(sch, kv_weight, SB[i // 2], g, i, m, store, needs, [name] if m == 15 else [])

    def q_proj(sch, g, i, name, needs):
        def store(lower, n, rows, v):
            QB[n][0, pl.ds(512 * lower + rows.start, 64), :] = v
        for m in range(8):
            strassen(sch, q_weight, SB[i // 2], g, i, m, store, needs, [name] if m == 7 else [])

    def o_proj(sch, g, i, m, needs, marks):
        def store(lower, n, rows, v):
            rows = pl.ds(512 * lower + rows.start, 64)
            X[n][g, rows, :] = X[n][g, rows, :] + v
        strassen(sch, o_weight, SB[2 + i // 2], g, i, m, store, needs, marks)

    def shift_block(g, i, name, needs):
        yield _Wait(*needs)
        j, z = g + 4 * i, opaque()
        for m in range(16):
            rows = pl.ds(64 * m, 64)
            for ref, to in ((KE, KS), (VE, VS)):
                v = pltpu.roll(ref[j + 4 + z, rows, :], 1, 1)
                if ref is VE:
                    v = jnp.where(_iota(64, 1) == 0, ref[4 + z, rows, :], v)
                to[j, rows, :] = v
                if i == 3:
                    ref[g, rows, :] = v
            yield _Step(12, delay=8 if i == 3 else 4, marks=[name] if m == 15 else [])

    def transpose_weight(w, quarters, name):
        for h in quarters:
            for r in range(4):
                v = WRAW[w, pl.ds(256 * r, 256), pl.ds(pl.multiple_of(256 * h, 256), 256)]
                v = pltpu.bitcast(v.T, U32)
                TR[2 * r], TR[2 * r + 1] = v[:, :128], v[:, 128:]
                yield _Step(40, delay=16)
            z = opaque()
            for c in range(8):
                WT[w][pl.ds(pl.multiple_of(128 * h, 128), 128), pl.ds(128 * c, 128)] = jnp.concatenate(
                    [TR[c + z, pl.ds(u, 8, stride=16), :] for u in range(16)], 0)
                yield _Step(20, delay=4, marks=[name] if c == 7 else [])

    def transpose_wo(name):
        for c in range(8):
            for h in range(4):
                v = jnp.concatenate([wou[c, pl.ds(128 * h + u, 8, stride=16), :] for u in range(16)], 0)
                WP[pl.ds(64 * c, 64), pl.ds(256 * h, 256)] = pltpu.bitcast(_bf(v).T, U32)
                yield _Step(20, delay=10, marks=[name] if c == 7 and h == 3 else [])

    def prep_spectral_weights(c2):
        lane = _iota(8, 1)
        order = jnp.where(lane > 64, 192 - lane, lane)

        def words(k2):
            re, im = (wsu[u, k2, pl.ds(c2, 64, stride=4), :] for u in range(2))
            return ((re & np.uint32(0xFFFF)) | (im << 16), (re >> 16) | (im & np.uint32(0xFFFF0000)))

        def arrange(w, below):
            w = jnp.where(_iota(w.shape[0], 1) < 64, w, below)
            return jnp.concatenate([jnp.take_along_axis(w[u:u + 8], order, axis=1)
                                    for u in range(0, w.shape[0], 8)], 0)

        below = words(15)
        for k2 in range(16):
            here = words(k2)
            for e in range(2):
                cl = 2 * c2 + e
                w = arrange(here[e], below[e])
                WS[k2, pl.ds(64 * cl, 64), :] = pltpu.roll(w, 1, 0) if cl > 4 else w
            below = here
            yield _Step(100)
        if c2 == 0:
            def nyquist(k2):
                re, im = (jnp.broadcast_to(WN[u, :, pl.ds(128 * k2, 128)].astype(F32), (8, 128))
                          for u in range(2))
                return pltpu.pack_elementwise([re, im], packed_dtype=BF16)
            for k2 in range(16):
                WS[k2, pl.ds(512, 8), :] = arrange(nyquist(k2), nyquist((k2 + 15) % 16))

    def write_out(p, c, name, needs):
        yield _Wait(*needs)
        rows = pl.ds(pl.multiple_of(128 * c, 128), 128)
        g, i = 2 * p % 4 + opaque(), p // 2
        w = pltpu.pack_elementwise([X[i][g, rows, :], X[i][g + 1, rows, :]], packed_dtype=BF16)
        xru[c, pl.ds(p, 128, stride=8), :] = w.T
        yield _Step(30, marks=[name])

    for c in range(8):
        x_copy(c).start()
    for c in range(5):
        mats[M_R + c] = d_mats[c]

    def make_twiddle(k):
        PB = temps[0][2]
        PB[0, pl.ds(0, 128), :] = lane_vec(L_TWID + k, 128)
        twid[k] = PB[opaque(), pl.ds(0, 128), :].T

    _loop(6, make_twiddle, "make_twiddle")

    def make_dft(j):
        fa, fb = lanes[pl.ds(L_FA, 128), :], lanes[pl.ds(L_FB, 128), :]
        c, sn = lane_vec(L_COS + j, 128), lane_vec(L_SIN + j, 128)
        UB, _, _, ubu, _ = temps[0]
        UB[0, pl.ds(0, 128), :] = (fa * c + fb * sn).astype(BF16)
        UB[0, pl.ds(128, 128), :] = (fb * c - fa * sn).astype(BF16)
        mats[M_FA + j], mats[M_FB + j] = ubu[0, pl.ds(0, 64), :], ubu[0, pl.ds(64, 64), :]

    _loop(NB, make_dft, "make_dft")

    def load_x(c):
        x_copy(c).wait()
        pl.when(c == 5)(lambda: start_all(spec_copies[0]))
        pl.when(c == 7)(lambda: start_all(spec_copies[1]))
        rows = pl.ds(pl.multiple_of(128 * c, 128), 128)
        for p in range(8):
            w = xru[c, pl.ds(p, 128, stride=8), :].T
            for e, bits in enumerate((w << 16, w & np.uint32(0xFFFF0000))):
                g, i = 2 * p % 4 + e, p // 2
                v = pltpu.bitcast(bits, F32)
                X[i][g, rows, :] = v
                v = v.reshape(16, 8, 128)
                mean = _all_sublanes(v.sum(0), jnp.add, 0) * (1.0 / 128)
                STAT[4 * g + i, c] = mean
                STAT[4 * g + i, 8 + c] = _all_sublanes(((v - mean) ** 2).sum(0), jnp.add, 0)

    _loop(8, load_x, "load_x")

    def after(name, action):
        yield _Wait(name)
        action()

    def spectral_weights():
        yield _Wait(("f", 2, 1))
        for c in spec_copies[0] + spec_copies[1]:
            c.wait()
        for c2 in range(4):
            yield from prep_spectral_weights(c2)

    with jax.named_scope("first_forward"):
        sch = _Sched(0.92)
        sch.add(after(("f", 0, 1), w_copies[1].start), "k")
        sch.add(after(("f", 1, 1), w_copies[2].start), "v")
        sch.add(after(("f", 2, 3), w_copies[0].start), "q")
        for g in range(4):
            for i in range(4):
                sch.add(fwd_block(g, i, ("f", g, i), [("f", g - 1, i)] if g else [],
                                  [("r", g - 1)] if g else [], True), ("f", g, i))
            sch.add(group_stage(g, ("r", g), [("f", g, i) for i in range(4)], False), ("r", g))
        sch.add(spectral_weights(), "s")
        sch.drive()
    start_all(wo_copies)

    def keys_values(layer, g):
        sch = _Sched(0.42 if layer == 0 else 0.40)
        nxt = (g + 1) % 4
        sch.add(inv_block(g, 2, ("i", 2), []), ("i", 2))
        sch.add(inv_block(g, 3, ("i", 3), [("read", ("i", 2))]), ("i", 3))
        sch.add(right_sums(SB[1], g, 2, ("b", 2), [("i", 2), ("i", 3)]), ("b", 2))
        sch.add(group_stage(nxt, "r", [("read", ("i", 3))], True), "r")
        sch.add(inv_block(nxt, 0, ("i", 4), ["r", ("i", 2)], n=g + 1), ("i", 4))
        sch.add(inv_block(nxt, 1, ("i", 5), [("read", ("i", 4)), ("i", 3)], n=g + 1), ("i", 5))
        if layer == 0:
            sch.add(transpose_weight(0, [g], "w"), "w")
            sch.add(left_sums(q_weight, 128 * (g % 2), 128, ["w"]), "sums")
        for i in (2, 3):
            sch.add(shift_block((g + 3) % 4, i, ("s", i), []), ("s", i))
        for i in (0, 1):
            sch.add(shift_block(g, i, ("s", i), [("kv", 0)]), ("s", i))
        sch.add(right_sums(SB[0], g + 1, 0, ("b", 4), [("i", 4), ("i", 5), ("kv", 0)]), ("b", 4))
        kv_proj(sch, g, 0, ("kv", 0), [])
        kv_proj(sch, g, 2, ("kv", 2), [("b", 2)])
        sch.finish()

    def mix(g, after, last, write):
        sch = _Sched(0.62)
        tail = after is None
        pace = 0.36 if tail else 0.33 if last else 0.29
        ahead = [(g, 2), (g, 3)] + ([] if tail else [(after, 0), (after, 1)])
        for n, block in enumerate(ahead):
            sch.add(attend(*block, ("a", n), [[], [("a", 0)], [("a", 1), ("q", 0)], [("a", 2)]][n]),
                    ("a", n), pace=pace)
            if n % 2:
                sch.add(right_sums(SB[2 + block[1] // 2], block[0], block[1] - 1, ("b", n),
                                   [("a", n)] + ([("o", 0, 0, "all")] if n == 3 else [])), ("b", n))
        for i in () if tail else (0, 2):
            sch.add(right_sums(SB[i // 2], after, i, ("h", i), [("q", 0)] if i else []), ("h", i))
        if not last:
            sch.add(group_stage((g + 3) % 4, "r", [], False), "r")
            for i in range(4):
                sch.add(fwd_block(g, i, ("f", i), [("o", i - i % 2, 7)], ["r"]), ("f", i))
        now = 6 if last else 8
        for i in range(4 if write else 0):
            for c in (0, 4, 1, 5, 2, 6):
                sch.add(write_out(2 * i + g // 2, c, ("w", i, c), [("o", i - i % 2, 2 * (c % 4) + 1)]),
                        ("w", i, c))
        for i in (0, 2):
            for m in range(now):
                o_proj(sch, g, i, m, [("b", 1)] if i else [],
                       [("o", i, m)] + ([("o", i, 0, "all")] if m == now - 1 else []))
            if not tail:
                q_proj(sch, after, i, ("q", i), [("h", i)])
        if tail and not last:
            sch.add(group_stage(g, "s", [("f", i) for i in range(4)], False), "s")
        sch.share = 0.92
        sch.drive()

    def postponed():
        sch = _Sched(0.5)
        pairs = [(g, i) for g in range(4) for i in (0, 2)]
        for n, (g, i) in enumerate(pairs):
            sch.add(right_sums(SB[2 + i // 2], g, i, ("b", n), [("o", n - 2)] if n >= 2 else []), ("b", n))
            for c in (3, 7) if g % 2 else ():
                for e in (i, i + 1):
                    sch.add(write_out(2 * e + g // 2, c, ("w", n, c, e), [("o", n)]), ("w", n, c, e))
        for n, (g, i) in enumerate(pairs):
            for m in (6, 7):
                o_proj(sch, g, i, m, [("b", n)], [("o", n)] if m == 7 else [])
        sch.finish()

    def first_queries(layer):
        sch = _Sched(0.62)
        sch.add(right_sums(SB[0], 0, 0, ("h", 0), []), ("h", 0))
        sch.add(right_sums(SB[1], 0, 2, ("h", 2), []), ("h", 2))
        sch.add(shift_block(3, 2, "s", []), "s")
        sch.add(attend(0, 0, ("a", 0), ["q"]), ("a", 0), pace=0.4)
        sch.add(attend(0, 1, ("a", 1), [("a", 0)]), ("a", 1), pace=0.4)
        sch.add(right_sums(SB[2], 0, 0, "b", [("a", 1)]), "b")
        sch.add(shift_block(3, 3, "t", []), "t")
        if layer == 0:
            for c in wo_copies:
                c.wait()
            sch.add(transpose_wo("w"), "w")
            sch.add(left_sums(o_weight, 0, 256, ["w"]), "sums")
        q_proj(sch, 0, 0, "q", [("h", 0)])
        q_proj(sch, 0, 2, None, [("h", 2)])
        sch.finish()

    def spectral_and_weights(h):
        for _ in transpose_weight(1, [h], None):
            pass
        spectral_rows(h)
        for _ in transpose_weight(2, [h], None):
            pass
        for _ in left_sums(kv_weight, 128 * h, 128):
            pass

    for layer in range(2):
        with jax.named_scope("spectral"):
            if layer == 0:
                w_copies[1].wait()
                w_copies[2].wait()
                _loop(4, spectral_and_weights, "rows")
            else:
                _loop(4, spectral_rows, "rows")
            spectral(512, 8)
        sch = _Sched(0.92)
        sch.add(group_stage(0, "r", [], True), "r")
        sch.add(inv_block(0, 0, ("i", 0), ["r"]), ("i", 0))
        sch.add(inv_block(0, 1, ("i", 1), ["r"]), ("i", 1))
        sch.add(right_sums(SB[0], 0, 0, "b", [("i", 0), ("i", 1)]), "b")
        sch.drive()
        if layer == 0:
            w_copies[0].wait()
        _loop(4, lambda g: keys_values(layer, g), "keys_values")
        first_queries(layer)
        if layer == 0:
            pl.when(never)(lambda: [spectral_rows(c % 4) for c in range(5)] and None)
        if layer == 0:
            _loop(3, lambda g: mix(g, g + 1, False, False), "mix")
            mix(3, None, False, False)
        else:
            _loop(2, lambda u: mix(2 * u, 2 - u, True, False), "mix")
            mix(1, 3, True, True)
            mix(3, None, True, True)
    for c in (0, 1, 2, 4, 5, 6):
        out_copy(c).start()
    with jax.named_scope("postponed"):
        postponed()
    for c in (3, 7):
        out_copy(c).start()
    for c in range(8):
        out_copy(c).wait()


@jax.jit
def pallas_interleave_layers__spectral_gfnet__sliding_local_dilated__prompt_kernel(
    A_x: jax.Array,
    A_w_r: jax.Array,
    A_w_i: jax.Array,
    B_x: jax.Array,
    B_wqkv: jax.Array,
    B_wo: jax.Array,
):
    del B_x
    hbm = pl.BlockSpec(memory_space=pl.ANY)
    smem = pl.BlockSpec(memory_space=pltpu.SMEM)
    out = pl.pallas_call(
        _kernel,
        out_shape=jax.ShapeDtypeStruct((S, D), BF16),
        in_specs=[smem, smem, pl.BlockSpec(), pl.BlockSpec(), hbm, hbm, hbm, hbm, hbm],
        out_specs=hbm,
        scratch_shapes=[
            pltpu.VMEM((37, 64, 128), U32),
            pltpu.VMEM((6, 128, 128), F32),
            pltpu.VMEM((NB, 16, 8, 128), F32),
            pltpu.VMEM((NB + 4, D, 128), F32),
            pltpu.VMEM((NB + 4, D, 128), F32),
            pltpu.VMEM((NB, D, 128), F32),
            pltpu.VMEM((NB, D, 128), F32),
            pltpu.VMEM((2 * NB + 1, ZR, 128), F32),
            pltpu.VMEM((9, ZR, 128), F32),
            pltpu.VMEM((NB, ZR, 128), U32),
            *4 * [pltpu.VMEM((D // 2, D), U32)],
            pltpu.VMEM((5, D // 2, D // 2), U32),
            *2 * [pltpu.VMEM((5, D // 4, D // 2), U32)],
            *4 * [pltpu.VMEM((5, D // 4, 128), U32)],
            pltpu.VMEM((8, S, 128), BF16),
            pltpu.VMEM((2, NB, D // 2, 128), BF16),
            pltpu.VMEM((2, 1, S), BF16),
            pltpu.VMEM((3, D, D), BF16),
            pltpu.VMEM((8, D, 128), BF16),
            pltpu.VMEM((8, 128, 128), U32),
            pltpu.VMEM((1, 128, 128), F32),
            pltpu.VMEM((1, 128, 128), F32),
            pltpu.SemaphoreType.DMA((24,)),
        ] + 4 * [
            pltpu.VMEM((5, D, 128), F32),
            pltpu.VMEM((5, D, 128), BF16),
            pltpu.VMEM((1, D, 128), F32),
            pltpu.VMEM((1, D, 128), BF16),
            pltpu.VMEM((1, 1152, 128), BF16),
            pltpu.VMEM((1, D, 128), F32),
        ],
        compiler_params=pltpu.CompilerParams(vmem_limit_bytes=126 * 2 ** 20),
    )(_ZERO, _ROT, _MATS, _LANES, A_x.reshape(S, D), A_w_r.T, A_w_i.T, B_wqkv, B_wo)
    return out.reshape(1, S, D)
```

```python
import functools

import numpy as np

import jax
import jax.numpy as jnp
import jax.experimental.pallas as pl
import jax.experimental.pallas.tpu as pltpu

S, D, NB = 2048, 1024, 16
ZR = 576
F32, BF16, U32, I32 = jnp.float32, jnp.bfloat16, jnp.uint32, jnp.int32
EPS = 1e-5
SCALE = 32 ** -0.5
RSQ2 = float(np.sqrt(0.5))
WAIT = 24
GRAIN = 1
SETTLE = 6
LAG = 3

_S_ROWS = [(32 * u, 32) for u in range(16)] + [(512, 8)]

M_FA, M_FB, M_R, M_C4, M_RT, M_C4T, M_R0T = 0, 16, 32, 33, 34, 35, 36
L_MU, L_NU, L_KU, L_KV, L_COS, L_SIN, L_TWID, L_FA, L_FB = 0, 16, 32, 48, 64, 80, 96, 104, 232


def _bf16_bits(a):
    u = np.ascontiguousarray(a, dtype=np.float32).view(np.uint32).astype(np.uint64)
    return ((u + 0x7FFF + ((u >> 16) & 1)) >> 16).astype(np.uint32)


def _constants():
    a = np.arange(128)
    k1 = np.arange(64)
    alt = (-1.0) ** a
    lanes = np.zeros((L_FB + 128, 128))
    t = 2 * np.pi * np.outer(a, k1) / 128
    fa = np.concatenate([np.cos(t), -np.sin(t)], 1)
    fb = np.concatenate([np.sin(t), -np.cos(t)], 1)
    fa[:, 0], fb[:, 0] = RSQ2, -RSQ2
    fa[:, 64], fb[:, 64] = alt, 0.0
    lanes[L_FA:L_FA + 128], lanes[L_FB:L_FB + 128] = fa, fb
    for j in range(NB):
        ang = 2 * np.pi * j / 32 + np.pi / 32
        p, q = (_bf16_bits([np.cos(ang), np.sin(ang)]) << 16).view(np.float32).astype(np.float64)
        turn = 2 * np.pi * j * np.tile(k1, 2) / S
        lanes[L_COS + j], lanes[L_SIN + j] = np.cos(turn), np.repeat([-1.0, 1.0], 64) * np.sin(turn)
        lanes[L_COS + j, 64], lanes[L_SIN + j, 64] = p, q
        lanes[L_MU + j, 0], lanes[L_MU + j, 64] = 1.0, (q / p + p / q) / 2
        lanes[L_NU + j, 0], lanes[L_NU + j, 64] = 0.0, (q / p - p / q) / 2
        lanes[L_KU + j, 0], lanes[L_KU + j, 64] = 1.0, q / p
        lanes[L_KV + j, 0], lanes[L_KV + j, 64] = 1.0, p / q
    for k in (1, 2, 3):
        lanes[L_TWID + 2 * k - 2] = np.cos(2 * np.pi * a * k / D)
        lanes[L_TWID + 2 * k - 1] = np.sin(2 * np.pi * a * k / D)
    th = 2 * np.pi * np.outer(k1, a) / 128
    r = np.concatenate([np.cos(th), -np.sin(th)], 0)
    r[64] = alt
    th = 2 * np.pi * np.outer(2 * k1 + 1, a) / 256
    c4 = np.concatenate([np.cos(th), -np.sin(th)], 0)
    inv = 2.0 / (S * D)
    r0t = inv * r.T
    r0t[:, 0::64] *= 0.5
    rows = np.arange(128).reshape(2, 4, 16).transpose(1, 0, 2).ravel()
    bits = _bf16_bits(np.stack([r[rows], c4[rows], inv * r.T, inv * c4.T, r0t]))
    ang = 2 * np.pi * np.outer(np.arange(4), np.arange(4)).ravel() / 16
    rot = np.concatenate([np.cos(ang), np.sin(ang)]).astype(np.float32)
    return bits[:, 0::2] | (bits[:, 1::2] << 16), lanes.astype(np.float32), rot


_MATS, _LANES, _ROT = _constants()
_ZERO = np.zeros((1,), np.int32)


class _Step:
    def __init__(self, cost, anchors=(), delay=0, marks=()):
        self.cost, self.anchors, self.delay, self.marks = cost, list(anchors), delay, list(marks)


class _Wait:
    def __init__(self, *names):
        self.names = names


class _Mat:
    def __init__(self, emit):
        self.emit = emit


class _Hold:
    def __init__(self, store):
        self.store = store


class _Task:
    def __init__(self, gen, pace):
        self.gen, self.pace, self.blocked, self.not_before, self.held = gen, pace, (), 0, None
        self.allowed = 0.0


class _Sched:
    def __init__(self, share=0.0):
        self.share = share
        self.tasks, self.done, self.producer = [], {}, {}
        self.slot, self.credit, self.anchors, self.results = 0, 0.0, [], []
        self.fresh = False

    def add(self, gen, name, pace=99):
        self.producer[name] = self.producer["read", name] = _Task(gen, pace)
        self.tasks.append(self.producer[name])

    def _ready(self, t):
        return t.not_before <= self.slot and all(
            n in self.done and self.done[n] <= self.slot for n in t.blocked)

    def _advance(self, t, mats=True):
        item, t.held = t.held or next(t.gen, None), None
        if item is None:
            self.tasks.remove(t)
        elif isinstance(item, _Wait):
            t.blocked = item.names
        elif isinstance(item, _Hold):
            if len(self.results) >= LAG:
                item.store(self.results[-LAG])
        elif isinstance(item, _Mat):
            if mats:
                t.not_before = float("inf")
                self.fresh = False
                self.credit -= item.emit(lambda: self.point(0.0)) or 0
                t.not_before = self.slot + WAIT
            else:
                t.held, t.not_before = item, self.slot + 1
        else:
            t.blocked = ()
            t.not_before = self.slot + item.delay
            self.credit -= item.cost
            self.anchors += item.anchors
            for n in item.marks:
                self.done[n] = self.slot + item.delay
            return True

    def run(self, *names):
        while not all(n in self.done for n in names):
            for n in names:
                if n not in self.done:
                    for b in self.producer[n].blocked:
                        self.run(b)
                    self._advance(self.producer[n])

    def drive(self):
        while self.tasks:
            ready = [t for t in self.tasks if self._ready(t)]
            if not ready:
                self.slot += 1
                continue
            self.anchors, self.credit = self.anchors[-2:], 0.0
            self._advance(next((t for t in ready if t.held), ready[0]))
            self.slot -= min(self.credit, 0.0) / 60

    def finish(self):
        self.run(*[n for n in self.producer if n[0] != "read"])

    def point(self, own):
        for t in self.tasks:
            t.allowed = min(t.allowed, 0.0) + t.pace
        while True:
            t = next((t for t in self.tasks if self._ready(t) and t.allowed > 0
                      and self.credit > 0), None)
            if t is None:
                break
            if self._advance(t, self.fresh):
                t.allowed -= 1
        anchors, self.anchors = self.anchors, []
        self.credit = min(self.credit, 10.0) + 64 * self.share - own
        self.fresh = False
        self.slot += 1
        return anchors


def _dot(a, b):
    return jnp.dot(a, b, preferred_element_type=F32)


def _dot_t(a, b):
    return jax.lax.dot_general(a, b, (((1,), (1,)), ((), ())), preferred_element_type=F32)


def _bf(u):
    return pltpu.bitcast(u, BF16)


def _iota(rows, dim):
    return jax.lax.broadcasted_iota(I32, (rows, 128), dim)


def _radix4(z, inverse):
    (r0, i0), (r1, i1), (r2, i2), (r3, i3) = z
    ar, ai, cr, ci = r0 + r2, i0 + i2, r0 - r2, i0 - i2
    br, bi, dr, di = r1 + r3, i1 + i3, r1 - r3, i1 - i3
    lo, hi = (cr + di, ci - dr), (cr - di, ci + dr)
    if inverse:
        lo, hi = hi, lo
    return [(ar + br, ai + bi), lo, (ar - br, ai - bi), hi]


def _all_sublanes(v, op, axis):
    for sh in (4, 2, 1):
        v = op(v, pltpu.roll(v, sh, axis))
    return v


def _loop(n, body, name):
    def step(i, carry):
        body(i)
        return carry
    with jax.named_scope(name):
        jax.lax.fori_loop(0, n, step, 0)


def _kernel(zero_ref, rot, d_mats, lanes, x_hbm, wr_hbm, wi_hbm, wqkv_hbm, wo_hbm, out_hbm,
            mats, twid, STAT, KE, VE, KS, VS, Z, ZT, WS, WQ, WK, WV, WP, WS5, WQ5, WP5, SB0, SB1, SB2, SB3, XR, WRI, WN, WRAW, WO, PW0, PW1, sems, *split):
    zero = zero_ref[0]
    never = zero != 0
    X, HB, QB = split[2::5], split[3::5], split[4::5]
    hbu = [r.bitcast(U32) for r in HB]
    xru, wsu, wou = XR.bitcast(U32), WRI.bitcast(U32), WO.bitcast(U32)
    temps = [(ub, ab, pb, ub.bitcast(U32), ab.bitcast(U32))
             for ub, ab, pb in zip(split[5::5], split[6::5], 2 * split[:2])]
    PW, SB, WT = (PW0, PW1), (SB0, SB1, SB2, SB3), (WQ, WK, WV, WP)
    counter = [0]

    def opaque():
        counter[0] += 1
        return zero * counter[0]

    def anchor(ref):
        at = (0,) * (len(ref.shape) - 2)
        return lambda: ref[(*at, pl.ds(pl.multiple_of(zero * 8, 8), 8), pl.ds(0, 128))]

    def settle(ref):
        return _Step(2, [anchor(ref)], delay=SETTLE)

    def hold(ref, spare, row=0):
        def store(v):
            ref[spare, pl.ds(pl.multiple_of(row + zero * 8, 8), 8), :] = v
        return _Hold(store)

    def tied(load, vregs, point):
        parts = []
        for r in range(vregs):
            anchors = [a for _ in range(GRAIN) for a in point()] if r % GRAIN == 0 else []
            u = load(8 * r)
            for a in anchors:
                u = jnp.where(never, pltpu.bitcast(a(), U32), u)
            parts.append(u)
        return jnp.concatenate(parts, 0)

    def mat(i):
        return _bf(mats[i])

    def d_stage(t, which):
        UB, AB, PB, ubu, abu = temps[t]

        def emit(point):
            z = opaque()
            for c in range(8):
                lhs = mat(which(c) + opaque()) if c % 4 else _bf(
                    tied(lambda r, u=which(c) + opaque(): mats[u, pl.ds(r, 8), :], 8, point))
                PB[0, pl.ds(128 * c, 128), :] = _dot(lhs, _bf(ubu[z, pl.ds(64 * c, 64), :]))
        return _Mat(emit)

    def lane_vec(i, rows):
        return jnp.broadcast_to(lanes[pl.ds(i, 1), :], (rows, 128))

    def x_copy(c):
        return pltpu.make_async_copy(
            x_hbm.at[:, pl.ds(pl.multiple_of(128 * c, 128), 128)], XR.at[c], sems.at[c])

    def out_copy(c):
        return pltpu.make_async_copy(
            XR.at[c], out_hbm.at[:, pl.ds(pl.multiple_of(128 * c, 128), 128)], sems.at[8 + c])

    spec_copies = [[pltpu.make_async_copy(w.at[pl.ds(0, 512), pl.ds(128 * k2, 128)], WRI.at[u, k2],
                                          sems.at[16 + u]) for k2 in range(16)]
                   + [pltpu.make_async_copy(w.at[pl.ds(512, 1), :], WN.at[u], sems.at[22 + u])]
                   for u, w in enumerate((wr_hbm, wi_hbm))]

    def start_all(copies):
        for c in copies:
            c.start()
    w_copies = [pltpu.make_async_copy(wqkv_hbm.at[:, pl.ds(D * w, D)], WRAW.at[w], sems.at[18 + w])
                for w in range(3)]
    wo_copies = [pltpu.make_async_copy(wo_hbm.at[:, pl.ds(128 * c, 128)], WO.at[c], sems.at[21])
                 for c in range(8)]

    def ln_rstd(g, i, mean):
        acc, m = None, g + opaque()
        for r in range(8):
            d = X[i][m, pl.ds(128 * r, 128), :].reshape(16, 8, 128) - mean[None]
            v = (d * d).sum(0)
            acc = v if acc is None else acc + v
            if r < 7:
                yield _Step(50, [lambda acc=acc: acc], delay=3)
        rstd = jax.lax.rsqrt(_all_sublanes(acc, jnp.add, 0) * (1.0 / D) + EPS)
        yield _Step(50, delay=8)
        yield _Step(10, [lambda: rstd], delay=1)
        return rstd

    def fwd_block(g, i, name, needs, free=(), known=False):
        j, t = g + 4 * i, i
        UB, AB, PB, ubu, abu = temps[t]
        yield _Wait(*needs)
        if known:
            means, squares = STAT[4 * g + i, pl.ds(0, 8)], STAT[4 * g + i, pl.ds(8, 8)]
            mean = means.sum(0) * 0.125
            var = (squares.sum(0) + 128.0 * ((means - mean) ** 2).sum(0)) * (1.0 / D)
            rstd = jax.lax.rsqrt(var + EPS)
            yield _Step(50, delay=6)
        else:
            yield settle(X[i])
            acc, m = None, g + opaque()
            for r in range(8):
                v = X[i][m, pl.ds(128 * r, 128), :].reshape(16, 8, 128).sum(0)
                acc = v if acc is None else acc + v
                if r % 2:
                    yield _Step(35, [lambda acc=acc: acc], delay=7 if r == 7 else 3)
            mean = _all_sublanes(acc, jnp.add, 0) * (1.0 / D)
            rstd = yield from ln_rstd(g, i, mean)
        mean8, rstd = (jnp.concatenate([v, v], 0) for v in (mean * 8.0, rstd))
        z = opaque()
        for r in range(8):
            rows = pl.ds(16 * r, 16)
            x = [X[i][g + z, pl.ds(128 * b + 16 * r, 16), :] for b in range(8)]
            s = [x[b] + x[b + 4] for b in range(4)]
            d = [x[b] - x[b + 4] for b in range(4)]
            e, o = s[0] + s[2], s[1] + s[3]
            UB[0, rows, :] = ((e + o - mean8) * rstd).astype(BF16)
            UB[0, pl.ds(128 + 16 * r, 16), :] = ((e - o) * rstd).astype(BF16)
            t1, t2 = (d[1] - d[3]) * RSQ2, (d[1] + d[3]) * RSQ2
            u = {1: (d[0] + t1, d[2] + t2), 2: (s[0] - s[2], s[1] - s[3]), 3: (d[0] - t1, d[2] - t2)}
            yield _Step(34, [anchor(ubu)], delay=1)
            for k in (1, 2, 3):
                c, sn = twid[z + 2 * k - 2, rows, :] * rstd, twid[z + 2 * k - 1, rows, :] * rstd
                re, m = u[k]
                if k == 3:
                    ur, ui = re * c + m * sn, m * c - re * sn
                else:
                    ur, ui = re * c - m * sn, m * c + re * sn
                UB[0, pl.ds(256 * k + 16 * r, 16), :] = ur.astype(BF16)
                UB[0, pl.ds(256 * k + 128 + 16 * r, 16), :] = ui.astype(BF16)
                yield _Step(26, [anchor(ubu)], delay=1)
        yield settle(ubu)

        def d_forward(point):
            z = opaque()
            first = _iota(8, 0) == 0

            def stage(c):
                u = (M_C4 if c == 1 else M_R) + opaque()
                lhs = mat(u) if c % 4 else _bf(tied(lambda r: mats[u, pl.ds(r, 8), :], 8, point))
                v = _dot(lhs, _bf(ubu[z, pl.ds(64 * c, 64), :]))
                return [(v[32 * u:32 * u + 16], v[32 * u + 16:32 * u + 32]) for u in range(4)]

            def put(row, u, v, v0=None):
                if u == 0 and v0 is not None:
                    v = jnp.concatenate([jnp.where(first, v0, v[:8]), v[8:]], 0)
                AB[0, pl.ds(row + 16 * u, 16), :] = v.astype(BF16)

            for u, (p1, p2) in enumerate(stage(0)):
                put(0, u, p1)
                put(528, u, p2, 0.0)
                if u == 0:
                    put(512, 0, jnp.zeros_like(p2), p2[:8])
            for u, (p1, p2) in enumerate(stage(1)):
                put(256, u, p1)
                put(528 + 256, u, p2)
            for k in (1, 2, 3):
                for u, ((p1, p2), (q1, q2)) in enumerate(zip(stage(2 * k), stage(2 * k + 1))):
                    if k == 3:
                        pr, pi, mr, mi = p1 - q2, p2 + q1, p1 + q2, p2 - q1
                        pi0, mi0 = q1[:8], -q2[:8]
                    else:
                        pr, pi, mr, mi = p1 + q2, p2 - q1, p1 - q2, p2 + q1
                        pi0, mi0 = -q1[:8], q2[:8]
                    put(64 * k, u, pr, p1[:8])
                    put(64 * (8 - k), u, mr, p2[:8])
                    put(528 + 64 * k, u, pi, pi0)
                    put(528 + 64 * (8 - k), u, mi, mi0)
            return 190

        yield _Mat(d_forward)
        yield settle(abu)
        yield _Wait(*free)

        def s_forward(point):
            z = opaque()
            fa, fb = mat(M_FA + j + z), mat(M_FB + j + z)
            for r0, rn in ((0, 256), (256, 272)):
                lhs = abu[z, pl.ds(r0 // 2, rn // 2), :] if r0 else tied(
                    lambda r: abu[z, pl.ds(r, 8), :], 16, point)
                u = _dot(_bf(lhs), fa)
                v = _dot(_bf(abu[z, pl.ds(264 + r0 // 2, 128), :]), fb)
                re, m = u[:256] + v, u[:256] - v
                if r0:
                    re, m = (jnp.concatenate([a, u[256:264]], 0) for a in (re, m))
                rn = re.shape[0]
                edge = (_iota(rn, 1) & 63) == 0
                ZT[2 * i, pl.ds(r0, rn), :] = re
                ZT[2 * i + 1, pl.ds(r0, rn), :] = jnp.where(
                    edge, lane_vec(L_MU + j, rn) * m + lane_vec(L_NU + j, rn) * re, pltpu.roll(m, 64, 1))
            return 400

        yield _Mat(s_forward)
        yield _Step(2, [anchor(ZT)], delay=SETTLE, marks=[name])

    def group_stage(g, name, needs, inverse):
        yield _Wait(*needs)

        def turn(z, k):
            if k == 0:
                return z
            c, s = rot[4 * g + k], rot[16 + 4 * g + k]
            if inverse:
                return z[0] * c - z[1] * s, z[1] * c + z[0] * s
            return z[0] * c + z[1] * s, z[1] * c - z[0] * s

        (src, a), (dst, b) = ((Z, 8 * g), (ZT, 0)) if inverse else ((ZT, opaque()), (Z, 8 * g))
        for r in range(65):
            if r % 4 == 0:
                yield hold(src, 2 * NB if inverse else 8)
            rows = pl.ds(8 * r, 8)
            z = [(src[a + 2 * i, rows, :], src[a + 2 * i + 1, rows, :]) for i in range(4)]
            if inverse:
                z = _radix4([turn(z[k], k) for k in range(4)], True)
            else:
                z = [turn(v, k) for k, v in enumerate(_radix4(z, False))]
            for i in range(4):
                dst[b + 2 * i, rows, :], dst[b + 2 * i + 1, rows, :] = z[i]
            yield _Step(35, [anchor(dst)], delay=1, marks=[name] if r == 64 else [])

    def spectral(row, size):
        rows = pl.ds(row, size)
        for k0 in range(4):
            z = _radix4([(Z[8 * g + 2 * k0, rows, :], Z[8 * g + 2 * k0 + 1, rows, :])
                         for g in range(4)], False)
            y = []
            for k1, (re, im) in enumerate(z):
                w = WS[k0 + 4 * k1, rows, :]
                wr = pltpu.bitcast(w << 16, F32)
                wi = pltpu.bitcast(w & np.uint32(0xFFFF0000), F32)
                y.append((re * wr - im * wi, re * wi + im * wr))
            y = _radix4(y, True)
            for g in range(4):
                Z[8 * g + 2 * k0, rows, :], Z[8 * g + 2 * k0 + 1, rows, :] = y[g]

    def spectral_rows(c2):
        for r in range(8):
            spectral(pl.multiple_of(128 * c2 + 16 * r, 16), 16)

    def inv_block(g, i, name, needs, n=None):
        j, t = g + 4 * i, i % 2
        UB, AB, PB, ubu, abu = temps[t]
        n = g if n is None else n
        z = opaque()
        yield _Wait(*needs)
        for r0, rn in _S_ROWS:
            if r0 == 0:
                yield hold(ZT, 8)
            re, im = ZT[z + 2 * i, pl.ds(r0, rn), :], ZT[z + 2 * i + 1, pl.ds(r0, rn), :]
            edge = (_iota(rn, 1) & 63) == 0
            rolled = pltpu.roll(im, 64, 1)
            u = re + jnp.where(edge, lane_vec(L_KU + j, rn) * im, rolled)
            if r0 < 512:
                v = re - jnp.where(edge, lane_vec(L_KV + j, rn) * im, rolled)
                AB[0, pl.ds(r0, rn), :] = u.astype(BF16)
                AB[0, pl.ds(528 + r0, rn), :] = v.astype(BF16)
            else:
                AB[0, pl.ds(512, 16), :] = jnp.concatenate([u, jnp.zeros_like(u)], 0).astype(BF16)
            yield _Step(rn, [anchor(abu)], delay=1, marks=[("read", name)] if r0 == 512 else [])
        yield settle(abu)

        def s_inverse(point):
            z = opaque()
            fa, fb = mat(M_FA + j + z), mat(M_FB + j + z)
            first = _iota(8, 0) == 0

            def put(row, v, v0=None):
                if v0 is not None:
                    v = jnp.concatenate([jnp.where(first, v0, v[:8]), v[8:]], 0)
                UB[0, pl.ds(row, 64), :] = v.astype(BF16)

            for k in range(4):
                lo, hi = 32 * k, 32 * (8 - k if k else 4)
                a = [abu[z, pl.ds(lo, 32), :], abu[z, pl.ds(hi, 32), :]] if k % 2 else [
                    tied(lambda r, o=o: abu[z, pl.ds(o + r, 8), :], 4, point) for o in (lo, hi)]
                if k == 0:
                    a.append(abu[z, pl.ds(256, 8), :])
                re = _dot_t(_bf(jnp.concatenate(a, 0)), fa)
                im = _dot_t(_bf(jnp.concatenate(
                    [abu[z, pl.ds(264 + lo, 32), :], abu[z, pl.ds(264 + hi, 32), :]], 0)), fb)
                pr, mr, pi, mi = re[:64], re[64:128], im[:64], im[64:]
                if k == 0:
                    put(0, pr)
                    put(64, pi, re[128:136])
                    put(128, mr)
                    put(192, mi)
                else:
                    put(256 * k, pr + mr, pr[:8])
                    put(256 * k + 64, pi + mi, mr[:8])
                    put(256 * k + 128, pi - mi, pi[:8])
                    put(256 * k + 192, mr - pr, -mi[:8])
            return 190

        yield _Mat(s_inverse)
        yield settle(ubu)
        yield d_stage(t, lambda c: {0: M_R0T, 1: M_C4T}.get(c, M_RT))
        yield settle(PB)
        z = opaque()
        acc = None
        for r in range(16):
            rows = pl.ds(8 * r, 8)
            t0, t4 = PB[z, rows, :], PB[z, pl.ds(128 + 8 * r, 8), :]
            tk = {}
            for k in (1, 2, 3):
                c, sn = twid[z + 2 * k - 2, rows, :], twid[z + 2 * k - 1, rows, :]
                re = PB[z, pl.ds(256 * k + 8 * r, 8), :]
                im = PB[z, pl.ds(256 * k + 128 + 8 * r, 8), :]
                tk[k] = (re * c - im * sn, re * sn + im * c)
            e0, e1 = t0 + t4, t0 - t4
            s = [e0 + tk[2][0], e1 - tk[2][1], e0 - tk[2][0], e1 + tk[2][1]]
            al, be = tk[1][0] - tk[3][0], tk[1][1] + tk[3][1]
            o = [tk[1][0] + tk[3][0], (al - be) * RSQ2, tk[3][1] - tk[1][1], (al + be) * -RSQ2]
            for b in range(8):
                y = s[b] + o[b] if b < 4 else s[b - 4] - o[b - 4]
                v = X[i][g, pl.ds(128 * b + 8 * r, 8), :] + y
                X[i][n, pl.ds(128 * b + 8 * r, 8), :] = v
                acc = v if acc is None else acc + v
            yield _Step(57, [lambda v=acc: v], delay=5 if r == 15 else 2)
        yield settle(X[i])
        mean = _all_sublanes(acc, jnp.add, 0) * (1.0 / D)
        rstd = yield from ln_rstd(n, i, mean)
        z = opaque()
        for r in range(8):
            v = X[i][n + z, pl.ds(128 * r, 128), :].reshape(16, 8, 128)
            HB[i][n, pl.ds(128 * r, 128), :] = ((v - mean[None]) * rstd[None]).reshape(128, 128).astype(BF16)
            yield _Step(41, [anchor(hbu[i])], delay=1, marks=[name] if r == 7 else [])

    def attend(g, i, name, needs):
        yield _Wait(*needs)
        yield settle(QB[i])
        j, z = g + 4 * i, opaque()
        even = (_iota(8, 0) & 1) == 0
        edge = _iota(8, 1) == 0

        def window(near, far, w, rows):
            return near[j + z + 4 - 2 * w, rows, :] if w <= 2 * i + 2 else far[j + z + 16 - 2 * w, rows, :]

        def mix_values(h, u):
            p = PW[h % 2][opaque()]
            for rows in (pl.ds(256 * h + 16 * u, 16), pl.ds(256 * h + 16 * u + 16, 16)):
                acc = functools.reduce(jnp.add, [p[16 * w:16 * w + 16] * window(VE, VS, w, rows)
                                                 for w in range(8)])
                HB[i][g, rows, :] = acc.astype(BF16)
            return _Step(63, [anchor(hbu[i])], delay=1, marks=[name] if (h, u) == (3, 14) else [])

        for h in range(5):
            logits = []
            for w0 in range(0, 8, 2):
                if h < 4:
                    rows = pl.ds(256 * h, 256)
                    q = QB[i][opaque(), rows, :]
                    for w in (w0, w0 + 1):
                        v = (q * window(KE, KS, w, rows)).reshape(16, 16, 128).sum(0)
                        v = jnp.where(even, v[:8] + pltpu.roll(v[:8], 7, 0), v[8:] + pltpu.roll(v[8:], 1, 0))
                        logits.append(jnp.where(edge & (2 * w > j), -1e9, v * SCALE) if w > 2 * i
                                      else v * SCALE)
                    yield _Step(138, [lambda v=v: v for v in logits[-2:]], delay=2)
                if h > 0:
                    yield mix_values(h - 1, 2 * w0)
                    yield mix_values(h - 1, 2 * w0 + 2)
            if h < 4:
                top = functools.reduce(jnp.maximum, logits)
                e = [jnp.exp(v - top) for v in logits]
                total = functools.reduce(jnp.add, e)
                yield _Step(30, [lambda v=total: v], delay=3)
                scale = 1.0 / total
                for w in range(8):
                    v = e[w] * scale
                    PW[h % 2][0, pl.ds(16 * w, 8), :] = jnp.where(even, v, pltpu.roll(v, 1, 0))
                    PW[h % 2][0, pl.ds(16 * w + 8, 8), :] = jnp.where(even, pltpu.roll(v, 7, 0), v)
                yield _Step(50, [anchor(PW[h % 2])], delay=6 if h == 3 else 1)

    def packed_sums(terms, signs):
        lo = [pltpu.bitcast(u << 16, F32) for u in terms]
        hi = [pltpu.bitcast(u & np.uint32(0xFFFF0000), F32) for u in terms]
        return [pltpu.pack_elementwise([v[p] + v[q] if s > 0 else v[p] - v[q] for v in (lo, hi)],
                                       packed_dtype=BF16) for p, s, q in signs]

    def half(ref, row):
        return lambda r, size, cols: ref[pl.ds(pl.multiple_of(row + r, 8), size), cols]

    kv_weight = (WS5, half(WK, 0), half(WV, 0))
    q_weight = (WQ5, half(WQ, 0), half(WQ, D // 4))
    o_weight = (WP5, half(WP, 0), half(WP, D // 4))

    def left_sums(weight, row, size, needs=()):
        yield _Wait(*needs)
        sums, top, bottom = weight
        for r in range(0, size, 8):
            a = [ref(row + r, 8, pl.ds(c, 512)) for ref in (top, bottom) for c in (0, 512)]
            for e, v in enumerate(packed_sums(a, ((0, 1, 3), (2, 1, 3), (0, 1, 1), (2, -1, 0), (1, -1, 3)))):
                sums[e, pl.ds(pl.multiple_of(row + r, 8), 8), :] = v
            yield _Step(92, [anchor(sums)], delay=2, marks=["sums"] if r == size - 8 else [])

    def right_sums(dst, g, i, name, needs):
        yield _Wait(*needs)
        z = g + opaque()
        for r in range(0, 256, 16):
            b = [hbu[n][z, pl.ds(k + r, 16), :] for k in (0, 256) for n in (i, i + 1)]
            for e, v in enumerate(packed_sums(b, ((0, 1, 3), (1, -1, 3), (2, -1, 0), (0, 1, 1), (2, 1, 3)))):
                dst[e, pl.ds(r, 16), :] = v
            yield _Step(47, [anchor(dst)], delay=SETTLE if r == 240 else 1,
                        marks=[name] if r == 240 else [])

    def strassen(sch, weight, right, g, i, m, store, needs, marks):
        for n in needs:
            sch.run(n)
        sums, top, bottom = weight
        rows = pl.ds(pl.multiple_of(64 * m, 64), 64)
        sch.fresh = True

        def product(left, b):
            head = tied(lambda r: left(32 * m + r, 8, pl.ds(0, 128)), 4, lambda: sch.point(8.0))
            return _dot(_bf(jnp.concatenate([head, left(32 * m, 32, pl.ds(128, 384))], 1)), _bf(b))

        def a(e):
            return lambda r, size, cols: sums[e, pl.ds(pl.multiple_of(r, 8), size), cols]

        def b(e):
            return right[e + opaque()]

        m2 = product(a(1), hbu[i][g + opaque(), pl.ds(0, 256), :])
        m4 = product(lambda r, size, cols: bottom(r, size, pl.ds(512 + cols.start, cols.size)), b(2))
        store(1, i, rows, m2 + m4)
        m1 = product(a(0), b(0))
        c11, c22 = m1 + m4, m1 - m2
        m5 = product(a(2), hbu[i + 1][g + opaque(), pl.ds(256, 256), :])
        c11 = c11 - m5
        store(0, i, rows, c11 + product(a(4), b(4)))
        m3 = product(top, b(1))
        store(0, i + 1, rows, m3 + m5)
        c22 = c22 + m3
        v = product(a(3), b(3))
        store(1, i + 1, rows, c22 + v)
        sch.results.append(v[:8])
        for name in marks:
            sch.done[name] = sch.slot + WAIT

    def kv_proj(sch, g, i, name, needs):
        def store(lower, n, rows, v):
            (KE, VE)[lower][g + 4 * n + 4, rows, :] = v
        for m in range(16):
            strassen(sch, kv_weight, SB[i // 2], g, i, m, store, needs, [name] if m == 15 else [])

    def q_proj(sch, g, i, name, needs):
        def store(lower, n, rows, v):
            QB[n][0, pl.ds(512 * lower + rows.start, 64), :] = v
        for m in range(8):
            strassen(sch, q_weight, SB[i // 2], g, i, m, store, needs, [name] if m == 7 else [])

    def o_proj(sch, g, i, m, needs, marks):
        def store(lower, n, rows, v):
            rows = pl.ds(512 * lower + rows.start, 64)
            X[n][g, rows, :] = X[n][g, rows, :] + v
        strassen(sch, o_weight, SB[2 + i // 2], g, i, m, store, needs, marks)

    def shift_block(g, i, name, needs):
        yield _Wait(*needs)
        j, z = g + 4 * i, opaque()
        for m in range(16):
            rows = pl.ds(64 * m, 64)
            for ref, to in ((KE, KS), (VE, VS)):
                v = pltpu.roll(ref[j + 4 + z, rows, :], 1, 1)
                if ref is VE:
                    v = jnp.where(_iota(64, 1) == 0, ref[4 + z, rows, :], v)
                to[j, rows, :] = v
                if i == 3:
                    ref[g, rows, :] = v
            yield _Step(12, delay=8 if i == 3 else 4, marks=[name] if m == 15 else [])

    def transpose_quarter(w, h, via):
        for r in range(4):
            v = WRAW[w, pl.ds(256 * r, 256), pl.ds(pl.multiple_of(256 * h, 256), 256)]
            v = pltpu.bitcast(v.T, F32)
            via[0, pl.ds(256 * r, 128), :], via[0, pl.ds(256 * r + 128, 128), :] = v[:, :128], v[:, 128:]
            yield _Step(40, delay=16)

    def reorder_quarter(w, h, via, name=None):
        z = opaque()
        for c in range(8):
            WT[w][pl.ds(pl.multiple_of(128 * h, 128), 128), pl.ds(128 * c, 128)] = pltpu.bitcast(
                jnp.concatenate([via[z, pl.ds(128 * c + u, 8, stride=16), :] for u in range(16)], 0), U32)
            yield _Step(20, delay=4, marks=[name] if c == 7 else [])

    def query_weight(h):
        yield from transpose_quarter(0, h, QB[0])
        yield from reorder_quarter(0, h, QB[0], "w")

    def transpose_wo(name):
        for c in range(8):
            for h in range(4):
                v = jnp.concatenate([wou[c, pl.ds(128 * h + u, 8, stride=16), :] for u in range(16)], 0)
                WP[pl.ds(64 * c, 64), pl.ds(256 * h, 256)] = pltpu.bitcast(_bf(v).T, U32)
                yield _Step(20, delay=10, marks=[name] if c == 7 and h == 3 else [])

    def prep_spectral_weights(c2):
        lane = _iota(8, 1)
        order = jnp.where(lane > 64, 192 - lane, lane)

        def words(k2):
            re, im = (wsu[u, k2, pl.ds(c2, 64, stride=4), :] for u in range(2))
            return ((re & np.uint32(0xFFFF)) | (im << 16), (re >> 16) | (im & np.uint32(0xFFFF0000)))

        def arrange(w, below):
            w = jnp.where(_iota(w.shape[0], 1) < 64, w, below)
            return jnp.concatenate([jnp.take_along_axis(w[u:u + 8], order, axis=1)
                                    for u in range(0, w.shape[0], 8)], 0)

        below = words(15)
        for k2 in range(16):
            here = words(k2)
            for e in range(2):
                cl = 2 * c2 + e
                w = arrange(here[e], below[e])
                WS[k2, pl.ds(64 * cl, 64), :] = pltpu.roll(w, 1, 0) if cl > 4 else w
            below = here
            yield _Step(100)
        if c2 == 0:
            def nyquist(k2):
                re, im = (jnp.broadcast_to(WN[u, :, pl.ds(128 * k2, 128)].astype(F32), (8, 128))
                          for u in range(2))
                return pltpu.pack_elementwise([re, im], packed_dtype=BF16)
            for k2 in range(16):
                WS[k2, pl.ds(512, 8), :] = arrange(nyquist(k2), nyquist((k2 + 15) % 16))

    def write_out(p, c, name, needs):
        yield _Wait(*needs)
        rows = pl.ds(pl.multiple_of(128 * c, 128), 128)
        g, i = 2 * p % 4 + opaque(), p // 2
        w = pltpu.pack_elementwise([X[i][g, rows, :], X[i][g + 1, rows, :]], packed_dtype=BF16)
        xru[c, pl.ds(p, 128, stride=8), :] = w.T
        yield _Step(30, marks=[name])

    for c in range(8):
        x_copy(c).start()
    for c in range(5):
        mats[M_R + c] = d_mats[c]

    def make_twiddle(k):
        PB = temps[0][2]
        PB[0, pl.ds(0, 128), :] = lane_vec(L_TWID + k, 128)
        twid[k] = PB[opaque(), pl.ds(0, 128), :].T

    _loop(6, make_twiddle, "make_twiddle")

    def make_dft(j):
        fa, fb = lanes[pl.ds(L_FA, 128), :], lanes[pl.ds(L_FB, 128), :]
        c, sn = lane_vec(L_COS + j, 128), lane_vec(L_SIN + j, 128)
        UB, _, _, ubu, _ = temps[0]
        UB[0, pl.ds(0, 128), :] = (fa * c + fb * sn).astype(BF16)
        UB[0, pl.ds(128, 128), :] = (fb * c - fa * sn).astype(BF16)
        mats[M_FA + j], mats[M_FB + j] = ubu[0, pl.ds(0, 64), :], ubu[0, pl.ds(64, 64), :]

    _loop(NB, make_dft, "make_dft")

    def load_x(c):
        x_copy(c).wait()
        pl.when(c == 6)(lambda: start_all(spec_copies[0]))
        pl.when(c == 7)(lambda: start_all(spec_copies[1]))
        rows = pl.ds(pl.multiple_of(128 * c, 128), 128)
        for p in range(8):
            w = xru[c, pl.ds(p, 128, stride=8), :].T
            for e, bits in enumerate((w << 16, w & np.uint32(0xFFFF0000))):
                g, i = 2 * p % 4 + e, p // 2
                v = pltpu.bitcast(bits, F32)
                X[i][g, rows, :] = v
                v = v.reshape(16, 8, 128)
                mean = _all_sublanes(v.sum(0), jnp.add, 0) * (1.0 / 128)
                STAT[4 * g + i, c] = mean
                STAT[4 * g + i, 8 + c] = _all_sublanes(((v - mean) ** 2).sum(0), jnp.add, 0)

    _loop(8, load_x, "load_x")

    def after(name, action):
        yield _Wait(name)
        action()

    def spectral_weights():
        yield _Wait(("f", 2, 1))
        for c in spec_copies[0] + spec_copies[1]:
            c.wait()
        for c2 in range(4):
            yield from prep_spectral_weights(c2)

    with jax.named_scope("first_forward"):
        sch = _Sched(0.80)
        sch.add(after(("f", 0, 1), w_copies[1].start), "k")
        sch.add(after(("f", 1, 1), w_copies[2].start), "v")
        sch.add(after(("f", 2, 3), w_copies[0].start), "q")
        for g in range(4):
            for i in range(4):
                sch.add(fwd_block(g, i, ("f", g, i), [("f", g - 1, i)] if g else [],
                                  [("r", g - 1)] if g else [], True), ("f", g, i))
            sch.add(group_stage(g, ("r", g), [("f", g, i) for i in range(4)], False), ("r", g))
        sch.add(spectral_weights(), "s")
        sch.drive()
    start_all(wo_copies)

    def keys_values(layer, g):
        sch = _Sched(0.42 if layer == 0 else 0.40)
        nxt = (g + 1) % 4
        sch.add(inv_block(g, 2, ("i", 2), []), ("i", 2))
        sch.add(inv_block(g, 3, ("i", 3), [("read", ("i", 2))]), ("i", 3))
        sch.add(right_sums(SB[1], g, 2, ("b", 2), [("i", 2), ("i", 3)]), ("b", 2))
        sch.add(group_stage(nxt, "r", [("read", ("i", 3))], True), "r")
        sch.add(inv_block(nxt, 0, ("i", 4), ["r", ("i", 2)], n=g + 1), ("i", 4))
        sch.add(inv_block(nxt, 1, ("i", 5), [("read", ("i", 4)), ("i", 3)], n=g + 1), ("i", 5))
        if layer == 0:
            sch.add(query_weight(g), "w")
            sch.add(left_sums(q_weight, 128 * (g % 2), 128, ["w"]), "sums")
        for i in (2, 3):
            sch.add(shift_block((g + 3) % 4, i, ("s", i), []), ("s", i))
        for i in (0, 1):
            sch.add(shift_block(g, i, ("s", i), [("kv", 0)]), ("s", i))
        sch.add(right_sums(SB[0], g + 1, 0, ("b", 4), [("i", 4), ("i", 5), ("kv", 0)]), ("b", 4))
        kv_proj(sch, g, 0, ("kv", 0), [])
        kv_proj(sch, g, 2, ("kv", 2), [("b", 2)])
        sch.finish()

    def mix(g, after, last, write):
        sch = _Sched(0.62)
        tail = after is None
        pace = 0.36 if tail else 0.33 if last else 0.29
        ahead = [(g, 2), (g, 3)] + ([] if tail else [(after, 0), (after, 1)])
        for n, block in enumerate(ahead):
            sch.add(attend(*block, ("a", n), [[], [("a", 0)], [("a", 1), ("q", 0)], [("a", 2)]][n]),
                    ("a", n), pace=pace)
            if n % 2:
                sch.add(right_sums(SB[2 + block[1] // 2], block[0], block[1] - 1, ("b", n),
                                   [("a", n)] + ([("o", 0, 0, "all")] if n == 3 else [])), ("b", n))
        for i in () if tail else (0, 2):
            sch.add(right_sums(SB[i // 2], after, i, ("h", i), [("q", 0)] if i else []), ("h", i))
        if not last:
            sch.add(group_stage((g + 3) % 4, "r", [], False), "r")
            for i in range(4):
                sch.add(fwd_block(g, i, ("f", i), [("o", i - i % 2, 7)], ["r"]), ("f", i))
        now = 6 if last else 8
        for i in range(4 if write else 0):
            for c in (0, 4, 1, 5, 2, 6):
                sch.add(write_out(2 * i + g // 2, c, ("w", i, c), [("o", i - i % 2, 2 * (c % 4) + 1)]),
                        ("w", i, c))
        for i in (0, 2):
            for m in range(now):
                o_proj(sch, g, i, m, [("b", 1)] if i else [],
                       [("o", i, m)] + ([("o", i, 0, "all")] if m == now - 1 else []))
            if not tail:
                q_proj(sch, after, i, ("q", i), [("h", i)])
        if tail and not last:
            sch.add(group_stage(g, "s", [("f", i) for i in range(4)], False), "s")
        sch.share = 0.92
        sch.drive()

    def postponed():
        sch = _Sched(0.5)
        pairs = [(g, i) for g in range(4) for i in (0, 2)]
        for n, (g, i) in enumerate(pairs):
            sch.add(right_sums(SB[2 + i // 2], g, i, ("b", n), [("o", n - 2)] if n >= 2 else []), ("b", n))
            for c in (3, 7) if g % 2 else ():
                for e in (i, i + 1):
                    sch.add(write_out(2 * e + g // 2, c, ("w", n, c, e), [("o", n)]), ("w", n, c, e))
        for n, (g, i) in enumerate(pairs):
            for m in (6, 7):
                o_proj(sch, g, i, m, [("b", n)], [("o", n)] if m == 7 else [])
        sch.finish()

    def first_queries(layer):
        sch = _Sched(0.62)
        sch.add(right_sums(SB[0], 0, 0, ("h", 0), []), ("h", 0))
        sch.add(right_sums(SB[1], 0, 2, ("h", 2), []), ("h", 2))
        sch.add(shift_block(3, 2, "s", []), "s")
        sch.add(attend(0, 0, ("a", 0), ["q"]), ("a", 0), pace=0.4)
        sch.add(attend(0, 1, ("a", 1), [("a", 0)]), ("a", 1), pace=0.4)
        sch.add(right_sums(SB[2], 0, 0, "b", [("a", 1)]), "b")
        sch.add(shift_block(3, 3, "t", []), "t")
        if layer == 0:
            for c in wo_copies:
                c.wait()
            sch.add(transpose_wo("w"), "w")
            sch.add(left_sums(o_weight, 0, 256, ["w"]), "sums")
        q_proj(sch, 0, 0, "q", [("h", 0)])
        q_proj(sch, 0, 2, None, [("h", 2)])
        sch.finish()

    def key_value_weights():
        w_copies[1].wait()
        w_copies[2].wait()
        for h in range(6):
            for w in (1, 2):
                if h < 4:
                    list(transpose_quarter(w, h, QB[2 * (h % 2) + w - 1]))
                if 0 < h < 5:
                    list(reorder_quarter(w, h - 1, QB[2 * ((h - 1) % 2) + w - 1]))
            if h > 1:
                list(left_sums(kv_weight, 128 * (h - 2), 128))

    for layer in range(2):
        with jax.named_scope("spectral"):
            _loop(4, spectral_rows, "rows")
            if layer == 0:
                _loop(zero + 1, lambda _: key_value_weights(), "weights")
            spectral(512, 8)
        sch = _Sched(0.92)
        sch.add(group_stage(0, "r", [], True), "r")
        sch.add(inv_block(0, 0, ("i", 0), ["r"]), ("i", 0))
        sch.add(inv_block(0, 1, ("i", 1), ["r"]), ("i", 1))
        sch.add(right_sums(SB[0], 0, 0, "b", [("i", 0), ("i", 1)]), "b")
        sch.drive()
        if layer == 0:
            w_copies[0].wait()
        _loop(4, lambda g: keys_values(layer, g), "keys_values")
        first_queries(layer)
        if layer == 0:
            pl.when(never)(lambda: [spectral_rows(c % 4) for c in range(5)] and None)
        if layer == 0:
            _loop(3, lambda g: mix(g, g + 1, False, False), "mix")
            mix(3, None, False, False)
        else:
            _loop(2, lambda u: mix(2 * u, 2 - u, True, False), "mix")
            mix(1, 3, True, True)
            mix(3, None, True, True)
    for c in (0, 1, 2, 4, 5, 6):
        out_copy(c).start()
    with jax.named_scope("postponed"):
        postponed()
    for c in (3, 7):
        out_copy(c).start()
    for c in range(8):
        out_copy(c).wait()


@jax.jit
def pallas_interleave_layers__spectral_gfnet__sliding_local_dilated__prompt_kernel(
    A_x: jax.Array,
    A_w_r: jax.Array,
    A_w_i: jax.Array,
    B_x: jax.Array,
    B_wqkv: jax.Array,
    B_wo: jax.Array,
):
    del B_x
    hbm = pl.BlockSpec(memory_space=pl.ANY)
    smem = pl.BlockSpec(memory_space=pltpu.SMEM)
    out = pl.pallas_call(
        _kernel,
        out_shape=jax.ShapeDtypeStruct((S, D), BF16),
        in_specs=[smem, smem, pl.BlockSpec(), pl.BlockSpec(), hbm, hbm, hbm, hbm, hbm],
        out_specs=hbm,
        scratch_shapes=[
            pltpu.VMEM((37, 64, 128), U32),
            pltpu.VMEM((6, 128, 128), F32),
            pltpu.VMEM((NB, 16, 8, 128), F32),
            pltpu.VMEM((NB + 4, D, 128), F32),
            pltpu.VMEM((NB + 4, D, 128), F32),
            pltpu.VMEM((NB, D, 128), F32),
            pltpu.VMEM((NB, D, 128), F32),
            pltpu.VMEM((2 * NB + 1, ZR, 128), F32),
            pltpu.VMEM((9, ZR, 128), F32),
            pltpu.VMEM((NB, ZR, 128), U32),
            *4 * [pltpu.VMEM((D // 2, D), U32)],
            pltpu.VMEM((5, D // 2, D // 2), U32),
            *2 * [pltpu.VMEM((5, D // 4, D // 2), U32)],
            *4 * [pltpu.VMEM((5, D // 4, 128), U32)],
            pltpu.VMEM((8, S, 128), BF16),
            pltpu.VMEM((2, NB, D // 2, 128), BF16),
            pltpu.VMEM((2, 1, S), BF16),
            pltpu.VMEM((3, D, D), BF16),
            pltpu.VMEM((8, D, 128), BF16),
            pltpu.VMEM((1, 128, 128), F32),
            pltpu.VMEM((1, 128, 128), F32),
            pltpu.SemaphoreType.DMA((24,)),
            *2 * [pltpu.VMEM((1, D, 128), F32)],
        ] + 4 * [
            pltpu.VMEM((5, D, 128), F32),
            pltpu.VMEM((5, D, 128), BF16),
            pltpu.VMEM((1, D, 128), F32),
            pltpu.VMEM((1, D, 128), BF16),
            pltpu.VMEM((1, 1152, 128), BF16),
        ],
        compiler_params=pltpu.CompilerParams(vmem_limit_bytes=126 * 2 ** 20),
    )(_ZERO, _ROT, _MATS, _LANES, A_x.reshape(S, D), A_w_r.T, A_w_i.T, B_wqkv, B_wo)
    return out.reshape(1, S, D)
```

```python
import functools

import numpy as np

import jax
import jax.numpy as jnp
import jax.experimental.pallas as pl
import jax.experimental.pallas.tpu as pltpu

S, D, NB = 2048, 1024, 16
ZR = 576
F32, BF16, U32, I32 = jnp.float32, jnp.bfloat16, jnp.uint32, jnp.int32
EPS = 1e-5
SCALE = 32 ** -0.5
RSQ2 = float(np.sqrt(0.5))
GRAIN = 1
SETTLE = 6
LAG = 3

_S_ROWS = [(32 * u, 32) for u in range(16)] + [(512, 8)]

M_FA, M_FB, M_R, M_C4, M_RT, M_C4T, M_R0T = 0, 16, 32, 33, 34, 35, 36
L_MU, L_NU, L_KU, L_KV, L_COS, L_SIN, L_TWID, L_FA, L_FB = 0, 16, 32, 48, 64, 80, 96, 104, 232


def _bf16_bits(a):
    u = np.ascontiguousarray(a, dtype=np.float32).view(np.uint32).astype(np.uint64)
    return ((u + 0x7FFF + ((u >> 16) & 1)) >> 16).astype(np.uint32)


def _constants():
    a = np.arange(128)
    k1 = np.arange(64)
    alt = (-1.0) ** a
    lanes = np.zeros((L_FB + 128, 128))
    t = 2 * np.pi * np.outer(a, k1) / 128
    fa = np.concatenate([np.cos(t), -np.sin(t)], 1)
    fb = np.concatenate([np.sin(t), -np.cos(t)], 1)
    fa[:, 0], fb[:, 0] = RSQ2, -RSQ2
    fa[:, 64], fb[:, 64] = alt, 0.0
    lanes[L_FA:L_FA + 128], lanes[L_FB:L_FB + 128] = fa, fb
    for j in range(NB):
        ang = 2 * np.pi * j / 32 + np.pi / 32
        p, q = (_bf16_bits([np.cos(ang), np.sin(ang)]) << 16).view(np.float32).astype(np.float64)
        turn = 2 * np.pi * j * np.tile(k1, 2) / S
        lanes[L_COS + j], lanes[L_SIN + j] = np.cos(turn), np.repeat([-1.0, 1.0], 64) * np.sin(turn)
        lanes[L_COS + j, 64], lanes[L_SIN + j, 64] = p, q
        lanes[L_MU + j, 0], lanes[L_MU + j, 64] = 1.0, (q / p + p / q) / 2
        lanes[L_NU + j, 0], lanes[L_NU + j, 64] = 0.0, (q / p - p / q) / 2
        lanes[L_KU + j, 0], lanes[L_KU + j, 64] = 1.0, q / p
        lanes[L_KV + j, 0], lanes[L_KV + j, 64] = 1.0, p / q
    for k in (1, 2, 3):
        lanes[L_TWID + 2 * k - 2] = np.cos(2 * np.pi * a * k / D)
        lanes[L_TWID + 2 * k - 1] = np.sin(2 * np.pi * a * k / D)
    th = 2 * np.pi * np.outer(k1, a) / 128
    r = np.concatenate([np.cos(th), -np.sin(th)], 0)
    r[64] = alt
    th = 2 * np.pi * np.outer(2 * k1 + 1, a) / 256
    c4 = np.concatenate([np.cos(th), -np.sin(th)], 0)
    inv = 2.0 / (S * D)
    r0t = inv * r.T
    r0t[:, 0::64] *= 0.5
    rows = np.arange(128).reshape(2, 4, 16).transpose(1, 0, 2).ravel()
    bits = _bf16_bits(np.stack([r[rows], c4[rows], inv * r.T, inv * c4.T, r0t]))
    ang = 2 * np.pi * np.outer(np.arange(4), np.arange(4)).ravel() / 16
    rot = np.concatenate([np.cos(ang), np.sin(ang)]).astype(np.float32)
    return bits[:, 0::2] | (bits[:, 1::2] << 16), lanes.astype(np.float32), rot


_MATS, _LANES, _ROT = _constants()
_ZERO = np.zeros((1,), np.int32)


class _Step:
    def __init__(self, cost, anchors=(), delay=0, marks=()):
        self.cost, self.anchors, self.delay, self.marks = cost, list(anchors), delay, list(marks)


class _Wait:
    def __init__(self, *names):
        self.names = names


class _Mat:
    def __init__(self, emit):
        self.emit = emit


class _Hold:
    def __init__(self, store):
        self.store = store


class _Task:
    def __init__(self, gen, pace):
        self.gen, self.pace, self.blocked, self.not_before, self.held = gen, pace, (), 0, None
        self.allowed = 0.0


class _Sched:
    def __init__(self, share=0.0, wait=24):
        self.wait = wait
        self.share = share
        self.tasks, self.done, self.producer = [], {}, {}
        self.slot, self.credit, self.anchors, self.results = 0, 0.0, [], []
        self.fresh = False

    def add(self, gen, name, pace=99):
        self.producer[name] = self.producer["read", name] = _Task(gen, pace)
        self.tasks.append(self.producer[name])

    def _ready(self, t):
        return t.not_before <= self.slot and all(
            n in self.done and self.done[n] <= self.slot for n in t.blocked)

    def _advance(self, t, mats=True):
        item, t.held = t.held or next(t.gen, None), None
        if item is None:
            self.tasks.remove(t)
        elif isinstance(item, _Wait):
            t.blocked = item.names
        elif isinstance(item, _Hold):
            if len(self.results) >= LAG:
                item.store(self.results[-LAG])
        elif isinstance(item, _Mat):
            if mats:
                t.not_before = float("inf")
                self.fresh = False
                self.credit -= item.emit(lambda: self.point(0.0)) or 0
                t.not_before = self.slot + self.wait
            else:
                t.held, t.not_before = item, self.slot + 1
        else:
            t.blocked = ()
            t.not_before = self.slot + item.delay
            self.credit -= item.cost
            self.anchors += item.anchors
            for n in item.marks:
                self.done[n] = self.slot + item.delay
            return True

    def run(self, *names):
        while not all(n in self.done for n in names):
            for n in names:
                if n not in self.done:
                    for b in self.producer[n].blocked:
                        self.run(b)
                    self._advance(self.producer[n])

    def drive(self):
        while self.tasks:
            ready = [t for t in self.tasks if self._ready(t)]
            if not ready:
                self.slot += 1
                continue
            self.anchors, self.credit = self.anchors[-2:], 0.0
            self._advance(next((t for t in ready if t.held), ready[0]))
            self.slot -= min(self.credit, 0.0) / 60

    def finish(self):
        self.run(*[n for n in self.producer if n[0] != "read"])

    def point(self, own):
        for t in self.tasks:
            t.allowed = min(t.allowed, 0.0) + t.pace
        while True:
            t = next((t for t in self.tasks if self._ready(t) and t.allowed > 0
                      and self.credit > 0), None)
            if t is None:
                break
            if self._advance(t, self.fresh):
                t.allowed -= 1
        anchors, self.anchors = self.anchors, []
        self.credit = min(self.credit, 10.0) + 64 * self.share - own
        self.fresh = False
        self.slot += 1
        return anchors


def _dot(a, b):
    return jnp.dot(a, b, preferred_element_type=F32)


def _dot_t(a, b):
    return jax.lax.dot_general(a, b, (((1,), (1,)), ((), ())), preferred_element_type=F32)


def _bf(u):
    return pltpu.bitcast(u, BF16)


def _iota(rows, dim):
    return jax.lax.broadcasted_iota(I32, (rows, 128), dim)


def _radix4(z, inverse):
    (r0, i0), (r1, i1), (r2, i2), (r3, i3) = z
    ar, ai, cr, ci = r0 + r2, i0 + i2, r0 - r2, i0 - i2
    br, bi, dr, di = r1 + r3, i1 + i3, r1 - r3, i1 - i3
    lo, hi = (cr + di, ci - dr), (cr - di, ci + dr)
    if inverse:
        lo, hi = hi, lo
    return [(ar + br, ai + bi), lo, (ar - br, ai - bi), hi]


def _all_sublanes(v, op, axis):
    for sh in (4, 2, 1):
        v = op(v, pltpu.roll(v, sh, axis))
    return v


def _loop(n, body, name):
    def step(i, carry):
        body(i)
        return carry
    with jax.named_scope(name):
        jax.lax.fori_loop(0, n, step, 0)


def _kernel(zero_ref, rot, d_mats, lanes, x_hbm, wr_hbm, wi_hbm, wqkv_hbm, wo_hbm, out_hbm,
            mats, twid, STAT, KE, VE, KS, VS, Z, ZT, WS, WQ, WK, WV, WP, WS5, WQ5, WP5, SB0, SB1, SB2, SB3, XR, WRI, WN, WRAW, WO, PW0, PW1, sems, *split):
    zero = zero_ref[0]
    never = zero != 0
    X, HB, QB = split[2::5], split[3::5], split[4::5]
    hbu = [r.bitcast(U32) for r in HB]
    xru, wsu, wou = XR.bitcast(U32), WRI.bitcast(U32), WO.bitcast(U32)
    temps = [(ub, ab, pb, ub.bitcast(U32), ab.bitcast(U32))
             for ub, ab, pb in zip(split[5::5], split[6::5], 2 * split[:2])]
    PW, SB, WT = (PW0, PW1), (SB0, SB1, SB2, SB3), (WQ, WK, WV, WP)
    counter = [0]

    def opaque():
        counter[0] += 1
        return zero * counter[0]

    def anchor(ref):
        at = (0,) * (len(ref.shape) - 2)
        return lambda: ref[(*at, pl.ds(pl.multiple_of(zero * 8, 8), 8), pl.ds(0, 128))]

    def settle(ref):
        return _Step(2, [anchor(ref)], delay=SETTLE)

    def hold(ref, spare, row=0):
        def store(v):
            ref[spare, pl.ds(pl.multiple_of(row + zero * 8, 8), 8), :] = v
        return _Hold(store)

    def tied(load, vregs, point):
        parts = []
        for r in range(vregs):
            anchors = [a for _ in range(GRAIN) for a in point()] if r % GRAIN == 0 else []
            u = load(8 * r)
            for a in anchors:
                u = jnp.where(never, pltpu.bitcast(a(), U32), u)
            parts.append(u)
        return jnp.concatenate(parts, 0)

    def mat(i):
        return _bf(mats[i])

    def d_stage(t, which):
        UB, AB, PB, ubu, abu = temps[t]

        def emit(point):
            z = opaque()
            for c in range(8):
                lhs = mat(which(c) + opaque()) if c % 4 else _bf(
                    tied(lambda r, u=which(c) + opaque(): mats[u, pl.ds(r, 8), :], 8, point))
                PB[0, pl.ds(128 * c, 128), :] = _dot(lhs, _bf(ubu[z, pl.ds(64 * c, 64), :]))
        return _Mat(emit)

    def lane_vec(i, rows):
        return jnp.broadcast_to(lanes[pl.ds(i, 1), :], (rows, 128))

    def x_copy(c):
        return pltpu.make_async_copy(
            x_hbm.at[:, pl.ds(pl.multiple_of(128 * c, 128), 128)], XR.at[c], sems.at[c])

    def out_copy(c):
        return pltpu.make_async_copy(
            XR.at[c], out_hbm.at[:, pl.ds(pl.multiple_of(128 * c, 128), 128)], sems.at[8 + c])

    spec_copies = [[pltpu.make_async_copy(w.at[pl.ds(0, 512), pl.ds(128 * k2, 128)], WRI.at[u, k2],
                                          sems.at[16 + u]) for k2 in range(16)]
                   + [pltpu.make_async_copy(w.at[pl.ds(512, 1), :], WN.at[u], sems.at[22 + u])]
                   for u, w in enumerate((wr_hbm, wi_hbm))]

    def start_all(copies):
        for c in copies:
            c.start()
    w_copies = [pltpu.make_async_copy(wqkv_hbm.at[:, pl.ds(D * w, D)], WRAW.at[w], sems.at[18 + w])
                for w in range(3)]
    wo_copies = [pltpu.make_async_copy(wo_hbm.at[:, pl.ds(128 * c, 128)], WO.at[c], sems.at[21])
                 for c in range(8)]

    def ln_rstd(g, i, mean):
        acc, m = None, g + opaque()
        for r in range(8):
            d = X[i][m, pl.ds(128 * r, 128), :].reshape(16, 8, 128) - mean[None]
            v = (d * d).sum(0)
            acc = v if acc is None else acc + v
            if r < 7:
                yield _Step(50, [lambda acc=acc: acc], delay=3)
        rstd = jax.lax.rsqrt(_all_sublanes(acc, jnp.add, 0) * (1.0 / D) + EPS)
        yield _Step(50, delay=8)
        yield _Step(10, [lambda: rstd], delay=1)
        return rstd

    def fwd_block(g, i, name, needs, free=(), known=False):
        j, t = g + 4 * i, i
        UB, AB, PB, ubu, abu = temps[t]
        yield _Wait(*needs)
        if known:
            means, squares = STAT[4 * g + i, pl.ds(0, 8)], STAT[4 * g + i, pl.ds(8, 8)]
            mean = means.sum(0) * 0.125
            var = (squares.sum(0) + 128.0 * ((means - mean) ** 2).sum(0)) * (1.0 / D)
            rstd = jax.lax.rsqrt(var + EPS)
            yield _Step(50, delay=6)
        else:
            yield settle(X[i])
            acc, m = None, g + opaque()
            for r in range(8):
                v = X[i][m, pl.ds(128 * r, 128), :].reshape(16, 8, 128).sum(0)
                acc = v if acc is None else acc + v
                if r % 2:
                    yield _Step(35, [lambda acc=acc: acc], delay=7 if r == 7 else 3)
            mean = _all_sublanes(acc, jnp.add, 0) * (1.0 / D)
            rstd = yield from ln_rstd(g, i, mean)
        mean8, rstd = (jnp.concatenate([v, v], 0) for v in (mean * 8.0, rstd))
        z = opaque()
        for r in range(8):
            rows = pl.ds(16 * r, 16)
            x = [X[i][g + z, pl.ds(128 * b + 16 * r, 16), :] for b in range(8)]
            s = [x[b] + x[b + 4] for b in range(4)]
            d = [x[b] - x[b + 4] for b in range(4)]
            e, o = s[0] + s[2], s[1] + s[3]
            UB[0, rows, :] = ((e + o - mean8) * rstd).astype(BF16)
            UB[0, pl.ds(128 + 16 * r, 16), :] = ((e - o) * rstd).astype(BF16)
            t1, t2 = (d[1] - d[3]) * RSQ2, (d[1] + d[3]) * RSQ2
            u = {1: (d[0] + t1, d[2] + t2), 2: (s[0] - s[2], s[1] - s[3]), 3: (d[0] - t1, d[2] - t2)}
            yield _Step(34, [anchor(ubu)], delay=1)
            for k in (1, 2, 3):
                c, sn = twid[z + 2 * k - 2, rows, :] * rstd, twid[z + 2 * k - 1, rows, :] * rstd
                re, m = u[k]
                if k == 3:
                    ur, ui = re * c + m * sn, m * c - re * sn
                else:
                    ur, ui = re * c - m * sn, m * c + re * sn
                UB[0, pl.ds(256 * k + 16 * r, 16), :] = ur.astype(BF16)
                UB[0, pl.ds(256 * k + 128 + 16 * r, 16), :] = ui.astype(BF16)
                yield _Step(26, [anchor(ubu)], delay=1)
        yield settle(ubu)

        def d_forward(point):
            z = opaque()
            first = _iota(8, 0) == 0

            def stage(c):
                u = (M_C4 if c == 1 else M_R) + opaque()
                lhs = mat(u) if c % 4 else _bf(tied(lambda r: mats[u, pl.ds(r, 8), :], 8, point))
                v = _dot(lhs, _bf(ubu[z, pl.ds(64 * c, 64), :]))
                return [(v[32 * u:32 * u + 16], v[32 * u + 16:32 * u + 32]) for u in range(4)]

            def put(row, u, v, v0=None):
                if u == 0 and v0 is not None:
                    v = jnp.concatenate([jnp.where(first, v0, v[:8]), v[8:]], 0)
                AB[0, pl.ds(row + 16 * u, 16), :] = v.astype(BF16)

            for u, (p1, p2) in enumerate(stage(0)):
                put(0, u, p1)
                put(528, u, p2, 0.0)
                if u == 0:
                    put(512, 0, jnp.zeros_like(p2), p2[:8])
            for u, (p1, p2) in enumerate(stage(1)):
                put(256, u, p1)
                put(528 + 256, u, p2)
            for k in (1, 2, 3):
                for u, ((p1, p2), (q1, q2)) in enumerate(zip(stage(2 * k), stage(2 * k + 1))):
                    if k == 3:
                        pr, pi, mr, mi = p1 - q2, p2 + q1, p1 + q2, p2 - q1
                        pi0, mi0 = q1[:8], -q2[:8]
                    else:
                        pr, pi, mr, mi = p1 + q2, p2 - q1, p1 - q2, p2 + q1
                        pi0, mi0 = -q1[:8], q2[:8]
                    put(64 * k, u, pr, p1[:8])
                    put(64 * (8 - k), u, mr, p2[:8])
                    put(528 + 64 * k, u, pi, pi0)
                    put(528 + 64 * (8 - k), u, mi, mi0)
            return 190

        yield _Mat(d_forward)
        yield settle(abu)
        yield _Wait(*free)

        def s_forward(point):
            z = opaque()
            fa, fb = mat(M_FA + j + z), mat(M_FB + j + z)
            for r0, rn in ((0, 256), (256, 272)):
                lhs = abu[z, pl.ds(r0 // 2, rn // 2), :] if r0 else tied(
                    lambda r: abu[z, pl.ds(r, 8), :], 16, point)
                u = _dot(_bf(lhs), fa)
                v = _dot(_bf(abu[z, pl.ds(264 + r0 // 2, 128), :]), fb)
                re, m = u[:256] + v, u[:256] - v
                if r0:
                    re, m = (jnp.concatenate([a, u[256:264]], 0) for a in (re, m))
                rn = re.shape[0]
                edge = (_iota(rn, 1) & 63) == 0
                ZT[2 * i, pl.ds(r0, rn), :] = re
                ZT[2 * i + 1, pl.ds(r0, rn), :] = jnp.where(
                    edge, lane_vec(L_MU + j, rn) * m + lane_vec(L_NU + j, rn) * re, pltpu.roll(m, 64, 1))
            return 400

        yield _Mat(s_forward)
        yield _Step(2, [anchor(ZT)], delay=SETTLE, marks=[name])

    def group_stage(g, name, needs, inverse):
        yield _Wait(*needs)

        def turn(z, k):
            if k == 0:
                return z
            c, s = rot[4 * g + k], rot[16 + 4 * g + k]
            if inverse:
                return z[0] * c - z[1] * s, z[1] * c + z[0] * s
            return z[0] * c + z[1] * s, z[1] * c - z[0] * s

        (src, a), (dst, b) = ((Z, 8 * g), (ZT, 0)) if inverse else ((ZT, opaque()), (Z, 8 * g))
        for r in range(65):
            if r % 4 == 0:
                yield hold(src, 2 * NB if inverse else 8)
            rows = pl.ds(8 * r, 8)
            z = [(src[a + 2 * i, rows, :], src[a + 2 * i + 1, rows, :]) for i in range(4)]
            if inverse:
                z = _radix4([turn(z[k], k) for k in range(4)], True)
            else:
                z = [turn(v, k) for k, v in enumerate(_radix4(z, False))]
            for i in range(4):
                dst[b + 2 * i, rows, :], dst[b + 2 * i + 1, rows, :] = z[i]
            yield _Step(35, [anchor(dst)], delay=1, marks=[name] if r == 64 else [])

    def spectral(row, size):
        rows = pl.ds(row, size)
        for k0 in range(4):
            z = _radix4([(Z[8 * g + 2 * k0, rows, :], Z[8 * g + 2 * k0 + 1, rows, :])
                         for g in range(4)], False)
            y = []
            for k1, (re, im) in enumerate(z):
                w = WS[k0 + 4 * k1, rows, :]
                wr = pltpu.bitcast(w << 16, F32)
                wi = pltpu.bitcast(w & np.uint32(0xFFFF0000), F32)
                y.append((re * wr - im * wi, re * wi + im * wr))
            y = _radix4(y, True)
            for g in range(4):
                Z[8 * g + 2 * k0, rows, :], Z[8 * g + 2 * k0 + 1, rows, :] = y[g]

    def spectral_rows(c2):
        for r in range(8):
            spectral(pl.multiple_of(128 * c2 + 16 * r, 16), 16)

    def inv_block(g, i, name, needs, n=None):
        j, t = g + 4 * i, i % 2
        UB, AB, PB, ubu, abu = temps[t]
        n = g if n is None else n
        z = opaque()
        yield _Wait(*needs)
        for r0, rn in _S_ROWS:
            if r0 == 0:
                yield hold(ZT, 8)
            re, im = ZT[z + 2 * i, pl.ds(r0, rn), :], ZT[z + 2 * i + 1, pl.ds(r0, rn), :]
            edge = (_iota(rn, 1) & 63) == 0
            rolled = pltpu.roll(im, 64, 1)
            u = re + jnp.where(edge, lane_vec(L_KU + j, rn) * im, rolled)
            if r0 < 512:
                v = re - jnp.where(edge, lane_vec(L_KV + j, rn) * im, rolled)
                AB[0, pl.ds(r0, rn), :] = u.astype(BF16)
                AB[0, pl.ds(528 + r0, rn), :] = v.astype(BF16)
            else:
                AB[0, pl.ds(512, 16), :] = jnp.concatenate([u, jnp.zeros_like(u)], 0).astype(BF16)
            yield _Step(rn, [anchor(abu)], delay=1, marks=[("read", name)] if r0 == 512 else [])
        yield settle(abu)

        def s_inverse(point):
            z = opaque()
            fa, fb = mat(M_FA + j + z), mat(M_FB + j + z)
            first = _iota(8, 0) == 0

            def put(row, v, v0=None):
                if v0 is not None:
                    v = jnp.concatenate([jnp.where(first, v0, v[:8]), v[8:]], 0)
                UB[0, pl.ds(row, 64), :] = v.astype(BF16)

            for k in range(4):
                lo, hi = 32 * k, 32 * (8 - k if k else 4)
                a = [abu[z, pl.ds(lo, 32), :], abu[z, pl.ds(hi, 32), :]] if k % 2 else [
                    tied(lambda r, o=o: abu[z, pl.ds(o + r, 8), :], 4, point) for o in (lo, hi)]
                if k == 0:
                    a.append(abu[z, pl.ds(256, 8), :])
                re = _dot_t(_bf(jnp.concatenate(a, 0)), fa)
                im = _dot_t(_bf(jnp.concatenate(
                    [abu[z, pl.ds(264 + lo, 32), :], abu[z, pl.ds(264 + hi, 32), :]], 0)), fb)
                pr, mr, pi, mi = re[:64], re[64:128], im[:64], im[64:]
                if k == 0:
                    put(0, pr)
                    put(64, pi, re[128:136])
                    put(128, mr)
                    put(192, mi)
                else:
                    put(256 * k, pr + mr, pr[:8])
                    put(256 * k + 64, pi + mi, mr[:8])
                    put(256 * k + 128, pi - mi, pi[:8])
                    put(256 * k + 192, mr - pr, -mi[:8])
            return 190

        yield _Mat(s_inverse)
        yield settle(ubu)
        yield d_stage(t, lambda c: {0: M_R0T, 1: M_C4T}.get(c, M_RT))
        yield settle(PB)
        z = opaque()
        acc = None
        for r in range(16):
            rows = pl.ds(8 * r, 8)
            t0, t4 = PB[z, rows, :], PB[z, pl.ds(128 + 8 * r, 8), :]
            tk = {}
            for k in (1, 2, 3):
                c, sn = twid[z + 2 * k - 2, rows, :], twid[z + 2 * k - 1, rows, :]
                re = PB[z, pl.ds(256 * k + 8 * r, 8), :]
                im = PB[z, pl.ds(256 * k + 128 + 8 * r, 8), :]
                tk[k] = (re * c - im * sn, re * sn + im * c)
            e0, e1 = t0 + t4, t0 - t4
            s = [e0 + tk[2][0], e1 - tk[2][1], e0 - tk[2][0], e1 + tk[2][1]]
            al, be = tk[1][0] - tk[3][0], tk[1][1] + tk[3][1]
            o = [tk[1][0] + tk[3][0], (al - be) * RSQ2, tk[3][1] - tk[1][1], (al + be) * -RSQ2]
            for b in range(8):
                y = s[b] + o[b] if b < 4 else s[b - 4] - o[b - 4]
                v = X[i][g, pl.ds(128 * b + 8 * r, 8), :] + y
                X[i][n, pl.ds(128 * b + 8 * r, 8), :] = v
                acc = v if acc is None else acc + v
            yield _Step(57, [lambda v=acc: v], delay=5 if r == 15 else 2)
        yield settle(X[i])
        mean = _all_sublanes(acc, jnp.add, 0) * (1.0 / D)
        rstd = yield from ln_rstd(n, i, mean)
        z = opaque()
        for r in range(8):
            v = X[i][n + z, pl.ds(128 * r, 128), :].reshape(16, 8, 128)
            HB[i][n, pl.ds(128 * r, 128), :] = ((v - mean[None]) * rstd[None]).reshape(128, 128).astype(BF16)
            yield _Step(41, [anchor(hbu[i])], delay=1, marks=[name] if r == 7 else [])

    def attend(g, i, name, needs):
        yield _Wait(*needs)
        yield settle(QB[i])
        j, z = g + 4 * i, opaque()
        even = (_iota(8, 0) & 1) == 0
        edge = _iota(8, 1) == 0

        def window(near, far, w, rows):
            return near[j + z + 4 - 2 * w, rows, :] if w <= 2 * i + 2 else far[j + z + 16 - 2 * w, rows, :]

        def mix_values(h, u):
            p = PW[h % 2][opaque()]
            for rows in (pl.ds(256 * h + 16 * u, 16), pl.ds(256 * h + 16 * u + 16, 16)):
                acc = functools.reduce(jnp.add, [p[16 * w:16 * w + 16] * window(VE, VS, w, rows)
                                                 for w in range(8)])
                HB[i][g, rows, :] = acc.astype(BF16)
            return _Step(63, [anchor(hbu[i])], delay=1, marks=[name] if (h, u) == (3, 14) else [])

        for h in range(5):
            logits = []
            for w0 in range(0, 8, 2):
                if h < 4:
                    rows = pl.ds(256 * h, 256)
                    q = q if w0 % 4 else QB[i][opaque(), rows, :]
                    for w in (w0, w0 + 1):
                        v = (q * window(KE, KS, w, rows)).reshape(16, 16, 128).sum(0)
                        v = jnp.where(even, v[:8] + pltpu.roll(v[:8], 7, 0), v[8:] + pltpu.roll(v[8:], 1, 0))
                        logits.append(jnp.where(edge & (2 * w > j), -1e9, v * SCALE) if w > 2 * i
                                      else v * SCALE)
                    yield _Step(138, [lambda v=v: v for v in logits[-2:]], delay=2)
                if h > 0:
                    yield mix_values(h - 1, 2 * w0)
                    yield mix_values(h - 1, 2 * w0 + 2)
            if h < 4:
                top = functools.reduce(jnp.maximum, logits)
                e = [jnp.exp(v - top) for v in logits]
                total = functools.reduce(jnp.add, e)
                yield _Step(30, [lambda v=total: v], delay=3)
                scale = 1.0 / total
                for w in range(8):
                    v = e[w] * scale
                    PW[h % 2][0, pl.ds(16 * w, 8), :] = jnp.where(even, v, pltpu.roll(v, 1, 0))
                    PW[h % 2][0, pl.ds(16 * w + 8, 8), :] = jnp.where(even, pltpu.roll(v, 7, 0), v)
                yield _Step(50, [anchor(PW[h % 2])], delay=6 if h == 3 else 1)

    def packed_sums(terms, signs):
        lo = [pltpu.bitcast(u << 16, F32) for u in terms]
        hi = [pltpu.bitcast(u & np.uint32(0xFFFF0000), F32) for u in terms]
        return [pltpu.pack_elementwise([v[p] + v[q] if s > 0 else v[p] - v[q] for v in (lo, hi)],
                                       packed_dtype=BF16) for p, s, q in signs]

    def half(ref, row):
        return lambda r, size, cols: ref[pl.ds(pl.multiple_of(row + r, 8), size), cols]

    kv_weight = (WS5, half(WK, 0), half(WV, 0))
    q_weight = (WQ5, half(WQ, 0), half(WQ, D // 4))
    o_weight = (WP5, *(lambda r, size, cols, e=e: WP[pl.ds(r + r // 32 * 32 + e, size), cols]
                       for e in (0, 32)))

    def left_sums(weight, row, size, needs=()):
        yield _Wait(*needs)
        sums, top, bottom = weight
        for r in range(0, size, 8):
            a = [ref(row + r, 8, pl.ds(c, 512)) for ref in (top, bottom) for c in (0, 512)]
            for e, v in enumerate(packed_sums(a, ((0, 1, 3), (2, 1, 3), (0, 1, 1), (2, -1, 0), (1, -1, 3)))):
                sums[e, pl.ds(pl.multiple_of(row + r, 8), 8), :] = v
            yield _Step(92, [anchor(sums)], delay=2, marks=["sums"] if r == size - 8 else [])

    def right_sums(dst, g, i, name, needs):
        yield _Wait(*needs)
        z = g + opaque()
        for r in range(0, 256, 16):
            b = [hbu[n][z, pl.ds(k + r, 16), :] for k in (0, 256) for n in (i, i + 1)]
            for e, v in enumerate(packed_sums(b, ((0, 1, 3), (1, -1, 3), (2, -1, 0), (0, 1, 1), (2, 1, 3)))):
                dst[e, pl.ds(r, 16), :] = v
            yield _Step(47, [anchor(dst)], delay=SETTLE if r == 240 else 1,
                        marks=[name] if r == 240 else [])

    def strassen(sch, weight, right, g, i, m, store, needs, marks):
        for n in needs:
            sch.run(n)
        sums, top, bottom = weight
        rows = pl.ds(pl.multiple_of(64 * m, 64), 64)
        sch.fresh = True

        def product(left, b):
            head = tied(lambda r: left(32 * m + r, 8, pl.ds(0, 128)), 4, lambda: sch.point(8.0))
            return _dot(_bf(jnp.concatenate([head, left(32 * m, 32, pl.ds(128, 384))], 1)), _bf(b))

        def a(e):
            return lambda r, size, cols: sums[e, pl.ds(pl.multiple_of(r, 8), size), cols]

        def b(e):
            return right[e + opaque()]

        m2 = product(a(1), hbu[i][g + opaque(), pl.ds(0, 256), :])
        m4 = product(lambda r, size, cols: bottom(r, size, pl.ds(512 + cols.start, cols.size)), b(2))
        store(1, i, rows, m2 + m4)
        m1 = product(a(0), b(0))
        c11, c22 = m1 + m4, m1 - m2
        c11 = c11 + product(a(4), b(4))
        c22 = c22 + product(a(3), b(3))
        m5 = product(a(2), hbu[i + 1][g + opaque(), pl.ds(256, 256), :])
        store(0, i, rows, c11 - m5)
        v = product(top, b(1))
        store(0, i + 1, rows, v + m5)
        store(1, i + 1, rows, c22 + v)
        sch.results.append(v[:8])
        for name in marks:
            sch.done[name] = sch.slot + sch.wait

    def kv_proj(sch, g, i, name, needs):
        def store(lower, n, rows, v):
            (KE, VE)[lower][g + 4 * n + 4, rows, :] = v
        for m in range(16):
            strassen(sch, kv_weight, SB[i // 2], g, i, m, store, needs, [name] if m == 15 else [])

    def q_proj(sch, g, i, name, needs):
        def store(lower, n, rows, v):
            QB[n][0, pl.ds(512 * lower + rows.start, 64), :] = v
        for m in range(8):
            strassen(sch, q_weight, SB[i // 2], g, i, m, store, needs, [name] if m == 7 else [])

    def o_proj(sch, g, i, m, needs, marks, right):
        def store(lower, n, rows, v):
            rows = pl.ds(128 * m + 64 * lower, 64)
            X[n][g, rows, :] = X[n][g, rows, :] + v
        strassen(sch, o_weight, right, g, i, m, store, needs, marks)

    def shift_block(g, i, name, needs):
        yield _Wait(*needs)
        j, z = g + 4 * i, opaque()
        for m in range(16):
            rows = pl.ds(64 * m, 64)
            for ref, to in ((KE, KS), (VE, VS)):
                v = pltpu.roll(ref[j + 4 + z, rows, :], 1, 1)
                if ref is VE:
                    v = jnp.where(_iota(64, 1) == 0, ref[4 + z, rows, :], v)
                to[j, rows, :] = v
                if i == 3:
                    ref[g, rows, :] = v
            yield _Step(12, delay=8, marks=[name] if m == 15 else [])

    def transpose_quarter(w, h, via):
        for r in range(4):
            v = WRAW[w, pl.ds(256 * r, 256), pl.ds(pl.multiple_of(256 * h, 256), 256)]
            v = pltpu.bitcast(v.T, F32)
            via[0, pl.ds(256 * r, 128), :], via[0, pl.ds(256 * r + 128, 128), :] = v[:, :128], v[:, 128:]
            yield _Step(40, delay=16)

    def reorder_quarter(w, h, via, name=None):
        z = opaque()
        for c in range(8):
            WT[w][pl.ds(pl.multiple_of(128 * h, 128), 128), pl.ds(128 * c, 128)] = pltpu.bitcast(
                jnp.concatenate([via[z, pl.ds(128 * c + u, 8, stride=16), :] for u in range(16)], 0), U32)
            yield _Step(20, delay=4, marks=[name] if c == 7 else [])

    def query_weight(h):
        yield from transpose_quarter(0, h, QB[0])
        yield from reorder_quarter(0, h, QB[0], "w")

    def transpose_wo(name):
        for c in range(8):
            for h in range(4):
                v = jnp.concatenate([wou[c, pl.ds(128 * h + u, 8, stride=16), :] for u in range(16)], 0)
                WP[pl.ds(64 * c, 64), pl.ds(256 * h, 256)] = pltpu.bitcast(_bf(v).T, U32)
                yield _Step(20, delay=10, marks=[name] if c == 7 and h == 3 else [])

    def prep_spectral_weights(c2):
        lane = _iota(8, 1)
        order = jnp.where(lane > 64, 192 - lane, lane)

        def words(k2):
            re, im = (wsu[u, k2, pl.ds(c2, 64, stride=4), :] for u in range(2))
            return ((re & np.uint32(0xFFFF)) | (im << 16), (re >> 16) | (im & np.uint32(0xFFFF0000)))

        def arrange(w, below):
            w = jnp.where(_iota(w.shape[0], 1) < 64, w, below)
            return jnp.concatenate([jnp.take_along_axis(w[u:u + 8], order, axis=1)
                                    for u in range(0, w.shape[0], 8)], 0)

        below = words(15)
        for k2 in range(16):
            here = words(k2)
            for e in range(2):
                cl = 2 * c2 + e
                w = arrange(here[e], below[e])
                WS[k2, pl.ds(64 * cl, 64), :] = pltpu.roll(w, 1, 0) if cl > 4 else w
            below = here
            yield _Step(100)
        if c2 == 0:
            def nyquist(k2):
                re, im = (jnp.broadcast_to(WN[u, :, pl.ds(128 * k2, 128)].astype(F32), (8, 128))
                          for u in range(2))
                return pltpu.pack_elementwise([re, im], packed_dtype=BF16)
            for k2 in range(16):
                WS[k2, pl.ds(512, 8), :] = arrange(nyquist(k2), nyquist((k2 + 15) % 16))

    def write_out(p, c, name, needs):
        yield _Wait(*needs)
        rows = pl.ds(pl.multiple_of(128 * c, 128), 128)
        g, i = 2 * p % 4 + opaque(), p // 2
        w = pltpu.pack_elementwise([X[i][g, rows, :], X[i][g + 1, rows, :]], packed_dtype=BF16)
        xru[c, pl.ds(p, 128, stride=8), :] = w.T
        yield _Step(30, marks=[name])

    for c in range(8):
        x_copy(c).start()
    for c in range(5):
        mats[M_R + c] = d_mats[c]

    def make_twiddle(k):
        PB = temps[0][2]
        PB[0, pl.ds(0, 128), :] = lane_vec(L_TWID + k, 128)
        twid[k] = PB[opaque(), pl.ds(0, 128), :].T

    _loop(6, make_twiddle, "make_twiddle")

    def make_dft(j):
        fa, fb = lanes[pl.ds(L_FA, 128), :], lanes[pl.ds(L_FB, 128), :]
        c, sn = lane_vec(L_COS + j, 128), lane_vec(L_SIN + j, 128)
        UB, _, _, ubu, _ = temps[0]
        UB[0, pl.ds(0, 128), :] = (fa * c + fb * sn).astype(BF16)
        UB[0, pl.ds(128, 128), :] = (fb * c - fa * sn).astype(BF16)
        mats[M_FA + j], mats[M_FB + j] = ubu[0, pl.ds(0, 64), :], ubu[0, pl.ds(64, 64), :]

    _loop(NB, make_dft, "make_dft")

    def load_x(c):
        x_copy(c).wait()
        pl.when(c == 6)(lambda: start_all(spec_copies[0]))
        pl.when(c == 7)(lambda: start_all(spec_copies[1]))
        rows = pl.ds(pl.multiple_of(128 * c, 128), 128)
        for p in range(8):
            w = xru[c, pl.ds(p, 128, stride=8), :].T
            for e, bits in enumerate((w << 16, w & np.uint32(0xFFFF0000))):
                g, i = 2 * p % 4 + e, p // 2
                v = pltpu.bitcast(bits, F32)
                X[i][g, rows, :] = v
                v = v.reshape(16, 8, 128)
                mean = _all_sublanes(v.sum(0), jnp.add, 0) * (1.0 / 128)
                STAT[4 * g + i, c] = mean
                STAT[4 * g + i, 8 + c] = _all_sublanes(((v - mean) ** 2).sum(0), jnp.add, 0)

    _loop(8, load_x, "load_x")

    def after(name, action):
        yield _Wait(name)
        action()

    def spectral_weights():
        yield _Wait(("f", 2, 1))
        for c in spec_copies[0] + spec_copies[1]:
            c.wait()
        for c2 in range(4):
            yield from prep_spectral_weights(c2)

    with jax.named_scope("first_forward"):
        sch = _Sched(0.80)
        sch.add(after(("f", 0, 1), w_copies[1].start), "k")
        sch.add(after(("f", 1, 1), w_copies[2].start), "v")
        sch.add(after(("f", 2, 3), w_copies[0].start), "q")
        for g in range(4):
            for i in range(4):
                sch.add(fwd_block(g, i, ("f", g, i), [("f", g - 1, i)] if g else [],
                                  [("r", g - 1)] if g else [], True), ("f", g, i))
            sch.add(group_stage(g, ("r", g), [("f", g, i) for i in range(4)], False), ("r", g))
        sch.add(spectral_weights(), "s")
        sch.drive()
    start_all(wo_copies)

    def keys_values(layer, g):
        sch = _Sched(0.42 if layer == 0 else 0.40, 32)
        nxt = (g + 1) % 4
        sch.add(inv_block(g, 2, ("i", 2), []), ("i", 2))
        sch.add(inv_block(g, 3, ("i", 3), [("read", ("i", 2))]), ("i", 3))
        sch.add(right_sums(SB[1], g, 2, ("b", 2), [("i", 2), ("i", 3)]), ("b", 2))
        sch.add(group_stage(nxt, "r", [("read", ("i", 3))], True), "r")
        sch.add(inv_block(nxt, 0, ("i", 4), ["r", ("i", 2)], n=g + 1), ("i", 4))
        sch.add(inv_block(nxt, 1, ("i", 5), [("read", ("i", 4)), ("i", 3)], n=g + 1), ("i", 5))
        if layer == 0:
            sch.add(query_weight(g), "w")
            sch.add(left_sums(q_weight, 128 * (g % 2), 128, ["w"]), "sums")
        for i in (2, 3):
            sch.add(shift_block((g + 3) % 4, i, ("s", i), []), ("s", i))
        for i in (0, 1):
            sch.add(shift_block(g, i, ("s", i), [("kv", 0)]), ("s", i))
        sch.add(right_sums(SB[0], g + 1, 0, ("b", 4), [("i", 4), ("i", 5), ("kv", 0)]), ("b", 4))
        kv_proj(sch, g, 0, ("kv", 0), [])
        kv_proj(sch, g, 2, ("kv", 2), [("b", 2)])
        sch.finish()

    def mix(g, after, last, write):
        sch = _Sched(0.66 if last else 0.62)
        tail = after is None
        pace = 0.36 if tail else 0.35 if last else 0.31
        ahead = [(g, 2), (g, 3)] + ([] if tail else [(after, 0), (after, 1)])
        for n, block in enumerate(ahead):
            sch.add(attend(*block, ("a", n), [[], [("a", 0)], [("a", 1), ("q", 0)], [("a", 2)]][n]),
                    ("a", n), pace=pace)
            if n % 2:
                sch.add(right_sums(SB[2 + block[1] // 2], block[0], block[1] - 1, ("b", n),
                                   [("a", n)] + ([("o", 0, 0, "all")] if n == 3 else [])), ("b", n))
        for i in () if tail else (0, 2):
            sch.add(right_sums(SB[i // 2], after, i, ("h", i), [("q", 0)] if i else []), ("h", i))
        if not last:
            sch.add(group_stage((g + 3) % 4, "r", [], False), "r")
            for i in range(4):
                sch.add(fwd_block(g, i, ("f", i), [("o", i - i % 2, 7)], ["r"]), ("f", i))
        now = 6 if last else 8
        for i in range(4 if write else 0):
            for c in range(now):
                sch.add(write_out(2 * i + g // 2, c, ("w", i, c), [("o", i - i % 2, c)]), ("w", i, c))
        for i in (0, 2):
            for m in range(now):
                o_proj(sch, g, i, m, [("b", 1)] if i else [],
                       [("o", i, m)] + ([("o", i, 0, "all")] if m == now - 1 else []), SB[2 + i // 2])
            if not tail:
                q_proj(sch, after, i, ("q", i), [("h", i)])
        if tail and not last:
            sch.add(group_stage(g, "s", [("f", i) for i in range(4)], False), "s")
        sch.share = 0.92
        sch.drive()

    def postponed(c):
        sch = _Sched(0.6, 12)
        pairs = [(g, i) for i in (0, 2) for g in range(4)]
        for n, (g, i) in enumerate(pairs):
            sch.add(right_sums(SB[n % 4], g, i, ("b", n), [("o", n - 4)] if n >= 4 else []), ("b", n))
            for e in (i, i + 1) if g % 2 else ():
                sch.add(write_out(2 * e + g // 2, c, ("w", n, e), [("o", n)]), ("w", n, e))
        for n, (g, i) in enumerate(pairs):
            o_proj(sch, g, i, c, [("b", n)], [("o", n)], SB[n % 4])
        sch.finish()
        out_copy(c).start()

    def first_queries(layer):
        sch = _Sched(0.62)
        sch.add(right_sums(SB[0], 0, 0, ("h", 0), []), ("h", 0))
        sch.add(right_sums(SB[1], 0, 2, ("h", 2), []), ("h", 2))
        sch.add(shift_block(3, 2, "s", []), "s")
        sch.add(attend(0, 0, ("a", 0), ["q"]), ("a", 0), pace=0.4)
        sch.add(attend(0, 1, ("a", 1), [("a", 0)]), ("a", 1), pace=0.4)
        sch.add(right_sums(SB[2], 0, 0, "b", [("a", 1)]), "b")
        sch.add(shift_block(3, 3, "t", []), "t")
        if layer == 0:
            for c in wo_copies:
                c.wait()
            sch.add(transpose_wo("w"), "w")
            sch.add(left_sums(o_weight, 0, 256, ["w"]), "sums")
        q_proj(sch, 0, 0, "q", [("h", 0)])
        q_proj(sch, 0, 2, None, [("h", 2)])
        sch.finish()

    def key_value_weights():
        w_copies[1].wait()
        w_copies[2].wait()
        for h in range(6):
            for w in (1, 2):
                if h < 4:
                    list(transpose_quarter(w, h, QB[2 * (h % 2) + w - 1]))
                if 0 < h < 5:
                    list(reorder_quarter(w, h - 1, QB[2 * ((h - 1) % 2) + w - 1]))
            if h > 1:
                list(left_sums(kv_weight, 128 * (h - 2), 128))

    for layer in range(2):
        with jax.named_scope("spectral"):
            _loop(4, spectral_rows, "rows")
            if layer == 0:
                _loop(zero + 1, lambda _: key_value_weights(), "weights")
            spectral(512, 8)
        sch = _Sched(0.92)
        sch.add(group_stage(0, "r", [], True), "r")
        sch.add(inv_block(0, 0, ("i", 0), ["r"]), ("i", 0))
        sch.add(inv_block(0, 1, ("i", 1), ["r"]), ("i", 1))
        sch.add(right_sums(SB[0], 0, 0, "b", [("i", 0), ("i", 1)]), "b")
        sch.drive()
        if layer == 0:
            w_copies[0].wait()
        _loop(4, lambda g: keys_values(layer, g), "keys_values")
        first_queries(layer)
        if layer == 0:
            pl.when(never)(lambda: [spectral_rows(c % 4) for c in range(5)] and None)
        if layer == 0:
            _loop(3, lambda g: mix(g, g + 1, False, False), "mix")
            mix(3, None, False, False)
        else:
            _loop(2, lambda u: mix(2 * u, 2 - u, True, False), "mix")
            mix(1, 3, True, True)
            mix(3, None, True, True)
    for c in range(6):
        out_copy(c).start()
    with jax.named_scope("postponed"):
        postponed(6)
        postponed(7)
    for c in range(8):
        out_copy(c).wait()


@jax.jit
def pallas_interleave_layers__spectral_gfnet__sliding_local_dilated__prompt_kernel(
    A_x: jax.Array,
    A_w_r: jax.Array,
    A_w_i: jax.Array,
    B_x: jax.Array,
    B_wqkv: jax.Array,
    B_wo: jax.Array,
):
    del B_x
    hbm = pl.BlockSpec(memory_space=pl.ANY)
    smem = pl.BlockSpec(memory_space=pltpu.SMEM)
    out = pl.pallas_call(
        _kernel,
        out_shape=jax.ShapeDtypeStruct((S, D), BF16),
        in_specs=[smem, smem, pl.BlockSpec(), pl.BlockSpec(), hbm, hbm, hbm, hbm, hbm],
        out_specs=hbm,
        scratch_shapes=[
            pltpu.VMEM((37, 64, 128), U32),
            pltpu.VMEM((6, 128, 128), F32),
            pltpu.VMEM((NB, 16, 8, 128), F32),
            pltpu.VMEM((NB + 4, D, 128), F32),
            pltpu.VMEM((NB + 4, D, 128), F32),
            pltpu.VMEM((NB, D, 128), F32),
            pltpu.VMEM((NB, D, 128), F32),
            pltpu.VMEM((2 * NB + 1, ZR, 128), F32),
            pltpu.VMEM((9, ZR, 128), F32),
            pltpu.VMEM((NB, ZR, 128), U32),
            *4 * [pltpu.VMEM((D // 2, D), U32)],
            pltpu.VMEM((5, D // 2, D // 2), U32),
            *2 * [pltpu.VMEM((5, D // 4, D // 2), U32)],
            *4 * [pltpu.VMEM((5, D // 4, 128), U32)],
            pltpu.VMEM((8, S, 128), BF16),
            pltpu.VMEM((2, NB, D // 2, 128), BF16),
            pltpu.VMEM((2, 1, S), BF16),
            pltpu.VMEM((3, D, D), BF16),
            pltpu.VMEM((8, D, 128), BF16),
            pltpu.VMEM((1, 128, 128), F32),
            pltpu.VMEM((1, 128, 128), F32),
            pltpu.SemaphoreType.DMA((24,)),
            *2 * [pltpu.VMEM((1, D, 128), F32)],
        ] + 4 * [
            pltpu.VMEM((5, D, 128), F32),
            pltpu.VMEM((5, D, 128), BF16),
            pltpu.VMEM((1, D, 128), F32),
            pltpu.VMEM((1, D, 128), BF16),
            pltpu.VMEM((1, 1152, 128), BF16),
        ],
        compiler_params=pltpu.CompilerParams(vmem_limit_bytes=126 * 2 ** 20),
    )(_ZERO, _ROT, _MATS, _LANES, A_x.reshape(S, D), A_w_r.T, A_w_i.T, B_wqkv, B_wo)
    return out.reshape(1, S, D)
```

```python
import functools
import itertools

import numpy as np

import jax
import jax.numpy as jnp
import jax.experimental.pallas as pl
import jax.experimental.pallas.tpu as pltpu

S, D, NB = 2048, 1024, 16
ZR = 576
F32, BF16, U32, I32 = jnp.float32, jnp.bfloat16, jnp.uint32, jnp.int32
EPS = 1e-5
SCALE = 32 ** -0.5
RSQ2 = float(np.sqrt(0.5))
GRAIN = 1
SETTLE = 6
LAG = 3

_S_ROWS = [(32 * u, 32) for u in range(16)] + [(512, 8)]

M_FA, M_FB, M_R, M_C4, M_RT, M_C4T, M_R0T = 0, 16, 32, 33, 34, 35, 36
L_MU, L_NU, L_KU, L_KV, L_COS, L_SIN, L_TWID, L_FA, L_FB = 0, 16, 32, 48, 64, 80, 96, 104, 232


def _bf16_bits(a):
    u = np.ascontiguousarray(a, dtype=np.float32).view(np.uint32).astype(np.uint64)
    return ((u + 0x7FFF + ((u >> 16) & 1)) >> 16).astype(np.uint32)


def _constants():
    a = np.arange(128)
    k1 = np.arange(64)
    alt = (-1.0) ** a
    lanes = np.zeros((L_FB + 128, 128))
    t = 2 * np.pi * np.outer(a, k1) / 128
    fa = np.concatenate([np.cos(t), -np.sin(t)], 1)
    fb = np.concatenate([np.sin(t), -np.cos(t)], 1)
    fa[:, 0], fb[:, 0] = RSQ2, -RSQ2
    fa[:, 64], fb[:, 64] = alt, 0.0
    lanes[L_FA:L_FA + 128], lanes[L_FB:L_FB + 128] = fa, fb
    for j in range(NB):
        ang = 2 * np.pi * j / 32 + np.pi / 32
        p, q = (_bf16_bits([np.cos(ang), np.sin(ang)]) << 16).view(np.float32).astype(np.float64)
        turn = 2 * np.pi * j * np.tile(k1, 2) / S
        lanes[L_COS + j], lanes[L_SIN + j] = np.cos(turn), np.repeat([-1.0, 1.0], 64) * np.sin(turn)
        lanes[L_COS + j, 64], lanes[L_SIN + j, 64] = p, q
        lanes[L_MU + j, 0], lanes[L_MU + j, 64] = 1.0, (q / p + p / q) / 2
        lanes[L_NU + j, 0], lanes[L_NU + j, 64] = 0.0, (q / p - p / q) / 2
        lanes[L_KU + j, 0], lanes[L_KU + j, 64] = 1.0, q / p
        lanes[L_KV + j, 0], lanes[L_KV + j, 64] = 1.0, p / q
    for k in (1, 2, 3):
        lanes[L_TWID + 2 * k - 2] = np.cos(2 * np.pi * a * k / D)
        lanes[L_TWID + 2 * k - 1] = np.sin(2 * np.pi * a * k / D)
    th = 2 * np.pi * np.outer(k1, a) / 128
    r = np.concatenate([np.cos(th), -np.sin(th)], 0)
    r[64] = alt
    th = 2 * np.pi * np.outer(2 * k1 + 1, a) / 256
    c4 = np.concatenate([np.cos(th), -np.sin(th)], 0)
    inv = 2.0 / (S * D)
    r0t = inv * r.T
    r0t[:, 0::64] *= 0.5
    rows = np.arange(128).reshape(2, 4, 16).transpose(1, 0, 2).ravel()
    bits = _bf16_bits(np.stack([r[rows], c4[rows], inv * r.T, inv * c4.T, r0t]))
    ang = 2 * np.pi * np.outer(np.arange(4), np.arange(4)).ravel() / 16
    rot = np.concatenate([np.cos(ang), np.sin(ang)]).astype(np.float32)
    return bits[:, 0::2] | (bits[:, 1::2] << 16), lanes.astype(np.float32), rot


_MATS, _LANES, _ROT = _constants()
_ZERO = np.zeros((1,), np.int32)


class _Step:
    def __init__(self, cost, anchors=(), delay=0, marks=()):
        self.cost, self.anchors, self.delay, self.marks = cost, list(anchors), delay, list(marks)


class _Wait:
    def __init__(self, *names):
        self.names = names


class _Mat:
    def __init__(self, emit):
        self.emit = emit


class _Hold:
    def __init__(self, store):
        self.store = store


class _Task:
    def __init__(self, gen, pace):
        self.gen, self.pace, self.blocked, self.not_before, self.held = gen, pace, (), 0, None
        self.allowed = 0.0


class _Sched:
    def __init__(self, share=0.0, wait=24):
        self.wait = wait
        self.share = share
        self.tasks, self.done, self.producer = [], {}, {}
        self.slot, self.credit, self.anchors, self.results = 0, 0.0, [], []
        self.fresh = False

    def add(self, gen, name, pace=99):
        self.producer[name] = self.producer["read", name] = _Task(gen, pace)
        self.tasks.append(self.producer[name])

    def _ready(self, t):
        return t.not_before <= self.slot and all(
            n in self.done and self.done[n] <= self.slot for n in t.blocked)

    def _advance(self, t, mats=True):
        item, t.held = t.held or next(t.gen, None), None
        if item is None:
            self.tasks.remove(t)
        elif isinstance(item, _Wait):
            t.blocked = item.names
        elif isinstance(item, _Hold):
            if len(self.results) >= LAG:
                item.store(self.results[-LAG])
        elif isinstance(item, _Mat):
            if mats:
                t.not_before = float("inf")
                self.fresh = False
                self.credit -= item.emit(lambda: self.point(0.0)) or 0
                t.not_before = self.slot + self.wait
            else:
                t.held, t.not_before = item, self.slot + 1
        else:
            t.blocked = ()
            t.not_before = self.slot + item.delay
            self.credit -= item.cost
            self.anchors += item.anchors
            for n in item.marks:
                self.done[n] = self.slot + item.delay
            return True

    def run(self, *names):
        while not all(n in self.done for n in names):
            for n in names:
                if n not in self.done:
                    for b in self.producer[n].blocked:
                        self.run(b)
                    self._advance(self.producer[n])

    def drive(self):
        while self.tasks:
            ready = [t for t in self.tasks if self._ready(t)]
            if not ready:
                self.slot += 1
                continue
            self.anchors, self.credit = self.anchors[-2:], 0.0
            self._advance(next((t for t in ready if t.held), ready[0]))
            self.slot -= min(self.credit, 0.0) / 60

    def finish(self):
        self.run(*[n for n in self.producer if n[0] != "read"])

    def point(self, own):
        for t in self.tasks:
            t.allowed = min(t.allowed, 0.0) + t.pace
        while True:
            t = next((t for t in self.tasks if self._ready(t) and t.allowed > 0
                      and self.credit > 0), None)
            if t is None:
                break
            if self._advance(t, self.fresh):
                t.allowed -= 1
        anchors, self.anchors = self.anchors, []
        self.credit = min(self.credit, 10.0) + 64 * self.share - own
        self.fresh = False
        self.slot += 1
        return anchors


def _dot(a, b):
    return jnp.dot(a, b, preferred_element_type=F32)


def _dot_t(a, b):
    return jax.lax.dot_general(a, b, (((1,), (1,)), ((), ())), preferred_element_type=F32)


def _bf(u):
    return pltpu.bitcast(u, BF16)


def _iota(rows, dim):
    return jax.lax.broadcasted_iota(I32, (rows, 128), dim)


def _radix4(z, inverse):
    (r0, i0), (r1, i1), (r2, i2), (r3, i3) = z
    ar, ai, cr, ci = r0 + r2, i0 + i2, r0 - r2, i0 - i2
    br, bi, dr, di = r1 + r3, i1 + i3, r1 - r3, i1 - i3
    lo, hi = (cr + di, ci - dr), (cr - di, ci + dr)
    if inverse:
        lo, hi = hi, lo
    return [(ar + br, ai + bi), lo, (ar - br, ai - bi), hi]


def _all_sublanes(v, op, axis):
    for sh in (4, 2, 1):
        v = op(v, pltpu.roll(v, sh, axis))
    return v


def _loop(n, body, name):
    def step(i, carry):
        body(i)
        return carry
    with jax.named_scope(name):
        jax.lax.fori_loop(0, n, step, 0)


def _kernel(zero_ref, rot, d_mats, lanes, x_hbm, wr_hbm, wi_hbm, wqkv_hbm, wo_hbm, out_hbm,
            mats, twid, STAT, KE, VE, KS, VS, Z, ZT, WS, WQ, WK, WV, WP, WS5, WQ5, WP5, SB0, SB1, SB2, SB3, XR, WRI, WN, WRAW, WO, PW0, PW1, sems, *split):
    zero = zero_ref[0]
    never = zero != 0
    X, HB, QB = split[2::5], split[3::5], split[4::5]
    hbu = [r.bitcast(U32) for r in HB]
    xru, wsu, wou = XR.bitcast(U32), WRI.bitcast(U32), WO.bitcast(U32)
    temps = [(ub, ab, pb, ub.bitcast(U32), ab.bitcast(U32))
             for ub, ab, pb in zip(split[5::5], split[6::5], 2 * split[:2])]
    PW, SB, WT = (PW0, PW1), (SB0, SB1, SB2, SB3), (WQ, WK, WV, WP)
    counter = [0]

    def opaque():
        counter[0] += 1
        return zero * counter[0]

    def anchor(ref):
        at = (0,) * (len(ref.shape) - 2)
        return lambda: ref[(*at, pl.ds(pl.multiple_of(zero * 8, 8), 8), pl.ds(0, 128))]

    def settle(ref):
        return _Step(2, [anchor(ref)], delay=SETTLE)

    def hold(ref, spare, row=0):
        def store(v):
            ref[spare, pl.ds(pl.multiple_of(row + zero * 8, 8), 8), :] = v
        return _Hold(store)

    def tied(load, vregs, point):
        parts = []
        for r in range(vregs):
            anchors = [a for _ in range(GRAIN) for a in point()] if r % GRAIN == 0 else []
            u = load(8 * r)
            for a in anchors:
                u = jnp.where(never, pltpu.bitcast(a(), U32), u)
            parts.append(u)
        return jnp.concatenate(parts, 0)

    def mat(i):
        return _bf(mats[i])

    def d_stage(t, which):
        UB, AB, PB, ubu, abu = temps[t]

        def emit(point):
            z = opaque()
            for c in range(8):
                lhs = mat(which(c) + opaque()) if c % 4 else _bf(
                    tied(lambda r, u=which(c) + opaque(): mats[u, pl.ds(r, 8), :], 8, point))
                PB[0, pl.ds(128 * c, 128), :] = _dot(lhs, _bf(ubu[z, pl.ds(64 * c, 64), :]))
        return _Mat(emit)

    def lane_vec(i, rows):
        return jnp.broadcast_to(lanes[pl.ds(i, 1), :], (rows, 128))

    def x_copy(c):
        return pltpu.make_async_copy(
            x_hbm.at[:, pl.ds(pl.multiple_of(128 * c, 128), 128)], XR.at[c], sems.at[c])

    def out_copy(c):
        return pltpu.make_async_copy(
            XR.at[c], out_hbm.at[:, pl.ds(pl.multiple_of(128 * c, 128), 128)], sems.at[8 + c])

    spec_copies = [[pltpu.make_async_copy(w.at[pl.ds(0, 512), pl.ds(128 * k2, 128)], WRI.at[u, k2],
                                          sems.at[16 + u]) for k2 in range(16)]
                   + [pltpu.make_async_copy(w.at[pl.ds(512, 1), :], WN.at[u], sems.at[22 + u])]
                   for u, w in enumerate((wr_hbm, wi_hbm))]

    def start_all(copies):
        for c in copies:
            c.start()
    w_copies = [pltpu.make_async_copy(wqkv_hbm.at[:, pl.ds(D * w, D)], WRAW.at[w], sems.at[18 + w])
                for w in range(3)]
    wo_copies = [pltpu.make_async_copy(wo_hbm.at[:, pl.ds(128 * c, 128)], WO.at[c], sems.at[21])
                 for c in range(8)]

    def ln_rstd(g, i, mean):
        acc, m = None, g + opaque()
        for r in range(8):
            d = X[i][m, pl.ds(128 * r, 128), :].reshape(16, 8, 128) - mean[None]
            v = (d * d).sum(0)
            acc = v if acc is None else acc + v
            if r < 7:
                yield _Step(50, [lambda acc=acc: acc], delay=3)
        rstd = jax.lax.rsqrt(_all_sublanes(acc, jnp.add, 0) * (1.0 / D) + EPS)
        yield _Step(50, delay=8)
        yield _Step(10, [lambda: rstd], delay=1)
        return rstd

    def fwd_block(g, i, name, needs, free=(), known=False):
        j, t = g + 4 * i, i
        UB, AB, PB, ubu, abu = temps[t]
        yield _Wait(*needs)
        if known:
            means, squares = STAT[4 * g + i, pl.ds(0, 8)], STAT[4 * g + i, pl.ds(8, 8)]
            mean = means.sum(0) * 0.125
            var = (squares.sum(0) + 128.0 * ((means - mean) ** 2).sum(0)) * (1.0 / D)
            rstd = jax.lax.rsqrt(var + EPS)
            yield _Step(50, delay=6)
        else:
            yield settle(X[i])
            acc, m = None, g + opaque()
            for r in range(8):
                v = X[i][m, pl.ds(128 * r, 128), :].reshape(16, 8, 128).sum(0)
                acc = v if acc is None else acc + v
                if r % 2:
                    yield _Step(35, [lambda acc=acc: acc], delay=7 if r == 7 else 3)
            mean = _all_sublanes(acc, jnp.add, 0) * (1.0 / D)
            rstd = yield from ln_rstd(g, i, mean)
        mean8, rstd = (jnp.concatenate([v, v], 0) for v in (mean * 8.0, rstd))
        z = opaque()
        for r in range(8):
            rows = pl.ds(16 * r, 16)
            x = [X[i][g + z, pl.ds(128 * b + 16 * r, 16), :] for b in range(8)]
            s = [x[b] + x[b + 4] for b in range(4)]
            d = [x[b] - x[b + 4] for b in range(4)]
            e, o = s[0] + s[2], s[1] + s[3]
            UB[0, rows, :] = ((e + o - mean8) * rstd).astype(BF16)
            UB[0, pl.ds(128 + 16 * r, 16), :] = ((e - o) * rstd).astype(BF16)
            t1, t2 = (d[1] - d[3]) * RSQ2, (d[1] + d[3]) * RSQ2
            u = {1: (d[0] + t1, d[2] + t2), 2: (s[0] - s[2], s[1] - s[3]), 3: (d[0] - t1, d[2] - t2)}
            yield _Step(34, [anchor(ubu)], delay=1)
            for k in (1, 2, 3):
                c, sn = twid[z + 2 * k - 2, rows, :] * rstd, twid[z + 2 * k - 1, rows, :] * rstd
                re, m = u[k]
                if k == 3:
                    ur, ui = re * c + m * sn, m * c - re * sn
                else:
                    ur, ui = re * c - m * sn, m * c + re * sn
                UB[0, pl.ds(256 * k + 16 * r, 16), :] = ur.astype(BF16)
                UB[0, pl.ds(256 * k + 128 + 16 * r, 16), :] = ui.astype(BF16)
                yield _Step(26, [anchor(ubu)], delay=1)
        yield settle(ubu)

        def d_forward(point):
            z = opaque()
            first = _iota(8, 0) == 0

            def stage(c):
                u = (M_C4 if c == 1 else M_R) + opaque()
                lhs = mat(u) if c % 4 else _bf(tied(lambda r: mats[u, pl.ds(r, 8), :], 8, point))
                v = _dot(lhs, _bf(ubu[z, pl.ds(64 * c, 64), :]))
                return [(v[32 * u:32 * u + 16], v[32 * u + 16:32 * u + 32]) for u in range(4)]

            def put(row, u, v, v0=None):
                if u == 0 and v0 is not None:
                    v = jnp.concatenate([jnp.where(first, v0, v[:8]), v[8:]], 0)
                AB[0, pl.ds(row + 16 * u, 16), :] = v.astype(BF16)

            for u, (p1, p2) in enumerate(stage(0)):
                put(0, u, p1)
                put(528, u, p2, 0.0)
                if u == 0:
                    put(512, 0, jnp.zeros_like(p2), p2[:8])
            for u, (p1, p2) in enumerate(stage(1)):
                put(256, u, p1)
                put(528 + 256, u, p2)
            for k in (1, 2, 3):
                for u, ((p1, p2), (q1, q2)) in enumerate(zip(stage(2 * k), stage(2 * k + 1))):
                    if k == 3:
                        pr, pi, mr, mi = p1 - q2, p2 + q1, p1 + q2, p2 - q1
                        pi0, mi0 = q1[:8], -q2[:8]
                    else:
                        pr, pi, mr, mi = p1 + q2, p2 - q1, p1 - q2, p2 + q1
                        pi0, mi0 = -q1[:8], q2[:8]
                    put(64 * k, u, pr, p1[:8])
                    put(64 * (8 - k), u, mr, p2[:8])
                    put(528 + 64 * k, u, pi, pi0)
                    put(528 + 64 * (8 - k), u, mi, mi0)
            return 190

        yield _Mat(d_forward)
        yield settle(abu)
        yield _Wait(*free)

        def s_forward(point):
            z = opaque()
            fa, fb = mat(M_FA + j + z), mat(M_FB + j + z)
            for r0, rn in ((0, 256), (256, 272)):
                lhs = abu[z, pl.ds(r0 // 2, rn // 2), :] if r0 else tied(
                    lambda r: abu[z, pl.ds(r, 8), :], 16, point)
                u = _dot(_bf(lhs), fa)
                v = _dot(_bf(abu[z, pl.ds(264 + r0 // 2, 128), :]), fb)
                re, m = u[:256] + v, u[:256] - v
                if r0:
                    re, m = (jnp.concatenate([a, u[256:264]], 0) for a in (re, m))
                rn = re.shape[0]
                edge = (_iota(rn, 1) & 63) == 0
                ZT[2 * i, pl.ds(r0, rn), :] = re
                ZT[2 * i + 1, pl.ds(r0, rn), :] = jnp.where(
                    edge, lane_vec(L_MU + j, rn) * m + lane_vec(L_NU + j, rn) * re, pltpu.roll(m, 64, 1))
            return 400

        yield _Mat(s_forward)
        yield _Step(2, [anchor(ZT)], delay=SETTLE, marks=[name])

    def group_stage(g, name, needs, inverse):
        yield _Wait(*needs)

        def turn(z, k):
            if k == 0:
                return z
            c, s = rot[4 * g + k], rot[16 + 4 * g + k]
            if inverse:
                return z[0] * c - z[1] * s, z[1] * c + z[0] * s
            return z[0] * c + z[1] * s, z[1] * c - z[0] * s

        (src, a), (dst, b) = ((Z, 8 * g), (ZT, 0)) if inverse else ((ZT, opaque()), (Z, 8 * g))
        for r in range(65):
            if r % 4 == 0:
                yield hold(src, 2 * NB if inverse else 8)
            rows = pl.ds(8 * r, 8)
            z = [(src[a + 2 * i, rows, :], src[a + 2 * i + 1, rows, :]) for i in range(4)]
            if inverse:
                z = _radix4([turn(z[k], k) for k in range(4)], True)
            else:
                z = [turn(v, k) for k, v in enumerate(_radix4(z, False))]
            for i in range(4):
                dst[b + 2 * i, rows, :], dst[b + 2 * i + 1, rows, :] = z[i]
            yield _Step(35, [anchor(dst)], delay=1, marks=[name] if r == 64 else [])

    def spectral(row, size):
        rows = pl.ds(row, size)
        for k0 in range(4):
            z = _radix4([(Z[8 * g + 2 * k0, rows, :], Z[8 * g + 2 * k0 + 1, rows, :])
                         for g in range(4)], False)
            y = []
            for k1, (re, im) in enumerate(z):
                w = WS[k0 + 4 * k1, rows, :]
                wr = pltpu.bitcast(w << 16, F32)
                wi = pltpu.bitcast(w & np.uint32(0xFFFF0000), F32)
                y.append((re * wr - im * wi, re * wi + im * wr))
            y = _radix4(y, True)
            for g in range(4):
                Z[8 * g + 2 * k0, rows, :], Z[8 * g + 2 * k0 + 1, rows, :] = y[g]

    def spectral_rows(c2):
        for r in range(8):
            spectral(pl.multiple_of(128 * c2 + 16 * r, 16), 16)

    def inv_block(g, i, name, needs, n=None):
        j, t = g + 4 * i, i % 2
        UB, AB, PB, ubu, abu = temps[t]
        n = g if n is None else n
        z = opaque()
        yield _Wait(*needs)
        for r0, rn in _S_ROWS:
            if r0 == 0:
                yield hold(ZT, 8)
            re, im = ZT[z + 2 * i, pl.ds(r0, rn), :], ZT[z + 2 * i + 1, pl.ds(r0, rn), :]
            edge = (_iota(rn, 1) & 63) == 0
            rolled = pltpu.roll(im, 64, 1)
            u = re + jnp.where(edge, lane_vec(L_KU + j, rn) * im, rolled)
            if r0 < 512:
                v = re - jnp.where(edge, lane_vec(L_KV + j, rn) * im, rolled)
                AB[0, pl.ds(r0, rn), :] = u.astype(BF16)
                AB[0, pl.ds(528 + r0, rn), :] = v.astype(BF16)
            else:
                AB[0, pl.ds(512, 16), :] = jnp.concatenate([u, jnp.zeros_like(u)], 0).astype(BF16)
            yield _Step(rn, [anchor(abu)], delay=1, marks=[("read", name)] if r0 == 512 else [])
        yield settle(abu)

        def s_inverse(point):
            z = opaque()
            fa, fb = mat(M_FA + j + z), mat(M_FB + j + z)
            first = _iota(8, 0) == 0

            def put(row, v, v0=None):
                if v0 is not None:
                    v = jnp.concatenate([jnp.where(first, v0, v[:8]), v[8:]], 0)
                UB[0, pl.ds(row, 64), :] = v.astype(BF16)

            for k in range(4):
                lo, hi = 32 * k, 32 * (8 - k if k else 4)
                a = [abu[z, pl.ds(lo, 32), :], abu[z, pl.ds(hi, 32), :]] if k % 2 else [
                    tied(lambda r, o=o: abu[z, pl.ds(o + r, 8), :], 4, point) for o in (lo, hi)]
                if k == 0:
                    a.append(abu[z, pl.ds(256, 8), :])
                re = _dot_t(_bf(jnp.concatenate(a, 0)), fa)
                im = _dot_t(_bf(jnp.concatenate(
                    [abu[z, pl.ds(264 + lo, 32), :], abu[z, pl.ds(264 + hi, 32), :]], 0)), fb)
                pr, mr, pi, mi = re[:64], re[64:128], im[:64], im[64:]
                if k == 0:
                    put(0, pr)
                    put(64, pi, re[128:136])
                    put(128, mr)
                    put(192, mi)
                else:
                    put(256 * k, pr + mr, pr[:8])
                    put(256 * k + 64, pi + mi, mr[:8])
                    put(256 * k + 128, pi - mi, pi[:8])
                    put(256 * k + 192, mr - pr, -mi[:8])
            return 190

        yield _Mat(s_inverse)
        yield settle(ubu)
        yield d_stage(t, lambda c: {0: M_R0T, 1: M_C4T}.get(c, M_RT))
        yield settle(PB)
        z = opaque()
        acc = None
        for r in range(16):
            rows = pl.ds(8 * r, 8)
            t0, t4 = PB[z, rows, :], PB[z, pl.ds(128 + 8 * r, 8), :]
            tk = {}
            for k in (1, 2, 3):
                c, sn = twid[z + 2 * k - 2, rows, :], twid[z + 2 * k - 1, rows, :]
                re = PB[z, pl.ds(256 * k + 8 * r, 8), :]
                im = PB[z, pl.ds(256 * k + 128 + 8 * r, 8), :]
                tk[k] = (re * c - im * sn, re * sn + im * c)
            e0, e1 = t0 + t4, t0 - t4
            s = [e0 + tk[2][0], e1 - tk[2][1], e0 - tk[2][0], e1 + tk[2][1]]
            al, be = tk[1][0] - tk[3][0], tk[1][1] + tk[3][1]
            o = [tk[1][0] + tk[3][0], (al - be) * RSQ2, tk[3][1] - tk[1][1], (al + be) * -RSQ2]
            for b in range(8):
                y = s[b] + o[b] if b < 4 else s[b - 4] - o[b - 4]
                v = X[i][g, pl.ds(128 * b + 8 * r, 8), :] + y
                X[i][n, pl.ds(128 * b + 8 * r, 8), :] = v
                acc = v if acc is None else acc + v
            yield _Step(57, [lambda v=acc: v], delay=5 if r == 15 else 2)
        yield settle(X[i])
        mean = _all_sublanes(acc, jnp.add, 0) * (1.0 / D)
        rstd = yield from ln_rstd(n, i, mean)
        z = opaque()
        for r in range(8):
            v = X[i][n + z, pl.ds(128 * r, 128), :].reshape(16, 8, 128)
            HB[i][n, pl.ds(128 * r, 128), :] = ((v - mean[None]) * rstd[None]).reshape(128, 128).astype(BF16)
            yield _Step(41, [anchor(hbu[i])], delay=1, marks=[name] if r == 7 else [])

    def attend(g, i, name, needs):
        yield _Wait(*needs)
        yield settle(QB[i])
        j, z = g + 4 * i, opaque()
        even = (_iota(8, 0) & 1) == 0
        edge = _iota(8, 1) == 0

        def window(near, far, w, rows):
            return near[j + z + 4 - 2 * w, rows, :] if w <= 2 * i + 2 else far[j + z + 16 - 2 * w, rows, :]

        def mix_values(h, u):
            p = PW[h % 2][opaque()]
            for rows in (pl.ds(256 * h + 16 * u, 16), pl.ds(256 * h + 16 * u + 16, 16)):
                acc = functools.reduce(jnp.add, [p[16 * w:16 * w + 16] * window(VE, VS, w, rows)
                                                 for w in range(8)])
                HB[i][g, rows, :] = acc.astype(BF16)
            return _Step(63, [anchor(hbu[i])], delay=1, marks=[name] if (h, u) == (3, 14) else [])

        for h in range(5):
            logits = []
            for w0 in range(0, 8, 2):
                if h < 4:
                    rows = pl.ds(256 * h, 256)
                    q = q if w0 % 4 else QB[i][opaque(), rows, :]
                    for w in (w0, w0 + 1):
                        v = (q * window(KE, KS, w, rows)).reshape(16, 16, 128).sum(0)
                        v = jnp.where(even, v[:8] + pltpu.roll(v[:8], 7, 0), v[8:] + pltpu.roll(v[8:], 1, 0))
                        logits.append(jnp.where(edge & (2 * w > j), -1e9, v * SCALE) if w > 2 * i
                                      else v * SCALE)
                    yield _Step(138, [lambda v=v: v for v in logits[-2:]], delay=2)
                if h > 0:
                    yield mix_values(h - 1, 2 * w0)
                    yield mix_values(h - 1, 2 * w0 + 2)
            if h < 4:
                top = functools.reduce(jnp.maximum, logits)
                e = [jnp.exp(v - top) for v in logits]
                total = functools.reduce(jnp.add, e)
                yield _Step(30, [lambda v=total: v], delay=3)
                scale = 1.0 / total
                for w in range(8):
                    v = e[w] * scale
                    PW[h % 2][0, pl.ds(16 * w, 8), :] = jnp.where(even, v, pltpu.roll(v, 1, 0))
                    PW[h % 2][0, pl.ds(16 * w + 8, 8), :] = jnp.where(even, pltpu.roll(v, 7, 0), v)
                yield _Step(50, [anchor(PW[h % 2])], delay=6 if h == 3 else 1)

    def packed_sums(terms, signs):
        lo = [pltpu.bitcast(u << 16, F32) for u in terms]
        hi = [pltpu.bitcast(u & np.uint32(0xFFFF0000), F32) for u in terms]
        return [pltpu.pack_elementwise([v[p] + v[q] if s > 0 else v[p] - v[q] for v in (lo, hi)],
                                       packed_dtype=BF16) for p, s, q in signs]

    def half(ref, row):
        return lambda r, size, cols: ref[pl.ds(pl.multiple_of(row + r, 8), size), cols]

    kv_weight = (WS5, half(WK, 0), half(WV, 0))
    q_weight = (WQ5, half(WQ, 0), half(WQ, D // 4))
    o_weight = (WP5, *(lambda r, size, cols, e=e: WP[pl.ds(r + r // 32 * 32 + e, size), cols]
                       for e in (0, 32)))

    def left_sums(weight, row, size, needs=()):
        yield _Wait(*needs)
        sums, top, bottom = weight
        for r in range(0, size, 8):
            a = [ref(row + r, 8, pl.ds(c, 512)) for ref in (top, bottom) for c in (0, 512)]
            for e, v in enumerate(packed_sums(a, ((0, 1, 3), (2, 1, 3), (0, 1, 1), (2, -1, 0), (1, -1, 3)))):
                sums[e, pl.ds(pl.multiple_of(row + r, 8), 8), :] = v
            yield _Step(92, [anchor(sums)], delay=2, marks=["sums"] if r == size - 8 else [])

    def right_sums(dst, g, i, name, needs):
        yield _Wait(*needs)
        z = g + opaque()
        for r in range(0, 256, 16):
            b = [hbu[n][z, pl.ds(k + r, 16), :] for k in (0, 256) for n in (i, i + 1)]
            for e, v in enumerate(packed_sums(b, ((0, 1, 3), (1, -1, 3), (2, -1, 0), (0, 1, 1), (2, 1, 3)))):
                dst[e, pl.ds(r, 16), :] = v
            yield _Step(47, [anchor(dst)], delay=SETTLE if r == 240 else 1,
                        marks=[name] if r == 240 else [])

    def strassen(sch, weight, right, g, i, m, store, needs, marks):
        for n in needs:
            sch.run(n)
        sums, top, bottom = weight
        rows = pl.ds(pl.multiple_of(64 * m, 64), 64)
        sch.fresh = True

        def product(left, b):
            head = tied(lambda r: left(32 * m + r, 8, pl.ds(0, 128)), 4, lambda: sch.point(8.0))
            return _dot(_bf(jnp.concatenate([head, left(32 * m, 32, pl.ds(128, 384))], 1)), _bf(b))

        def a(e):
            return lambda r, size, cols: sums[e, pl.ds(pl.multiple_of(r, 8), size), cols]

        def b(e):
            return right[e + opaque()]

        m2 = product(a(1), hbu[i][g + opaque(), pl.ds(0, 256), :])
        m4 = product(lambda r, size, cols: bottom(r, size, pl.ds(512 + cols.start, cols.size)), b(2))
        store(1, i, rows, m2 + m4)
        m1 = product(a(0), b(0))
        c11, c22 = m1 + m4, m1 - m2
        c11 = c11 + product(a(4), b(4))
        c22 = c22 + product(a(3), b(3))
        m5 = product(a(2), hbu[i + 1][g + opaque(), pl.ds(256, 256), :])
        store(0, i, rows, c11 - m5)
        v = product(top, b(1))
        store(0, i + 1, rows, v + m5)
        store(1, i + 1, rows, c22 + v)
        sch.results.append(v[:8])
        for name in marks:
            sch.done[name] = sch.slot + sch.wait

    def kv_proj(sch, g, i, name, needs):
        def store(lower, n, rows, v):
            (KE, VE)[lower][g + 4 * n + 4, rows, :] = v
        for m in range(16):
            strassen(sch, kv_weight, SB[i // 2], g, i, m, store, needs, [name] if m == 15 else [])

    def q_proj(sch, g, i, name, needs):
        def store(lower, n, rows, v):
            QB[n][0, pl.ds(512 * lower + rows.start, 64), :] = v
        for m in range(8):
            strassen(sch, q_weight, SB[i // 2], g, i, m, store, needs, [name] if m == 7 else [])

    def o_proj(sch, g, i, m, needs, marks, right):
        def store(lower, n, rows, v):
            rows = pl.ds(128 * m + 64 * lower, 64)
            X[n][g, rows, :] = X[n][g, rows, :] + v
        strassen(sch, o_weight, right, g, i, m, store, needs, marks)

    def shift_block(g, i, name, needs):
        yield _Wait(*needs)
        j, z = g + 4 * i, opaque()
        for m in range(16):
            rows = pl.ds(64 * m, 64)
            for ref, to in ((KE, KS), (VE, VS)):
                v = pltpu.roll(ref[j + 4 + z, rows, :], 1, 1)
                if ref is VE:
                    v = jnp.where(_iota(64, 1) == 0, ref[4 + z, rows, :], v)
                to[j, rows, :] = v
                if i == 3:
                    ref[g, rows, :] = v
            yield _Step(12, delay=8, marks=[name] if m == 15 else [])

    def transpose_quarter(w, h, via):
        for r in range(4):
            v = WRAW[w, pl.ds(256 * r, 256), pl.ds(pl.multiple_of(256 * h, 256), 256)]
            v = pltpu.bitcast(v.T, F32)
            via[0, pl.ds(256 * r, 128), :], via[0, pl.ds(256 * r + 128, 128), :] = v[:, :128], v[:, 128:]
            yield _Step(40, delay=16)

    def reorder_quarter(w, h, via, name=None):
        z = 0 if isinstance(h, int) else opaque()
        for c in range(8):
            WT[w][pl.ds(pl.multiple_of(128 * h, 128), 128), pl.ds(128 * c, 128)] = pltpu.bitcast(
                jnp.concatenate([via[z, pl.ds(128 * c + u, 8, stride=16), :] for u in range(16)], 0), U32)
            yield _Step(20, delay=4, marks=[name] if c == 7 else [])

    def query_weight(h):
        yield from transpose_quarter(0, h, QB[0])
        yield from reorder_quarter(0, h, QB[0], "w")

    def transpose_wo(name):
        for c in range(8):
            for h in range(4):
                v = jnp.concatenate([wou[c, pl.ds(128 * h + u, 8, stride=16), :] for u in range(16)], 0)
                WP[pl.ds(64 * c, 64), pl.ds(256 * h, 256)] = pltpu.bitcast(_bf(v).T, U32)
                yield _Step(20, delay=10, marks=[name] if c == 7 and h == 3 else [])

    def prep_spectral_weights(c2):
        lane = _iota(8, 1)
        order = jnp.where(lane > 64, 192 - lane, lane)

        def words(k2):
            re, im = (wsu[u, k2, pl.ds(c2, 64, stride=4), :] for u in range(2))
            return ((re & np.uint32(0xFFFF)) | (im << 16), (re >> 16) | (im & np.uint32(0xFFFF0000)))

        def arrange(w, below):
            w = jnp.where(_iota(w.shape[0], 1) < 64, w, below)
            return jnp.concatenate([jnp.take_along_axis(w[u:u + 8], order, axis=1)
                                    for u in range(0, w.shape[0], 8)], 0)

        below = words(15)
        for k2 in range(16):
            here = words(k2)
            for e in range(2):
                cl = 2 * c2 + e
                w = arrange(here[e], below[e])
                WS[k2, pl.ds(64 * cl, 64), :] = pltpu.roll(w, 1, 0) if cl > 4 else w
            below = here
            yield _Step(100)
        if c2 == 0:
            def nyquist(k2):
                re, im = (jnp.broadcast_to(WN[u, :, pl.ds(128 * k2, 128)].astype(F32), (8, 128))
                          for u in range(2))
                return pltpu.pack_elementwise([re, im], packed_dtype=BF16)
            for k2 in range(16):
                WS[k2, pl.ds(512, 8), :] = arrange(nyquist(k2), nyquist((k2 + 15) % 16))

    def write_out(p, c, name, needs):
        yield _Wait(*needs)
        rows = pl.ds(pl.multiple_of(128 * c, 128), 128)
        g, i = 2 * p % 4 + opaque(), p // 2
        w = pltpu.pack_elementwise([X[i][g, rows, :], X[i][g + 1, rows, :]], packed_dtype=BF16)
        xru[c, pl.ds(p, 128, stride=8), :] = w.T
        yield _Step(30, marks=[name])

    for c in range(8):
        x_copy(c).start()
    for c in range(5):
        mats[M_R + c] = d_mats[c]

    def make_twiddle(k):
        PB = temps[0][2]
        PB[0, pl.ds(0, 128), :] = lane_vec(L_TWID + k, 128)
        twid[k] = PB[opaque(), pl.ds(0, 128), :].T

    _loop(6, make_twiddle, "make_twiddle")

    def make_dft(j):
        fa, fb = lanes[pl.ds(L_FA, 128), :], lanes[pl.ds(L_FB, 128), :]
        c, sn = lane_vec(L_COS + j, 128), lane_vec(L_SIN + j, 128)
        UB, _, _, ubu, _ = temps[0]
        UB[0, pl.ds(0, 128), :] = (fa * c + fb * sn).astype(BF16)
        UB[0, pl.ds(128, 128), :] = (fb * c - fa * sn).astype(BF16)
        mats[M_FA + j], mats[M_FB + j] = ubu[0, pl.ds(0, 64), :], ubu[0, pl.ds(64, 64), :]

    _loop(NB, make_dft, "make_dft")

    def load_x(c):
        x_copy(c).wait()
        pl.when(c == 6)(lambda: start_all(spec_copies[0]))
        pl.when(c == 7)(lambda: start_all(spec_copies[1]))
        rows = pl.ds(pl.multiple_of(128 * c, 128), 128)
        for p in range(8):
            w = xru[c, pl.ds(p, 128, stride=8), :].T
            for e, bits in enumerate((w << 16, w & np.uint32(0xFFFF0000))):
                g, i = 2 * p % 4 + e, p // 2
                v = pltpu.bitcast(bits, F32)
                X[i][g, rows, :] = v
                v = v.reshape(16, 8, 128)
                mean = _all_sublanes(v.sum(0), jnp.add, 0) * (1.0 / 128)
                STAT[4 * g + i, c] = mean
                STAT[4 * g + i, 8 + c] = _all_sublanes(((v - mean) ** 2).sum(0), jnp.add, 0)

    _loop(8, load_x, "load_x")

    def after(name, action):
        yield _Wait(name)
        action()

    def spectral_weights():
        yield _Wait(("f", 2, 1))
        for c in spec_copies[0] + spec_copies[1]:
            c.wait()
        for c2 in range(4):
            yield from prep_spectral_weights(c2)

    with jax.named_scope("first_forward"):
        sch = _Sched(0.80)
        sch.add(after(("f", 0, 1), w_copies[1].start), "k")
        sch.add(after(("f", 1, 1), w_copies[2].start), "v")
        sch.add(after(("f", 2, 3), w_copies[0].start), "q")
        for g in range(4):
            for i in range(4):
                sch.add(fwd_block(g, i, ("f", g, i), [("f", g - 1, i)] if g else [],
                                  [("r", g - 1)] if g else [], True), ("f", g, i))
            sch.add(group_stage(g, ("r", g), [("f", g, i) for i in range(4)], False), ("r", g))
        sch.add(spectral_weights(), "s")
        sch.drive()
    start_all(wo_copies)

    def keys_values(layer, g):
        sch = _Sched(0.42 if layer == 0 else 0.40, 32)
        nxt = (g + 1) % 4
        sch.add(inv_block(g, 2, ("i", 2), []), ("i", 2))
        sch.add(inv_block(g, 3, ("i", 3), [("read", ("i", 2))]), ("i", 3))
        sch.add(right_sums(SB[1], g, 2, ("b", 2), [("i", 2), ("i", 3)]), ("b", 2))
        sch.add(group_stage(nxt, "r", [("read", ("i", 3))], True), "r")
        sch.add(inv_block(nxt, 0, ("i", 4), ["r", ("i", 2)], n=g + 1), ("i", 4))
        sch.add(inv_block(nxt, 1, ("i", 5), [("read", ("i", 4)), ("i", 3)], n=g + 1), ("i", 5))
        if layer == 0:
            sch.add(query_weight(g), "w")
            sch.add(left_sums(q_weight, 128 * (g % 2), 128, ["w"]), "sums")
        for i in (2, 3):
            sch.add(shift_block((g + 3) % 4, i, ("s", i), []), ("s", i))
        for i in (0, 1):
            sch.add(shift_block(g, i, ("s", i), [("kv", 0)]), ("s", i))
        sch.add(right_sums(SB[0], g + 1, 0, ("b", 4), [("i", 4), ("i", 5), ("kv", 0)]), ("b", 4))
        kv_proj(sch, g, 0, ("kv", 0), [])
        kv_proj(sch, g, 2, ("kv", 2), [("b", 2)])
        sch.finish()

    def mix(g, after, last):
        sch = _Sched(0.66 if last else 0.62)
        tail = after is None
        pace = 0.42 if tail else 0.35 if last else 0.31
        ahead = [(g, 2), (g, 3)] + ([] if tail else [(after, 0), (after, 1)])
        for n, block in enumerate(ahead):
            sch.add(attend(*block, ("a", n), [[], [("a", 0)], [("a", 1), ("q", 0)], [("a", 2)]][n]),
                    ("a", n), pace=pace)
            if n % 2:
                sch.add(right_sums(SB[2 + block[1] // 2], block[0], block[1] - 1, ("b", n),
                                   [("a", n)] + ([("o", 0)] if n == 3 else [])), ("b", n))
        for i in () if tail else (0, 2):
            sch.add(right_sums(SB[i // 2], after, i, ("h", i), [("q", 0)] if i else []), ("h", i))
        if not last:
            sch.add(group_stage((g + 3) % 4, "r", [], False), "r")
            for i in range(4):
                sch.add(fwd_block(g, i, ("f", i), [("o", i - i % 2)], ["r"]), ("f", i))
        now = 6 if last else 8
        for i in (0, 2):
            for m in range(now):
                o_proj(sch, g, i, m, [("b", 1)] if i else [], [("o", i)] if m == now - 1 else [],
                       SB[2 + i // 2])
            if not tail:
                q_proj(sch, after, i, ("q", i), [("h", i)])
        if tail:
            sch.add(group_stage(g, "s", [("f", i) for i in range(4)], False), "s")
        sch.share = 0.92
        sch.drive()

    def mix_odd():
        sch = _Sched(0.66)
        blocks = [(1, 2), (1, 3), (3, 0), (3, 1), (3, 2), (3, 3)]
        for n, (g, i) in enumerate(blocks):
            sch.add(attend(g, i, ("a", n), ([("a", n - 1)] if n else []) + ([("q", i)] if n in (2, 4) else [])),
                    ("a", n), pace=0.32)
            if n % 2:
                sch.add(right_sums(SB[(3, 2, 0)[n // 2]], g, i - 1, ("b", g, i - 1),
                                   [("a", n)] + ([("o", 1, 0, 5)] if n > 1 else [])), ("b", g, i - 1))
        for i in (0, 2):
            sch.add(right_sums(SB[i // 2], 3, i, ("h", i), []), ("h", i))
        for g in (1, 3):
            for i in range(4):
                for c in range(6):
                    sch.add(write_out(2 * i + g // 2, c, ("w", g, i, c), [("o", g, i - i % 2, c)]),
                            ("w", g, i, c))
        for g, i, slot, count in ((1, 0, 2, 6), (1, 2, 3, 8), (3, 0, 2, 8), (3, 2, 0, 6)):
            for m in range(count):
                o_proj(sch, g, i, m, [("b", g, i)] if (g, i) != (1, 0) else [], [("o", g, i, m)], SB[slot])
            for e in (0, 2) if (g, i) == (1, 0) else ():
                q_proj(sch, 3, e, ("q", e), [("h", e)] + ([("a", 1)] if e else []))
        sch.share = 0.92
        sch.drive()

    def postponed():
        sch = _Sched(0.7, 12)
        slots = {(3, 2): 0, (2, 2): 1, (0, 2): 2, (2, 0): 3, (0, 0): 0, (1, 0): 1}
        for n, (pair, slot) in enumerate(slots.items()):
            if n:
                sch.add(right_sums(SB[slot], *pair, pair, [(list(slots)[n - 4], 7)] if n >= 4 else []), pair)
        for p, pairs in enumerate(2 * [[(0, 0), (1, 0)], [(2, 0)]] + 2 * [[(0, 2)], [(2, 2), (3, 2)]]):
            for c in (6, 7):
                sch.add(write_out(p, c, ("w", p, c), [(pair, c) for pair in pairs]), ("w", p, c))

        def copy_out():
            yield _Wait(*[("w", p, 6) for p in range(8)])
            out_copy(6).start()

        sch.add(copy_out(), "copy")
        for part in (list(slots)[:2], list(slots)[2:]):
            for c in (6, 7):
                for pair in part:
                    o_proj(sch, *pair, c, [pair] if pair != (3, 2) else [], [(pair, c)], SB[slots[pair]])
        sch.drive()
        out_copy(7).start()

    def first_queries(layer):
        sch = _Sched(0.62)
        sch.add(right_sums(SB[0], 0, 0, ("h", 0), []), ("h", 0))
        sch.add(right_sums(SB[1], 0, 2, ("h", 2), []), ("h", 2))
        sch.add(shift_block(3, 2, "s", []), "s")
        sch.add(attend(0, 0, ("a", 0), ["q"]), ("a", 0), pace=0.4)
        sch.add(attend(0, 1, ("a", 1), [("a", 0)]), ("a", 1), pace=0.4)
        sch.add(right_sums(SB[2], 0, 0, "b", [("a", 1)]), "b")
        sch.add(shift_block(3, 3, "t", []), "t")
        if layer == 0:
            for c in wo_copies:
                c.wait()
            sch.add(transpose_wo("w"), "w")
            sch.add(left_sums(o_weight, 0, 256, ["w"]), "sums")
        q_proj(sch, 0, 0, "q", [("h", 0)])
        q_proj(sch, 0, 2, None, [("h", 2)])
        sch.finish()

    def key_value_weights():
        w_copies[1].wait()
        w_copies[2].wait()
        for h in range(6):
            work = []
            for w in (1, 2):
                if h < 4:
                    work.append(transpose_quarter(w, h, QB[2 * (h % 2) + w - 1]))
                if 0 < h < 5:
                    work.append(reorder_quarter(w, h - 1, QB[2 * ((h - 1) % 2) + w - 1]))
            if h > 1:
                work.append(left_sums(kv_weight, 128 * (h - 2), 128))
            list(itertools.zip_longest(*work))

    for layer in range(2):
        with jax.named_scope("spectral"):
            _loop(4, spectral_rows, "rows")
            if layer == 0:
                _loop(zero + 1, lambda _: key_value_weights(), "weights")
            spectral(512, 8)
        sch = _Sched(0.92)
        sch.add(group_stage(0, "r", [], True), "r")
        sch.add(inv_block(0, 0, ("i", 0), ["r"]), ("i", 0))
        sch.add(inv_block(0, 1, ("i", 1), ["r"]), ("i", 1))
        sch.add(right_sums(SB[0], 0, 0, "b", [("i", 0), ("i", 1)]), "b")
        sch.drive()
        if layer == 0:
            w_copies[0].wait()
        _loop(4, lambda g: keys_values(layer, g), "keys_values")
        first_queries(layer)
        if layer == 0:
            pl.when(never)(lambda: [spectral_rows(c % 4) for c in range(5)] and None)
        if layer == 0:
            _loop(3, lambda g: mix(g, g + 1, False), "mix")
            mix(3, None, False)
        else:
            _loop(2, lambda u: mix(2 * u, 2 - u, True), "mix")
            mix_odd()
    for c in range(6):
        out_copy(c).start()
    with jax.named_scope("postponed"):
        postponed()
    for c in range(8):
        out_copy(c).wait()


@jax.jit
def pallas_interleave_layers__spectral_gfnet__sliding_local_dilated__prompt_kernel(
    A_x: jax.Array,
    A_w_r: jax.Array,
    A_w_i: jax.Array,
    B_x: jax.Array,
    B_wqkv: jax.Array,
    B_wo: jax.Array,
):
    del B_x
    hbm = pl.BlockSpec(memory_space=pl.ANY)
    smem = pl.BlockSpec(memory_space=pltpu.SMEM)
    out = pl.pallas_call(
        _kernel,
        out_shape=jax.ShapeDtypeStruct((S, D), BF16),
        in_specs=[smem, smem, pl.BlockSpec(), pl.BlockSpec(), hbm, hbm, hbm, hbm, hbm],
        out_specs=hbm,
        scratch_shapes=[
            pltpu.VMEM((37, 64, 128), U32),
            pltpu.VMEM((6, 128, 128), F32),
            pltpu.VMEM((NB, 16, 8, 128), F32),
            pltpu.VMEM((NB + 4, D, 128), F32),
            pltpu.VMEM((NB + 4, D, 128), F32),
            pltpu.VMEM((NB, D, 128), F32),
            pltpu.VMEM((NB, D, 128), F32),
            pltpu.VMEM((2 * NB + 1, ZR, 128), F32),
            pltpu.VMEM((9, ZR, 128), F32),
            pltpu.VMEM((NB, ZR, 128), U32),
            *4 * [pltpu.VMEM((D // 2, D), U32)],
            pltpu.VMEM((5, D // 2, D // 2), U32),
            *2 * [pltpu.VMEM((5, D // 4, D // 2), U32)],
            *4 * [pltpu.VMEM((5, D // 4, 128), U32)],
            pltpu.VMEM((8, S, 128), BF16),
            pltpu.VMEM((2, NB, D // 2, 128), BF16),
            pltpu.VMEM((2, 1, S), BF16),
            pltpu.VMEM((3, D, D), BF16),
            pltpu.VMEM((8, D, 128), BF16),
            pltpu.VMEM((1, 128, 128), F32),
            pltpu.VMEM((1, 128, 128), F32),
            pltpu.SemaphoreType.DMA((24,)),
            *2 * [pltpu.VMEM((1, D, 128), F32)],
        ] + 4 * [
            pltpu.VMEM((5, D, 128), F32),
            pltpu.VMEM((5, D, 128), BF16),
            pltpu.VMEM((1, D, 128), F32),
            pltpu.VMEM((1, D, 128), BF16),
            pltpu.VMEM((1, 1152, 128), BF16),
        ],
        compiler_params=pltpu.CompilerParams(vmem_limit_bytes=126 * 2 ** 20),
    )(_ZERO, _ROT, _MATS, _LANES, A_x.reshape(S, D), A_w_r.T, A_w_i.T, B_wqkv, B_wo)
    return out.reshape(1, S, D)
```

```python
import functools
import itertools

import numpy as np

import jax
import jax.numpy as jnp
import jax.experimental.pallas as pl
import jax.experimental.pallas.tpu as pltpu

S, D, NB = 2048, 1024, 16
ZR = 576
F32, BF16, U32, I32 = jnp.float32, jnp.bfloat16, jnp.uint32, jnp.int32
EPS = 1e-5
SCALE = 32 ** -0.5
RSQ2 = float(np.sqrt(0.5))
GRAIN = 1
SETTLE = 4
LAG = 3

_S_ROWS = [(32 * u, 32) for u in range(16)] + [(512, 8)]

M_FA, M_FB, M_R, M_C4, M_RT, M_C4T, M_R0T = 0, 16, 32, 33, 34, 35, 36
L_MU, L_NU, L_KU, L_KV, L_COS, L_SIN, L_TWID, L_FA, L_FB = 0, 16, 32, 48, 64, 80, 96, 104, 232


def _bf16_bits(a):
    u = np.ascontiguousarray(a, dtype=np.float32).view(np.uint32).astype(np.uint64)
    return ((u + 0x7FFF + ((u >> 16) & 1)) >> 16).astype(np.uint32)


def _constants():
    a = np.arange(128)
    k1 = np.arange(64)
    alt = (-1.0) ** a
    lanes = np.zeros((L_FB + 128, 128))
    t = 2 * np.pi * np.outer(a, k1) / 128
    fa = np.concatenate([np.cos(t), -np.sin(t)], 1)
    fb = np.concatenate([np.sin(t), -np.cos(t)], 1)
    fa[:, 0], fb[:, 0] = RSQ2, -RSQ2
    fa[:, 64], fb[:, 64] = alt, 0.0
    lanes[L_FA:L_FA + 128], lanes[L_FB:L_FB + 128] = fa, fb
    for j in range(NB):
        ang = 2 * np.pi * j / 32 + np.pi / 32
        p, q = (_bf16_bits([np.cos(ang), np.sin(ang)]) << 16).view(np.float32).astype(np.float64)
        turn = 2 * np.pi * j * np.tile(k1, 2) / S
        lanes[L_COS + j], lanes[L_SIN + j] = np.cos(turn), np.repeat([-1.0, 1.0], 64) * np.sin(turn)
        lanes[L_COS + j, 64], lanes[L_SIN + j, 64] = p, q
        lanes[L_MU + j, 0], lanes[L_MU + j, 64] = 1.0, (q / p + p / q) / 2
        lanes[L_NU + j, 0], lanes[L_NU + j, 64] = 0.0, (q / p - p / q) / 2
        lanes[L_KU + j, 0], lanes[L_KU + j, 64] = 1.0, q / p
        lanes[L_KV + j, 0], lanes[L_KV + j, 64] = 1.0, p / q
    for k in (1, 2, 3):
        lanes[L_TWID + 2 * k - 2] = np.cos(2 * np.pi * a * k / D)
        lanes[L_TWID + 2 * k - 1] = np.sin(2 * np.pi * a * k / D)
    th = 2 * np.pi * np.outer(k1, a) / 128
    r = np.concatenate([np.cos(th), -np.sin(th)], 0)
    r[64] = alt
    th = 2 * np.pi * np.outer(2 * k1 + 1, a) / 256
    c4 = np.concatenate([np.cos(th), -np.sin(th)], 0)
    inv = 2.0 / (S * D)
    r0t = inv * r.T
    r0t[:, 0::64] *= 0.5
    rows = np.arange(128).reshape(2, 4, 16).transpose(1, 0, 2).ravel()
    bits = _bf16_bits(np.stack([r[rows], c4[rows], inv * r.T, inv * c4.T, r0t]))
    ang = 2 * np.pi * np.outer(np.arange(4), np.arange(4)).ravel() / 16
    rot = np.concatenate([np.cos(ang), np.sin(ang)]).astype(np.float32)
    return bits[:, 0::2] | (bits[:, 1::2] << 16), lanes.astype(np.float32), rot


_MATS, _LANES, _ROT = _constants()
_ZERO = np.zeros((1,), np.int32)


class _Step:
    def __init__(self, cost, anchors=(), delay=0, marks=()):
        self.cost, self.anchors, self.delay, self.marks = cost, list(anchors), delay, list(marks)


class _Wait:
    def __init__(self, *names):
        self.names = names


class _Mat:
    def __init__(self, emit):
        self.emit = emit


class _Hold:
    def __init__(self, store):
        self.store = store


class _Task:
    def __init__(self, gen, pace):
        self.gen, self.pace, self.blocked, self.not_before, self.held = gen, pace, (), 0, None
        self.allowed = 0.0


class _Sched:
    def __init__(self, share=0.0, wait=28):
        self.wait = wait
        self.share = share
        self.tasks, self.done, self.producer = [], {}, {}
        self.slot, self.credit, self.anchors, self.results = 0, 0.0, [], []
        self.fresh = False

    def add(self, gen, name, pace=99):
        self.producer[name] = self.producer["read", name] = _Task(gen, pace)
        self.tasks.append(self.producer[name])

    def _ready(self, t):
        return t.not_before <= self.slot and all(
            n in self.done and self.done[n] <= self.slot for n in t.blocked)

    def _advance(self, t, mats=True):
        item, t.held = t.held or next(t.gen, None), None
        if item is None:
            self.tasks.remove(t)
        elif isinstance(item, _Wait):
            t.blocked = item.names
        elif isinstance(item, _Hold):
            if len(self.results) >= LAG:
                item.store(self.results[-LAG])
        elif isinstance(item, _Mat):
            if mats:
                t.not_before = float("inf")
                self.fresh = False
                self.credit -= item.emit(lambda: self.point(0.0)) or 0
                t.not_before = self.slot + self.wait
            else:
                t.held, t.not_before = item, self.slot + 1
        else:
            t.blocked = ()
            t.not_before = self.slot + item.delay
            self.credit -= item.cost
            self.anchors += item.anchors
            for n in item.marks:
                self.done[n] = self.slot + item.delay
            return True

    def run(self, *names):
        while not all(n in self.done for n in names):
            for n in names:
                if n not in self.done:
                    for b in self.producer[n].blocked:
                        self.run(b)
                    self._advance(self.producer[n])

    def drive(self):
        while self.tasks:
            ready = [t for t in self.tasks if self._ready(t)]
            if not ready:
                self.slot += 1
                continue
            self.anchors, self.credit = self.anchors[-2:], 0.0
            self._advance(next((t for t in ready if t.held), ready[0]))
            self.slot -= min(self.credit, 0.0) / 60

    def finish(self):
        self.run(*[n for n in self.producer if n[0] != "read"])

    def point(self, own):
        for t in self.tasks:
            t.allowed = min(t.allowed, 0.0) + t.pace
        while True:
            t = next((t for t in self.tasks if self._ready(t) and t.allowed > 0
                      and self.credit > 0), None)
            if t is None:
                break
            if self._advance(t, self.fresh):
                t.allowed -= 1
        anchors, self.anchors = self.anchors, []
        self.credit = min(self.credit, 10.0) + 64 * self.share - own
        self.fresh = False
        self.slot += 1
        return anchors


def _dot(a, b):
    return jnp.dot(a, b, preferred_element_type=F32)


def _dot_t(a, b):
    return jax.lax.dot_general(a, b, (((1,), (1,)), ((), ())), preferred_element_type=F32)


def _bf(u):
    return pltpu.bitcast(u, BF16)


def _iota(rows, dim):
    return jax.lax.broadcasted_iota(I32, (rows, 128), dim)


def _radix4(z, inverse):
    (r0, i0), (r1, i1), (r2, i2), (r3, i3) = z
    ar, ai, cr, ci = r0 + r2, i0 + i2, r0 - r2, i0 - i2
    br, bi, dr, di = r1 + r3, i1 + i3, r1 - r3, i1 - i3
    lo, hi = (cr + di, ci - dr), (cr - di, ci + dr)
    if inverse:
        lo, hi = hi, lo
    return [(ar + br, ai + bi), lo, (ar - br, ai - bi), hi]


def _all_sublanes(v, op, axis):
    for sh in (4, 2, 1):
        v = op(v, pltpu.roll(v, sh, axis))
    return v


def _loop(n, body, name):
    def step(i, carry):
        body(i)
        return carry
    with jax.named_scope(name):
        jax.lax.fori_loop(0, n, step, 0)


def _kernel(zero_ref, rot, d_mats, lanes, x_hbm, wr_hbm, wi_hbm, wqkv_hbm, wo_hbm, out_hbm,
            mats, twid, STAT, KE, VE, KS, VS, Z, ZT, WS, WQ, WK, WV, WP, WS5, WQ5, WP5, SB0, SB1, SB2, SB3, XR, WRI, WN, WRAW, WO, PW0, PW1, sems, *split):
    zero = zero_ref[0]
    never = zero != 0
    X, HB, QB = split[2::5], split[3::5], split[4::5]
    hbu = [r.bitcast(U32) for r in HB]
    xru, wsu, wou = XR.bitcast(U32), WRI.bitcast(U32), WO.bitcast(U32)
    temps = [(ub, ab, pb, ub.bitcast(U32), ab.bitcast(U32))
             for ub, ab, pb in zip(split[5::5], split[6::5], 2 * split[:2])]
    PW, SB, WT = (PW0, PW1), (SB0, SB1, SB2, SB3), (WQ, WK, WV, WP)
    counter = [0]

    def opaque():
        counter[0] += 1
        return zero * counter[0]

    def anchor(ref):
        at = (0,) * (len(ref.shape) - 2)
        return lambda: ref[(*at, pl.ds(pl.multiple_of(zero * 8, 8), 8), pl.ds(0, 128))]

    def settle(ref):
        return _Step(2, [anchor(ref)], delay=SETTLE)

    def hold(ref, spare, row=0):
        def store(v):
            ref[spare, pl.ds(pl.multiple_of(row + zero * 8, 8), 8), :] = v
        return _Hold(store)

    def tied(load, vregs, point):
        parts = []
        for r in range(vregs):
            anchors = [a for _ in range(GRAIN) for a in point()] if r % GRAIN == 0 else []
            u = load(8 * r)
            for a in anchors:
                u = jnp.where(never, pltpu.bitcast(a(), U32), u)
            parts.append(u)
        return jnp.concatenate(parts, 0)

    def mat(i):
        return _bf(mats[i])

    def d_stage(t, which):
        UB, AB, PB, ubu, abu = temps[t]

        def emit(point):
            z = opaque()
            for c in range(8):
                lhs = mat(which(c) + opaque()) if c % 4 else _bf(
                    tied(lambda r, u=which(c) + opaque(): mats[u, pl.ds(r, 8), :], 8, point))
                PB[0, pl.ds(128 * c, 128), :] = _dot(lhs, _bf(ubu[z, pl.ds(64 * c, 64), :]))
        return _Mat(emit)

    def lane_vec(i, rows):
        return jnp.broadcast_to(lanes[pl.ds(i, 1), :], (rows, 128))

    def x_copy(c):
        return pltpu.make_async_copy(
            x_hbm.at[:, pl.ds(pl.multiple_of(128 * c, 128), 128)], XR.at[c], sems.at[c])

    def out_copy(c):
        return pltpu.make_async_copy(
            XR.at[c], out_hbm.at[:, pl.ds(pl.multiple_of(128 * c, 128), 128)], sems.at[8 + c])

    spec_copies = [[pltpu.make_async_copy(w.at[pl.ds(0, 512), pl.ds(128 * k2, 128)], WRI.at[u, k2],
                                          sems.at[16 + u]) for k2 in range(16)]
                   + [pltpu.make_async_copy(w.at[pl.ds(512, 1), :], WN.at[u], sems.at[22 + u])]
                   for u, w in enumerate((wr_hbm, wi_hbm))]

    def start_all(copies):
        for c in copies:
            c.start()
    w_copies = [pltpu.make_async_copy(wqkv_hbm.at[:, pl.ds(D * w, D)], WRAW.at[w], sems.at[18 + w])
                for w in range(3)]
    wo_copies = [pltpu.make_async_copy(wo_hbm.at[:, pl.ds(128 * c, 128)], WO.at[c], sems.at[21])
                 for c in range(8)]

    def ln_rstd(g, i, mean):
        acc, m = None, g + opaque()
        for r in range(8):
            d = X[i][m, pl.ds(128 * r, 128), :].reshape(16, 8, 128) - mean[None]
            v = (d * d).sum(0)
            acc = v if acc is None else acc + v
            if r < 7:
                yield _Step(50, [lambda acc=acc: acc], delay=3)
        rstd = jax.lax.rsqrt(_all_sublanes(acc, jnp.add, 0) * (1.0 / D) + EPS)
        yield _Step(50, delay=8)
        yield _Step(10, [lambda: rstd], delay=1)
        return rstd

    def fwd_block(g, i, name, needs, free=(), known=False):
        j, t = g + 4 * i, i
        UB, AB, PB, ubu, abu = temps[t]
        yield _Wait(*needs)
        if known:
            means, squares = STAT[4 * g + i, pl.ds(0, 8)], STAT[4 * g + i, pl.ds(8, 8)]
            mean = means.sum(0) * 0.125
            var = (squares.sum(0) + 128.0 * ((means - mean) ** 2).sum(0)) * (1.0 / D)
            rstd = jax.lax.rsqrt(var + EPS)
            yield _Step(50, delay=6)
        else:
            yield settle(X[i])
            acc, m = None, g + opaque()
            for r in range(8):
                v = X[i][m, pl.ds(128 * r, 128), :].reshape(16, 8, 128).sum(0)
                acc = v if acc is None else acc + v
                if r % 2:
                    yield _Step(35, [lambda acc=acc: acc], delay=7 if r == 7 else 3)
            mean = _all_sublanes(acc, jnp.add, 0) * (1.0 / D)
            rstd = yield from ln_rstd(g, i, mean)
        mean8, rstd = (jnp.concatenate([v, v], 0) for v in (mean * 8.0, rstd))
        z = opaque()
        for r in range(8):
            rows = pl.ds(16 * r, 16)
            x = [X[i][g + z, pl.ds(128 * b + 16 * r, 16), :] for b in range(8)]
            s = [x[b] + x[b + 4] for b in range(4)]
            d = [x[b] - x[b + 4] for b in range(4)]
            e, o = s[0] + s[2], s[1] + s[3]
            UB[0, rows, :] = ((e + o - mean8) * rstd).astype(BF16)
            UB[0, pl.ds(128 + 16 * r, 16), :] = ((e - o) * rstd).astype(BF16)
            t1, t2 = (d[1] - d[3]) * RSQ2, (d[1] + d[3]) * RSQ2
            u = {1: (d[0] + t1, d[2] + t2), 2: (s[0] - s[2], s[1] - s[3]), 3: (d[0] - t1, d[2] - t2)}
            yield _Step(34, [anchor(ubu)], delay=1)
            for k in (1, 2, 3):
                c, sn = twid[z + 2 * k - 2, rows, :] * rstd, twid[z + 2 * k - 1, rows, :] * rstd
                re, m = u[k]
                if k == 3:
                    ur, ui = re * c + m * sn, m * c - re * sn
                else:
                    ur, ui = re * c - m * sn, m * c + re * sn
                UB[0, pl.ds(256 * k + 16 * r, 16), :] = ur.astype(BF16)
                UB[0, pl.ds(256 * k + 128 + 16 * r, 16), :] = ui.astype(BF16)
                yield _Step(26, [anchor(ubu)], delay=1)
        yield settle(ubu)

        def d_forward(point):
            z = opaque()
            first = _iota(8, 0) == 0

            def stage(c):
                u = (M_C4 if c == 1 else M_R) + opaque()
                lhs = mat(u) if c % 4 else _bf(tied(lambda r: mats[u, pl.ds(r, 8), :], 8, point))
                v = _dot(lhs, _bf(ubu[z, pl.ds(64 * c, 64), :]))
                return [(v[32 * u:32 * u + 16], v[32 * u + 16:32 * u + 32]) for u in range(4)]

            def put(row, u, v, v0=None):
                if u == 0 and v0 is not None:
                    v = jnp.concatenate([jnp.where(first, v0, v[:8]), v[8:]], 0)
                AB[0, pl.ds(row + 16 * u, 16), :] = v.astype(BF16)

            for u, (p1, p2) in enumerate(stage(0)):
                put(0, u, p1)
                put(528, u, p2, 0.0)
                if u == 0:
                    put(512, 0, jnp.zeros_like(p2), p2[:8])
            for u, (p1, p2) in enumerate(stage(1)):
                put(256, u, p1)
                put(528 + 256, u, p2)
            for k in (1, 2, 3):
                for u, ((p1, p2), (q1, q2)) in enumerate(zip(stage(2 * k), stage(2 * k + 1))):
                    if k == 3:
                        pr, pi, mr, mi = p1 - q2, p2 + q1, p1 + q2, p2 - q1
                        pi0, mi0 = q1[:8], -q2[:8]
                    else:
                        pr, pi, mr, mi = p1 + q2, p2 - q1, p1 - q2, p2 + q1
                        pi0, mi0 = -q1[:8], q2[:8]
                    put(64 * k, u, pr, p1[:8])
                    put(64 * (8 - k), u, mr, p2[:8])
                    put(528 + 64 * k, u, pi, pi0)
                    put(528 + 64 * (8 - k), u, mi, mi0)
            return 190

        yield _Mat(d_forward)
        yield settle(abu)
        yield _Wait(*free)

        def s_forward(point):
            z = opaque()
            fa, fb = mat(M_FA + j + z), mat(M_FB + j + z)
            for r0, rn in ((0, 256), (256, 272)):
                lhs = abu[z, pl.ds(r0 // 2, rn // 2), :] if r0 else tied(
                    lambda r: abu[z, pl.ds(r, 8), :], 16, point)
                u = _dot(_bf(lhs), fa)
                v = _dot(_bf(abu[z, pl.ds(264 + r0 // 2, 128), :]), fb)
                re, m = u[:256] + v, u[:256] - v
                if r0:
                    re, m = (jnp.concatenate([a, u[256:264]], 0) for a in (re, m))
                rn = re.shape[0]
                edge = (_iota(rn, 1) & 63) == 0
                ZT[2 * i, pl.ds(r0, rn), :] = re
                ZT[2 * i + 1, pl.ds(r0, rn), :] = jnp.where(
                    edge, lane_vec(L_MU + j, rn) * m + lane_vec(L_NU + j, rn) * re, pltpu.roll(m, 64, 1))
            return 400

        yield _Mat(s_forward)
        yield _Step(2, [anchor(ZT)], delay=SETTLE, marks=[name])

    def group_stage(g, name, needs, inverse):
        yield _Wait(*needs)

        def turn(z, k):
            if k == 0:
                return z
            c, s = rot[4 * g + k], rot[16 + 4 * g + k]
            if inverse:
                return z[0] * c - z[1] * s, z[1] * c + z[0] * s
            return z[0] * c + z[1] * s, z[1] * c - z[0] * s

        (src, a), (dst, b) = ((Z, 8 * g), (ZT, 0)) if inverse else ((ZT, opaque()), (Z, 8 * g))
        for r in range(65):
            if r % 16 == 0:
                yield hold(src, 2 * NB if inverse else 8)
            rows = pl.ds(8 * r, 8)
            z = [(src[a + 2 * i, rows, :], src[a + 2 * i + 1, rows, :]) for i in range(4)]
            if inverse:
                z = _radix4([turn(z[k], k) for k in range(4)], True)
            else:
                z = [turn(v, k) for k, v in enumerate(_radix4(z, False))]
            for i in range(4):
                dst[b + 2 * i, rows, :], dst[b + 2 * i + 1, rows, :] = z[i]
            yield _Step(35, [anchor(dst)], delay=1, marks=[name] if r == 64 else [])

    def spectral(row, size):
        rows = pl.ds(row, size)
        for k0 in range(4):
            z = _radix4([(Z[8 * g + 2 * k0, rows, :], Z[8 * g + 2 * k0 + 1, rows, :])
                         for g in range(4)], False)
            y = []
            for k1, (re, im) in enumerate(z):
                w = WS[k0 + 4 * k1, rows, :]
                wr = pltpu.bitcast(w << 16, F32)
                wi = pltpu.bitcast(w & np.uint32(0xFFFF0000), F32)
                y.append((re * wr - im * wi, re * wi + im * wr))
            y = _radix4(y, True)
            for g in range(4):
                Z[8 * g + 2 * k0, rows, :], Z[8 * g + 2 * k0 + 1, rows, :] = y[g]

    def spectral_rows(c2):
        for r in range(8):
            spectral(pl.multiple_of(128 * c2 + 16 * r, 16), 16)

    def inv_block(g, i, name, needs, n=None):
        j, t = g + 4 * i, i % 2
        UB, AB, PB, ubu, abu = temps[t]
        n = g if n is None else n
        z = opaque()
        yield _Wait(*needs)
        for r0, rn in _S_ROWS:
            if r0 == 0:
                yield hold(ZT, 8)
            re, im = ZT[z + 2 * i, pl.ds(r0, rn), :], ZT[z + 2 * i + 1, pl.ds(r0, rn), :]
            edge = (_iota(rn, 1) & 63) == 0
            rolled = pltpu.roll(im, 64, 1)
            u = re + jnp.where(edge, lane_vec(L_KU + j, rn) * im, rolled)
            if r0 < 512:
                v = re - jnp.where(edge, lane_vec(L_KV + j, rn) * im, rolled)
                AB[0, pl.ds(r0, rn), :] = u.astype(BF16)
                AB[0, pl.ds(528 + r0, rn), :] = v.astype(BF16)
            else:
                AB[0, pl.ds(512, 16), :] = jnp.concatenate([u, jnp.zeros_like(u)], 0).astype(BF16)
            yield _Step(rn, [anchor(abu)], delay=1, marks=[("read", name)] if r0 == 512 else [])
        yield settle(abu)

        def s_inverse(point):
            z = opaque()
            fa, fb = mat(M_FA + j + z), mat(M_FB + j + z)
            first = _iota(8, 0) == 0

            def put(row, v, v0=None):
                if v0 is not None:
                    v = jnp.concatenate([jnp.where(first, v0, v[:8]), v[8:]], 0)
                UB[0, pl.ds(row, 64), :] = v.astype(BF16)

            for k in range(4):
                lo, hi = 32 * k, 32 * (8 - k if k else 4)
                a = [abu[z, pl.ds(lo, 32), :], abu[z, pl.ds(hi, 32), :]] if k % 2 else [
                    tied(lambda r, o=o: abu[z, pl.ds(o + r, 8), :], 4, point) for o in (lo, hi)]
                if k == 0:
                    a.append(abu[z, pl.ds(256, 8), :])
                re = _dot_t(_bf(jnp.concatenate(a, 0)), fa)
                im = _dot_t(_bf(jnp.concatenate(
                    [abu[z, pl.ds(264 + lo, 32), :], abu[z, pl.ds(264 + hi, 32), :]], 0)), fb)
                pr, mr, pi, mi = re[:64], re[64:128], im[:64], im[64:]
                if k == 0:
                    put(0, pr)
                    put(64, pi, re[128:136])
                    put(128, mr)
                    put(192, mi)
                else:
                    put(256 * k, pr + mr, pr[:8])
                    put(256 * k + 64, pi + mi, mr[:8])
                    put(256 * k + 128, pi - mi, pi[:8])
                    put(256 * k + 192, mr - pr, -mi[:8])
            return 190

        yield _Mat(s_inverse)
        yield settle(ubu)
        yield d_stage(t, lambda c: {0: M_R0T, 1: M_C4T}.get(c, M_RT))
        yield settle(PB)
        z = opaque()
        acc = None
        for r in range(16):
            rows = pl.ds(8 * r, 8)
            t0, t4 = PB[z, rows, :], PB[z, pl.ds(128 + 8 * r, 8), :]
            tk = {}
            for k in (1, 2, 3):
                c, sn = twid[z + 2 * k - 2, rows, :], twid[z + 2 * k - 1, rows, :]
                re = PB[z, pl.ds(256 * k + 8 * r, 8), :]
                im = PB[z, pl.ds(256 * k + 128 + 8 * r, 8), :]
                tk[k] = (re * c - im * sn, re * sn + im * c)
            e0, e1 = t0 + t4, t0 - t4
            s = [e0 + tk[2][0], e1 - tk[2][1], e0 - tk[2][0], e1 + tk[2][1]]
            al, be = tk[1][0] - tk[3][0], tk[1][1] + tk[3][1]
            o = [tk[1][0] + tk[3][0], (al - be) * RSQ2, tk[3][1] - tk[1][1], (al + be) * -RSQ2]
            for b in range(8):
                y = s[b] + o[b] if b < 4 else s[b - 4] - o[b - 4]
                v = X[i][g, pl.ds(128 * b + 8 * r, 8), :] + y
                X[i][n, pl.ds(128 * b + 8 * r, 8), :] = v
                acc = v if acc is None else acc + v
            yield _Step(57, [lambda v=acc: v], delay=5 if r == 15 else 2)
        yield settle(X[i])
        mean = _all_sublanes(acc, jnp.add, 0) * (1.0 / D)
        rstd = yield from ln_rstd(n, i, mean)
        z = opaque()
        for r in range(8):
            v = X[i][n + z, pl.ds(128 * r, 128), :].reshape(16, 8, 128)
            HB[i][n, pl.ds(128 * r, 128), :] = ((v - mean[None]) * rstd[None]).reshape(128, 128).astype(BF16)
            yield _Step(41, [anchor(hbu[i])], delay=1, marks=[name] if r == 7 else [])

    def attend(g, i, name, needs):
        yield _Wait(*needs)
        yield settle(QB[i])
        j, z = g + 4 * i, opaque()
        even = (_iota(8, 0) & 1) == 0
        edge = _iota(8, 1) == 0

        def window(near, far, w, rows):
            return near[j + z + 4 - 2 * w, rows, :] if w <= 2 * i + 2 else far[j + z + 16 - 2 * w, rows, :]

        def mix_values(h, u):
            p = PW[h % 2][opaque()]
            for rows in (pl.ds(256 * h + 16 * u, 16), pl.ds(256 * h + 16 * u + 16, 16)):
                acc = functools.reduce(jnp.add, [p[16 * w:16 * w + 16] * window(VE, VS, w, rows)
                                                 for w in range(8)])
                HB[i][g, rows, :] = acc.astype(BF16)
            return _Step(63, [anchor(hbu[i])], delay=1, marks=[name] if (h, u) == (3, 14) else [])

        for h in range(5):
            logits = []
            for w0 in range(0, 8, 2):
                if h < 4:
                    rows = pl.ds(256 * h, 256)
                    q = q if w0 % 4 else QB[i][opaque(), rows, :]
                    for w in (w0, w0 + 1):
                        v = (q * window(KE, KS, w, rows)).reshape(16, 16, 128).sum(0)
                        v = jnp.where(even, v[:8] + pltpu.roll(v[:8], 7, 0), v[8:] + pltpu.roll(v[8:], 1, 0))
                        logits.append(jnp.where(edge & (2 * w > j), -1e9, v * SCALE) if w > 2 * i
                                      else v * SCALE)
                    yield _Step(138, [lambda v=v: v for v in logits[-2:]], delay=2)
                if h > 0:
                    yield mix_values(h - 1, 2 * w0)
                    yield mix_values(h - 1, 2 * w0 + 2)
            if h < 4:
                top = functools.reduce(jnp.maximum, logits)
                e = [jnp.exp(v - top) for v in logits]
                total = functools.reduce(jnp.add, e)
                yield _Step(30, [lambda v=total: v], delay=3)
                scale = 1.0 / total
                for w in range(8):
                    v = e[w] * scale
                    PW[h % 2][0, pl.ds(16 * w, 8), :] = jnp.where(even, v, pltpu.roll(v, 1, 0))
                    PW[h % 2][0, pl.ds(16 * w + 8, 8), :] = jnp.where(even, pltpu.roll(v, 7, 0), v)
                yield _Step(50, [anchor(PW[h % 2])], delay=6 if h == 3 else 1)

    def packed_sums(terms, signs):
        lo = [pltpu.bitcast(u << 16, F32) for u in terms]
        hi = [pltpu.bitcast(u & np.uint32(0xFFFF0000), F32) for u in terms]
        return [pltpu.pack_elementwise([v[p] + v[q] if s > 0 else v[p] - v[q] for v in (lo, hi)],
                                       packed_dtype=BF16) for p, s, q in signs]

    def half(ref, row):
        return lambda r, size, cols: ref[pl.ds(pl.multiple_of(row + r, 8), size), cols]

    kv_weight = (WS5, half(WK, 0), half(WV, 0))
    q_weight = (WQ5, half(WQ, 0), half(WQ, D // 4))
    o_weight = (WP5, *(lambda r, size, cols, e=e: WP[pl.ds(r + r // 32 * 32 + e, size), cols]
                       for e in (0, 32)))

    def left_sums(weight, row, size, needs=()):
        yield _Wait(*needs)
        sums, top, bottom = weight
        for r in range(0, size, 8):
            a = [ref(row + r, 8, pl.ds(c, 512)) for ref in (top, bottom) for c in (0, 512)]
            for e, v in enumerate(packed_sums(a, ((0, 1, 3), (2, 1, 3), (0, 1, 1), (2, -1, 0), (1, -1, 3)))):
                sums[e, pl.ds(pl.multiple_of(row + r, 8), 8), :] = v
            yield _Step(92, [anchor(sums)], delay=2, marks=["sums"] if r == size - 8 else [])

    def right_sums(dst, g, i, name, needs):
        yield _Wait(*needs)
        z = g + opaque()
        for r in range(0, 256, 16):
            b = [hbu[n][z, pl.ds(k + r, 16), :] for k in (0, 256) for n in (i, i + 1)]
            for e, v in enumerate(packed_sums(b, ((0, 1, 3), (1, -1, 3), (2, -1, 0), (0, 1, 1), (2, 1, 3)))):
                dst[e, pl.ds(r, 16), :] = v
            yield _Step(47, [anchor(dst)], delay=SETTLE if r == 240 else 1,
                        marks=[name] if r == 240 else [])

    def strassen(sch, weight, right, g, i, m, store, needs, marks):
        for n in needs:
            sch.run(n)
        sums, top, bottom = weight
        rows = pl.ds(pl.multiple_of(64 * m, 64), 64)

        def product(left, b):
            sch.fresh = True
            head = tied(lambda r: left(32 * m + r, 8, pl.ds(0, 128)), 4, lambda: sch.point(8.0))
            return _dot(_bf(jnp.concatenate([head, left(32 * m, 32, pl.ds(128, 384))], 1)), _bf(b))

        def a(e):
            return lambda r, size, cols: sums[e, pl.ds(pl.multiple_of(r, 8), size), cols]

        def b(e):
            return right[e + opaque()]

        m2 = product(a(1), hbu[i][g + opaque(), pl.ds(0, 256), :])
        m4 = product(lambda r, size, cols: bottom(r, size, pl.ds(512 + cols.start, cols.size)), b(2))
        store(1, i, rows, m2 + m4)
        m1 = product(a(0), b(0))
        c11, c22 = m1 + m4, m1 - m2
        c11 = c11 + product(a(4), b(4))
        c22 = c22 + product(a(3), b(3))
        m5 = product(a(2), hbu[i + 1][g + opaque(), pl.ds(256, 256), :])
        store(0, i, rows, c11 - m5)
        v = product(top, b(1))
        store(0, i + 1, rows, v + m5)
        store(1, i + 1, rows, c22 + v)
        sch.results.append(v[:8])
        for name in marks:
            sch.done[name] = sch.slot + sch.wait

    def kv_proj(sch, g, i, name, needs):
        def store(lower, n, rows, v):
            (KE, VE)[lower][g + 4 * n + 4, rows, :] = v
        for m in range(16):
            strassen(sch, kv_weight, SB[i // 2], g, i, m, store, needs, [name] if m == 15 else [])

    def q_proj(sch, g, i, name, needs):
        def store(lower, n, rows, v):
            QB[n][0, pl.ds(512 * lower + rows.start, 64), :] = v
        for m in range(8):
            strassen(sch, q_weight, SB[i // 2], g, i, m, store, needs, [name] if m == 7 else [])

    def o_proj(sch, g, i, m, needs, marks, right):
        def store(lower, n, rows, v):
            rows = pl.ds(128 * m + 64 * lower, 64)
            X[n][g, rows, :] = X[n][g, rows, :] + v
        strassen(sch, o_weight, right, g, i, m, store, needs, marks)

    def shift_block(g, i, name, needs):
        yield _Wait(*needs)
        j, z = g + 4 * i, opaque()
        for m in range(16):
            rows = pl.ds(64 * m, 64)
            for ref, to in ((KE, KS), (VE, VS)):
                v = pltpu.roll(ref[j + 4 + z, rows, :], 1, 1)
                if ref is VE:
                    v = jnp.where(_iota(64, 1) == 0, ref[4 + z, rows, :], v)
                to[j, rows, :] = v
                if i == 3:
                    ref[g, rows, :] = v
            yield _Step(12, delay=8, marks=[name] if m == 15 else [])

    def transpose_quarter(w, h, via):
        for r in range(4):
            v = WRAW[w, pl.ds(256 * r, 256), pl.ds(pl.multiple_of(256 * h, 256), 256)]
            v = pltpu.bitcast(v.T, F32)
            via[0, pl.ds(256 * r, 128), :], via[0, pl.ds(256 * r + 128, 128), :] = v[:, :128], v[:, 128:]
            yield _Step(40, delay=16)

    def reorder_quarter(w, h, via, name=None):
        z = 0 if isinstance(h, int) else opaque()
        for c in range(8):
            WT[w][pl.ds(pl.multiple_of(128 * h, 128), 128), pl.ds(128 * c, 128)] = pltpu.bitcast(
                jnp.concatenate([via[z, pl.ds(128 * c + u, 8, stride=16), :] for u in range(16)], 0), U32)
            yield _Step(20, delay=4, marks=[name] if c == 7 else [])

    def query_weight(h):
        yield from transpose_quarter(0, h, QB[0])
        yield from reorder_quarter(0, h, QB[0], "w")

    def transpose_wo(name):
        for c in range(8):
            for h in range(4):
                v = jnp.concatenate([wou[c, pl.ds(128 * h + u, 8, stride=16), :] for u in range(16)], 0)
                WP[pl.ds(64 * c, 64), pl.ds(256 * h, 256)] = pltpu.bitcast(_bf(v).T, U32)
                yield _Step(20, delay=10, marks=[name] if c == 7 and h == 3 else [])

    def prep_spectral_weights(c2):
        lane = _iota(8, 1)
        order = jnp.where(lane > 64, 192 - lane, lane)

        def words(k2):
            re, im = (wsu[u, k2, pl.ds(c2, 64, stride=4), :] for u in range(2))
            return ((re & np.uint32(0xFFFF)) | (im << 16), (re >> 16) | (im & np.uint32(0xFFFF0000)))

        def arrange(w, below):
            w = jnp.where(_iota(w.shape[0], 1) < 64, w, below)
            return jnp.concatenate([jnp.take_along_axis(w[u:u + 8], order, axis=1)
                                    for u in range(0, w.shape[0], 8)], 0)

        below = words(15)
        for k2 in range(16):
            here = words(k2)
            for e in range(2):
                cl = 2 * c2 + e
                w = arrange(here[e], below[e])
                WS[k2, pl.ds(64 * cl, 64), :] = pltpu.roll(w, 1, 0) if cl > 4 else w
            below = here
            yield _Step(100)
        if c2 == 0:
            def nyquist(k2):
                re, im = (jnp.broadcast_to(WN[u, :, pl.ds(128 * k2, 128)].astype(F32), (8, 128))
                          for u in range(2))
                return pltpu.pack_elementwise([re, im], packed_dtype=BF16)
            for k2 in range(16):
                WS[k2, pl.ds(512, 8), :] = arrange(nyquist(k2), nyquist((k2 + 15) % 16))

    def write_out(p, c, name, needs):
        yield _Wait(*needs)
        rows = pl.ds(pl.multiple_of(128 * c, 128), 128)
        g, i = 2 * p % 4 + opaque(), p // 2
        w = pltpu.pack_elementwise([X[i][g, rows, :], X[i][g + 1, rows, :]], packed_dtype=BF16)
        xru[c, pl.ds(p, 128, stride=8), :] = w.T
        yield _Step(30, marks=[name])

    for c in range(8):
        x_copy(c).start()
    for c in range(5):
        mats[M_R + c] = d_mats[c]

    def make_twiddle(k):
        PB = temps[0][2]
        PB[0, pl.ds(0, 128), :] = lane_vec(L_TWID + k, 128)
        twid[k] = PB[opaque(), pl.ds(0, 128), :].T

    _loop(6, make_twiddle, "make_twiddle")

    def make_dft(j):
        fa, fb = lanes[pl.ds(L_FA, 128), :], lanes[pl.ds(L_FB, 128), :]
        c, sn = lane_vec(L_COS + j, 128), lane_vec(L_SIN + j, 128)
        UB, _, _, ubu, _ = temps[0]
        UB[0, pl.ds(0, 128), :] = (fa * c + fb * sn).astype(BF16)
        UB[0, pl.ds(128, 128), :] = (fb * c - fa * sn).astype(BF16)
        mats[M_FA + j], mats[M_FB + j] = ubu[0, pl.ds(0, 64), :], ubu[0, pl.ds(64, 64), :]

    _loop(NB, make_dft, "make_dft")

    def load_x(c):
        x_copy(c).wait()
        pl.when(c == 6)(lambda: start_all(spec_copies[0]))
        pl.when(c == 7)(lambda: start_all(spec_copies[1]))
        rows = pl.ds(pl.multiple_of(128 * c, 128), 128)
        for p in range(8):
            w = xru[c, pl.ds(p, 128, stride=8), :].T
            for e, bits in enumerate((w << 16, w & np.uint32(0xFFFF0000))):
                g, i = 2 * p % 4 + e, p // 2
                v = pltpu.bitcast(bits, F32)
                X[i][g, rows, :] = v
                v = v.reshape(16, 8, 128)
                mean = _all_sublanes(v.sum(0), jnp.add, 0) * (1.0 / 128)
                STAT[4 * g + i, c] = mean
                STAT[4 * g + i, 8 + c] = _all_sublanes(((v - mean) ** 2).sum(0), jnp.add, 0)

    _loop(8, load_x, "load_x")

    def after(name, action):
        yield _Wait(name)
        action()

    def spectral_weights():
        yield _Wait(("f", 2, 1))
        for c in spec_copies[0] + spec_copies[1]:
            c.wait()
        for c2 in range(4):
            yield from prep_spectral_weights(c2)

    with jax.named_scope("first_forward"):
        sch = _Sched(0.80)
        sch.add(after(("f", 0, 1), w_copies[1].start), "k")
        sch.add(after(("f", 1, 1), w_copies[2].start), "v")
        sch.add(after(("f", 2, 3), w_copies[0].start), "q")
        for g in range(4):
            for i in range(4):
                sch.add(fwd_block(g, i, ("f", g, i), [("f", g - 1, i)] if g else [],
                                  [("r", g - 1)] if g else [], True), ("f", g, i))
            sch.add(group_stage(g, ("r", g), [("f", g, i) for i in range(4)], False), ("r", g))
        sch.add(spectral_weights(), "s")
        sch.drive()
    start_all(wo_copies)

    def keys_values(layer, g):
        sch = _Sched(0.41 if layer == 0 else 0.36, 32 if layer == 0 else 28)
        nxt = (g + 1) % 4
        sch.add(inv_block(g, 2, ("i", 2), []), ("i", 2))
        sch.add(inv_block(g, 3, ("i", 3), [("read", ("i", 2))]), ("i", 3))
        sch.add(right_sums(SB[1], g, 2, ("b", 2), [("i", 2), ("i", 3)]), ("b", 2))
        sch.add(group_stage(nxt, "r", [("read", ("i", 3))], True), "r")
        sch.add(inv_block(nxt, 0, ("i", 4), ["r", ("i", 2)], n=g + 1), ("i", 4))
        sch.add(inv_block(nxt, 1, ("i", 5), [("read", ("i", 4)), ("i", 3)], n=g + 1), ("i", 5))
        if layer == 0:
            sch.add(query_weight(g), "w")
            sch.add(left_sums(q_weight, 128 * (g % 2), 128, ["w"]), "sums")
        for i in (2, 3):
            sch.add(shift_block((g + 3) % 4, i, ("s", i), []), ("s", i))
        for i in (0, 1):
            sch.add(shift_block(g, i, ("s", i), [("kv", 0)]), ("s", i))
        sch.add(right_sums(SB[0], nxt, 0, ("b", 4), [("i", 4), ("i", 5), ("kv", 0)]), ("b", 4))
        kv_proj(sch, g, 0, ("kv", 0), [])
        kv_proj(sch, g, 2, ("kv", 2), [("b", 2)])
        sch.finish()

    def mix(g, after, last):
        tail = after is None
        sch = _Sched(0.66 if last else 0.63 if tail else 0.59)
        pace = 0.48 if tail else 0.35 if last else 0.31
        ahead = [(g, 2), (g, 3)] + ([] if tail else [(after, 0), (after, 1)])
        for n, block in enumerate(ahead):
            sch.add(attend(*block, ("a", n), [[], [("a", 0)], [("a", 1), ("q", 0)], [("a", 2)]][n]),
                    ("a", n), pace=pace)
            if n % 2:
                sch.add(right_sums(SB[2 + block[1] // 2], block[0], block[1] - 1, ("b", n),
                                   [("a", n)] + ([("o", 0)] if n == 3 else [])), ("b", n))
        for i in () if tail else (0, 2):
            sch.add(right_sums(SB[i // 2], after, i, ("h", i), [("q", 0)] if i else []), ("h", i))
        if not last:
            sch.add(group_stage((g + 3) % 4, "r", [], False), "r")
            for i in range(4):
                sch.add(fwd_block(g, i, ("f", i), [("o", i - i % 2)], ["r"]), ("f", i))
        now = 6 if last else 8
        for i in (0, 2):
            for m in range(now):
                o_proj(sch, g, i, m, [("b", 1)] if i else [], [("o", i)] if m == now - 1 else [],
                       SB[2 + i // 2])
            if not tail:
                q_proj(sch, after, i, ("q", i), [("h", i)])
        if tail:
            sch.add(group_stage(g, "s", [("f", i) for i in range(4)], False), "s")
        sch.share = 0.92
        sch.drive()

    def mix_odd():
        sch = _Sched(0.66)
        blocks = [(1, 2), (1, 3), (3, 0), (3, 1), (3, 2), (3, 3)]
        for n, (g, i) in enumerate(blocks):
            sch.add(attend(g, i, ("a", n), ([("a", n - 1)] if n else []) + ([("q", i)] if n in (2, 4) else [])),
                    ("a", n), pace=0.32)
            if n % 2:
                sch.add(right_sums(SB[(3, 2, 0)[n // 2]], g, i - 1, ("b", g, i - 1),
                                   [("a", n)] + ([("o", 1, 0, 5)] if n > 1 else [])), ("b", g, i - 1))
        for i in (0, 2):
            sch.add(right_sums(SB[i // 2], 3, i, ("h", i), []), ("h", i))
        for g in (1, 3):
            for i in range(4):
                for c in range(6):
                    sch.add(write_out(2 * i + g // 2, c, ("w", g, i, c), [("o", g, i - i % 2, c)]),
                            ("w", g, i, c))
        for g, i, slot, count in ((1, 0, 2, 6), (1, 2, 3, 8), (3, 0, 2, 8), (3, 2, 0, 6)):
            for m in range(count):
                o_proj(sch, g, i, m, [("b", g, i)] if (g, i) != (1, 0) else [], [("o", g, i, m)], SB[slot])
            for e in (0, 2) if (g, i) == (1, 0) else ():
                q_proj(sch, 3, e, ("q", e), [("h", e)] + ([("a", 1)] if e else []))
        sch.share = 0.92
        sch.drive()

    def postponed():
        sch = _Sched(0.7, 12)
        slots = {(3, 2): 0, (2, 2): 1, (0, 2): 2, (2, 0): 3, (0, 0): 0, (1, 0): 1}
        for n, (pair, slot) in enumerate(slots.items()):
            if n:
                sch.add(right_sums(SB[slot], *pair, pair, [(list(slots)[n - 4], 7)] if n >= 4 else []), pair)
        for p, pairs in enumerate(2 * [[(0, 0), (1, 0)], [(2, 0)]] + 2 * [[(0, 2)], [(2, 2), (3, 2)]]):
            for c in (6, 7):
                sch.add(write_out(p, c, ("w", p, c), [(pair, c) for pair in pairs]), ("w", p, c))

        def copy_out():
            yield _Wait(*[("w", p, 6) for p in range(8)])
            out_copy(6).start()

        sch.add(copy_out(), "copy")
        for part in (list(slots)[:2], list(slots)[2:]):
            for c in (6, 7):
                for pair in part:
                    o_proj(sch, *pair, c, [pair] if pair != (3, 2) else [], [(pair, c)], SB[slots[pair]])
        sch.drive()
        out_copy(7).start()

    def first_queries(layer):
        sch = _Sched(0.68)
        sch.add(right_sums(SB[1], 0, 2, ("h", 2), []), ("h", 2))
        sch.add(shift_block(3, 2, "s", []), "s")
        sch.add(attend(0, 0, ("a", 0), ["q"]), ("a", 0), pace=0.4)
        sch.add(attend(0, 1, ("a", 1), [("a", 0)]), ("a", 1), pace=0.4)
        sch.add(right_sums(SB[2], 0, 0, "b", [("a", 1)]), "b")
        sch.add(shift_block(3, 3, "t", []), "t")
        if layer == 0:
            for c in wo_copies:
                c.wait()
            sch.add(transpose_wo("w"), "w")
            sch.add(left_sums(o_weight, 0, 256, ["w"]), "sums")
        q_proj(sch, 0, 0, "q", [])
        q_proj(sch, 0, 2, None, [("h", 2)])
        sch.finish()

    def key_value_weights():
        w_copies[1].wait()
        w_copies[2].wait()
        for h in range(6):
            work = []
            for w in (1, 2):
                if h < 4:
                    work.append(transpose_quarter(w, h, QB[2 * (h % 2) + w - 1]))
                if 0 < h < 5:
                    work.append(reorder_quarter(w, h - 1, QB[2 * ((h - 1) % 2) + w - 1]))
            if h > 1:
                work.append(left_sums(kv_weight, 128 * (h - 2), 128))
            list(itertools.zip_longest(*work))

    for layer in range(2):
        with jax.named_scope("spectral"):
            _loop(4, spectral_rows, "rows")
            if layer == 0:
                _loop(zero + 1, lambda _: key_value_weights(), "weights")
            spectral(512, 8)
        sch = _Sched(0.92)
        sch.add(group_stage(0, "r", [], True), "r")
        sch.add(inv_block(0, 0, ("i", 0), ["r"]), ("i", 0))
        sch.add(inv_block(0, 1, ("i", 1), ["r"]), ("i", 1))
        sch.add(right_sums(SB[0], 0, 0, "b", [("i", 0), ("i", 1)]), "b")
        sch.drive()
        if layer == 0:
            w_copies[0].wait()
        _loop(4, lambda g: keys_values(layer, g), "keys_values")
        first_queries(layer)
        if layer == 0:
            pl.when(never)(lambda: [spectral_rows(c % 4) for c in range(5)] and None)
        if layer == 0:
            _loop(3, lambda g: mix(g, g + 1, False), "mix")
            mix(3, None, False)
        else:
            _loop(2, lambda u: mix(2 * u, 2 - u, True), "mix")
            mix_odd()
    for c in range(6):
        out_copy(c).start()
    with jax.named_scope("postponed"):
        postponed()
    for c in range(8):
        out_copy(c).wait()


@jax.jit
def pallas_interleave_layers__spectral_gfnet__sliding_local_dilated__prompt_kernel(
    A_x: jax.Array,
    A_w_r: jax.Array,
    A_w_i: jax.Array,
    B_x: jax.Array,
    B_wqkv: jax.Array,
    B_wo: jax.Array,
):
    del B_x
    hbm = pl.BlockSpec(memory_space=pl.ANY)
    smem = pl.BlockSpec(memory_space=pltpu.SMEM)
    out = pl.pallas_call(
        _kernel,
        out_shape=jax.ShapeDtypeStruct((S, D), BF16),
        in_specs=[smem, smem, pl.BlockSpec(), pl.BlockSpec(), hbm, hbm, hbm, hbm, hbm],
        out_specs=hbm,
        scratch_shapes=[
            pltpu.VMEM((37, 64, 128), U32),
            pltpu.VMEM((6, 128, 128), F32),
            pltpu.VMEM((NB, 16, 8, 128), F32),
            pltpu.VMEM((NB + 4, D, 128), F32),
            pltpu.VMEM((NB + 4, D, 128), F32),
            pltpu.VMEM((NB, D, 128), F32),
            pltpu.VMEM((NB, D, 128), F32),
            pltpu.VMEM((2 * NB + 1, ZR, 128), F32),
            pltpu.VMEM((9, ZR, 128), F32),
            pltpu.VMEM((NB, ZR, 128), U32),
            *4 * [pltpu.VMEM((D // 2, D), U32)],
            pltpu.VMEM((5, D // 2, D // 2), U32),
            *2 * [pltpu.VMEM((5, D // 4, D // 2), U32)],
            *4 * [pltpu.VMEM((5, D // 4, 128), U32)],
            pltpu.VMEM((8, S, 128), BF16),
            pltpu.VMEM((2, NB, D // 2, 128), BF16),
            pltpu.VMEM((2, 1, S), BF16),
            pltpu.VMEM((3, D, D), BF16),
            pltpu.VMEM((8, D, 128), BF16),
            pltpu.VMEM((1, 128, 128), F32),
            pltpu.VMEM((1, 128, 128), F32),
            pltpu.SemaphoreType.DMA((24,)),
            *2 * [pltpu.VMEM((1, D, 128), F32)],
        ] + 4 * [
            pltpu.VMEM((5, D, 128), F32),
            pltpu.VMEM((5, D, 128), BF16),
            pltpu.VMEM((1, D, 128), F32),
            pltpu.VMEM((1, D, 128), BF16),
            pltpu.VMEM((1, 1152, 128), BF16),
        ],
        compiler_params=pltpu.CompilerParams(vmem_limit_bytes=126 * 2 ** 20),
    )(_ZERO, _ROT, _MATS, _LANES, A_x.reshape(S, D), A_w_r.T, A_w_i.T, B_wqkv, B_wo)
    return out.reshape(1, S, D)
```

```python
import functools
import itertools

import numpy as np

import jax
import jax.numpy as jnp
import jax.experimental.pallas as pl
import jax.experimental.pallas.tpu as pltpu

S, D, NB = 2048, 1024, 16
ZR = 576
F32, BF16, U32, I32 = jnp.float32, jnp.bfloat16, jnp.uint32, jnp.int32
EPS = 1e-5
SCALE = 32 ** -0.5
RSQ2 = float(np.sqrt(0.5))
GRAIN = 1
SETTLE = 6

_S_ROWS = [(32 * u, 32) for u in range(16)] + [(512, 8)]

M_FA, M_FB, M_R, M_C4, M_RT, M_C4T, M_R0T = 0, 16, 32, 33, 34, 35, 36
L_MU, L_NU, L_KU, L_KV, L_COS, L_SIN, L_TWID, L_FA, L_FB = 0, 16, 32, 48, 64, 80, 96, 104, 232


def _bf16_bits(a):
    u = np.ascontiguousarray(a, dtype=np.float32).view(np.uint32).astype(np.uint64)
    return ((u + 0x7FFF + ((u >> 16) & 1)) >> 16).astype(np.uint32)


def _constants():
    a = np.arange(128)
    k1 = np.arange(64)
    alt = (-1.0) ** a
    lanes = np.zeros((L_FB + 128, 128))
    t = 2 * np.pi * np.outer(a, k1) / 128
    fa = np.concatenate([np.cos(t), -np.sin(t)], 1)
    fb = np.concatenate([np.sin(t), -np.cos(t)], 1)
    fa[:, 0], fb[:, 0] = RSQ2, -RSQ2
    fa[:, 64], fb[:, 64] = alt, 0.0
    lanes[L_FA:L_FA + 128], lanes[L_FB:L_FB + 128] = fa, fb
    for j in range(NB):
        ang = 2 * np.pi * j / 32 + np.pi / 32
        p, q = (_bf16_bits([np.cos(ang), np.sin(ang)]) << 16).view(np.float32).astype(np.float64)
        turn = 2 * np.pi * j * np.tile(k1, 2) / S
        lanes[L_COS + j], lanes[L_SIN + j] = np.cos(turn), np.repeat([-1.0, 1.0], 64) * np.sin(turn)
        lanes[L_COS + j, 64], lanes[L_SIN + j, 64] = p, q
        lanes[L_MU + j, 0], lanes[L_MU + j, 64] = 1.0, (q / p + p / q) / 2
        lanes[L_NU + j, 0], lanes[L_NU + j, 64] = 0.0, (q / p - p / q) / 2
        lanes[L_KU + j, 0], lanes[L_KU + j, 64] = 1.0, q / p
        lanes[L_KV + j, 0], lanes[L_KV + j, 64] = 1.0, p / q
    for k in (1, 2, 3):
        lanes[L_TWID + 2 * k - 2] = np.cos(2 * np.pi * a * k / D)
        lanes[L_TWID + 2 * k - 1] = np.sin(2 * np.pi * a * k / D)
    th = 2 * np.pi * np.outer(k1, a) / 128
    r = np.concatenate([np.cos(th), -np.sin(th)], 0)
    r[64] = alt
    th = 2 * np.pi * np.outer(2 * k1 + 1, a) / 256
    c4 = np.concatenate([np.cos(th), -np.sin(th)], 0)
    inv = 2.0 / (S * D)
    r0t = inv * r.T
    r0t[:, 0::64] *= 0.5
    rows = np.arange(128).reshape(2, 4, 16).transpose(1, 0, 2).ravel()
    bits = _bf16_bits(np.stack([r[rows], c4[rows], inv * r.T, inv * c4.T, r0t]))
    ang = 2 * np.pi * np.outer(np.arange(4), np.arange(4)).ravel() / 16
    rot = np.concatenate([np.cos(ang), np.sin(ang)]).astype(np.float32)
    return bits[:, 0::2] | (bits[:, 1::2] << 16), lanes.astype(np.float32), rot


_MATS, _LANES, _ROT = _constants()
_ZERO = np.zeros((1,), np.int32)


class _Step:
    def __init__(self, cost, anchors=(), delay=0, marks=()):
        self.cost, self.anchors, self.delay, self.marks = cost, list(anchors), delay, list(marks)


class _Wait:
    def __init__(self, *names):
        self.names = names


class _Mat:
    def __init__(self, emit):
        self.emit = emit


class _Hold:
    def __init__(self, store):
        self.store = store


class _Task:
    def __init__(self, gen, pace):
        self.gen, self.pace, self.blocked, self.not_before, self.held = gen, pace, (), 0, None
        self.allowed = 0.0


class _Sched:
    def __init__(self, share=0.0, wait=28, lag=3):
        self.lag = lag
        self.wait = wait
        self.share = share
        self.tasks, self.done, self.producer = [], {}, {}
        self.slot, self.credit, self.anchors, self.results = 0, 0.0, [], []
        self.fresh = False

    def add(self, gen, name, pace=99):
        self.producer[name] = self.producer["read", name] = _Task(gen, pace)
        self.tasks.append(self.producer[name])

    def _ready(self, t):
        return t.not_before <= self.slot and all(
            n in self.done and self.done[n] <= self.slot for n in t.blocked)

    def _advance(self, t, mats=True):
        item, t.held = t.held or next(t.gen, None), None
        if item is None:
            self.tasks.remove(t)
        elif isinstance(item, _Wait):
            t.blocked = item.names
        elif isinstance(item, _Hold):
            if len(self.results) >= self.lag:
                item.store(self.results[-self.lag])
        elif isinstance(item, _Mat):
            if mats:
                t.not_before = float("inf")
                self.fresh = False
                self.credit -= item.emit(lambda: self.point(0.0)) or 0
                t.not_before = self.slot + self.wait
            else:
                t.held, t.not_before = item, self.slot + 1
        else:
            t.blocked = ()
            t.not_before = self.slot + item.delay
            self.credit -= item.cost
            self.anchors += item.anchors
            for n in item.marks:
                self.done[n] = self.slot + item.delay
            return True

    def run(self, *names):
        while not all(n in self.done for n in names):
            for n in names:
                if n not in self.done:
                    for b in self.producer[n].blocked:
                        self.run(b)
                    self._advance(self.producer[n])

    def drive(self):
        while self.tasks:
            ready = [t for t in self.tasks if self._ready(t)]
            if not ready:
                self.slot += 1
                continue
            self.anchors, self.credit = self.anchors[-2:], 0.0
            self._advance(next((t for t in ready if t.held), ready[0]))
            self.slot -= min(self.credit, 0.0) / 60

    def finish(self):
        self.run(*[n for n in self.producer if n[0] != "read"])

    def point(self, own):
        for t in self.tasks:
            t.allowed = min(t.allowed, 0.0) + t.pace
        while True:
            t = next((t for t in self.tasks if self._ready(t) and t.allowed > 0
                      and self.credit > 0), None)
            if t is None:
                break
            if self._advance(t, self.fresh):
                t.allowed -= 1
        anchors, self.anchors = self.anchors, []
        self.credit = min(self.credit, 10.0) + 64 * self.share - own
        self.fresh = False
        self.slot += 1
        return anchors


def _dot(a, b):
    return jnp.dot(a, b, preferred_element_type=F32)


def _dot_t(a, b):
    return jax.lax.dot_general(a, b, (((1,), (1,)), ((), ())), preferred_element_type=F32)


def _bf(u):
    return pltpu.bitcast(u, BF16)


def _iota(rows, dim):
    return jax.lax.broadcasted_iota(I32, (rows, 128), dim)


def _radix4(z, inverse):
    (r0, i0), (r1, i1), (r2, i2), (r3, i3) = z
    ar, ai, cr, ci = r0 + r2, i0 + i2, r0 - r2, i0 - i2
    br, bi, dr, di = r1 + r3, i1 + i3, r1 - r3, i1 - i3
    lo, hi = (cr + di, ci - dr), (cr - di, ci + dr)
    if inverse:
        lo, hi = hi, lo
    return [(ar + br, ai + bi), lo, (ar - br, ai - bi), hi]


def _all_sublanes(v, op, axis):
    for sh in (4, 2, 1):
        v = op(v, pltpu.roll(v, sh, axis))
    return v


def _loop(n, body, name):
    def step(i, carry):
        body(i)
        return carry
    with jax.named_scope(name):
        jax.lax.fori_loop(0, n, step, 0)


def _kernel(zero_ref, rot, d_mats, lanes, x_hbm, wr_hbm, wi_hbm, wqkv_hbm, wo_hbm, out_hbm,
            mats, twid, STAT, KE, VE, KS, VS, Z, ZT, WS, WQ, WK, WV, WP, WS5, WQ5, WP5, SB0, SB1, SB2, SB3, XR, WRI, WN, WRAW, WO, PW0, PW1, sems, *split):
    zero = zero_ref[0]
    never = zero != 0
    X, HB, QB = split[2::5], split[3::5], split[4::5]
    hbu = [r.bitcast(U32) for r in HB]
    xru, wsu, wou = XR.bitcast(U32), WRI.bitcast(U32), WO.bitcast(U32)
    temps = [(ub, ab, pb, ub.bitcast(U32), ab.bitcast(U32))
             for ub, ab, pb in zip(split[5::5], split[6::5], 2 * split[:2])]
    PW, SB, WT = (PW0, PW1), (SB0, SB1, SB2, SB3), (WQ, WK, WV, WP)
    counter = [0]

    def opaque():
        counter[0] += 1
        return zero * counter[0]

    def anchor(ref):
        at = (0,) * (len(ref.shape) - 2)
        return lambda: ref[(*at, pl.ds(pl.multiple_of(zero * 8, 8), 8), pl.ds(0, 128))]

    def settle(ref, points=SETTLE):
        return _Step(2, [anchor(ref)], delay=points)

    def hold(ref, spare, row=0):
        def store(v):
            ref[spare, pl.ds(pl.multiple_of(row + zero * 8, 8), 8), :] = v
        return _Hold(store)

    def tied(load, vregs, point):
        parts = []
        for r in range(vregs):
            anchors = [a for _ in range(GRAIN) for a in point()] if r % GRAIN == 0 else []
            u = load(8 * r)
            for a in anchors:
                u = jnp.where(never, pltpu.bitcast(a(), U32), u)
            parts.append(u)
        return jnp.concatenate(parts, 0)

    def mat(i):
        return _bf(mats[i])

    def d_stage(t, which):
        UB, AB, PB, ubu, abu = temps[t]

        def emit(point):
            z = opaque()
            for c in range(8):
                lhs = mat(which(c) + opaque()) if c % 4 else _bf(
                    tied(lambda r, u=which(c) + opaque(): mats[u, pl.ds(r, 8), :], 8, point))
                PB[0, pl.ds(128 * c, 128), :] = _dot(lhs, _bf(ubu[z, pl.ds(64 * c, 64), :]))
        return _Mat(emit)

    def lane_vec(i, rows):
        return jnp.broadcast_to(lanes[pl.ds(i, 1), :], (rows, 128))

    def x_copy(c):
        return pltpu.make_async_copy(
            x_hbm.at[:, pl.ds(pl.multiple_of(128 * c, 128), 128)], XR.at[c], sems.at[c])

    def out_copy(c):
        return pltpu.make_async_copy(
            XR.at[c], out_hbm.at[:, pl.ds(pl.multiple_of(128 * c, 128), 128)], sems.at[8 + c])

    spec_copies = [[pltpu.make_async_copy(w.at[pl.ds(0, 512), pl.ds(128 * k2, 128)], WRI.at[u, k2],
                                          sems.at[16 + u]) for k2 in range(16)]
                   + [pltpu.make_async_copy(w.at[pl.ds(512, 1), :], WN.at[u], sems.at[22 + u])]
                   for u, w in enumerate((wr_hbm, wi_hbm))]

    def start_all(copies):
        for c in copies:
            c.start()
    w_copies = [pltpu.make_async_copy(wqkv_hbm.at[:, pl.ds(D * w, D)], WRAW.at[w], sems.at[18 + w])
                for w in range(3)]
    wo_copies = [pltpu.make_async_copy(wo_hbm.at[:, pl.ds(128 * c, 128)], WO.at[c], sems.at[21])
                 for c in range(8)]

    def ln_rstd(g, i, mean):
        acc, m = None, g + opaque()
        for r in range(8):
            d = X[i][m, pl.ds(128 * r, 128), :].reshape(16, 8, 128) - mean[None]
            v = (d * d).sum(0)
            acc = v if acc is None else acc + v
            if r < 7:
                yield _Step(50, [lambda acc=acc: acc], delay=3)
        rstd = jax.lax.rsqrt(_all_sublanes(acc, jnp.add, 0) * (1.0 / D) + EPS)
        yield _Step(50, delay=8)
        yield _Step(10, [lambda: rstd], delay=1)
        return rstd

    def fwd_block(g, i, name, needs, free=(), known=False):
        j, t = g + 4 * i, i
        UB, AB, PB, ubu, abu = temps[t]
        yield _Wait(*needs)
        if known:
            means, squares = STAT[4 * g + i, pl.ds(0, 8)], STAT[4 * g + i, pl.ds(8, 8)]
            mean = means.sum(0) * 0.125
            var = (squares.sum(0) + 128.0 * ((means - mean) ** 2).sum(0)) * (1.0 / D)
            rstd = jax.lax.rsqrt(var + EPS)
            yield _Step(50, delay=6)
        else:
            yield settle(X[i])
            acc, m = None, g + opaque()
            for r in range(8):
                v = X[i][m, pl.ds(128 * r, 128), :].reshape(16, 8, 128).sum(0)
                acc = v if acc is None else acc + v
                if r % 2:
                    yield _Step(35, [lambda acc=acc: acc], delay=7 if r == 7 else 3)
            mean = _all_sublanes(acc, jnp.add, 0) * (1.0 / D)
            rstd = yield from ln_rstd(g, i, mean)
        mean8, rstd = (jnp.concatenate([v, v], 0) for v in (mean * 8.0, rstd))
        z = opaque()
        for r in range(8):
            rows = pl.ds(16 * r, 16)
            x = [X[i][g + z, pl.ds(128 * b + 16 * r, 16), :] for b in range(8)]
            s = [x[b] + x[b + 4] for b in range(4)]
            d = [x[b] - x[b + 4] for b in range(4)]
            e, o = s[0] + s[2], s[1] + s[3]
            UB[0, rows, :] = ((e + o - mean8) * rstd).astype(BF16)
            UB[0, pl.ds(128 + 16 * r, 16), :] = ((e - o) * rstd).astype(BF16)
            t1, t2 = (d[1] - d[3]) * RSQ2, (d[1] + d[3]) * RSQ2
            u = {1: (d[0] + t1, d[2] + t2), 2: (s[0] - s[2], s[1] - s[3]), 3: (d[0] - t1, d[2] - t2)}
            yield _Step(34, [anchor(ubu)], delay=1)
            for k in (1, 2, 3):
                c, sn = twid[z + 2 * k - 2, rows, :] * rstd, twid[z + 2 * k - 1, rows, :] * rstd
                re, m = u[k]
                if k == 3:
                    ur, ui = re * c + m * sn, m * c - re * sn
                else:
                    ur, ui = re * c - m * sn, m * c + re * sn
                UB[0, pl.ds(256 * k + 16 * r, 16), :] = ur.astype(BF16)
                UB[0, pl.ds(256 * k + 128 + 16 * r, 16), :] = ui.astype(BF16)
                yield _Step(26, [anchor(ubu)], delay=1)
        yield settle(ubu)

        def d_forward(point):
            z = opaque()
            first = _iota(8, 0) == 0

            def stage(c):
                u = (M_C4 if c == 1 else M_R) + opaque()
                lhs = mat(u) if c % 4 else _bf(tied(lambda r: mats[u, pl.ds(r, 8), :], 8, point))
                v = _dot(lhs, _bf(ubu[z, pl.ds(64 * c, 64), :]))
                return [(v[32 * u:32 * u + 16], v[32 * u + 16:32 * u + 32]) for u in range(4)]

            def put(row, u, v, v0=None):
                if u == 0 and v0 is not None:
                    v = jnp.concatenate([jnp.where(first, v0, v[:8]), v[8:]], 0)
                AB[0, pl.ds(row + 16 * u, 16), :] = v.astype(BF16)

            for u, (p1, p2) in enumerate(stage(0)):
                put(0, u, p1)
                put(528, u, p2, 0.0)
                if u == 0:
                    put(512, 0, jnp.zeros_like(p2), p2[:8])
            for u, (p1, p2) in enumerate(stage(1)):
                put(256, u, p1)
                put(528 + 256, u, p2)
            for k in (1, 2, 3):
                for u, ((p1, p2), (q1, q2)) in enumerate(zip(stage(2 * k), stage(2 * k + 1))):
                    if k == 3:
                        pr, pi, mr, mi = p1 - q2, p2 + q1, p1 + q2, p2 - q1
                        pi0, mi0 = q1[:8], -q2[:8]
                    else:
                        pr, pi, mr, mi = p1 + q2, p2 - q1, p1 - q2, p2 + q1
                        pi0, mi0 = -q1[:8], q2[:8]
                    put(64 * k, u, pr, p1[:8])
                    put(64 * (8 - k), u, mr, p2[:8])
                    put(528 + 64 * k, u, pi, pi0)
                    put(528 + 64 * (8 - k), u, mi, mi0)
            return 190

        yield _Mat(d_forward)
        yield settle(abu)
        yield _Wait(*free)

        def s_forward(point):
            z = opaque()
            fa, fb = mat(M_FA + j + z), mat(M_FB + j + z)
            for r0, rn in ((0, 256), (256, 272)):
                lhs = abu[z, pl.ds(r0 // 2, rn // 2), :] if r0 else tied(
                    lambda r: abu[z, pl.ds(r, 8), :], 16, point)
                u = _dot(_bf(lhs), fa)
                v = _dot(_bf(abu[z, pl.ds(264 + r0 // 2, 128), :]), fb)
                re, m = u[:256] + v, u[:256] - v
                if r0:
                    re, m = (jnp.concatenate([a, u[256:264]], 0) for a in (re, m))
                rn = re.shape[0]
                edge = (_iota(rn, 1) & 63) == 0
                ZT[2 * i, pl.ds(r0, rn), :] = re
                ZT[2 * i + 1, pl.ds(r0, rn), :] = jnp.where(
                    edge, lane_vec(L_MU + j, rn) * m + lane_vec(L_NU + j, rn) * re, pltpu.roll(m, 64, 1))
            return 400

        yield _Mat(s_forward)
        yield _Step(2, [anchor(ZT)], delay=SETTLE, marks=[name])

    def group_stage(g, name, needs, inverse):
        yield _Wait(*needs)

        def turn(z, k):
            if k == 0:
                return z
            c, s = rot[4 * g + k], rot[16 + 4 * g + k]
            if inverse:
                return z[0] * c - z[1] * s, z[1] * c + z[0] * s
            return z[0] * c + z[1] * s, z[1] * c - z[0] * s

        (src, a), (dst, b) = ((Z, 8 * g), (ZT, 0)) if inverse else ((ZT, opaque()), (Z, 8 * g))
        for r in range(65):
            if r % (16 if inverse else 64) == 0:
                yield hold(src, 2 * NB if inverse else 8)
            rows = pl.ds(8 * r, 8)
            z = [(src[a + 2 * i, rows, :], src[a + 2 * i + 1, rows, :]) for i in range(4)]
            if inverse:
                z = _radix4([turn(z[k], k) for k in range(4)], True)
            else:
                z = [turn(v, k) for k, v in enumerate(_radix4(z, False))]
            for i in range(4):
                dst[b + 2 * i, rows, :], dst[b + 2 * i + 1, rows, :] = z[i]
            yield _Step(35, [anchor(dst)], delay=1, marks=[name] if r == 64 else [])

    def spectral(row, size):
        rows = pl.ds(row, size)
        for k0 in range(4):
            z = _radix4([(Z[8 * g + 2 * k0, rows, :], Z[8 * g + 2 * k0 + 1, rows, :])
                         for g in range(4)], False)
            y = []
            for k1, (re, im) in enumerate(z):
                w = WS[k0 + 4 * k1, rows, :]
                wr = pltpu.bitcast(w << 16, F32)
                wi = pltpu.bitcast(w & np.uint32(0xFFFF0000), F32)
                y.append((re * wr - im * wi, re * wi + im * wr))
            y = _radix4(y, True)
            for g in range(4):
                Z[8 * g + 2 * k0, rows, :], Z[8 * g + 2 * k0 + 1, rows, :] = y[g]

    def spectral_rows(c2):
        for r in range(8):
            spectral(pl.multiple_of(128 * c2 + 16 * r, 16), 16)

    def inv_block(g, i, name, needs, n=None):
        j, t = g + 4 * i, i % 2
        UB, AB, PB, ubu, abu = temps[t]
        n = g if n is None else n
        z = opaque()
        yield _Wait(*needs)
        for r0, rn in _S_ROWS:
            if r0 == 0:
                yield hold(ZT, 8)
            re, im = ZT[z + 2 * i, pl.ds(r0, rn), :], ZT[z + 2 * i + 1, pl.ds(r0, rn), :]
            edge = (_iota(rn, 1) & 63) == 0
            rolled = pltpu.roll(im, 64, 1)
            u = re + jnp.where(edge, lane_vec(L_KU + j, rn) * im, rolled)
            if r0 < 512:
                v = re - jnp.where(edge, lane_vec(L_KV + j, rn) * im, rolled)
                AB[0, pl.ds(r0, rn), :] = u.astype(BF16)
                AB[0, pl.ds(528 + r0, rn), :] = v.astype(BF16)
            else:
                AB[0, pl.ds(512, 16), :] = jnp.concatenate([u, jnp.zeros_like(u)], 0).astype(BF16)
            yield _Step(rn, [anchor(abu)], delay=1, marks=[("read", name)] if r0 == 512 else [])
        yield settle(abu, 4)

        def s_inverse(point):
            z = opaque()
            fa, fb = mat(M_FA + j + z), mat(M_FB + j + z)
            first = _iota(8, 0) == 0

            def put(row, v, v0=None):
                if v0 is not None:
                    v = jnp.concatenate([jnp.where(first, v0, v[:8]), v[8:]], 0)
                UB[0, pl.ds(row, 64), :] = v.astype(BF16)

            for k in range(4):
                lo, hi = 32 * k, 32 * (8 - k if k else 4)
                a = [abu[z, pl.ds(lo, 32), :], abu[z, pl.ds(hi, 32), :]] if k % 2 else [
                    tied(lambda r, o=o: abu[z, pl.ds(o + r, 8), :], 4, point) for o in (lo, hi)]
                if k == 0:
                    a.append(abu[z, pl.ds(256, 8), :])
                re = _dot_t(_bf(jnp.concatenate(a, 0)), fa)
                im = _dot_t(_bf(jnp.concatenate(
                    [abu[z, pl.ds(264 + lo, 32), :], abu[z, pl.ds(264 + hi, 32), :]], 0)), fb)
                pr, mr, pi, mi = re[:64], re[64:128], im[:64], im[64:]
                if k == 0:
                    put(0, pr)
                    put(64, pi, re[128:136])
                    put(128, mr)
                    put(192, mi)
                else:
                    put(256 * k, pr + mr, pr[:8])
                    put(256 * k + 64, pi + mi, mr[:8])
                    put(256 * k + 128, pi - mi, pi[:8])
                    put(256 * k + 192, mr - pr, -mi[:8])
            return 190

        yield _Mat(s_inverse)
        yield settle(ubu, 4)
        yield d_stage(t, lambda c: {0: M_R0T, 1: M_C4T}.get(c, M_RT))
        yield settle(PB, 4)
        z = opaque()
        acc = None
        for r in range(16):
            rows = pl.ds(8 * r, 8)
            t0, t4 = PB[z, rows, :], PB[z, pl.ds(128 + 8 * r, 8), :]
            tk = {}
            for k in (1, 2, 3):
                c, sn = twid[z + 2 * k - 2, rows, :], twid[z + 2 * k - 1, rows, :]
                re = PB[z, pl.ds(256 * k + 8 * r, 8), :]
                im = PB[z, pl.ds(256 * k + 128 + 8 * r, 8), :]
                tk[k] = (re * c - im * sn, re * sn + im * c)
            e0, e1 = t0 + t4, t0 - t4
            s = [e0 + tk[2][0], e1 - tk[2][1], e0 - tk[2][0], e1 + tk[2][1]]
            al, be = tk[1][0] - tk[3][0], tk[1][1] + tk[3][1]
            o = [tk[1][0] + tk[3][0], (al - be) * RSQ2, tk[3][1] - tk[1][1], (al + be) * -RSQ2]
            for b in range(8):
                y = s[b] + o[b] if b < 4 else s[b - 4] - o[b - 4]
                v = X[i][g, pl.ds(128 * b + 8 * r, 8), :] + y
                X[i][n, pl.ds(128 * b + 8 * r, 8), :] = v
                acc = v if acc is None else acc + v
            yield _Step(57, [lambda v=acc: v], delay=5 if r == 15 else 2)
        yield settle(X[i], 4)
        mean = _all_sublanes(acc, jnp.add, 0) * (1.0 / D)
        rstd = yield from ln_rstd(n, i, mean)
        z = opaque()
        for r in range(8):
            v = X[i][n + z, pl.ds(128 * r, 128), :].reshape(16, 8, 128)
            HB[i][n, pl.ds(128 * r, 128), :] = ((v - mean[None]) * rstd[None]).reshape(128, 128).astype(BF16)
            yield _Step(41, [anchor(hbu[i])], delay=1, marks=[name] if r == 7 else [])

    def attend(g, i, name, needs):
        yield _Wait(*needs)
        yield settle(QB[i])
        j, z = g + 4 * i, opaque()
        even = (_iota(8, 0) & 1) == 0
        edge = _iota(8, 1) == 0

        def window(near, far, w, rows):
            return near[j + z + 4 - 2 * w, rows, :] if w <= 2 * i + 2 else far[j + z + 16 - 2 * w, rows, :]

        def mix_values(h, u):
            p = PW[h % 2][opaque()]
            for rows in (pl.ds(256 * h + 16 * u, 16), pl.ds(256 * h + 16 * u + 16, 16)):
                acc = functools.reduce(jnp.add, [p[16 * w:16 * w + 16] * window(VE, VS, w, rows)
                                                 for w in range(8)])
                HB[i][g, rows, :] = acc.astype(BF16)
            return _Step(63, [anchor(hbu[i])], delay=2, marks=[name] if (h, u) == (3, 14) else [])

        for h in range(5):
            logits = []
            for w0 in range(0, 8, 2):
                if h < 4:
                    rows = pl.ds(256 * h, 256)
                    q = q if w0 % 4 else QB[i][opaque(), rows, :]
                    for w in (w0, w0 + 1):
                        v = (q * window(KE, KS, w, rows)).reshape(16, 16, 128).sum(0)
                        v = jnp.where(even, v[:8] + pltpu.roll(v[:8], 7, 0), v[8:] + pltpu.roll(v[8:], 1, 0))
                        logits.append(jnp.where(edge & (2 * w > j), -1e9, v * SCALE) if w > 2 * i
                                      else v * SCALE)
                    yield _Step(138, [lambda v=v: v for v in logits[-2:]], delay=4)
                if h > 0:
                    yield mix_values(h - 1, 2 * w0)
                    yield mix_values(h - 1, 2 * w0 + 2)
            if h < 4:
                top = functools.reduce(jnp.maximum, logits)
                e = [jnp.exp(v - top) for v in logits]
                total = functools.reduce(jnp.add, e)
                yield _Step(30, [lambda v=total: v], delay=3)
                scale = 1.0 / total
                for w in range(8):
                    v = e[w] * scale
                    PW[h % 2][0, pl.ds(16 * w, 8), :] = jnp.where(even, v, pltpu.roll(v, 1, 0))
                    PW[h % 2][0, pl.ds(16 * w + 8, 8), :] = jnp.where(even, pltpu.roll(v, 7, 0), v)
                yield _Step(50, [anchor(PW[h % 2])], delay=6 if h == 3 else 1)

    def packed_sums(terms, signs):
        lo = [pltpu.bitcast(u << 16, F32) for u in terms]
        hi = [pltpu.bitcast(u & np.uint32(0xFFFF0000), F32) for u in terms]
        return [pltpu.pack_elementwise([v[p] + v[q] if s > 0 else v[p] - v[q] for v in (lo, hi)],
                                       packed_dtype=BF16) for p, s, q in signs]

    def half(ref, row):
        return lambda r, size, cols: ref[pl.ds(pl.multiple_of(row + r, 8), size), cols]

    kv_weight = (WS5, half(WK, 0), half(WV, 0))
    q_weight = (WQ5, half(WQ, 0), half(WQ, D // 4))
    o_weight = (WP5, *(lambda r, size, cols, e=e: WP[pl.ds(r + r // 32 * 32 + e, size), cols]
                       for e in (0, 32)))

    def left_sums(weight, row, size, needs=()):
        yield _Wait(*needs)
        sums, top, bottom = weight
        for r in range(0, size, 8):
            a = [ref(row + r, 8, pl.ds(c, 512)) for ref in (top, bottom) for c in (0, 512)]
            for e, v in enumerate(packed_sums(a, ((0, 1, 3), (2, 1, 3), (0, 1, 1), (2, -1, 0), (1, -1, 3)))):
                sums[e, pl.ds(pl.multiple_of(row + r, 8), 8), :] = v
            yield _Step(92, [anchor(sums)], delay=2, marks=["sums"] if r == size - 8 else [])

    def right_sums(dst, g, i, name, needs):
        yield _Wait(*needs)
        z = g + opaque()
        for r in range(0, 256, 16):
            b = [hbu[n][z, pl.ds(k + r, 16), :] for k in (0, 256) for n in (i, i + 1)]
            for e, v in enumerate(packed_sums(b, ((0, 1, 3), (1, -1, 3), (2, -1, 0), (0, 1, 1), (2, 1, 3)))):
                dst[e, pl.ds(r, 16), :] = v
            yield _Step(47, [anchor(dst)], delay=SETTLE if r == 240 else 1,
                        marks=[name] if r == 240 else [])

    def strassen(sch, weight, right, g, i, m, store, needs, marks):
        for n in needs:
            sch.run(n)
        sums, top, bottom = weight
        rows = pl.ds(pl.multiple_of(64 * m, 64), 64)

        def product(left, b):
            sch.fresh = True
            head = tied(lambda r: left(32 * m + r, 8, pl.ds(0, 128)), 4, lambda: sch.point(8.0))
            return _dot(_bf(jnp.concatenate([head, left(32 * m, 32, pl.ds(128, 384))], 1)), _bf(b))

        def a(e):
            return lambda r, size, cols: sums[e, pl.ds(pl.multiple_of(r, 8), size), cols]

        def b(e):
            return right[e + opaque()]

        m2 = product(a(1), hbu[i][g + opaque(), pl.ds(0, 256), :])
        m4 = product(lambda r, size, cols: bottom(r, size, pl.ds(512 + cols.start, cols.size)), b(2))
        store(1, i, rows, m2 + m4)
        m1 = product(a(0), b(0))
        c11, c22 = m1 + m4, m1 - m2
        c11 = c11 + product(a(4), b(4))
        c22 = c22 + product(a(3), b(3))
        m5 = product(a(2), hbu[i + 1][g + opaque(), pl.ds(256, 256), :])
        store(0, i, rows, c11 - m5)
        v = product(top, b(1))
        store(0, i + 1, rows, v + m5)
        store(1, i + 1, rows, c22 + v)
        sch.results.append(v[:8])
        for name in marks:
            sch.done[name] = sch.slot + sch.wait

    def kv_proj(sch, g, i, name, needs):
        def store(lower, n, rows, v):
            (KE, VE)[lower][g + 4 * n + 4, rows, :] = v
        for m in range(16):
            strassen(sch, kv_weight, SB[i // 2], g, i, m, store, needs, [name] if m == 15 else [])

    def q_proj(sch, g, i, name, needs):
        def store(lower, n, rows, v):
            QB[n][0, pl.ds(512 * lower + rows.start, 64), :] = v
        for m in range(8):
            strassen(sch, q_weight, SB[i // 2], g, i, m, store, needs, [name] if m == 7 else [])

    def o_proj(sch, g, i, m, needs, marks, right):
        def store(lower, n, rows, v):
            rows = pl.ds(128 * m + 64 * lower, 64)
            X[n][g, rows, :] = X[n][g, rows, :] + v
        strassen(sch, o_weight, right, g, i, m, store, needs, marks)

    def shift_block(g, i, name, needs):
        yield _Wait(*needs)
        j, z = g + 4 * i, opaque()
        for m in range(16):
            rows = pl.ds(64 * m, 64)
            for ref, to in ((KE, KS), (VE, VS)):
                v = pltpu.roll(ref[j + 4 + z, rows, :], 1, 1)
                if ref is VE:
                    v = jnp.where(_iota(64, 1) == 0, ref[4 + z, rows, :], v)
                to[j, rows, :] = v
                if i == 3:
                    ref[g, rows, :] = v
            yield _Step(12, delay=8, marks=[name] if m == 15 else [])

    def transpose_quarter(w, h, via):
        for r in range(4):
            v = WRAW[w, pl.ds(256 * r, 256), pl.ds(pl.multiple_of(256 * h, 256), 256)]
            v = pltpu.bitcast(v.T, F32)
            via[0, pl.ds(256 * r, 128), :], via[0, pl.ds(256 * r + 128, 128), :] = v[:, :128], v[:, 128:]
            yield _Step(40, delay=16)

    def reorder_quarter(w, h, via, name=None):
        z = 0 if isinstance(h, int) else opaque()
        for c in range(8):
            WT[w][pl.ds(pl.multiple_of(128 * h, 128), 128), pl.ds(128 * c, 128)] = pltpu.bitcast(
                jnp.concatenate([via[z, pl.ds(128 * c + u, 8, stride=16), :] for u in range(16)], 0), U32)
            yield _Step(20, delay=4, marks=[name] if c == 7 else [])

    def query_weight(h):
        yield from transpose_quarter(0, h, QB[0])
        yield from reorder_quarter(0, h, QB[0], "w")

    def transpose_wo(name):
        for c in range(8):
            for h in range(4):
                v = jnp.concatenate([wou[c, pl.ds(128 * h + u, 8, stride=16), :] for u in range(16)], 0)
                WP[pl.ds(64 * c, 64), pl.ds(256 * h, 256)] = pltpu.bitcast(_bf(v).T, U32)
                yield _Step(20, delay=10, marks=[name] if c == 7 and h == 3 else [])

    def prep_spectral_weights(c2):
        lane = _iota(8, 1)
        order = jnp.where(lane > 64, 192 - lane, lane)

        def words(k2):
            re, im = (wsu[u, k2, pl.ds(c2, 64, stride=4), :] for u in range(2))
            return ((re & np.uint32(0xFFFF)) | (im << 16), (re >> 16) | (im & np.uint32(0xFFFF0000)))

        def arrange(w, below):
            w = jnp.where(_iota(w.shape[0], 1) < 64, w, below)
            return jnp.concatenate([jnp.take_along_axis(w[u:u + 8], order, axis=1)
                                    for u in range(0, w.shape[0], 8)], 0)

        below = words(15)
        for k2 in range(16):
            here = words(k2)
            for e in range(2):
                cl = 2 * c2 + e
                w = arrange(here[e], below[e])
                WS[k2, pl.ds(64 * cl, 64), :] = pltpu.roll(w, 1, 0) if cl > 4 else w
            below = here
            yield _Step(100)
        if c2 == 0:
            def nyquist(k2):
                re, im = (jnp.broadcast_to(WN[u, :, pl.ds(128 * k2, 128)].astype(F32), (8, 128))
                          for u in range(2))
                return pltpu.pack_elementwise([re, im], packed_dtype=BF16)
            for k2 in range(16):
                WS[k2, pl.ds(512, 8), :] = arrange(nyquist(k2), nyquist((k2 + 15) % 16))

    def write_out(p, c, name, needs):
        yield _Wait(*needs)
        rows = pl.ds(pl.multiple_of(128 * c, 128), 128)
        g, i = 2 * p % 4 + opaque(), p // 2
        w = pltpu.pack_elementwise([X[i][g, rows, :], X[i][g + 1, rows, :]], packed_dtype=BF16)
        xru[c, pl.ds(p, 128, stride=8), :] = w.T
        yield _Step(30, marks=[name])

    for c in range(8):
        x_copy(c).start()
    for c in range(5):
        mats[M_R + c] = d_mats[c]

    def make_twiddle(k):
        PB = temps[0][2]
        PB[0, pl.ds(0, 128), :] = lane_vec(L_TWID + k, 128)
        twid[k] = PB[opaque(), pl.ds(0, 128), :].T

    _loop(6, make_twiddle, "make_twiddle")

    def make_dft(j):
        fa, fb = lanes[pl.ds(L_FA, 128), :], lanes[pl.ds(L_FB, 128), :]
        c, sn = lane_vec(L_COS + j, 128), lane_vec(L_SIN + j, 128)
        UB, _, _, ubu, _ = temps[0]
        UB[0, pl.ds(0, 128), :] = (fa * c + fb * sn).astype(BF16)
        UB[0, pl.ds(128, 128), :] = (fb * c - fa * sn).astype(BF16)
        mats[M_FA + j], mats[M_FB + j] = ubu[0, pl.ds(0, 64), :], ubu[0, pl.ds(64, 64), :]

    _loop(NB, make_dft, "make_dft")

    def load_x(c):
        x_copy(c).wait()
        pl.when(c == 6)(lambda: start_all(spec_copies[0]))
        pl.when(c == 7)(lambda: start_all(spec_copies[1]))
        rows = pl.ds(pl.multiple_of(128 * c, 128), 128)
        for p in range(8):
            w = xru[c, pl.ds(p, 128, stride=8), :].T
            for e, bits in enumerate((w << 16, w & np.uint32(0xFFFF0000))):
                g, i = 2 * p % 4 + e, p // 2
                v = pltpu.bitcast(bits, F32)
                X[i][g, rows, :] = v
                v = v.reshape(16, 8, 128)
                mean = _all_sublanes(v.sum(0), jnp.add, 0) * (1.0 / 128)
                STAT[4 * g + i, c] = mean
                STAT[4 * g + i, 8 + c] = _all_sublanes(((v - mean) ** 2).sum(0), jnp.add, 0)

    _loop(8, load_x, "load_x")

    def after(name, action):
        yield _Wait(name)
        action()

    def spectral_weights():
        yield _Wait(("f", 2, 1))
        for c in spec_copies[0] + spec_copies[1]:
            c.wait()
        for c2 in range(4):
            yield from prep_spectral_weights(c2)

    with jax.named_scope("first_forward"):
        sch = _Sched(0.72, 20)
        sch.add(after(("f", 0, 1), w_copies[1].start), "k")
        sch.add(after(("f", 1, 1), w_copies[2].start), "v")
        sch.add(after(("f", 2, 3), w_copies[0].start), "q")
        for g in range(4):
            for i in range(4):
                sch.add(fwd_block(g, i, ("f", g, i), [("f", g - 1, i)] if g else [],
                                  [("r", g - 1)] if g else [], True), ("f", g, i))
            sch.add(group_stage(g, ("r", g), [("f", g, i) for i in range(4)], False), ("r", g))
        sch.add(spectral_weights(), "s")
        sch.drive()
    start_all(wo_copies)

    def keys_values(layer, g):
        sch = _Sched(0.41, 32, 3) if layer == 0 else _Sched(0.36, 28, 2)
        nxt = (g + 1) % 4
        sch.add(inv_block(g, 2, ("i", 2), []), ("i", 2))
        sch.add(inv_block(g, 3, ("i", 3), [("read", ("i", 2))]), ("i", 3))
        sch.add(right_sums(SB[1], g, 2, ("b", 2), [("i", 2), ("i", 3)]), ("b", 2))
        sch.add(group_stage(nxt, "r", [("read", ("i", 3))], True), "r")
        sch.add(inv_block(nxt, 0, ("i", 4), ["r", ("i", 2)], n=g + 1), ("i", 4))
        sch.add(inv_block(nxt, 1, ("i", 5), [("read", ("i", 4)), ("i", 3)], n=g + 1), ("i", 5))
        if layer == 0:
            sch.add(query_weight(g), "w")
            sch.add(left_sums(q_weight, 128 * (g % 2), 128, ["w"]), "sums")
        for i in (2, 3):
            sch.add(shift_block((g + 3) % 4, i, ("s", i), []), ("s", i))
        for i in (0, 1):
            sch.add(shift_block(g, i, ("s", i), [("kv", 0)]), ("s", i))
        sch.add(right_sums(SB[0], nxt, 0, ("b", 4), [("i", 4), ("i", 5), ("kv", 0)]), ("b", 4))
        kv_proj(sch, g, 0, ("kv", 0), [])
        kv_proj(sch, g, 2, ("kv", 2), [("b", 2)])
        sch.finish()

    def mix(g, after, last):
        tail = after is None
        sch = _Sched(0.66 if last else 0.63, 28 if last else 32)
        pace = 0.48 if tail else 0.35 if last else 0.32
        ahead = [(g, 2), (g, 3)] + ([] if tail else [(after, 0), (after, 1)])
        for n, block in enumerate(ahead):
            sch.add(attend(*block, ("a", n), [[], [("a", 0)], [("a", 1), ("q", 0)], [("a", 2)]][n]),
                    ("a", n), pace=pace)
            if n % 2:
                sch.add(right_sums(SB[2 + block[1] // 2], block[0], block[1] - 1, ("b", n),
                                   [("a", n)] + ([("o", 0)] if n == 3 else [])), ("b", n))
        for i in () if tail else (0, 2):
            sch.add(right_sums(SB[i // 2], after, i, ("h", i), [("q", 0)] if i else []), ("h", i))
        if not last:
            sch.add(group_stage((g + 3) % 4, "r", [], False), "r")
            for i in range(4):
                sch.add(fwd_block(g, i, ("f", i), [("o", i - i % 2)], ["r"]), ("f", i))
        now = 6 if last else 8
        for i in (0, 2):
            for m in range(now):
                o_proj(sch, g, i, m, [("b", 1)] if i else [], [("o", i)] if m == now - 1 else [],
                       SB[2 + i // 2])
            if not tail:
                q_proj(sch, after, i, ("q", i), [("h", i)])
        if tail:
            sch.add(group_stage(g, "s", [("f", i) for i in range(4)], False), "s")
        sch.share = 0.92
        sch.drive()

    def mix_odd():
        sch = _Sched(0.66)
        blocks = [(1, 2), (1, 3), (3, 0), (3, 1), (3, 2), (3, 3)]
        for n, (g, i) in enumerate(blocks):
            sch.add(attend(g, i, ("a", n), ([("a", n - 1)] if n else []) + ([("q", i)] if n in (2, 4) else [])),
                    ("a", n), pace=0.32)
            if n % 2:
                sch.add(right_sums(SB[(3, 2, 0)[n // 2]], g, i - 1, ("b", g, i - 1),
                                   [("a", n)] + ([("o", 1, 0, 5)] if n > 1 else [])), ("b", g, i - 1))
        for i in (0, 2):
            sch.add(right_sums(SB[i // 2], 3, i, ("h", i), []), ("h", i))
        for g in (1, 3):
            for i in range(4):
                for c in range(6):
                    sch.add(write_out(2 * i + g // 2, c, ("w", g, i, c), [("o", g, i - i % 2, c)]),
                            ("w", g, i, c))
        for g, i, slot, count in ((1, 0, 2, 6), (1, 2, 3, 8), (3, 0, 2, 8), (3, 2, 0, 6)):
            for m in range(count):
                o_proj(sch, g, i, m, [("b", g, i)] if (g, i) != (1, 0) else [], [("o", g, i, m)], SB[slot])
            for e in (0, 2) if (g, i) == (1, 0) else ():
                q_proj(sch, 3, e, ("q", e), [("h", e)] + ([("a", 1)] if e else []))
        sch.share = 0.92
        sch.drive()

    def postponed():
        sch = _Sched(0.7, 12)
        slots = {(3, 2): 0, (2, 2): 1, (0, 2): 2, (2, 0): 3, (0, 0): 0, (1, 0): 1}
        for n, (pair, slot) in enumerate(slots.items()):
            if n:
                sch.add(right_sums(SB[slot], *pair, pair, [(list(slots)[n - 4], 7)] if n >= 4 else []), pair)
        for p, pairs in enumerate(2 * [[(0, 0), (1, 0)], [(2, 0)]] + 2 * [[(0, 2)], [(2, 2), (3, 2)]]):
            for c in (6, 7):
                sch.add(write_out(p, c, ("w", p, c), [(pair, c) for pair in pairs]), ("w", p, c))

        def copy_out():
            yield _Wait(*[("w", p, 6) for p in range(8)])
            out_copy(6).start()

        sch.add(copy_out(), "copy")
        for part in (list(slots)[:2], list(slots)[2:]):
            for c in (6, 7):
                for pair in part:
                    o_proj(sch, *pair, c, [pair] if pair != (3, 2) else [], [(pair, c)], SB[slots[pair]])
        sch.drive()
        out_copy(7).start()

    def first_queries(layer):
        sch = _Sched(0.68)
        sch.add(right_sums(SB[1], 0, 2, ("h", 2), []), ("h", 2))
        sch.add(shift_block(3, 2, "s", []), "s")
        sch.add(attend(0, 0, ("a", 0), ["q"]), ("a", 0), pace=0.4)
        sch.add(attend(0, 1, ("a", 1), [("a", 0)]), ("a", 1), pace=0.4)
        sch.add(right_sums(SB[2], 0, 0, "b", [("a", 1)]), "b")
        sch.add(shift_block(3, 3, "t", []), "t")
        if layer == 0:
            for c in wo_copies:
                c.wait()
            sch.add(transpose_wo("w"), "w")
            sch.add(left_sums(o_weight, 0, 256, ["w"]), "sums")
        q_proj(sch, 0, 0, "q", [])
        q_proj(sch, 0, 2, None, [("h", 2)])
        sch.finish()

    def key_value_weights():
        w_copies[1].wait()
        w_copies[2].wait()
        for h in range(6):
            work = []
            for w in (1, 2):
                if h < 4:
                    work.append(transpose_quarter(w, h, QB[2 * (h % 2) + w - 1]))
                if 0 < h < 5:
                    work.append(reorder_quarter(w, h - 1, QB[2 * ((h - 1) % 2) + w - 1]))
            if h > 1:
                work.append(left_sums(kv_weight, 128 * (h - 2), 128))
            list(itertools.zip_longest(*work))

    for layer in range(2):
        with jax.named_scope("spectral"):
            _loop(4, spectral_rows, "rows")
            if layer == 0:
                _loop(zero + 1, lambda _: key_value_weights(), "weights")
            spectral(512, 8)
        sch = _Sched(0.92)
        sch.add(group_stage(0, "r", [], True), "r")
        sch.add(inv_block(0, 0, ("i", 0), ["r"]), ("i", 0))
        sch.add(inv_block(0, 1, ("i", 1), ["r"]), ("i", 1))
        sch.add(right_sums(SB[0], 0, 0, "b", [("i", 0), ("i", 1)]), "b")
        sch.drive()
        if layer == 0:
            w_copies[0].wait()
        _loop(4, lambda g: keys_values(layer, g), "keys_values")
        first_queries(layer)
        if layer == 0:
            pl.when(never)(lambda: [spectral_rows(c % 4) for c in range(5)] and None)
        if layer == 0:
            _loop(3, lambda g: mix(g, g + 1, False), "mix")
            mix(3, None, False)
        else:
            _loop(2, lambda u: mix(2 * u, 2 - u, True), "mix")
            mix_odd()
    for c in range(6):
        out_copy(c).start()
    with jax.named_scope("postponed"):
        postponed()
    for c in range(8):
        out_copy(c).wait()


@jax.jit
def pallas_interleave_layers__spectral_gfnet__sliding_local_dilated__prompt_kernel(
    A_x: jax.Array,
    A_w_r: jax.Array,
    A_w_i: jax.Array,
    B_x: jax.Array,
    B_wqkv: jax.Array,
    B_wo: jax.Array,
):
    del B_x
    hbm = pl.BlockSpec(memory_space=pl.ANY)
    smem = pl.BlockSpec(memory_space=pltpu.SMEM)
    out = pl.pallas_call(
        _kernel,
        out_shape=jax.ShapeDtypeStruct((S, D), BF16),
        in_specs=[smem, smem, pl.BlockSpec(), pl.BlockSpec(), hbm, hbm, hbm, hbm, hbm],
        out_specs=hbm,
        scratch_shapes=[
            pltpu.VMEM((37, 64, 128), U32),
            pltpu.VMEM((6, 128, 128), F32),
            pltpu.VMEM((NB, 16, 8, 128), F32),
            pltpu.VMEM((NB + 4, D, 128), F32),
            pltpu.VMEM((NB + 4, D, 128), F32),
            pltpu.VMEM((NB, D, 128), F32),
            pltpu.VMEM((NB, D, 128), F32),
            pltpu.VMEM((2 * NB + 1, ZR, 128), F32),
            pltpu.VMEM((9, ZR, 128), F32),
            pltpu.VMEM((NB, ZR, 128), U32),
            *4 * [pltpu.VMEM((D // 2, D), U32)],
            pltpu.VMEM((5, D // 2, D // 2), U32),
            *2 * [pltpu.VMEM((5, D // 4, D // 2), U32)],
            *4 * [pltpu.VMEM((5, D // 4, 128), U32)],
            pltpu.VMEM((8, S, 128), BF16),
            pltpu.VMEM((2, NB, D // 2, 128), BF16),
            pltpu.VMEM((2, 1, S), BF16),
            pltpu.VMEM((3, D, D), BF16),
            pltpu.VMEM((8, D, 128), BF16),
            pltpu.VMEM((1, 128, 128), F32),
            pltpu.VMEM((1, 128, 128), F32),
            pltpu.SemaphoreType.DMA((24,)),
            *2 * [pltpu.VMEM((1, D, 128), F32)],
        ] + 4 * [
            pltpu.VMEM((5, D, 128), F32),
            pltpu.VMEM((5, D, 128), BF16),
            pltpu.VMEM((1, D, 128), F32),
            pltpu.VMEM((1, D, 128), BF16),
            pltpu.VMEM((1, 1152, 128), BF16),
        ],
        compiler_params=pltpu.CompilerParams(vmem_limit_bytes=126 * 2 ** 20),
    )(_ZERO, _ROT, _MATS, _LANES, A_x.reshape(S, D), A_w_r.T, A_w_i.T, B_wqkv, B_wo)
    return out.reshape(1, S, D)
```

```python
import functools
import itertools

import numpy as np

import jax
import jax.numpy as jnp
import jax.experimental.pallas as pl
import jax.experimental.pallas.tpu as pltpu

S, D, NB = 2048, 1024, 16
ZR = 576
F32, BF16, U32, I32 = jnp.float32, jnp.bfloat16, jnp.uint32, jnp.int32
EPS = 1e-5
SCALE = 32 ** -0.5
RSQ2 = float(np.sqrt(0.5))
GRAIN = 1
SETTLE = 6

_S_ROWS = [(32 * u, 32) for u in range(16)] + [(512, 8)]

M_FA, M_FB, M_R, M_C4, M_RT, M_C4T, M_R0T = 0, 16, 32, 33, 34, 35, 36
L_MU, L_NU, L_KU, L_KV, L_COS, L_SIN, L_TWID, L_FA, L_FB = 0, 16, 32, 48, 64, 80, 96, 104, 232


def _bf16_bits(a):
    u = np.ascontiguousarray(a, dtype=np.float32).view(np.uint32).astype(np.uint64)
    return ((u + 0x7FFF + ((u >> 16) & 1)) >> 16).astype(np.uint32)


def _constants():
    a = np.arange(128)
    k1 = np.arange(64)
    alt = (-1.0) ** a
    lanes = np.zeros((L_FB + 128, 128))
    t = 2 * np.pi * np.outer(a, k1) / 128
    fa = np.concatenate([np.cos(t), -np.sin(t)], 1)
    fb = np.concatenate([np.sin(t), -np.cos(t)], 1)
    fa[:, 0], fb[:, 0] = RSQ2, -RSQ2
    fa[:, 64], fb[:, 64] = alt, 0.0
    lanes[L_FA:L_FA + 128], lanes[L_FB:L_FB + 128] = fa, fb
    for j in range(NB):
        ang = 2 * np.pi * j / 32 + np.pi / 32
        p, q = (_bf16_bits([np.cos(ang), np.sin(ang)]) << 16).view(np.float32).astype(np.float64)
        turn = 2 * np.pi * j * np.tile(k1, 2) / S
        lanes[L_COS + j], lanes[L_SIN + j] = np.cos(turn), np.repeat([-1.0, 1.0], 64) * np.sin(turn)
        lanes[L_COS + j, 64], lanes[L_SIN + j, 64] = p, q
        lanes[L_MU + j, 0], lanes[L_MU + j, 64] = 1.0, (q / p + p / q) / 2
        lanes[L_NU + j, 0], lanes[L_NU + j, 64] = 0.0, (q / p - p / q) / 2
        lanes[L_KU + j, 0], lanes[L_KU + j, 64] = 1.0, q / p
        lanes[L_KV + j, 0], lanes[L_KV + j, 64] = 1.0, p / q
    for k in (1, 2, 3):
        lanes[L_TWID + 2 * k - 2] = np.cos(2 * np.pi * a * k / D)
        lanes[L_TWID + 2 * k - 1] = np.sin(2 * np.pi * a * k / D)
    th = 2 * np.pi * np.outer(k1, a) / 128
    r = np.concatenate([np.cos(th), -np.sin(th)], 0)
    r[64] = alt
    th = 2 * np.pi * np.outer(2 * k1 + 1, a) / 256
    c4 = np.concatenate([np.cos(th), -np.sin(th)], 0)
    inv = 2.0 / (S * D)
    r0t = inv * r.T
    r0t[:, 0::64] *= 0.5
    rows = np.arange(128).reshape(2, 4, 16).transpose(1, 0, 2).ravel()
    bits = _bf16_bits(np.stack([r[rows], c4[rows], inv * r.T, inv * c4.T, r0t]))
    ang = 2 * np.pi * np.outer(np.arange(4), np.arange(4)).ravel() / 16
    rot = np.concatenate([np.cos(ang), np.sin(ang)]).astype(np.float32)
    return bits[:, 0::2] | (bits[:, 1::2] << 16), lanes.astype(np.float32), rot


_MATS, _LANES, _ROT = _constants()
_ZERO = np.zeros((1,), np.int32)


class _Step:
    def __init__(self, cost, anchors=(), delay=0, marks=()):
        self.cost, self.anchors, self.delay, self.marks = cost, list(anchors), delay, list(marks)


class _Wait:
    def __init__(self, *names):
        self.names = names


class _Mat:
    def __init__(self, emit):
        self.emit = emit


class _Hold:
    def __init__(self, store):
        self.store = store


class _Task:
    def __init__(self, gen, pace):
        self.gen, self.pace, self.blocked, self.not_before, self.held = gen, pace, (), 0, None
        self.allowed = 0.0


class _Sched:
    def __init__(self, share=0.0, wait=28, lag=3):
        self.lag = lag
        self.wait = wait
        self.share = share
        self.tasks, self.done, self.producer = [], {}, {}
        self.slot, self.credit, self.anchors, self.results = 0, 0.0, [], []
        self.fresh = False

    def add(self, gen, name, pace=99):
        self.producer[name] = self.producer["read", name] = _Task(gen, pace)
        self.tasks.append(self.producer[name])

    def _ready(self, t):
        return t.not_before <= self.slot and all(
            n in self.done and self.done[n] <= self.slot for n in t.blocked)

    def _advance(self, t, mats=True):
        item, t.held = t.held or next(t.gen, None), None
        if item is None:
            self.tasks.remove(t)
        elif isinstance(item, _Wait):
            t.blocked = item.names
        elif isinstance(item, _Hold):
            if len(self.results) >= self.lag:
                item.store(self.results[-self.lag])
        elif isinstance(item, _Mat):
            if mats:
                t.not_before = float("inf")
                self.fresh = False
                self.credit -= item.emit(lambda: self.point(0.0)) or 0
                t.not_before = self.slot + self.wait
            else:
                t.held, t.not_before = item, self.slot + 1
        else:
            t.blocked = ()
            t.not_before = self.slot + item.delay
            self.credit -= item.cost
            self.anchors += item.anchors
            for n in item.marks:
                self.done[n] = self.slot + item.delay
            return True

    def run(self, *names):
        while not all(n in self.done for n in names):
            for n in names:
                if n not in self.done:
                    for b in self.producer[n].blocked:
                        self.run(b)
                    self._advance(self.producer[n])

    def drive(self):
        while self.tasks:
            ready = [t for t in self.tasks if self._ready(t)]
            if not ready:
                self.slot += 1
                continue
            self.anchors, self.credit = self.anchors[-2:], 0.0
            self._advance(next((t for t in ready if t.held), ready[0]))
            self.slot -= min(self.credit, 0.0) / 60

    def finish(self):
        self.run(*[n for n in self.producer if n[0] != "read"])

    def point(self, own):
        for t in self.tasks:
            t.allowed = min(t.allowed, 0.0) + t.pace
        while True:
            t = next((t for t in self.tasks if self._ready(t) and t.allowed > 0
                      and self.credit > 0), None)
            if t is None:
                break
            if self._advance(t, self.fresh):
                t.allowed -= 1
        anchors, self.anchors = self.anchors, []
        self.credit = min(self.credit, 10.0) + 64 * self.share - own
        self.fresh = False
        self.slot += 1
        return anchors


def _dot(a, b):
    return jnp.dot(a, b, preferred_element_type=F32)


def _dot_t(a, b):
    return jax.lax.dot_general(a, b, (((1,), (1,)), ((), ())), preferred_element_type=F32)


def _bf(u):
    return pltpu.bitcast(u, BF16)


def _iota(rows, dim):
    return jax.lax.broadcasted_iota(I32, (rows, 128), dim)


def _radix4(z, inverse):
    (r0, i0), (r1, i1), (r2, i2), (r3, i3) = z
    ar, ai, cr, ci = r0 + r2, i0 + i2, r0 - r2, i0 - i2
    br, bi, dr, di = r1 + r3, i1 + i3, r1 - r3, i1 - i3
    lo, hi = (cr + di, ci - dr), (cr - di, ci + dr)
    if inverse:
        lo, hi = hi, lo
    return [(ar + br, ai + bi), lo, (ar - br, ai - bi), hi]


def _all_sublanes(v, op, axis):
    for sh in (4, 2, 1):
        v = op(v, pltpu.roll(v, sh, axis))
    return v


def _loop(n, body, name):
    def step(i, carry):
        body(i)
        return carry
    with jax.named_scope(name):
        jax.lax.fori_loop(0, n, step, 0)


def _kernel(zero_ref, rot, d_mats, lanes, x_hbm, wr_hbm, wi_hbm, wqkv_hbm, wo_hbm, out_hbm,
            mats, twid, STAT, KE, VE, KS, VS, Z, ZT, WS, WQ, WK, WV, WP, WS5, WQ5, WP5, SB0, SB1, SB2, SB3, XR, WRI, WN, WRAW, WO, PW0, PW1, sems, *split):
    zero = zero_ref[0]
    never = zero != 0
    X, HB, QB = split[2::5], split[3::5], split[4::5]
    hbu = [r.bitcast(U32) for r in HB]
    xru, wsu, wou = XR.bitcast(U32), WRI.bitcast(U32), WO.bitcast(U32)
    temps = [(ub, ab, pb, ub.bitcast(U32), ab.bitcast(U32))
             for ub, ab, pb in zip(split[5::5], split[6::5], 2 * split[:2])]
    PW, SB, WT = (PW0, PW1), (SB0, SB1, SB2, SB3), (WQ, WK, WV, WP)
    counter = [0]

    def opaque():
        counter[0] += 1
        return zero * counter[0]

    def anchor(ref):
        at = (0,) * (len(ref.shape) - 2)
        return lambda: ref[(*at, pl.ds(pl.multiple_of(zero * 8, 8), 8), pl.ds(0, 128))]

    def settle(ref, points=SETTLE):
        return _Step(2, [anchor(ref)], delay=points)

    def hold(ref, spare, row=0):
        def store(v):
            ref[spare, pl.ds(pl.multiple_of(row + zero * 8, 8), 8), :] = v
        return _Hold(store)

    def tied(load, vregs, point):
        parts = []
        for r in range(vregs):
            anchors = [a for _ in range(GRAIN) for a in point()] if r % GRAIN == 0 else []
            u = load(8 * r)
            for a in anchors:
                u = jnp.where(never, pltpu.bitcast(a(), U32), u)
            parts.append(u)
        return jnp.concatenate(parts, 0)

    def mat(i):
        return _bf(mats[i])

    def d_stage(t, which):
        UB, AB, PB, ubu, abu = temps[t]

        def emit(point):
            z = opaque()
            for c in range(8):
                lhs = mat(which(c) + opaque()) if c % 4 else _bf(
                    tied(lambda r, u=which(c) + opaque(): mats[u, pl.ds(r, 8), :], 8, point))
                PB[0, pl.ds(128 * c, 128), :] = _dot(lhs, _bf(ubu[z, pl.ds(64 * c, 64), :]))
        return _Mat(emit)

    def lane_vec(i, rows):
        return jnp.broadcast_to(lanes[pl.ds(i, 1), :], (rows, 128))

    def x_copy(c):
        return pltpu.make_async_copy(
            x_hbm.at[:, pl.ds(pl.multiple_of(128 * c, 128), 128)], XR.at[c], sems.at[c])

    def out_copy(c):
        return pltpu.make_async_copy(
            XR.at[c], out_hbm.at[:, pl.ds(pl.multiple_of(128 * c, 128), 128)], sems.at[8 + c])

    spec_copies = [[pltpu.make_async_copy(w.at[pl.ds(0, 512), pl.ds(128 * k2, 128)], WRI.at[u, k2],
                                          sems.at[16 + u]) for k2 in range(16)]
                   + [pltpu.make_async_copy(w.at[pl.ds(512, 1), :], WN.at[u], sems.at[22 + u])]
                   for u, w in enumerate((wr_hbm, wi_hbm))]

    def start_all(copies):
        for c in copies:
            c.start()
    w_copies = [pltpu.make_async_copy(wqkv_hbm.at[:, pl.ds(D * w, D)], WRAW.at[w], sems.at[18 + w])
                for w in range(3)]
    wo_copies = [pltpu.make_async_copy(wo_hbm.at[:, pl.ds(128 * c, 128)], WO.at[c], sems.at[21])
                 for c in range(8)]

    def ln_rstd(g, i, mean):
        acc, m = None, g + opaque()
        for r in range(8):
            d = X[i][m, pl.ds(128 * r, 128), :].reshape(16, 8, 128) - mean[None]
            v = (d * d).sum(0)
            acc = v if acc is None else acc + v
            if r < 7:
                yield _Step(50, [lambda acc=acc: acc], delay=3)
        rstd = jax.lax.rsqrt(_all_sublanes(acc, jnp.add, 0) * (1.0 / D) + EPS)
        yield _Step(50, delay=8)
        yield _Step(10, [lambda: rstd], delay=1)
        return rstd

    def fwd_block(g, i, name, needs, free=(), known=False):
        j, t = g + 4 * i, i
        UB, AB, PB, ubu, abu = temps[t]
        yield _Wait(*needs)
        if known:
            means, squares = STAT[4 * g + i, pl.ds(0, 8)], STAT[4 * g + i, pl.ds(8, 8)]
            mean = means.sum(0) * 0.125
            var = (squares.sum(0) + 128.0 * ((means - mean) ** 2).sum(0)) * (1.0 / D)
            rstd = jax.lax.rsqrt(var + EPS)
            yield _Step(50, delay=6)
        else:
            yield settle(X[i])
            acc, m = None, g + opaque()
            for r in range(8):
                v = X[i][m, pl.ds(128 * r, 128), :].reshape(16, 8, 128).sum(0)
                acc = v if acc is None else acc + v
                if r % 2:
                    yield _Step(35, [lambda acc=acc: acc], delay=7 if r == 7 else 3)
            mean = _all_sublanes(acc, jnp.add, 0) * (1.0 / D)
            rstd = yield from ln_rstd(g, i, mean)
        mean8, rstd = (jnp.concatenate([v, v], 0) for v in (mean * 8.0, rstd))
        z = opaque()
        for r in range(8):
            rows = pl.ds(16 * r, 16)
            x = [X[i][g + z, pl.ds(128 * b + 16 * r, 16), :] for b in range(8)]
            s = [x[b] + x[b + 4] for b in range(4)]
            d = [x[b] - x[b + 4] for b in range(4)]
            e, o = s[0] + s[2], s[1] + s[3]
            UB[0, rows, :] = ((e + o - mean8) * rstd).astype(BF16)
            UB[0, pl.ds(128 + 16 * r, 16), :] = ((e - o) * rstd).astype(BF16)
            t1, t2 = (d[1] - d[3]) * RSQ2, (d[1] + d[3]) * RSQ2
            u = {1: (d[0] + t1, d[2] + t2), 2: (s[0] - s[2], s[1] - s[3]), 3: (d[0] - t1, d[2] - t2)}
            yield _Step(34, [anchor(ubu)], delay=1)
            for k in (1, 2, 3):
                c, sn = twid[z + 2 * k - 2, rows, :] * rstd, twid[z + 2 * k - 1, rows, :] * rstd
                re, m = u[k]
                if k == 3:
                    ur, ui = re * c + m * sn, m * c - re * sn
                else:
                    ur, ui = re * c - m * sn, m * c + re * sn
                UB[0, pl.ds(256 * k + 16 * r, 16), :] = ur.astype(BF16)
                UB[0, pl.ds(256 * k + 128 + 16 * r, 16), :] = ui.astype(BF16)
                yield _Step(26, [anchor(ubu)], delay=1)
        yield settle(ubu)

        def d_forward(point):
            z = opaque()
            first = _iota(8, 0) == 0

            def stage(c):
                u = (M_C4 if c == 1 else M_R) + opaque()
                lhs = mat(u) if c % 4 else _bf(tied(lambda r: mats[u, pl.ds(r, 8), :], 8, point))
                v = _dot(lhs, _bf(ubu[z, pl.ds(64 * c, 64), :]))
                return [(v[32 * u:32 * u + 16], v[32 * u + 16:32 * u + 32]) for u in range(4)]

            def put(row, u, v, v0=None):
                if u == 0 and v0 is not None:
                    v = jnp.concatenate([jnp.where(first, v0, v[:8]), v[8:]], 0)
                AB[0, pl.ds(row + 16 * u, 16), :] = v.astype(BF16)

            for u, (p1, p2) in enumerate(stage(0)):
                put(0, u, p1)
                put(528, u, p2, 0.0)
                if u == 0:
                    put(512, 0, jnp.zeros_like(p2), p2[:8])
            for u, (p1, p2) in enumerate(stage(1)):
                put(256, u, p1)
                put(528 + 256, u, p2)
            for k in (1, 2, 3):
                for u, ((p1, p2), (q1, q2)) in enumerate(zip(stage(2 * k), stage(2 * k + 1))):
                    if k == 3:
                        pr, pi, mr, mi = p1 - q2, p2 + q1, p1 + q2, p2 - q1
                        pi0, mi0 = q1[:8], -q2[:8]
                    else:
                        pr, pi, mr, mi = p1 + q2, p2 - q1, p1 - q2, p2 + q1
                        pi0, mi0 = -q1[:8], q2[:8]
                    put(64 * k, u, pr, p1[:8])
                    put(64 * (8 - k), u, mr, p2[:8])
                    put(528 + 64 * k, u, pi, pi0)
                    put(528 + 64 * (8 - k), u, mi, mi0)
            return 190

        yield _Mat(d_forward)
        yield settle(abu)
        yield _Wait(*free)

        def s_forward(point):
            z = opaque()
            fa, fb = mat(M_FA + j + z), mat(M_FB + j + z)
            for r0, rn in ((0, 256), (256, 272)):
                lhs = abu[z, pl.ds(r0 // 2, rn // 2), :] if r0 else tied(
                    lambda r: abu[z, pl.ds(r, 8), :], 16, point)
                u = _dot(_bf(lhs), fa)
                v = _dot(_bf(abu[z, pl.ds(264 + r0 // 2, 128), :]), fb)
                re, m = u[:256] + v, u[:256] - v
                if r0:
                    re, m = (jnp.concatenate([a, u[256:264]], 0) for a in (re, m))
                rn = re.shape[0]
                edge = (_iota(rn, 1) & 63) == 0
                ZT[2 * i, pl.ds(r0, rn), :] = re
                ZT[2 * i + 1, pl.ds(r0, rn), :] = jnp.where(
                    edge, lane_vec(L_MU + j, rn) * m + lane_vec(L_NU + j, rn) * re, pltpu.roll(m, 64, 1))
            return 400

        yield _Mat(s_forward)
        yield _Step(2, [anchor(ZT)], delay=SETTLE, marks=[name])

    def group_stage(g, name, needs, inverse):
        yield _Wait(*needs)

        def turn(z, k):
            if k == 0:
                return z
            c, s = rot[4 * g + k], rot[16 + 4 * g + k]
            if inverse:
                return z[0] * c - z[1] * s, z[1] * c + z[0] * s
            return z[0] * c + z[1] * s, z[1] * c - z[0] * s

        (src, a), (dst, b) = ((Z, 8 * g), (ZT, 0)) if inverse else ((ZT, opaque()), (Z, 8 * g))
        for r in range(65):
            if r % (16 if inverse else 64) == 0:
                yield hold(src, 2 * NB if inverse else 8)
            rows = pl.ds(8 * r, 8)
            z = [(src[a + 2 * i, rows, :], src[a + 2 * i + 1, rows, :]) for i in range(4)]
            if inverse:
                z = _radix4([turn(z[k], k) for k in range(4)], True)
            else:
                z = [turn(v, k) for k, v in enumerate(_radix4(z, False))]
            for i in range(4):
                dst[b + 2 * i, rows, :], dst[b + 2 * i + 1, rows, :] = z[i]
            yield _Step(35, [anchor(dst)], delay=1, marks=[name] if r == 64 else [])

    def spectral(row, size):
        rows = pl.ds(row, size)
        for k0 in range(4):
            z = _radix4([(Z[8 * g + 2 * k0, rows, :], Z[8 * g + 2 * k0 + 1, rows, :])
                         for g in range(4)], False)
            y = []
            for k1, (re, im) in enumerate(z):
                w = WS[k0 + 4 * k1, rows, :]
                wr = pltpu.bitcast(w << 16, F32)
                wi = pltpu.bitcast(w & np.uint32(0xFFFF0000), F32)
                y.append((re * wr - im * wi, re * wi + im * wr))
            y = _radix4(y, True)
            for g in range(4):
                Z[8 * g + 2 * k0, rows, :], Z[8 * g + 2 * k0 + 1, rows, :] = y[g]

    def spectral_rows(c2):
        for r in range(8):
            spectral(pl.multiple_of(128 * c2 + 16 * r, 16), 16)

    def inv_block(g, i, name, needs, n=None):
        j, t = g + 4 * i, i % 2
        UB, AB, PB, ubu, abu = temps[t]
        n = g if n is None else n
        z = opaque()
        yield _Wait(*needs)
        for r0, rn in _S_ROWS:
            if r0 == 0:
                yield hold(ZT, 8)
            re, im = ZT[z + 2 * i, pl.ds(r0, rn), :], ZT[z + 2 * i + 1, pl.ds(r0, rn), :]
            edge = (_iota(rn, 1) & 63) == 0
            rolled = pltpu.roll(im, 64, 1)
            u = re + jnp.where(edge, lane_vec(L_KU + j, rn) * im, rolled)
            if r0 < 512:
                v = re - jnp.where(edge, lane_vec(L_KV + j, rn) * im, rolled)
                AB[0, pl.ds(r0, rn), :] = u.astype(BF16)
                AB[0, pl.ds(528 + r0, rn), :] = v.astype(BF16)
            else:
                AB[0, pl.ds(512, 16), :] = jnp.concatenate([u, jnp.zeros_like(u)], 0).astype(BF16)
            yield _Step(rn, [anchor(abu)], delay=1, marks=[("read", name)] if r0 == 512 else [])
        yield settle(abu, 4)

        def s_inverse(point):
            z = opaque()
            fa, fb = mat(M_FA + j + z), mat(M_FB + j + z)
            first = _iota(8, 0) == 0

            def put(row, v, v0=None):
                if v0 is not None:
                    v = jnp.concatenate([jnp.where(first, v0, v[:8]), v[8:]], 0)
                UB[0, pl.ds(row, 64), :] = v.astype(BF16)

            for k in range(4):
                lo, hi = 32 * k, 32 * (8 - k if k else 4)
                a = [abu[z, pl.ds(lo, 32), :], abu[z, pl.ds(hi, 32), :]] if k % 2 else [
                    tied(lambda r, o=o: abu[z, pl.ds(o + r, 8), :], 4, point) for o in (lo, hi)]
                if k == 0:
                    a.append(abu[z, pl.ds(256, 8), :])
                re = _dot_t(_bf(jnp.concatenate(a, 0)), fa)
                im = _dot_t(_bf(jnp.concatenate(
                    [abu[z, pl.ds(264 + lo, 32), :], abu[z, pl.ds(264 + hi, 32), :]], 0)), fb)
                pr, mr, pi, mi = re[:64], re[64:128], im[:64], im[64:]
                if k == 0:
                    put(0, pr)
                    put(64, pi, re[128:136])
                    put(128, mr)
                    put(192, mi)
                else:
                    put(256 * k, pr + mr, pr[:8])
                    put(256 * k + 64, pi + mi, mr[:8])
                    put(256 * k + 128, pi - mi, pi[:8])
                    put(256 * k + 192, mr - pr, -mi[:8])
            return 190

        yield _Mat(s_inverse)
        yield settle(ubu, 4)
        yield d_stage(t, lambda c: {0: M_R0T, 1: M_C4T}.get(c, M_RT))
        yield settle(PB, 4)
        z = opaque()
        acc = None
        for r in range(16):
            rows = pl.ds(8 * r, 8)
            t0, t4 = PB[z, rows, :], PB[z, pl.ds(128 + 8 * r, 8), :]
            tk = {}
            for k in (1, 2, 3):
                c, sn = twid[z + 2 * k - 2, rows, :], twid[z + 2 * k - 1, rows, :]
                re = PB[z, pl.ds(256 * k + 8 * r, 8), :]
                im = PB[z, pl.ds(256 * k + 128 + 8 * r, 8), :]
                tk[k] = (re * c - im * sn, re * sn + im * c)
            e0, e1 = t0 + t4, t0 - t4
            s = [e0 + tk[2][0], e1 - tk[2][1], e0 - tk[2][0], e1 + tk[2][1]]
            al, be = tk[1][0] - tk[3][0], tk[1][1] + tk[3][1]
            o = [tk[1][0] + tk[3][0], (al - be) * RSQ2, tk[3][1] - tk[1][1], (al + be) * -RSQ2]
            for b in range(8):
                y = s[b] + o[b] if b < 4 else s[b - 4] - o[b - 4]
                v = X[i][g, pl.ds(128 * b + 8 * r, 8), :] + y
                X[i][n, pl.ds(128 * b + 8 * r, 8), :] = v
                acc = v if acc is None else acc + v
            yield _Step(57, [lambda v=acc: v], delay=5 if r == 15 else 2)
        yield settle(X[i], 4)
        mean = _all_sublanes(acc, jnp.add, 0) * (1.0 / D)
        rstd = yield from ln_rstd(n, i, mean)
        z = opaque()
        for r in range(8):
            v = X[i][n + z, pl.ds(128 * r, 128), :].reshape(16, 8, 128)
            HB[i][n, pl.ds(128 * r, 128), :] = ((v - mean[None]) * rstd[None]).reshape(128, 128).astype(BF16)
            yield _Step(41, [anchor(hbu[i])], delay=1, marks=[name] if r == 7 else [])

    def attend(g, i, name, needs):
        yield _Wait(*needs)
        yield settle(QB[i])
        j, z = g + 4 * i, opaque()
        even = (_iota(8, 0) & 1) == 0
        edge = _iota(8, 1) == 0

        def window(near, far, w, rows):
            return near[j + z + 4 - 2 * w, rows, :] if w <= 2 * i + 2 else far[j + z + 16 - 2 * w, rows, :]

        def mix_values(h, u):
            p = PW[h % 2][opaque()]
            for rows in (pl.ds(256 * h + 16 * u, 16), pl.ds(256 * h + 16 * u + 16, 16)):
                acc = functools.reduce(jnp.add, [p[16 * w:16 * w + 16] * window(VE, VS, w, rows)
                                                 for w in range(8)])
                HB[i][g, rows, :] = acc.astype(BF16)
            return _Step(63, [anchor(hbu[i])], delay=2, marks=[name] if (h, u) == (3, 14) else [])

        for h in range(5):
            logits = []
            for w0 in range(0, 8, 2):
                if h < 4:
                    rows = pl.ds(256 * h, 256)
                    q = q if w0 % 4 else QB[i][opaque(), rows, :]
                    for w in (w0, w0 + 1):
                        v = (q * window(KE, KS, w, rows)).reshape(16, 16, 128).sum(0)
                        v = jnp.where(even, v[:8] + pltpu.roll(v[:8], 7, 0), v[8:] + pltpu.roll(v[8:], 1, 0))
                        logits.append(jnp.where(edge & (2 * w > j), -1e9, v * SCALE) if w > 2 * i
                                      else v * SCALE)
                    yield _Step(138, [lambda v=v: v for v in logits[-2:]], delay=4)
                if h > 0:
                    yield mix_values(h - 1, 2 * w0)
                    yield mix_values(h - 1, 2 * w0 + 2)
            if h < 4:
                top = functools.reduce(jnp.maximum, logits)
                e = [jnp.exp(v - top) for v in logits]
                total = functools.reduce(jnp.add, e)
                yield _Step(30, [lambda v=total: v], delay=3)
                scale = 1.0 / total
                for w in range(8):
                    v = e[w] * scale
                    PW[h % 2][0, pl.ds(16 * w, 8), :] = jnp.where(even, v, pltpu.roll(v, 1, 0))
                    PW[h % 2][0, pl.ds(16 * w + 8, 8), :] = jnp.where(even, pltpu.roll(v, 7, 0), v)
                yield _Step(50, [anchor(PW[h % 2])], delay=6 if h == 3 else 1)

    def packed_sums(terms, signs):
        lo = [pltpu.bitcast(u << 16, F32) for u in terms]
        hi = [pltpu.bitcast(u & np.uint32(0xFFFF0000), F32) for u in terms]
        return [pltpu.pack_elementwise([v[p] + v[q] if s > 0 else v[p] - v[q] for v in (lo, hi)],
                                       packed_dtype=BF16) for p, s, q in signs]

    def half(ref, row):
        return lambda r, size, cols: ref[pl.ds(pl.multiple_of(row + r, 8), size), cols]

    kv_weight = (WS5, half(WK, 0), half(WV, 0))
    q_weight = (WQ5, half(WQ, 0), half(WQ, D // 4))
    o_weight = (WP5, *(lambda r, size, cols, e=e: WP[pl.ds(r + r // 32 * 32 + e, size), cols]
                       for e in (0, 32)))

    def left_sums(weight, row, size, needs=()):
        yield _Wait(*needs)
        sums, top, bottom = weight
        for r in range(0, size, 8):
            a = [ref(row + r, 8, pl.ds(c, 512)) for ref in (top, bottom) for c in (0, 512)]
            for e, v in enumerate(packed_sums(a, ((0, 1, 3), (2, 1, 3), (0, 1, 1), (2, -1, 0), (1, -1, 3)))):
                sums[e, pl.ds(pl.multiple_of(row + r, 8), 8), :] = v
            yield _Step(92, [anchor(sums)], delay=2, marks=["sums"] if r == size - 8 else [])

    def right_sums(dst, g, i, name, needs):
        yield _Wait(*needs)
        z = g + opaque()
        for r in range(0, 256, 16):
            b = [hbu[n][z, pl.ds(k + r, 16), :] for k in (0, 256) for n in (i, i + 1)]
            for e, v in enumerate(packed_sums(b, ((0, 1, 3), (1, -1, 3), (2, -1, 0), (0, 1, 1), (2, 1, 3)))):
                dst[e, pl.ds(r, 16), :] = v
            yield _Step(47, [anchor(dst)], delay=SETTLE if r == 240 else 1,
                        marks=[name] if r == 240 else [])

    def strassen(sch, weight, right, g, i, m, store, needs, marks):
        for n in needs:
            sch.run(n)
        sums, top, bottom = weight
        rows = pl.ds(pl.multiple_of(64 * m, 64), 64)

        def product(left, b):
            sch.fresh = True
            head = tied(lambda r: left(32 * m + r, 8, pl.ds(0, 128)), 4, lambda: sch.point(8.0))
            return _dot(_bf(jnp.concatenate([head, left(32 * m, 32, pl.ds(128, 384))], 1)), _bf(b))

        def a(e):
            return lambda r, size, cols: sums[e, pl.ds(pl.multiple_of(r, 8), size), cols]

        def b(e):
            return right[e + opaque()]

        m2 = product(a(1), hbu[i][g + opaque(), pl.ds(0, 256), :])
        m4 = product(lambda r, size, cols: bottom(r, size, pl.ds(512 + cols.start, cols.size)), b(2))
        store(1, i, rows, m2 + m4)
        m1 = product(a(0), b(0))
        c11, c22 = m1 + m4, m1 - m2
        c11 = c11 + product(a(4), b(4))
        c22 = c22 + product(a(3), b(3))
        m5 = product(a(2), hbu[i + 1][g + opaque(), pl.ds(256, 256), :])
        store(0, i, rows, c11 - m5)
        v = product(top, b(1))
        store(0, i + 1, rows, v + m5)
        store(1, i + 1, rows, c22 + v)
        sch.results.append(v[:8])
        for name in marks:
            sch.done[name] = sch.slot + sch.wait

    def kv_proj(sch, g, i, name, needs):
        def store(lower, n, rows, v):
            (KE, VE)[lower][g + 4 * n + 4, rows, :] = v
        for m in range(16):
            strassen(sch, kv_weight, SB[i // 2], g, i, m, store, needs, [name] if m == 15 else [])

    def q_proj(sch, g, i, name, needs):
        def store(lower, n, rows, v):
            QB[n][0, pl.ds(512 * lower + rows.start, 64), :] = v
        for m in range(8):
            strassen(sch, q_weight, SB[i // 2], g, i, m, store, needs, [name] if m == 7 else [])

    def o_proj(sch, g, i, m, needs, marks, right):
        def store(lower, n, rows, v):
            rows = pl.ds(128 * m + 64 * lower, 64)
            X[n][g, rows, :] = X[n][g, rows, :] + v
        strassen(sch, o_weight, right, g, i, m, store, needs, marks)

    def shift_block(g, i, name, needs):
        yield _Wait(*needs)
        j, z = g + 4 * i, opaque()
        for m in range(16):
            rows = pl.ds(64 * m, 64)
            for ref, to in ((KE, KS), (VE, VS)):
                v = pltpu.roll(ref[j + 4 + z, rows, :], 1, 1)
                if ref is VE:
                    v = jnp.where(_iota(64, 1) == 0, ref[4 + z, rows, :], v)
                to[j, rows, :] = v
                if i == 3:
                    ref[g, rows, :] = v
            yield _Step(12, delay=8, marks=[name] if m == 15 else [])

    def transpose_quarter(w, h, via):
        for r in range(4):
            v = WRAW[w, pl.ds(256 * r, 256), pl.ds(pl.multiple_of(256 * h, 256), 256)]
            v = pltpu.bitcast(v.T, F32)
            via[0, pl.ds(256 * r, 128), :], via[0, pl.ds(256 * r + 128, 128), :] = v[:, :128], v[:, 128:]
            yield _Step(40, delay=16)

    def reorder_quarter(w, h, via, name=None):
        z = 0 if isinstance(h, int) else opaque()
        for c in range(8):
            WT[w][pl.ds(pl.multiple_of(128 * h, 128), 128), pl.ds(128 * c, 128)] = pltpu.bitcast(
                jnp.concatenate([via[z, pl.ds(128 * c + u, 8, stride=16), :] for u in range(16)], 0), U32)
            yield _Step(20, delay=4, marks=[name] if c == 7 else [])

    def query_weight(h):
        yield from transpose_quarter(0, h, QB[0])
        yield from reorder_quarter(0, h, QB[0], "w")

    def transpose_wo(name):
        for c in range(8):
            for h in range(4):
                v = jnp.concatenate([wou[c, pl.ds(128 * h + u, 8, stride=16), :] for u in range(16)], 0)
                WP[pl.ds(64 * c, 64), pl.ds(256 * h, 256)] = pltpu.bitcast(_bf(v).T, U32)
                yield _Step(20, delay=10, marks=[name] if c == 7 and h == 3 else [])

    def prep_spectral_weights(c2):
        lane = _iota(8, 1)
        order = jnp.where(lane > 64, 192 - lane, lane)

        def words(k2):
            re, im = (wsu[u, k2, pl.ds(c2, 64, stride=4), :] for u in range(2))
            return ((re & np.uint32(0xFFFF)) | (im << 16), (re >> 16) | (im & np.uint32(0xFFFF0000)))

        def arrange(w, below):
            w = jnp.where(_iota(w.shape[0], 1) < 64, w, below)
            return jnp.concatenate([jnp.take_along_axis(w[u:u + 8], order, axis=1)
                                    for u in range(0, w.shape[0], 8)], 0)

        below = words(15)
        for k2 in range(16):
            here = words(k2)
            for e in range(2):
                cl = 2 * c2 + e
                w = arrange(here[e], below[e])
                WS[k2, pl.ds(64 * cl, 64), :] = pltpu.roll(w, 1, 0) if cl > 4 else w
            below = here
            yield _Step(100)
        if c2 == 0:
            def nyquist(k2):
                re, im = (jnp.broadcast_to(WN[u, :, pl.ds(128 * k2, 128)].astype(F32), (8, 128))
                          for u in range(2))
                return pltpu.pack_elementwise([re, im], packed_dtype=BF16)
            for k2 in range(16):
                WS[k2, pl.ds(512, 8), :] = arrange(nyquist(k2), nyquist((k2 + 15) % 16))

    def write_out(p, c, name, needs):
        yield _Wait(*needs)
        rows = pl.ds(pl.multiple_of(128 * c, 128), 128)
        g, i = 2 * p % 4 + opaque(), p // 2
        w = pltpu.pack_elementwise([X[i][g, rows, :], X[i][g + 1, rows, :]], packed_dtype=BF16)
        xru[c, pl.ds(p, 128, stride=8), :] = w.T
        yield _Step(30, marks=[name])

    for c in range(8):
        x_copy(c).start()
    for c in range(5):
        mats[M_R + c] = d_mats[c]

    def make_twiddle(k):
        PB = temps[0][2]
        PB[0, pl.ds(0, 128), :] = lane_vec(L_TWID + k, 128)
        twid[k] = PB[opaque(), pl.ds(0, 128), :].T

    _loop(6, make_twiddle, "make_twiddle")

    def make_dft(j):
        fa, fb = lanes[pl.ds(L_FA, 128), :], lanes[pl.ds(L_FB, 128), :]
        c, sn = lane_vec(L_COS + j, 128), lane_vec(L_SIN + j, 128)
        UB, _, _, ubu, _ = temps[0]
        UB[0, pl.ds(0, 128), :] = (fa * c + fb * sn).astype(BF16)
        UB[0, pl.ds(128, 128), :] = (fb * c - fa * sn).astype(BF16)
        mats[M_FA + j], mats[M_FB + j] = ubu[0, pl.ds(0, 64), :], ubu[0, pl.ds(64, 64), :]

    _loop(NB, make_dft, "make_dft")

    def load_x(c):
        x_copy(c).wait()
        pl.when(c == 6)(lambda: start_all(spec_copies[0]))
        pl.when(c == 7)(lambda: start_all(spec_copies[1]))
        rows = pl.ds(pl.multiple_of(128 * c, 128), 128)
        for p in range(8):
            w = xru[c, pl.ds(p, 128, stride=8), :].T
            for e, bits in enumerate((w << 16, w & np.uint32(0xFFFF0000))):
                g, i = 2 * p % 4 + e, p // 2
                v = pltpu.bitcast(bits, F32)
                X[i][g, rows, :] = v
                v = v.reshape(16, 8, 128)
                mean = _all_sublanes(v.sum(0), jnp.add, 0) * (1.0 / 128)
                STAT[4 * g + i, c] = mean
                STAT[4 * g + i, 8 + c] = _all_sublanes(((v - mean) ** 2).sum(0), jnp.add, 0)

    _loop(8, load_x, "load_x")

    def after(name, action):
        yield _Wait(name)
        action()

    def spectral_weights():
        yield _Wait(("f", 2, 1))
        for c in spec_copies[0] + spec_copies[1]:
            c.wait()
        for c2 in range(4):
            yield from prep_spectral_weights(c2)

    with jax.named_scope("first_forward"):
        sch = _Sched(0.72, 20)
        sch.add(after(("f", 0, 1), w_copies[1].start), "k")
        sch.add(after(("f", 1, 1), w_copies[2].start), "v")
        sch.add(after(("f", 2, 3), w_copies[0].start), "q")
        for g in range(4):
            for i in range(4):
                sch.add(fwd_block(g, i, ("f", g, i), [("f", g - 1, i)] if g else [],
                                  [("r", g - 1)] if g else [], True), ("f", g, i))
            sch.add(group_stage(g, ("r", g), [("f", g, i) for i in range(4)], False), ("r", g))
        sch.add(spectral_weights(), "s")
        sch.drive()
    start_all(wo_copies)

    def keys_values(layer, g):
        sch = _Sched(0.41, 32, 3) if layer == 0 else _Sched(0.36, 28, 2)
        nxt = (g + 1) % 4
        sch.add(inv_block(g, 2, ("i", 2), []), ("i", 2))
        sch.add(inv_block(g, 3, ("i", 3), [("read", ("i", 2))]), ("i", 3))
        sch.add(right_sums(SB[1], g, 2, ("b", 2), [("i", 2), ("i", 3)]), ("b", 2))
        sch.add(group_stage(nxt, "r", [("read", ("i", 3))], True), "r")
        sch.add(inv_block(nxt, 0, ("i", 4), ["r", ("i", 2)], n=g + 1), ("i", 4))
        sch.add(inv_block(nxt, 1, ("i", 5), [("read", ("i", 4)), ("i", 3)], n=g + 1), ("i", 5))
        if layer == 0:
            sch.add(query_weight(g), "w")
            sch.add(left_sums(q_weight, 128 * (g % 2), 128, ["w"]), "sums")
        for i in (2, 3):
            sch.add(shift_block((g + 3) % 4, i, ("s", i), []), ("s", i))
        for i in (0, 1):
            sch.add(shift_block(g, i, ("s", i), [("kv", 0)]), ("s", i))
        sch.add(right_sums(SB[0], nxt, 0, ("b", 4), [("i", 4), ("i", 5), ("kv", 0)]), ("b", 4))
        kv_proj(sch, g, 0, ("kv", 0), [])
        kv_proj(sch, g, 2, ("kv", 2), [("b", 2)])
        sch.finish()

    def mix(g, after, last):
        tail = after is None
        sch = _Sched(0.66 if last else 0.63, 28 if last else 32)
        pace = 0.48 if tail else 0.35 if last else 0.32
        ahead = [(g, 2), (g, 3)] + ([] if tail else [(after, 0), (after, 1)])
        for n, block in enumerate(ahead):
            sch.add(attend(*block, ("a", n), [[], [("a", 0)], [("a", 1), ("q", 0)], [("a", 2)]][n]),
                    ("a", n), pace=pace)
            if n % 2:
                sch.add(right_sums(SB[2 + block[1] // 2], block[0], block[1] - 1, ("b", n),
                                   [("a", n)] + ([("o", 0)] if n == 3 else [])), ("b", n))
        for i in () if tail else (0, 2):
            sch.add(right_sums(SB[i // 2], after, i, ("h", i), [("q", 0)] if i else []), ("h", i))
        if not last:
            sch.add(group_stage((g + 3) % 4, "r", [], False), "r")
            for i in range(4):
                sch.add(fwd_block(g, i, ("f", i), [("o", i - i % 2)], ["r"]), ("f", i))
        now = 6 if last else 8
        for i in (0, 2):
            for m in range(now):
                o_proj(sch, g, i, m, [("b", 1)] if i else [], [("o", i)] if m == now - 1 else [],
                       SB[2 + i // 2])
            if not tail:
                q_proj(sch, after, i, ("q", i), [("h", i)])
        if tail:
            sch.add(group_stage(g, "s", [("f", i) for i in range(4)], False), "s")
        sch.share = 0.92
        sch.drive()

    def mix_odd():
        sch = _Sched(0.66)
        blocks = [(1, 2), (1, 3), (3, 0), (3, 1), (3, 2), (3, 3)]
        for n, (g, i) in enumerate(blocks):
            sch.add(attend(g, i, ("a", n), ([("a", n - 1)] if n else []) + ([("q", i)] if n in (2, 4) else [])),
                    ("a", n), pace=0.32)
            if n % 2:
                sch.add(right_sums(SB[(3, 2, 0)[n // 2]], g, i - 1, ("b", g, i - 1),
                                   [("a", n)] + ([("o", 1, 0, 5)] if n > 1 else [])), ("b", g, i - 1))
        for i in (0, 2):
            sch.add(right_sums(SB[i // 2], 3, i, ("h", i), []), ("h", i))
        for g in (1, 3):
            for i in range(4):
                for c in range(6):
                    sch.add(write_out(2 * i + g // 2, c, ("w", g, i, c), [("o", g, i - i % 2, c)]),
                            ("w", g, i, c))
        for g, i, slot, count in ((1, 0, 2, 6), (1, 2, 3, 8), (3, 0, 2, 8), (3, 2, 0, 6)):
            for m in range(count):
                o_proj(sch, g, i, m, [("b", g, i)] if (g, i) != (1, 0) else [], [("o", g, i, m)], SB[slot])
            for e in (0, 2) if (g, i) == (1, 0) else ():
                q_proj(sch, 3, e, ("q", e), [("h", e)] + ([("a", 1)] if e else []))
        sch.share = 0.92
        sch.drive()

    def copy_out(chunks):
        def start(_):
            for c in chunks:
                out_copy(c).start()
        _loop(zero + 1, start, "copy_out")

    def postponed():
        slots = {(3, 2): 0, (2, 2): 1, (0, 2): 2, (2, 0): 3, (0, 0): 0, (1, 0): 1}
        early, late = list(slots)[:2], list(slots)[2:]
        sources = 2 * [[(0, 0), (1, 0)], [(2, 0)]] + 2 * [[(0, 2)], []]
        for c in (6, 7):
            sch = _Sched(0.7, 12)
            for n, (pair, slot) in enumerate(slots.items()) if c == 6 else ():
                if n:
                    sch.add(right_sums(SB[slot], *pair, pair, [(early[n - 4], 7)] if n >= 4 else []), pair)
            for p in (5, 7, 4, 6, 1, 3, 0, 2):
                sch.add(write_out(p, c, ("w", p), [(pair, c) for pair in sources[p] or early * (c == 6)]),
                        ("w", p))
            for pair, m in [(pair, m) for m in (6, 7) for pair in early] * (c == 6) + [(v, c) for v in late]:
                o_proj(sch, *pair, m, [pair] if c == 6 and pair != (3, 2) else [], [(pair, m)],
                       SB[slots[pair]])
            sch.drive()
            copy_out([c])

    def first_queries(layer):
        sch = _Sched(0.68)
        sch.add(right_sums(SB[1], 0, 2, ("h", 2), []), ("h", 2))
        sch.add(shift_block(3, 2, "s", []), "s")
        sch.add(attend(0, 0, ("a", 0), ["q"]), ("a", 0), pace=0.4)
        sch.add(attend(0, 1, ("a", 1), [("a", 0)]), ("a", 1), pace=0.4)
        sch.add(right_sums(SB[2], 0, 0, "b", [("a", 1)]), "b")
        sch.add(shift_block(3, 3, "t", []), "t")
        if layer == 0:
            for c in wo_copies:
                c.wait()
            sch.add(transpose_wo("w"), "w")
            sch.add(left_sums(o_weight, 0, 256, ["w"]), "sums")
        q_proj(sch, 0, 0, "q", [])
        q_proj(sch, 0, 2, None, [("h", 2)])
        sch.finish()

    def key_value_weights():
        w_copies[1].wait()
        w_copies[2].wait()
        for h in range(6):
            work = []
            for w in (1, 2):
                if h < 4:
                    work.append(transpose_quarter(w, h, QB[2 * (h % 2) + w - 1]))
                if 0 < h < 5:
                    work.append(reorder_quarter(w, h - 1, QB[2 * ((h - 1) % 2) + w - 1]))
            if h > 1:
                work.append(left_sums(kv_weight, 128 * (h - 2), 128))
            list(itertools.zip_longest(*work))

    for layer in range(2):
        with jax.named_scope("spectral"):
            _loop(4, spectral_rows, "rows")
            if layer == 0:
                _loop(zero + 1, lambda _: key_value_weights(), "weights")
            spectral(512, 8)
        sch = _Sched(0.92)
        sch.add(group_stage(0, "r", [], True), "r")
        sch.add(inv_block(0, 0, ("i", 0), ["r"]), ("i", 0))
        sch.add(inv_block(0, 1, ("i", 1), ["r"]), ("i", 1))
        sch.add(right_sums(SB[0], 0, 0, "b", [("i", 0), ("i", 1)]), "b")
        sch.drive()
        if layer == 0:
            w_copies[0].wait()
        _loop(4, lambda g: keys_values(layer, g), "keys_values")
        first_queries(layer)
        if layer == 0:
            pl.when(never)(lambda: spectral_rows(0))
        if layer == 0:
            _loop(3, lambda g: mix(g, g + 1, False), "mix")
            mix(3, None, False)
        else:
            _loop(2, lambda u: mix(2 * u, 2 - u, True), "mix")
            mix_odd()
    copy_out(range(6))
    postponed()
    for c in range(8):
        out_copy(c).wait()


@jax.jit
def pallas_interleave_layers__spectral_gfnet__sliding_local_dilated__prompt_kernel(
    A_x: jax.Array,
    A_w_r: jax.Array,
    A_w_i: jax.Array,
    B_x: jax.Array,
    B_wqkv: jax.Array,
    B_wo: jax.Array,
):
    del B_x
    hbm = pl.BlockSpec(memory_space=pl.ANY)
    smem = pl.BlockSpec(memory_space=pltpu.SMEM)
    out = pl.pallas_call(
        _kernel,
        out_shape=jax.ShapeDtypeStruct((S, D), BF16),
        in_specs=[smem, smem, pl.BlockSpec(), pl.BlockSpec(), hbm, hbm, hbm, hbm, hbm],
        out_specs=hbm,
        scratch_shapes=[
            pltpu.VMEM((37, 64, 128), U32),
            pltpu.VMEM((6, 128, 128), F32),
            pltpu.VMEM((NB, 16, 8, 128), F32),
            pltpu.VMEM((NB + 4, D, 128), F32),
            pltpu.VMEM((NB + 4, D, 128), F32),
            pltpu.VMEM((NB, D, 128), F32),
            pltpu.VMEM((NB, D, 128), F32),
            pltpu.VMEM((2 * NB + 1, ZR, 128), F32),
            pltpu.VMEM((9, ZR, 128), F32),
            pltpu.VMEM((NB, ZR, 128), U32),
            *4 * [pltpu.VMEM((D // 2, D), U32)],
            pltpu.VMEM((5, D // 2, D // 2), U32),
            *2 * [pltpu.VMEM((5, D // 4, D // 2), U32)],
            *4 * [pltpu.VMEM((5, D // 4, 128), U32)],
            pltpu.VMEM((8, S, 128), BF16),
            pltpu.VMEM((2, NB, D // 2, 128), BF16),
            pltpu.VMEM((2, 1, S), BF16),
            pltpu.VMEM((3, D, D), BF16),
            pltpu.VMEM((8, D, 128), BF16),
            pltpu.VMEM((1, 128, 128), F32),
            pltpu.VMEM((1, 128, 128), F32),
            pltpu.SemaphoreType.DMA((24,)),
            *2 * [pltpu.VMEM((1, D, 128), F32)],
        ] + 4 * [
            pltpu.VMEM((5, D, 128), F32),
            pltpu.VMEM((5, D, 128), BF16),
            pltpu.VMEM((1, D, 128), F32),
            pltpu.VMEM((1, D, 128), BF16),
            pltpu.VMEM((1, 1152, 128), BF16),
        ],
        compiler_params=pltpu.CompilerParams(vmem_limit_bytes=126 * 2 ** 20),
    )(_ZERO, _ROT, _MATS, _LANES, A_x.reshape(S, D), A_w_r.T, A_w_i.T, B_wqkv, B_wo)
    return out.reshape(1, S, D)
```

```python
import functools
import itertools

import numpy as np

import jax
import jax.numpy as jnp
import jax.experimental.pallas as pl
import jax.experimental.pallas.tpu as pltpu

S, D, NB = 2048, 1024, 16
ZR = 576
F32, BF16, U32, I32 = jnp.float32, jnp.bfloat16, jnp.uint32, jnp.int32
EPS = 1e-5
SCALE = 32 ** -0.5
RSQ2 = float(np.sqrt(0.5))
SETTLE = 6

_S_ROWS = [(32 * u, 32) for u in range(16)] + [(512, 8)]

M_FA, M_FB, M_R, M_C4, M_RT, M_C4T, M_R0T = 0, 16, 32, 33, 34, 35, 36
L_MU, L_NU, L_KU, L_KV, L_COS, L_SIN, L_TWID, L_FA, L_FB = 0, 16, 32, 48, 64, 80, 96, 104, 232


def _bf16_bits(a):
    u = np.ascontiguousarray(a, dtype=np.float32).view(np.uint32).astype(np.uint64)
    return ((u + 0x7FFF + ((u >> 16) & 1)) >> 16).astype(np.uint32)


def _constants():
    a = np.arange(128)
    k1 = np.arange(64)
    alt = (-1.0) ** a
    lanes = np.zeros((L_FB + 128, 128))
    t = 2 * np.pi * np.outer(a, k1) / 128
    fa = np.concatenate([np.cos(t), -np.sin(t)], 1)
    fb = np.concatenate([np.sin(t), -np.cos(t)], 1)
    fa[:, 0], fb[:, 0] = RSQ2, -RSQ2
    fa[:, 64], fb[:, 64] = alt, 0.0
    lanes[L_FA:L_FA + 128], lanes[L_FB:L_FB + 128] = fa, fb
    for j in range(NB):
        ang = 2 * np.pi * j / 32 + np.pi / 32
        p, q = (_bf16_bits([np.cos(ang), np.sin(ang)]) << 16).view(np.float32).astype(np.float64)
        turn = 2 * np.pi * j * np.tile(k1, 2) / S
        lanes[L_COS + j], lanes[L_SIN + j] = np.cos(turn), np.repeat([-1.0, 1.0], 64) * np.sin(turn)
        lanes[L_COS + j, 64], lanes[L_SIN + j, 64] = p, q
        lanes[L_MU + j, 0], lanes[L_MU + j, 64] = 1.0, (q / p + p / q) / 2
        lanes[L_NU + j, 0], lanes[L_NU + j, 64] = 0.0, (q / p - p / q) / 2
        lanes[L_KU + j, 0], lanes[L_KU + j, 64] = 1.0, q / p
        lanes[L_KV + j, 0], lanes[L_KV + j, 64] = 1.0, p / q
    for k in (1, 2, 3):
        lanes[L_TWID + 2 * k - 2] = np.cos(2 * np.pi * a * k / D)
        lanes[L_TWID + 2 * k - 1] = np.sin(2 * np.pi * a * k / D)
    th = 2 * np.pi * np.outer(k1, a) / 128
    r = np.concatenate([np.cos(th), -np.sin(th)], 0)
    r[64] = alt
    th = 2 * np.pi * np.outer(2 * k1 + 1, a) / 256
    c4 = np.concatenate([np.cos(th), -np.sin(th)], 0)
    inv = 2.0 / (S * D)
    r0t = inv * r.T
    r0t[:, 0::64] *= 0.5
    rows = np.arange(128).reshape(2, 4, 16).transpose(1, 0, 2).ravel()
    bits = _bf16_bits(np.stack([r[rows], c4[rows], inv * r.T, inv * c4.T, r0t]))
    ang = 2 * np.pi * np.outer(np.arange(4), np.arange(4)).ravel() / 16
    rot = np.concatenate([np.cos(ang), np.sin(ang)]).astype(np.float32)
    return bits[:, 0::2] | (bits[:, 1::2] << 16), lanes.astype(np.float32), rot


_MATS, _LANES, _ROT = _constants()
_ZERO = np.zeros((1,), np.int32)


class _Step:
    def __init__(self, cost, anchors=(), delay=0, marks=()):
        self.cost, self.anchors, self.delay, self.marks = cost, list(anchors), delay, list(marks)


class _Wait:
    def __init__(self, *names):
        self.names = names


class _Mat:
    def __init__(self, emit):
        self.emit = emit


class _Hold:
    def __init__(self, store):
        self.store = store


class _Task:
    def __init__(self, gen, pace):
        self.gen, self.pace, self.blocked, self.not_before, self.held = gen, pace, (), 0, None
        self.allowed = 0.0


class _Sched:
    def __init__(self, share=0.0, wait=28, lag=3):
        self.lag = lag
        self.wait = wait
        self.share = share
        self.tasks, self.done, self.producer = [], {}, {}
        self.slot, self.credit, self.anchors, self.results = 0, 0.0, [], []
        self.fresh = False

    def add(self, gen, name, pace=99):
        self.producer[name] = self.producer["read", name] = _Task(gen, pace)
        self.tasks.append(self.producer[name])

    def _ready(self, t):
        return t.not_before <= self.slot and all(
            n in self.done and self.done[n] <= self.slot for n in t.blocked)

    def _advance(self, t, mats=True):
        item, t.held = t.held or next(t.gen, None), None
        if item is None:
            self.tasks.remove(t)
        elif isinstance(item, _Wait):
            t.blocked = item.names
        elif isinstance(item, _Hold):
            if len(self.results) >= self.lag:
                item.store(self.results[-self.lag])
        elif isinstance(item, _Mat):
            if mats:
                t.not_before = float("inf")
                self.fresh = False
                self.credit -= item.emit(lambda: self.point(0.0)) or 0
                t.not_before = self.slot + self.wait
            else:
                t.held, t.not_before = item, self.slot + 1
        else:
            t.blocked = ()
            t.not_before = self.slot + item.delay
            self.credit -= item.cost
            self.anchors += item.anchors
            for n in item.marks:
                self.done[n] = self.slot + item.delay
            return True

    def run(self, *names):
        while not all(n in self.done for n in names):
            for n in names:
                if n not in self.done:
                    for b in self.producer[n].blocked:
                        self.run(b)
                    self._advance(self.producer[n])

    def drive(self):
        while self.tasks:
            ready = [t for t in self.tasks if self._ready(t)]
            if not ready:
                self.slot += 1
                continue
            self.anchors, self.credit = self.anchors[-2:], 0.0
            self._advance(next((t for t in ready if t.held), ready[0]))
            self.slot -= min(self.credit, 0.0) / 60

    def finish(self):
        self.run(*[n for n in self.producer if n[0] != "read"])

    def point(self, own):
        for t in self.tasks:
            t.allowed = min(t.allowed, 0.0) + t.pace
        while True:
            t = next((t for t in self.tasks if self._ready(t) and t.allowed > 0
                      and self.credit > 0), None)
            if t is None:
                break
            if self._advance(t, self.fresh):
                t.allowed -= 1
        anchors, self.anchors = self.anchors, []
        self.credit = min(self.credit, 10.0) + 64 * self.share - own
        self.fresh = False
        self.slot += 1
        return anchors


def _dot(a, b):
    return jnp.dot(a, b, preferred_element_type=F32)


def _dot_t(a, b):
    return jax.lax.dot_general(a, b, (((1,), (1,)), ((), ())), preferred_element_type=F32)


def _bf(u):
    return pltpu.bitcast(u, BF16)


def _iota(rows, dim):
    return jax.lax.broadcasted_iota(I32, (rows, 128), dim)


def _radix4(z, inverse):
    (r0, i0), (r1, i1), (r2, i2), (r3, i3) = z
    ar, ai, cr, ci = r0 + r2, i0 + i2, r0 - r2, i0 - i2
    br, bi, dr, di = r1 + r3, i1 + i3, r1 - r3, i1 - i3
    lo, hi = (cr + di, ci - dr), (cr - di, ci + dr)
    if inverse:
        lo, hi = hi, lo
    return [(ar + br, ai + bi), lo, (ar - br, ai - bi), hi]


def _all_sublanes(v, op, axis):
    for sh in (4, 2, 1):
        v = op(v, pltpu.roll(v, sh, axis))
    return v


def _loop(n, body, name):
    def step(i, carry):
        body(i)
        return carry
    with jax.named_scope(name):
        jax.lax.fori_loop(0, n, step, 0)


def _kernel(zero_ref, rot, d_mats, lanes, x_hbm, wr_hbm, wi_hbm, wqkv_hbm, wo_hbm, out_hbm,
            mats, twid, STAT, KE, VE, KS, VS, Z, ZT, WS, WQ, WK, WV, WP, WS5, WQ5, WP5,
            SB0, SB1, SB2, SB3, XR, WRI, WN, WRAW, WO, PW0, PW1, sems, *split):
    zero = zero_ref[0]
    never = zero != 0
    X, HB, QB = split[2::5], split[3::5], split[4::5]
    hbu = [r.bitcast(U32) for r in HB]
    xru, wsu, wou = XR.bitcast(U32), WRI.bitcast(U32), WO.bitcast(U32)
    temps = [(ub, ab, pb, ub.bitcast(U32), ab.bitcast(U32))
             for ub, ab, pb in zip(split[5::5], split[6::5], 2 * split[:2])]
    PW, SB, WT = (PW0, PW1), (SB0, SB1, SB2, SB3), (WQ, WK, WV, WP)
    counter = [0]

    def opaque():
        counter[0] += 1
        return zero * counter[0]

    def anchor(ref):
        at = (0,) * (len(ref.shape) - 2)
        return lambda: ref[(*at, pl.ds(pl.multiple_of(zero * 8, 8), 8), pl.ds(0, 128))]

    def settle(ref, points=SETTLE):
        return _Step(2, [anchor(ref)], delay=points)

    def hold(ref, spare):
        def store(v):
            ref[spare, pl.ds(pl.multiple_of(zero * 8, 8), 8), :] = v
        return _Hold(store)

    def tied(load, vregs, point):
        parts = []
        for r in range(vregs):
            anchors = point()
            u = load(8 * r)
            for a in anchors:
                u = jnp.where(never, pltpu.bitcast(a(), U32), u)
            parts.append(u)
        return jnp.concatenate(parts, 0)

    def mat(i):
        return _bf(mats[i])

    def d_stage(t, which):
        UB, AB, PB, ubu, abu = temps[t]

        def emit(point):
            z = opaque()
            for c in range(8):
                lhs = mat(which(c) + opaque()) if c % 4 else _bf(
                    tied(lambda r, u=which(c) + opaque(): mats[u, pl.ds(r, 8), :], 8, point))
                PB[0, pl.ds(128 * c, 128), :] = _dot(lhs, _bf(ubu[z, pl.ds(64 * c, 64), :]))
        return _Mat(emit)

    def lane_vec(i, rows):
        return jnp.broadcast_to(lanes[pl.ds(i, 1), :], (rows, 128))

    def x_copy(c):
        return pltpu.make_async_copy(
            x_hbm.at[:, pl.ds(pl.multiple_of(128 * c, 128), 128)], XR.at[c], sems.at[c])

    def out_copy(c):
        return pltpu.make_async_copy(
            XR.at[c], out_hbm.at[:, pl.ds(pl.multiple_of(128 * c, 128), 128)], sems.at[8 + c])

    spec_copies = [[pltpu.make_async_copy(w.at[pl.ds(0, 512), pl.ds(128 * k2, 128)], WRI.at[u, k2],
                                          sems.at[16 + u]) for k2 in range(16)]
                   + [pltpu.make_async_copy(w.at[pl.ds(512, 1), :], WN.at[u], sems.at[22 + u])]
                   for u, w in enumerate((wr_hbm, wi_hbm))]

    def start_all(copies):
        for c in copies:
            c.start()
    w_copies = [pltpu.make_async_copy(wqkv_hbm.at[:, pl.ds(D * w, D)], WRAW.at[w], sems.at[18 + w])
                for w in range(3)]
    wo_copies = [pltpu.make_async_copy(wo_hbm.at[:, pl.ds(128 * c, 128)], WO.at[c], sems.at[21])
                 for c in range(8)]

    def ln_rstd(g, i, mean):
        acc, m = None, g + opaque()
        for r in range(8):
            d = X[i][m, pl.ds(128 * r, 128), :].reshape(16, 8, 128) - mean[None]
            v = (d * d).sum(0)
            acc = v if acc is None else acc + v
            if r < 7:
                yield _Step(50, [lambda acc=acc: acc], delay=3)
        rstd = jax.lax.rsqrt(_all_sublanes(acc, jnp.add, 0) * (1.0 / D) + EPS)
        yield _Step(50, delay=8)
        yield _Step(10, [lambda: rstd], delay=1)
        return rstd

    def fwd_block(g, i, name, needs, free=(), known=False):
        j, t = g + 4 * i, i
        UB, AB, PB, ubu, abu = temps[t]
        yield _Wait(*needs)
        if known:
            means, squares = STAT[4 * g + i, pl.ds(0, 8)], STAT[4 * g + i, pl.ds(8, 8)]
            mean = means.sum(0) * 0.125
            var = (squares.sum(0) + 128.0 * ((means - mean) ** 2).sum(0)) * (1.0 / D)
            rstd = jax.lax.rsqrt(var + EPS)
            yield _Step(50, delay=6)
        else:
            yield settle(X[i])
            acc, m = None, g + opaque()
            for r in range(8):
                v = X[i][m, pl.ds(128 * r, 128), :].reshape(16, 8, 128).sum(0)
                acc = v if acc is None else acc + v
                if r % 2:
                    yield _Step(35, [lambda acc=acc: acc], delay=7 if r == 7 else 3)
            mean = _all_sublanes(acc, jnp.add, 0) * (1.0 / D)
            rstd = yield from ln_rstd(g, i, mean)
        mean8, rstd = (jnp.concatenate([v, v], 0) for v in (mean * 8.0, rstd))
        z = opaque()
        for r in range(8):
            rows = pl.ds(16 * r, 16)
            x = [X[i][g + z, pl.ds(128 * b + 16 * r, 16), :] for b in range(8)]
            s = [x[b] + x[b + 4] for b in range(4)]
            d = [x[b] - x[b + 4] for b in range(4)]
            e, o = s[0] + s[2], s[1] + s[3]
            UB[0, rows, :] = ((e + o - mean8) * rstd).astype(BF16)
            UB[0, pl.ds(128 + 16 * r, 16), :] = ((e - o) * rstd).astype(BF16)
            t1, t2 = (d[1] - d[3]) * RSQ2, (d[1] + d[3]) * RSQ2
            u = {1: (d[0] + t1, d[2] + t2), 2: (s[0] - s[2], s[1] - s[3]), 3: (d[0] - t1, d[2] - t2)}
            yield _Step(34, [anchor(ubu)], delay=1)
            for k in (1, 2, 3):
                c, sn = twid[z + 2 * k - 2, rows, :] * rstd, twid[z + 2 * k - 1, rows, :] * rstd
                re, m = u[k]
                if k == 3:
                    ur, ui = re * c + m * sn, m * c - re * sn
                else:
                    ur, ui = re * c - m * sn, m * c + re * sn
                UB[0, pl.ds(256 * k + 16 * r, 16), :] = ur.astype(BF16)
                UB[0, pl.ds(256 * k + 128 + 16 * r, 16), :] = ui.astype(BF16)
                yield _Step(26, [anchor(ubu)], delay=1)
        yield settle(ubu)

        def d_forward(point):
            z = opaque()
            first = _iota(8, 0) == 0

            def stage(c):
                u = (M_C4 if c == 1 else M_R) + opaque()
                lhs = mat(u) if c % 4 else _bf(tied(lambda r: mats[u, pl.ds(r, 8), :], 8, point))
                v = _dot(lhs, _bf(ubu[z, pl.ds(64 * c, 64), :]))
                return [(v[32 * u:32 * u + 16], v[32 * u + 16:32 * u + 32]) for u in range(4)]

            def put(row, u, v, v0=None):
                if u == 0 and v0 is not None:
                    v = jnp.concatenate([jnp.where(first, v0, v[:8]), v[8:]], 0)
                AB[0, pl.ds(row + 16 * u, 16), :] = v.astype(BF16)

            for u, (p1, p2) in enumerate(stage(0)):
                put(0, u, p1)
                put(528, u, p2, 0.0)
                if u == 0:
                    put(512, 0, jnp.zeros_like(p2), p2[:8])
            for u, (p1, p2) in enumerate(stage(1)):
                put(256, u, p1)
                put(528 + 256, u, p2)
            for k in (1, 2, 3):
                for u, ((p1, p2), (q1, q2)) in enumerate(zip(stage(2 * k), stage(2 * k + 1))):
                    if k == 3:
                        pr, pi, mr, mi = p1 - q2, p2 + q1, p1 + q2, p2 - q1
                        pi0, mi0 = q1[:8], -q2[:8]
                    else:
                        pr, pi, mr, mi = p1 + q2, p2 - q1, p1 - q2, p2 + q1
                        pi0, mi0 = -q1[:8], q2[:8]
                    put(64 * k, u, pr, p1[:8])
                    put(64 * (8 - k), u, mr, p2[:8])
                    put(528 + 64 * k, u, pi, pi0)
                    put(528 + 64 * (8 - k), u, mi, mi0)
            return 190

        yield _Mat(d_forward)
        yield settle(abu)
        yield _Wait(*free)

        def s_forward(point):
            z = opaque()
            fa, fb = mat(M_FA + j + z), mat(M_FB + j + z)
            for r0, rn in ((0, 256), (256, 272)):
                lhs = abu[z, pl.ds(r0 // 2, rn // 2), :] if r0 else tied(
                    lambda r: abu[z, pl.ds(r, 8), :], 16, point)
                u = _dot(_bf(lhs), fa)
                v = _dot(_bf(abu[z, pl.ds(264 + r0 // 2, 128), :]), fb)
                re, m = u[:256] + v, u[:256] - v
                if r0:
                    re, m = (jnp.concatenate([a, u[256:264]], 0) for a in (re, m))
                rn = re.shape[0]
                edge = (_iota(rn, 1) & 63) == 0
                ZT[2 * i, pl.ds(r0, rn), :] = re
                ZT[2 * i + 1, pl.ds(r0, rn), :] = jnp.where(
                    edge, lane_vec(L_MU + j, rn) * m + lane_vec(L_NU + j, rn) * re, pltpu.roll(m, 64, 1))
            return 400

        yield _Mat(s_forward)
        yield _Step(2, [anchor(ZT)], delay=SETTLE, marks=[name])

    def group_stage(g, name, needs, inverse):
        yield _Wait(*needs)

        def turn(z, k):
            if k == 0:
                return z
            c, s = rot[4 * g + k], rot[16 + 4 * g + k]
            if inverse:
                return z[0] * c - z[1] * s, z[1] * c + z[0] * s
            return z[0] * c + z[1] * s, z[1] * c - z[0] * s

        (src, a), (dst, b) = ((Z, 8 * g), (ZT, 0)) if inverse else ((ZT, opaque()), (Z, 8 * g))
        for r in range(65):
            if r % (16 if inverse else 64) == 0:
                yield hold(src, 2 * NB if inverse else 8)
            rows = pl.ds(8 * r, 8)
            z = [(src[a + 2 * i, rows, :], src[a + 2 * i + 1, rows, :]) for i in range(4)]
            if inverse:
                z = _radix4([turn(z[k], k) for k in range(4)], True)
            else:
                z = [turn(v, k) for k, v in enumerate(_radix4(z, False))]
            for i in range(4):
                dst[b + 2 * i, rows, :], dst[b + 2 * i + 1, rows, :] = z[i]
            yield _Step(35, [anchor(dst)], delay=1, marks=[name] if r == 64 else [])

    def spectral(row, size):
        rows = pl.ds(row, size)
        for k0 in range(4):
            z = _radix4([(Z[8 * g + 2 * k0, rows, :], Z[8 * g + 2 * k0 + 1, rows, :])
                         for g in range(4)], False)
            y = []
            for k1, (re, im) in enumerate(z):
                w = WS[k0 + 4 * k1, rows, :]
                wr = pltpu.bitcast(w << 16, F32)
                wi = pltpu.bitcast(w & np.uint32(0xFFFF0000), F32)
                y.append((re * wr - im * wi, re * wi + im * wr))
            y = _radix4(y, True)
            for g in range(4):
                Z[8 * g + 2 * k0, rows, :], Z[8 * g + 2 * k0 + 1, rows, :] = y[g]

    def spectral_rows(c2):
        for r in range(8):
            spectral(pl.multiple_of(128 * c2 + 16 * r, 16), 16)

    def inv_block(g, i, name, needs, n=None):
        j, t = g + 4 * i, i % 2
        UB, AB, PB, ubu, abu = temps[t]
        n = g if n is None else n
        z = opaque()
        yield _Wait(*needs)
        for r0, rn in _S_ROWS:
            if r0 == 0:
                yield hold(ZT, 8)
            re, im = ZT[z + 2 * i, pl.ds(r0, rn), :], ZT[z + 2 * i + 1, pl.ds(r0, rn), :]
            edge = (_iota(rn, 1) & 63) == 0
            rolled = pltpu.roll(im, 64, 1)
            u = re + jnp.where(edge, lane_vec(L_KU + j, rn) * im, rolled)
            if r0 < 512:
                v = re - jnp.where(edge, lane_vec(L_KV + j, rn) * im, rolled)
                AB[0, pl.ds(r0, rn), :] = u.astype(BF16)
                AB[0, pl.ds(528 + r0, rn), :] = v.astype(BF16)
            else:
                AB[0, pl.ds(512, 16), :] = jnp.concatenate([u, jnp.zeros_like(u)], 0).astype(BF16)
            yield _Step(rn, [anchor(abu)], delay=1, marks=[("read", name)] if r0 == 512 else [])
        yield settle(abu, 4)

        def s_inverse(point):
            z = opaque()
            fa, fb = mat(M_FA + j + z), mat(M_FB + j + z)
            first = _iota(8, 0) == 0

            def put(row, v, v0=None):
                if v0 is not None:
                    v = jnp.concatenate([jnp.where(first, v0, v[:8]), v[8:]], 0)
                UB[0, pl.ds(row, 64), :] = v.astype(BF16)

            for k in range(4):
                lo, hi = 32 * k, 32 * (8 - k if k else 4)
                a = [abu[z, pl.ds(lo, 32), :], abu[z, pl.ds(hi, 32), :]] if k % 2 else [
                    tied(lambda r, o=o: abu[z, pl.ds(o + r, 8), :], 4, point) for o in (lo, hi)]
                if k == 0:
                    a.append(abu[z, pl.ds(256, 8), :])
                re = _dot_t(_bf(jnp.concatenate(a, 0)), fa)
                im = _dot_t(_bf(jnp.concatenate(
                    [abu[z, pl.ds(264 + lo, 32), :], abu[z, pl.ds(264 + hi, 32), :]], 0)), fb)
                pr, mr, pi, mi = re[:64], re[64:128], im[:64], im[64:]
                if k == 0:
                    put(0, pr)
                    put(64, pi, re[128:136])
                    put(128, mr)
                    put(192, mi)
                else:
                    put(256 * k, pr + mr, pr[:8])
                    put(256 * k + 64, pi + mi, mr[:8])
                    put(256 * k + 128, pi - mi, pi[:8])
                    put(256 * k + 192, mr - pr, -mi[:8])
            return 190

        yield _Mat(s_inverse)
        yield settle(ubu, 4)
        yield d_stage(t, lambda c: {0: M_R0T, 1: M_C4T}.get(c, M_RT))
        yield settle(PB, 4)
        z = opaque()
        acc = None
        for r in range(16):
            rows = pl.ds(8 * r, 8)
            t0, t4 = PB[z, rows, :], PB[z, pl.ds(128 + 8 * r, 8), :]
            tk = {}
            for k in (1, 2, 3):
                c, sn = twid[z + 2 * k - 2, rows, :], twid[z + 2 * k - 1, rows, :]
                re = PB[z, pl.ds(256 * k + 8 * r, 8), :]
                im = PB[z, pl.ds(256 * k + 128 + 8 * r, 8), :]
                tk[k] = (re * c - im * sn, re * sn + im * c)
            e0, e1 = t0 + t4, t0 - t4
            s = [e0 + tk[2][0], e1 - tk[2][1], e0 - tk[2][0], e1 + tk[2][1]]
            al, be = tk[1][0] - tk[3][0], tk[1][1] + tk[3][1]
            o = [tk[1][0] + tk[3][0], (al - be) * RSQ2, tk[3][1] - tk[1][1], (al + be) * -RSQ2]
            for b in range(8):
                y = s[b] + o[b] if b < 4 else s[b - 4] - o[b - 4]
                v = X[i][g, pl.ds(128 * b + 8 * r, 8), :] + y
                X[i][n, pl.ds(128 * b + 8 * r, 8), :] = v
                acc = v if acc is None else acc + v
            yield _Step(57, [lambda v=acc: v], delay=5 if r == 15 else 2)
        yield settle(X[i], 4)
        mean = _all_sublanes(acc, jnp.add, 0) * (1.0 / D)
        rstd = yield from ln_rstd(n, i, mean)
        z = opaque()
        for r in range(8):
            v = X[i][n + z, pl.ds(128 * r, 128), :].reshape(16, 8, 128)
            HB[i][n, pl.ds(128 * r, 128), :] = ((v - mean[None]) * rstd[None]).reshape(128, 128).astype(BF16)
            yield _Step(41, [anchor(hbu[i])], delay=1, marks=[name] if r == 7 else [])

    def attend(g, i, name, needs):
        yield _Wait(*needs)
        yield settle(QB[i])
        j, z = g + 4 * i, opaque()
        even = (_iota(8, 0) & 1) == 0
        edge = _iota(8, 1) == 0

        def window(near, far, w, rows):
            return near[j + z + 4 - 2 * w, rows, :] if w <= 2 * i + 2 else far[j + z + 16 - 2 * w, rows, :]

        def mix_values(h, u):
            p = PW[h % 2][opaque()]
            for rows in (pl.ds(256 * h + 16 * u, 16), pl.ds(256 * h + 16 * u + 16, 16)):
                acc = functools.reduce(jnp.add, [p[16 * w:16 * w + 16] * window(VE, VS, w, rows)
                                                 for w in range(8)])
                HB[i][g, rows, :] = acc.astype(BF16)
            return _Step(63, [anchor(hbu[i])], delay=2, marks=[name] if (h, u) == (3, 14) else [])

        for h in range(5):
            logits = []
            for w0 in range(0, 8, 2):
                if h < 4:
                    rows = pl.ds(256 * h, 256)
                    q = q if w0 % 4 else QB[i][opaque(), rows, :]
                    for w in (w0, w0 + 1):
                        v = (q * window(KE, KS, w, rows)).reshape(16, 16, 128).sum(0)
                        v = jnp.where(even, v[:8] + pltpu.roll(v[:8], 7, 0), v[8:] + pltpu.roll(v[8:], 1, 0))
                        logits.append(jnp.where(edge & (2 * w > j), -1e9, v * SCALE) if w > 2 * i
                                      else v * SCALE)
                    yield _Step(138, [lambda v=v: v for v in logits[-2:]], delay=4)
                if h > 0:
                    yield mix_values(h - 1, 2 * w0)
                    yield mix_values(h - 1, 2 * w0 + 2)
            if h < 4:
                top = functools.reduce(jnp.maximum, logits)
                e = [jnp.exp(v - top) for v in logits]
                total = functools.reduce(jnp.add, e)
                yield _Step(30, [lambda v=total: v], delay=3)
                scale = 1.0 / total
                for w in range(8):
                    v = e[w] * scale
                    PW[h % 2][0, pl.ds(16 * w, 8), :] = jnp.where(even, v, pltpu.roll(v, 1, 0))
                    PW[h % 2][0, pl.ds(16 * w + 8, 8), :] = jnp.where(even, pltpu.roll(v, 7, 0), v)
                yield _Step(50, [anchor(PW[h % 2])], delay=6 if h == 3 else 1)

    def packed_sums(terms, signs):
        lo = [pltpu.bitcast(u << 16, F32) for u in terms]
        hi = [pltpu.bitcast(u & np.uint32(0xFFFF0000), F32) for u in terms]
        return [pltpu.pack_elementwise([v[p] + v[q] if s > 0 else v[p] - v[q] for v in (lo, hi)],
                                       packed_dtype=BF16) for p, s, q in signs]

    def half(ref, row):
        return lambda r, size, cols: ref[pl.ds(pl.multiple_of(row + r, 8), size), cols]

    kv_weight = (WS5, half(WK, 0), half(WV, 0))
    q_weight = (WQ5, half(WQ, 0), half(WQ, D // 4))
    o_weight = (WP5, *(lambda r, size, cols, e=e: WP[pl.ds(r + r // 32 * 32 + e, size), cols]
                       for e in (0, 32)))

    def left_sums(weight, row, size, needs=()):
        yield _Wait(*needs)
        sums, top, bottom = weight
        for r in range(0, size, 8):
            a = [ref(row + r, 8, pl.ds(c, 512)) for ref in (top, bottom) for c in (0, 512)]
            for e, v in enumerate(packed_sums(a, ((0, 1, 3), (2, 1, 3), (0, 1, 1), (2, -1, 0), (1, -1, 3)))):
                sums[e, pl.ds(pl.multiple_of(row + r, 8), 8), :] = v
            yield _Step(92, [anchor(sums)], delay=2, marks=["sums"] if r == size - 8 else [])

    def right_sums(dst, g, i, name, needs):
        yield _Wait(*needs)
        z = g + opaque()
        for r in range(0, 256, 16):
            b = [hbu[n][z, pl.ds(k + r, 16), :] for k in (0, 256) for n in (i, i + 1)]
            for e, v in enumerate(packed_sums(b, ((0, 1, 3), (1, -1, 3), (2, -1, 0), (0, 1, 1), (2, 1, 3)))):
                dst[e, pl.ds(r, 16), :] = v
            yield _Step(47, [anchor(dst)], delay=SETTLE if r == 240 else 1,
                        marks=[name] if r == 240 else [])

    def strassen(sch, weight, right, g, i, m, store, needs, marks):
        for n in needs:
            sch.run(n)
        sums, top, bottom = weight
        rows = pl.ds(pl.multiple_of(64 * m, 64), 64)

        def product(left, b):
            sch.fresh = True
            head = tied(lambda r: left(32 * m + r, 8, pl.ds(0, 128)), 4, lambda: sch.point(8.0))
            return _dot(_bf(jnp.concatenate([head, left(32 * m, 32, pl.ds(128, 384))], 1)), _bf(b))

        def a(e):
            return lambda r, size, cols: sums[e, pl.ds(pl.multiple_of(r, 8), size), cols]

        def b(e):
            return right[e + opaque()]

        m2 = product(a(1), hbu[i][g + opaque(), pl.ds(0, 256), :])
        m4 = product(lambda r, size, cols: bottom(r, size, pl.ds(512 + cols.start, cols.size)), b(2))
        store(1, i, rows, m2 + m4)
        m1 = product(a(0), b(0))
        c11, c22 = m1 + m4, m1 - m2
        c11 = c11 + product(a(4), b(4))
        c22 = c22 + product(a(3), b(3))
        m5 = product(a(2), hbu[i + 1][g + opaque(), pl.ds(256, 256), :])
        store(0, i, rows, c11 - m5)
        v = product(top, b(1))
        store(0, i + 1, rows, v + m5)
        store(1, i + 1, rows, c22 + v)
        sch.results.append(v[:8])
        for name in marks:
            sch.done[name] = sch.slot + sch.wait

    def kv_proj(sch, g, i, name, needs):
        def store(lower, n, rows, v):
            (KE, VE)[lower][g + 4 * n + 4, rows, :] = v
        for m in range(16):
            strassen(sch, kv_weight, SB[i // 2], g, i, m, store, needs, [name] if m == 15 else [])

    def q_proj(sch, g, i, name, needs):
        def store(lower, n, rows, v):
            QB[n][0, pl.ds(512 * lower + rows.start, 64), :] = v
        for m in range(8):
            strassen(sch, q_weight, SB[i // 2], g, i, m, store, needs, [name] if m == 7 else [])

    def o_proj(sch, g, i, m, needs, marks, right):
        def store(lower, n, rows, v):
            rows = pl.ds(128 * m + 64 * lower, 64)
            X[n][g, rows, :] = X[n][g, rows, :] + v
        strassen(sch, o_weight, right, g, i, m, store, needs, marks)

    def shift_block(g, i, name, needs):
        yield _Wait(*needs)
        j, z = g + 4 * i, opaque()
        for m in range(16):
            rows = pl.ds(64 * m, 64)
            for ref, to in ((KE, KS), (VE, VS)):
                v = pltpu.roll(ref[j + 4 + z, rows, :], 1, 1)
                if ref is VE:
                    v = jnp.where(_iota(64, 1) == 0, ref[4 + z, rows, :], v)
                to[j, rows, :] = v
                if i == 3:
                    ref[g, rows, :] = v
            yield _Step(12, delay=8, marks=[name] if m == 15 else [])

    def transpose_quarter(w, h, via):
        for r in range(4):
            v = WRAW[w, pl.ds(256 * r, 256), pl.ds(pl.multiple_of(256 * h, 256), 256)]
            v = pltpu.bitcast(v.T, F32)
            via[0, pl.ds(256 * r, 128), :], via[0, pl.ds(256 * r + 128, 128), :] = v[:, :128], v[:, 128:]
            yield _Step(40, delay=16)

    def reorder_quarter(w, h, via, name=None):
        z = 0 if isinstance(h, int) else opaque()
        for c in range(8):
            WT[w][pl.ds(pl.multiple_of(128 * h, 128), 128), pl.ds(128 * c, 128)] = pltpu.bitcast(
                jnp.concatenate([via[z, pl.ds(128 * c + u, 8, stride=16), :] for u in range(16)], 0), U32)
            yield _Step(20, delay=4, marks=[name] if c == 7 else [])

    def query_weight(h):
        yield from transpose_quarter(0, h, QB[0])
        yield from reorder_quarter(0, h, QB[0], "w")

    def transpose_wo(name):
        for c in range(8):
            for h in range(4):
                v = jnp.concatenate([wou[c, pl.ds(128 * h + u, 8, stride=16), :] for u in range(16)], 0)
                WP[pl.ds(64 * c, 64), pl.ds(256 * h, 256)] = pltpu.bitcast(_bf(v).T, U32)
                yield _Step(20, delay=10, marks=[name] if c == 7 and h == 3 else [])

    def prep_spectral_weights(c2):
        lane = _iota(8, 1)
        order = jnp.where(lane > 64, 192 - lane, lane)

        def words(k2):
            re, im = (wsu[u, k2, pl.ds(c2, 64, stride=4), :] for u in range(2))
            return ((re & np.uint32(0xFFFF)) | (im << 16), (re >> 16) | (im & np.uint32(0xFFFF0000)))

        def arrange(w, below):
            w = jnp.where(_iota(w.shape[0], 1) < 64, w, below)
            return jnp.concatenate([jnp.take_along_axis(w[u:u + 8], order, axis=1)
                                    for u in range(0, w.shape[0], 8)], 0)

        below = words(15)
        for k2 in range(16):
            here = words(k2)
            for e in range(2):
                cl = 2 * c2 + e
                w = arrange(here[e], below[e])
                WS[k2, pl.ds(64 * cl, 64), :] = pltpu.roll(w, 1, 0) if cl > 4 else w
            below = here
            yield _Step(100)
        if c2 == 0:
            def nyquist(k2):
                re, im = (jnp.broadcast_to(WN[u, :, pl.ds(128 * k2, 128)].astype(F32), (8, 128))
                          for u in range(2))
                return pltpu.pack_elementwise([re, im], packed_dtype=BF16)
            for k2 in range(16):
                WS[k2, pl.ds(512, 8), :] = arrange(nyquist(k2), nyquist((k2 + 15) % 16))

    def write_out(p, c, name, needs):
        yield _Wait(*needs)
        rows = pl.ds(pl.multiple_of(128 * c, 128), 128)
        g, i = 2 * p % 4 + opaque(), p // 2
        w = pltpu.pack_elementwise([X[i][g, rows, :], X[i][g + 1, rows, :]], packed_dtype=BF16)
        xru[c, pl.ds(p, 128, stride=8), :] = w.T
        yield _Step(30, marks=[name])

    for c in range(8):
        x_copy(c).start()
    for c in range(5):
        mats[M_R + c] = d_mats[c]

    def make_twiddle(k):
        PB = temps[0][2]
        PB[0, pl.ds(0, 128), :] = lane_vec(L_TWID + k, 128)
        twid[k] = PB[opaque(), pl.ds(0, 128), :].T

    _loop(6, make_twiddle, "make_twiddle")

    def make_dft(j):
        fa, fb = lanes[pl.ds(L_FA, 128), :], lanes[pl.ds(L_FB, 128), :]
        c, sn = lane_vec(L_COS + j, 128), lane_vec(L_SIN + j, 128)
        UB, _, _, ubu, _ = temps[0]
        UB[0, pl.ds(0, 128), :] = (fa * c + fb * sn).astype(BF16)
        UB[0, pl.ds(128, 128), :] = (fb * c - fa * sn).astype(BF16)
        mats[M_FA + j], mats[M_FB + j] = ubu[0, pl.ds(0, 64), :], ubu[0, pl.ds(64, 64), :]

    _loop(NB, make_dft, "make_dft")

    def load_x(c):
        x_copy(c).wait()
        pl.when(c == 6)(lambda: start_all(spec_copies[0]))
        pl.when(c == 7)(lambda: start_all(spec_copies[1]))
        rows = pl.ds(pl.multiple_of(128 * c, 128), 128)
        for p in range(8):
            w = xru[c, pl.ds(p, 128, stride=8), :].T
            for e, bits in enumerate((w << 16, w & np.uint32(0xFFFF0000))):
                g, i = 2 * p % 4 + e, p // 2
                v = pltpu.bitcast(bits, F32)
                X[i][g, rows, :] = v
                v = v.reshape(16, 8, 128)
                mean = _all_sublanes(v.sum(0), jnp.add, 0) * (1.0 / 128)
                STAT[4 * g + i, c] = mean
                STAT[4 * g + i, 8 + c] = _all_sublanes(((v - mean) ** 2).sum(0), jnp.add, 0)

    _loop(8, load_x, "load_x")

    def after(name, action):
        yield _Wait(name)
        action()

    def spectral_weights():
        yield _Wait(("f", 2, 1))
        for c in spec_copies[0] + spec_copies[1]:
            c.wait()
        for c2 in range(4):
            yield from prep_spectral_weights(c2)

    with jax.named_scope("first_forward"):
        sch = _Sched(0.72, 20)
        sch.add(after(("f", 0, 1), w_copies[1].start), "k")
        sch.add(after(("f", 1, 1), w_copies[2].start), "v")
        sch.add(after(("f", 2, 3), w_copies[0].start), "q")
        for g in range(4):
            for i in range(4):
                sch.add(fwd_block(g, i, ("f", g, i), [("f", g - 1, i)] if g else [],
                                  [("r", g - 1)] if g else [], True), ("f", g, i))
            sch.add(group_stage(g, ("r", g), [("f", g, i) for i in range(4)], False), ("r", g))
        sch.add(spectral_weights(), "s")
        sch.drive()
    start_all(wo_copies)

    def keys_values(layer, g):
        sch = _Sched(0.41, 32, 3) if layer == 0 else _Sched(0.36, 28, 2)
        nxt = (g + 1) % 4
        sch.add(inv_block(g, 2, ("i", 2), []), ("i", 2))
        sch.add(inv_block(g, 3, ("i", 3), [("read", ("i", 2))]), ("i", 3))
        sch.add(right_sums(SB[1], g, 2, ("b", 2), [("i", 2), ("i", 3)]), ("b", 2))
        sch.add(group_stage(nxt, "r", [("read", ("i", 3))], True), "r")
        sch.add(inv_block(nxt, 0, ("i", 4), ["r", ("i", 2)], n=g + 1), ("i", 4))
        sch.add(inv_block(nxt, 1, ("i", 5), [("read", ("i", 4)), ("i", 3)], n=g + 1), ("i", 5))
        if layer == 0:
            sch.add(query_weight(g), "w")
            sch.add(left_sums(q_weight, 128 * (g % 2), 128, ["w"]), "sums")
        for i in (2, 3):
            sch.add(shift_block((g + 3) % 4, i, ("s", i), []), ("s", i))
        for i in (0, 1):
            sch.add(shift_block(g, i, ("s", i), [("kv", 0)]), ("s", i))
        sch.add(right_sums(SB[0], nxt, 0, ("b", 4), [("i", 4), ("i", 5), ("kv", 0)]), ("b", 4))
        kv_proj(sch, g, 0, ("kv", 0), [])
        kv_proj(sch, g, 2, ("kv", 2), [("b", 2)])
        sch.finish()

    def mix(g, after, last):
        tail = after is None
        sch = _Sched(0.66 if last else 0.63, 28 if last else 32)
        pace = 0.48 if tail else 0.35 if last else 0.32
        ahead = [(g, 2), (g, 3)] + ([] if tail else [(after, 0), (after, 1)])
        for n, block in enumerate(ahead):
            sch.add(attend(*block, ("a", n), [[], [("a", 0)], [("a", 1), ("q", 0)], [("a", 2)]][n]),
                    ("a", n), pace=pace)
            if n % 2:
                sch.add(right_sums(SB[2 + block[1] // 2], block[0], block[1] - 1, ("b", n),
                                   [("a", n)] + ([("o", 0)] if n == 3 else [])), ("b", n))
        for i in () if tail else (0, 2):
            sch.add(right_sums(SB[i // 2], after, i, ("h", i), [("q", 0)] if i else []), ("h", i))
        if not last:
            sch.add(group_stage((g + 3) % 4, "r", [], False), "r")
            for i in range(4):
                sch.add(fwd_block(g, i, ("f", i), [("o", i - i % 2)], ["r"]), ("f", i))
        now = 6 if last else 8
        for i in (0, 2):
            for m in range(now):
                o_proj(sch, g, i, m, [("b", 1)] if i else [], [("o", i)] if m == now - 1 else [],
                       SB[2 + i // 2])
            if not tail:
                q_proj(sch, after, i, ("q", i), [("h", i)])
        if tail:
            sch.add(group_stage(g, "s", [("f", i) for i in range(4)], False), "s")
        sch.share = 0.92
        sch.drive()

    def mix_odd():
        sch = _Sched(0.66)
        blocks = [(1, 2), (1, 3), (3, 0), (3, 1), (3, 2), (3, 3)]
        for n, (g, i) in enumerate(blocks):
            sch.add(attend(g, i, ("a", n), ([("a", n - 1)] if n else []) + ([("q", i)] if n in (2, 4) else [])),
                    ("a", n), pace=0.32)
            if n % 2:
                sch.add(right_sums(SB[(3, 2, 0)[n // 2]], g, i - 1, ("b", g, i - 1),
                                   [("a", n)] + ([("o", 1, 0, 5)] if n > 1 else [])), ("b", g, i - 1))
        for i in (0, 2):
            sch.add(right_sums(SB[i // 2], 3, i, ("h", i), []), ("h", i))
        for g in (1, 3):
            for i in range(4):
                for c in range(6):
                    sch.add(write_out(2 * i + g // 2, c, ("w", g, i, c), [("o", g, i - i % 2, c)]),
                            ("w", g, i, c))
        for g, i, slot, count in ((1, 0, 2, 6), (1, 2, 3, 8), (3, 0, 2, 8), (3, 2, 0, 6)):
            for m in range(count):
                o_proj(sch, g, i, m, [("b", g, i)] if (g, i) != (1, 0) else [], [("o", g, i, m)], SB[slot])
            for e in (0, 2) if (g, i) == (1, 0) else ():
                q_proj(sch, 3, e, ("q", e), [("h", e)] + ([("a", 1)] if e else []))
        sch.share = 0.92
        sch.drive()

    def copy_out(chunks):
        def start(_):
            for c in chunks:
                out_copy(c).start()
        _loop(zero + 1, start, "copy_out")

    def postponed():
        slots = {(3, 2): 0, (2, 2): 1, (0, 2): 2, (2, 0): 3, (0, 0): 0, (1, 0): 1}
        early, late = list(slots)[:2], list(slots)[2:]
        sources = 2 * [[(0, 0), (1, 0)], [(2, 0)]] + 2 * [[(0, 2)], []]
        for c in (6, 7):
            sch = _Sched(0.7, 12)
            for n, (pair, slot) in enumerate(slots.items()) if c == 6 else ():
                if n:
                    sch.add(right_sums(SB[slot], *pair, pair, [(early[n - 4], 7)] if n >= 4 else []), pair)
            for p in (5, 7, 4, 6, 1, 3, 0, 2):
                sch.add(write_out(p, c, ("w", p), [(pair, c) for pair in sources[p] or early * (c == 6)]),
                        ("w", p))
            for pair, m in [(pair, m) for m in (6, 7) for pair in early] * (c == 6) + [(v, c) for v in late]:
                o_proj(sch, *pair, m, [pair] if c == 6 and pair != (3, 2) else [], [(pair, m)],
                       SB[slots[pair]])
            sch.drive()
            copy_out([c])

    def first_queries(layer):
        sch = _Sched(0.68)
        sch.add(right_sums(SB[1], 0, 2, ("h", 2), []), ("h", 2))
        sch.add(shift_block(3, 2, "s", []), "s")
        sch.add(attend(0, 0, ("a", 0), ["q"]), ("a", 0), pace=0.4)
        sch.add(attend(0, 1, ("a", 1), [("a", 0)]), ("a", 1), pace=0.4)
        sch.add(right_sums(SB[2], 0, 0, "b", [("a", 1)]), "b")
        sch.add(shift_block(3, 3, "t", []), "t")
        if layer == 0:
            for c in wo_copies:
                c.wait()
            sch.add(transpose_wo("w"), "w")
            sch.add(left_sums(o_weight, 0, 256, ["w"]), "sums")
        q_proj(sch, 0, 0, "q", [])
        q_proj(sch, 0, 2, None, [("h", 2)])
        sch.finish()

    def key_value_weights():
        w_copies[1].wait()
        w_copies[2].wait()
        for h in range(6):
            work = []
            for w in (1, 2):
                if h < 4:
                    work.append(transpose_quarter(w, h, QB[2 * (h % 2) + w - 1]))
                if 0 < h < 5:
                    work.append(reorder_quarter(w, h - 1, QB[2 * ((h - 1) % 2) + w - 1]))
            if h > 1:
                work.append(left_sums(kv_weight, 128 * (h - 2), 128))
            list(itertools.zip_longest(*work))

    for layer in range(2):
        with jax.named_scope("spectral"):
            _loop(4, spectral_rows, "rows")
            if layer == 0:
                _loop(zero + 1, lambda _: key_value_weights(), "weights")
            spectral(512, 8)
        sch = _Sched(0.92)
        sch.add(group_stage(0, "r", [], True), "r")
        sch.add(inv_block(0, 0, ("i", 0), ["r"]), ("i", 0))
        sch.add(inv_block(0, 1, ("i", 1), ["r"]), ("i", 1))
        sch.add(right_sums(SB[0], 0, 0, "b", [("i", 0), ("i", 1)]), "b")
        sch.drive()
        if layer == 0:
            w_copies[0].wait()
        _loop(4, lambda g: keys_values(layer, g), "keys_values")
        first_queries(layer)
        if layer == 0:
            pl.when(never)(lambda: spectral_rows(0))
        if layer == 0:
            _loop(3, lambda g: mix(g, g + 1, False), "mix")
            mix(3, None, False)
        else:
            _loop(2, lambda u: mix(2 * u, 2 - u, True), "mix")
            mix_odd()
    copy_out(range(6))
    postponed()
    for c in range(8):
        out_copy(c).wait()


@jax.jit
def pallas_interleave_layers__spectral_gfnet__sliding_local_dilated__prompt_kernel(
    A_x: jax.Array,
    A_w_r: jax.Array,
    A_w_i: jax.Array,
    B_x: jax.Array,
    B_wqkv: jax.Array,
    B_wo: jax.Array,
):
    del B_x
    hbm = pl.BlockSpec(memory_space=pl.ANY)
    smem = pl.BlockSpec(memory_space=pltpu.SMEM)
    out = pl.pallas_call(
        _kernel,
        out_shape=jax.ShapeDtypeStruct((S, D), BF16),
        in_specs=[smem, smem, pl.BlockSpec(), pl.BlockSpec(), hbm, hbm, hbm, hbm, hbm],
        out_specs=hbm,
        scratch_shapes=[
            pltpu.VMEM((37, 64, 128), U32),
            pltpu.VMEM((6, 128, 128), F32),
            pltpu.VMEM((NB, 16, 8, 128), F32),
            pltpu.VMEM((NB + 4, D, 128), F32),
            pltpu.VMEM((NB + 4, D, 128), F32),
            pltpu.VMEM((NB, D, 128), F32),
            pltpu.VMEM((NB, D, 128), F32),
            pltpu.VMEM((2 * NB + 1, ZR, 128), F32),
            pltpu.VMEM((9, ZR, 128), F32),
            pltpu.VMEM((NB, ZR, 128), U32),
            *4 * [pltpu.VMEM((D // 2, D), U32)],
            pltpu.VMEM((5, D // 2, D // 2), U32),
            *2 * [pltpu.VMEM((5, D // 4, D // 2), U32)],
            *4 * [pltpu.VMEM((5, D // 4, 128), U32)],
            pltpu.VMEM((8, S, 128), BF16),
            pltpu.VMEM((2, NB, D // 2, 128), BF16),
            pltpu.VMEM((2, 1, S), BF16),
            pltpu.VMEM((3, D, D), BF16),
            pltpu.VMEM((8, D, 128), BF16),
            pltpu.VMEM((1, 128, 128), F32),
            pltpu.VMEM((1, 128, 128), F32),
            pltpu.SemaphoreType.DMA((24,)),
            *2 * [pltpu.VMEM((1, D, 128), F32)],
        ] + 4 * [
            pltpu.VMEM((5, D, 128), F32),
            pltpu.VMEM((5, D, 128), BF16),
            pltpu.VMEM((1, D, 128), F32),
            pltpu.VMEM((1, D, 128), BF16),
            pltpu.VMEM((1, 1152, 128), BF16),
        ],
        compiler_params=pltpu.CompilerParams(vmem_limit_bytes=126 * 2 ** 20),
    )(_ZERO, _ROT, _MATS, _LANES, A_x.reshape(S, D), A_w_r.T, A_w_i.T, B_wqkv, B_wo)
    return out.reshape(1, S, D)
```

```python
import functools
import itertools

import numpy as np

import jax
import jax.numpy as jnp
import jax.experimental.pallas as pl
import jax.experimental.pallas.tpu as pltpu

S, D, NB = 2048, 1024, 16
ZR = 576
F32, BF16, U32, I32 = jnp.float32, jnp.bfloat16, jnp.uint32, jnp.int32
EPS = 1e-5
SCALE = 32 ** -0.5
RSQ2 = float(np.sqrt(0.5))
SETTLE = 6

_S_ROWS = [(32 * u, 32) for u in range(16)] + [(512, 8)]

M_FA, M_FB, M_R, M_C4, M_RT, M_C4T, M_R0T = 0, 16, 32, 33, 34, 35, 36
L_MU, L_NU, L_KU, L_KV, L_COS, L_SIN, L_TWID, L_FA, L_FB = 0, 16, 32, 48, 64, 80, 96, 104, 232


def _bf16_bits(a):
    u = np.ascontiguousarray(a, dtype=np.float32).view(np.uint32).astype(np.uint64)
    return ((u + 0x7FFF + ((u >> 16) & 1)) >> 16).astype(np.uint32)


def _constants():
    a = np.arange(128)
    k1 = np.arange(64)
    alt = (-1.0) ** a
    lanes = np.zeros((L_FB + 128, 128))
    t = 2 * np.pi * np.outer(a, k1) / 128
    fa = np.concatenate([np.cos(t), -np.sin(t)], 1)
    fb = np.concatenate([np.sin(t), -np.cos(t)], 1)
    fa[:, 0], fb[:, 0] = RSQ2, -RSQ2
    fa[:, 64], fb[:, 64] = alt, 0.0
    lanes[L_FA:L_FA + 128], lanes[L_FB:L_FB + 128] = fa, fb
    for j in range(NB):
        ang = 2 * np.pi * j / 32 + np.pi / 32
        p, q = (_bf16_bits([np.cos(ang), np.sin(ang)]) << 16).view(np.float32).astype(np.float64)
        turn = 2 * np.pi * j * np.tile(k1, 2) / S
        lanes[L_COS + j], lanes[L_SIN + j] = np.cos(turn), np.repeat([-1.0, 1.0], 64) * np.sin(turn)
        lanes[L_COS + j, 64], lanes[L_SIN + j, 64] = p, q
        lanes[L_MU + j, 0], lanes[L_MU + j, 64] = 1.0, (q / p + p / q) / 2
        lanes[L_NU + j, 0], lanes[L_NU + j, 64] = 0.0, (q / p - p / q) / 2
        lanes[L_KU + j, 0], lanes[L_KU + j, 64] = 1.0, q / p
        lanes[L_KV + j, 0], lanes[L_KV + j, 64] = 1.0, p / q
    lanes[:, 65:] = lanes[:, :64:-1].copy()
    for k in (1, 2, 3):
        lanes[L_TWID + 2 * k - 2] = np.cos(2 * np.pi * a * k / D)
        lanes[L_TWID + 2 * k - 1] = np.sin(2 * np.pi * a * k / D)
    th = 2 * np.pi * np.outer(k1, a) / 128
    r = np.concatenate([np.cos(th), -np.sin(th)], 0)
    r[64] = alt
    th = 2 * np.pi * np.outer(2 * k1 + 1, a) / 256
    c4 = np.concatenate([np.cos(th), -np.sin(th)], 0)
    inv = 2.0 / (S * D)
    r0t = inv * r.T
    r0t[:, 0::64] *= 0.5
    rows = np.arange(128).reshape(2, 4, 16).transpose(1, 0, 2).ravel()
    bits = _bf16_bits(np.stack([r[rows], c4[rows], inv * r.T, inv * c4.T, r0t]))
    ang = 2 * np.pi * np.outer(np.arange(4), np.arange(4)).ravel() / 16
    rot = np.concatenate([np.cos(ang), np.sin(ang)]).astype(np.float32)
    return bits[:, 0::2] | (bits[:, 1::2] << 16), lanes.astype(np.float32), rot


_MATS, _LANES, _ROT = _constants()
_ZERO = np.zeros((1,), np.int32)


class _Step:
    def __init__(self, cost, anchors=(), delay=0, marks=()):
        self.cost, self.anchors, self.delay, self.marks = cost, list(anchors), delay, list(marks)


class _Wait:
    def __init__(self, *names):
        self.names = names


class _Mat:
    def __init__(self, emit):
        self.emit = emit


class _Hold:
    def __init__(self, store):
        self.store = store


class _Task:
    def __init__(self, gen, pace):
        self.gen, self.pace, self.blocked, self.not_before, self.held = gen, pace, (), 0, None
        self.allowed = 0.0


class _Sched:
    def __init__(self, share=0.0, wait=28, lag=3):
        self.lag = lag
        self.wait = wait
        self.share = share
        self.tasks, self.done, self.producer = [], {}, {}
        self.slot, self.credit, self.anchors, self.results = 0, 0.0, [], []
        self.fresh = False

    def add(self, gen, name, pace=99):
        self.producer[name] = self.producer["read", name] = _Task(gen, pace)
        self.tasks.append(self.producer[name])

    def _ready(self, t):
        return t.not_before <= self.slot and all(
            n in self.done and self.done[n] <= self.slot for n in t.blocked)

    def _advance(self, t, mats=True):
        item, t.held = t.held or next(t.gen, None), None
        if item is None:
            self.tasks.remove(t)
        elif isinstance(item, _Wait):
            t.blocked = item.names
        elif isinstance(item, _Hold):
            if len(self.results) >= self.lag:
                item.store(self.results[-self.lag])
        elif isinstance(item, _Mat):
            if mats:
                t.not_before = float("inf")
                self.fresh = False
                self.credit -= item.emit(lambda: self.point(0.0)) or 0
                t.not_before = self.slot + self.wait
            else:
                t.held, t.not_before = item, self.slot + 1
        else:
            t.blocked = ()
            t.not_before = self.slot + item.delay
            self.credit -= item.cost
            self.anchors += item.anchors
            for n in item.marks:
                self.done[n] = self.slot + item.delay
            return True

    def run(self, *names):
        while not all(n in self.done for n in names):
            for n in names:
                if n not in self.done:
                    for b in self.producer[n].blocked:
                        self.run(b)
                    self._advance(self.producer[n])

    def drive(self):
        while self.tasks:
            ready = [t for t in self.tasks if self._ready(t)]
            if not ready:
                self.slot += 1
                continue
            self.anchors, self.credit = self.anchors[-2:], 0.0
            self._advance(next((t for t in ready if t.held), ready[0]))
            self.slot -= min(self.credit, 0.0) / 60

    def finish(self):
        self.run(*[n for n in self.producer if n[0] != "read"])

    def point(self, own):
        for t in self.tasks:
            t.allowed = min(t.allowed, 0.0) + t.pace
        while True:
            t = next((t for t in self.tasks if self._ready(t) and t.allowed > 0
                      and self.credit > 0), None)
            if t is None:
                break
            if self._advance(t, self.fresh):
                t.allowed -= 1
        anchors, self.anchors = self.anchors, []
        self.credit = min(self.credit, 10.0) + 64 * self.share - own
        self.fresh = False
        self.slot += 1
        return anchors


def _dot(a, b):
    return jnp.dot(a, b, preferred_element_type=F32)


def _dot_t(a, b):
    return jax.lax.dot_general(a, b, (((1,), (1,)), ((), ())), preferred_element_type=F32)


def _bf(u):
    return pltpu.bitcast(u, BF16)


def _iota(rows, dim):
    return jax.lax.broadcasted_iota(I32, (rows, 128), dim)


def _mirror(v):
    index = -_iota(8, 1) & 127
    return jnp.concatenate([jnp.take_along_axis(v[r:r + 8], index, axis=1)
                            for r in range(0, v.shape[0], 8)], 0)


def _radix4(z, inverse):
    (r0, i0), (r1, i1), (r2, i2), (r3, i3) = z
    ar, ai, cr, ci = r0 + r2, i0 + i2, r0 - r2, i0 - i2
    br, bi, dr, di = r1 + r3, i1 + i3, r1 - r3, i1 - i3
    lo, hi = (cr + di, ci - dr), (cr - di, ci + dr)
    if inverse:
        lo, hi = hi, lo
    return [(ar + br, ai + bi), lo, (ar - br, ai - bi), hi]


def _all_sublanes(v, op, axis):
    for sh in (4, 2, 1):
        v = op(v, pltpu.roll(v, sh, axis))
    return v


def _loop(n, body, name):
    def step(i, carry):
        body(i)
        return carry
    with jax.named_scope(name):
        jax.lax.fori_loop(0, n, step, 0)


def _kernel(zero_ref, rot, d_mats, lanes, x_hbm, wr_hbm, wi_hbm, wqkv_hbm, wo_hbm, out_hbm,
            mats, twid, STAT, KE, VE, KS, VS, Z, ZT, WS, WQ, WK, WV, WP, WS5, WQ5, WP5,
            SB0, SB1, SB2, SB3, XR, WRI, WN, WRAW, WO, PW0, PW1, sems, *split):
    zero = zero_ref[0]
    never = zero != 0
    X, HB, QB = split[2::5], split[3::5], split[4::5]
    hbu = [r.bitcast(U32) for r in HB]
    xru, wsu, wou = XR.bitcast(U32), WRI.bitcast(U32), WO.bitcast(U32)
    temps = [(ub, ab, pb, ub.bitcast(U32), ab.bitcast(U32))
             for ub, ab, pb in zip(split[5::5], split[6::5], 2 * split[:2])]
    PW, SB, WT = (PW0, PW1), (SB0, SB1, SB2, SB3), (WQ, WK, WV, WP)
    counter = [0]

    def opaque():
        counter[0] += 1
        return zero * counter[0]

    def anchor(ref):
        at = (0,) * (len(ref.shape) - 2)
        return lambda: ref[(*at, pl.ds(pl.multiple_of(zero * 8, 8), 8), pl.ds(0, 128))]

    def settle(ref, points=SETTLE):
        return _Step(2, [anchor(ref)], delay=points)

    def hold(ref, spare):
        def store(v):
            ref[spare, pl.ds(pl.multiple_of(zero * 8, 8), 8), :] = v
        return _Hold(store)

    def tied(load, vregs, point):
        parts = []
        for r in range(vregs):
            anchors = point()
            u = load(8 * r)
            for a in anchors:
                u = jnp.where(never, pltpu.bitcast(a(), U32), u)
            parts.append(u)
        return jnp.concatenate(parts, 0)

    def mat(i):
        return _bf(mats[i])

    def d_stage(t, which):
        UB, AB, PB, ubu, abu = temps[t]

        def emit(point):
            z = opaque()
            for c in range(8):
                lhs = mat(which(c) + opaque()) if c % 4 else _bf(
                    tied(lambda r, u=which(c) + opaque(): mats[u, pl.ds(r, 8), :], 8, point))
                PB[0, pl.ds(128 * c, 128), :] = _dot(lhs, _bf(ubu[z, pl.ds(64 * c, 64), :]))
        return _Mat(emit)

    def lane_vec(i, rows):
        return jnp.broadcast_to(lanes[pl.ds(i, 1), :], (rows, 128))

    def x_copy(c):
        return pltpu.make_async_copy(
            x_hbm.at[:, pl.ds(pl.multiple_of(128 * c, 128), 128)], XR.at[c], sems.at[c])

    def out_copy(c):
        return pltpu.make_async_copy(
            XR.at[c], out_hbm.at[:, pl.ds(pl.multiple_of(128 * c, 128), 128)], sems.at[8 + c])

    spec_copies = [[pltpu.make_async_copy(w.at[pl.ds(0, 512), pl.ds(128 * k2, 128)], WRI.at[u, k2],
                                          sems.at[16 + u]) for k2 in range(16)]
                   + [pltpu.make_async_copy(w.at[pl.ds(512, 1), :], WN.at[u], sems.at[22 + u])]
                   for u, w in enumerate((wr_hbm, wi_hbm))]

    def start_all(copies):
        for c in copies:
            c.start()
    w_copies = [pltpu.make_async_copy(wqkv_hbm.at[:, pl.ds(D * w, D)], WRAW.at[w], sems.at[18 + w])
                for w in range(3)]
    wo_copies = [pltpu.make_async_copy(wo_hbm.at[:, pl.ds(128 * c, 128)], WO.at[c], sems.at[21])
                 for c in range(8)]

    def ln_rstd(g, i, mean):
        acc, m = None, g + opaque()
        for r in range(8):
            d = X[i][m, pl.ds(128 * r, 128), :].reshape(16, 8, 128) - mean[None]
            v = (d * d).sum(0)
            acc = v if acc is None else acc + v
            if r < 7:
                yield _Step(50, [lambda acc=acc: acc], delay=3)
        rstd = jax.lax.rsqrt(_all_sublanes(acc, jnp.add, 0) * (1.0 / D) + EPS)
        yield _Step(50, delay=8)
        yield _Step(10, [lambda: rstd], delay=1)
        return rstd

    def fwd_block(g, i, name, needs, free=(), known=False):
        j, t = g + 4 * i, i
        UB, AB, PB, ubu, abu = temps[t]
        yield _Wait(*needs)
        if known:
            means, squares = STAT[4 * g + i, pl.ds(0, 8)], STAT[4 * g + i, pl.ds(8, 8)]
            mean = means.sum(0) * 0.125
            var = (squares.sum(0) + 128.0 * ((means - mean) ** 2).sum(0)) * (1.0 / D)
            rstd = jax.lax.rsqrt(var + EPS)
            yield _Step(50, delay=6)
        else:
            yield settle(X[i])
            acc, m = None, g + opaque()
            for r in range(8):
                v = X[i][m, pl.ds(128 * r, 128), :].reshape(16, 8, 128).sum(0)
                acc = v if acc is None else acc + v
                if r % 2:
                    yield _Step(35, [lambda acc=acc: acc], delay=7 if r == 7 else 3)
            mean = _all_sublanes(acc, jnp.add, 0) * (1.0 / D)
            rstd = yield from ln_rstd(g, i, mean)
        mean8, rstd = (jnp.concatenate([v, v], 0) for v in (mean * 8.0, rstd))
        z = opaque()
        for r in range(8):
            rows = pl.ds(16 * r, 16)
            x = [X[i][g + z, pl.ds(128 * b + 16 * r, 16), :] for b in range(8)]
            s = [x[b] + x[b + 4] for b in range(4)]
            d = [x[b] - x[b + 4] for b in range(4)]
            e, o = s[0] + s[2], s[1] + s[3]
            UB[0, rows, :] = ((e + o - mean8) * rstd).astype(BF16)
            UB[0, pl.ds(128 + 16 * r, 16), :] = ((e - o) * rstd).astype(BF16)
            t1, t2 = (d[1] - d[3]) * RSQ2, (d[1] + d[3]) * RSQ2
            u = {1: (d[0] + t1, d[2] + t2), 2: (s[0] - s[2], s[1] - s[3]), 3: (d[0] - t1, d[2] - t2)}
            yield _Step(34, [anchor(ubu)], delay=1)
            for k in (1, 2, 3):
                c, sn = twid[z + 2 * k - 2, rows, :] * rstd, twid[z + 2 * k - 1, rows, :] * rstd
                re, m = u[k]
                if k == 3:
                    ur, ui = re * c + m * sn, m * c - re * sn
                else:
                    ur, ui = re * c - m * sn, m * c + re * sn
                UB[0, pl.ds(256 * k + 16 * r, 16), :] = ur.astype(BF16)
                UB[0, pl.ds(256 * k + 128 + 16 * r, 16), :] = ui.astype(BF16)
                yield _Step(26, [anchor(ubu)], delay=1)
        yield settle(ubu)

        def d_forward(point):
            z = opaque()
            first = _iota(8, 0) == 0

            def stage(c):
                u = (M_C4 if c == 1 else M_R) + opaque()
                lhs = mat(u) if c % 4 else _bf(tied(lambda r: mats[u, pl.ds(r, 8), :], 8, point))
                v = _dot(lhs, _bf(ubu[z, pl.ds(64 * c, 64), :]))
                return [(v[32 * u:32 * u + 16], v[32 * u + 16:32 * u + 32]) for u in range(4)]

            def put(row, u, v, v0=None):
                if u == 0 and v0 is not None:
                    v = jnp.concatenate([jnp.where(first, v0, v[:8]), v[8:]], 0)
                AB[0, pl.ds(row + 16 * u, 16), :] = v.astype(BF16)

            for u, (p1, p2) in enumerate(stage(0)):
                put(0, u, p1)
                put(528, u, p2, 0.0)
                if u == 0:
                    put(512, 0, jnp.zeros_like(p2), p2[:8])
            for u, (p1, p2) in enumerate(stage(1)):
                put(256, u, p1)
                put(528 + 256, u, p2)
            for k in (1, 2, 3):
                for u, ((p1, p2), (q1, q2)) in enumerate(zip(stage(2 * k), stage(2 * k + 1))):
                    if k == 3:
                        pr, pi, mr, mi = p1 - q2, p2 + q1, p1 + q2, p2 - q1
                        pi0, mi0 = q1[:8], -q2[:8]
                    else:
                        pr, pi, mr, mi = p1 + q2, p2 - q1, p1 - q2, p2 + q1
                        pi0, mi0 = -q1[:8], q2[:8]
                    put(64 * k, u, pr, p1[:8])
                    put(64 * (8 - k), u, mr, p2[:8])
                    put(528 + 64 * k, u, pi, pi0)
                    put(528 + 64 * (8 - k), u, mi, mi0)
            return 190

        yield _Mat(d_forward)
        yield settle(abu)
        yield _Wait(*free)

        def s_forward(point):
            z = opaque()
            fa, fb = mat(M_FA + j + z), mat(M_FB + j + z)
            for r0, rn in ((0, 256), (256, 272)):
                lhs = abu[z, pl.ds(r0 // 2, rn // 2), :] if r0 else tied(
                    lambda r: abu[z, pl.ds(r, 8), :], 16, point)
                u = _dot(_bf(lhs), fa)
                v = _dot(_bf(abu[z, pl.ds(264 + r0 // 2, 128), :]), fb)
                re, m = u[:256] + v, u[:256] - v
                if r0:
                    re, m = (jnp.concatenate([a, u[256:264]], 0) for a in (re, m))
                rn = re.shape[0]
                edge = (_iota(rn, 1) & 63) == 0
                ZT[2 * i, pl.ds(r0, rn), :] = re
                ZT[2 * i + 1, pl.ds(r0, rn), :] = jnp.where(
                    edge, lane_vec(L_MU + j, rn) * m + lane_vec(L_NU + j, rn) * re, _mirror(m))
            return 400

        yield _Mat(s_forward)
        yield _Step(2, [anchor(ZT)], delay=SETTLE, marks=[name])

    def group_stage(g, name, needs, inverse):
        yield _Wait(*needs)

        def turn(z, k):
            if k == 0:
                return z
            c, s = rot[4 * g + k], rot[16 + 4 * g + k]
            if inverse:
                return z[0] * c - z[1] * s, z[1] * c + z[0] * s
            return z[0] * c + z[1] * s, z[1] * c - z[0] * s

        (src, a), (dst, b) = ((Z, 8 * g), (ZT, 0)) if inverse else ((ZT, opaque()), (Z, 8 * g))
        for r in range(65):
            if r % (16 if inverse else 64) == 0:
                yield hold(src, 2 * NB if inverse else 8)
            rows = pl.ds(8 * r, 8)
            z = [(src[a + 2 * i, rows, :], src[a + 2 * i + 1, rows, :]) for i in range(4)]
            if inverse:
                z = _radix4([turn(z[k], k) for k in range(4)], True)
            else:
                z = [turn(v, k) for k, v in enumerate(_radix4(z, False))]
            for i in range(4):
                dst[b + 2 * i, rows, :], dst[b + 2 * i + 1, rows, :] = z[i]
            yield _Step(35, [anchor(dst)], delay=1, marks=[name] if r == 64 else [])

    def spectral(row, size):
        rows = pl.ds(row, size)
        for k0 in range(4):
            z = _radix4([(Z[8 * g + 2 * k0, rows, :], Z[8 * g + 2 * k0 + 1, rows, :])
                         for g in range(4)], False)
            y = []
            for k1, (re, im) in enumerate(z):
                w = WS[k0 + 4 * k1, rows, :]
                wr = pltpu.bitcast(w << 16, F32)
                wi = pltpu.bitcast(w & np.uint32(0xFFFF0000), F32)
                y.append((re * wr - im * wi, re * wi + im * wr))
            y = _radix4(y, True)
            for g in range(4):
                Z[8 * g + 2 * k0, rows, :], Z[8 * g + 2 * k0 + 1, rows, :] = y[g]

    def spectral_rows(c2):
        for r in range(8):
            spectral(pl.multiple_of(128 * c2 + 16 * r, 16), 16)

    def inv_block(g, i, name, needs, n=None):
        j, t = g + 4 * i, i % 2
        UB, AB, PB, ubu, abu = temps[t]
        n = g if n is None else n
        z = opaque()
        yield _Wait(*needs)
        for r0, rn in _S_ROWS:
            if r0 == 0:
                yield hold(ZT, 8)
            re, im = ZT[z + 2 * i, pl.ds(r0, rn), :], ZT[z + 2 * i + 1, pl.ds(r0, rn), :]
            edge = (_iota(rn, 1) & 63) == 0
            rolled = _mirror(im)
            u = re + jnp.where(edge, lane_vec(L_KU + j, rn) * im, rolled)
            if r0 < 512:
                v = re - jnp.where(edge, lane_vec(L_KV + j, rn) * im, rolled)
                AB[0, pl.ds(r0, rn), :] = u.astype(BF16)
                AB[0, pl.ds(528 + r0, rn), :] = v.astype(BF16)
            else:
                AB[0, pl.ds(512, 16), :] = jnp.concatenate([u, jnp.zeros_like(u)], 0).astype(BF16)
            yield _Step(rn, [anchor(abu)], delay=1, marks=[("read", name)] if r0 == 512 else [])
        yield settle(abu, 4)

        def s_inverse(point):
            z = opaque()
            fa, fb = mat(M_FA + j + z), mat(M_FB + j + z)
            first = _iota(8, 0) == 0

            def put(row, v, v0=None):
                if v0 is not None:
                    v = jnp.concatenate([jnp.where(first, v0, v[:8]), v[8:]], 0)
                UB[0, pl.ds(row, 64), :] = v.astype(BF16)

            for k in range(4):
                lo, hi = 32 * k, 32 * (8 - k if k else 4)
                a = [abu[z, pl.ds(lo, 32), :], abu[z, pl.ds(hi, 32), :]] if k % 2 else [
                    tied(lambda r, o=o: abu[z, pl.ds(o + r, 8), :], 4, point) for o in (lo, hi)]
                if k == 0:
                    a.append(abu[z, pl.ds(256, 8), :])
                re = _dot_t(_bf(jnp.concatenate(a, 0)), fa)
                im = _dot_t(_bf(jnp.concatenate(
                    [abu[z, pl.ds(264 + lo, 32), :], abu[z, pl.ds(264 + hi, 32), :]], 0)), fb)
                pr, mr, pi, mi = re[:64], re[64:128], im[:64], im[64:]
                if k == 0:
                    put(0, pr)
                    put(64, pi, re[128:136])
                    put(128, mr)
                    put(192, mi)
                else:
                    put(256 * k, pr + mr, pr[:8])
                    put(256 * k + 64, pi + mi, mr[:8])
                    put(256 * k + 128, pi - mi, pi[:8])
                    put(256 * k + 192, mr - pr, -mi[:8])
            return 190

        yield _Mat(s_inverse)
        yield settle(ubu, 4)
        yield d_stage(t, lambda c: {0: M_R0T, 1: M_C4T}.get(c, M_RT))
        yield settle(PB, 4)
        z = opaque()
        acc = None
        for r in range(16):
            rows = pl.ds(8 * r, 8)
            t0, t4 = PB[z, rows, :], PB[z, pl.ds(128 + 8 * r, 8), :]
            tk = {}
            for k in (1, 2, 3):
                c, sn = twid[z + 2 * k - 2, rows, :], twid[z + 2 * k - 1, rows, :]
                re = PB[z, pl.ds(256 * k + 8 * r, 8), :]
                im = PB[z, pl.ds(256 * k + 128 + 8 * r, 8), :]
                tk[k] = (re * c - im * sn, re * sn + im * c)
            e0, e1 = t0 + t4, t0 - t4
            s = [e0 + tk[2][0], e1 - tk[2][1], e0 - tk[2][0], e1 + tk[2][1]]
            al, be = tk[1][0] - tk[3][0], tk[1][1] + tk[3][1]
            o = [tk[1][0] + tk[3][0], (al - be) * RSQ2, tk[3][1] - tk[1][1], (al + be) * -RSQ2]
            for b in range(8):
                y = s[b] + o[b] if b < 4 else s[b - 4] - o[b - 4]
                v = X[i][g, pl.ds(128 * b + 8 * r, 8), :] + y
                X[i][n, pl.ds(128 * b + 8 * r, 8), :] = v
                acc = v if acc is None else acc + v
            yield _Step(57, [lambda v=acc: v], delay=5 if r == 15 else 2)
        yield settle(X[i], 4)
        mean = _all_sublanes(acc, jnp.add, 0) * (1.0 / D)
        rstd = yield from ln_rstd(n, i, mean)
        z = opaque()
        for r in range(8):
            v = X[i][n + z, pl.ds(128 * r, 128), :].reshape(16, 8, 128)
            HB[i][n, pl.ds(128 * r, 128), :] = ((v - mean[None]) * rstd[None]).reshape(128, 128).astype(BF16)
            yield _Step(41, [anchor(hbu[i])], delay=1, marks=[name] if r == 7 else [])

    def attend(g, i, name, needs):
        yield _Wait(*needs)
        yield settle(QB[i])
        j, z = g + 4 * i, opaque()
        even = (_iota(8, 0) & 1) == 0
        edge = _iota(8, 1) == 0

        def window(near, far, w, rows):
            return near[j + z + 4 - 2 * w, rows, :] if w <= 2 * i + 2 else far[j + z + 16 - 2 * w, rows, :]

        def mix_values(h, u):
            p = PW[h % 2][opaque()]
            for rows in (pl.ds(256 * h + 16 * u, 16), pl.ds(256 * h + 16 * u + 16, 16)):
                acc = functools.reduce(jnp.add, [p[16 * w:16 * w + 16] * window(VE, VS, w, rows)
                                                 for w in range(8)])
                HB[i][g, rows, :] = acc.astype(BF16)
            return _Step(63, [anchor(hbu[i])], delay=2, marks=[name] if (h, u) == (3, 14) else [])

        for h in range(5):
            logits = []
            for w0 in range(0, 8, 2):
                if h < 4:
                    rows = pl.ds(256 * h, 256)
                    q = q if w0 % 4 else QB[i][opaque(), rows, :]
                    for w in (w0, w0 + 1):
                        v = (q * window(KE, KS, w, rows)).reshape(16, 16, 128).sum(0)
                        v = jnp.where(even, v[:8] + pltpu.roll(v[:8], 7, 0), v[8:] + pltpu.roll(v[8:], 1, 0))
                        logits.append(jnp.where(edge & (2 * w > j), -1e9, v * SCALE) if w > 2 * i
                                      else v * SCALE)
                    yield _Step(138, [lambda v=v: v for v in logits[-2:]], delay=4)
                if h > 0:
                    yield mix_values(h - 1, 2 * w0)
                    yield mix_values(h - 1, 2 * w0 + 2)
            if h < 4:
                top = functools.reduce(jnp.maximum, logits)
                e = [jnp.exp(v - top) for v in logits]
                total = functools.reduce(jnp.add, e)
                yield _Step(30, [lambda v=total: v], delay=3)
                scale = 1.0 / total
                for w in range(8):
                    v = e[w] * scale
                    PW[h % 2][0, pl.ds(16 * w, 8), :] = jnp.where(even, v, pltpu.roll(v, 1, 0))
                    PW[h % 2][0, pl.ds(16 * w + 8, 8), :] = jnp.where(even, pltpu.roll(v, 7, 0), v)
                yield _Step(50, [anchor(PW[h % 2])], delay=6 if h == 3 else 1)

    def packed_sums(terms, signs):
        lo = [pltpu.bitcast(u << 16, F32) for u in terms]
        hi = [pltpu.bitcast(u & np.uint32(0xFFFF0000), F32) for u in terms]
        return [pltpu.pack_elementwise([v[p] + v[q] if s > 0 else v[p] - v[q] for v in (lo, hi)],
                                       packed_dtype=BF16) for p, s, q in signs]

    def half(ref, row):
        return lambda r, size, cols: ref[pl.ds(pl.multiple_of(row + r, 8), size), cols]

    kv_weight = (WS5, half(WK, 0), half(WV, 0))
    q_weight = (WQ5, half(WQ, 0), half(WQ, D // 4))
    o_weight = (WP5, *(lambda r, size, cols, e=e: WP[pl.ds(r + r // 32 * 32 + e, size), cols]
                       for e in (0, 32)))

    def left_sums(weight, row, size, needs=()):
        yield _Wait(*needs)
        sums, top, bottom = weight
        for r in range(0, size, 8):
            a = [ref(row + r, 8, pl.ds(c, 512)) for ref in (top, bottom) for c in (0, 512)]
            for e, v in enumerate(packed_sums(a, ((0, 1, 3), (2, 1, 3), (0, 1, 1), (2, -1, 0), (1, -1, 3)))):
                sums[e, pl.ds(pl.multiple_of(row + r, 8), 8), :] = v
            yield _Step(92, [anchor(sums)], delay=2, marks=["sums"] if r == size - 8 else [])

    def right_sums(dst, g, i, name, needs):
        yield _Wait(*needs)
        z = g + opaque()
        for r in range(0, 256, 16):
            b = [hbu[n][z, pl.ds(k + r, 16), :] for k in (0, 256) for n in (i, i + 1)]
            for e, v in enumerate(packed_sums(b, ((0, 1, 3), (1, -1, 3), (2, -1, 0), (0, 1, 1), (2, 1, 3)))):
                dst[e, pl.ds(r, 16), :] = v
            yield _Step(47, [anchor(dst)], delay=SETTLE if r == 240 else 1,
                        marks=[name] if r == 240 else [])

    def strassen(sch, weight, right, g, i, m, store, needs, marks):
        for n in needs:
            sch.run(n)
        sums, top, bottom = weight
        rows = pl.ds(pl.multiple_of(64 * m, 64), 64)

        def product(left, b):
            sch.fresh = True
            head = tied(lambda r: left(32 * m + r, 8, pl.ds(0, 128)), 4, lambda: sch.point(8.0))
            return _dot(_bf(jnp.concatenate([head, left(32 * m, 32, pl.ds(128, 384))], 1)), _bf(b))

        def a(e):
            return lambda r, size, cols: sums[e, pl.ds(pl.multiple_of(r, 8), size), cols]

        def b(e):
            return right[e + opaque()]

        m2 = product(a(1), hbu[i][g + opaque(), pl.ds(0, 256), :])
        m4 = product(lambda r, size, cols: bottom(r, size, pl.ds(512 + cols.start, cols.size)), b(2))
        store(1, i, rows, m2 + m4)
        m1 = product(a(0), b(0))
        c11, c22 = m1 + m4, m1 - m2
        c11 = c11 + product(a(4), b(4))
        c22 = c22 + product(a(3), b(3))
        m5 = product(a(2), hbu[i + 1][g + opaque(), pl.ds(256, 256), :])
        store(0, i, rows, c11 - m5)
        v = product(top, b(1))
        store(0, i + 1, rows, v + m5)
        store(1, i + 1, rows, c22 + v)
        sch.results.append(v[:8])
        for name in marks:
            sch.done[name] = sch.slot + sch.wait

    def kv_proj(sch, g, i, name, needs):
        def store(lower, n, rows, v):
            (KE, VE)[lower][g + 4 * n + 4, rows, :] = v
        for m in range(16):
            strassen(sch, kv_weight, SB[i // 2], g, i, m, store, needs, [name] if m == 15 else [])

    def q_proj(sch, g, i, name, needs):
        def store(lower, n, rows, v):
            QB[n][0, pl.ds(512 * lower + rows.start, 64), :] = v
        for m in range(8):
            strassen(sch, q_weight, SB[i // 2], g, i, m, store, needs, [name] if m == 7 else [])

    def o_proj(sch, g, i, m, needs, marks, right):
        def store(lower, n, rows, v):
            rows = pl.ds(128 * m + 64 * lower, 64)
            X[n][g, rows, :] = X[n][g, rows, :] + v
        strassen(sch, o_weight, right, g, i, m, store, needs, marks)

    def shift_block(g, i, name, needs):
        yield _Wait(*needs)
        j, z = g + 4 * i, opaque()
        for m in range(16):
            rows = pl.ds(64 * m, 64)
            for ref, to in ((KE, KS), (VE, VS)):
                v = pltpu.roll(ref[j + 4 + z, rows, :], 1, 1)
                if ref is VE:
                    v = jnp.where(_iota(64, 1) == 0, ref[4 + z, rows, :], v)
                to[j, rows, :] = v
                if i == 3:
                    ref[g, rows, :] = v
            yield _Step(12, delay=8, marks=[name] if m == 15 else [])

    def transpose_quarter(w, h, via):
        for r in range(4):
            v = WRAW[w, pl.ds(256 * r, 256), pl.ds(pl.multiple_of(256 * h, 256), 256)]
            v = pltpu.bitcast(v.T, F32)
            via[0, pl.ds(256 * r, 128), :], via[0, pl.ds(256 * r + 128, 128), :] = v[:, :128], v[:, 128:]
            yield _Step(40, delay=16)

    def reorder_quarter(w, h, via, name=None):
        z = 0 if isinstance(h, int) else opaque()
        for c in range(8):
            WT[w][pl.ds(pl.multiple_of(128 * h, 128), 128), pl.ds(128 * c, 128)] = pltpu.bitcast(
                jnp.concatenate([via[z, pl.ds(128 * c + u, 8, stride=16), :] for u in range(16)], 0), U32)
            yield _Step(20, delay=4, marks=[name] if c == 7 else [])

    def query_weight(h):
        yield from transpose_quarter(0, h, QB[0])
        yield from reorder_quarter(0, h, QB[0], "w")

    def transpose_wo(name):
        for c in range(8):
            for h in range(4):
                v = jnp.concatenate([wou[c, pl.ds(128 * h + u, 8, stride=16), :] for u in range(16)], 0)
                WP[pl.ds(64 * c, 64), pl.ds(256 * h, 256)] = pltpu.bitcast(_bf(v).T, U32)
                yield _Step(20, delay=10, marks=[name] if c == 7 and h == 3 else [])

    def prep_spectral_weights(c2):
        def words(k2):
            re, im = (wsu[u, k2, pl.ds(c2, 64, stride=4), :] for u in range(2))
            return ((re & np.uint32(0xFFFF)) | (im << 16), (re >> 16) | (im & np.uint32(0xFFFF0000)))

        def arrange(w, below):
            return jnp.where(_iota(w.shape[0], 1) < 64, w, below)

        below = words(15)
        for k2 in range(16):
            here = words(k2)
            for e in range(2):
                cl = 2 * c2 + e
                w = arrange(here[e], below[e])
                WS[k2, pl.ds(64 * cl, 64), :] = pltpu.roll(w, 1, 0) if cl > 4 else w
            below = here
            yield _Step(90, delay=3)
        if c2 == 0:
            def nyquist(k2):
                re, im = (jnp.broadcast_to(WN[u, :, pl.ds(128 * k2, 128)].astype(F32), (8, 128))
                          for u in range(2))
                return pltpu.pack_elementwise([re, im], packed_dtype=BF16)
            for k2 in range(16):
                WS[k2, pl.ds(512, 8), :] = arrange(nyquist(k2), nyquist((k2 + 15) % 16))

    def write_out(p, c, name, needs):
        yield _Wait(*needs)
        rows = pl.ds(pl.multiple_of(128 * c, 128), 128)
        g, i = 2 * p % 4 + opaque(), p // 2
        w = pltpu.pack_elementwise([X[i][g, rows, :], X[i][g + 1, rows, :]], packed_dtype=BF16)
        xru[c, pl.ds(p, 128, stride=8), :] = w.T
        yield _Step(30, marks=[name])

    for c in range(8):
        x_copy(c).start()
    for c in range(5):
        mats[M_R + c] = d_mats[c]

    def make_twiddle(k):
        PB = temps[0][2]
        PB[0, pl.ds(0, 128), :] = lane_vec(L_TWID + k, 128)
        twid[k] = PB[opaque(), pl.ds(0, 128), :].T

    _loop(6, make_twiddle, "make_twiddle")

    def make_dft(j):
        fa, fb = lanes[pl.ds(L_FA, 128), :], lanes[pl.ds(L_FB, 128), :]
        c, sn = lane_vec(L_COS + j, 128), lane_vec(L_SIN + j, 128)
        UB, _, _, ubu, _ = temps[0]
        UB[0, pl.ds(0, 128), :] = (fa * c + fb * sn).astype(BF16)
        UB[0, pl.ds(128, 128), :] = (fb * c - fa * sn).astype(BF16)
        mats[M_FA + j], mats[M_FB + j] = ubu[0, pl.ds(0, 64), :], ubu[0, pl.ds(64, 64), :]

    _loop(NB, make_dft, "make_dft")

    def load_x(c):
        x_copy(c).wait()
        pl.when(c == 6)(lambda: start_all(spec_copies[0]))
        pl.when(c == 7)(lambda: start_all(spec_copies[1]))
        rows = pl.ds(pl.multiple_of(128 * c, 128), 128)
        for p in range(8):
            w = xru[c, pl.ds(p, 128, stride=8), :].T
            for e, bits in enumerate((w << 16, w & np.uint32(0xFFFF0000))):
                g, i = 2 * p % 4 + e, p // 2
                v = pltpu.bitcast(bits, F32)
                X[i][g, rows, :] = v
                v = v.reshape(16, 8, 128)
                mean = _all_sublanes(v.sum(0), jnp.add, 0) * (1.0 / 128)
                STAT[4 * g + i, c] = mean
                STAT[4 * g + i, 8 + c] = _all_sublanes(((v - mean) ** 2).sum(0), jnp.add, 0)

    _loop(8, load_x, "load_x")

    def after(name, action):
        yield _Wait(name)
        action()

    def spectral_weights():
        yield _Wait(("f", 2, 1))
        for c in spec_copies[0] + spec_copies[1]:
            c.wait()
        for c2 in range(4):
            yield from prep_spectral_weights(c2)

    with jax.named_scope("first_forward"):
        sch = _Sched(0.72, 20)
        sch.add(after(("f", 0, 1), w_copies[1].start), "k")
        sch.add(after(("f", 1, 1), w_copies[2].start), "v")
        sch.add(after(("f", 2, 3), w_copies[0].start), "q")
        for g in range(4):
            for i in range(4):
                sch.add(fwd_block(g, i, ("f", g, i), [("f", g - 1, i)] if g else [],
                                  [("r", g - 1)] if g else [], True), ("f", g, i))
            sch.add(group_stage(g, ("r", g), [("f", g, i) for i in range(4)], False), ("r", g))
        sch.add(spectral_weights(), "s")
        sch.drive()
    start_all(wo_copies)

    def keys_values(layer, g):
        sch = _Sched(0.41, 32, 3) if layer == 0 else _Sched(0.36, 28, 2)
        nxt = (g + 1) % 4
        sch.add(inv_block(g, 2, ("i", 2), []), ("i", 2))
        sch.add(inv_block(g, 3, ("i", 3), [("read", ("i", 2))]), ("i", 3))
        sch.add(right_sums(SB[1], g, 2, ("b", 2), [("i", 2), ("i", 3)]), ("b", 2))
        sch.add(group_stage(nxt, "r", [("read", ("i", 3))], True), "r")
        sch.add(inv_block(nxt, 0, ("i", 4), ["r", ("i", 2)], n=g + 1), ("i", 4))
        sch.add(inv_block(nxt, 1, ("i", 5), [("read", ("i", 4)), ("i", 3)], n=g + 1), ("i", 5))
        if layer == 0:
            sch.add(query_weight(g), "w")
            sch.add(left_sums(q_weight, 128 * (g % 2), 128, ["w"]), "sums")
        for i in (2, 3):
            sch.add(shift_block((g + 3) % 4, i, ("s", i), []), ("s", i))
        for i in (0, 1):
            sch.add(shift_block(g, i, ("s", i), [("kv", 0)]), ("s", i))
        sch.add(right_sums(SB[0], nxt, 0, ("b", 4), [("i", 4), ("i", 5), ("kv", 0)]), ("b", 4))
        kv_proj(sch, g, 0, ("kv", 0), [])
        kv_proj(sch, g, 2, ("kv", 2), [("b", 2)])
        sch.finish()

    def mix(g, after, last):
        tail = after is None
        sch = _Sched(0.66 if last else 0.63, 28 if last else 32)
        pace = 0.48 if tail else 0.35 if last else 0.32
        ahead = [(g, 2), (g, 3)] + ([] if tail else [(after, 0), (after, 1)])
        for n, block in enumerate(ahead):
            sch.add(attend(*block, ("a", n), [[], [("a", 0)], [("a", 1), ("q", 0)], [("a", 2)]][n]),
                    ("a", n), pace=pace)
            if n % 2:
                sch.add(right_sums(SB[2 + block[1] // 2], block[0], block[1] - 1, ("b", n),
                                   [("a", n)] + ([("o", 0)] if n == 3 else [])), ("b", n))
        for i in () if tail else (0, 2):
            sch.add(right_sums(SB[i // 2], after, i, ("h", i), [("q", 0)] if i else []), ("h", i))
        if not last:
            sch.add(group_stage((g + 3) % 4, "r", [], False), "r")
            for i in range(4):
                sch.add(fwd_block(g, i, ("f", i), [("o", i - i % 2)], ["r"]), ("f", i))
        now = 6 if last else 8
        for i in (0, 2):
            for m in range(now):
                o_proj(sch, g, i, m, [("b", 1)] if i else [], [("o", i)] if m == now - 1 else [],
                       SB[2 + i // 2])
            if not tail:
                q_proj(sch, after, i, ("q", i), [("h", i)])
        if tail:
            sch.add(group_stage(g, "s", [("f", i) for i in range(4)], False), "s")
        sch.share = 0.92
        sch.drive()

    def mix_odd():
        sch = _Sched(0.66)
        blocks = [(1, 2), (1, 3), (3, 0), (3, 1), (3, 2), (3, 3)]
        for n, (g, i) in enumerate(blocks):
            sch.add(attend(g, i, ("a", n), ([("a", n - 1)] if n else []) + ([("q", i)] if n in (2, 4) else [])),
                    ("a", n), pace=0.32)
            if n % 2:
                sch.add(right_sums(SB[(3, 2, 0)[n // 2]], g, i - 1, ("b", g, i - 1),
                                   [("a", n)] + ([("o", 1, 0, 5)] if n > 1 else [])), ("b", g, i - 1))
        for i in (0, 2):
            sch.add(right_sums(SB[i // 2], 3, i, ("h", i), []), ("h", i))
        for g in (1, 3):
            for i in range(4):
                for c in range(6):
                    sch.add(write_out(2 * i + g // 2, c, ("w", g, i, c), [("o", g, i - i % 2, c)]),
                            ("w", g, i, c))
        for g, i, slot, count in ((1, 0, 2, 6), (1, 2, 3, 8), (3, 0, 2, 8), (3, 2, 0, 6)):
            for m in range(count):
                o_proj(sch, g, i, m, [("b", g, i)] if (g, i) != (1, 0) else [], [("o", g, i, m)], SB[slot])
            for e in (0, 2) if (g, i) == (1, 0) else ():
                q_proj(sch, 3, e, ("q", e), [("h", e)] + ([("a", 1)] if e else []))
        sch.share = 0.92
        sch.drive()

    def copy_out(chunks):
        def start(_):
            for c in chunks:
                out_copy(c).start()
        _loop(zero + 1, start, "copy_out")

    def postponed():
        slots = {(3, 2): 0, (2, 2): 1, (0, 2): 2, (2, 0): 3, (0, 0): 0, (1, 0): 1}
        early, late = list(slots)[:2], list(slots)[2:]
        sources = 2 * [[(0, 0), (1, 0)], [(2, 0)]] + 2 * [[(0, 2)], []]
        for c in (6, 7):
            sch = _Sched(0.7, 12)
            for n, (pair, slot) in enumerate(slots.items()) if c == 6 else ():
                if n:
                    sch.add(right_sums(SB[slot], *pair, pair, [(early[n - 4], 7)] if n >= 4 else []), pair)
            for p in (5, 7, 4, 6, 1, 3, 0, 2):
                sch.add(write_out(p, c, ("w", p), [(pair, c) for pair in sources[p] or early * (c == 6)]),
                        ("w", p))
            for pair, m in [(pair, m) for m in (6, 7) for pair in early] * (c == 6) + [(v, c) for v in late]:
                o_proj(sch, *pair, m, [pair] if c == 6 and pair != (3, 2) else [], [(pair, m)],
                       SB[slots[pair]])
            sch.drive()
            copy_out([c])

    def first_queries(layer):
        sch = _Sched(0.68)
        sch.add(right_sums(SB[1], 0, 2, ("h", 2), []), ("h", 2))
        sch.add(shift_block(3, 2, "s", []), "s")
        sch.add(attend(0, 0, ("a", 0), ["q"]), ("a", 0), pace=0.4)
        sch.add(attend(0, 1, ("a", 1), [("a", 0)]), ("a", 1), pace=0.4)
        sch.add(right_sums(SB[2], 0, 0, "b", [("a", 1)]), "b")
        sch.add(shift_block(3, 3, "t", []), "t")
        if layer == 0:
            for c in wo_copies:
                c.wait()
            sch.add(transpose_wo("w"), "w")
            sch.add(left_sums(o_weight, 0, 256, ["w"]), "sums")
        q_proj(sch, 0, 0, "q", [])
        q_proj(sch, 0, 2, None, [("h", 2)])
        sch.finish()

    def key_value_weights():
        w_copies[1].wait()
        w_copies[2].wait()
        for h in range(6):
            work = []
            for w in (1, 2):
                if h < 4:
                    work.append(transpose_quarter(w, h, QB[2 * (h % 2) + w - 1]))
                if 0 < h < 5:
                    work.append(reorder_quarter(w, h - 1, QB[2 * ((h - 1) % 2) + w - 1]))
            if h > 1:
                work.append(left_sums(kv_weight, 128 * (h - 2), 128))
            list(itertools.zip_longest(*work))

    for layer in range(2):
        with jax.named_scope("spectral"):
            _loop(4, spectral_rows, "rows")
            if layer == 0:
                _loop(zero + 1, lambda _: key_value_weights(), "weights")
            spectral(512, 8)
        sch = _Sched(0.92)
        sch.add(group_stage(0, "r", [], True), "r")
        sch.add(inv_block(0, 0, ("i", 0), ["r"]), ("i", 0))
        sch.add(inv_block(0, 1, ("i", 1), ["r"]), ("i", 1))
        sch.add(right_sums(SB[0], 0, 0, "b", [("i", 0), ("i", 1)]), "b")
        sch.drive()
        if layer == 0:
            w_copies[0].wait()
        _loop(4, lambda g: keys_values(layer, g), "keys_values")
        first_queries(layer)
        if layer == 0:
            pl.when(never)(lambda: spectral_rows(0))
        if layer == 0:
            _loop(3, lambda g: mix(g, g + 1, False), "mix")
            mix(3, None, False)
        else:
            _loop(2, lambda u: mix(2 * u, 2 - u, True), "mix")
            mix_odd()
    copy_out(range(6))
    postponed()
    for c in range(8):
        out_copy(c).wait()


@jax.jit
def pallas_interleave_layers__spectral_gfnet__sliding_local_dilated__prompt_kernel(
    A_x: jax.Array,
    A_w_r: jax.Array,
    A_w_i: jax.Array,
    B_x: jax.Array,
    B_wqkv: jax.Array,
    B_wo: jax.Array,
):
    del B_x
    hbm = pl.BlockSpec(memory_space=pl.ANY)
    smem = pl.BlockSpec(memory_space=pltpu.SMEM)
    out = pl.pallas_call(
        _kernel,
        out_shape=jax.ShapeDtypeStruct((S, D), BF16),
        in_specs=[smem, smem, pl.BlockSpec(), pl.BlockSpec(), hbm, hbm, hbm, hbm, hbm],
        out_specs=hbm,
        scratch_shapes=[
            pltpu.VMEM((37, 64, 128), U32),
            pltpu.VMEM((6, 128, 128), F32),
            pltpu.VMEM((NB, 16, 8, 128), F32),
            pltpu.VMEM((NB + 4, D, 128), F32),
            pltpu.VMEM((NB + 4, D, 128), F32),
            pltpu.VMEM((NB, D, 128), F32),
            pltpu.VMEM((NB, D, 128), F32),
            pltpu.VMEM((2 * NB + 1, ZR, 128), F32),
            pltpu.VMEM((9, ZR, 128), F32),
            pltpu.VMEM((NB, ZR, 128), U32),
            *4 * [pltpu.VMEM((D // 2, D), U32)],
            pltpu.VMEM((5, D // 2, D // 2), U32),
            *2 * [pltpu.VMEM((5, D // 4, D // 2), U32)],
            *4 * [pltpu.VMEM((5, D // 4, 128), U32)],
            pltpu.VMEM((8, S, 128), BF16),
            pltpu.VMEM((2, NB, D // 2, 128), BF16),
            pltpu.VMEM((2, 1, S), BF16),
            pltpu.VMEM((3, D, D), BF16),
            pltpu.VMEM((8, D, 128), BF16),
            pltpu.VMEM((1, 128, 128), F32),
            pltpu.VMEM((1, 128, 128), F32),
            pltpu.SemaphoreType.DMA((24,)),
            *2 * [pltpu.VMEM((1, D, 128), F32)],
        ] + 4 * [
            pltpu.VMEM((5, D, 128), F32),
            pltpu.VMEM((5, D, 128), BF16),
            pltpu.VMEM((1, D, 128), F32),
            pltpu.VMEM((1, D, 128), BF16),
            pltpu.VMEM((1, 1152, 128), BF16),
        ],
        compiler_params=pltpu.CompilerParams(vmem_limit_bytes=126 * 2 ** 20),
    )(_ZERO, _ROT, _MATS, _LANES, A_x.reshape(S, D), A_w_r.T, A_w_i.T, B_wqkv, B_wo)
    return out.reshape(1, S, D)
```

```python
import functools
import itertools

import numpy as np

import jax
import jax.numpy as jnp
import jax.experimental.pallas as pl
import jax.experimental.pallas.tpu as pltpu

S, D, NB = 2048, 1024, 16
ZR = 576
F32, BF16, U32, I32 = jnp.float32, jnp.bfloat16, jnp.uint32, jnp.int32
EPS = 1e-5
SCALE = 32 ** -0.5
RSQ2 = float(np.sqrt(0.5))
SETTLE = 6

_S_ROWS = [(32 * u, 32) for u in range(16)] + [(512, 8)]

M_FA, M_FB, M_R, M_C4, M_RT, M_C4T, M_R0T = 0, 16, 32, 33, 34, 35, 36
L_MU, L_NU, L_KU, L_KV, L_COS, L_SIN, L_TWID, L_FA, L_FB = 0, 16, 32, 48, 64, 80, 96, 104, 232


def _bf16_bits(a):
    u = np.ascontiguousarray(a, dtype=np.float32).view(np.uint32).astype(np.uint64)
    return ((u + 0x7FFF + ((u >> 16) & 1)) >> 16).astype(np.uint32)


def _constants():
    a = np.arange(128)
    k1 = np.arange(64)
    alt = (-1.0) ** a
    lanes = np.zeros((384, 128))
    t = 2 * np.pi * np.outer(a, k1) / 128
    fa = np.concatenate([np.cos(t), -np.sin(t)], 1)
    fb = np.concatenate([np.sin(t), -np.cos(t)], 1)
    fa[:, 0], fb[:, 0] = RSQ2, -RSQ2
    fa[:, 64], fb[:, 64] = alt, 0.0
    lanes[L_FA:L_FA + 128], lanes[L_FB:L_FB + 128] = fa, fb
    for j in range(NB):
        ang = 2 * np.pi * j / 32 + np.pi / 32
        p, q = (_bf16_bits([np.cos(ang), np.sin(ang)]) << 16).view(np.float32).astype(np.float64)
        turn = 2 * np.pi * j * np.tile(k1, 2) / S
        lanes[L_COS + j], lanes[L_SIN + j] = np.cos(turn), np.repeat([-1.0, 1.0], 64) * np.sin(turn)
        lanes[L_COS + j, 64], lanes[L_SIN + j, 64] = p, q
        lanes[L_MU + j, 0], lanes[L_MU + j, 64] = 1.0, (q / p + p / q) / 2
        lanes[L_NU + j, 0], lanes[L_NU + j, 64] = 0.0, (q / p - p / q) / 2
        lanes[L_KU + j, 0], lanes[L_KU + j, 64] = 1.0, q / p
        lanes[L_KV + j, 0], lanes[L_KV + j, 64] = 1.0, p / q
    lanes[:, 65:] = lanes[:, :64:-1].copy()
    for k in (1, 2, 3):
        lanes[L_TWID + 2 * k - 2] = np.cos(2 * np.pi * a * k / D)
        lanes[L_TWID + 2 * k - 1] = np.sin(2 * np.pi * a * k / D)
    th = 2 * np.pi * np.outer(k1, a) / 128
    r = np.concatenate([np.cos(th), -np.sin(th)], 0)
    r[64] = alt
    th = 2 * np.pi * np.outer(2 * k1 + 1, a) / 256
    c4 = np.concatenate([np.cos(th), -np.sin(th)], 0)
    inv = 2.0 / (S * D)
    r0t = inv * r.T
    r0t[:, 0::64] *= 0.5
    rows = np.arange(128).reshape(2, 4, 16).transpose(1, 0, 2).ravel()
    bits = _bf16_bits(np.stack([r[rows], c4[rows], inv * r.T, inv * c4.T, r0t]))
    ang = 2 * np.pi * np.outer(np.arange(4), np.arange(4)).ravel() / 16
    rot = np.concatenate([np.cos(ang), np.sin(ang)]).astype(np.float32)
    return bits[:, 0::2] | (bits[:, 1::2] << 16), lanes.astype(np.float32), rot


_MATS, _LANES, _ROT = _constants()
_ZERO = np.zeros((1,), np.int32)


class _Step:
    def __init__(self, cost, anchors=(), delay=0, marks=()):
        self.cost, self.anchors, self.delay, self.marks = cost, list(anchors), delay, list(marks)


class _Wait:
    def __init__(self, *names):
        self.names = names


class _Mat:
    def __init__(self, emit):
        self.emit = emit


class _Hold:
    def __init__(self, store):
        self.store = store


class _Task:
    def __init__(self, gen, pace):
        self.gen, self.pace, self.blocked, self.not_before, self.held = gen, pace, (), 0, None
        self.allowed = 0.0


class _Sched:
    def __init__(self, share=0.0, wait=28, lag=3):
        self.lag = lag
        self.wait = wait
        self.share = share
        self.tasks, self.done, self.producer = [], {}, {}
        self.slot, self.credit, self.anchors, self.results = 0, 0.0, [], []
        self.fresh = False

    def add(self, gen, name, pace=99):
        self.producer[name] = self.producer["read", name] = _Task(gen, pace)
        self.tasks.append(self.producer[name])

    def _ready(self, t):
        return t.not_before <= self.slot and all(
            n in self.done and self.done[n] <= self.slot for n in t.blocked)

    def _advance(self, t, mats=True):
        item, t.held = t.held or next(t.gen, None), None
        if item is None:
            self.tasks.remove(t)
        elif isinstance(item, _Wait):
            t.blocked = item.names
        elif isinstance(item, _Hold):
            if len(self.results) >= self.lag:
                item.store(self.results[-self.lag])
        elif isinstance(item, _Mat):
            if mats:
                t.not_before = float("inf")
                self.fresh = False
                self.credit -= item.emit(lambda: self.point(0.0)) or 0
                t.not_before = self.slot + self.wait
            else:
                t.held, t.not_before = item, self.slot + 1
        else:
            t.blocked = ()
            t.not_before = self.slot + item.delay
            self.credit -= item.cost
            self.anchors += item.anchors
            for n in item.marks:
                self.done[n] = self.slot + item.delay
            return True

    def run(self, *names):
        while not all(n in self.done for n in names):
            for n in names:
                if n not in self.done:
                    for b in self.producer[n].blocked:
                        self.run(b)
                    self._advance(self.producer[n])

    def drive(self):
        while self.tasks:
            ready = [t for t in self.tasks if self._ready(t)]
            if not ready:
                self.slot += 1
                continue
            self.anchors, self.credit = self.anchors[-2:], 0.0
            self._advance(next((t for t in ready if t.held), ready[0]))
            self.slot -= min(self.credit, 0.0) / 60

    def finish(self):
        self.run(*[n for n in self.producer if n[0] != "read"])

    def point(self, own):
        for t in self.tasks:
            t.allowed = min(t.allowed, 0.0) + t.pace
        while True:
            t = next((t for t in self.tasks if self._ready(t) and t.allowed > 0
                      and self.credit > 0), None)
            if t is None:
                break
            if self._advance(t, self.fresh):
                t.allowed -= 1
        anchors, self.anchors = self.anchors, []
        self.credit = min(self.credit, 10.0) + 64 * self.share - own
        self.fresh = False
        self.slot += 1
        return anchors


def _dot(a, b):
    return jnp.dot(a, b, preferred_element_type=F32)


def _dot_t(a, b):
    return jax.lax.dot_general(a, b, (((1,), (1,)), ((), ())), preferred_element_type=F32)


def _bf(u):
    return pltpu.bitcast(u, BF16)


def _iota(rows, dim):
    return jax.lax.broadcasted_iota(I32, (rows, 128), dim)


def _mirror(v):
    index = -_iota(8, 1) & 127
    return jnp.concatenate([jnp.take_along_axis(v[r:r + 8], index, axis=1)
                            for r in range(0, v.shape[0], 8)], 0)


def _radix4(z, inverse):
    (r0, i0), (r1, i1), (r2, i2), (r3, i3) = z
    ar, ai, cr, ci = r0 + r2, i0 + i2, r0 - r2, i0 - i2
    br, bi, dr, di = r1 + r3, i1 + i3, r1 - r3, i1 - i3
    lo, hi = (cr + di, ci - dr), (cr - di, ci + dr)
    if inverse:
        lo, hi = hi, lo
    return [(ar + br, ai + bi), lo, (ar - br, ai - bi), hi]


def _all_sublanes(v, op, axis):
    for sh in (4, 2, 1):
        v = op(v, pltpu.roll(v, sh, axis))
    return v


def _loop(n, body, name):
    def step(i, carry):
        body(i)
        return carry
    with jax.named_scope(name):
        jax.lax.fori_loop(0, n, step, 0)


def _kernel(zero_ref, rot, mats_hbm, lanes_hbm, x_hbm, wr_hbm, wi_hbm, wqkv_hbm, wo_hbm, out_hbm,
            lanes, mats, twid, STAT, KE, VE, KS, VS, Z, ZT, WS, WQ, WK, WV, WP, WS5, WQ5, WP5,
            SB0, SB1, SB2, SB3, XR, WRI, WN, WRAW, WO, PW0, PW1, sems, *split):
    zero = zero_ref[0]
    never = zero != 0
    X, HB, QB = split[2::5], split[3::5], split[4::5]
    hbu = [r.bitcast(U32) for r in HB]
    xru, wsu, wou = XR.bitcast(U32), WRI.bitcast(U32), WO.bitcast(U32)
    temps = [(ub, ab, pb, ub.bitcast(U32), ab.bitcast(U32))
             for ub, ab, pb in zip(split[5::5], split[6::5], 2 * split[:2])]
    PW, SB, WT = (PW0, PW1), (SB0, SB1, SB2, SB3), (WQ, WK, WV, WP)
    counter = [0]

    def opaque():
        counter[0] += 1
        return zero * counter[0]

    def anchor(ref):
        at = (0,) * (len(ref.shape) - 2)
        return lambda: ref[(*at, pl.ds(pl.multiple_of(zero * 8, 8), 8), pl.ds(0, 128))]

    def settle(ref, points=SETTLE):
        return _Step(2, [anchor(ref)], delay=points)

    def hold(ref, spare):
        def store(v):
            ref[spare, pl.ds(pl.multiple_of(zero * 8, 8), 8), :] = v
        return _Hold(store)

    def tied(load, vregs, point):
        parts = []
        for r in range(vregs):
            anchors = point()
            u = load(8 * r)
            for a in anchors:
                u = jnp.where(never, pltpu.bitcast(a(), U32), u)
            parts.append(u)
        return jnp.concatenate(parts, 0)

    def mat(i):
        return _bf(mats[i])

    def d_stage(t, which):
        UB, AB, PB, ubu, abu = temps[t]

        def emit(point):
            z = opaque()
            for c in range(8):
                lhs = mat(which(c) + opaque()) if c % 4 else _bf(
                    tied(lambda r, u=which(c) + opaque(): mats[u, pl.ds(r, 8), :], 8, point))
                PB[0, pl.ds(128 * c, 128), :] = _dot(lhs, _bf(ubu[z, pl.ds(64 * c, 64), :]))
        return _Mat(emit)

    def lane_vec(i, rows):
        return jnp.broadcast_to(lanes[pl.ds(i, 1), :], (rows, 128))

    def x_copy(c):
        return pltpu.make_async_copy(
            x_hbm.at[:, pl.ds(pl.multiple_of(128 * c, 128), 128)], XR.at[c], sems.at[c])

    def out_copy(c):
        return pltpu.make_async_copy(
            XR.at[c], out_hbm.at[:, pl.ds(pl.multiple_of(128 * c, 128), 128)], sems.at[8 + c])

    spec_copies = [[pltpu.make_async_copy(w.at[pl.ds(0, 512), pl.ds(128 * k2, 128)], WRI.at[u, k2],
                                          sems.at[16 + u]) for k2 in range(16)]
                   + [pltpu.make_async_copy(w.at[pl.ds(512, 1), :], WN.at[u], sems.at[22 + u])]
                   for u, w in enumerate((wr_hbm, wi_hbm))]

    def start_all(copies):
        for c in copies:
            c.start()
    w_copies = [pltpu.make_async_copy(wqkv_hbm.at[:, pl.ds(D * w, D)], WRAW.at[w], sems.at[18 + w])
                for w in range(3)]
    wo_copies = [pltpu.make_async_copy(wo_hbm.at[:, pl.ds(128 * c, 128)], WO.at[c], sems.at[21])
                 for c in range(8)]

    def ln_rstd(g, i, mean):
        acc, m = None, g + opaque()
        for r in range(8):
            d = X[i][m, pl.ds(128 * r, 128), :].reshape(16, 8, 128) - mean[None]
            v = (d * d).sum(0)
            acc = v if acc is None else acc + v
            if r < 7:
                yield _Step(50, [lambda acc=acc: acc], delay=3)
        rstd = jax.lax.rsqrt(_all_sublanes(acc, jnp.add, 0) * (1.0 / D) + EPS)
        yield _Step(50, delay=8)
        yield _Step(10, [lambda: rstd], delay=1)
        return rstd

    def fwd_block(g, i, name, needs, free=(), known=False):
        j, t = g + 4 * i, i
        UB, AB, PB, ubu, abu = temps[t]
        yield _Wait(*needs)
        if known:
            means, squares = STAT[4 * g + i, pl.ds(0, 8)], STAT[4 * g + i, pl.ds(8, 8)]
            mean = means.sum(0) * 0.125
            var = (squares.sum(0) + 128.0 * ((means - mean) ** 2).sum(0)) * (1.0 / D)
            rstd = jax.lax.rsqrt(var + EPS)
            yield _Step(50, delay=6)
        else:
            yield settle(X[i])
            acc, m = None, g + opaque()
            for r in range(8):
                v = X[i][m, pl.ds(128 * r, 128), :].reshape(16, 8, 128).sum(0)
                acc = v if acc is None else acc + v
                if r % 2:
                    yield _Step(35, [lambda acc=acc: acc], delay=7 if r == 7 else 3)
            mean = _all_sublanes(acc, jnp.add, 0) * (1.0 / D)
            rstd = yield from ln_rstd(g, i, mean)
        mean8, rstd = (jnp.concatenate([v, v], 0) for v in (mean * 8.0, rstd))
        z = opaque()
        for r in range(8):
            rows = pl.ds(16 * r, 16)
            x = [X[i][g + z, pl.ds(128 * b + 16 * r, 16), :] for b in range(8)]
            s = [x[b] + x[b + 4] for b in range(4)]
            d = [x[b] - x[b + 4] for b in range(4)]
            e, o = s[0] + s[2], s[1] + s[3]
            UB[0, rows, :] = ((e + o - mean8) * rstd).astype(BF16)
            UB[0, pl.ds(128 + 16 * r, 16), :] = ((e - o) * rstd).astype(BF16)
            t1, t2 = (d[1] - d[3]) * RSQ2, (d[1] + d[3]) * RSQ2
            u = {1: (d[0] + t1, d[2] + t2), 2: (s[0] - s[2], s[1] - s[3]), 3: (d[0] - t1, d[2] - t2)}
            yield _Step(34, [anchor(ubu)], delay=1)
            for k in (1, 2, 3):
                c, sn = twid[z + 2 * k - 2, rows, :] * rstd, twid[z + 2 * k - 1, rows, :] * rstd
                re, m = u[k]
                if k == 3:
                    ur, ui = re * c + m * sn, m * c - re * sn
                else:
                    ur, ui = re * c - m * sn, m * c + re * sn
                UB[0, pl.ds(256 * k + 16 * r, 16), :] = ur.astype(BF16)
                UB[0, pl.ds(256 * k + 128 + 16 * r, 16), :] = ui.astype(BF16)
                yield _Step(26, [anchor(ubu)], delay=1)
        yield settle(ubu)

        def d_forward(point):
            z = opaque()
            first = _iota(8, 0) == 0

            def stage(c):
                u = (M_C4 if c == 1 else M_R) + opaque()
                lhs = mat(u) if c % 4 else _bf(tied(lambda r: mats[u, pl.ds(r, 8), :], 8, point))
                v = _dot(lhs, _bf(ubu[z, pl.ds(64 * c, 64), :]))
                return [(v[32 * u:32 * u + 16], v[32 * u + 16:32 * u + 32]) for u in range(4)]

            def put(row, u, v, v0=None):
                if u == 0 and v0 is not None:
                    v = jnp.concatenate([jnp.where(first, v0, v[:8]), v[8:]], 0)
                AB[0, pl.ds(row + 16 * u, 16), :] = v.astype(BF16)

            for u, (p1, p2) in enumerate(stage(0)):
                put(0, u, p1)
                put(528, u, p2, 0.0)
                if u == 0:
                    put(512, 0, jnp.zeros_like(p2), p2[:8])
            for u, (p1, p2) in enumerate(stage(1)):
                put(256, u, p1)
                put(528 + 256, u, p2)
            for k in (1, 2, 3):
                for u, ((p1, p2), (q1, q2)) in enumerate(zip(stage(2 * k), stage(2 * k + 1))):
                    if k == 3:
                        pr, pi, mr, mi = p1 - q2, p2 + q1, p1 + q2, p2 - q1
                        pi0, mi0 = q1[:8], -q2[:8]
                    else:
                        pr, pi, mr, mi = p1 + q2, p2 - q1, p1 - q2, p2 + q1
                        pi0, mi0 = -q1[:8], q2[:8]
                    put(64 * k, u, pr, p1[:8])
                    put(64 * (8 - k), u, mr, p2[:8])
                    put(528 + 64 * k, u, pi, pi0)
                    put(528 + 64 * (8 - k), u, mi, mi0)
            return 190

        yield _Mat(d_forward)
        yield settle(abu)
        yield _Wait(*free)

        def s_forward(point):
            z = opaque()
            fa, fb = mat(M_FA + j + z), mat(M_FB + j + z)
            for r0, rn in ((0, 256), (256, 272)):
                lhs = abu[z, pl.ds(r0 // 2, rn // 2), :] if r0 else tied(
                    lambda r: abu[z, pl.ds(r, 8), :], 16, point)
                u = _dot(_bf(lhs), fa)
                v = _dot(_bf(abu[z, pl.ds(264 + r0 // 2, 128), :]), fb)
                re, m = u[:256] + v, u[:256] - v
                if r0:
                    re, m = (jnp.concatenate([a, u[256:264]], 0) for a in (re, m))
                rn = re.shape[0]
                edge = (_iota(rn, 1) & 63) == 0
                ZT[2 * i, pl.ds(r0, rn), :] = re
                ZT[2 * i + 1, pl.ds(r0, rn), :] = jnp.where(
                    edge, lane_vec(L_MU + j, rn) * m + lane_vec(L_NU + j, rn) * re, _mirror(m))
            return 400

        yield _Mat(s_forward)
        yield _Step(2, [anchor(ZT)], delay=SETTLE, marks=[name])

    def group_stage(g, name, needs, inverse):
        yield _Wait(*needs)

        def turn(z, k):
            if k == 0:
                return z
            c, s = rot[4 * g + k], rot[16 + 4 * g + k]
            if inverse:
                return z[0] * c - z[1] * s, z[1] * c + z[0] * s
            return z[0] * c + z[1] * s, z[1] * c - z[0] * s

        (src, a), (dst, b) = ((Z, 8 * g), (ZT, 0)) if inverse else ((ZT, opaque()), (Z, 8 * g))
        for r in range(65):
            if r % (16 if inverse else 64) == 0:
                yield hold(src, 2 * NB if inverse else 8)
            rows = pl.ds(8 * r, 8)
            z = [(src[a + 2 * i, rows, :], src[a + 2 * i + 1, rows, :]) for i in range(4)]
            if inverse:
                z = _radix4([turn(z[k], k) for k in range(4)], True)
            else:
                z = [turn(v, k) for k, v in enumerate(_radix4(z, False))]
            for i in range(4):
                dst[b + 2 * i, rows, :], dst[b + 2 * i + 1, rows, :] = z[i]
            yield _Step(35, [anchor(dst)], delay=1, marks=[name] if r == 64 else [])

    def spectral(row, size):
        rows = pl.ds(row, size)
        for k0 in range(4):
            z = _radix4([(Z[8 * g + 2 * k0, rows, :], Z[8 * g + 2 * k0 + 1, rows, :])
                         for g in range(4)], False)
            y = []
            for k1, (re, im) in enumerate(z):
                w = WS[k0 + 4 * k1, rows, :]
                wr = pltpu.bitcast(w << 16, F32)
                wi = pltpu.bitcast(w & np.uint32(0xFFFF0000), F32)
                y.append((re * wr - im * wi, re * wi + im * wr))
            y = _radix4(y, True)
            for g in range(4):
                Z[8 * g + 2 * k0, rows, :], Z[8 * g + 2 * k0 + 1, rows, :] = y[g]

    def spectral_rows(c2):
        for r in range(8):
            spectral(pl.multiple_of(128 * c2 + 16 * r, 16), 16)

    def inv_block(g, i, name, needs, n=None):
        j, t = g + 4 * i, i % 2
        UB, AB, PB, ubu, abu = temps[t]
        n = g if n is None else n
        z = opaque()
        yield _Wait(*needs)
        for r0, rn in _S_ROWS:
            if r0 == 0:
                yield hold(ZT, 8)
            re, im = ZT[z + 2 * i, pl.ds(r0, rn), :], ZT[z + 2 * i + 1, pl.ds(r0, rn), :]
            edge = (_iota(rn, 1) & 63) == 0
            rolled = _mirror(im)
            u = re + jnp.where(edge, lane_vec(L_KU + j, rn) * im, rolled)
            if r0 < 512:
                v = re - jnp.where(edge, lane_vec(L_KV + j, rn) * im, rolled)
                AB[0, pl.ds(r0, rn), :] = u.astype(BF16)
                AB[0, pl.ds(528 + r0, rn), :] = v.astype(BF16)
            else:
                AB[0, pl.ds(512, 16), :] = jnp.concatenate([u, jnp.zeros_like(u)], 0).astype(BF16)
            yield _Step(rn, [anchor(abu)], delay=1, marks=[("read", name)] if r0 == 512 else [])
        yield settle(abu, 4)

        def s_inverse(point):
            z = opaque()
            fa, fb = mat(M_FA + j + z), mat(M_FB + j + z)
            first = _iota(8, 0) == 0

            def put(row, v, v0=None):
                if v0 is not None:
                    v = jnp.concatenate([jnp.where(first, v0, v[:8]), v[8:]], 0)
                UB[0, pl.ds(row, 64), :] = v.astype(BF16)

            for k in range(4):
                lo, hi = 32 * k, 32 * (8 - k if k else 4)
                a = [abu[z, pl.ds(lo, 32), :], abu[z, pl.ds(hi, 32), :]] if k % 2 else [
                    tied(lambda r, o=o: abu[z, pl.ds(o + r, 8), :], 4, point) for o in (lo, hi)]
                if k == 0:
                    a.append(abu[z, pl.ds(256, 8), :])
                re = _dot_t(_bf(jnp.concatenate(a, 0)), fa)
                im = _dot_t(_bf(jnp.concatenate(
                    [abu[z, pl.ds(264 + lo, 32), :], abu[z, pl.ds(264 + hi, 32), :]], 0)), fb)
                pr, mr, pi, mi = re[:64], re[64:128], im[:64], im[64:]
                if k == 0:
                    put(0, pr)
                    put(64, pi, re[128:136])
                    put(128, mr)
                    put(192, mi)
                else:
                    put(256 * k, pr + mr, pr[:8])
                    put(256 * k + 64, pi + mi, mr[:8])
                    put(256 * k + 128, pi - mi, pi[:8])
                    put(256 * k + 192, mr - pr, -mi[:8])
            return 190

        yield _Mat(s_inverse)
        yield settle(ubu, 4)
        yield d_stage(t, lambda c: {0: M_R0T, 1: M_C4T}.get(c, M_RT))
        yield settle(PB, 4)
        z = opaque()
        acc = None
        for r in range(16):
            rows = pl.ds(8 * r, 8)
            t0, t4 = PB[z, rows, :], PB[z, pl.ds(128 + 8 * r, 8), :]
            tk = {}
            for k in (1, 2, 3):
                c, sn = twid[z + 2 * k - 2, rows, :], twid[z + 2 * k - 1, rows, :]
                re = PB[z, pl.ds(256 * k + 8 * r, 8), :]
                im = PB[z, pl.ds(256 * k + 128 + 8 * r, 8), :]
                tk[k] = (re * c - im * sn, re * sn + im * c)
            e0, e1 = t0 + t4, t0 - t4
            s = [e0 + tk[2][0], e1 - tk[2][1], e0 - tk[2][0], e1 + tk[2][1]]
            al, be = tk[1][0] - tk[3][0], tk[1][1] + tk[3][1]
            o = [tk[1][0] + tk[3][0], (al - be) * RSQ2, tk[3][1] - tk[1][1], (al + be) * -RSQ2]
            for b in range(8):
                y = s[b] + o[b] if b < 4 else s[b - 4] - o[b - 4]
                v = X[i][g, pl.ds(128 * b + 8 * r, 8), :] + y
                X[i][n, pl.ds(128 * b + 8 * r, 8), :] = v
                acc = v if acc is None else acc + v
            yield _Step(57, [lambda v=acc: v], delay=5 if r == 15 else 2)
        yield settle(X[i], 4)
        mean = _all_sublanes(acc, jnp.add, 0) * (1.0 / D)
        rstd = yield from ln_rstd(n, i, mean)
        z = opaque()
        for r in range(8):
            v = X[i][n + z, pl.ds(128 * r, 128), :].reshape(16, 8, 128)
            HB[i][n, pl.ds(128 * r, 128), :] = ((v - mean[None]) * rstd[None]).reshape(128, 128).astype(BF16)
            yield _Step(41, [anchor(hbu[i])], delay=1, marks=[name] if r == 7 else [])

    def attend(g, i, name, needs):
        yield _Wait(*needs)
        yield settle(QB[i])
        j, z = g + 4 * i, opaque()
        even = (_iota(8, 0) & 1) == 0
        edge = _iota(8, 1) == 0

        def window(near, far, w, rows):
            return near[j + z + 4 - 2 * w, rows, :] if w <= 2 * i + 2 else far[j + z + 16 - 2 * w, rows, :]

        def mix_values(h, u):
            p = PW[h % 2][opaque()]
            for rows in (pl.ds(256 * h + 16 * u, 16), pl.ds(256 * h + 16 * u + 16, 16)):
                acc = functools.reduce(jnp.add, [p[16 * w:16 * w + 16] * window(VE, VS, w, rows)
                                                 for w in range(8)])
                HB[i][g, rows, :] = acc.astype(BF16)
            return _Step(63, [anchor(hbu[i])], delay=2, marks=[name] if (h, u) == (3, 14) else [])

        for h in range(5):
            logits = []
            for w0 in range(0, 8, 2):
                if h < 4:
                    rows = pl.ds(256 * h, 256)
                    q = q if w0 % 4 else QB[i][opaque(), rows, :]
                    for w in (w0, w0 + 1):
                        v = (q * window(KE, KS, w, rows)).reshape(16, 16, 128).sum(0)
                        v = jnp.where(even, v[:8] + pltpu.roll(v[:8], 7, 0), v[8:] + pltpu.roll(v[8:], 1, 0))
                        logits.append(jnp.where(edge & (2 * w > j), -1e9, v * SCALE) if w > 2 * i
                                      else v * SCALE)
                    yield _Step(138, [lambda v=v: v for v in logits[-2:]], delay=4)
                if h > 0:
                    yield mix_values(h - 1, 2 * w0)
                    yield mix_values(h - 1, 2 * w0 + 2)
            if h < 4:
                top = functools.reduce(jnp.maximum, logits)
                e = [jnp.exp(v - top) for v in logits]
                total = functools.reduce(jnp.add, e)
                yield _Step(30, [lambda v=total: v], delay=3)
                scale = 1.0 / total
                for w in range(8):
                    v = e[w] * scale
                    PW[h % 2][0, pl.ds(16 * w, 8), :] = jnp.where(even, v, pltpu.roll(v, 1, 0))
                    PW[h % 2][0, pl.ds(16 * w + 8, 8), :] = jnp.where(even, pltpu.roll(v, 7, 0), v)
                yield _Step(50, [anchor(PW[h % 2])], delay=6 if h == 3 else 1)

    def packed_sums(terms, signs):
        lo = [pltpu.bitcast(u << 16, F32) for u in terms]
        hi = [pltpu.bitcast(u & np.uint32(0xFFFF0000), F32) for u in terms]
        return [pltpu.pack_elementwise([v[p] + v[q] if s > 0 else v[p] - v[q] for v in (lo, hi)],
                                       packed_dtype=BF16) for p, s, q in signs]

    def half(ref, row):
        return lambda r, size, cols: ref[pl.ds(pl.multiple_of(row + r, 8), size), cols]

    kv_weight = (WS5, half(WK, 0), half(WV, 0))
    q_weight = (WQ5, half(WQ, 0), half(WQ, D // 4))
    o_weight = (WP5, *(lambda r, size, cols, e=e: WP[pl.ds(r + r // 32 * 32 + e, size), cols]
                       for e in (0, 32)))

    def left_sums(weight, row, size, needs=()):
        yield _Wait(*needs)
        sums, top, bottom = weight
        for r in range(0, size, 8):
            a = [ref(row + r, 8, pl.ds(c, 512)) for ref in (top, bottom) for c in (0, 512)]
            for e, v in enumerate(packed_sums(a, ((0, 1, 3), (2, 1, 3), (0, 1, 1), (2, -1, 0), (1, -1, 3)))):
                sums[e, pl.ds(pl.multiple_of(row + r, 8), 8), :] = v
            yield _Step(92, [anchor(sums)], delay=2, marks=["sums"] if r == size - 8 else [])

    def right_sums(dst, g, i, name, needs):
        yield _Wait(*needs)
        z = g + opaque()
        for r in range(0, 256, 16):
            b = [hbu[n][z, pl.ds(k + r, 16), :] for k in (0, 256) for n in (i, i + 1)]
            for e, v in enumerate(packed_sums(b, ((0, 1, 3), (1, -1, 3), (2, -1, 0), (0, 1, 1), (2, 1, 3)))):
                dst[e, pl.ds(r, 16), :] = v
            yield _Step(47, [anchor(dst)], delay=SETTLE if r == 240 else 1,
                        marks=[name] if r == 240 else [])

    def strassen(sch, weight, right, g, i, m, store, needs, marks):
        for n in needs:
            sch.run(n)
        sums, top, bottom = weight
        rows = pl.ds(pl.multiple_of(64 * m, 64), 64)

        def product(left, b):
            sch.fresh = True
            head = tied(lambda r: left(32 * m + r, 8, pl.ds(0, 128)), 4, lambda: sch.point(8.0))
            return _dot(_bf(jnp.concatenate([head, left(32 * m, 32, pl.ds(128, 384))], 1)), _bf(b))

        def a(e):
            return lambda r, size, cols: sums[e, pl.ds(pl.multiple_of(r, 8), size), cols]

        def b(e):
            return right[e + opaque()]

        m2 = product(a(1), hbu[i][g + opaque(), pl.ds(0, 256), :])
        m4 = product(lambda r, size, cols: bottom(r, size, pl.ds(512 + cols.start, cols.size)), b(2))
        store(1, i, rows, m2 + m4)
        m1 = product(a(0), b(0))
        c11, c22 = m1 + m4, m1 - m2
        c11 = c11 + product(a(4), b(4))
        c22 = c22 + product(a(3), b(3))
        m5 = product(a(2), hbu[i + 1][g + opaque(), pl.ds(256, 256), :])
        store(0, i, rows, c11 - m5)
        v = product(top, b(1))
        store(0, i + 1, rows, v + m5)
        store(1, i + 1, rows, c22 + v)
        sch.results.append(v[:8])
        for name in marks:
            sch.done[name] = sch.slot + sch.wait

    def kv_proj(sch, g, i, name, needs):
        def store(lower, n, rows, v):
            (KE, VE)[lower][g + 4 * n + 4, rows, :] = v
        for m in range(16):
            strassen(sch, kv_weight, SB[i // 2], g, i, m, store, needs, [name] if m == 15 else [])

    def q_proj(sch, g, i, name, needs):
        def store(lower, n, rows, v):
            QB[n][0, pl.ds(512 * lower + rows.start, 64), :] = v
        for m in range(8):
            strassen(sch, q_weight, SB[i // 2], g, i, m, store, needs, [name] if m == 7 else [])

    def o_proj(sch, g, i, m, needs, marks, right):
        def store(lower, n, rows, v):
            rows = pl.ds(128 * m + 64 * lower, 64)
            X[n][g, rows, :] = X[n][g, rows, :] + v
        strassen(sch, o_weight, right, g, i, m, store, needs, marks)

    def shift_block(g, i, name, needs):
        yield _Wait(*needs)
        j, z = g + 4 * i, opaque()
        for m in range(16):
            rows = pl.ds(64 * m, 64)
            for ref, to in ((KE, KS), (VE, VS)):
                v = pltpu.roll(ref[j + 4 + z, rows, :], 1, 1)
                if ref is VE:
                    v = jnp.where(_iota(64, 1) == 0, ref[4 + z, rows, :], v)
                to[j, rows, :] = v
                if i == 3:
                    ref[g, rows, :] = v
            yield _Step(12, delay=8, marks=[name] if m == 15 else [])

    def transpose_quarter(w, h, via):
        for r in range(4):
            v = WRAW[w, pl.ds(256 * r, 256), pl.ds(pl.multiple_of(256 * h, 256), 256)]
            v = pltpu.bitcast(v.T, F32)
            via[0, pl.ds(256 * r, 128), :], via[0, pl.ds(256 * r + 128, 128), :] = v[:, :128], v[:, 128:]
            yield _Step(40, delay=16)

    def reorder_quarter(w, h, via, name=None):
        z = 0 if isinstance(h, int) else opaque()
        for c in range(8):
            WT[w][pl.ds(pl.multiple_of(128 * h, 128), 128), pl.ds(128 * c, 128)] = pltpu.bitcast(
                jnp.concatenate([via[z, pl.ds(128 * c + u, 8, stride=16), :] for u in range(16)], 0), U32)
            yield _Step(20, delay=4, marks=[name] if c == 7 else [])

    def query_weight(h):
        yield from transpose_quarter(0, h, QB[0])
        yield from reorder_quarter(0, h, QB[0], "w")

    def transpose_wo(name):
        for c in range(8):
            for h in range(4):
                v = jnp.concatenate([wou[c, pl.ds(128 * h + u, 8, stride=16), :] for u in range(16)], 0)
                WP[pl.ds(64 * c, 64), pl.ds(256 * h, 256)] = pltpu.bitcast(_bf(v).T, U32)
                yield _Step(20, delay=10, marks=[name] if c == 7 and h == 3 else [])

    def prep_spectral_weights(c2):
        def words(k2):
            re, im = (wsu[u, k2, pl.ds(c2, 64, stride=4), :] for u in range(2))
            return ((re & np.uint32(0xFFFF)) | (im << 16), (re >> 16) | (im & np.uint32(0xFFFF0000)))

        def arrange(w, below):
            return jnp.where(_iota(w.shape[0], 1) < 64, w, below)

        below = words(15)
        for k2 in range(16):
            here = words(k2)
            for e in range(2):
                cl = 2 * c2 + e
                w = arrange(here[e], below[e])
                WS[k2, pl.ds(64 * cl, 64), :] = pltpu.roll(w, 1, 0) if cl > 4 else w
            below = here
            yield _Step(90, delay=3)
        if c2 == 0:
            def nyquist(k2):
                re, im = (jnp.broadcast_to(WN[u, :, pl.ds(128 * k2, 128)].astype(F32), (8, 128))
                          for u in range(2))
                return pltpu.pack_elementwise([re, im], packed_dtype=BF16)
            for k2 in range(16):
                WS[k2, pl.ds(512, 8), :] = arrange(nyquist(k2), nyquist((k2 + 15) % 16))

    def write_out(p, c, name, needs):
        yield _Wait(*needs)
        rows = pl.ds(pl.multiple_of(128 * c, 128), 128)
        g, i = 2 * p % 4 + opaque(), p // 2
        w = pltpu.pack_elementwise([X[i][g, rows, :], X[i][g + 1, rows, :]], packed_dtype=BF16)
        xru[c, pl.ds(p, 128, stride=8), :] = w.T
        yield _Step(30, marks=[name])

    tables = [pltpu.make_async_copy(lanes_hbm, lanes, sems.at[24]),
              pltpu.make_async_copy(mats_hbm, mats.at[pl.ds(M_R, 5)], sems.at[25])]
    start_all(tables + [x_copy(c) for c in range(8)])
    for c in tables:
        c.wait()

    def make_twiddle(k):
        PB = temps[0][2]
        PB[0, pl.ds(0, 128), :] = lane_vec(L_TWID + k, 128)
        twid[k] = PB[opaque(), pl.ds(0, 128), :].T

    _loop(6, make_twiddle, "make_twiddle")

    def make_dft(j):
        fa, fb = lanes[pl.ds(L_FA, 128), :], lanes[pl.ds(L_FB, 128), :]
        c, sn = lane_vec(L_COS + j, 128), lane_vec(L_SIN + j, 128)
        UB, _, _, ubu, _ = temps[0]
        UB[0, pl.ds(0, 128), :] = (fa * c + fb * sn).astype(BF16)
        UB[0, pl.ds(128, 128), :] = (fb * c - fa * sn).astype(BF16)
        mats[M_FA + j], mats[M_FB + j] = ubu[0, pl.ds(0, 64), :], ubu[0, pl.ds(64, 64), :]

    _loop(NB, make_dft, "make_dft")

    def load_x(c):
        x_copy(c).wait()
        pl.when(c == 6)(lambda: start_all(spec_copies[0]))
        pl.when(c == 7)(lambda: start_all(spec_copies[1]))
        rows = pl.ds(pl.multiple_of(128 * c, 128), 128)
        for p in range(8):
            w = xru[c, pl.ds(p, 128, stride=8), :].T
            for e, bits in enumerate((w << 16, w & np.uint32(0xFFFF0000))):
                g, i = 2 * p % 4 + e, p // 2
                v = pltpu.bitcast(bits, F32)
                X[i][g, rows, :] = v
                v = v.reshape(16, 8, 128)
                mean = _all_sublanes(v.sum(0), jnp.add, 0) * (1.0 / 128)
                STAT[4 * g + i, c] = mean
                STAT[4 * g + i, 8 + c] = _all_sublanes(((v - mean) ** 2).sum(0), jnp.add, 0)

    _loop(8, load_x, "load_x")

    def after(name, action):
        yield _Wait(name)
        action()

    def spectral_weights():
        yield _Wait(("f", 2, 1))
        for c in spec_copies[0] + spec_copies[1]:
            c.wait()
        for c2 in range(4):
            yield from prep_spectral_weights(c2)

    with jax.named_scope("first_forward"):
        sch = _Sched(0.72, 20)
        sch.add(after(("f", 0, 1), w_copies[1].start), "k")
        sch.add(after(("f", 1, 1), w_copies[2].start), "v")
        sch.add(after(("f", 2, 3), w_copies[0].start), "q")
        for g in range(4):
            for i in range(4):
                sch.add(fwd_block(g, i, ("f", g, i), [("f", g - 1, i)] if g else [],
                                  [("r", g - 1)] if g else [], True), ("f", g, i))
            sch.add(group_stage(g, ("r", g), [("f", g, i) for i in range(4)], False), ("r", g))
        sch.add(spectral_weights(), "s")
        sch.drive()
    start_all(wo_copies)

    def keys_values(layer, g):
        sch = _Sched(0.41, 32, 3) if layer == 0 else _Sched(0.36, 28, 2)
        nxt = (g + 1) % 4
        sch.add(inv_block(g, 2, ("i", 2), []), ("i", 2))
        sch.add(inv_block(g, 3, ("i", 3), [("read", ("i", 2))]), ("i", 3))
        sch.add(right_sums(SB[1], g, 2, ("b", 2), [("i", 2), ("i", 3)]), ("b", 2))
        sch.add(group_stage(nxt, "r", [("read", ("i", 3))], True), "r")
        sch.add(inv_block(nxt, 0, ("i", 4), ["r", ("i", 2)], n=g + 1), ("i", 4))
        sch.add(inv_block(nxt, 1, ("i", 5), [("read", ("i", 4)), ("i", 3)], n=g + 1), ("i", 5))
        if layer == 0:
            sch.add(query_weight(g), "w")
            sch.add(left_sums(q_weight, 128 * (g % 2), 128, ["w"]), "sums")
        for i in (2, 3):
            sch.add(shift_block((g + 3) % 4, i, ("s", i), []), ("s", i))
        for i in (0, 1):
            sch.add(shift_block(g, i, ("s", i), [("kv", 0)]), ("s", i))
        sch.add(right_sums(SB[0], nxt, 0, ("b", 4), [("i", 4), ("i", 5), ("kv", 0)]), ("b", 4))
        kv_proj(sch, g, 0, ("kv", 0), [])
        kv_proj(sch, g, 2, ("kv", 2), [("b", 2)])
        sch.finish()

    def mix(g, after, last):
        tail = after is None
        sch = _Sched(0.66 if last else 0.63, 28 if last else 32)
        pace = 0.48 if tail else 0.35 if last else 0.32
        ahead = [(g, 2), (g, 3)] + ([] if tail else [(after, 0), (after, 1)])
        for n, block in enumerate(ahead):
            sch.add(attend(*block, ("a", n), [[], [("a", 0)], [("a", 1), ("q", 0)], [("a", 2)]][n]),
                    ("a", n), pace=pace)
            if n % 2:
                sch.add(right_sums(SB[2 + block[1] // 2], block[0], block[1] - 1, ("b", n),
                                   [("a", n)] + ([("o", 0)] if n == 3 else [])), ("b", n))
        for i in () if tail else (0, 2):
            sch.add(right_sums(SB[i // 2], after, i, ("h", i), [("q", 0)] if i else []), ("h", i))
        if not last:
            sch.add(group_stage((g + 3) % 4, "r", [], False), "r")
            for i in range(4):
                sch.add(fwd_block(g, i, ("f", i), [("o", i - i % 2)], ["r"]), ("f", i))
        now = 6 if last else 8
        for i in (0, 2):
            for m in range(now):
                o_proj(sch, g, i, m, [("b", 1)] if i else [], [("o", i)] if m == now - 1 else [],
                       SB[2 + i // 2])
            if not tail:
                q_proj(sch, after, i, ("q", i), [("h", i)])
        if tail:
            sch.add(group_stage(g, "s", [("f", i) for i in range(4)], False), "s")
        sch.share = 0.92
        sch.drive()

    def mix_odd():
        sch = _Sched(0.66)
        blocks = [(1, 2), (1, 3), (3, 0), (3, 1), (3, 2), (3, 3)]
        for n, (g, i) in enumerate(blocks):
            sch.add(attend(g, i, ("a", n), ([("a", n - 1)] if n else []) + ([("q", i)] if n in (2, 4) else [])),
                    ("a", n), pace=0.32)
            if n % 2:
                sch.add(right_sums(SB[(3, 2, 0)[n // 2]], g, i - 1, ("b", g, i - 1),
                                   [("a", n)] + ([("o", 1, 0, 5)] if n > 1 else [])), ("b", g, i - 1))
        for i in (0, 2):
            sch.add(right_sums(SB[i // 2], 3, i, ("h", i), []), ("h", i))
        for g in (1, 3):
            for i in range(4):
                for c in range(6):
                    sch.add(write_out(2 * i + g // 2, c, ("w", g, i, c), [("o", g, i - i % 2, c)]),
                            ("w", g, i, c))
        for g, i, slot, count in ((1, 0, 2, 6), (1, 2, 3, 8), (3, 0, 2, 8), (3, 2, 0, 6)):
            for m in range(count):
                o_proj(sch, g, i, m, [("b", g, i)] if (g, i) != (1, 0) else [], [("o", g, i, m)], SB[slot])
            for e in (0, 2) if (g, i) == (1, 0) else ():
                q_proj(sch, 3, e, ("q", e), [("h", e)] + ([("a", 1)] if e else []))
        sch.share = 0.92
        sch.drive()

    def copy_out(chunks):
        def start(_):
            for c in chunks:
                out_copy(c).start()
        _loop(zero + 1, start, "copy_out")

    def postponed():
        slots = {(3, 2): 0, (2, 2): 1, (0, 2): 2, (2, 0): 3, (0, 0): 0, (1, 0): 1}
        early, late = list(slots)[:2], list(slots)[2:]
        sources = 2 * [[(0, 0), (1, 0)], [(2, 0)]] + 2 * [[(0, 2)], []]
        for c in (6, 7):
            sch = _Sched(0.7, 12)
            for n, (pair, slot) in enumerate(slots.items()) if c == 6 else ():
                if n:
                    sch.add(right_sums(SB[slot], *pair, pair, [(early[n - 4], 7)] if n >= 4 else []), pair)
            for p in (5, 7, 4, 6, 1, 3, 0, 2):
                sch.add(write_out(p, c, ("w", p), [(pair, c) for pair in sources[p] or early * (c == 6)]),
                        ("w", p))
            for pair, m in [(pair, m) for m in (6, 7) for pair in early] * (c == 6) + [(v, c) for v in late]:
                o_proj(sch, *pair, m, [pair] if c == 6 and pair != (3, 2) else [], [(pair, m)],
                       SB[slots[pair]])
            sch.drive()
            copy_out([c])

    def first_queries(layer):
        sch = _Sched(0.68)
        sch.add(right_sums(SB[1], 0, 2, ("h", 2), []), ("h", 2))
        sch.add(shift_block(3, 2, "s", []), "s")
        sch.add(attend(0, 0, ("a", 0), ["q"]), ("a", 0), pace=0.4)
        sch.add(attend(0, 1, ("a", 1), [("a", 0)]), ("a", 1), pace=0.4)
        sch.add(right_sums(SB[2], 0, 0, "b", [("a", 1)]), "b")
        sch.add(shift_block(3, 3, "t", []), "t")
        if layer == 0:
            for c in wo_copies:
                c.wait()
            sch.add(transpose_wo("w"), "w")
            sch.add(left_sums(o_weight, 0, 256, ["w"]), "sums")
        q_proj(sch, 0, 0, "q", [])
        q_proj(sch, 0, 2, None, [("h", 2)])
        sch.finish()

    def key_value_weights():
        w_copies[1].wait()
        w_copies[2].wait()
        for h in range(6):
            work = []
            for w in (1, 2):
                if h < 4:
                    work.append(transpose_quarter(w, h, QB[2 * (h % 2) + w - 1]))
                if 0 < h < 5:
                    work.append(reorder_quarter(w, h - 1, QB[2 * ((h - 1) % 2) + w - 1]))
            if h > 1:
                work.append(left_sums(kv_weight, 128 * (h - 2), 128))
            list(itertools.zip_longest(*work))

    for layer in range(2):
        with jax.named_scope("spectral"):
            _loop(4, spectral_rows, "rows")
            if layer == 0:
                _loop(zero + 1, lambda _: key_value_weights(), "weights")
            spectral(512, 8)
        sch = _Sched(0.92)
        sch.add(group_stage(0, "r", [], True), "r")
        sch.add(inv_block(0, 0, ("i", 0), ["r"]), ("i", 0))
        sch.add(inv_block(0, 1, ("i", 1), ["r"]), ("i", 1))
        sch.add(right_sums(SB[0], 0, 0, "b", [("i", 0), ("i", 1)]), "b")
        sch.drive()
        if layer == 0:
            w_copies[0].wait()
        _loop(4, lambda g: keys_values(layer, g), "keys_values")
        first_queries(layer)
        if layer == 0:
            pl.when(never)(lambda: spectral_rows(0))
        if layer == 0:
            _loop(3, lambda g: mix(g, g + 1, False), "mix")
            mix(3, None, False)
        else:
            _loop(2, lambda u: mix(2 * u, 2 - u, True), "mix")
            mix_odd()
    copy_out(range(6))
    postponed()
    for c in range(8):
        out_copy(c).wait()


@jax.jit
def pallas_interleave_layers__spectral_gfnet__sliding_local_dilated__prompt_kernel(
    A_x: jax.Array,
    A_w_r: jax.Array,
    A_w_i: jax.Array,
    B_x: jax.Array,
    B_wqkv: jax.Array,
    B_wo: jax.Array,
):
    del B_x
    hbm = pl.BlockSpec(memory_space=pl.ANY)
    smem = pl.BlockSpec(memory_space=pltpu.SMEM)
    out = pl.pallas_call(
        _kernel,
        out_shape=jax.ShapeDtypeStruct((S, D), BF16),
        in_specs=[smem, smem, hbm, hbm, hbm, hbm, hbm, hbm, hbm],
        out_specs=hbm,
        scratch_shapes=[
            pltpu.VMEM(_LANES.shape, F32),
            pltpu.VMEM((37, 64, 128), U32),
            pltpu.VMEM((6, 128, 128), F32),
            pltpu.VMEM((NB, 16, 8, 128), F32),
            pltpu.VMEM((NB + 4, D, 128), F32),
            pltpu.VMEM((NB + 4, D, 128), F32),
            pltpu.VMEM((NB, D, 128), F32),
            pltpu.VMEM((NB, D, 128), F32),
            pltpu.VMEM((2 * NB + 1, ZR, 128), F32),
            pltpu.VMEM((9, ZR, 128), F32),
            pltpu.VMEM((NB, ZR, 128), U32),
            *4 * [pltpu.VMEM((D // 2, D), U32)],
            pltpu.VMEM((5, D // 2, D // 2), U32),
            *2 * [pltpu.VMEM((5, D // 4, D // 2), U32)],
            *4 * [pltpu.VMEM((5, D // 4, 128), U32)],
            pltpu.VMEM((8, S, 128), BF16),
            pltpu.VMEM((2, NB, D // 2, 128), BF16),
            pltpu.VMEM((2, 1, S), BF16),
            pltpu.VMEM((3, D, D), BF16),
            pltpu.VMEM((8, D, 128), BF16),
            pltpu.VMEM((1, 128, 128), F32),
            pltpu.VMEM((1, 128, 128), F32),
            pltpu.SemaphoreType.DMA((26,)),
            *2 * [pltpu.VMEM((1, D, 128), F32)],
        ] + 4 * [
            pltpu.VMEM((5, D, 128), F32),
            pltpu.VMEM((5, D, 128), BF16),
            pltpu.VMEM((1, D, 128), F32),
            pltpu.VMEM((1, D, 128), BF16),
            pltpu.VMEM((1, 1152, 128), BF16),
        ],
        compiler_params=pltpu.CompilerParams(vmem_limit_bytes=126 * 2 ** 20),
    )(_ZERO, _ROT, _MATS, _LANES, A_x.reshape(S, D), A_w_r.T, A_w_i.T, B_wqkv, B_wo)
    return out.reshape(1, S, D)
```

```python
import functools
import itertools

import numpy as np

import jax
import jax.numpy as jnp
import jax.experimental.pallas as pl
import jax.experimental.pallas.tpu as pltpu

S, D, NB = 2048, 1024, 16
ZR = 576
F32, BF16, U32, I32 = jnp.float32, jnp.bfloat16, jnp.uint32, jnp.int32
EPS = 1e-5
SCALE = 32 ** -0.5
RSQ2 = float(np.sqrt(0.5))
SETTLE = 6

_S_ROWS = [(32 * u, 32) for u in range(16)] + [(512, 8)]

M_FA, M_FB, M_R, M_C4, M_RT, M_C4T, M_R0T = 0, 16, 32, 33, 34, 35, 36
L_MU, L_NU, L_KU, L_KV, L_COS, L_SIN, L_TWID, L_FA, L_FB = 0, 16, 32, 48, 64, 80, 96, 104, 232


def _bf16_bits(a):
    u = np.ascontiguousarray(a, dtype=np.float32).view(np.uint32).astype(np.uint64)
    return ((u + 0x7FFF + ((u >> 16) & 1)) >> 16).astype(np.uint32)


def _constants():
    a = np.arange(128)
    k1 = np.arange(64)
    alt = (-1.0) ** a
    lanes = np.zeros((384, 128))
    t = 2 * np.pi * np.outer(a, k1) / 128
    fa = np.concatenate([np.cos(t), -np.sin(t)], 1)
    fb = np.concatenate([np.sin(t), -np.cos(t)], 1)
    fa[:, 0], fb[:, 0] = RSQ2, -RSQ2
    fa[:, 64], fb[:, 64] = alt, 0.0
    lanes[L_FA:L_FA + 128], lanes[L_FB:L_FB + 128] = fa, fb
    for j in range(NB):
        ang = 2 * np.pi * j / 32 + np.pi / 32
        p, q = (_bf16_bits([np.cos(ang), np.sin(ang)]) << 16).view(np.float32).astype(np.float64)
        turn = 2 * np.pi * j * np.tile(k1, 2) / S
        lanes[L_COS + j], lanes[L_SIN + j] = np.cos(turn), np.repeat([-1.0, 1.0], 64) * np.sin(turn)
        lanes[L_COS + j, 64], lanes[L_SIN + j, 64] = p, q
        lanes[L_MU + j, 0], lanes[L_MU + j, 64] = 1.0, (q / p + p / q) / 2
        lanes[L_NU + j, 0], lanes[L_NU + j, 64] = 0.0, (q / p - p / q) / 2
        lanes[L_KU + j, 0], lanes[L_KU + j, 64] = 1.0, q / p
        lanes[L_KV + j, 0], lanes[L_KV + j, 64] = 1.0, p / q
    lanes[:, 65:] = lanes[:, :64:-1].copy()
    for k in (1, 2, 3):
        lanes[L_TWID + 2 * k - 2] = np.cos(2 * np.pi * a * k / D)
        lanes[L_TWID + 2 * k - 1] = np.sin(2 * np.pi * a * k / D)
    th = 2 * np.pi * np.outer(k1, a) / 128
    r = np.concatenate([np.cos(th), -np.sin(th)], 0)
    r[64] = alt
    th = 2 * np.pi * np.outer(2 * k1 + 1, a) / 256
    c4 = np.concatenate([np.cos(th), -np.sin(th)], 0)
    inv = 2.0 / (S * D)
    r0t = inv * r.T
    r0t[:, 0::64] *= 0.5
    rows = np.arange(128).reshape(2, 4, 16).transpose(1, 0, 2).ravel()
    bits = _bf16_bits(np.stack([r[rows], c4[rows], inv * r.T, inv * c4.T, r0t]))
    ang = 2 * np.pi * np.outer(np.arange(4), np.arange(4)).ravel() / 16
    rot = np.concatenate([np.cos(ang), np.sin(ang)]).astype(np.float32)
    return bits[:, 0::2] | (bits[:, 1::2] << 16), lanes.astype(np.float32), rot


_MATS, _LANES, _ROT = _constants()
_ZERO = np.zeros((1,), np.int32)


class _Step:
    def __init__(self, cost, anchors=(), delay=0, marks=()):
        self.cost, self.anchors, self.delay, self.marks = cost, list(anchors), delay, list(marks)


class _Wait:
    def __init__(self, *names):
        self.names = names


class _Mat:
    def __init__(self, emit):
        self.emit = emit


class _Hold:
    def __init__(self, store):
        self.store = store


class _Task:
    def __init__(self, gen, pace):
        self.gen, self.pace, self.blocked, self.not_before, self.held = gen, pace, (), 0, None
        self.allowed = 0.0


class _Sched:
    def __init__(self, share=0.0, wait=28, lag=3):
        self.lag = lag
        self.wait = wait
        self.share = share
        self.tasks, self.done, self.producer = [], {}, {}
        self.slot, self.credit, self.anchors, self.results = 0, 0.0, [], []
        self.fresh = False

    def add(self, gen, name, pace=99):
        self.producer[name] = self.producer["read", name] = _Task(gen, pace)
        self.tasks.append(self.producer[name])

    def _ready(self, t):
        return t.not_before <= self.slot and all(
            n in self.done and self.done[n] <= self.slot for n in t.blocked)

    def _advance(self, t, mats=True):
        item, t.held = t.held or next(t.gen, None), None
        if item is None:
            self.tasks.remove(t)
        elif isinstance(item, _Wait):
            t.blocked = item.names
        elif isinstance(item, _Hold):
            if len(self.results) >= self.lag:
                item.store(self.results[-self.lag])
        elif isinstance(item, _Mat):
            if mats:
                t.not_before = float("inf")
                self.fresh = False
                self.credit -= item.emit(lambda: self.point(0.0)) or 0
                t.not_before = self.slot + self.wait
            else:
                t.held, t.not_before = item, self.slot + 1
        else:
            t.blocked = ()
            t.not_before = self.slot + item.delay
            self.credit -= item.cost
            self.anchors += item.anchors
            for n in item.marks:
                self.done[n] = self.slot + item.delay
            return True

    def run(self, *names):
        while not all(n in self.done for n in names):
            for n in names:
                if n not in self.done:
                    for b in self.producer[n].blocked:
                        self.run(b)
                    self._advance(self.producer[n])

    def drive(self):
        while self.tasks:
            ready = [t for t in self.tasks if self._ready(t)]
            if not ready:
                self.slot += 1
                continue
            self.anchors, self.credit = self.anchors[-2:], 0.0
            self._advance(next((t for t in ready if t.held), ready[0]))
            self.slot -= min(self.credit, 0.0) / 60

    def finish(self):
        self.run(*[n for n in self.producer if n[0] != "read"])

    def point(self, own):
        for t in self.tasks:
            t.allowed = min(t.allowed, 0.0) + t.pace
        while True:
            t = next((t for t in self.tasks if self._ready(t) and t.allowed > 0
                      and self.credit > 0), None)
            if t is None:
                break
            if self._advance(t, self.fresh):
                t.allowed -= 1
        anchors, self.anchors = self.anchors, []
        self.credit = min(self.credit, 10.0) + 64 * self.share - own
        self.fresh = False
        self.slot += 1
        return anchors


def _dot(a, b):
    return jnp.dot(a, b, preferred_element_type=F32)


def _dot_t(a, b):
    return jax.lax.dot_general(a, b, (((1,), (1,)), ((), ())), preferred_element_type=F32)


def _bf(u):
    return pltpu.bitcast(u, BF16)


def _iota(rows, dim):
    return jax.lax.broadcasted_iota(I32, (rows, 128), dim)


def _mirror(v):
    index = -_iota(8, 1) & 127
    return jnp.concatenate([jnp.take_along_axis(v[r:r + 8], index, axis=1)
                            for r in range(0, v.shape[0], 8)], 0)


def _radix4(z, inverse):
    (r0, i0), (r1, i1), (r2, i2), (r3, i3) = z
    ar, ai, cr, ci = r0 + r2, i0 + i2, r0 - r2, i0 - i2
    br, bi, dr, di = r1 + r3, i1 + i3, r1 - r3, i1 - i3
    lo, hi = (cr + di, ci - dr), (cr - di, ci + dr)
    if inverse:
        lo, hi = hi, lo
    return [(ar + br, ai + bi), lo, (ar - br, ai - bi), hi]


def _all_sublanes(v, op, axis):
    for sh in (4, 2, 1):
        v = op(v, pltpu.roll(v, sh, axis))
    return v


def _loop(n, body, name):
    def step(i, carry):
        body(i)
        return carry
    with jax.named_scope(name):
        jax.lax.fori_loop(0, n, step, 0)


def _kernel(zero_ref, rot, mats_hbm, lanes_hbm, x_hbm, wr_hbm, wi_hbm, wqkv_hbm, wo_hbm, out_hbm,
            lanes, mats, twid, STAT, KE, VE, KS, VS, Z, ZT, WS, WQ, WK, WV, WP, WS5, WQ5, WP5,
            SB0, SB1, SB2, SB3, XR, WRI, WN, WRAW, WO, PW0, PW1, sems, *split):
    zero = zero_ref[0]
    never = zero != 0
    X, HB, QB = split[2::5], split[3::5], split[4::5]
    hbu = [r.bitcast(U32) for r in HB]
    xru, wsu, wou = XR.bitcast(U32), WRI.bitcast(U32), WO.bitcast(U32)
    temps = [(ub, ab, pb, ub.bitcast(U32), ab.bitcast(U32))
             for ub, ab, pb in zip(split[5::5], split[6::5], 2 * split[:2])]
    PW, SB, WT = (PW0, PW1), (SB0, SB1, SB2, SB3), (WQ, WK, WV, WP)
    counter = [0]

    def opaque():
        counter[0] += 1
        return zero * counter[0]

    def anchor(ref):
        at = (0,) * (len(ref.shape) - 2)
        return lambda: ref[(*at, pl.ds(pl.multiple_of(zero * 8, 8), 8), pl.ds(0, 128))]

    def settle(ref, points=SETTLE):
        return _Step(2, [anchor(ref)], delay=points)

    def hold(ref, spare):
        def store(v):
            ref[spare, pl.ds(pl.multiple_of(zero * 8, 8), 8), :] = v
        return _Hold(store)

    def tied(load, vregs, point):
        parts = []
        for r in range(vregs):
            anchors = point()
            u = load(8 * r)
            for a in anchors:
                u = jnp.where(never, pltpu.bitcast(a(), U32), u)
            parts.append(u)
        return jnp.concatenate(parts, 0)

    def mat(i):
        return _bf(mats[i])

    def d_stage(t, which):
        UB, AB, PB, ubu, abu = temps[t]

        def emit(point):
            z = opaque()
            for c in range(8):
                lhs = mat(which(c) + opaque()) if c % 4 else _bf(
                    tied(lambda r, u=which(c) + opaque(): mats[u, pl.ds(r, 8), :], 8, point))
                PB[0, pl.ds(128 * c, 128), :] = _dot(lhs, _bf(ubu[z, pl.ds(64 * c, 64), :]))
        return _Mat(emit)

    def lane_vec(i, rows):
        return jnp.broadcast_to(lanes[pl.ds(i, 1), :], (rows, 128))

    def x_copy(c):
        return pltpu.make_async_copy(
            x_hbm.at[:, pl.ds(pl.multiple_of(128 * c, 128), 128)], XR.at[c], sems.at[c])

    def out_copy(c):
        return pltpu.make_async_copy(
            XR.at[c], out_hbm.at[:, pl.ds(pl.multiple_of(128 * c, 128), 128)], sems.at[8 + c])

    spec_copies = [[pltpu.make_async_copy(w.at[pl.ds(0, 512), pl.ds(128 * k2, 128)], WRI.at[u, k2],
                                          sems.at[16 + u]) for k2 in range(16)]
                   + [pltpu.make_async_copy(w.at[pl.ds(512, 1), :], WN.at[u], sems.at[22 + u])]
                   for u, w in enumerate((wr_hbm, wi_hbm))]

    def start_all(copies):
        for c in copies:
            c.start()
    w_copies = [pltpu.make_async_copy(wqkv_hbm.at[:, pl.ds(D * w, D)], WRAW.at[w], sems.at[18 + w])
                for w in range(3)]
    wo_copies = [pltpu.make_async_copy(wo_hbm.at[:, pl.ds(128 * c, 128)], WO.at[c], sems.at[21])
                 for c in range(8)]

    def ln_rstd(g, i, mean):
        acc, m = None, g + opaque()
        for r in range(8):
            d = X[i][m, pl.ds(128 * r, 128), :].reshape(16, 8, 128) - mean[None]
            v = (d * d).sum(0)
            acc = v if acc is None else acc + v
            if r < 7:
                yield _Step(50, [lambda acc=acc: acc], delay=3)
        rstd = jax.lax.rsqrt(_all_sublanes(acc, jnp.add, 0) * (1.0 / D) + EPS)
        yield _Step(50, delay=8)
        yield _Step(10, [lambda: rstd], delay=1)
        return rstd

    def fwd_block(g, i, name, needs, free=(), known=False):
        j, t = g + 4 * i, i
        UB, AB, PB, ubu, abu = temps[t]
        yield _Wait(*needs)
        if known:
            means, squares = STAT[4 * g + i, pl.ds(0, 8)], STAT[4 * g + i, pl.ds(8, 8)]
            mean = means.sum(0) * 0.125
            var = (squares.sum(0) + 128.0 * ((means - mean) ** 2).sum(0)) * (1.0 / D)
            rstd = jax.lax.rsqrt(var + EPS)
            yield _Step(50, delay=6)
        else:
            yield settle(X[i])
            acc, m = None, g + opaque()
            for r in range(8):
                v = X[i][m, pl.ds(128 * r, 128), :].reshape(16, 8, 128).sum(0)
                acc = v if acc is None else acc + v
                if r % 2:
                    yield _Step(35, [lambda acc=acc: acc], delay=7 if r == 7 else 3)
            mean = _all_sublanes(acc, jnp.add, 0) * (1.0 / D)
            rstd = yield from ln_rstd(g, i, mean)
        mean8, rstd = (jnp.concatenate([v, v], 0) for v in (mean * 8.0, rstd))
        z = opaque()
        for r in range(8):
            rows = pl.ds(16 * r, 16)
            x = [X[i][g + z, pl.ds(128 * b + 16 * r, 16), :] for b in range(8)]
            s = [x[b] + x[b + 4] for b in range(4)]
            d = [x[b] - x[b + 4] for b in range(4)]
            e, o = s[0] + s[2], s[1] + s[3]
            UB[0, rows, :] = ((e + o - mean8) * rstd).astype(BF16)
            UB[0, pl.ds(128 + 16 * r, 16), :] = ((e - o) * rstd).astype(BF16)
            t1, t2 = (d[1] - d[3]) * RSQ2, (d[1] + d[3]) * RSQ2
            u = {1: (d[0] + t1, d[2] + t2), 2: (s[0] - s[2], s[1] - s[3]), 3: (d[0] - t1, d[2] - t2)}
            yield _Step(34, [anchor(ubu)], delay=1)
            for k in (1, 2, 3):
                c, sn = twid[z + 2 * k - 2, rows, :] * rstd, twid[z + 2 * k - 1, rows, :] * rstd
                re, m = u[k]
                if k == 3:
                    ur, ui = re * c + m * sn, m * c - re * sn
                else:
                    ur, ui = re * c - m * sn, m * c + re * sn
                UB[0, pl.ds(256 * k + 16 * r, 16), :] = ur.astype(BF16)
                UB[0, pl.ds(256 * k + 128 + 16 * r, 16), :] = ui.astype(BF16)
                yield _Step(26, [anchor(ubu)], delay=1)
        yield settle(ubu)

        def d_forward(point):
            z = opaque()
            first = _iota(8, 0) == 0

            def stage(c):
                u = (M_C4 if c == 1 else M_R) + opaque()
                lhs = mat(u) if c % 4 else _bf(tied(lambda r: mats[u, pl.ds(r, 8), :], 8, point))
                v = _dot(lhs, _bf(ubu[z, pl.ds(64 * c, 64), :]))
                return [(v[32 * u:32 * u + 16], v[32 * u + 16:32 * u + 32]) for u in range(4)]

            def put(row, u, v, v0=None):
                if u == 0 and v0 is not None:
                    v = jnp.concatenate([jnp.where(first, v0, v[:8]), v[8:]], 0)
                AB[0, pl.ds(row + 16 * u, 16), :] = v.astype(BF16)

            for u, (p1, p2) in enumerate(stage(0)):
                put(0, u, p1)
                put(528, u, p2, 0.0)
                if u == 0:
                    put(512, 0, jnp.zeros_like(p2), p2[:8])
            for u, (p1, p2) in enumerate(stage(1)):
                put(256, u, p1)
                put(528 + 256, u, p2)
            for k in (1, 2, 3):
                for u, ((p1, p2), (q1, q2)) in enumerate(zip(stage(2 * k), stage(2 * k + 1))):
                    if k == 3:
                        pr, pi, mr, mi = p1 - q2, p2 + q1, p1 + q2, p2 - q1
                        pi0, mi0 = q1[:8], -q2[:8]
                    else:
                        pr, pi, mr, mi = p1 + q2, p2 - q1, p1 - q2, p2 + q1
                        pi0, mi0 = -q1[:8], q2[:8]
                    put(64 * k, u, pr, p1[:8])
                    put(64 * (8 - k), u, mr, p2[:8])
                    put(528 + 64 * k, u, pi, pi0)
                    put(528 + 64 * (8 - k), u, mi, mi0)
            return 190

        yield _Mat(d_forward)
        yield settle(abu)
        yield _Wait(*free)

        def s_forward(point):
            z = opaque()
            fa, fb = mat(M_FA + j + z), mat(M_FB + j + z)
            for r0, rn in ((0, 256), (256, 272)):
                lhs = abu[z, pl.ds(r0 // 2, rn // 2), :] if r0 else tied(
                    lambda r: abu[z, pl.ds(r, 8), :], 16, point)
                u = _dot(_bf(lhs), fa)
                v = _dot(_bf(abu[z, pl.ds(264 + r0 // 2, 128), :]), fb)
                re, m = u[:256] + v, u[:256] - v
                if r0:
                    re, m = (jnp.concatenate([a, u[256:264]], 0) for a in (re, m))
                rn = re.shape[0]
                edge = (_iota(rn, 1) & 63) == 0
                ZT[2 * i, pl.ds(r0, rn), :] = re
                ZT[2 * i + 1, pl.ds(r0, rn), :] = jnp.where(
                    edge, lane_vec(L_MU + j, rn) * m + lane_vec(L_NU + j, rn) * re, _mirror(m))
            return 400

        yield _Mat(s_forward)
        yield _Step(2, [anchor(ZT)], delay=SETTLE, marks=[name])

    def group_stage(g, name, needs, inverse):
        yield _Wait(*needs)

        def turn(z, k):
            if k == 0:
                return z
            c, s = rot[4 * g + k], rot[16 + 4 * g + k]
            if inverse:
                return z[0] * c - z[1] * s, z[1] * c + z[0] * s
            return z[0] * c + z[1] * s, z[1] * c - z[0] * s

        (src, a), (dst, b) = ((Z, 8 * g), (ZT, 0)) if inverse else ((ZT, opaque()), (Z, 8 * g))
        for r in range(65):
            if r % (16 if inverse else 64) == 0:
                yield hold(src, 2 * NB if inverse else 8)
            rows = pl.ds(8 * r, 8)
            z = [(src[a + 2 * i, rows, :], src[a + 2 * i + 1, rows, :]) for i in range(4)]
            if inverse:
                z = _radix4([turn(z[k], k) for k in range(4)], True)
            else:
                z = [turn(v, k) for k, v in enumerate(_radix4(z, False))]
            for i in range(4):
                dst[b + 2 * i, rows, :], dst[b + 2 * i + 1, rows, :] = z[i]
            yield _Step(35, [anchor(dst)], delay=1, marks=[name] if r == 64 else [])

    def spectral(row, size):
        rows = pl.ds(row, size)
        for k0 in range(4):
            z = _radix4([(Z[8 * g + 2 * k0, rows, :], Z[8 * g + 2 * k0 + 1, rows, :])
                         for g in range(4)], False)
            y = []
            for k1, (re, im) in enumerate(z):
                w = WS[k0 + 4 * k1, rows, :]
                wr = pltpu.bitcast(w << 16, F32)
                wi = pltpu.bitcast(w & np.uint32(0xFFFF0000), F32)
                y.append((re * wr - im * wi, re * wi + im * wr))
            y = _radix4(y, True)
            for g in range(4):
                Z[8 * g + 2 * k0, rows, :], Z[8 * g + 2 * k0 + 1, rows, :] = y[g]

    def spectral_rows(c2):
        for r in range(8):
            spectral(pl.multiple_of(128 * c2 + 16 * r, 16), 16)

    def inv_block(g, i, name, needs, n=None):
        j, t = g + 4 * i, i % 2
        UB, AB, PB, ubu, abu = temps[t]
        n = g if n is None else n
        z = opaque()
        yield _Wait(*needs)
        for r0, rn in _S_ROWS:
            if r0 == 0:
                yield hold(ZT, 8)
            re, im = ZT[z + 2 * i, pl.ds(r0, rn), :], ZT[z + 2 * i + 1, pl.ds(r0, rn), :]
            edge = (_iota(rn, 1) & 63) == 0
            rolled = _mirror(im)
            u = re + jnp.where(edge, lane_vec(L_KU + j, rn) * im, rolled)
            if r0 < 512:
                v = re - jnp.where(edge, lane_vec(L_KV + j, rn) * im, rolled)
                AB[0, pl.ds(r0, rn), :] = u.astype(BF16)
                AB[0, pl.ds(528 + r0, rn), :] = v.astype(BF16)
            else:
                AB[0, pl.ds(512, 16), :] = jnp.concatenate([u, jnp.zeros_like(u)], 0).astype(BF16)
            yield _Step(rn, [anchor(abu)], delay=1, marks=[("read", name)] if r0 == 512 else [])
        yield settle(abu, 4)

        def s_inverse(point):
            z = opaque()
            fa, fb = mat(M_FA + j + z), mat(M_FB + j + z)
            first = _iota(8, 0) == 0

            def put(row, v, v0=None):
                if v0 is not None:
                    v = jnp.concatenate([jnp.where(first, v0, v[:8]), v[8:]], 0)
                UB[0, pl.ds(row, 64), :] = v.astype(BF16)

            for k in range(4):
                lo, hi = 32 * k, 32 * (8 - k if k else 4)
                a = [abu[z, pl.ds(lo, 32), :], abu[z, pl.ds(hi, 32), :]] if k % 2 else [
                    tied(lambda r, o=o: abu[z, pl.ds(o + r, 8), :], 4, point) for o in (lo, hi)]
                if k == 0:
                    a.append(abu[z, pl.ds(256, 8), :])
                re = _dot_t(_bf(jnp.concatenate(a, 0)), fa)
                im = _dot_t(_bf(jnp.concatenate(
                    [abu[z, pl.ds(264 + lo, 32), :], abu[z, pl.ds(264 + hi, 32), :]], 0)), fb)
                pr, mr, pi, mi = re[:64], re[64:128], im[:64], im[64:]
                if k == 0:
                    put(0, pr)
                    put(64, pi, re[128:136])
                    put(128, mr)
                    put(192, mi)
                else:
                    put(256 * k, pr + mr, pr[:8])
                    put(256 * k + 64, pi + mi, mr[:8])
                    put(256 * k + 128, pi - mi, pi[:8])
                    put(256 * k + 192, mr - pr, -mi[:8])
            return 190

        yield _Mat(s_inverse)
        yield settle(ubu, 4)
        yield d_stage(t, lambda c: {0: M_R0T, 1: M_C4T}.get(c, M_RT))
        yield settle(PB, 4)
        z = opaque()
        acc = None
        for r in range(16):
            rows = pl.ds(8 * r, 8)
            t0, t4 = PB[z, rows, :], PB[z, pl.ds(128 + 8 * r, 8), :]
            tk = {}
            for k in (1, 2, 3):
                c, sn = twid[z + 2 * k - 2, rows, :], twid[z + 2 * k - 1, rows, :]
                re = PB[z, pl.ds(256 * k + 8 * r, 8), :]
                im = PB[z, pl.ds(256 * k + 128 + 8 * r, 8), :]
                tk[k] = (re * c - im * sn, re * sn + im * c)
            e0, e1 = t0 + t4, t0 - t4
            s = [e0 + tk[2][0], e1 - tk[2][1], e0 - tk[2][0], e1 + tk[2][1]]
            al, be = tk[1][0] - tk[3][0], tk[1][1] + tk[3][1]
            o = [tk[1][0] + tk[3][0], (al - be) * RSQ2, tk[3][1] - tk[1][1], (al + be) * -RSQ2]
            for b in range(8):
                y = s[b] + o[b] if b < 4 else s[b - 4] - o[b - 4]
                v = X[i][g, pl.ds(128 * b + 8 * r, 8), :] + y
                X[i][n, pl.ds(128 * b + 8 * r, 8), :] = v
                acc = v if acc is None else acc + v
            yield _Step(57, [lambda v=acc: v], delay=5 if r == 15 else 2)
        yield settle(X[i], 4)
        mean = _all_sublanes(acc, jnp.add, 0) * (1.0 / D)
        rstd = yield from ln_rstd(n, i, mean)
        z = opaque()
        for r in range(8):
            v = X[i][n + z, pl.ds(128 * r, 128), :].reshape(16, 8, 128)
            HB[i][n, pl.ds(128 * r, 128), :] = ((v - mean[None]) * rstd[None]).reshape(128, 128).astype(BF16)
            yield _Step(41, [anchor(hbu[i])], delay=1, marks=[name] if r == 7 else [])

    def attend(g, i, name, needs):
        yield _Wait(*needs)
        yield settle(QB[i])
        j, z = g + 4 * i, opaque()
        even = (_iota(8, 0) & 1) == 0
        edge = _iota(8, 1) == 0

        def window(near, far, w, rows):
            return near[j + z + 4 - 2 * w, rows, :] if w <= 2 * i + 2 else far[j + z + 16 - 2 * w, rows, :]

        def mix_values(h, u):
            p = PW[h % 2][opaque()]
            for rows in (pl.ds(256 * h + 16 * u, 16), pl.ds(256 * h + 16 * u + 16, 16)):
                acc = functools.reduce(jnp.add, [p[16 * w:16 * w + 16] * window(VE, VS, w, rows)
                                                 for w in range(8)])
                HB[i][g, rows, :] = acc.astype(BF16)
            return _Step(63, [anchor(hbu[i])], delay=2, marks=[name] if (h, u) == (3, 14) else [])

        for h in range(5):
            logits = []
            for w0 in range(0, 8, 2):
                if h < 4:
                    rows = pl.ds(256 * h, 256)
                    q = q if w0 % 4 else QB[i][opaque(), rows, :]
                    for w in (w0, w0 + 1):
                        v = (q * window(KE, KS, w, rows)).reshape(16, 16, 128).sum(0)
                        v = jnp.where(even, v[:8] + pltpu.roll(v[:8], 7, 0), v[8:] + pltpu.roll(v[8:], 1, 0))
                        logits.append(jnp.where(edge & (2 * w > j), -1e9, v * SCALE) if w > 2 * i
                                      else v * SCALE)
                    yield _Step(138, [lambda v=v: v for v in logits[-2:]], delay=4)
                if h > 0:
                    yield mix_values(h - 1, 2 * w0)
                    yield mix_values(h - 1, 2 * w0 + 2)
            if h < 4:
                top = functools.reduce(jnp.maximum, logits)
                e = [jnp.exp(v - top) for v in logits]
                total = functools.reduce(jnp.add, e)
                yield _Step(30, [lambda v=total: v], delay=3)
                scale = 1.0 / total
                for w in range(8):
                    v = e[w] * scale
                    PW[h % 2][0, pl.ds(16 * w, 8), :] = jnp.where(even, v, pltpu.roll(v, 1, 0))
                    PW[h % 2][0, pl.ds(16 * w + 8, 8), :] = jnp.where(even, pltpu.roll(v, 7, 0), v)
                yield _Step(50, [anchor(PW[h % 2])], delay=6 if h == 3 else 1)

    def packed_sums(terms, signs):
        lo = [pltpu.bitcast(u << 16, F32) for u in terms]
        hi = [pltpu.bitcast(u & np.uint32(0xFFFF0000), F32) for u in terms]
        return [pltpu.pack_elementwise([v[p] + v[q] if s > 0 else v[p] - v[q] for v in (lo, hi)],
                                       packed_dtype=BF16) for p, s, q in signs]

    def half(ref, row):
        return lambda r, size, cols: ref[pl.ds(pl.multiple_of(row + r, 8), size), cols]

    kv_weight = (WS5, half(WK, 0), half(WV, 0))
    q_weight = (WQ5, half(WQ, 0), half(WQ, D // 4))
    o_weight = (WP5, *(lambda r, size, cols, e=e: WP[pl.ds(r + r // 32 * 32 + e, size), cols]
                       for e in (0, 32)))

    def left_sums(weight, row, size, needs=()):
        yield _Wait(*needs)
        sums, top, bottom = weight
        for r in range(0, size, 8):
            a = [ref(row + r, 8, pl.ds(c, 512)) for ref in (top, bottom) for c in (0, 512)]
            for e, v in enumerate(packed_sums(a, ((0, 1, 3), (2, 1, 3), (0, 1, 1), (2, -1, 0), (1, -1, 3)))):
                sums[e, pl.ds(pl.multiple_of(row + r, 8), 8), :] = v
            yield _Step(92, [anchor(sums)], delay=2, marks=["sums"] if r == size - 8 else [])

    def right_sums(dst, g, i, name, needs):
        yield _Wait(*needs)
        z = g + opaque()
        for r in range(0, 256, 16):
            b = [hbu[n][z, pl.ds(k + r, 16), :] for k in (0, 256) for n in (i, i + 1)]
            for e, v in enumerate(packed_sums(b, ((0, 1, 3), (1, -1, 3), (2, -1, 0), (0, 1, 1), (2, 1, 3)))):
                dst[e, pl.ds(r, 16), :] = v
            yield _Step(47, [anchor(dst)], delay=SETTLE if r == 240 else 1,
                        marks=[name] if r == 240 else [])

    def strassen(sch, weight, right, g, i, m, store, needs, marks):
        for n in needs:
            sch.run(n)
        sums, top, bottom = weight
        rows = pl.ds(pl.multiple_of(64 * m, 64), 64)

        def product(left, b):
            sch.fresh = True
            head = tied(lambda r: left(32 * m + r, 8, pl.ds(0, 128)), 4, lambda: sch.point(8.0))
            return _dot(_bf(jnp.concatenate([head, left(32 * m, 32, pl.ds(128, 384))], 1)), _bf(b))

        def a(e):
            return lambda r, size, cols: sums[e, pl.ds(pl.multiple_of(r, 8), size), cols]

        def b(e):
            return right[e + opaque()]

        m2 = product(a(1), hbu[i][g + opaque(), pl.ds(0, 256), :])
        m4 = product(lambda r, size, cols: bottom(r, size, pl.ds(512 + cols.start, cols.size)), b(2))
        store(1, i, rows, m2 + m4)
        m1 = product(a(0), b(0))
        c11, c22 = m1 + m4, m1 - m2
        c11 = c11 + product(a(4), b(4))
        c22 = c22 + product(a(3), b(3))
        m5 = product(a(2), hbu[i + 1][g + opaque(), pl.ds(256, 256), :])
        store(0, i, rows, c11 - m5)
        v = product(top, b(1))
        store(0, i + 1, rows, v + m5)
        store(1, i + 1, rows, c22 + v)
        sch.results.append(v[:8])
        for name in marks:
            sch.done[name] = sch.slot + sch.wait

    def kv_proj(sch, g, i, name, needs):
        def store(lower, n, rows, v):
            (KE, VE)[lower][g + 4 * n + 4, rows, :] = v
        for m in range(16):
            strassen(sch, kv_weight, SB[i // 2], g, i, m, store, needs, [name] if m == 15 else [])

    def q_proj(sch, g, i, name, needs):
        def store(lower, n, rows, v):
            QB[n][0, pl.ds(512 * lower + rows.start, 64), :] = v
        for m in range(8):
            strassen(sch, q_weight, SB[i // 2], g, i, m, store, needs, [name] if m == 7 else [])

    def o_proj(sch, g, i, m, needs, marks, right):
        def store(lower, n, rows, v):
            rows = pl.ds(128 * m + 64 * lower, 64)
            X[n][g, rows, :] = X[n][g, rows, :] + v
        strassen(sch, o_weight, right, g, i, m, store, needs, marks)

    def shift_block(g, i, name, needs):
        yield _Wait(*needs)
        j, z = g + 4 * i, opaque()
        for m in range(16):
            rows = pl.ds(64 * m, 64)
            for ref, to in ((KE, KS), (VE, VS)):
                v = pltpu.roll(ref[j + 4 + z, rows, :], 1, 1)
                if ref is VE:
                    v = jnp.where(_iota(64, 1) == 0, ref[4 + z, rows, :], v)
                to[j, rows, :] = v
                if i == 3:
                    ref[g, rows, :] = v
            yield _Step(12, delay=8, marks=[name] if m == 15 else [])

    def transpose_quarter(w, h, via):
        for r in range(4):
            v = WRAW[w, pl.ds(256 * r, 256), pl.ds(pl.multiple_of(256 * h, 256), 256)]
            v = pltpu.bitcast(v.T, F32)
            via[0, pl.ds(256 * r, 128), :], via[0, pl.ds(256 * r + 128, 128), :] = v[:, :128], v[:, 128:]
            yield _Step(40, delay=16)

    def reorder_quarter(w, h, via, name=None):
        z = 0 if isinstance(h, int) else opaque()
        for c in range(8):
            WT[w][pl.ds(pl.multiple_of(128 * h, 128), 128), pl.ds(128 * c, 128)] = pltpu.bitcast(
                jnp.concatenate([via[z, pl.ds(128 * c + u, 8, stride=16), :] for u in range(16)], 0), U32)
            yield _Step(20, delay=4, marks=[name] if c == 7 else [])

    def query_weight(h):
        yield from transpose_quarter(0, h, QB[0])
        yield from reorder_quarter(0, h, QB[0], "w")

    def transpose_wo(name):
        for c in range(8):
            for h, e in itertools.product(range(4), range(2)):
                v = jnp.concatenate([wou[c, pl.ds(128 * h + 8 * e + u, 8, stride=16), :]
                                     for u in range(8)], 0)
                WP[pl.ds(64 * c, 64), pl.ds(256 * h + 128 * e, 128)] = pltpu.bitcast(_bf(v).T, U32)
                yield _Step(10, delay=5, marks=[name] if (c, h, e) == (7, 3, 1) else [])

    def prep_spectral_weights(c2):
        def words(k2):
            re, im = (wsu[u, k2, pl.ds(c2, 64, stride=4), :] for u in range(2))
            return ((re & np.uint32(0xFFFF)) | (im << 16), (re >> 16) | (im & np.uint32(0xFFFF0000)))

        def arrange(w, below):
            return jnp.where(_iota(w.shape[0], 1) < 64, w, below)

        below = words(15)
        for k2 in range(16):
            here = words(k2)
            for e in range(2):
                cl = 2 * c2 + e
                w = arrange(here[e], below[e])
                WS[k2, pl.ds(64 * cl, 64), :] = pltpu.roll(w, 1, 0) if cl > 4 else w
            below = here
            yield _Step(90, delay=3)
        if c2 == 0:
            def nyquist(k2):
                re, im = (jnp.broadcast_to(WN[u, :, pl.ds(128 * k2, 128)].astype(F32), (8, 128))
                          for u in range(2))
                return pltpu.pack_elementwise([re, im], packed_dtype=BF16)
            for k2 in range(16):
                WS[k2, pl.ds(512, 8), :] = arrange(nyquist(k2), nyquist((k2 + 15) % 16))

    def write_out(p, c, name, needs):
        yield _Wait(*needs)
        rows = pl.ds(pl.multiple_of(128 * c, 128), 128)
        g, i = 2 * p % 4 + opaque(), p // 2
        w = pltpu.pack_elementwise([X[i][g, rows, :], X[i][g + 1, rows, :]], packed_dtype=BF16)
        xru[c, pl.ds(p, 128, stride=8), :] = w.T
        yield _Step(30, marks=[name])

    tables = [pltpu.make_async_copy(lanes_hbm, lanes, sems.at[24]),
              pltpu.make_async_copy(mats_hbm, mats.at[pl.ds(M_R, 5)], sems.at[25])]
    start_all(tables + [x_copy(c) for c in range(8)])
    for c in tables:
        c.wait()

    def make_twiddle(k):
        PB = temps[0][2]
        PB[0, pl.ds(0, 128), :] = lane_vec(L_TWID + k, 128)
        twid[k] = PB[opaque(), pl.ds(0, 128), :].T

    _loop(6, make_twiddle, "make_twiddle")

    def make_dft(j):
        fa, fb = lanes[pl.ds(L_FA, 128), :], lanes[pl.ds(L_FB, 128), :]
        c, sn = lane_vec(L_COS + j, 128), lane_vec(L_SIN + j, 128)
        UB, _, _, ubu, _ = temps[0]
        UB[0, pl.ds(0, 128), :] = (fa * c + fb * sn).astype(BF16)
        UB[0, pl.ds(128, 128), :] = (fb * c - fa * sn).astype(BF16)
        mats[M_FA + j], mats[M_FB + j] = ubu[0, pl.ds(0, 64), :], ubu[0, pl.ds(64, 64), :]

    _loop(NB, make_dft, "make_dft")

    def load_x(c):
        x_copy(c).wait()
        pl.when(c == 6)(lambda: start_all(spec_copies[0]))
        pl.when(c == 7)(lambda: start_all(spec_copies[1]))
        rows = pl.ds(pl.multiple_of(128 * c, 128), 128)
        for p in range(8):
            w = xru[c, pl.ds(p, 128, stride=8), :].T
            for e, bits in enumerate((w << 16, w & np.uint32(0xFFFF0000))):
                g, i = 2 * p % 4 + e, p // 2
                v = pltpu.bitcast(bits, F32)
                X[i][g, rows, :] = v
                v = v.reshape(16, 8, 128)
                mean = _all_sublanes(v.sum(0), jnp.add, 0) * (1.0 / 128)
                STAT[4 * g + i, c] = mean
                STAT[4 * g + i, 8 + c] = _all_sublanes(((v - mean) ** 2).sum(0), jnp.add, 0)

    _loop(8, load_x, "load_x")

    def after(name, action):
        yield _Wait(name)
        action()

    def spectral_weights():
        yield _Wait(("f", 2, 1))
        for c in spec_copies[0] + spec_copies[1]:
            c.wait()
        for c2 in range(4):
            yield from prep_spectral_weights(c2)

    with jax.named_scope("first_forward"):
        sch = _Sched(0.72, 20)
        sch.add(after(("f", 0, 1), w_copies[1].start), "k")
        sch.add(after(("f", 1, 1), w_copies[2].start), "v")
        sch.add(after(("f", 2, 3), w_copies[0].start), "q")
        for g in range(4):
            for i in range(4):
                sch.add(fwd_block(g, i, ("f", g, i), [("f", g - 1, i)] if g else [],
                                  [("r", g - 1)] if g else [], True), ("f", g, i))
            sch.add(group_stage(g, ("r", g), [("f", g, i) for i in range(4)], False), ("r", g))
        sch.add(spectral_weights(), "s")
        sch.drive()
    start_all(wo_copies)

    def keys_values(layer, g):
        sch = _Sched(0.41, 32, 3) if layer == 0 else _Sched(0.36, 28, 2)
        nxt = (g + 1) % 4
        sch.add(inv_block(g, 2, ("i", 2), []), ("i", 2))
        sch.add(inv_block(g, 3, ("i", 3), [("read", ("i", 2))]), ("i", 3))
        sch.add(right_sums(SB[1], g, 2, ("b", 2), [("i", 2), ("i", 3)]), ("b", 2))
        sch.add(group_stage(nxt, "r", [("read", ("i", 3))], True), "r")
        sch.add(inv_block(nxt, 0, ("i", 4), ["r", ("i", 2)], n=g + 1), ("i", 4))
        sch.add(inv_block(nxt, 1, ("i", 5), [("read", ("i", 4)), ("i", 3)], n=g + 1), ("i", 5))
        if layer == 0:
            sch.add(query_weight(g), "w")
            sch.add(left_sums(q_weight, 128 * (g % 2), 128, ["w"]), "sums")
        for i in (2, 3):
            sch.add(shift_block((g + 3) % 4, i, ("s", i), []), ("s", i))
        for i in (0, 1):
            sch.add(shift_block(g, i, ("s", i), [("kv", 0)]), ("s", i))
        sch.add(right_sums(SB[0], nxt, 0, ("b", 4), [("i", 4), ("i", 5), ("kv", 0)]), ("b", 4))
        kv_proj(sch, g, 0, ("kv", 0), [])
        kv_proj(sch, g, 2, ("kv", 2), [("b", 2)])
        sch.finish()

    def mix(g, after, last):
        tail = after is None
        sch = _Sched(0.66 if last else 0.63, 28 if last else 32)
        pace = 0.48 if tail else 0.35 if last else 0.32
        ahead = [(g, 2), (g, 3)] + ([] if tail else [(after, 0), (after, 1)])
        for n, block in enumerate(ahead):
            sch.add(attend(*block, ("a", n), [[], [("a", 0)], [("a", 1), ("q", 0)], [("a", 2)]][n]),
                    ("a", n), pace=pace)
            if n % 2:
                sch.add(right_sums(SB[2 + block[1] // 2], block[0], block[1] - 1, ("b", n),
                                   [("a", n)] + ([("o", 0)] if n == 3 else [])), ("b", n))
        for i in () if tail else (0, 2):
            sch.add(right_sums(SB[i // 2], after, i, ("h", i), [("q", 0)] if i else []), ("h", i))
        if not last:
            sch.add(group_stage((g + 3) % 4, "r", [], False), "r")
            for i in range(4):
                sch.add(fwd_block(g, i, ("f", i), [("o", i - i % 2)], ["r"]), ("f", i))
        now = 6 if last else 8
        for i in (0, 2):
            for m in range(now):
                o_proj(sch, g, i, m, [("b", 1)] if i else [], [("o", i)] if m == now - 1 else [],
                       SB[2 + i // 2])
            if not tail:
                q_proj(sch, after, i, ("q", i), [("h", i)])
        if tail:
            sch.add(group_stage(g, "s", [("f", i) for i in range(4)], False), "s")
        sch.share = 0.92
        sch.drive()

    def mix_odd():
        sch = _Sched(0.66)
        blocks = [(1, 2), (1, 3), (3, 0), (3, 1), (3, 2), (3, 3)]
        for n, (g, i) in enumerate(blocks):
            sch.add(attend(g, i, ("a", n), ([("a", n - 1)] if n else []) + ([("q", i)] if n in (2, 4) else [])),
                    ("a", n), pace=0.32)
            if n % 2:
                sch.add(right_sums(SB[(3, 2, 0)[n // 2]], g, i - 1, ("b", g, i - 1),
                                   [("a", n)] + ([("o", 1, 0, 5)] if n > 1 else [])), ("b", g, i - 1))
        for i in (0, 2):
            sch.add(right_sums(SB[i // 2], 3, i, ("h", i), []), ("h", i))
        for g in (1, 3):
            for i in range(4):
                for c in range(6):
                    sch.add(write_out(2 * i + g // 2, c, ("w", g, i, c), [("o", g, i - i % 2, c)]),
                            ("w", g, i, c))
        for g, i, slot, count in ((1, 0, 2, 6), (1, 2, 3, 8), (3, 0, 2, 8), (3, 2, 0, 6)):
            for m in range(count):
                o_proj(sch, g, i, m, [("b", g, i)] if (g, i) != (1, 0) else [], [("o", g, i, m)], SB[slot])
            for e in (0, 2) if (g, i) == (1, 0) else ():
                q_proj(sch, 3, e, ("q", e), [("h", e)] + ([("a", 1)] if e else []))
        sch.share = 0.92
        sch.drive()

    def copy_out(chunks):
        def start(_):
            for c in chunks:
                out_copy(c).start()
        _loop(zero + 1, start, "copy_out")

    def postponed():
        slots = {(3, 2): 0, (2, 2): 1, (0, 2): 2, (2, 0): 3, (0, 0): 0, (1, 0): 1}
        early, late = list(slots)[:2], list(slots)[2:]
        sources = 2 * [[(0, 0), (1, 0)], [(2, 0)]] + 2 * [[(0, 2)], []]
        for c in (6, 7):
            sch = _Sched(0.7, 12)
            for n, (pair, slot) in enumerate(slots.items()) if c == 6 else ():
                if n:
                    sch.add(right_sums(SB[slot], *pair, pair, [(early[n - 4], 7)] if n >= 4 else []), pair)
            for p in (5, 7, 4, 6, 1, 3, 0, 2):
                sch.add(write_out(p, c, ("w", p), [(pair, c) for pair in sources[p] or early * (c == 6)]),
                        ("w", p))
            for pair, m in [(pair, m) for m in (6, 7) for pair in early] * (c == 6) + [(v, c) for v in late]:
                o_proj(sch, *pair, m, [pair] if c == 6 and pair != (3, 2) else [], [(pair, m)],
                       SB[slots[pair]])
            sch.drive()
            copy_out([c])

    def first_queries(layer):
        sch = _Sched(0.68)
        sch.add(right_sums(SB[1], 0, 2, ("h", 2), []), ("h", 2))
        sch.add(shift_block(3, 2, "s", []), "s")
        sch.add(attend(0, 0, ("a", 0), ["q"]), ("a", 0), pace=0.4)
        sch.add(attend(0, 1, ("a", 1), [("a", 0)]), ("a", 1), pace=0.4)
        sch.add(right_sums(SB[2], 0, 0, "b", [("a", 1)]), "b")
        sch.add(shift_block(3, 3, "t", []), "t")
        if layer == 0:
            for c in wo_copies:
                c.wait()
            sch.add(transpose_wo("w"), "w")
            sch.add(left_sums(o_weight, 0, 256, ["w"]), "sums")
        q_proj(sch, 0, 0, "q", [])
        q_proj(sch, 0, 2, None, [("h", 2)])
        sch.finish()

    def key_value_weights():
        w_copies[1].wait()
        w_copies[2].wait()
        for h in range(6):
            work = []
            for w in (1, 2):
                if h < 4:
                    work.append(transpose_quarter(w, h, QB[2 * (h % 2) + w - 1]))
                if 0 < h < 5:
                    work.append(reorder_quarter(w, h - 1, QB[2 * ((h - 1) % 2) + w - 1]))
            if h > 1:
                work.append(left_sums(kv_weight, 128 * (h - 2), 128))
            list(itertools.zip_longest(*work))

    for layer in range(2):
        with jax.named_scope("spectral"):
            _loop(4, spectral_rows, "rows")
            if layer == 0:
                _loop(zero + 1, lambda _: key_value_weights(), "weights")
            spectral(512, 8)
        sch = _Sched(0.92)
        sch.add(group_stage(0, "r", [], True), "r")
        sch.add(inv_block(0, 0, ("i", 0), ["r"]), ("i", 0))
        sch.add(inv_block(0, 1, ("i", 1), ["r"]), ("i", 1))
        sch.add(right_sums(SB[0], 0, 0, "b", [("i", 0), ("i", 1)]), "b")
        sch.drive()
        if layer == 0:
            w_copies[0].wait()
        _loop(4, lambda g: keys_values(layer, g), "keys_values")
        first_queries(layer)
        if layer == 0:
            pl.when(never)(lambda: [spectral_rows(c) for c in range(3)] and None)
        if layer == 0:
            _loop(3, lambda g: mix(g, g + 1, False), "mix")
            mix(3, None, False)
        else:
            _loop(2, lambda u: mix(2 * u, 2 - u, True), "mix")
            mix_odd()
    copy_out(range(6))
    postponed()
    for c in range(8):
        out_copy(c).wait()


@jax.jit
def pallas_interleave_layers__spectral_gfnet__sliding_local_dilated__prompt_kernel(
    A_x: jax.Array,
    A_w_r: jax.Array,
    A_w_i: jax.Array,
    B_x: jax.Array,
    B_wqkv: jax.Array,
    B_wo: jax.Array,
):
    del B_x
    hbm = pl.BlockSpec(memory_space=pl.ANY)
    smem = pl.BlockSpec(memory_space=pltpu.SMEM)
    out = pl.pallas_call(
        _kernel,
        out_shape=jax.ShapeDtypeStruct((S, D), BF16),
        in_specs=[smem, smem, hbm, hbm, hbm, hbm, hbm, hbm, hbm],
        out_specs=hbm,
        scratch_shapes=[
            pltpu.VMEM(_LANES.shape, F32),
            pltpu.VMEM((37, 64, 128), U32),
            pltpu.VMEM((6, 128, 128), F32),
            pltpu.VMEM((NB, 16, 8, 128), F32),
            pltpu.VMEM((NB + 4, D, 128), F32),
            pltpu.VMEM((NB + 4, D, 128), F32),
            pltpu.VMEM((NB, D, 128), F32),
            pltpu.VMEM((NB, D, 128), F32),
            pltpu.VMEM((2 * NB + 1, ZR, 128), F32),
            pltpu.VMEM((9, ZR, 128), F32),
            pltpu.VMEM((NB, ZR, 128), U32),
            *4 * [pltpu.VMEM((D // 2, D), U32)],
            pltpu.VMEM((5, D // 2, D // 2), U32),
            *2 * [pltpu.VMEM((5, D // 4, D // 2), U32)],
            *4 * [pltpu.VMEM((5, D // 4, 128), U32)],
            pltpu.VMEM((8, S, 128), BF16),
            pltpu.VMEM((2, NB, D // 2, 128), BF16),
            pltpu.VMEM((2, 1, S), BF16),
            pltpu.VMEM((3, D, D), BF16),
            pltpu.VMEM((8, D, 128), BF16),
            pltpu.VMEM((1, 128, 128), F32),
            pltpu.VMEM((1, 128, 128), F32),
            pltpu.SemaphoreType.DMA((26,)),
            *2 * [pltpu.VMEM((1, D, 128), F32)],
        ] + 4 * [
            pltpu.VMEM((5, D, 128), F32),
            pltpu.VMEM((5, D, 128), BF16),
            pltpu.VMEM((1, D, 128), F32),
            pltpu.VMEM((1, D, 128), BF16),
            pltpu.VMEM((1, 1152, 128), BF16),
        ],
        compiler_params=pltpu.CompilerParams(vmem_limit_bytes=126 * 2 ** 20),
    )(_ZERO, _ROT, _MATS, _LANES, A_x.reshape(S, D), A_w_r.T, A_w_i.T, B_wqkv, B_wo)
    return out.reshape(1, S, D)
```

```python
import functools
import itertools

import numpy as np

import jax
import jax.numpy as jnp
import jax.experimental.pallas as pl
import jax.experimental.pallas.tpu as pltpu

S, D, NB = 2048, 1024, 16
ZR = 576
F32, BF16, U32, I32 = jnp.float32, jnp.bfloat16, jnp.uint32, jnp.int32
EPS = 1e-5
SCALE = 32 ** -0.5
RSQ2 = float(np.sqrt(0.5))
SETTLE = 6

_S_ROWS = [(32 * u, 32) for u in range(16)] + [(512, 8)]

M_FA, M_FB, M_R, M_C4, M_RT, M_C4T, M_R0T = 0, 16, 32, 33, 34, 35, 36
L_MU, L_NU, L_KU, L_KV, L_COS, L_SIN, L_TWID, L_FA, L_FB = 0, 16, 32, 48, 64, 80, 96, 104, 232


def _bf16_bits(a):
    u = np.ascontiguousarray(a, dtype=np.float32).view(np.uint32).astype(np.uint64)
    return ((u + 0x7FFF + ((u >> 16) & 1)) >> 16).astype(np.uint32)


def _constants():
    a = np.arange(128)
    k1 = np.arange(64)
    alt = (-1.0) ** a
    lanes = np.zeros((384, 128))
    t = 2 * np.pi * np.outer(a, k1) / 128
    fa = np.concatenate([np.cos(t), -np.sin(t)], 1)
    fb = np.concatenate([np.sin(t), -np.cos(t)], 1)
    fa[:, 0], fb[:, 0] = RSQ2, -RSQ2
    fa[:, 64], fb[:, 64] = alt, 0.0
    lanes[L_FA:L_FA + 128], lanes[L_FB:L_FB + 128] = fa, fb
    for j in range(NB):
        ang = 2 * np.pi * j / 32 + np.pi / 32
        p, q = (_bf16_bits([np.cos(ang), np.sin(ang)]) << 16).view(np.float32).astype(np.float64)
        turn = 2 * np.pi * j * np.tile(k1, 2) / S
        lanes[L_COS + j], lanes[L_SIN + j] = np.cos(turn), np.repeat([-1.0, 1.0], 64) * np.sin(turn)
        lanes[L_COS + j, 64], lanes[L_SIN + j, 64] = p, q
        lanes[L_MU + j, 0], lanes[L_MU + j, 64] = 1.0, (q / p + p / q) / 2
        lanes[L_NU + j, 0], lanes[L_NU + j, 64] = 0.0, (q / p - p / q) / 2
        lanes[L_KU + j, 0], lanes[L_KU + j, 64] = 1.0, q / p
        lanes[L_KV + j, 0], lanes[L_KV + j, 64] = 1.0, p / q
    lanes[:, 65:] = lanes[:, :64:-1].copy()
    for k in (1, 2, 3):
        lanes[L_TWID + 2 * k - 2] = np.cos(2 * np.pi * a * k / D)
        lanes[L_TWID + 2 * k - 1] = np.sin(2 * np.pi * a * k / D)
    th = 2 * np.pi * np.outer(k1, a) / 128
    r = np.concatenate([np.cos(th), -np.sin(th)], 0)
    r[64] = alt
    th = 2 * np.pi * np.outer(2 * k1 + 1, a) / 256
    c4 = np.concatenate([np.cos(th), -np.sin(th)], 0)
    inv = 2.0 / (S * D)
    r0t = inv * r.T
    r0t[:, 0::64] *= 0.5
    rows = np.arange(128).reshape(2, 4, 16).transpose(1, 0, 2).ravel()
    bits = _bf16_bits(np.stack([r[rows], c4[rows], inv * r.T, inv * c4.T, r0t]))
    ang = 2 * np.pi * np.outer(np.arange(4), np.arange(4)).ravel() / 16
    rot = np.concatenate([np.cos(ang), np.sin(ang)]).astype(np.float32)
    return bits[:, 0::2] | (bits[:, 1::2] << 16), lanes.astype(np.float32), rot


_MATS, _LANES, _ROT = _constants()
_ZERO = np.zeros((1,), np.int32)


class _Step:
    def __init__(self, cost, anchors=(), delay=0, marks=()):
        self.cost, self.anchors, self.delay, self.marks = cost, list(anchors), delay, list(marks)


class _Wait:
    def __init__(self, *names):
        self.names = names


class _Mat:
    def __init__(self, emit):
        self.emit = emit


class _Hold:
    def __init__(self, store):
        self.store = store


class _Task:
    def __init__(self, gen, pace):
        self.gen, self.pace, self.blocked, self.not_before, self.held = gen, pace, (), 0, None
        self.allowed = 0.0


class _Sched:
    def __init__(self, share=0.0, wait=28, lag=3):
        self.lag = lag
        self.wait = wait
        self.share = share
        self.tasks, self.done, self.producer = [], {}, {}
        self.slot, self.credit, self.anchors, self.results = 0, 0.0, [], []
        self.fresh = False

    def add(self, gen, name, pace=99):
        self.producer[name] = self.producer["read", name] = _Task(gen, pace)
        self.tasks.append(self.producer[name])

    def _ready(self, t):
        return t.not_before <= self.slot and all(
            n in self.done and self.done[n] <= self.slot for n in t.blocked)

    def _advance(self, t, mats=True):
        item, t.held = t.held or next(t.gen, None), None
        if item is None:
            self.tasks.remove(t)
        elif isinstance(item, _Wait):
            t.blocked = item.names
        elif isinstance(item, _Hold):
            if len(self.results) >= self.lag:
                item.store(self.results[-self.lag])
        elif isinstance(item, _Mat):
            if mats:
                t.not_before = float("inf")
                self.fresh = False
                self.credit -= item.emit(lambda: self.point(0.0)) or 0
                t.not_before = self.slot + self.wait
            else:
                t.held, t.not_before = item, self.slot + 1
        else:
            t.blocked = ()
            t.not_before = self.slot + item.delay
            self.credit -= item.cost
            self.anchors += item.anchors
            for n in item.marks:
                self.done[n] = self.slot + item.delay
            return True

    def run(self, *names):
        while not all(n in self.done for n in names):
            for n in names:
                if n not in self.done:
                    for b in self.producer[n].blocked:
                        self.run(b)
                    self._advance(self.producer[n])

    def drive(self):
        while self.tasks:
            ready = [t for t in self.tasks if self._ready(t)]
            if not ready:
                self.slot += 1
                continue
            self.anchors, self.credit = self.anchors[-2:], 0.0
            self._advance(next((t for t in ready if t.held), ready[0]))
            self.slot -= min(self.credit, 0.0) / 60

    def finish(self):
        self.run(*[n for n in self.producer if n[0] != "read"])

    def point(self, own):
        for t in self.tasks:
            t.allowed = min(t.allowed, 0.0) + t.pace
        while True:
            t = next((t for t in self.tasks if self._ready(t) and t.allowed > 0
                      and self.credit > 0), None)
            if t is None:
                break
            if self._advance(t, self.fresh):
                t.allowed -= 1
        anchors, self.anchors = self.anchors, []
        self.credit = min(self.credit, 10.0) + 64 * self.share - own
        self.fresh = False
        self.slot += 1
        return anchors


def _dot(a, b):
    return jnp.dot(a, b, preferred_element_type=F32)


def _dot_t(a, b):
    return jax.lax.dot_general(a, b, (((1,), (1,)), ((), ())), preferred_element_type=F32)


def _bf(u):
    return pltpu.bitcast(u, BF16)


def _iota(rows, dim):
    return jax.lax.broadcasted_iota(I32, (rows, 128), dim)


def _mirror(v):
    index = -_iota(8, 1) & 127
    return jnp.concatenate([jnp.take_along_axis(v[r:r + 8], index, axis=1)
                            for r in range(0, v.shape[0], 8)], 0)


def _radix4(z, inverse):
    (r0, i0), (r1, i1), (r2, i2), (r3, i3) = z
    ar, ai, cr, ci = r0 + r2, i0 + i2, r0 - r2, i0 - i2
    br, bi, dr, di = r1 + r3, i1 + i3, r1 - r3, i1 - i3
    lo, hi = (cr + di, ci - dr), (cr - di, ci + dr)
    if inverse:
        lo, hi = hi, lo
    return [(ar + br, ai + bi), lo, (ar - br, ai - bi), hi]


def _all_sublanes(v, op, axis):
    for sh in (4, 2, 1):
        v = op(v, pltpu.roll(v, sh, axis))
    return v


def _loop(n, body, name):
    def step(i, carry):
        body(i)
        return carry
    with jax.named_scope(name):
        jax.lax.fori_loop(0, n, step, 0)


def _kernel(zero_ref, rot, mats_hbm, lanes_hbm, x_hbm, wr_hbm, wi_hbm, wqkv_hbm, wo_hbm, out_hbm,
            lanes, mats, twid, STAT, KE, VE, KS, VS, Z, ZT, WS, WQ, WK, WV, WP, WS5, WQ5, WP5,
            SB0, SB1, SB2, SB3, XR, WRI, WN, WRAW, WO, PW0, PW1, sems, *split):
    zero = zero_ref[0]
    never = zero != 0
    X, HB, QB = split[2::5], split[3::5], split[4::5]
    hbu = [r.bitcast(U32) for r in HB]
    xru, wsu, wou = XR.bitcast(U32), WRI.bitcast(U32), WO.bitcast(U32)
    temps = [(ub, ab, pb, ub.bitcast(U32), ab.bitcast(U32))
             for ub, ab, pb in zip(split[5::5], split[6::5], 2 * split[:2])]
    PW, SB, WT = (PW0, PW1), (SB0, SB1, SB2, SB3), (WQ, WK, WV, WP)
    counter = [0]

    def opaque():
        counter[0] += 1
        return zero * counter[0]

    def anchor(ref):
        at = (0,) * (len(ref.shape) - 2)
        return lambda: ref[(*at, pl.ds(pl.multiple_of(zero * 8, 8), 8), pl.ds(0, 128))]

    def settle(ref, points=SETTLE):
        return _Step(2, [anchor(ref)], delay=points)

    def hold(ref, spare):
        def store(v):
            ref[spare, pl.ds(pl.multiple_of(zero * 8, 8), 8), :] = v
        return _Hold(store)

    def tied(load, vregs, point):
        parts = []
        for r in range(vregs):
            anchors = point()
            u = load(8 * r)
            for a in anchors:
                u = jnp.where(never, pltpu.bitcast(a(), U32), u)
            parts.append(u)
        return jnp.concatenate(parts, 0)

    def mat(i):
        return _bf(mats[i])

    def d_stage(t, which):
        UB, AB, PB, ubu, abu = temps[t]

        def emit(point):
            z = opaque()
            for c in range(8):
                lhs = mat(which(c) + opaque()) if c % 4 else _bf(
                    tied(lambda r, u=which(c) + opaque(): mats[u, pl.ds(r, 8), :], 8, point))
                PB[0, pl.ds(128 * c, 128), :] = _dot(lhs, _bf(ubu[z, pl.ds(64 * c, 64), :]))
        return _Mat(emit)

    def lane_vec(i, rows):
        return jnp.broadcast_to(lanes[pl.ds(i, 1), :], (rows, 128))

    def x_copy(c):
        return pltpu.make_async_copy(
            x_hbm.at[:, pl.ds(pl.multiple_of(128 * c, 128), 128)], XR.at[c], sems.at[c])

    def out_copy(c):
        return pltpu.make_async_copy(
            XR.at[c], out_hbm.at[:, pl.ds(pl.multiple_of(128 * c, 128), 128)], sems.at[8 + c])

    spec_copies = [[pltpu.make_async_copy(w.at[pl.ds(0, 512), pl.ds(128 * k2, 128)], WRI.at[u, k2],
                                          sems.at[16 + u]) for k2 in range(16)]
                   + [pltpu.make_async_copy(w.at[pl.ds(512, 1), :], WN.at[u], sems.at[22 + u])]
                   for u, w in enumerate((wr_hbm, wi_hbm))]

    def start_all(copies):
        for c in copies:
            c.start()
    w_copies = [pltpu.make_async_copy(wqkv_hbm.at[:, pl.ds(D * w, D)], WRAW.at[w], sems.at[18 + w])
                for w in range(3)]
    wo_copies = [pltpu.make_async_copy(wo_hbm.at[:, pl.ds(128 * c, 128)], WO.at[c], sems.at[21])
                 for c in range(8)]

    def ln_rstd(g, i, mean):
        acc, m = None, g + opaque()
        for r in range(8):
            d = X[i][m, pl.ds(128 * r, 128), :].reshape(16, 8, 128) - mean[None]
            v = (d * d).sum(0)
            acc = v if acc is None else acc + v
            if r < 7:
                yield _Step(50, [lambda acc=acc: acc], delay=3)
        rstd = jax.lax.rsqrt(_all_sublanes(acc, jnp.add, 0) * (1.0 / D) + EPS)
        yield _Step(50, delay=8)
        yield _Step(10, [lambda: rstd], delay=1)
        return rstd

    def fwd_block(g, i, name, needs, free=(), known=False):
        j, t = g + 4 * i, i
        UB, AB, PB, ubu, abu = temps[t]
        yield _Wait(*needs)
        if known:
            means, squares = STAT[4 * g + i, pl.ds(0, 8)], STAT[4 * g + i, pl.ds(8, 8)]
            mean = means.sum(0) * 0.125
            var = (squares.sum(0) + 128.0 * ((means - mean) ** 2).sum(0)) * (1.0 / D)
            rstd = jax.lax.rsqrt(var + EPS)
            yield _Step(50, delay=6)
        else:
            yield settle(X[i])
            acc, m = None, g + opaque()
            for r in range(8):
                v = X[i][m, pl.ds(128 * r, 128), :].reshape(16, 8, 128).sum(0)
                acc = v if acc is None else acc + v
                if r % 2:
                    yield _Step(35, [lambda acc=acc: acc], delay=7 if r == 7 else 3)
            mean = _all_sublanes(acc, jnp.add, 0) * (1.0 / D)
            rstd = yield from ln_rstd(g, i, mean)
        mean8, rstd = (jnp.concatenate([v, v], 0) for v in (mean * 8.0, rstd))
        z = opaque()
        for r in range(8):
            rows = pl.ds(16 * r, 16)
            x = [X[i][g + z, pl.ds(128 * b + 16 * r, 16), :] for b in range(8)]
            s = [x[b] + x[b + 4] for b in range(4)]
            d = [x[b] - x[b + 4] for b in range(4)]
            e, o = s[0] + s[2], s[1] + s[3]
            UB[0, rows, :] = ((e + o - mean8) * rstd).astype(BF16)
            UB[0, pl.ds(128 + 16 * r, 16), :] = ((e - o) * rstd).astype(BF16)
            t1, t2 = (d[1] - d[3]) * RSQ2, (d[1] + d[3]) * RSQ2
            u = {1: (d[0] + t1, d[2] + t2), 2: (s[0] - s[2], s[1] - s[3]), 3: (d[0] - t1, d[2] - t2)}
            yield _Step(34, [anchor(ubu)], delay=1)
            for k in (1, 2, 3):
                c, sn = twid[z + 2 * k - 2, rows, :] * rstd, twid[z + 2 * k - 1, rows, :] * rstd
                re, m = u[k]
                if k == 3:
                    ur, ui = re * c + m * sn, m * c - re * sn
                else:
                    ur, ui = re * c - m * sn, m * c + re * sn
                UB[0, pl.ds(256 * k + 16 * r, 16), :] = ur.astype(BF16)
                UB[0, pl.ds(256 * k + 128 + 16 * r, 16), :] = ui.astype(BF16)
                yield _Step(26, [anchor(ubu)], delay=1)
        yield settle(ubu)

        def d_forward(point):
            z = opaque()
            first = _iota(8, 0) == 0

            def stage(c):
                u = (M_C4 if c == 1 else M_R) + opaque()
                lhs = mat(u) if c % 4 else _bf(tied(lambda r: mats[u, pl.ds(r, 8), :], 8, point))
                v = _dot(lhs, _bf(ubu[z, pl.ds(64 * c, 64), :]))
                return [(v[32 * u:32 * u + 16], v[32 * u + 16:32 * u + 32]) for u in range(4)]

            def put(row, u, v, v0=None):
                if u == 0 and v0 is not None:
                    v = jnp.concatenate([jnp.where(first, v0, v[:8]), v[8:]], 0)
                AB[0, pl.ds(row + 16 * u, 16), :] = v.astype(BF16)

            for u, (p1, p2) in enumerate(stage(0)):
                put(0, u, p1)
                put(528, u, p2, 0.0)
                if u == 0:
                    put(512, 0, jnp.zeros_like(p2), p2[:8])
            for u, (p1, p2) in enumerate(stage(1)):
                put(256, u, p1)
                put(528 + 256, u, p2)
            for k in (1, 2, 3):
                for u, ((p1, p2), (q1, q2)) in enumerate(zip(stage(2 * k), stage(2 * k + 1))):
                    if k == 3:
                        pr, pi, mr, mi = p1 - q2, p2 + q1, p1 + q2, p2 - q1
                        pi0, mi0 = q1[:8], -q2[:8]
                    else:
                        pr, pi, mr, mi = p1 + q2, p2 - q1, p1 - q2, p2 + q1
                        pi0, mi0 = -q1[:8], q2[:8]
                    put(64 * k, u, pr, p1[:8])
                    put(64 * (8 - k), u, mr, p2[:8])
                    put(528 + 64 * k, u, pi, pi0)
                    put(528 + 64 * (8 - k), u, mi, mi0)
            return 190

        yield _Mat(d_forward)
        yield settle(abu)
        yield _Wait(*free)

        def s_forward(point):
            z = opaque()
            fa, fb = mat(M_FA + j + z), mat(M_FB + j + z)
            for r0, rn in ((0, 256), (256, 272)):
                lhs = abu[z, pl.ds(r0 // 2, rn // 2), :] if r0 else tied(
                    lambda r: abu[z, pl.ds(r, 8), :], 16, point)
                u = _dot(_bf(lhs), fa)
                v = _dot(_bf(abu[z, pl.ds(264 + r0 // 2, 128), :]), fb)
                re, m = u[:256] + v, u[:256] - v
                if r0:
                    re, m = (jnp.concatenate([a, u[256:264]], 0) for a in (re, m))
                rn = re.shape[0]
                edge = (_iota(rn, 1) & 63) == 0
                ZT[2 * i, pl.ds(r0, rn), :] = re
                ZT[2 * i + 1, pl.ds(r0, rn), :] = jnp.where(
                    edge, lane_vec(L_MU + j, rn) * m + lane_vec(L_NU + j, rn) * re, _mirror(m))
            return 400

        yield _Mat(s_forward)
        yield _Step(2, [anchor(ZT)], delay=SETTLE, marks=[name])

    def group_stage(g, name, needs, inverse):
        yield _Wait(*needs)

        def turn(z, k):
            if k == 0 or (isinstance(g, int) and g == 0):
                return z
            if isinstance(g, int) and g * k == 4:
                return (-z[1], z[0]) if inverse else (z[1], -z[0])
            c, s = rot[4 * g + k], rot[16 + 4 * g + k]
            if inverse:
                return z[0] * c - z[1] * s, z[1] * c + z[0] * s
            return z[0] * c + z[1] * s, z[1] * c - z[0] * s

        (src, a), (dst, b) = ((Z, 8 * g), (ZT, 0)) if inverse else ((ZT, opaque()), (Z, 8 * g))
        for r in range(65):
            if r % (16 if inverse else 64) == 0:
                yield hold(src, 2 * NB if inverse else 8)
            rows = pl.ds(8 * r, 8)
            z = [(src[a + 2 * i, rows, :], src[a + 2 * i + 1, rows, :]) for i in range(4)]
            if inverse:
                z = _radix4([turn(z[k], k) for k in range(4)], True)
            else:
                z = [turn(v, k) for k, v in enumerate(_radix4(z, False))]
            for i in range(4):
                dst[b + 2 * i, rows, :], dst[b + 2 * i + 1, rows, :] = z[i]
            yield _Step(18 if isinstance(g, int) and g == 0 else 35, [anchor(dst)], delay=1, marks=[name] if r == 64 else [])

    def spectral(row, size):
        rows = pl.ds(row, size)
        for k0 in range(4):
            z = _radix4([(Z[8 * g + 2 * k0, rows, :], Z[8 * g + 2 * k0 + 1, rows, :])
                         for g in range(4)], False)
            y = []
            for k1, (re, im) in enumerate(z):
                w = WS[k0 + 4 * k1, rows, :]
                wr = pltpu.bitcast(w << 16, F32)
                wi = pltpu.bitcast(w & np.uint32(0xFFFF0000), F32)
                y.append((re * wr - im * wi, re * wi + im * wr))
            y = _radix4(y, True)
            for g in range(4):
                Z[8 * g + 2 * k0, rows, :], Z[8 * g + 2 * k0 + 1, rows, :] = y[g]

    def spectral_rows(c2):
        for r in range(8):
            spectral(pl.multiple_of(128 * c2 + 16 * r, 16), 16)

    def inv_block(g, i, name, needs, n=None):
        j, t = g + 4 * i, i % 2
        UB, AB, PB, ubu, abu = temps[t]
        n = g if n is None else n
        z = opaque()
        yield _Wait(*needs)
        for r0, rn in _S_ROWS:
            if r0 == 0:
                yield hold(ZT, 8)
            re, im = ZT[z + 2 * i, pl.ds(r0, rn), :], ZT[z + 2 * i + 1, pl.ds(r0, rn), :]
            edge = (_iota(rn, 1) & 63) == 0
            rolled = _mirror(im)
            u = re + jnp.where(edge, lane_vec(L_KU + j, rn) * im, rolled)
            if r0 < 512:
                v = re - jnp.where(edge, lane_vec(L_KV + j, rn) * im, rolled)
                AB[0, pl.ds(r0, rn), :] = u.astype(BF16)
                AB[0, pl.ds(528 + r0, rn), :] = v.astype(BF16)
            else:
                AB[0, pl.ds(512, 16), :] = jnp.concatenate([u, jnp.zeros_like(u)], 0).astype(BF16)
            yield _Step(rn, [anchor(abu)], delay=1, marks=[("read", name)] if r0 == 512 else [])
        yield settle(abu, 4)

        def s_inverse(point):
            z = opaque()
            fa, fb = mat(M_FA + j + z), mat(M_FB + j + z)
            first = _iota(8, 0) == 0

            def put(row, v, v0=None):
                if v0 is not None:
                    v = jnp.concatenate([jnp.where(first, v0, v[:8]), v[8:]], 0)
                UB[0, pl.ds(row, 64), :] = v.astype(BF16)

            for k in range(4):
                lo, hi = 32 * k, 32 * (8 - k if k else 4)
                a = [abu[z, pl.ds(lo, 32), :], abu[z, pl.ds(hi, 32), :]] if k % 2 else [
                    tied(lambda r, o=o: abu[z, pl.ds(o + r, 8), :], 4, point) for o in (lo, hi)]
                if k == 0:
                    a.append(abu[z, pl.ds(256, 8), :])
                re = _dot_t(_bf(jnp.concatenate(a, 0)), fa)
                im = _dot_t(_bf(jnp.concatenate(
                    [abu[z, pl.ds(264 + lo, 32), :], abu[z, pl.ds(264 + hi, 32), :]], 0)), fb)
                pr, mr, pi, mi = re[:64], re[64:128], im[:64], im[64:]
                if k == 0:
                    put(0, pr)
                    put(64, pi, re[128:136])
                    put(128, mr)
                    put(192, mi)
                else:
                    put(256 * k, pr + mr, pr[:8])
                    put(256 * k + 64, pi + mi, mr[:8])
                    put(256 * k + 128, pi - mi, pi[:8])
                    put(256 * k + 192, mr - pr, -mi[:8])
            return 190

        yield _Mat(s_inverse)
        yield settle(ubu, 4)
        yield d_stage(t, lambda c: {0: M_R0T, 1: M_C4T}.get(c, M_RT))
        yield settle(PB, 4)
        z = opaque()
        acc = None
        for r in range(16):
            rows = pl.ds(8 * r, 8)
            t0, t4 = PB[z, rows, :], PB[z, pl.ds(128 + 8 * r, 8), :]
            tk = {}
            for k in (1, 2, 3):
                c, sn = twid[z + 2 * k - 2, rows, :], twid[z + 2 * k - 1, rows, :]
                re = PB[z, pl.ds(256 * k + 8 * r, 8), :]
                im = PB[z, pl.ds(256 * k + 128 + 8 * r, 8), :]
                tk[k] = (re * c - im * sn, re * sn + im * c)
            e0, e1 = t0 + t4, t0 - t4
            s = [e0 + tk[2][0], e1 - tk[2][1], e0 - tk[2][0], e1 + tk[2][1]]
            al, be = tk[1][0] - tk[3][0], tk[1][1] + tk[3][1]
            o = [tk[1][0] + tk[3][0], (al - be) * RSQ2, tk[3][1] - tk[1][1], (al + be) * -RSQ2]
            for b in range(8):
                y = s[b] + o[b] if b < 4 else s[b - 4] - o[b - 4]
                v = X[i][g, pl.ds(128 * b + 8 * r, 8), :] + y
                X[i][n, pl.ds(128 * b + 8 * r, 8), :] = v
                acc = v if acc is None else acc + v
            yield _Step(57, [lambda v=acc: v], delay=5 if r == 15 else 2)
        yield settle(X[i], 4)
        mean = _all_sublanes(acc, jnp.add, 0) * (1.0 / D)
        rstd = yield from ln_rstd(n, i, mean)
        z = opaque()
        for r in range(8):
            v = X[i][n + z, pl.ds(128 * r, 128), :].reshape(16, 8, 128)
            HB[i][n, pl.ds(128 * r, 128), :] = ((v - mean[None]) * rstd[None]).reshape(128, 128).astype(BF16)
            yield _Step(41, [anchor(hbu[i])], delay=1, marks=[name] if r == 7 else [])

    def attend(g, i, name, needs):
        yield _Wait(*needs)
        yield settle(QB[i])
        j, z = g + 4 * i, opaque()
        even = (_iota(8, 0) & 1) == 0
        edge = _iota(8, 1) == 0

        def window(near, far, w, rows):
            return near[j + z + 4 - 2 * w, rows, :] if w <= 2 * i + 2 else far[j + z + 16 - 2 * w, rows, :]

        def mix_values(h, u):
            p = PW[h % 2][opaque()]
            for rows in (pl.ds(256 * h + 16 * u, 16), pl.ds(256 * h + 16 * u + 16, 16)):
                acc = functools.reduce(jnp.add, [p[16 * w:16 * w + 16] * window(VE, VS, w, rows)
                                                 for w in range(8)])
                HB[i][g, rows, :] = acc.astype(BF16)
            return _Step(63, [anchor(hbu[i])], delay=2, marks=[name] if (h, u) == (3, 14) else [])

        for h in range(5):
            logits = []
            for w0 in range(0, 8, 2):
                if h < 4:
                    rows = pl.ds(256 * h, 256)
                    q = q if w0 % 4 else QB[i][opaque(), rows, :]
                    for w in (w0, w0 + 1):
                        v = (q * window(KE, KS, w, rows)).reshape(16, 16, 128).sum(0)
                        v = jnp.where(even, v[:8] + pltpu.roll(v[:8], 7, 0), v[8:] + pltpu.roll(v[8:], 1, 0))
                        logits.append(jnp.where(edge & (2 * w > j), -1e9, v * SCALE) if w > 2 * i
                                      else v * SCALE)
                    yield _Step(138, [lambda v=v: v for v in logits[-2:]], delay=4)
                if h > 0:
                    yield mix_values(h - 1, 2 * w0)
                    yield mix_values(h - 1, 2 * w0 + 2)
            if h < 4:
                top = functools.reduce(jnp.maximum, logits)
                e = [jnp.exp(v - top) for v in logits]
                total = functools.reduce(jnp.add, e)
                yield _Step(30, [lambda v=total: v], delay=3)
                scale = 1.0 / total
                for w in range(8):
                    v = e[w] * scale
                    PW[h % 2][0, pl.ds(16 * w, 8), :] = jnp.where(even, v, pltpu.roll(v, 1, 0))
                    PW[h % 2][0, pl.ds(16 * w + 8, 8), :] = jnp.where(even, pltpu.roll(v, 7, 0), v)
                yield _Step(50, [anchor(PW[h % 2])], delay=6 if h == 3 else 1)

    def packed_sums(terms, signs):
        lo = [pltpu.bitcast(u << 16, F32) for u in terms]
        hi = [pltpu.bitcast(u & np.uint32(0xFFFF0000), F32) for u in terms]
        return [pltpu.pack_elementwise([v[p] + v[q] if s > 0 else v[p] - v[q] for v in (lo, hi)],
                                       packed_dtype=BF16) for p, s, q in signs]

    def half(ref, row):
        return lambda r, size, cols: ref[pl.ds(pl.multiple_of(row + r, 8), size), cols]

    kv_weight = (WS5, half(WK, 0), half(WV, 0))
    q_weight = (WQ5, half(WQ, 0), half(WQ, D // 4))
    o_weight = (WP5, *(lambda r, size, cols, e=e: WP[pl.ds(r + r // 32 * 32 + e, size), cols]
                       for e in (0, 32)))

    def left_sums(weight, row, size, needs=()):
        yield _Wait(*needs)
        sums, top, bottom = weight
        for r in range(0, size, 8):
            a = [ref(row + r, 8, pl.ds(c, 512)) for ref in (top, bottom) for c in (0, 512)]
            for e, v in enumerate(packed_sums(a, ((0, 1, 3), (2, 1, 3), (0, 1, 1), (2, -1, 0), (1, -1, 3)))):
                sums[e, pl.ds(pl.multiple_of(row + r, 8), 8), :] = v
            yield _Step(92, [anchor(sums)], delay=2, marks=["sums"] if r == size - 8 else [])

    def right_sums(dst, g, i, name, needs):
        yield _Wait(*needs)
        z = g + opaque()
        for r in range(0, 256, 16):
            b = [hbu[n][z, pl.ds(k + r, 16), :] for k in (0, 256) for n in (i, i + 1)]
            for e, v in enumerate(packed_sums(b, ((0, 1, 3), (1, -1, 3), (2, -1, 0), (0, 1, 1), (2, 1, 3)))):
                dst[e, pl.ds(r, 16), :] = v
            yield _Step(47, [anchor(dst)], delay=SETTLE if r == 240 else 1,
                        marks=[name] if r == 240 else [])

    def strassen(sch, weight, right, g, i, m, store, needs, marks):
        for n in needs:
            sch.run(n)
        sums, top, bottom = weight
        rows = pl.ds(pl.multiple_of(64 * m, 64), 64)

        def product(left, b):
            sch.fresh = True
            head = tied(lambda r: left(32 * m + r, 8, pl.ds(0, 128)), 4, lambda: sch.point(8.0))
            return _dot(_bf(jnp.concatenate([head, left(32 * m, 32, pl.ds(128, 384))], 1)), _bf(b))

        def a(e):
            return lambda r, size, cols: sums[e, pl.ds(pl.multiple_of(r, 8), size), cols]

        def b(e):
            return right[e + opaque()]

        m2 = product(a(1), hbu[i][g + opaque(), pl.ds(0, 256), :])
        m4 = product(lambda r, size, cols: bottom(r, size, pl.ds(512 + cols.start, cols.size)), b(2))
        store(1, i, rows, m2 + m4)
        m1 = product(a(0), b(0))
        c11, c22 = m1 + m4, m1 - m2
        c11 = c11 + product(a(4), b(4))
        c22 = c22 + product(a(3), b(3))
        m5 = product(a(2), hbu[i + 1][g + opaque(), pl.ds(256, 256), :])
        store(0, i, rows, c11 - m5)
        v = product(top, b(1))
        store(0, i + 1, rows, v + m5)
        store(1, i + 1, rows, c22 + v)
        sch.results.append(v[:8])
        for name in marks:
            sch.done[name] = sch.slot + sch.wait

    def kv_proj(sch, g, i, name, needs):
        def store(lower, n, rows, v):
            (KE, VE)[lower][g + 4 * n + 4, rows, :] = v
        for m in range(16):
            strassen(sch, kv_weight, SB[i // 2], g, i, m, store, needs, [name] if m == 15 else [])

    def q_proj(sch, g, i, name, needs):
        def store(lower, n, rows, v):
            QB[n][0, pl.ds(512 * lower + rows.start, 64), :] = v
        for m in range(8):
            strassen(sch, q_weight, SB[i // 2], g, i, m, store, needs, [name] if m == 7 else [])

    def o_proj(sch, g, i, m, needs, marks, right):
        def store(lower, n, rows, v):
            rows = pl.ds(128 * m + 64 * lower, 64)
            X[n][g, rows, :] = X[n][g, rows, :] + v
        strassen(sch, o_weight, right, g, i, m, store, needs, marks)

    def shift_block(g, i, name, needs):
        yield _Wait(*needs)
        j, z = g + 4 * i, opaque()
        for m in range(16):
            rows = pl.ds(64 * m, 64)
            for ref, to in ((KE, KS), (VE, VS)):
                v = pltpu.roll(ref[j + 4 + z, rows, :], 1, 1)
                if ref is VE:
                    v = jnp.where(_iota(64, 1) == 0, ref[4 + z, rows, :], v)
                to[j, rows, :] = v
                if i == 3:
                    ref[g, rows, :] = v
            yield _Step(12, delay=8, marks=[name] if m == 15 else [])

    def transpose_quarter(w, h, via):
        for r in range(4):
            v = WRAW[w, pl.ds(256 * r, 256), pl.ds(pl.multiple_of(256 * h, 256), 256)]
            v = pltpu.bitcast(v.T, F32)
            via[0, pl.ds(256 * r, 128), :], via[0, pl.ds(256 * r + 128, 128), :] = v[:, :128], v[:, 128:]
            yield _Step(40, delay=16)

    def reorder_quarter(w, h, via, name=None):
        z = 0 if isinstance(h, int) else opaque()
        for c in range(8):
            WT[w][pl.ds(pl.multiple_of(128 * h, 128), 128), pl.ds(128 * c, 128)] = pltpu.bitcast(
                jnp.concatenate([via[z, pl.ds(128 * c + u, 8, stride=16), :] for u in range(16)], 0), U32)
            yield _Step(20, delay=4, marks=[name] if c == 7 else [])

    def query_weight(h):
        yield from transpose_quarter(0, h, QB[0])
        yield from reorder_quarter(0, h, QB[0], "w")

    def transpose_wo(name):
        for c in range(8):
            for h, e in itertools.product(range(4), range(2)):
                v = jnp.concatenate([wou[c, pl.ds(128 * h + 8 * e + u, 8, stride=16), :]
                                     for u in range(8)], 0)
                WP[pl.ds(64 * c, 64), pl.ds(256 * h + 128 * e, 128)] = pltpu.bitcast(_bf(v).T, U32)
                yield _Step(10, delay=5, marks=[name] if (c, h, e) == (7, 3, 1) else [])

    def prep_spectral_weights(c2):
        def words(k2):
            re, im = (wsu[u, k2, pl.ds(c2, 64, stride=4), :] for u in range(2))
            return ((re & np.uint32(0xFFFF)) | (im << 16), (re >> 16) | (im & np.uint32(0xFFFF0000)))

        def arrange(w, below):
            return jnp.where(_iota(w.shape[0], 1) < 64, w, below)

        below = words(15)
        for k2 in range(16):
            here = words(k2)
            for e in range(2):
                cl = 2 * c2 + e
                w = arrange(here[e], below[e])
                WS[k2, pl.ds(64 * cl, 64), :] = pltpu.roll(w, 1, 0) if cl > 4 else w
            below = here
            yield _Step(90, delay=3)
        if c2 == 0:
            def nyquist(k2):
                re, im = (jnp.broadcast_to(WN[u, :, pl.ds(128 * k2, 128)].astype(F32), (8, 128))
                          for u in range(2))
                return pltpu.pack_elementwise([re, im], packed_dtype=BF16)
            for k2 in range(16):
                WS[k2, pl.ds(512, 8), :] = arrange(nyquist(k2), nyquist((k2 + 15) % 16))

    def write_out(p, c, name, needs):
        yield _Wait(*needs)
        rows = pl.ds(pl.multiple_of(128 * c, 128), 128)
        g, i = 2 * p % 4 + opaque(), p // 2
        w = pltpu.pack_elementwise([X[i][g, rows, :], X[i][g + 1, rows, :]], packed_dtype=BF16)
        xru[c, pl.ds(p, 128, stride=8), :] = w.T
        yield _Step(30, marks=[name])

    tables = [pltpu.make_async_copy(lanes_hbm, lanes, sems.at[24]),
              pltpu.make_async_copy(mats_hbm, mats.at[pl.ds(M_R, 5)], sems.at[25])]
    start_all(tables + [x_copy(c) for c in range(8)])
    for c in tables:
        c.wait()

    def make_twiddle(k):
        PB = temps[0][2]
        PB[0, pl.ds(0, 128), :] = lane_vec(L_TWID + k, 128)
        twid[k] = PB[opaque(), pl.ds(0, 128), :].T

    _loop(6, make_twiddle, "make_twiddle")

    def make_dft(j):
        fa, fb = lanes[pl.ds(L_FA, 128), :], lanes[pl.ds(L_FB, 128), :]
        c, sn = lane_vec(L_COS + j, 128), lane_vec(L_SIN + j, 128)
        UB, _, _, ubu, _ = temps[0]
        UB[0, pl.ds(0, 128), :] = (fa * c + fb * sn).astype(BF16)
        UB[0, pl.ds(128, 128), :] = (fb * c - fa * sn).astype(BF16)
        mats[M_FA + j], mats[M_FB + j] = ubu[0, pl.ds(0, 64), :], ubu[0, pl.ds(64, 64), :]

    _loop(NB, make_dft, "make_dft")

    def load_x(c):
        x_copy(c).wait()
        pl.when(c == 6)(lambda: start_all(spec_copies[0]))
        pl.when(c == 7)(lambda: start_all(spec_copies[1]))
        rows = pl.ds(pl.multiple_of(128 * c, 128), 128)
        for p in range(8):
            w = xru[c, pl.ds(p, 128, stride=8), :].T
            for e, bits in enumerate((w << 16, w & np.uint32(0xFFFF0000))):
                g, i = 2 * p % 4 + e, p // 2
                v = pltpu.bitcast(bits, F32)
                X[i][g, rows, :] = v
                v = v.reshape(16, 8, 128)
                mean = _all_sublanes(v.sum(0), jnp.add, 0) * (1.0 / 128)
                STAT[4 * g + i, c] = mean
                STAT[4 * g + i, 8 + c] = _all_sublanes(((v - mean) ** 2).sum(0), jnp.add, 0)

    _loop(8, load_x, "load_x")

    def after(name, action):
        yield _Wait(name)
        action()

    def spectral_weights():
        yield _Wait(("f", 2, 1))
        for c in spec_copies[0] + spec_copies[1]:
            c.wait()
        for c2 in range(4):
            yield from prep_spectral_weights(c2)

    with jax.named_scope("first_forward"):
        sch = _Sched(0.72, 20)
        sch.add(after(("f", 0, 1), w_copies[1].start), "k")
        sch.add(after(("f", 1, 1), w_copies[2].start), "v")
        sch.add(after(("f", 2, 3), w_copies[0].start), "q")
        for g in range(4):
            for i in range(4):
                sch.add(fwd_block(g, i, ("f", g, i), [("f", g - 1, i)] if g else [],
                                  [("r", g - 1)] if g else [], True), ("f", g, i))
            sch.add(group_stage(g, ("r", g), [("f", g, i) for i in range(4)], False), ("r", g))
        sch.add(spectral_weights(), "s")
        sch.drive()
    start_all(wo_copies)

    def keys_values(layer, g):
        sch = _Sched(0.41, 32, 3) if layer == 0 else _Sched(0.36, 28, 2)
        nxt = (g + 1) % 4
        sch.add(inv_block(g, 2, ("i", 2), []), ("i", 2))
        sch.add(inv_block(g, 3, ("i", 3), [("read", ("i", 2))]), ("i", 3))
        sch.add(right_sums(SB[1], g, 2, ("b", 2), [("i", 2), ("i", 3)]), ("b", 2))
        sch.add(group_stage(nxt, "r", [("read", ("i", 3))], True), "r")
        sch.add(inv_block(nxt, 0, ("i", 4), ["r", ("i", 2)], n=g + 1), ("i", 4))
        sch.add(inv_block(nxt, 1, ("i", 5), [("read", ("i", 4)), ("i", 3)], n=g + 1), ("i", 5))
        if layer == 0:
            sch.add(query_weight(g), "w")
            sch.add(left_sums(q_weight, 128 * (g % 2), 128, ["w"]), "sums")
        for i in (2, 3):
            sch.add(shift_block((g + 3) % 4, i, ("s", i), []), ("s", i))
        for i in (0, 1):
            sch.add(shift_block(g, i, ("s", i), [("kv", 0)]), ("s", i))
        sch.add(right_sums(SB[0], nxt, 0, ("b", 4), [("i", 4), ("i", 5), ("kv", 0)]), ("b", 4))
        kv_proj(sch, g, 0, ("kv", 0), [])
        kv_proj(sch, g, 2, ("kv", 2), [("b", 2)])
        sch.finish()

    def mix(g, after, last):
        tail = after is None
        sch = _Sched(0.66 if last else 0.63, 28 if last else 32)
        pace = 0.48 if tail else 0.35 if last else 0.32
        ahead = [(g, 2), (g, 3)] + ([] if tail else [(after, 0), (after, 1)])
        for n, block in enumerate(ahead):
            sch.add(attend(*block, ("a", n), [[], [("a", 0)], [("a", 1), ("q", 0)], [("a", 2)]][n]),
                    ("a", n), pace=pace)
            if n % 2:
                sch.add(right_sums(SB[2 + block[1] // 2], block[0], block[1] - 1, ("b", n),
                                   [("a", n)] + ([("o", 0)] if n == 3 else [])), ("b", n))
        for i in () if tail else (0, 2):
            sch.add(right_sums(SB[i // 2], after, i, ("h", i), [("q", 0)] if i else []), ("h", i))
        if not last:
            sch.add(group_stage((g + 3) % 4, "r", [], False), "r")
            for i in range(4):
                sch.add(fwd_block(g, i, ("f", i), [("o", i - i % 2)], ["r"]), ("f", i))
        now = 6 if last else 8
        for i in (0, 2):
            for m in range(now):
                o_proj(sch, g, i, m, [("b", 1)] if i else [], [("o", i)] if m == now - 1 else [],
                       SB[2 + i // 2])
            if not tail:
                q_proj(sch, after, i, ("q", i), [("h", i)])
        if tail:
            sch.add(group_stage(g, "s", [("f", i) for i in range(4)], False), "s")
        sch.share = 0.92
        sch.drive()

    def mix_odd():
        sch = _Sched(0.66)
        blocks = [(1, 2), (1, 3), (3, 0), (3, 1), (3, 2), (3, 3)]
        for n, (g, i) in enumerate(blocks):
            sch.add(attend(g, i, ("a", n), ([("a", n - 1)] if n else []) + ([("q", i)] if n in (2, 4) else [])),
                    ("a", n), pace=0.32)
            if n % 2:
                sch.add(right_sums(SB[(3, 2, 0)[n // 2]], g, i - 1, ("b", g, i - 1),
                                   [("a", n)] + ([("o", 1, 0, 5)] if n > 1 else [])), ("b", g, i - 1))
        for i in (0, 2):
            sch.add(right_sums(SB[i // 2], 3, i, ("h", i), []), ("h", i))
        for g in (1, 3):
            for i in range(4):
                for c in range(6):
                    sch.add(write_out(2 * i + g // 2, c, ("w", g, i, c), [("o", g, i - i % 2, c)]),
                            ("w", g, i, c))
        for g, i, slot, count in ((1, 0, 2, 6), (1, 2, 3, 8), (3, 0, 2, 8), (3, 2, 0, 6)):
            for m in range(count):
                o_proj(sch, g, i, m, [("b", g, i)] if (g, i) != (1, 0) else [], [("o", g, i, m)], SB[slot])
            for e in (0, 2) if (g, i) == (1, 0) else ():
                q_proj(sch, 3, e, ("q", e), [("h", e)] + ([("a", 1)] if e else []))
        sch.share = 0.92
        sch.drive()

    def copy_out(chunks):
        def start(_):
            for c in chunks:
                out_copy(c).start()
        _loop(zero + 1, start, "copy_out")

    def postponed():
        slots = {(3, 2): 0, (2, 2): 1, (0, 2): 2, (2, 0): 3, (0, 0): 0, (1, 0): 1}
        early, late = list(slots)[:2], list(slots)[2:]
        sources = 2 * [[(0, 0), (1, 0)], [(2, 0)]] + 2 * [[(0, 2)], []]
        for c in (6, 7):
            sch = _Sched(0.7, 12)
            for n, (pair, slot) in enumerate(slots.items()) if c == 6 else ():
                if n:
                    sch.add(right_sums(SB[slot], *pair, pair, [(early[n - 4], 7)] if n >= 4 else []), pair)
            for p in (5, 7, 4, 6, 1, 3, 0, 2):
                sch.add(write_out(p, c, ("w", p), [(pair, c) for pair in sources[p] or early * (c == 6)]),
                        ("w", p))
            for pair, m in [(pair, m) for m in (6, 7) for pair in early] * (c == 6) + [(v, c) for v in late]:
                o_proj(sch, *pair, m, [pair] if c == 6 and pair != (3, 2) else [], [(pair, m)],
                       SB[slots[pair]])
            sch.drive()
            copy_out([c])

    def first_queries(layer):
        sch = _Sched(0.68)
        sch.add(right_sums(SB[1], 0, 2, ("h", 2), []), ("h", 2))
        sch.add(shift_block(3, 2, "s", []), "s")
        sch.add(attend(0, 0, ("a", 0), ["q"]), ("a", 0), pace=0.4)
        sch.add(attend(0, 1, ("a", 1), [("a", 0)]), ("a", 1), pace=0.4)
        sch.add(right_sums(SB[2], 0, 0, "b", [("a", 1)]), "b")
        sch.add(shift_block(3, 3, "t", []), "t")
        if layer == 0:
            for c in wo_copies:
                c.wait()
            sch.add(transpose_wo("w"), "w")
            sch.add(left_sums(o_weight, 0, 256, ["w"]), "sums")
        q_proj(sch, 0, 0, "q", [])
        q_proj(sch, 0, 2, None, [("h", 2)])
        sch.finish()

    def key_value_weights():
        w_copies[1].wait()
        w_copies[2].wait()
        for h in range(6):
            work = []
            for w in (1, 2):
                if h < 4:
                    work.append(transpose_quarter(w, h, QB[2 * (h % 2) + w - 1]))
                if 0 < h < 5:
                    work.append(reorder_quarter(w, h - 1, QB[2 * ((h - 1) % 2) + w - 1]))
            if h > 1:
                work.append(left_sums(kv_weight, 128 * (h - 2), 128))
            list(itertools.zip_longest(*work))

    for layer in range(2):
        with jax.named_scope("spectral"):
            _loop(4, spectral_rows, "rows")
            if layer == 0:
                _loop(zero + 1, lambda _: key_value_weights(), "weights")
            spectral(512, 8)
        sch = _Sched(0.92)
        sch.add(group_stage(0, "r", [], True), "r")
        sch.add(inv_block(0, 0, ("i", 0), ["r"]), ("i", 0))
        sch.add(inv_block(0, 1, ("i", 1), ["r"]), ("i", 1))
        sch.add(right_sums(SB[0], 0, 0, "b", [("i", 0), ("i", 1)]), "b")
        sch.drive()
        if layer == 0:
            w_copies[0].wait()
        _loop(4, lambda g: keys_values(layer, g), "keys_values")
        first_queries(layer)
        if layer == 0:
            pl.when(never)(lambda: [spectral_rows(c) for c in range(3)] and None)
        if layer == 0:
            _loop(3, lambda g: mix(g, g + 1, False), "mix")
            mix(3, None, False)
        else:
            _loop(2, lambda u: mix(2 * u, 2 - u, True), "mix")
            mix_odd()
    copy_out(range(6))
    postponed()
    for c in range(8):
        out_copy(c).wait()


@jax.jit
def pallas_interleave_layers__spectral_gfnet__sliding_local_dilated__prompt_kernel(
    A_x: jax.Array,
    A_w_r: jax.Array,
    A_w_i: jax.Array,
    B_x: jax.Array,
    B_wqkv: jax.Array,
    B_wo: jax.Array,
):
    del B_x
    hbm = pl.BlockSpec(memory_space=pl.ANY)
    smem = pl.BlockSpec(memory_space=pltpu.SMEM)
    out = pl.pallas_call(
        _kernel,
        out_shape=jax.ShapeDtypeStruct((S, D), BF16),
        in_specs=[smem, smem, hbm, hbm, hbm, hbm, hbm, hbm, hbm],
        out_specs=hbm,
        scratch_shapes=[
            pltpu.VMEM(_LANES.shape, F32),
            pltpu.VMEM((37, 64, 128), U32),
            pltpu.VMEM((6, 128, 128), F32),
            pltpu.VMEM((NB, 16, 8, 128), F32),
            pltpu.VMEM((NB + 4, D, 128), F32),
            pltpu.VMEM((NB + 4, D, 128), F32),
            pltpu.VMEM((NB, D, 128), F32),
            pltpu.VMEM((NB, D, 128), F32),
            pltpu.VMEM((2 * NB + 1, ZR, 128), F32),
            pltpu.VMEM((9, ZR, 128), F32),
            pltpu.VMEM((NB, ZR, 128), U32),
            *4 * [pltpu.VMEM((D // 2, D), U32)],
            pltpu.VMEM((5, D // 2, D // 2), U32),
            *2 * [pltpu.VMEM((5, D // 4, D // 2), U32)],
            *4 * [pltpu.VMEM((5, D // 4, 128), U32)],
            pltpu.VMEM((8, S, 128), BF16),
            pltpu.VMEM((2, NB, D // 2, 128), BF16),
            pltpu.VMEM((2, 1, S), BF16),
            pltpu.VMEM((3, D, D), BF16),
            pltpu.VMEM((8, D, 128), BF16),
            pltpu.VMEM((1, 128, 128), F32),
            pltpu.VMEM((1, 128, 128), F32),
            pltpu.SemaphoreType.DMA((26,)),
            *2 * [pltpu.VMEM((1, D, 128), F32)],
        ] + 4 * [
            pltpu.VMEM((5, D, 128), F32),
            pltpu.VMEM((5, D, 128), BF16),
            pltpu.VMEM((1, D, 128), F32),
            pltpu.VMEM((1, D, 128), BF16),
            pltpu.VMEM((1, 1152, 128), BF16),
        ],
        compiler_params=pltpu.CompilerParams(vmem_limit_bytes=126 * 2 ** 20),
    )(_ZERO, _ROT, _MATS, _LANES, A_x.reshape(S, D), A_w_r.T, A_w_i.T, B_wqkv, B_wo)
    return out.reshape(1, S, D)
```

```python
import functools
import itertools

import numpy as np

import jax
import jax.numpy as jnp
import jax.experimental.pallas as pl
import jax.experimental.pallas.tpu as pltpu

S, D, NB = 2048, 1024, 16
ZR = 576
F32, BF16, U32, I32 = jnp.float32, jnp.bfloat16, jnp.uint32, jnp.int32
EPS = 1e-5
SCALE = 32 ** -0.5
RSQ2 = float(np.sqrt(0.5))
SETTLE = 6

_S_ROWS = [(32 * u, 32) for u in range(16)] + [(512, 8)]

M_FA, M_FB, M_R, M_C4, M_RT, M_C4T, M_R0T = 0, 16, 32, 33, 34, 35, 36
L_MU, L_NU, L_KU, L_KV, L_COS, L_SIN, L_TWID, L_FA, L_FB = 0, 16, 32, 48, 64, 80, 96, 104, 232


def _bf16_bits(a):
    u = np.ascontiguousarray(a, dtype=np.float32).view(np.uint32).astype(np.uint64)
    return ((u + 0x7FFF + ((u >> 16) & 1)) >> 16).astype(np.uint32)


def _constants():
    a = np.arange(128)
    k1 = np.arange(64)
    alt = (-1.0) ** a
    lanes = np.zeros((384, 128))
    t = 2 * np.pi * np.outer(a, k1) / 128
    fa = np.concatenate([np.cos(t), -np.sin(t)], 1)
    fb = np.concatenate([np.sin(t), -np.cos(t)], 1)
    fa[:, 0], fb[:, 0] = RSQ2, -RSQ2
    fa[:, 64], fb[:, 64] = alt, 0.0
    lanes[L_FA:L_FA + 128], lanes[L_FB:L_FB + 128] = fa, fb
    for j in range(NB):
        ang = 2 * np.pi * j / 32 + np.pi / 32
        p, q = (_bf16_bits([np.cos(ang), np.sin(ang)]) << 16).view(np.float32).astype(np.float64)
        turn = 2 * np.pi * j * np.tile(k1, 2) / S
        lanes[L_COS + j], lanes[L_SIN + j] = np.cos(turn), np.repeat([-1.0, 1.0], 64) * np.sin(turn)
        lanes[L_COS + j, 64], lanes[L_SIN + j, 64] = p, q
        lanes[L_MU + j, 0], lanes[L_MU + j, 64] = 1.0, (q / p + p / q) / 2
        lanes[L_NU + j, 0], lanes[L_NU + j, 64] = 0.0, (q / p - p / q) / 2
        lanes[L_KU + j, 0], lanes[L_KU + j, 64] = 1.0, q / p
        lanes[L_KV + j, 0], lanes[L_KV + j, 64] = 1.0, p / q
    lanes[:, 65:] = lanes[:, :64:-1].copy()
    for k in (1, 2, 3):
        lanes[L_TWID + 2 * k - 2] = np.cos(2 * np.pi * a * k / D)
        lanes[L_TWID + 2 * k - 1] = np.sin(2 * np.pi * a * k / D)
    th = 2 * np.pi * np.outer(k1, a) / 128
    r = np.concatenate([np.cos(th), -np.sin(th)], 0)
    r[64] = alt
    th = 2 * np.pi * np.outer(2 * k1 + 1, a) / 256
    c4 = np.concatenate([np.cos(th), -np.sin(th)], 0)
    inv = 2.0 / (S * D)
    r0t = inv * r.T
    r0t[:, 0::64] *= 0.5
    rows = np.arange(128).reshape(2, 4, 16).transpose(1, 0, 2).ravel()
    bits = _bf16_bits(np.stack([r[rows], c4[rows], inv * r.T, inv * c4.T, r0t]))
    ang = 2 * np.pi * np.outer(np.arange(4), np.arange(4)).ravel() / 16
    rot = np.concatenate([np.cos(ang), np.sin(ang)]).astype(np.float32)
    return bits[:, 0::2] | (bits[:, 1::2] << 16), lanes.astype(np.float32), rot


_MATS, _LANES, _ROT = _constants()
_ZERO = np.zeros((1,), np.int32)


class _Step:
    def __init__(self, cost, anchors=(), delay=0, marks=()):
        self.cost, self.anchors, self.delay, self.marks = cost, list(anchors), delay, list(marks)


class _Wait:
    def __init__(self, *names):
        self.names = names


class _Mat:
    def __init__(self, emit):
        self.emit = emit


class _Hold:
    def __init__(self, store):
        self.store = store


class _Task:
    def __init__(self, gen, pace):
        self.gen, self.pace, self.blocked, self.not_before, self.held = gen, pace, (), 0, None
        self.allowed = 0.0


class _Sched:
    def __init__(self, share=0.0, wait=28, lag=3):
        self.lag = lag
        self.wait = wait
        self.share = share
        self.tasks, self.done, self.producer = [], {}, {}
        self.slot, self.credit, self.anchors, self.results = 0, 0.0, [], []
        self.fresh = False

    def add(self, gen, name, pace=99):
        self.producer[name] = self.producer["read", name] = _Task(gen, pace)
        self.tasks.append(self.producer[name])

    def _ready(self, t):
        return t.not_before <= self.slot and all(
            n in self.done and self.done[n] <= self.slot for n in t.blocked)

    def _advance(self, t, mats=True):
        item, t.held = t.held or next(t.gen, None), None
        if item is None:
            self.tasks.remove(t)
        elif isinstance(item, _Wait):
            t.blocked = item.names
        elif isinstance(item, _Hold):
            if len(self.results) >= self.lag:
                item.store(self.results[-self.lag])
        elif isinstance(item, _Mat):
            if mats:
                t.not_before = float("inf")
                self.fresh = False
                self.credit -= item.emit(lambda: self.point(0.0)) or 0
                t.not_before = self.slot + self.wait
            else:
                t.held, t.not_before = item, self.slot + 1
        else:
            t.blocked = ()
            t.not_before = self.slot + item.delay
            self.credit -= item.cost
            self.anchors += item.anchors
            for n in item.marks:
                self.done[n] = self.slot + item.delay
            return True

    def run(self, *names):
        while not all(n in self.done for n in names):
            for n in names:
                if n not in self.done:
                    for b in self.producer[n].blocked:
                        self.run(b)
                    self._advance(self.producer[n])

    def drive(self):
        while self.tasks:
            ready = [t for t in self.tasks if self._ready(t)]
            if not ready:
                self.slot += 1
                continue
            self.anchors, self.credit = self.anchors[-2:], 0.0
            self._advance(next((t for t in ready if t.held), ready[0]))
            self.slot -= min(self.credit, 0.0) / 60

    def finish(self):
        self.run(*[n for n in self.producer if n[0] != "read"])

    def point(self, own):
        for t in self.tasks:
            t.allowed = min(t.allowed, 0.0) + t.pace
        while True:
            t = next((t for t in self.tasks if self._ready(t) and t.allowed > 0
                      and self.credit > 0), None)
            if t is None:
                break
            if self._advance(t, self.fresh):
                t.allowed -= 1
        anchors, self.anchors = self.anchors, []
        self.credit = min(self.credit, 10.0) + 64 * self.share - own
        self.fresh = False
        self.slot += 1
        return anchors


def _dot(a, b):
    return jnp.dot(a, b, preferred_element_type=F32)


def _dot_t(a, b):
    return jax.lax.dot_general(a, b, (((1,), (1,)), ((), ())), preferred_element_type=F32)


def _bf(u):
    return pltpu.bitcast(u, BF16)


def _iota(rows, dim):
    return jax.lax.broadcasted_iota(I32, (rows, 128), dim)


def _mirror(v):
    index = -_iota(8, 1) & 127
    return jnp.concatenate([jnp.take_along_axis(v[r:r + 8], index, axis=1)
                            for r in range(0, v.shape[0], 8)], 0)


def _radix4(z, inverse):
    (r0, i0), (r1, i1), (r2, i2), (r3, i3) = z
    ar, ai, cr, ci = r0 + r2, i0 + i2, r0 - r2, i0 - i2
    br, bi, dr, di = r1 + r3, i1 + i3, r1 - r3, i1 - i3
    lo, hi = (cr + di, ci - dr), (cr - di, ci + dr)
    if inverse:
        lo, hi = hi, lo
    return [(ar + br, ai + bi), lo, (ar - br, ai - bi), hi]


def _all_sublanes(v, op, axis):
    for sh in (4, 2, 1):
        v = op(v, pltpu.roll(v, sh, axis))
    return v


def _loop(n, body, name):
    def step(i, carry):
        body(i)
        return carry
    with jax.named_scope(name):
        jax.lax.fori_loop(0, n, step, 0)


def _kernel(zero_ref, rot, mats_hbm, lanes_hbm, x_hbm, wr_hbm, wi_hbm, wqkv_hbm, wo_hbm, out_hbm,
            lanes, mats, twid, STAT, KE, VE, KS, VS, Z, ZT, WS, WQ, WK, WV, WP, WS5, WQ5, WP5,
            SB0, SB1, SB2, SB3, XR, WRI, WN, WRAW, WO, PW0, PW1, sems, *split):
    zero = zero_ref[0]
    never = zero != 0
    X, HB, QB = split[2::5], split[3::5], split[4::5]
    hbu = [r.bitcast(U32) for r in HB]
    xru, wsu, wou = XR.bitcast(U32), WRI.bitcast(U32), WO.bitcast(U32)
    temps = [(ub, ab, pb, ub.bitcast(U32), ab.bitcast(U32))
             for ub, ab, pb in zip(split[5::5], split[6::5], 2 * split[:2])]
    PW, SB, WT = (PW0, PW1), (SB0, SB1, SB2, SB3), (WQ, WK, WV, WP)
    counter = [0]

    def opaque():
        counter[0] += 1
        return zero * counter[0]

    def anchor(ref):
        at = (0,) * (len(ref.shape) - 2)
        return lambda: ref[(*at, pl.ds(pl.multiple_of(zero * 8, 8), 8), pl.ds(0, 128))]

    def settle(ref, points=SETTLE):
        return _Step(2, [anchor(ref)], delay=points)

    def hold(ref, spare):
        def store(v):
            ref[spare, pl.ds(pl.multiple_of(zero * 8, 8), 8), :] = v
        return _Hold(store)

    def tied(load, vregs, point):
        parts = []
        for r in range(vregs):
            anchors = point()
            u = load(8 * r)
            for a in anchors:
                u = jnp.where(never, pltpu.bitcast(a(), U32), u)
            parts.append(u)
        return jnp.concatenate(parts, 0)

    def mat(i):
        return _bf(mats[i])

    def d_stage(t, which):
        UB, AB, PB, ubu, abu = temps[t]

        def emit(point):
            z = opaque()
            for c in range(8):
                lhs = mat(which(c) + opaque()) if c % 4 else _bf(
                    tied(lambda r, u=which(c) + opaque(): mats[u, pl.ds(r, 8), :], 8, point))
                PB[0, pl.ds(128 * c, 128), :] = _dot(lhs, _bf(ubu[z, pl.ds(64 * c, 64), :]))
        return _Mat(emit)

    def lane_vec(i, rows):
        return jnp.broadcast_to(lanes[pl.ds(i, 1), :], (rows, 128))

    def x_copy(c):
        return pltpu.make_async_copy(
            x_hbm.at[:, pl.ds(pl.multiple_of(128 * c, 128), 128)], XR.at[c], sems.at[c])

    def out_copy(c):
        return pltpu.make_async_copy(
            XR.at[c], out_hbm.at[:, pl.ds(pl.multiple_of(128 * c, 128), 128)], sems.at[8 + c])

    spec_copies = [[pltpu.make_async_copy(w.at[pl.ds(0, 512), pl.ds(128 * k2, 128)], WRI.at[u, k2],
                                          sems.at[16 + u]) for k2 in range(16)]
                   + [pltpu.make_async_copy(w.at[pl.ds(512, 1), :], WN.at[u], sems.at[22 + u])]
                   for u, w in enumerate((wr_hbm, wi_hbm))]

    def start_all(copies):
        for c in copies:
            c.start()
    w_copies = [pltpu.make_async_copy(wqkv_hbm.at[:, pl.ds(D * w, D)], WRAW.at[w], sems.at[18 + w])
                for w in range(3)]
    wo_copies = [pltpu.make_async_copy(wo_hbm.at[:, pl.ds(128 * c, 128)], WO.at[c], sems.at[21])
                 for c in range(8)]

    def ln_rstd(g, i, mean):
        acc, m = None, g + opaque()
        for r in range(8):
            d = X[i][m, pl.ds(128 * r, 128), :].reshape(16, 8, 128) - mean[None]
            v = (d * d).sum(0)
            acc = v if acc is None else acc + v
            if r < 7:
                yield _Step(50, [lambda acc=acc: acc], delay=3)
        rstd = jax.lax.rsqrt(_all_sublanes(acc, jnp.add, 0) * (1.0 / D) + EPS)
        yield _Step(50, delay=8)
        yield _Step(10, [lambda: rstd], delay=1)
        return rstd

    def fwd_block(g, i, name, needs, free=(), known=False):
        j, t = g + 4 * i, i
        UB, AB, PB, ubu, abu = temps[t]
        yield _Wait(*needs)
        if known:
            means, squares = STAT[4 * g + i, pl.ds(0, 8)], STAT[4 * g + i, pl.ds(8, 8)]
            mean = means.sum(0) * 0.125
            var = (squares.sum(0) + 128.0 * ((means - mean) ** 2).sum(0)) * (1.0 / D)
            rstd = jax.lax.rsqrt(var + EPS)
            yield _Step(50, delay=6)
        else:
            yield settle(X[i])
            acc, m = None, g + opaque()
            for r in range(8):
                v = X[i][m, pl.ds(128 * r, 128), :].reshape(16, 8, 128).sum(0)
                acc = v if acc is None else acc + v
                if r % 2:
                    yield _Step(35, [lambda acc=acc: acc], delay=7 if r == 7 else 3)
            mean = _all_sublanes(acc, jnp.add, 0) * (1.0 / D)
            rstd = yield from ln_rstd(g, i, mean)
        mean8, rstd = (jnp.concatenate([v, v], 0) for v in (mean * 8.0, rstd))
        z = opaque()
        for r in range(8):
            rows = pl.ds(16 * r, 16)
            x = [X[i][g + z, pl.ds(128 * b + 16 * r, 16), :] for b in range(8)]
            s = [x[b] + x[b + 4] for b in range(4)]
            d = [x[b] - x[b + 4] for b in range(4)]
            e, o = s[0] + s[2], s[1] + s[3]
            UB[0, rows, :] = ((e + o - mean8) * rstd).astype(BF16)
            UB[0, pl.ds(128 + 16 * r, 16), :] = ((e - o) * rstd).astype(BF16)
            t1, t2 = (d[1] - d[3]) * RSQ2, (d[1] + d[3]) * RSQ2
            u = {1: (d[0] + t1, d[2] + t2), 2: (s[0] - s[2], s[1] - s[3]), 3: (d[0] - t1, d[2] - t2)}
            yield _Step(34, [anchor(ubu)], delay=1)
            for k in (1, 2, 3):
                c, sn = twid[z + 2 * k - 2, rows, :] * rstd, twid[z + 2 * k - 1, rows, :] * rstd
                re, m = u[k]
                if k == 3:
                    ur, ui = re * c + m * sn, m * c - re * sn
                else:
                    ur, ui = re * c - m * sn, m * c + re * sn
                UB[0, pl.ds(256 * k + 16 * r, 16), :] = ur.astype(BF16)
                UB[0, pl.ds(256 * k + 128 + 16 * r, 16), :] = ui.astype(BF16)
                yield _Step(26, [anchor(ubu)], delay=1)
        yield settle(ubu)

        def d_forward(point):
            z = opaque()
            first = _iota(8, 0) == 0

            def stage(c):
                u = (M_C4 if c == 1 else M_R) + opaque()
                lhs = mat(u) if c % 4 else _bf(tied(lambda r: mats[u, pl.ds(r, 8), :], 8, point))
                v = _dot(lhs, _bf(ubu[z, pl.ds(64 * c, 64), :]))
                return [(v[32 * u:32 * u + 16], v[32 * u + 16:32 * u + 32]) for u in range(4)]

            def put(row, u, v, v0=None):
                if u == 0 and v0 is not None:
                    v = jnp.concatenate([jnp.where(first, v0, v[:8]), v[8:]], 0)
                AB[0, pl.ds(row + 16 * u, 16), :] = v.astype(BF16)

            for u, (p1, p2) in enumerate(stage(0)):
                put(0, u, p1)
                put(528, u, p2, 0.0)
                if u == 0:
                    put(512, 0, jnp.zeros_like(p2), p2[:8])
            for u, (p1, p2) in enumerate(stage(1)):
                put(256, u, p1)
                put(528 + 256, u, p2)
            for k in (1, 2, 3):
                for u, ((p1, p2), (q1, q2)) in enumerate(zip(stage(2 * k), stage(2 * k + 1))):
                    if k == 3:
                        pr, pi, mr, mi = p1 - q2, p2 + q1, p1 + q2, p2 - q1
                        pi0, mi0 = q1[:8], -q2[:8]
                    else:
                        pr, pi, mr, mi = p1 + q2, p2 - q1, p1 - q2, p2 + q1
                        pi0, mi0 = -q1[:8], q2[:8]
                    put(64 * k, u, pr, p1[:8])
                    put(64 * (8 - k), u, mr, p2[:8])
                    put(528 + 64 * k, u, pi, pi0)
                    put(528 + 64 * (8 - k), u, mi, mi0)
            return 190

        yield _Mat(d_forward)
        yield settle(abu)
        yield _Wait(*free)

        def s_forward(point):
            z = opaque()
            fa, fb = mat(M_FA + j + z), mat(M_FB + j + z)
            for r0, rn in ((0, 256), (256, 272)):
                lhs = abu[z, pl.ds(r0 // 2, rn // 2), :] if r0 else tied(
                    lambda r: abu[z, pl.ds(r, 8), :], 16, point)
                u = _dot(_bf(lhs), fa)
                v = _dot(_bf(abu[z, pl.ds(264 + r0 // 2, 128), :]), fb)
                re, m = u[:256] + v, u[:256] - v
                if r0:
                    re, m = (jnp.concatenate([a, u[256:264]], 0) for a in (re, m))
                rn = re.shape[0]
                edge = (_iota(rn, 1) & 63) == 0
                ZT[2 * i, pl.ds(r0, rn), :] = re
                ZT[2 * i + 1, pl.ds(r0, rn), :] = jnp.where(
                    edge, lane_vec(L_MU + j, rn) * m + lane_vec(L_NU + j, rn) * re, _mirror(m))
            return 400

        yield _Mat(s_forward)
        yield _Step(2, [anchor(ZT)], delay=SETTLE, marks=[name])

    def group_stage(g, name, needs, inverse):
        yield _Wait(*needs)

        def turn(z, k):
            if k == 0 or (isinstance(g, int) and g == 0):
                return z
            if isinstance(g, int) and g * k == 4:
                return (-z[1], z[0]) if inverse else (z[1], -z[0])
            c, s = rot[4 * g + k], rot[16 + 4 * g + k]
            if inverse:
                return z[0] * c - z[1] * s, z[1] * c + z[0] * s
            return z[0] * c + z[1] * s, z[1] * c - z[0] * s

        (src, a), (dst, b) = ((Z, 8 * g), (ZT, 0)) if inverse else ((ZT, opaque()), (Z, 8 * g))
        for r in range(65):
            if r % (16 if inverse else 64) == 0:
                yield hold(src, 2 * NB if inverse else 8)
            rows = pl.ds(8 * r, 8)
            z = [(src[a + 2 * i, rows, :], src[a + 2 * i + 1, rows, :]) for i in range(4)]
            if inverse:
                z = _radix4([turn(z[k], k) for k in range(4)], True)
            else:
                z = [turn(v, k) for k, v in enumerate(_radix4(z, False))]
            for i in range(4):
                dst[b + 2 * i, rows, :], dst[b + 2 * i + 1, rows, :] = z[i]
            yield _Step(18 if isinstance(g, int) and g == 0 else 35, [anchor(dst)], delay=1, marks=[name] if r == 64 else [])

    def spectral(row, size):
        rows = pl.ds(row, size)
        for k0 in range(4):
            z = _radix4([(Z[8 * g + 2 * k0, rows, :], Z[8 * g + 2 * k0 + 1, rows, :])
                         for g in range(4)], False)
            y = []
            for k1, (re, im) in enumerate(z):
                w = WS[k0 + 4 * k1, rows, :]
                wr = pltpu.bitcast(w << 16, F32)
                wi = pltpu.bitcast(w & np.uint32(0xFFFF0000), F32)
                y.append((re * wr - im * wi, re * wi + im * wr))
            y = _radix4(y, True)
            for g in range(4):
                Z[8 * g + 2 * k0, rows, :], Z[8 * g + 2 * k0 + 1, rows, :] = y[g]

    def spectral_rows(c2):
        for r in range(8):
            spectral(pl.multiple_of(128 * c2 + 16 * r, 16), 16)

    def inv_block(g, i, name, needs, n=None):
        j, t = g + 4 * i, i % 2
        UB, AB, PB, ubu, abu = temps[t]
        n = g if n is None else n
        z = opaque()
        yield _Wait(*needs)
        for r0, rn in _S_ROWS:
            if r0 == 0:
                yield hold(ZT, 8)
            re, im = ZT[z + 2 * i, pl.ds(r0, rn), :], ZT[z + 2 * i + 1, pl.ds(r0, rn), :]
            edge = (_iota(rn, 1) & 63) == 0
            rolled = _mirror(im)
            u = re + jnp.where(edge, lane_vec(L_KU + j, rn) * im, rolled)
            if r0 < 512:
                v = re - jnp.where(edge, lane_vec(L_KV + j, rn) * im, rolled)
                AB[0, pl.ds(r0, rn), :] = u.astype(BF16)
                AB[0, pl.ds(528 + r0, rn), :] = v.astype(BF16)
            else:
                AB[0, pl.ds(512, 16), :] = jnp.concatenate([u, jnp.zeros_like(u)], 0).astype(BF16)
            yield _Step(rn, [anchor(abu)], delay=1, marks=[("read", name)] if r0 == 512 else [])
        yield settle(abu, 4)

        def s_inverse(point):
            z = opaque()
            fa, fb = mat(M_FA + j + z), mat(M_FB + j + z)
            first = _iota(8, 0) == 0

            def put(row, v, v0=None):
                if v0 is not None:
                    v = jnp.concatenate([jnp.where(first, v0, v[:8]), v[8:]], 0)
                UB[0, pl.ds(row, 64), :] = v.astype(BF16)

            for k in range(4):
                lo, hi = 32 * k, 32 * (8 - k if k else 4)
                a = [abu[z, pl.ds(lo, 32), :], abu[z, pl.ds(hi, 32), :]] if k % 2 else [
                    tied(lambda r, o=o: abu[z, pl.ds(o + r, 8), :], 4, point) for o in (lo, hi)]
                if k == 0:
                    a.append(abu[z, pl.ds(256, 8), :])
                re = _dot_t(_bf(jnp.concatenate(a, 0)), fa)
                im = _dot_t(_bf(jnp.concatenate(
                    [abu[z, pl.ds(264 + lo, 32), :], abu[z, pl.ds(264 + hi, 32), :]], 0)), fb)
                pr, mr, pi, mi = re[:64], re[64:128], im[:64], im[64:]
                if k == 0:
                    put(0, pr)
                    put(64, pi, re[128:136])
                    put(128, mr)
                    put(192, mi)
                else:
                    put(256 * k, pr + mr, pr[:8])
                    put(256 * k + 64, pi + mi, mr[:8])
                    put(256 * k + 128, pi - mi, pi[:8])
                    put(256 * k + 192, mr - pr, -mi[:8])
            return 190

        yield _Mat(s_inverse)
        yield settle(ubu, 4)
        yield d_stage(t, lambda c: {0: M_R0T, 1: M_C4T}.get(c, M_RT))
        yield settle(PB, 4)
        z = opaque()
        acc = None
        for r in range(16):
            rows = pl.ds(8 * r, 8)
            t0, t4 = PB[z, rows, :], PB[z, pl.ds(128 + 8 * r, 8), :]
            tk = {}
            for k in (1, 2, 3):
                c, sn = twid[z + 2 * k - 2, rows, :], twid[z + 2 * k - 1, rows, :]
                re = PB[z, pl.ds(256 * k + 8 * r, 8), :]
                im = PB[z, pl.ds(256 * k + 128 + 8 * r, 8), :]
                tk[k] = (re * c - im * sn, re * sn + im * c)
            e0, e1 = t0 + t4, t0 - t4
            s = [e0 + tk[2][0], e1 - tk[2][1], e0 - tk[2][0], e1 + tk[2][1]]
            al, be = tk[1][0] - tk[3][0], tk[1][1] + tk[3][1]
            o = [tk[1][0] + tk[3][0], (al - be) * RSQ2, tk[3][1] - tk[1][1], (al + be) * -RSQ2]
            for b in range(8):
                y = s[b] + o[b] if b < 4 else s[b - 4] - o[b - 4]
                v = X[i][g, pl.ds(128 * b + 8 * r, 8), :] + y
                X[i][n, pl.ds(128 * b + 8 * r, 8), :] = v
                acc = v if acc is None else acc + v
            yield _Step(57, [lambda v=acc: v], delay=5 if r == 15 else 2)
        yield settle(X[i], 4)
        mean = _all_sublanes(acc, jnp.add, 0) * (1.0 / D)
        rstd = yield from ln_rstd(n, i, mean)
        z = opaque()
        for r in range(8):
            v = X[i][n + z, pl.ds(128 * r, 128), :].reshape(16, 8, 128)
            HB[i][n, pl.ds(128 * r, 128), :] = ((v - mean[None]) * rstd[None]).reshape(128, 128).astype(BF16)
            yield _Step(41, [anchor(hbu[i])], delay=1, marks=[name] if r == 7 else [])

    def attend(g, i, name, needs):
        yield _Wait(*needs)
        yield settle(QB[i])
        j, z = g + 4 * i, opaque()
        even = (_iota(8, 0) & 1) == 0
        edge = _iota(8, 1) == 0

        def window(near, far, w, rows):
            return near[j + z + 4 - 2 * w, rows, :] if w <= 2 * i + 2 else far[j + z + 16 - 2 * w, rows, :]

        def mix_values(h, u):
            p = PW[h % 2][opaque()]
            for rows in (pl.ds(256 * h + 16 * u, 16), pl.ds(256 * h + 16 * u + 16, 16)):
                acc = functools.reduce(jnp.add, [p[16 * w:16 * w + 16] * window(VE, VS, w, rows)
                                                 for w in range(8)])
                HB[i][g, rows, :] = acc.astype(BF16)
            return _Step(63, [anchor(hbu[i])], delay=2, marks=[name] if (h, u) == (3, 14) else [])

        for h in range(5):
            logits = []
            for w0 in range(0, 8, 2):
                if h < 4:
                    rows = pl.ds(256 * h, 256)
                    q = q if w0 % 4 else QB[i][opaque(), rows, :]
                    for w in (w0, w0 + 1):
                        v = (q * window(KE, KS, w, rows)).reshape(16, 16, 128).sum(0)
                        v = jnp.where(even, v[:8] + pltpu.roll(v[:8], 7, 0), v[8:] + pltpu.roll(v[8:], 1, 0))
                        logits.append(jnp.where(edge & (2 * w > j), -1e9, v * SCALE) if w > 2 * i
                                      else v * SCALE)
                    yield _Step(138, [lambda v=v: v for v in logits[-2:]], delay=4)
                if h > 0:
                    yield mix_values(h - 1, 2 * w0)
                    yield mix_values(h - 1, 2 * w0 + 2)
            if h < 4:
                top = functools.reduce(jnp.maximum, logits)
                e = [jnp.exp(v - top) for v in logits]
                total = functools.reduce(jnp.add, e)
                yield _Step(30, [lambda v=total: v], delay=3)
                scale = 1.0 / total
                for w in range(8):
                    v = e[w] * scale
                    PW[h % 2][0, pl.ds(16 * w, 8), :] = jnp.where(even, v, pltpu.roll(v, 1, 0))
                    PW[h % 2][0, pl.ds(16 * w + 8, 8), :] = jnp.where(even, pltpu.roll(v, 7, 0), v)
                yield _Step(50, [anchor(PW[h % 2])], delay=6 if h == 3 else 1)

    def packed_sums(terms, signs):
        lo = [pltpu.bitcast(u << 16, F32) for u in terms]
        hi = [pltpu.bitcast(u & np.uint32(0xFFFF0000), F32) for u in terms]
        return [pltpu.pack_elementwise([v[p] + v[q] if s > 0 else v[p] - v[q] for v in (lo, hi)],
                                       packed_dtype=BF16) for p, s, q in signs]

    def half(ref, row):
        return lambda r, size, cols: ref[pl.ds(pl.multiple_of(row + r, 8), size), cols]

    kv_weight = (WS5, half(WK, 0), half(WV, 0))
    q_weight = (WQ5, half(WQ, 0), half(WQ, D // 4))
    o_weight = (WP5, *(lambda r, size, cols, e=e: WP[pl.ds(r + r // 32 * 32 + e, size), cols]
                       for e in (0, 32)))

    def left_sums(weight, row, size, needs=()):
        yield _Wait(*needs)
        sums, top, bottom = weight
        for r in range(0, size, 8):
            a = [ref(row + r, 8, pl.ds(c, 512)) for ref in (top, bottom) for c in (0, 512)]
            for e, v in enumerate(packed_sums(a, ((0, 1, 3), (2, 1, 3), (0, 1, 1), (2, -1, 0), (1, -1, 3)))):
                sums[e, pl.ds(pl.multiple_of(row + r, 8), 8), :] = v
            yield _Step(92, [anchor(sums)], delay=2, marks=["sums"] if r == size - 8 else [])

    def right_sums(dst, g, i, name, needs):
        yield _Wait(*needs)
        z = g + opaque()
        for r in range(0, 256, 16):
            b = [hbu[n][z, pl.ds(k + r, 16), :] for k in (0, 256) for n in (i, i + 1)]
            for e, v in enumerate(packed_sums(b, ((0, 1, 3), (1, -1, 3), (2, -1, 0), (0, 1, 1), (2, 1, 3)))):
                dst[e, pl.ds(r, 16), :] = v
            yield _Step(47, [anchor(dst)], delay=SETTLE if r == 240 else 1,
                        marks=[name] if r == 240 else [])

    def strassen(sch, weight, right, g, i, m, store, needs, marks):
        for n in needs:
            sch.run(n)
        sums, top, bottom = weight
        rows = pl.ds(pl.multiple_of(64 * m, 64), 64)

        def product(left, b):
            sch.fresh = True
            head = tied(lambda r: left(32 * m + r, 8, pl.ds(0, 128)), 4, lambda: sch.point(8.0))
            return _dot(_bf(jnp.concatenate([head, left(32 * m, 32, pl.ds(128, 384))], 1)), _bf(b))

        def a(e):
            return lambda r, size, cols: sums[e, pl.ds(pl.multiple_of(r, 8), size), cols]

        def b(e):
            return right[e + opaque()]

        m2 = product(a(1), hbu[i][g + opaque(), pl.ds(0, 256), :])
        m4 = product(lambda r, size, cols: bottom(r, size, pl.ds(512 + cols.start, cols.size)), b(2))
        store(1, i, rows, m2 + m4)
        m1 = product(a(0), b(0))
        c11, c22 = m1 + m4, m1 - m2
        c11 = c11 + product(a(4), b(4))
        c22 = c22 + product(a(3), b(3))
        m5 = product(a(2), hbu[i + 1][g + opaque(), pl.ds(256, 256), :])
        store(0, i, rows, c11 - m5)
        v = product(top, b(1))
        store(0, i + 1, rows, v + m5)
        store(1, i + 1, rows, c22 + v)
        sch.results.append(v[:8])
        for name in marks:
            sch.done[name] = sch.slot + sch.wait

    def kv_proj(sch, g, i, name, needs):
        def store(lower, n, rows, v):
            (KE, VE)[lower][g + 4 * n + 4, rows, :] = v
        for m in range(16):
            strassen(sch, kv_weight, SB[i // 2], g, i, m, store, needs, [name] if m == 15 else [])

    def q_proj(sch, g, i, name, needs):
        def store(lower, n, rows, v):
            QB[n][0, pl.ds(512 * lower + rows.start, 64), :] = v
        for m in range(8):
            strassen(sch, q_weight, SB[i // 2], g, i, m, store, needs, [name] if m == 7 else [])

    def o_proj(sch, g, i, m, needs, marks, right):
        def store(lower, n, rows, v):
            rows = pl.ds(128 * m + 64 * lower, 64)
            X[n][g, rows, :] = X[n][g, rows, :] + v
        strassen(sch, o_weight, right, g, i, m, store, needs, marks)

    def shift_block(g, i, name, needs):
        yield _Wait(*needs)
        j, z = g + 4 * i, opaque()
        for m in range(16):
            rows = pl.ds(64 * m, 64)
            for ref, to in ((KE, KS), (VE, VS)):
                v = pltpu.roll(ref[j + 4 + z, rows, :], 1, 1)
                if ref is VE:
                    v = jnp.where(_iota(64, 1) == 0, ref[4 + z, rows, :], v)
                to[j, rows, :] = v
                if i == 3:
                    ref[g, rows, :] = v
            yield _Step(12, delay=8, marks=[name] if m == 15 else [])

    def transpose_quarter(w, h, via):
        for r in range(4):
            v = WRAW[w, pl.ds(256 * r, 256), pl.ds(pl.multiple_of(256 * h, 256), 256)]
            v = pltpu.bitcast(v.T, F32)
            via[0, pl.ds(256 * r, 128), :], via[0, pl.ds(256 * r + 128, 128), :] = v[:, :128], v[:, 128:]
            yield _Step(40, delay=16)

    def reorder_quarter(w, h, via, name=None):
        z = 0 if isinstance(h, int) else opaque()
        for c in range(8):
            WT[w][pl.ds(pl.multiple_of(128 * h, 128), 128), pl.ds(128 * c, 128)] = pltpu.bitcast(
                jnp.concatenate([via[z, pl.ds(128 * c + u, 8, stride=16), :] for u in range(16)], 0), U32)
            yield _Step(20, delay=4, marks=[name] if c == 7 else [])

    def query_weight(h):
        yield from transpose_quarter(0, h, QB[0])
        yield from reorder_quarter(0, h, QB[0], "w")

    def transpose_wo(name):
        for c in range(8):
            for h, e in itertools.product(range(4), range(2)):
                v = jnp.concatenate([wou[c, pl.ds(128 * h + 8 * e + u, 8, stride=16), :]
                                     for u in range(8)], 0)
                WP[pl.ds(64 * c, 64), pl.ds(256 * h + 128 * e, 128)] = pltpu.bitcast(_bf(v).T, U32)
                yield _Step(10, delay=6, marks=[name] if (c, h, e) == (7, 3, 1) else [])

    def prep_spectral_weights(c2):
        def words(k2):
            re, im = (wsu[u, k2, pl.ds(c2, 64, stride=4), :] for u in range(2))
            return ((re & np.uint32(0xFFFF)) | (im << 16), (re >> 16) | (im & np.uint32(0xFFFF0000)))

        def arrange(w, below):
            return jnp.where(_iota(w.shape[0], 1) < 64, w, below)

        below = words(15)
        for k2 in range(16):
            here = words(k2)
            for e in range(2):
                cl = 2 * c2 + e
                w = arrange(here[e], below[e])
                WS[k2, pl.ds(64 * cl, 64), :] = pltpu.roll(w, 1, 0) if cl > 4 else w
            below = here
            yield _Step(90, delay=3)
        if c2 == 0:
            def nyquist(k2):
                re, im = (jnp.broadcast_to(WN[u, :, pl.ds(128 * k2, 128)].astype(F32), (8, 128))
                          for u in range(2))
                return pltpu.pack_elementwise([re, im], packed_dtype=BF16)
            for k2 in range(16):
                WS[k2, pl.ds(512, 8), :] = arrange(nyquist(k2), nyquist((k2 + 15) % 16))

    def write_out(p, c, name, needs):
        yield _Wait(*needs)
        rows = pl.ds(pl.multiple_of(128 * c, 128), 128)
        g, i = 2 * p % 4 + opaque(), p // 2
        w = pltpu.pack_elementwise([X[i][g, rows, :], X[i][g + 1, rows, :]], packed_dtype=BF16)
        xru[c, pl.ds(p, 128, stride=8), :] = w.T
        yield _Step(30, marks=[name])

    tables = [pltpu.make_async_copy(lanes_hbm, lanes, sems.at[24]),
              pltpu.make_async_copy(mats_hbm, mats.at[pl.ds(M_R, 5)], sems.at[25])]
    start_all(tables + [x_copy(c) for c in range(8)])
    for c in tables:
        c.wait()

    def make_twiddle(k):
        PB = temps[0][2]
        PB[0, pl.ds(0, 128), :] = lane_vec(L_TWID + k, 128)
        twid[k] = PB[opaque(), pl.ds(0, 128), :].T

    _loop(6, make_twiddle, "make_twiddle")

    def make_dft(j):
        fa, fb = lanes[pl.ds(L_FA, 128), :], lanes[pl.ds(L_FB, 128), :]
        c, sn = lane_vec(L_COS + j, 128), lane_vec(L_SIN + j, 128)
        UB, _, _, ubu, _ = temps[0]
        UB[0, pl.ds(0, 128), :] = (fa * c + fb * sn).astype(BF16)
        UB[0, pl.ds(128, 128), :] = (fb * c - fa * sn).astype(BF16)
        mats[M_FA + j], mats[M_FB + j] = ubu[0, pl.ds(0, 64), :], ubu[0, pl.ds(64, 64), :]

    _loop(NB, make_dft, "make_dft")

    def load_x(c):
        x_copy(c).wait()
        pl.when(c == 6)(lambda: start_all(spec_copies[0]))
        pl.when(c == 7)(lambda: start_all(spec_copies[1]))
        rows = pl.ds(pl.multiple_of(128 * c, 128), 128)
        for p in range(8):
            w = xru[c, pl.ds(p, 128, stride=8), :].T
            for e, bits in enumerate((w << 16, w & np.uint32(0xFFFF0000))):
                g, i = 2 * p % 4 + e, p // 2
                v = pltpu.bitcast(bits, F32)
                X[i][g, rows, :] = v
                v = v.reshape(16, 8, 128)
                mean = _all_sublanes(v.sum(0), jnp.add, 0) * (1.0 / 128)
                STAT[4 * g + i, c] = mean
                STAT[4 * g + i, 8 + c] = _all_sublanes(((v - mean) ** 2).sum(0), jnp.add, 0)

    _loop(8, load_x, "load_x")

    def after(name, action):
        yield _Wait(name)
        action()

    def spectral_weights():
        yield _Wait(("f", 2, 1))
        for c in spec_copies[0] + spec_copies[1]:
            c.wait()
        for c2 in range(4):
            yield from prep_spectral_weights(c2)

    with jax.named_scope("first_forward"):
        sch = _Sched(0.72, 20)
        sch.add(after(("f", 0, 1), w_copies[1].start), "k")
        sch.add(after(("f", 1, 1), w_copies[2].start), "v")
        sch.add(after(("f", 2, 3), w_copies[0].start), "q")
        for g in range(4):
            for i in range(4):
                sch.add(fwd_block(g, i, ("f", g, i), [("f", g - 1, i)] if g else [],
                                  [("r", g - 1)] if g else [], True), ("f", g, i))
            sch.add(group_stage(g, ("r", g), [("f", g, i) for i in range(4)], False), ("r", g))
        sch.add(spectral_weights(), "s")
        sch.drive()
    start_all(wo_copies)

    def keys_values(layer, g):
        sch = _Sched(0.405, 32, 3) if layer == 0 else _Sched(0.355, 28, 2)
        nxt = (g + 1) % 4
        sch.add(inv_block(g, 2, ("i", 2), []), ("i", 2))
        sch.add(inv_block(g, 3, ("i", 3), [("read", ("i", 2))]), ("i", 3))
        sch.add(right_sums(SB[1], g, 2, ("b", 2), [("i", 2), ("i", 3)]), ("b", 2))
        sch.add(group_stage(nxt, "r", [("read", ("i", 3))], True), "r")
        sch.add(inv_block(nxt, 0, ("i", 4), ["r", ("i", 2)], n=g + 1), ("i", 4))
        sch.add(inv_block(nxt, 1, ("i", 5), [("read", ("i", 4)), ("i", 3)], n=g + 1), ("i", 5))
        if layer == 0:
            sch.add(query_weight(g), "w")
            sch.add(left_sums(q_weight, 128 * (g % 2), 128, ["w"]), "sums")
        for i in (2, 3):
            sch.add(shift_block((g + 3) % 4, i, ("s", i), []), ("s", i))
        for i in (0, 1):
            sch.add(shift_block(g, i, ("s", i), [("kv", 0)]), ("s", i))
        sch.add(right_sums(SB[0], nxt, 0, ("b", 4), [("i", 4), ("i", 5), ("kv", 0)]), ("b", 4))
        kv_proj(sch, g, 0, ("kv", 0), [])
        kv_proj(sch, g, 2, ("kv", 2), [("b", 2)])
        sch.finish()

    def mix(g, after, last):
        tail = after is None
        sch = _Sched(0.70 if last else 0.65, 28 if last else 36)
        pace = 0.48 if tail else 0.35 if last else 0.32
        ahead = [(g, 2), (g, 3)] + ([] if tail else [(after, 0), (after, 1)])
        for n, block in enumerate(ahead):
            sch.add(attend(*block, ("a", n), [[], [("a", 0)], [("a", 1), ("q", 0)], [("a", 2)]][n]),
                    ("a", n), pace=pace)
            if n % 2:
                sch.add(right_sums(SB[2 + block[1] // 2], block[0], block[1] - 1, ("b", n),
                                   [("a", n)] + ([("o", 0)] if n == 3 else [])), ("b", n))
        for i in () if tail else (0, 2):
            sch.add(right_sums(SB[i // 2], after, i, ("h", i), [("q", 0)] if i else []), ("h", i))
        if not last:
            sch.add(group_stage((g + 3) % 4, "r", [], False), "r")
            for i in range(4):
                sch.add(fwd_block(g, i, ("f", i), [("o", i - i % 2)], ["r"]), ("f", i))
        now = 6 if last else 8
        for i in (0, 2):
            for m in range(now):
                o_proj(sch, g, i, m, [("b", 1)] if i else [], [("o", i)] if m == now - 1 else [],
                       SB[2 + i // 2])
            if not tail:
                q_proj(sch, after, i, ("q", i), [("h", i)])
        if tail:
            sch.add(group_stage(g, "s", [("f", i) for i in range(4)], False), "s")
        sch.share = 0.92
        sch.drive()

    def mix_odd():
        sch = _Sched(0.66, 20)
        blocks = [(1, 2), (1, 3), (3, 0), (3, 1), (3, 2), (3, 3)]
        for n, (g, i) in enumerate(blocks):
            sch.add(attend(g, i, ("a", n), ([("a", n - 1)] if n else []) + ([("q", i)] if n in (2, 4) else [])),
                    ("a", n), pace=0.32)
            if n % 2:
                sch.add(right_sums(SB[(3, 2, 0)[n // 2]], g, i - 1, ("b", g, i - 1),
                                   [("a", n)] + ([("o", 1, 0, 5)] if n > 1 else [])), ("b", g, i - 1))
        for i in (0, 2):
            sch.add(right_sums(SB[i // 2], 3, i, ("h", i), []), ("h", i))
        for g in (1, 3):
            for i in range(4):
                for c in range(6):
                    sch.add(write_out(2 * i + g // 2, c, ("w", g, i, c), [("o", g, i - i % 2, c)]),
                            ("w", g, i, c))
        for g, i, slot, count in ((1, 0, 2, 6), (1, 2, 3, 8), (3, 0, 2, 8), (3, 2, 0, 6)):
            for m in range(count):
                o_proj(sch, g, i, m, [("b", g, i)] if (g, i) != (1, 0) else [], [("o", g, i, m)], SB[slot])
            for e in (0, 2) if (g, i) == (1, 0) else ():
                q_proj(sch, 3, e, ("q", e), [("h", e)] + ([("a", 1)] if e else []))
        sch.share = 0.92
        sch.drive()

    def copy_out(chunks):
        def start(_):
            for c in chunks:
                out_copy(c).start()
        _loop(zero + 1, start, "copy_out")

    def postponed():
        slots = {(3, 2): 0, (2, 2): 1, (0, 2): 2, (2, 0): 3, (0, 0): 0, (1, 0): 1}
        early, late = list(slots)[:2], list(slots)[2:]
        sources = 2 * [[(0, 0), (1, 0)], [(2, 0)]] + 2 * [[(0, 2)], []]
        for c in (6, 7):
            sch = _Sched(0.7, 12)
            for n, (pair, slot) in enumerate(slots.items()) if c == 6 else ():
                if n:
                    sch.add(right_sums(SB[slot], *pair, pair, [(early[n - 4], 7)] if n >= 4 else []), pair)
            for p in (5, 7, 4, 6, 1, 3, 0, 2):
                sch.add(write_out(p, c, ("w", p), [(pair, c) for pair in sources[p] or early * (c == 6)]),
                        ("w", p))
            for pair, m in [(pair, m) for m in (6, 7) for pair in early] * (c == 6) + [(v, c) for v in late]:
                o_proj(sch, *pair, m, [pair] if c == 6 and pair != (3, 2) else [], [(pair, m)],
                       SB[slots[pair]])
            sch.drive()
            copy_out([c])

    def first_queries(layer):
        sch = _Sched(0.68)
        sch.add(right_sums(SB[1], 0, 2, ("h", 2), []), ("h", 2))
        sch.add(shift_block(3, 2, "s", []), "s")
        sch.add(attend(0, 0, ("a", 0), ["q"]), ("a", 0), pace=0.4)
        sch.add(attend(0, 1, ("a", 1), [("a", 0)]), ("a", 1), pace=0.4)
        sch.add(right_sums(SB[2], 0, 0, "b", [("a", 1)]), "b")
        sch.add(shift_block(3, 3, "t", []), "t")
        if layer == 0:
            for c in wo_copies:
                c.wait()
            sch.add(transpose_wo("w"), "w")
            sch.add(left_sums(o_weight, 0, 256, ["w"]), "sums")
        q_proj(sch, 0, 0, "q", [])
        q_proj(sch, 0, 2, None, [("h", 2)])
        sch.finish()

    def key_value_weights():
        w_copies[1].wait()
        w_copies[2].wait()
        for h in range(6):
            work = []
            for w in (1, 2):
                if h < 4:
                    work.append(transpose_quarter(w, h, QB[2 * (h % 2) + w - 1]))
                if 0 < h < 5:
                    work.append(reorder_quarter(w, h - 1, QB[2 * ((h - 1) % 2) + w - 1]))
            if h > 1:
                work.append(left_sums(kv_weight, 128 * (h - 2), 128))
            list(itertools.zip_longest(*work))

    for layer in range(2):
        with jax.named_scope("spectral"):
            _loop(4, spectral_rows, "rows")
            if layer == 0:
                _loop(zero + 1, lambda _: key_value_weights(), "weights")
            spectral(512, 8)
        sch = _Sched(0.92)
        sch.add(group_stage(0, "r", [], True), "r")
        sch.add(inv_block(0, 0, ("i", 0), ["r"]), ("i", 0))
        sch.add(inv_block(0, 1, ("i", 1), ["r"]), ("i", 1))
        sch.add(right_sums(SB[0], 0, 0, "b", [("i", 0), ("i", 1)]), "b")
        sch.drive()
        if layer == 0:
            w_copies[0].wait()
        _loop(4, lambda g: keys_values(layer, g), "keys_values")
        first_queries(layer)
        if layer == 0:
            pl.when(never)(lambda: [spectral_rows(c) for c in range(3)] and None)
        if layer == 0:
            _loop(3, lambda g: mix(g, g + 1, False), "mix")
            mix(3, None, False)
        else:
            _loop(2, lambda u: mix(2 * u, 2 - u, True), "mix")
            mix_odd()
    copy_out(range(6))
    postponed()
    for c in range(8):
        out_copy(c).wait()


@jax.jit
def pallas_interleave_layers__spectral_gfnet__sliding_local_dilated__prompt_kernel(
    A_x: jax.Array,
    A_w_r: jax.Array,
    A_w_i: jax.Array,
    B_x: jax.Array,
    B_wqkv: jax.Array,
    B_wo: jax.Array,
):
    del B_x
    hbm = pl.BlockSpec(memory_space=pl.ANY)
    smem = pl.BlockSpec(memory_space=pltpu.SMEM)
    out = pl.pallas_call(
        _kernel,
        out_shape=jax.ShapeDtypeStruct((S, D), BF16),
        in_specs=[smem, smem, hbm, hbm, hbm, hbm, hbm, hbm, hbm],
        out_specs=hbm,
        scratch_shapes=[
            pltpu.VMEM(_LANES.shape, F32),
            pltpu.VMEM((37, 64, 128), U32),
            pltpu.VMEM((6, 128, 128), F32),
            pltpu.VMEM((NB, 16, 8, 128), F32),
            pltpu.VMEM((NB + 4, D, 128), F32),
            pltpu.VMEM((NB + 4, D, 128), F32),
            pltpu.VMEM((NB, D, 128), F32),
            pltpu.VMEM((NB, D, 128), F32),
            pltpu.VMEM((2 * NB + 1, ZR, 128), F32),
            pltpu.VMEM((9, ZR, 128), F32),
            pltpu.VMEM((NB, ZR, 128), U32),
            *4 * [pltpu.VMEM((D // 2, D), U32)],
            pltpu.VMEM((5, D // 2, D // 2), U32),
            *2 * [pltpu.VMEM((5, D // 4, D // 2), U32)],
            *4 * [pltpu.VMEM((5, D // 4, 128), U32)],
            pltpu.VMEM((8, S, 128), BF16),
            pltpu.VMEM((2, NB, D // 2, 128), BF16),
            pltpu.VMEM((2, 1, S), BF16),
            pltpu.VMEM((3, D, D), BF16),
            pltpu.VMEM((8, D, 128), BF16),
            pltpu.VMEM((1, 128, 128), F32),
            pltpu.VMEM((1, 128, 128), F32),
            pltpu.SemaphoreType.DMA((26,)),
            *2 * [pltpu.VMEM((1, D, 128), F32)],
        ] + 4 * [
            pltpu.VMEM((5, D, 128), F32),
            pltpu.VMEM((5, D, 128), BF16),
            pltpu.VMEM((1, D, 128), F32),
            pltpu.VMEM((1, D, 128), BF16),
            pltpu.VMEM((1, 1152, 128), BF16),
        ],
        compiler_params=pltpu.CompilerParams(vmem_limit_bytes=126 * 2 ** 20),
    )(_ZERO, _ROT, _MATS, _LANES, A_x.reshape(S, D), A_w_r.T, A_w_i.T, B_wqkv, B_wo)
    return out.reshape(1, S, D)
```
